```python
import jax
import jax.numpy as jnp

def _softmax(x, axis=-1):
    return jax.nn.softmax(x, axis=axis)
def _gelu(x):
    return jax.nn.gelu(x, approximate=True)
def _silu(x):
    return jax.nn.silu(x)
def _sigmoid(x):
    return jax.nn.sigmoid(x)
def _layernorm(x, axis=-1, eps=1e-5):
    m = jnp.mean(x, axis=axis, keepdims=True)
    v = jnp.var(x, axis=axis, keepdims=True)
    return (x - m) / jnp.sqrt(v + eps)
def _scatter_add(tgt, idx, src, axis=0):
    return tgt.at[idx].add(src)
def _segment_sum(src, seg, n):
    return jax.ops.segment_sum(src, seg, n)
class _Rng:
    def __init__(self, key):
        self._k = key
    def _next(self):
        self._k, sub = jax.random.split(self._k)
        return sub
    def normal(self, shape):
        return jax.random.normal(self._next(), shape, dtype=jnp.bfloat16)
    def randint(self, lo, hi, shape):
        return jax.random.randint(self._next(), shape, lo, hi, dtype=jnp.int32)
    def uniform(self, shape, lo=0.0, hi=1.0):
        return jax.random.uniform(self._next(), shape, jnp.bfloat16, lo, hi)
    def permutation(self, n):
        return jax.random.permutation(self._next(), n)


kernel_name = 'gated_mix__compressed_kv_cla__ssm_conv_s5__prompt'

def setup_inputs():
    _rng = _Rng(jax.random.key(int.from_bytes(__import__("os").urandom(4), "little")))
    _w = (lambda a: (lambda t: t.astype(jnp.bfloat16) if jnp.issubdtype(t.dtype, jnp.floating) else t)(jnp.asarray(a)))
    def _A_setup():
        B, H, Sq, Sk, D, M = 1, 16, 2048, 2048, 256, 448
        Dc = 4 * D
        return {
            "x": _w((lambda *s: _rng.normal(s) * 0.05)(B, Sq, M)),
            "c_kv": _w((lambda *s: _rng.normal(s) * 0.05)(B, Sk, Dc)),
            "w_q": _w((lambda *s: _rng.normal(s) * 0.05)(M, H, D) * (M ** -0.5)),
            "w_uk": _w((lambda *s: _rng.normal(s) * 0.05)(Dc, H, D) * (Dc ** -0.5)),
            "w_uv": _w((lambda *s: _rng.normal(s) * 0.05)(Dc, H, D) * (Dc ** -0.5)),
            "w_o": _w((lambda *s: _rng.normal(s) * 0.05)(H, D, M) * ((H * D) ** -0.5)),
        }
    _A_in = _A_setup()

    def _B_setup():
        B, S, D = 1, 2048, 448
        P = D
        Lambda_re = -0.5 * jnp.exp((lambda *s: _rng.normal(s) * 0.05)(P))
        Lambda_im = (lambda *s: _rng.normal(s) * 0.05)(P) * 1.0
        B_re = (lambda *s: _rng.normal(s) * 0.05)(P, D) * (D ** -0.5)
        B_im = (lambda *s: _rng.normal(s) * 0.05)(P, D) * (D ** -0.5)
        C_re = (lambda *s: _rng.normal(s) * 0.05)(D, P) * (P ** -0.5)
        C_im = (lambda *s: _rng.normal(s) * 0.05)(D, P) * (P ** -0.5)
        log_dt = (lambda *s: _rng.normal(s) * 0.05)(P) * 0.3 - 2.0
        Dskip = (lambda *s: _rng.normal(s) * 0.05)(D)
        return {
            "x": _w((lambda *s: _rng.normal(s) * 0.05)(B, S, D)),
            "Lambda_re": _w(Lambda_re),
            "Lambda_im": _w(Lambda_im),
            "B_re": _w(B_re),
            "B_im": _w(B_im),
            "C_re": _w(C_re),
            "C_im": _w(C_im),
            "log_dt": _w(log_dt),
            "Dskip": _w(Dskip),
        }
    _B_in = _B_setup()

    return {
        "A_x": _A_in["x"],
        "A_c_kv": _A_in["c_kv"],
        "A_w_q": _A_in["w_q"],
        "A_w_uk": _A_in["w_uk"],
        "A_w_uv": _A_in["w_uv"],
        "A_w_o": _A_in["w_o"],
        "B_x": _B_in["x"],
        "B_Lambda_re": _B_in["Lambda_re"],
        "B_Lambda_im": _B_in["Lambda_im"],
        "B_B_re": _B_in["B_re"],
        "B_B_im": _B_in["B_im"],
        "B_C_re": _B_in["C_re"],
        "B_C_im": _B_in["C_im"],
        "B_log_dt": _B_in["log_dt"],
        "B_Dskip": _B_in["Dskip"],
        "gate_w": _w((lambda *s: _rng.normal(s) * 0.05)(448)),
    }

def reference(A_x, A_c_kv, A_w_q, A_w_uk, A_w_uv, A_w_o, B_x, B_Lambda_re, B_Lambda_im, B_B_re, B_B_im, B_C_re, B_C_im, B_log_dt, B_Dskip, gate_w):
    def _A_ref(x, c_kv, w_q, w_uk, w_uv, w_o):
        B, Sq, M = x.shape[0], x.shape[1], x.shape[2]
        Sk = c_kv.shape[1]
        H, D = w_q.shape[1], w_q.shape[2]
        q = jnp.einsum("bqm,mhd->bhqd", x, w_q)
        k = jnp.einsum("bkc,chd->bhkd", c_kv, w_uk)
        v = jnp.einsum("bkc,chd->bhkd", c_kv, w_uv)
        scores = jnp.einsum("bhqd,bhkd->bhqk", q, k) * (D ** -0.5)
        off = Sk - Sq
        qi = jnp.arange(Sq)[:, None]
        kj = jnp.arange(Sk)[None, :]
        cmask = kj <= (qi + off)
        scores = jnp.where(cmask[None, None], scores, -1e9)
        p = _softmax(scores, axis=-1)
        ctx = jnp.einsum("bhqk,bhkd->bhqd", p, v)
        return jnp.einsum("bhqd,hdm->bqm", ctx, w_o)

    def _B_ref(x, Lambda_re, Lambda_im, B_re, B_im, C_re, C_im, log_dt, Dskip):
        Bsz, L, H = x.shape
        Lam = Lambda_re + 1j * Lambda_im
        Bmat = B_re + 1j * B_im
        Cmat = C_re + 1j * C_im
        dt = jnp.exp(log_dt)
        Lam_bar = jnp.exp(dt * Lam)
        B_bar = ((Lam_bar - 1.0) / Lam)[:, None] * Bmat
        Bu = jnp.einsum("bld,pd->blp", x + 0j, B_bar)
        h = jnp.zeros_like(Bu[:, 0, :])
        hs = []
        for t in range(L):
            h = Lam_bar[None, :] * h + Bu[:, t, :]
            hs.append(h)
        hseq = jnp.stack(hs, 1)
        y = 2.0 * jnp.einsum("blp,dp->bld", hseq, Cmat).real + x * Dskip[None, None, :]
        return y

    x = A_x
    g = _sigmoid((x * gate_w).sum(-1, keepdims=True))
    a = _A_ref(x, A_c_kv, A_w_q, A_w_uk, A_w_uv, A_w_o)
    b = _B_ref(x, B_Lambda_re, B_Lambda_im, B_B_re, B_B_im, B_C_re, B_C_im, B_log_dt, B_Dskip)
    return g * a + (1 - g) * b
```

```python
import jax
import jax.numpy as jnp
from jax import lax
import jax.experimental.pallas as pl
import jax.experimental.pallas.tpu as pltpu

S = 2048
M = 448
H = 16
D = 256
DC = 1024
TQ = 128
NQ = S // TQ
PA = 384
PB = M - PA
TC = 256
LOG2E = 1.4426950408889634

f32 = jnp.float32
bf16 = jnp.bfloat16
u32 = jnp.uint32


def _dot(a, b, dims):
    return lax.dot_general(a, b, (dims, ((), ())), preferred_element_type=f32)


_NN = ((1,), (0,))
_NT = ((1,), (1,))
_TN = ((0,), (0,))
_TT = ((0,), (1,))


def _cmul(ar, ai, br, bi):
    return ar * br - ai * bi, ar * bi + ai * br


def _weight_copies(w_hbm, raw, sem, sem0):
    return [
        pltpu.make_async_copy(
            w_hbm.at[:, ht * 8:(ht + 1) * 8, dt * 128:(dt + 1) * 128],
            raw.at[ht * 2 + dt], sem.at[sem0 + ht * 2 + dt])
        for ht in range(2) for dt in range(2)
    ]


def _stage(raw, stg, k, c0, nc):
    v = raw[k, pl.ds(c0, nc)].reshape(nc * 8, 128)
    stg[k, pl.ds(pl.multiple_of(c0 * 4, 8), nc * 4), :] = pltpu.bitcast(v, u32)


def _stage_slice(raws, stgs, group, sl):
    for raw, stg, rows in zip(raws, stgs, (M, DC, DC)):
        for dt in range(2):
            _stage(raw, stg, group * 2 + dt, sl * (rows // 4), rows // 4)


def _head_weight(stg, h, rows):
    ht = lax.shift_right_logical(h, 3)
    pr = lax.shift_right_logical(h & 7, 1)
    sh = (16 * (1 - (h & 1))).astype(u32)
    halves = []
    for dt in range(2):
        u = stg[ht * 2 + dt, pl.ds(pr, rows, stride=4), :]
        halves.append(pltpu.bitcast((u << sh) & jnp.uint32(0xFFFF0000), f32))
    return jnp.concatenate(halves, axis=1)


def _ssm_and_gate(xT_ref, bre_ref, bim_ref, cre_ref, cim_ref, lre_ref, lim_ref,
                  ldt_ref, dsk_ref, gw_ref, o_ref, g_s, b_s, c_s, lam_s, col_s, u_s, h_s):
    row = lambda r: r[...].astype(f32).reshape(1, M)
    lre, lim = row(lre_ref), row(lim_ref)
    dt = jnp.exp(row(ldt_ref)).astype(bf16).astype(f32)
    mag = jnp.exp(dt * lre)
    ang = dt * lim
    lr, li = mag * jnp.cos(ang), mag * jnp.sin(ang)
    den = lre * lre + lim * lim
    nr = lr - 1.0
    cr = (nr * lre + li * lim) / den
    ci = (li * lre - nr * lim) / den
    c_re, c_im = cre_ref[...].astype(f32), cim_ref[...].astype(f32)
    cp_re, cp_im = _cmul(c_re, c_im, 2.0 * cr, 2.0 * ci)
    c_s[...] = jnp.concatenate(
        [cp_re[:, :PA], -cp_im[:, :PA], cp_re[:, PA:], -cp_im[:, PA:]], axis=1).astype(bf16)
    b_s[0:PA, :] = bre_ref[0:PA, :]
    b_s[PA:2 * PA, :] = bim_ref[0:PA, :]
    b_s[2 * PA:2 * PA + PB, :] = bre_ref[PA:M, :]
    b_s[2 * PA + PB:2 * M, :] = bim_ref[PA:M, :]

    er = jnp.concatenate([lr, lr[:, PA:]], axis=1)
    ei = jnp.concatenate([li, -li[:, PA:]], axis=1)
    pw = [(er, ei)]
    for _ in range(7):
        pw.append(_cmul(pw[-1][0], pw[-1][1], er, ei))
    sub = lax.broadcasted_iota(jnp.int32, (8, 512), 0)
    for n, d in enumerate((1, 2, 4)):
        lam_s[2 * n] = jnp.where(sub >= d, pw[d - 1][0], 0.0)
        lam_s[2 * n + 1] = jnp.where(sub >= d, pw[d - 1][1], 0.0)
    lcr = jnp.zeros((8, 512), f32)
    lci = jnp.zeros((8, 512), f32)
    for r in range(8):
        lcr = jnp.where(sub == r, pw[r][0], lcr)
        lci = jnp.where(sub == r, pw[r][1], lci)
    lam_s[6] = lcr
    lam_s[7] = lci

    def col(r):
        v = jnp.concatenate([row(r), jnp.zeros((1, 512 - M), f32)], axis=1)
        return jnp.broadcast_to(v, (128, 512)).T[:M]
    col_s[0] = col(dsk_ref)
    col_s[1] = col(gw_ref)

    def lanes(lo, n):
        return pl.ds(lo if isinstance(lo, int) else pl.multiple_of(lo, 128), n)

    def bu(i):
        return _dot(xT_ref[:, lanes(i * TC, TC)], b_s[...], _TT)

    def scan(u, carry):
        nb = TC // 8
        mixed = u[:, 2 * PA:]
        hr = jnp.concatenate([u[:, :PA], mixed], axis=1).reshape(nb, 8, 512)
        hi = jnp.concatenate([u[:, PA:2 * PA], pltpu.roll(mixed, PB, 1)], axis=1).reshape(nb, 8, 512)
        for n, d in enumerate((1, 2, 4)):
            sr, si = pltpu.roll(hr, d, 1), pltpu.roll(hi, d, 1)
            tr, ti = _cmul(sr, si, lam_s[2 * n][None], lam_s[2 * n + 1][None])
            hr, hi = hr + tr, hi + ti
        lcr, lci = lam_s[6], lam_s[7]
        car, cai = carry
        outr, outi = [], []
        for b in range(nb):
            tr, ti = _cmul(lcr, lci, car, cai)
            br, bi = hr[b] + tr, hi[b] + ti
            outr.append(br)
            outi.append(bi)
            car, cai = br[7:8, :], bi[7:8, :]
        hr = jnp.concatenate(outr, axis=0)
        hi = jnp.concatenate(outi, axis=0)
        h = jnp.concatenate([hr[:, :PA], hi[:, :PA], hr[:, PA:]], axis=1).astype(bf16)
        return h, (car, cai)

    def finish(i, h):
        yT = _dot(c_s[...], h, _NT)
        for t in range(TC // 128):
            sl = lanes(i * TC + t * 128, 128)
            xf = xT_ref[:, sl].astype(f32)
            g = jax.nn.sigmoid(jnp.sum(xf * col_s[1], axis=0, keepdims=True))
            g_s[:, sl] = g
            o_ref[:, sl] = (1.0 - g) * (yT[:, t * 128:(t + 1) * 128] + xf * col_s[0])

    nc = S // TC
    zero = jnp.zeros((1, 512), f32)
    u0 = bu(0)
    u_s[...] = bu(1)
    h0, carry = scan(u0, (zero, zero))
    h_s[...] = h0

    def body(k, carry):
        i = 2 * k + 1
        ua = u_s[...]
        hp = h_s[...]
        ub = bu(i + 1)
        h1, carry = scan(ua, carry)
        finish(i - 1, hp)
        u_s[...] = bu(i + 2)
        h2, carry = scan(ub, carry)
        finish(i, h1)
        h_s[...] = h2
        return carry

    carry = lax.fori_loop(0, nc // 2 - 1, body, carry)
    hl, _ = scan(u_s[...], carry)
    finish(nc - 2, h_s[...])
    finish(nc - 1, hl)


def _kernel(xT_ref, bre_ref, bim_ref, cre_ref, cim_ref, lre_ref, lim_ref, ldt_ref,
            dsk_ref, gw_ref, woT_ref, ckv_hbm, wq_hbm, wk_hbm, wv_hbm,
            o_ref,
            ckv_s, rq, rk, rv, sq, sk, sv, k_s, vT_s, qT_s, cT_s, g_s,
            b_s, c_s, lam_s, col_s, u_s, h_s, sem):
    h = pl.program_id(0)
    raws, stgs = (rq, rk, rv), (sq, sk, sv)
    cp_ckv = pltpu.make_async_copy(ckv_hbm, ckv_s, sem.at[12])
    cps = [_weight_copies(w, raw, sem, 4 * n)
           for n, (w, raw) in enumerate(zip((wq_hbm, wk_hbm, wv_hbm), raws))]

    @pl.when(h == 0)
    def _():
        cp_ckv.start()
        for k in range(4):
            for cp in cps:
                cp[k].start()
        _ssm_and_gate(xT_ref, bre_ref, bim_ref, cre_ref, cim_ref, lre_ref, lim_ref,
                      ldt_ref, dsk_ref, gw_ref, o_ref, g_s, b_s, c_s, lam_s, col_s, u_s, h_s)
        cp_ckv.wait()
        for k in range(2):
            for cp in cps:
                cp[k].wait()

        def stage0(sl, carry):
            _stage_slice(raws, stgs, 0, sl)
            return carry
        lax.fori_loop(0, 4, stage0, 0)

    @pl.when(h == 4)
    def _():
        for k in range(2, 4):
            for cp in cps:
                cp[k].wait()

    ckv = ckv_s[...]
    wk = _head_weight(sk, h, DC).astype(bf16)
    k_s[...] = _dot(ckv, wk, _NN).astype(bf16)
    wq = _head_weight(sq, h, M).astype(bf16)
    qT_s[...] = (_dot(wq, xT_ref[...], _TN) * (LOG2E * D ** -0.5)).astype(bf16)
    wv = _head_weight(sv, h, DC).astype(bf16)
    vT_s[...] = _dot(wv, ckv, _TT).astype(bf16)
    _stage_slice(raws, stgs, (h >= 4).astype(jnp.int32), h & 3)

    key = lax.broadcasted_iota(jnp.int32, (TQ, TQ), 0)
    qry = lax.broadcasted_iota(jnp.int32, (TQ, TQ), 1)
    causal = key <= qry

    def qk(j):
        kv = (j + 1) * TQ
        s = _dot(k_s[0:kv, :], qT_s[:, j * TQ:(j + 1) * TQ], _NN)
        sd = jnp.where(causal, s[kv - TQ:kv], -1e30)
        return jnp.concatenate([s[:kv - TQ], sd], axis=0) if j > 0 else sd

    def softmax_pv(j, s):
        kv = (j + 1) * TQ
        parts = [jnp.max(s[a:min(a + 512, kv)], axis=0, keepdims=True) for a in range(0, kv, 512)]
        m = parts[0]
        for part in parts[1:]:
            m = jnp.maximum(m, part)
        p = jnp.exp2(s - m)
        l = jnp.sum(p, axis=0, keepdims=True)
        c = _dot(vT_s[:, 0:kv], p.astype(bf16), _NN)
        scale = g_s[:, j * TQ:(j + 1) * TQ] / l
        cT_s[:, j * TQ:(j + 1) * TQ] = (c * scale).astype(bf16)

    ss = {0: qk(0), 1: qk(1)}
    for j in range(NQ):
        if j + 2 < NQ:
            ss[j + 2] = qk(j + 2)
        softmax_pv(j, ss.pop(j))

    o_ref[...] += _dot(woT_ref[...], cT_s[...], _NN)


@jax.jit
def pallas_gated_mix__compressed_kv_cla__ssm_conv_s5__prompt_kernel(
    A_x: jax.Array,
    A_c_kv: jax.Array,
    A_w_q: jax.Array,
    A_w_uk: jax.Array,
    A_w_uv: jax.Array,
    A_w_o: jax.Array,
    B_x: jax.Array,
    B_Lambda_re: jax.Array,
    B_Lambda_im: jax.Array,
    B_B_re: jax.Array,
    B_B_im: jax.Array,
    B_C_re: jax.Array,
    B_C_im: jax.Array,
    B_log_dt: jax.Array,
    B_Dskip: jax.Array,
    gate_w: jax.Array,
):
    del B_x
    xT = jnp.transpose(A_x[0])
    woT = jnp.transpose(A_w_o, (0, 2, 1))
    ckv = A_c_kv[0]

    full2 = lambda shape: pl.BlockSpec(shape, lambda h: (0, 0))
    vec = pl.BlockSpec((M,), lambda h: (0,))
    hbm = pl.BlockSpec(memory_space=pl.ANY)
    outT = pl.pallas_call(
        _kernel,
        grid=(H,),
        in_specs=[full2((M, S)), full2((M, M)), full2((M, M)), full2((M, M)), full2((M, M)),
                  vec, vec, vec, vec, vec,
                  pl.BlockSpec((None, M, D), lambda h: (h, 0, 0)),
                  hbm, hbm, hbm, hbm],
        out_specs=full2((M, S)),
        out_shape=jax.ShapeDtypeStruct((M, S), f32),
        scratch_shapes=[
            pltpu.VMEM((S, DC), bf16),
            pltpu.VMEM((4, M, 8, 128), bf16),
            pltpu.VMEM((4, DC, 8, 128), bf16),
            pltpu.VMEM((4, DC, 8, 128), bf16),
            pltpu.VMEM((4, M * 4, 128), u32),
            pltpu.VMEM((4, DC * 4, 128), u32),
            pltpu.VMEM((4, DC * 4, 128), u32),
            pltpu.VMEM((S, D), bf16),
            pltpu.VMEM((D, S), bf16),
            pltpu.VMEM((D, S), bf16),
            pltpu.VMEM((D, S), bf16),
            pltpu.VMEM((1, S), f32),
            pltpu.VMEM((2 * M, M), bf16),
            pltpu.VMEM((M, 2 * M), bf16),
            pltpu.VMEM((8, 8, 512), f32),
            pltpu.VMEM((2, M, 128), f32),
            pltpu.VMEM((TC, 2 * M), f32),
            pltpu.VMEM((TC, 2 * M), bf16),
            pltpu.SemaphoreType.DMA((13,)),
        ],
        compiler_params=pltpu.CompilerParams(
            dimension_semantics=("arbitrary",),
            vmem_limit_bytes=110 * 1024 * 1024,
        ),
    )(xT, B_B_re, B_B_im, B_C_re, B_C_im, B_Lambda_re, B_Lambda_im, B_log_dt,
      B_Dskip, gate_w, woT, ckv, A_w_q, A_w_uk, A_w_uv)
    return jnp.transpose(outT)[None]
```

```python
import jax
import jax.numpy as jnp
from jax import lax
import jax.experimental.pallas as pl
import jax.experimental.pallas.tpu as pltpu

S = 2048
M = 448
H = 16
D = 256
DC = 1024
TQ = 128
NQ = S // TQ
PA = 384
PB = M - PA
TC = 256
LOG2E = 1.4426950408889634

f32 = jnp.float32
bf16 = jnp.bfloat16
u32 = jnp.uint32


def _dot(a, b, dims):
    return lax.dot_general(a, b, (dims, ((), ())), preferred_element_type=f32)


_NN = ((1,), (0,))
_NT = ((1,), (1,))
_TN = ((0,), (0,))
_TT = ((0,), (1,))


def _cmul(ar, ai, br, bi):
    return ar * br - ai * bi, ar * bi + ai * br


def _strassen_a(a11, a12, a21, a22):
    return [a11 + a22, a21 + a22, a11, a22, a11 + a12, a21 - a11, a12 - a22]


def _strassen_b(b11, b12, b21, b22):
    return [b11 + b22, b11, b12 - b22, b21 - b11, b22, b11 + b12, b21 + b22]


def _strassen_c(m):
    c11 = (m[0] + m[3]) + (m[6] - m[4])
    c12 = m[2] + m[4]
    c21 = m[1] + m[3]
    c22 = (m[0] - m[1]) + (m[2] + m[5])
    return c11, c12, c21, c22


def _weight_copies(w_hbm, raw, sem, sem0):
    return [
        pltpu.make_async_copy(
            w_hbm.at[:, ht * 8:(ht + 1) * 8, dt * 128:(dt + 1) * 128],
            raw.at[ht * 2 + dt], sem.at[sem0 + ht * 2 + dt])
        for ht in range(2) for dt in range(2)
    ]


def _stage(raw, stg, k, c0, nc):
    v = raw[k, pl.ds(c0, nc)].reshape(nc * 8, 128)
    stg[k, pl.ds(pl.multiple_of(c0 * 4, 8), nc * 4), :] = pltpu.bitcast(v, u32)


def _stage_slice(raws, stgs, group, sl):
    for raw, stg, rows in zip(raws, stgs, (M, DC, DC)):
        for dt in range(2):
            _stage(raw, stg, group * 2 + dt, sl * (rows // 4), rows // 4)


def _head_weight(stg, h, rows):
    ht = lax.shift_right_logical(h, 3)
    pr = lax.shift_right_logical(h & 7, 1)
    sh = (16 * (1 - (h & 1))).astype(u32)
    halves = []
    for dt in range(2):
        u = stg[ht * 2 + dt, pl.ds(pr, rows, stride=4), :]
        halves.append(pltpu.bitcast((u << sh) & jnp.uint32(0xFFFF0000), f32))
    r = rows // 2
    ops = _strassen_b(halves[0][:r], halves[1][:r], halves[0][r:], halves[1][r:])
    return [o.astype(bf16) for o in ops]


def _ssm_and_gate(xT_ref, bre_ref, bim_ref, cre_ref, cim_ref, lre_ref, lim_ref,
                  ldt_ref, dsk_ref, gw_ref, o_ref, g_s, b_s, c_s, lam_s, col_s, u_s, h_s):
    row = lambda r: r[...].astype(f32).reshape(1, M)
    lre, lim = row(lre_ref), row(lim_ref)
    dt = jnp.exp(row(ldt_ref)).astype(bf16).astype(f32)
    mag = jnp.exp(dt * lre)
    ang = dt * lim
    lr, li = mag * jnp.cos(ang), mag * jnp.sin(ang)
    den = lre * lre + lim * lim
    nr = lr - 1.0
    cr = (nr * lre + li * lim) / den
    ci = (li * lre - nr * lim) / den
    c_re, c_im = cre_ref[...].astype(f32), cim_ref[...].astype(f32)
    cp_re, cp_im = _cmul(c_re, c_im, 2.0 * cr, 2.0 * ci)
    c_s[...] = jnp.concatenate(
        [cp_re[:, :PA], -cp_im[:, :PA], cp_re[:, PA:], -cp_im[:, PA:]], axis=1).astype(bf16)
    b_s[0:PA, :] = bre_ref[0:PA, :]
    b_s[PA:2 * PA, :] = bim_ref[0:PA, :]
    b_s[2 * PA:2 * PA + PB, :] = bre_ref[PA:M, :]
    b_s[2 * PA + PB:2 * M, :] = bim_ref[PA:M, :]

    er = jnp.concatenate([lr, lr[:, PA:]], axis=1)
    ei = jnp.concatenate([li, -li[:, PA:]], axis=1)
    pw = [(er, ei)]
    for _ in range(7):
        pw.append(_cmul(pw[-1][0], pw[-1][1], er, ei))
    sub = lax.broadcasted_iota(jnp.int32, (8, 512), 0)
    for n, d in enumerate((1, 2, 4)):
        lam_s[2 * n] = jnp.where(sub >= d, pw[d - 1][0], 0.0)
        lam_s[2 * n + 1] = jnp.where(sub >= d, pw[d - 1][1], 0.0)
    lcr = jnp.zeros((8, 512), f32)
    lci = jnp.zeros((8, 512), f32)
    for r in range(8):
        lcr = jnp.where(sub == r, pw[r][0], lcr)
        lci = jnp.where(sub == r, pw[r][1], lci)
    lam_s[6] = lcr
    lam_s[7] = lci

    def col(r):
        v = jnp.concatenate([row(r), jnp.zeros((1, 512 - M), f32)], axis=1)
        return jnp.broadcast_to(v, (128, 512)).T[:M]
    col_s[0] = col(dsk_ref)
    col_s[1] = col(gw_ref)

    def lanes(lo, n):
        return pl.ds(lo if isinstance(lo, int) else pl.multiple_of(lo, 128), n)

    def bu(i):
        return _dot(xT_ref[:, lanes(i * TC, TC)], b_s[...], _TT)

    def scan(u, carry):
        nb = TC // 8
        mixed = u[:, 2 * PA:]
        hr = jnp.concatenate([u[:, :PA], mixed], axis=1).reshape(nb, 8, 512)
        hi = jnp.concatenate([u[:, PA:2 * PA], pltpu.roll(mixed, PB, 1)], axis=1).reshape(nb, 8, 512)
        for n, d in enumerate((1, 2, 4)):
            sr, si = pltpu.roll(hr, d, 1), pltpu.roll(hi, d, 1)
            tr, ti = _cmul(sr, si, lam_s[2 * n][None], lam_s[2 * n + 1][None])
            hr, hi = hr + tr, hi + ti
        lcr, lci = lam_s[6], lam_s[7]
        car, cai = carry
        outr, outi = [], []
        for b in range(nb):
            tr, ti = _cmul(lcr, lci, car, cai)
            br, bi = hr[b] + tr, hi[b] + ti
            outr.append(br)
            outi.append(bi)
            car, cai = br[7:8, :], bi[7:8, :]
        hr = jnp.concatenate(outr, axis=0)
        hi = jnp.concatenate(outi, axis=0)
        h = jnp.concatenate([hr[:, :PA], hi[:, :PA], hr[:, PA:]], axis=1).astype(bf16)
        return h, (car, cai)

    def finish(i, h):
        yT = _dot(c_s[...], h, _NT)
        for t in range(TC // 128):
            sl = lanes(i * TC + t * 128, 128)
            xf = xT_ref[:, sl].astype(f32)
            g = jax.nn.sigmoid(jnp.sum(xf * col_s[1], axis=0, keepdims=True))
            g_s[:, sl] = g
            o_ref[:, sl] = (1.0 - g) * (yT[:, t * 128:(t + 1) * 128] + xf * col_s[0])

    nc = S // TC
    zero = jnp.zeros((1, 512), f32)
    u0 = bu(0)
    u_s[...] = bu(1)
    h0, carry = scan(u0, (zero, zero))
    h_s[...] = h0

    def body(k, carry):
        i = 2 * k + 1
        ua = u_s[...]
        hp = h_s[...]
        ub = bu(i + 1)
        h1, carry = scan(ua, carry)
        finish(i - 1, hp)
        u_s[...] = bu(i + 2)
        h2, carry = scan(ub, carry)
        finish(i, h1)
        h_s[...] = h2
        return carry

    carry = lax.fori_loop(0, nc // 2 - 1, body, carry)
    hl, _ = scan(u_s[...], carry)
    finish(nc - 2, h_s[...])
    finish(nc - 1, hl)


def _kernel(xT_ref, bre_ref, bim_ref, cre_ref, cim_ref, lre_ref, lim_ref, ldt_ref,
            dsk_ref, gw_ref, woT_ref, ckv_hbm, wq_hbm, wk_hbm, wv_hbm,
            o_ref,
            ckv_s, rq, rk, rv, sq, sk, sv, k_s, vT_s, qT_s, cT_s, g_s,
            b_s, c_s, lam_s, col_s, u_s, h_s, a_s, xa_s, sem):
    h = pl.program_id(0)
    raws, stgs = (rq, rk, rv), (sq, sk, sv)
    cp_ckv = pltpu.make_async_copy(ckv_hbm, ckv_s, sem.at[12])
    cps = [_weight_copies(w, raw, sem, 4 * n)
           for n, (w, raw) in enumerate(zip((wq_hbm, wk_hbm, wv_hbm), raws))]

    @pl.when(h == 0)
    def _():
        cp_ckv.start()
        for k in range(4):
            for cp in cps:
                cp[k].start()
        _ssm_and_gate(xT_ref, bre_ref, bim_ref, cre_ref, cim_ref, lre_ref, lim_ref,
                      ldt_ref, dsk_ref, gw_ref, o_ref, g_s, b_s, c_s, lam_s, col_s, u_s, h_s)
        cp_ckv.wait()
        for k in range(2):
            for cp in cps:
                cp[k].wait()

        def stage0(sl, carry):
            _stage_slice(raws, stgs, 0, sl)
            r = S // 8
            top = pl.ds(pl.multiple_of(sl * r, r), r)
            bot = pl.ds(pl.multiple_of(S // 2 + sl * r, r), r)
            ops = _strassen_a(ckv_s[top, 0:DC // 2].astype(f32), ckv_s[top, DC // 2:DC].astype(f32),
                              ckv_s[bot, 0:DC // 2].astype(f32), ckv_s[bot, DC // 2:DC].astype(f32))
            for i in range(7):
                a_s[i, top, :] = ops[i].astype(bf16)
            ops = _strassen_a(xT_ref[0:M // 2, top].astype(f32), xT_ref[M // 2:M, top].astype(f32),
                              xT_ref[0:M // 2, bot].astype(f32), xT_ref[M // 2:M, bot].astype(f32))
            for i in range(7):
                xa_s[i, :, top] = ops[i].astype(bf16)
            return carry
        lax.fori_loop(0, 4, stage0, 0)

    @pl.when(h == 4)
    def _():
        for k in range(2, 4):
            for cp in cps:
                cp[k].wait()

    hs, hd = S // 2, D // 2
    wk = _head_weight(sk, h, DC)
    c11, c12, c21, c22 = _strassen_c([_dot(a_s[i], wk[i], _NN) for i in range(7)])
    k_s[0:hs, 0:hd] = c11.astype(bf16)
    k_s[0:hs, hd:D] = c12.astype(bf16)
    k_s[hs:S, 0:hd] = c21.astype(bf16)
    k_s[hs:S, hd:D] = c22.astype(bf16)

    wq = _head_weight(sq, h, M)
    c11, c12, c21, c22 = _strassen_c([_dot(wq[i], xa_s[i], _TN) for i in range(7)])
    qs = LOG2E * D ** -0.5
    qT_s[0:hd, 0:hs] = (c11 * qs).astype(bf16)
    qT_s[hd:D, 0:hs] = (c12 * qs).astype(bf16)
    qT_s[0:hd, hs:S] = (c21 * qs).astype(bf16)
    qT_s[hd:D, hs:S] = (c22 * qs).astype(bf16)

    wv = _head_weight(sv, h, DC)
    c11, c12, c21, c22 = _strassen_c([_dot(wv[i], a_s[i], _TT) for i in range(7)])
    vT_s[0:hd, 0:hs] = c11.astype(bf16)
    vT_s[hd:D, 0:hs] = c12.astype(bf16)
    vT_s[0:hd, hs:S] = c21.astype(bf16)
    vT_s[hd:D, hs:S] = c22.astype(bf16)
    _stage_slice(raws, stgs, (h >= 4).astype(jnp.int32), h & 3)

    key = lax.broadcasted_iota(jnp.int32, (TQ, TQ), 0)
    qry = lax.broadcasted_iota(jnp.int32, (TQ, TQ), 1)
    causal = key <= qry

    def qk(j):
        kv = (j + 1) * TQ
        s = _dot(k_s[0:kv, :], qT_s[:, j * TQ:(j + 1) * TQ], _NN)
        sd = jnp.where(causal, s[kv - TQ:kv], -1e30)
        return jnp.concatenate([s[:kv - TQ], sd], axis=0) if j > 0 else sd

    def softmax_pv(j, s):
        kv = (j + 1) * TQ
        parts = [jnp.max(s[a:min(a + 512, kv)], axis=0, keepdims=True) for a in range(0, kv, 512)]
        m = parts[0]
        for part in parts[1:]:
            m = jnp.maximum(m, part)
        p = jnp.exp2(s - m)
        l = jnp.sum(p, axis=0, keepdims=True)
        c = _dot(vT_s[:, 0:kv], p.astype(bf16), _NN)
        scale = g_s[:, j * TQ:(j + 1) * TQ] / l
        cT_s[:, j * TQ:(j + 1) * TQ] = (c * scale).astype(bf16)

    ss = {0: qk(0), 1: qk(1)}
    for j in range(NQ):
        if j + 2 < NQ:
            ss[j + 2] = qk(j + 2)
        softmax_pv(j, ss.pop(j))

    o_ref[...] += _dot(woT_ref[...], cT_s[...], _NN)


@jax.jit
def pallas_gated_mix__compressed_kv_cla__ssm_conv_s5__prompt_kernel(
    A_x: jax.Array,
    A_c_kv: jax.Array,
    A_w_q: jax.Array,
    A_w_uk: jax.Array,
    A_w_uv: jax.Array,
    A_w_o: jax.Array,
    B_x: jax.Array,
    B_Lambda_re: jax.Array,
    B_Lambda_im: jax.Array,
    B_B_re: jax.Array,
    B_B_im: jax.Array,
    B_C_re: jax.Array,
    B_C_im: jax.Array,
    B_log_dt: jax.Array,
    B_Dskip: jax.Array,
    gate_w: jax.Array,
):
    del B_x
    xT = jnp.transpose(A_x[0])
    woT = jnp.transpose(A_w_o, (0, 2, 1))
    ckv = A_c_kv[0]

    full2 = lambda shape: pl.BlockSpec(shape, lambda h: (0, 0))
    vec = pl.BlockSpec((M,), lambda h: (0,))
    hbm = pl.BlockSpec(memory_space=pl.ANY)
    outT = pl.pallas_call(
        _kernel,
        grid=(H,),
        in_specs=[full2((M, S)), full2((M, M)), full2((M, M)), full2((M, M)), full2((M, M)),
                  vec, vec, vec, vec, vec,
                  pl.BlockSpec((None, M, D), lambda h: (h, 0, 0)),
                  hbm, hbm, hbm, hbm],
        out_specs=full2((M, S)),
        out_shape=jax.ShapeDtypeStruct((M, S), f32),
        scratch_shapes=[
            pltpu.VMEM((S, DC), bf16),
            pltpu.VMEM((4, M, 8, 128), bf16),
            pltpu.VMEM((4, DC, 8, 128), bf16),
            pltpu.VMEM((4, DC, 8, 128), bf16),
            pltpu.VMEM((4, M * 4, 128), u32),
            pltpu.VMEM((4, DC * 4, 128), u32),
            pltpu.VMEM((4, DC * 4, 128), u32),
            pltpu.VMEM((S, D), bf16),
            pltpu.VMEM((D, S), bf16),
            pltpu.VMEM((D, S), bf16),
            pltpu.VMEM((D, S), bf16),
            pltpu.VMEM((1, S), f32),
            pltpu.VMEM((2 * M, M), bf16),
            pltpu.VMEM((M, 2 * M), bf16),
            pltpu.VMEM((8, 8, 512), f32),
            pltpu.VMEM((2, M, 128), f32),
            pltpu.VMEM((TC, 2 * M), f32),
            pltpu.VMEM((TC, 2 * M), bf16),
            pltpu.VMEM((7, S // 2, DC // 2), bf16),
            pltpu.VMEM((7, M // 2, S // 2), bf16),
            pltpu.SemaphoreType.DMA((13,)),
        ],
        compiler_params=pltpu.CompilerParams(
            dimension_semantics=("arbitrary",),
            vmem_limit_bytes=110 * 1024 * 1024,
        ),
    )(xT, B_B_re, B_B_im, B_C_re, B_C_im, B_Lambda_re, B_Lambda_im, B_log_dt,
      B_Dskip, gate_w, woT, ckv, A_w_q, A_w_uk, A_w_uv)
    return jnp.transpose(outT)[None]
```

```python
import jax
import jax.numpy as jnp
from jax import lax
import jax.experimental.pallas as pl
import jax.experimental.pallas.tpu as pltpu

S = 2048
M = 448
H = 16
D = 256
DC = 1024
T = 128
NT = S // T
NP = NT // 2
HD = D // 2
HM = M // 2
PA = 384
PB = M - PA
TA = 512
TC = 256
CS = DC // NP
LOG2E = 1.4426950408889634

f32 = jnp.float32
bf16 = jnp.bfloat16
u32 = jnp.uint32

SEM_VEC, SEM_B, SEM_X, SEM_WQ, SEM_C, SEM_SL, SEM_WO, SEM_OUT = 0, 1, 2, 6, 7, 8, 16, 17
NSEM = 18


def _dot(a, b, dims):
    return lax.dot_general(a, b, (dims, ((), ())), preferred_element_type=f32)


_NN = ((1,), (0,))
_NT = ((1,), (1,))
_TN = ((0,), (0,))
_TT = ((0,), (1,))


def _pk(x):
    return pltpu.bitcast(x, u32)


def _up(x):
    return pltpu.bitcast(x, bf16)


def _cmul(ar, ai, br, bi):
    return ar * br - ai * bi, ar * bi + ai * br


def _ds(lo, n, align):
    return pl.ds(lo if isinstance(lo, int) else pl.multiple_of(lo, align), n)


def _strassen_a(a11, a12, a21, a22):
    ops = [a11 + a22, a21 + a22, a11, a22, a11 + a12, a21 - a11, a12 - a22]
    return [o.astype(bf16) for o in ops]


def _strassen_b(b11, b12, b21, b22):
    ops = [b11 + b22, b11, b12 - b22, b21 - b11, b22, b11 + b12, b21 + b22]
    return [o.astype(bf16) for o in ops]


def _strassen_c(m):
    c11 = (m[0] + m[3]) + (m[6] - m[4])
    c12 = m[2] + m[4]
    c21 = m[1] + m[3]
    c22 = (m[0] - m[1]) + (m[2] + m[5])
    return c11, c12, c21, c22


def _stage(raw, stg, c0, nc):
    for ht in range(2):
        for dt in range(2):
            v = raw[pl.ds(c0, nc), ht * 8:(ht + 1) * 8, dt * 128:(dt + 1) * 128]
            stg[ht * 2 + dt, _ds(c0 * 4, nc * 4, 8), :] = _pk(v.reshape(nc * 8, 128))


def _pair_words(stg, pair, rows):
    ht = lax.shift_right_logical(pair, 2)
    return [stg[ht * 2 + dt, pl.ds(pair & 3, rows, stride=4), :] for dt in range(2)]


def _weight_ops(halves, rows):
    r = rows // 2
    return _strassen_b(halves[0][:r], halves[1][:r], halves[0][r:], halves[1][r:])


def _head_weight_ops(stg, h, rows):
    sh = (16 * (1 - (h & 1))).astype(u32)
    words = _pair_words(stg, lax.shift_right_logical(h, 1), rows)
    halves = [pltpu.bitcast((u << sh) & jnp.uint32(0xFFFF0000), f32) for u in words]
    return _weight_ops(halves, rows)


def _ssm_params(vec_s, craw_s, c_s, lam_s, col_s):
    row = lambda r: r[...].astype(f32).reshape(1, M)
    lre, lim, ldt, dsk, gw = [row(v) for v in vec_s]
    dt = jnp.exp(ldt).astype(bf16).astype(f32)
    mag = jnp.exp(dt * lre)
    ang = dt * lim
    lr, li = mag * jnp.cos(ang), mag * jnp.sin(ang)
    den = lre * lre + lim * lim
    nr = lr - 1.0
    cr = (nr * lre + li * lim) / den
    ci = (li * lre - nr * lim) / den
    cp_re, cp_im = _cmul(craw_s[0].astype(f32), craw_s[1].astype(f32), 2.0 * cr, 2.0 * ci)
    c_s[...] = _pk(jnp.concatenate(
        [cp_re[:, :PA], -cp_im[:, :PA], cp_re[:, PA:], -cp_im[:, PA:]], axis=1).astype(bf16))

    er = jnp.concatenate([lr, lr[:, PA:]], axis=1)
    ei = jnp.concatenate([li, -li[:, PA:]], axis=1)
    pw = [(er, ei)]
    for _ in range(7):
        pw.append(_cmul(pw[-1][0], pw[-1][1], er, ei))
    sub = lax.broadcasted_iota(jnp.int32, (8, 512), 0)
    for n, d in enumerate((1, 2, 4)):
        lam_s[2 * n] = jnp.where(sub >= d, pw[d - 1][0], 0.0)
        lam_s[2 * n + 1] = jnp.where(sub >= d, pw[d - 1][1], 0.0)
    lcr = jnp.zeros((8, 512), f32)
    lci = jnp.zeros((8, 512), f32)
    for r in range(8):
        lcr = jnp.where(sub == r, pw[r][0], lcr)
        lci = jnp.where(sub == r, pw[r][1], lci)
    lam_s[6] = lcr
    lam_s[7] = lci

    def col(v):
        v = jnp.concatenate([v, jnp.zeros((1, 512 - M), f32)], axis=1)
        return jnp.broadcast_to(v, (128, 512)).T[:M]
    col_s[0] = col(dsk)
    col_s[1] = col(gw)


def _ssm_scan(u_s, t0, carry, lam_s):
    car, cai = carry
    out = []
    for b in range(TC // 8):
        u = u_s[_ds(t0 + b * 8, 8, 8), :]
        mixed = u[:, 2 * PA:]
        hr = jnp.concatenate([u[:, :PA], mixed], axis=1)
        hi = jnp.concatenate([u[:, PA:2 * PA], pltpu.roll(mixed, PB, 1)], axis=1)
        for n, d in enumerate((1, 2, 4)):
            sr, si = pltpu.roll(hr, d, 0), pltpu.roll(hi, d, 0)
            tr, ti = _cmul(sr, si, lam_s[2 * n], lam_s[2 * n + 1])
            hr, hi = hr + tr, hi + ti
        tr, ti = _cmul(lam_s[6], lam_s[7], car, cai)
        hr, hi = hr + tr, hi + ti
        car, cai = hr[7:8, :], hi[7:8, :]
        out.append(jnp.concatenate([hr[:, :PA], hi[:, :PA], hr[:, PA:]], axis=1))
    return jnp.concatenate(out, axis=0).astype(bf16), (car, cai)


def _kernel(xT_hbm, bre_hbm, bim_hbm, cre_hbm, cim_hbm, lre_hbm, lim_hbm, ldt_hbm,
            dsk_hbm, gw_hbm, woT_hbm, ckv_hbm, wq_hbm, wk_hbm, wv_hbm,
            out_hbm,
            xT_s, v0, v1, v2, v3, v4, b_s, craw_s, c_s, lam_s, col_s, u_s, g_s,
            ckv_s, rq, rk, rv, sq, sk, sv, a_s, xa_s, q_s, wo_s,
            k_s, vT_s, o_s, s_s, sem):
    h = pl.program_id(0)
    vec_s = (v0, v1, v2, v3, v4)

    def slice_copies(i):
        s = sem.at[SEM_SL + i]
        rows = _ds(i * 2 * T, 2 * T, 2 * T)
        cs = pl.ds(i * CS, CS)
        return [pltpu.make_async_copy(ckv_hbm.at[rows], ckv_s.at[rows], s),
                pltpu.make_async_copy(wk_hbm.at[cs], rk.at[cs], s),
                pltpu.make_async_copy(wv_hbm.at[cs], rv.at[cs], s)]

    def x_copy(i):
        cols = _ds(i * TA, TA, TA)
        return pltpu.make_async_copy(xT_hbm.at[:, cols], xT_s.at[:, cols], sem.at[SEM_X + i])

    def out_copy(jp):
        cols = pl.ds(jp * 2 * T, 2 * T)
        return pltpu.make_async_copy(o_s.at[:, cols], out_hbm.at[:, cols], sem.at[SEM_OUT])

    @pl.when(h == 0)
    def _():
        cp_vec = [pltpu.make_async_copy(src, dst, sem.at[SEM_VEC])
                  for src, dst in zip((lre_hbm, lim_hbm, ldt_hbm, dsk_hbm, gw_hbm), vec_s)]
        cp_b = [pltpu.make_async_copy(src.at[pl.ds(lo, n)], b_s.at[pl.ds(dst, n)], sem.at[SEM_B])
                for src, lo, n, dst in ((bre_hbm, 0, PA, 0), (bim_hbm, 0, PA, PA),
                                        (bre_hbm, PA, PB, 2 * PA), (bim_hbm, PA, PB, 2 * PA + PB))]
        cp_wq = [pltpu.make_async_copy(wq_hbm, rq, sem.at[SEM_WQ])]
        cp_c = [pltpu.make_async_copy(src, craw_s.at[n], sem.at[SEM_C])
                for n, src in enumerate((cre_hbm, cim_hbm))]
        cp_wo = pltpu.make_async_copy(woT_hbm, wo_s, sem.at[SEM_WO])
        for cp in cp_b:
            cp.start()
        for i in range(S // TA):
            x_copy(i).start()
        for cp in cp_vec + cp_wq + cp_c:
            cp.start()
        for i in range(NP):
            for cp in slice_copies(i):
                cp.start()
        cp_wo.start()

        def phase1(i):
            x_copy(i).wait()
            u_s[_ds(i * TA, TA, TA), :] = _dot(xT_s[:, _ds(i * TA, TA, TA)], b_s[...], _TT)
            for t in range(TA // (2 * T)):
                ev = _ds(i * TA + 2 * t * T, T, T)
                od = _ds(i * TA + (2 * t + 1) * T, T, T)
                ops = _strassen_a(xT_s[0:HM, ev].astype(f32), xT_s[HM:M, ev].astype(f32),
                                  xT_s[0:HM, od].astype(f32), xT_s[HM:M, od].astype(f32))
                for n in range(7):
                    xa_s[n, :, _ds(i * (TA // 2) + t * T, T, T)] = _pk(ops[n])

        for cp in cp_b:
            cp.wait()

        def phase1_body(i, carry):
            phase1(i)
            return carry
        lax.fori_loop(0, S // TA - 1, phase1_body, 0)
        for cp in cp_vec + cp_wq + cp_c:
            cp.wait()
        phase1(S // TA - 1)
        _stage(rq, sq, 0, M)
        _ssm_params(vec_s, craw_s, c_s, lam_s, col_s)

        def phase2(i, carry):
            for cp in slice_copies(i):
                cp.wait()
            words = _pair_words(sq, i, M)
            lo = _weight_ops([pltpu.bitcast(u << 16, f32) for u in words], M)
            hi = _weight_ops([pltpu.bitcast(u & jnp.uint32(0xFFFF0000), f32) for u in words], M)
            prods = [_dot(jnp.concatenate([lo[n], hi[n]], axis=1), _up(xa_s[n]), _TN) for n in range(7)]
            qs = LOG2E * D ** -0.5
            for n, c in enumerate(_strassen_c(prods)):
                c = c * qs
                rows = pl.ds((n % 2) * (HD // 2), HD // 2)
                q_s[2 * i, n // 2, rows, :] = _pk(c[:HD].astype(bf16))
                q_s[2 * i + 1, n // 2, rows, :] = _pk(c[HD:].astype(bf16))

            hseq, carry = _ssm_scan(u_s, i * TC, carry, lam_s)
            yT = _dot(_up(c_s[...]), hseq, _NT)
            for t in range(TC // T):
                cols = _ds(i * TC + t * T, T, T)
                xf = xT_s[:, cols].astype(f32)
                g = jax.nn.sigmoid(jnp.sum(xf * col_s[1], axis=0, keepdims=True))
                g_s[:, cols] = g
                o_s[:, cols] = (1.0 - g) * (yT[:, t * T:(t + 1) * T] + xf * col_s[0])

            _stage(rk, sk, i * CS, CS)
            _stage(rv, sv, i * CS, CS)
            ev = _ds(i * 2 * T, T, T)
            od = _ds(i * 2 * T + T, T, T)
            hc = DC // 2
            ops = _strassen_a(ckv_s[ev, 0:hc].astype(f32), ckv_s[ev, hc:DC].astype(f32),
                              ckv_s[od, 0:hc].astype(f32), ckv_s[od, hc:DC].astype(f32))
            for n in range(7):
                a_s[n, _ds(i * (T // 2), T // 2, T // 2), :] = _pk(ops[n])
            return carry

        zero = jnp.zeros((1, 512), f32)
        lax.fori_loop(0, NP, phase2, (zero, zero))
        cp_wo.wait()

    wk = _head_weight_ops(sk, h, DC)
    for n, c in enumerate(_strassen_c([_dot(_up(a_s[i]), wk[i], _NN) for i in range(7)])):
        for t in range(NP):
            k_s[pl.ds((2 * t + n // 2) * (T // 2), T // 2), pl.ds((n % 2) * HD, HD)] = (
                _pk(c[t * T:(t + 1) * T].astype(bf16)))

    wv = _head_weight_ops(sv, h, DC)
    for n, c in enumerate(_strassen_c([_dot(wv[i], _up(a_s[i]), _TT) for i in range(7)])):
        for t in range(NP):
            vT_s[pl.ds((n % 2) * (HD // 2), HD // 2), pl.ds((2 * t + n // 2) * T, T)] = (
                _pk(c[:, t * T:(t + 1) * T].astype(bf16)))

    wo = wo_s[h].astype(f32)
    wo = _strassen_a(wo[:HM, :HD], wo[:HM, HD:], wo[HM:, :HD], wo[HM:, HD:])

    key = lax.broadcasted_iota(jnp.int32, (T, T), 0)
    qry = lax.broadcasted_iota(jnp.int32, (T, T), 1)
    causal = key <= qry

    def qk(j):
        kv = (j + 1) * T
        qT = _up(q_s[h, j % 2, :, pl.ds((j // 2) * T, T)])
        s = _dot(_up(k_s[0:kv // 2, :]), qT, _NN)
        sd = jnp.where(causal, s[kv - T:kv], -1e30)
        s = jnp.concatenate([s[:kv - T], sd], axis=0) if j > 0 else sd
        s_s[j % 3, 0:kv, :] = s
        parts = [jnp.max(s[a:min(a + 512, kv)], axis=0, keepdims=True) for a in range(0, kv, 512)]
        m = parts[0]
        for part in parts[1:]:
            m = jnp.maximum(m, part)
        return m

    def softmax_pv(j, m):
        kv = (j + 1) * T
        p = jnp.exp2(s_s[j % 3, 0:kv, :] - m)
        l = jnp.sum(p, axis=0, keepdims=True)
        c = _dot(_up(vT_s[:, 0:kv]), p.astype(bf16), _NN)
        return c * (g_s[:, j * T:(j + 1) * T] / l)

    def oproj(jp, ce, co):
        ops = _strassen_b(ce[:HD], co[:HD], ce[HD:], co[HD:])
        for n, c in enumerate(_strassen_c([_dot(wo[i], ops[i], _NN) for i in range(7)])):
            rows = pl.ds((n // 2) * HM, HM)
            cols = pl.ds((2 * jp + n % 2) * T, T)
            o_s[rows, cols] += c

        @pl.when(h == H - 1)
        def _():
            out_copy(jp).start()

    ss = {0: qk(0), 1: qk(1)}
    cs = {}
    for j in range(NT):
        if j + 2 < NT:
            ss[j + 2] = qk(j + 2)
        cs[j] = softmax_pv(j, ss.pop(j))
        if j >= 2 and j % 2 == 0:
            oproj(j // 2 - 1, cs.pop(j - 2), cs.pop(j - 1))
    oproj(NP - 1, cs.pop(NT - 2), cs.pop(NT - 1))

    @pl.when(h == H - 1)
    def _():
        for jp in range(NP):
            out_copy(jp).wait()


@jax.jit
def pallas_gated_mix__compressed_kv_cla__ssm_conv_s5__prompt_kernel(
    A_x: jax.Array,
    A_c_kv: jax.Array,
    A_w_q: jax.Array,
    A_w_uk: jax.Array,
    A_w_uv: jax.Array,
    A_w_o: jax.Array,
    B_x: jax.Array,
    B_Lambda_re: jax.Array,
    B_Lambda_im: jax.Array,
    B_B_re: jax.Array,
    B_B_im: jax.Array,
    B_C_re: jax.Array,
    B_C_im: jax.Array,
    B_log_dt: jax.Array,
    B_Dskip: jax.Array,
    gate_w: jax.Array,
):
    del B_x
    xT = jnp.transpose(A_x[0])
    woT = jnp.transpose(A_w_o, (0, 2, 1))
    ckv = A_c_kv[0]

    hbm = pl.BlockSpec(memory_space=pl.ANY)
    vmem = pltpu.VMEM
    outT = pl.pallas_call(
        _kernel,
        grid=(H,),
        in_specs=[hbm] * 15,
        out_specs=hbm,
        out_shape=jax.ShapeDtypeStruct((M, S), f32),
        scratch_shapes=[
            vmem((M, S), bf16),
            vmem((M,), bf16), vmem((M,), bf16), vmem((M,), bf16), vmem((M,), bf16), vmem((M,), bf16),
            vmem((2 * M, M), bf16),
            vmem((2, M, M), bf16),
            vmem((M // 2, 2 * M), u32),
            vmem((8, 8, 512), f32),
            vmem((2, M, 128), f32),
            vmem((S, 2 * M), f32),
            vmem((1, S), f32),
            vmem((S, DC), bf16),
            vmem((M, H, D), bf16),
            vmem((DC, H, D), bf16),
            vmem((DC, H, D), bf16),
            vmem((4, M * 4, 128), u32),
            vmem((4, DC * 4, 128), u32),
            vmem((4, DC * 4, 128), u32),
            vmem((7, S // 4, DC // 2), u32),
            vmem((7, HM // 2, S // 2), u32),
            vmem((H, 2, D // 2, S // 2), u32),
            vmem((H, M, D), bf16),
            vmem((S // 2, D), u32),
            vmem((D // 2, S), u32),
            vmem((M, S), f32),
            vmem((3, S, T), f32),
            pltpu.SemaphoreType.DMA((NSEM,)),
        ],
        compiler_params=pltpu.CompilerParams(
            dimension_semantics=("arbitrary",),
            vmem_limit_bytes=120 * 1024 * 1024,
        ),
    )(xT, B_B_re, B_B_im, B_C_re, B_C_im, B_Lambda_re, B_Lambda_im, B_log_dt,
      B_Dskip, gate_w, woT, ckv, A_w_q, A_w_uk, A_w_uv)
    return jnp.transpose(outT)[None]
```

```python
import jax
import jax.numpy as jnp
from jax import lax
import jax.experimental.pallas as pl
import jax.experimental.pallas.tpu as pltpu

S = 2048
M = 448
H = 16
D = 256
DC = 1024
T = 128
NT = S // T
NP = NT // 2
HD = D // 2
HM = M // 2
PA = 384
PB = M - PA
TA = 512
TC = 256
CS = DC // NP
LOG2E = 1.4426950408889634

f32 = jnp.float32
bf16 = jnp.bfloat16
u32 = jnp.uint32

SEM_VEC, SEM_B, SEM_X, SEM_WQ, SEM_C, SEM_SL, SEM_WO, SEM_OUT = 0, 1, 2, 6, 7, 8, 16, 17
NSEM = 18


def _dot(a, b, dims):
    return lax.dot_general(a, b, (dims, ((), ())), preferred_element_type=f32)


_NN = ((1,), (0,))
_NT = ((1,), (1,))
_TN = ((0,), (0,))
_TT = ((0,), (1,))


def _pk(x):
    return pltpu.bitcast(x, u32)


def _up(x):
    return pltpu.bitcast(x, bf16)


def _cmul(ar, ai, br, bi):
    return ar * br - ai * bi, ar * bi + ai * br


def _ds(lo, n, align):
    return pl.ds(lo if isinstance(lo, int) else pl.multiple_of(lo, align), n)


def _strassen_a(a11, a12, a21, a22):
    ops = [a11 + a22, a21 + a22, a11, a22, a11 + a12, a21 - a11, a12 - a22]
    return [o.astype(bf16) for o in ops]


def _strassen_b(b11, b12, b21, b22):
    ops = [b11 + b22, b11, b12 - b22, b21 - b11, b22, b11 + b12, b21 + b22]
    return [o.astype(bf16) for o in ops]


def _strassen_c(m):
    c11 = (m[0] + m[3]) + (m[6] - m[4])
    c12 = m[2] + m[4]
    c21 = m[1] + m[3]
    c22 = (m[0] - m[1]) + (m[2] + m[5])
    return c11, c12, c21, c22


def _stage(raw, stg, c0, nc):
    for ht in range(2):
        for dt in range(2):
            v = raw[pl.ds(c0, nc), ht * 8:(ht + 1) * 8, dt * 128:(dt + 1) * 128]
            stg[ht * 2 + dt, _ds(c0 * 4, nc * 4, 8), :] = _pk(v.reshape(nc * 8, 128))


def _pair_words(stg, pair, rows):
    ht = lax.shift_right_logical(pair, 2)
    return [stg[ht * 2 + dt, pl.ds(pair & 3, rows, stride=4), :] for dt in range(2)]


def _weight_ops(halves, rows):
    r = rows // 2
    return _strassen_b(halves[0][:r], halves[1][:r], halves[0][r:], halves[1][r:])


def _head_weight_ops(stg, h, rows):
    sh = (16 * (1 - (h & 1))).astype(u32)
    words = _pair_words(stg, lax.shift_right_logical(h, 1), rows)
    halves = [pltpu.bitcast((u << sh) & jnp.uint32(0xFFFF0000), f32) for u in words]
    return _weight_ops(halves, rows)


def _ssm_cmat(craw_s, coef_s, c_s):
    cr, ci = coef_s[0:1, :], coef_s[1:2, :]
    for r in range(0, M, 16):
        cp_re, cp_im = _cmul(craw_s[0, r:r + 16, :].astype(f32), craw_s[1, r:r + 16, :].astype(f32), cr, ci)
        c_s[r // 2:r // 2 + 8, :] = _pk(jnp.concatenate(
            [cp_re[:, :PA], -cp_im[:, :PA], cp_re[:, PA:], -cp_im[:, PA:]], axis=1).astype(bf16))


def _ssm_params(vec_s, coef_s, lam_s, col_s):
    row = lambda r: r[...].astype(f32).reshape(1, M)
    lre, lim, ldt, dsk, gw = [row(v) for v in vec_s]
    dt = jnp.exp(ldt).astype(bf16).astype(f32)
    mag = jnp.exp(dt * lre)
    ang = dt * lim
    lr, li = mag * jnp.cos(ang), mag * jnp.sin(ang)
    den = lre * lre + lim * lim
    nr = lr - 1.0
    coef_s[0:1, :] = 2.0 * ((nr * lre + li * lim) / den)
    coef_s[1:2, :] = 2.0 * ((li * lre - nr * lim) / den)

    er = jnp.concatenate([lr, lr[:, PA:]], axis=1)
    ei = jnp.concatenate([li, -li[:, PA:]], axis=1)
    pw = [(er, ei)]
    for _ in range(7):
        pw.append(_cmul(pw[-1][0], pw[-1][1], er, ei))
    sub = lax.broadcasted_iota(jnp.int32, (8, 512), 0)
    for n, d in enumerate((1, 2, 4)):
        lam_s[2 * n] = jnp.where(sub >= d, pw[d - 1][0], 0.0)
        lam_s[2 * n + 1] = jnp.where(sub >= d, pw[d - 1][1], 0.0)
    lcr = jnp.zeros((8, 512), f32)
    lci = jnp.zeros((8, 512), f32)
    for r in range(8):
        lcr = jnp.where(sub == r, pw[r][0], lcr)
        lci = jnp.where(sub == r, pw[r][1], lci)
    lam_s[6] = lcr
    lam_s[7] = lci

    def col(v):
        v = jnp.concatenate([v, jnp.zeros((1, 512 - M), f32)], axis=1)
        return jnp.broadcast_to(v, (128, 512)).T[:M]
    col_s[0] = col(dsk)
    col_s[1] = col(gw)


def _ssm_scan(u_s, t0, carry, lam_s, h_s):
    car, cai = carry
    out = []
    for b in range(TC // 8):
        u = u_s[_ds(t0 + b * 8, 8, 8), :]
        mixed = u[:, 2 * PA:]
        hr = jnp.concatenate([u[:, :PA], mixed], axis=1)
        hi = jnp.concatenate([u[:, PA:2 * PA], pltpu.roll(mixed, PB, 1)], axis=1)
        for n, d in enumerate((1, 2, 4)):
            sr, si = pltpu.roll(hr, d, 0), pltpu.roll(hi, d, 0)
            tr, ti = _cmul(sr, si, lam_s[2 * n], lam_s[2 * n + 1])
            hr, hi = hr + tr, hi + ti
        tr, ti = _cmul(lam_s[6], lam_s[7], car, cai)
        hr, hi = hr + tr, hi + ti
        car, cai = hr[7:8, :], hi[7:8, :]
        out.append(jnp.concatenate([hr[:, :PA], hi[:, :PA], hr[:, PA:]], axis=1))
        if b % 2 == 1:
            h_s[(b // 2) * 8:(b // 2 + 1) * 8, :] = _pk(jnp.concatenate(out, axis=0).astype(bf16))
            out = []
    return car, cai


def _kernel(xT_hbm, bre_hbm, bim_hbm, cre_hbm, cim_hbm, lre_hbm, lim_hbm, ldt_hbm,
            dsk_hbm, gw_hbm, woT_hbm, ckv_hbm, wq_hbm, wk_hbm, wv_hbm,
            out_hbm,
            xT_s, v0, v1, v2, v3, v4, b_s, craw_s, c_s, coef_s, lam_s, col_s, u_s, g_s,
            ckv_s, rq, rk, rv, sq, sk, sv, a_s, xa_s, q_s, wo_s,
            k_s, vT_s, o_s, s_s, h_s, sem):
    h = pl.program_id(0)
    vec_s = (v0, v1, v2, v3, v4)

    def slice_copies(i):
        s = sem.at[SEM_SL + i]
        rows = _ds(i * 2 * T, 2 * T, 2 * T)
        cs = pl.ds(i * CS, CS)
        return [pltpu.make_async_copy(ckv_hbm.at[rows], ckv_s.at[rows], s),
                pltpu.make_async_copy(wk_hbm.at[cs], rk.at[cs], s),
                pltpu.make_async_copy(wv_hbm.at[cs], rv.at[cs], s)]

    def x_copy(i):
        cols = _ds(i * TA, TA, TA)
        return pltpu.make_async_copy(xT_hbm.at[:, cols], xT_s.at[:, cols], sem.at[SEM_X + i])

    def out_copy(jp):
        cols = pl.ds(jp * 2 * T, 2 * T)
        return pltpu.make_async_copy(o_s.at[:, cols], out_hbm.at[:, cols], sem.at[SEM_OUT])

    @pl.when(h == 0)
    def _():
        cp_vec = [pltpu.make_async_copy(src, dst, sem.at[SEM_VEC])
                  for src, dst in zip((lre_hbm, lim_hbm, ldt_hbm, dsk_hbm, gw_hbm), vec_s)]
        cp_b = [pltpu.make_async_copy(src.at[pl.ds(lo, n)], b_s.at[pl.ds(dst, n)], sem.at[SEM_B])
                for src, lo, n, dst in ((bre_hbm, 0, PA, 0), (bim_hbm, 0, PA, PA),
                                        (bre_hbm, PA, PB, 2 * PA), (bim_hbm, PA, PB, 2 * PA + PB))]
        cp_wq = [pltpu.make_async_copy(wq_hbm, rq, sem.at[SEM_WQ])]
        cp_c = [pltpu.make_async_copy(src, craw_s.at[n], sem.at[SEM_C])
                for n, src in enumerate((cre_hbm, cim_hbm))]
        cp_wo = pltpu.make_async_copy(woT_hbm, wo_s, sem.at[SEM_WO])
        for cp in cp_vec + cp_b:
            cp.start()
        for i in range(S // TA):
            x_copy(i).start()
        for cp in cp_wq + cp_c:
            cp.start()
        for i in range(NP):
            for cp in slice_copies(i):
                cp.start()
        cp_wo.start()

        def phase1(i):
            x_copy(i).wait()
            u_s[_ds(i * TA, TA, TA), :] = _dot(xT_s[:, _ds(i * TA, TA, TA)], b_s[...], _TT)
            for t in range(TA // (2 * T)):
                ev = _ds(i * TA + 2 * t * T, T, T)
                od = _ds(i * TA + (2 * t + 1) * T, T, T)
                for r in range(0, HM, 32):
                    top, bot = pl.ds(r, 32), pl.ds(HM + r, 32)
                    ops = _strassen_a(xT_s[top, ev].astype(f32), xT_s[bot, ev].astype(f32),
                                      xT_s[top, od].astype(f32), xT_s[bot, od].astype(f32))
                    for n in range(7):
                        xa_s[n, r // 2:r // 2 + 16, _ds(i * (TA // 2) + t * T, T, T)] = _pk(ops[n])

        for cp in cp_vec:
            cp.wait()
        _ssm_params(vec_s, coef_s, lam_s, col_s)
        for cp in cp_b:
            cp.wait()

        def phase1_body(i, carry):
            phase1(i)
            return carry
        lax.fori_loop(0, S // TA - 1, phase1_body, 0)
        for cp in cp_wq + cp_c:
            cp.wait()
        phase1(S // TA - 1)
        _stage(rq, sq, 0, M)
        _ssm_cmat(craw_s, coef_s, c_s)
        zero = jnp.zeros((1, 512), f32)
        carry0 = _ssm_scan(u_s, 0, (zero, zero), lam_s, h_s)

        def phase2(i, carry):
            for cp in slice_copies(i):
                cp.wait()
            yT = _dot(_up(c_s[...]), _up(h_s[...]), _NT)
            for t in range(TC // T):
                cols = _ds(i * TC + t * T, T, T)
                acc = jnp.zeros((8, T), f32)
                for r in range(0, M, 32):
                    xg = xT_s[r:r + 32, cols].astype(f32) * col_s[1, r:r + 32, :]
                    acc = acc + jnp.sum(xg.reshape(4, 8, T), axis=0)
                g = jax.nn.sigmoid(jnp.sum(acc, axis=0, keepdims=True))
                g_s[:, cols] = g
                for r in range(0, M, 32):
                    skip = xT_s[r:r + 32, cols].astype(f32) * col_s[0, r:r + 32, :]
                    o_s[r:r + 32, cols] = (1.0 - g) * (yT[r:r + 32, t * T:(t + 1) * T] + skip)

            words = _pair_words(sq, i, M)
            lo = _weight_ops([pltpu.bitcast(u << 16, f32) for u in words], M)
            hi = _weight_ops([pltpu.bitcast(u & jnp.uint32(0xFFFF0000), f32) for u in words], M)
            prods = [_dot(jnp.concatenate([lo[n], hi[n]], axis=1), _up(xa_s[n]), _TN) for n in range(7)]
            qs = LOG2E * D ** -0.5
            for n, c in enumerate(_strassen_c(prods)):
                c = c * qs
                rows = pl.ds((n % 2) * (HD // 2), HD // 2)
                q_s[2 * i, n // 2, rows, :] = _pk(c[:HD].astype(bf16))
                q_s[2 * i + 1, n // 2, rows, :] = _pk(c[HD:].astype(bf16))

            carry = _ssm_scan(u_s, jnp.minimum(i + 1, NP - 1) * TC, carry, lam_s, h_s)

            _stage(rk, sk, i * CS, CS)
            _stage(rv, sv, i * CS, CS)
            hc = DC // 2
            for r in range(0, T, 16):
                ev = _ds(i * 2 * T + r, 16, 16)
                od = _ds(i * 2 * T + T + r, 16, 16)
                for c0 in range(0, hc, 256):
                    lf, rt = pl.ds(c0, 256), pl.ds(hc + c0, 256)
                    ops = _strassen_a(ckv_s[ev, lf].astype(f32), ckv_s[ev, rt].astype(f32),
                                      ckv_s[od, lf].astype(f32), ckv_s[od, rt].astype(f32))
                    for n in range(7):
                        a_s[n, _ds(i * (T // 2) + r // 2, 8, 8), lf] = _pk(ops[n])
            return carry

        lax.fori_loop(0, NP, phase2, carry0)
        cp_wo.wait()

    wk = _head_weight_ops(sk, h, DC)
    for n, c in enumerate(_strassen_c([_dot(_up(a_s[i]), wk[i], _NN) for i in range(7)])):
        for t in range(NP):
            k_s[pl.ds((2 * t + n // 2) * (T // 2), T // 2), pl.ds((n % 2) * HD, HD)] = (
                _pk(c[t * T:(t + 1) * T].astype(bf16)))

    wv = _head_weight_ops(sv, h, DC)
    for n, c in enumerate(_strassen_c([_dot(wv[i], _up(a_s[i]), _TT) for i in range(7)])):
        for t in range(NP):
            vT_s[pl.ds((n % 2) * (HD // 2), HD // 2), pl.ds((2 * t + n // 2) * T, T)] = (
                _pk(c[:, t * T:(t + 1) * T].astype(bf16)))

    wo = wo_s[h].astype(f32)
    wo = _strassen_a(wo[:HM, :HD], wo[:HM, HD:], wo[HM:, :HD], wo[HM:, HD:])

    key = lax.broadcasted_iota(jnp.int32, (T, T), 0)
    qry = lax.broadcasted_iota(jnp.int32, (T, T), 1)
    causal = key <= qry

    def qk(j):
        kv = (j + 1) * T
        qT = _up(q_s[h, j % 2, :, pl.ds((j // 2) * T, T)])
        s = _dot(_up(k_s[0:kv // 2, :]), qT, _NN)
        sd = jnp.where(causal, s[kv - T:kv], -1e30)
        s = jnp.concatenate([s[:kv - T], sd], axis=0) if j > 0 else sd
        s_s[j % 3, 0:kv, :] = s
        parts = [jnp.max(s[a:min(a + 512, kv)], axis=0, keepdims=True) for a in range(0, kv, 512)]
        m = parts[0]
        for part in parts[1:]:
            m = jnp.maximum(m, part)
        return m

    def softmax_pv(j, m):
        kv = (j + 1) * T
        p = jnp.exp2(s_s[j % 3, 0:kv, :] - m)
        l = jnp.sum(p, axis=0, keepdims=True)
        c = _dot(_up(vT_s[:, 0:kv]), p.astype(bf16), _NN)
        return c * (g_s[:, j * T:(j + 1) * T] / l)

    def oproj(jp, ce, co):
        ops = _strassen_b(ce[:HD], co[:HD], ce[HD:], co[HD:])
        for n, c in enumerate(_strassen_c([_dot(wo[i], ops[i], _NN) for i in range(7)])):
            rows = pl.ds((n // 2) * HM, HM)
            cols = pl.ds((2 * jp + n % 2) * T, T)
            o_s[rows, cols] += c

        @pl.when(h == H - 1)
        def _():
            out_copy(jp).start()

    ss = {0: qk(0), 1: qk(1)}
    cs = {}
    for j in range(NT):
        if j + 2 < NT:
            ss[j + 2] = qk(j + 2)
        cs[j] = softmax_pv(j, ss.pop(j))
        if j >= 2 and j % 2 == 0:
            oproj(j // 2 - 1, cs.pop(j - 2), cs.pop(j - 1))
    oproj(NP - 1, cs.pop(NT - 2), cs.pop(NT - 1))

    @pl.when(h == H - 1)
    def _():
        for jp in range(NP):
            out_copy(jp).wait()


@jax.jit
def pallas_gated_mix__compressed_kv_cla__ssm_conv_s5__prompt_kernel(
    A_x: jax.Array,
    A_c_kv: jax.Array,
    A_w_q: jax.Array,
    A_w_uk: jax.Array,
    A_w_uv: jax.Array,
    A_w_o: jax.Array,
    B_x: jax.Array,
    B_Lambda_re: jax.Array,
    B_Lambda_im: jax.Array,
    B_B_re: jax.Array,
    B_B_im: jax.Array,
    B_C_re: jax.Array,
    B_C_im: jax.Array,
    B_log_dt: jax.Array,
    B_Dskip: jax.Array,
    gate_w: jax.Array,
):
    del B_x
    xT = jnp.transpose(A_x[0])
    woT = jnp.transpose(A_w_o, (0, 2, 1))
    ckv = A_c_kv[0]

    hbm = pl.BlockSpec(memory_space=pl.ANY)
    vmem = pltpu.VMEM
    outT = pl.pallas_call(
        _kernel,
        grid=(H,),
        in_specs=[hbm] * 15,
        out_specs=hbm,
        out_shape=jax.ShapeDtypeStruct((M, S), f32),
        scratch_shapes=[
            vmem((M, S), bf16),
            vmem((M,), bf16), vmem((M,), bf16), vmem((M,), bf16), vmem((M,), bf16), vmem((M,), bf16),
            vmem((2 * M, M), bf16),
            vmem((2, M, M), bf16),
            vmem((M // 2, 2 * M), u32),
            vmem((2, M), f32),
            vmem((8, 8, 512), f32),
            vmem((2, M, 128), f32),
            vmem((S, 2 * M), f32),
            vmem((1, S), f32),
            vmem((S, DC), bf16),
            vmem((M, H, D), bf16),
            vmem((DC, H, D), bf16),
            vmem((DC, H, D), bf16),
            vmem((4, M * 4, 128), u32),
            vmem((4, DC * 4, 128), u32),
            vmem((4, DC * 4, 128), u32),
            vmem((7, S // 4, DC // 2), u32),
            vmem((7, HM // 2, S // 2), u32),
            vmem((H, 2, D // 2, S // 2), u32),
            vmem((H, M, D), bf16),
            vmem((S // 2, D), u32),
            vmem((D // 2, S), u32),
            vmem((M, S), f32),
            vmem((3, S, T), f32),
            vmem((TC // 2, 2 * M), u32),
            pltpu.SemaphoreType.DMA((NSEM,)),
        ],
        compiler_params=pltpu.CompilerParams(
            dimension_semantics=("arbitrary",),
            vmem_limit_bytes=120 * 1024 * 1024,
        ),
    )(xT, B_B_re, B_B_im, B_C_re, B_C_im, B_Lambda_re, B_Lambda_im, B_log_dt,
      B_Dskip, gate_w, woT, ckv, A_w_q, A_w_uk, A_w_uv)
    return jnp.transpose(outT)[None]
```

```python
import jax
import jax.numpy as jnp
from jax import lax
import jax.experimental.pallas as pl
import jax.experimental.pallas.tpu as pltpu

S = 2048
M = 448
H = 16
D = 256
DC = 1024
T = 128
NT = S // T
NP = NT // 2
HD = D // 2
HM = M // 2
PA = 384
PB = M - PA
TA = 512
TC = 256
CS = DC // NP
LOG2E = 1.4426950408889634

f32 = jnp.float32
bf16 = jnp.bfloat16
u32 = jnp.uint32

SEM_VEC, SEM_B, SEM_X, SEM_WQ, SEM_C, SEM_SL, SEM_WO, SEM_OUT = 0, 1, 2, 6, 7, 8, 16, 17
NSEM = 18


def _dot(a, b, dims):
    return lax.dot_general(a, b, (dims, ((), ())), preferred_element_type=f32)


_NN = ((1,), (0,))
_NT = ((1,), (1,))
_TN = ((0,), (0,))
_TT = ((0,), (1,))


def _pk(x):
    return pltpu.bitcast(x, u32)


def _up(x):
    return pltpu.bitcast(x, bf16)


def _tie(x, clock):
    if clock is None:
        return x
    never, tick = clock
    r, c = x.shape
    if tick.dtype != x.dtype:
        tick = pltpu.bitcast(tick, x.dtype)
    tile = lambda v: jnp.tile(v, (r // 8, c // 128))
    return jnp.where(tile(never), tile(tick), x)


def _cmul(ar, ai, br, bi):
    return ar * br - ai * bi, ar * bi + ai * br


def _ds(lo, n, align):
    return pl.ds(lo if isinstance(lo, int) else pl.multiple_of(lo, align), n)


def _strassen_a(a11, a12, a21, a22):
    ops = [a11 + a22, a21 + a22, a11, a22, a11 + a12, a21 - a11, a12 - a22]
    return [o.astype(bf16) for o in ops]


def _strassen_b(b11, b12, b21, b22):
    ops = [b11 + b22, b11, b12 - b22, b21 - b11, b22, b11 + b12, b21 + b22]
    return [o.astype(bf16) for o in ops]


def _strassen_c(m):
    c11 = (m[0] + m[3]) + (m[6] - m[4])
    c12 = m[2] + m[4]
    c21 = m[1] + m[3]
    c22 = (m[0] - m[1]) + (m[2] + m[5])
    return c11, c12, c21, c22


def _stage(raw, stg, c0, nc, clock=None):
    for ht in range(2):
        for dt in range(2):
            v = raw[pl.ds(c0, nc), ht * 8:(ht + 1) * 8, dt * 128:(dt + 1) * 128]
            stg[ht * 2 + dt, _ds(c0 * 4, nc * 4, 8), :] = _tie(_pk(v.reshape(nc * 8, 128)), clock)


def _pair_words(stg, pair, rows):
    ht = lax.shift_right_logical(pair, 2)
    return [stg[ht * 2 + dt, pl.ds(pair & 3, rows, stride=4), :] for dt in range(2)]


def _weight_ops(halves, rows):
    r = rows // 2
    return _strassen_b(halves[0][:r], halves[1][:r], halves[0][r:], halves[1][r:])


def _head_weight_ops(stg, h, rows):
    sh = (16 * (1 - (h & 1))).astype(u32)
    words = _pair_words(stg, lax.shift_right_logical(h, 1), rows)
    halves = [pltpu.bitcast((u << sh) & jnp.uint32(0xFFFF0000), f32) for u in words]
    return _weight_ops(halves, rows)


def _ssm_cmat(craw_s, coef_s, c_s, clocks):
    for r in range(0, M, 16):
        coef = _tie(coef_s[...], clocks(r // 16, M // 16))
        cr, ci = coef[0:1, :M], coef[1:2, :M]
        cp_re, cp_im = _cmul(craw_s[0, r:r + 16, :].astype(f32), craw_s[1, r:r + 16, :].astype(f32), cr, ci)
        c_s[r // 2:r // 2 + 8, :] = _pk(jnp.concatenate(
            [cp_re[:, :PA], -cp_im[:, :PA], cp_re[:, PA:], -cp_im[:, PA:]], axis=1).astype(bf16))


def _ssm_params(vec_s, coef_s, lam_s, col_s, zero_s):
    row = lambda r: r[...].astype(f32).reshape(1, M)
    lre, lim, ldt, dsk, gw = [row(v) for v in vec_s]
    dt = jnp.exp(ldt).astype(bf16).astype(f32)
    mag = jnp.exp(dt * lre)
    ang = dt * lim
    lr, li = mag * jnp.cos(ang), mag * jnp.sin(ang)
    den = lre * lre + lim * lim
    nr = lr - 1.0
    coef_s[...] = jnp.zeros(coef_s.shape, f32)
    coef_s[0:1, 0:M] = 2.0 * ((nr * lre + li * lim) / den)
    coef_s[1:2, 0:M] = 2.0 * ((li * lre - nr * lim) / den)
    zero_s[...] = jnp.zeros(zero_s.shape, f32)

    er = jnp.concatenate([lr, lr[:, PA:]], axis=1)
    ei = jnp.concatenate([li, -li[:, PA:]], axis=1)
    pw = [(er, ei)]
    for _ in range(7):
        pw.append(_cmul(pw[-1][0], pw[-1][1], er, ei))
    sub = lax.broadcasted_iota(jnp.int32, (8, 512), 0)
    for n, d in enumerate((1, 2, 4)):
        lam_s[2 * n] = jnp.where(sub >= d, pw[d - 1][0], 0.0)
        lam_s[2 * n + 1] = jnp.where(sub >= d, pw[d - 1][1], 0.0)
    lcr = jnp.zeros((8, 512), f32)
    lci = jnp.zeros((8, 512), f32)
    for r in range(8):
        lcr = jnp.where(sub == r, pw[r][0], lcr)
        lci = jnp.where(sub == r, pw[r][1], lci)
    lam_s[6] = lcr
    lam_s[7] = lci

    def col(v):
        v = jnp.concatenate([v, jnp.zeros((1, 512 - M), f32)], axis=1)
        return jnp.broadcast_to(v, (128, 512)).T[:M]
    col_s[0] = col(dsk)
    col_s[1] = col(gw)


def _ssm_scan(u_s, t0, carry, lam_s, h_s, clocks):
    car, cai = carry
    out = []
    for b in range(TC // 8):
        u = u_s[_ds(t0 + b * 8, 8, 8), :]
        mixed = u[:, 2 * PA:]
        hr = _tie(jnp.concatenate([u[:, :PA], mixed], axis=1), clocks(b, TC // 8))
        hi = jnp.concatenate([u[:, PA:2 * PA], pltpu.roll(mixed, PB, 1)], axis=1)
        for n, d in enumerate((1, 2, 4)):
            sr, si = pltpu.roll(hr, d, 0), pltpu.roll(hi, d, 0)
            tr, ti = _cmul(sr, si, lam_s[2 * n], lam_s[2 * n + 1])
            hr, hi = hr + tr, hi + ti
        tr, ti = _cmul(lam_s[6], lam_s[7], car, cai)
        hr, hi = hr + tr, hi + ti
        car, cai = hr[7:8, :], hi[7:8, :]
        out.append(jnp.concatenate([hr[:, :PA], hi[:, :PA], hr[:, PA:]], axis=1))
        if b % 2 == 1:
            h_s[(b // 2) * 8:(b // 2 + 1) * 8, :] = _pk(jnp.concatenate(out, axis=0).astype(bf16))
            out = []
    return car, cai


def _kernel(xT_hbm, bre_hbm, bim_hbm, cre_hbm, cim_hbm, lre_hbm, lim_hbm, ldt_hbm,
            dsk_hbm, gw_hbm, woT_hbm, ckv_hbm, wq_hbm, wk_hbm, wv_hbm,
            out_hbm,
            xT_s, v0, v1, v2, v3, v4, b_s, craw_s, c_s, coef_s, lam_s, col_s, u_s, g_s,
            ckv_s, rq, rk, rv, sq, sk, sv, a_s, xa_s, q_s, wo_s,
            k_s, vT_s, o_s, s_s, h_s, zero_s, sem):
    h = pl.program_id(0)
    vec_s = (v0, v1, v2, v3, v4)

    def slice_copies(i):
        s = sem.at[SEM_SL + i]
        rows = _ds(i * 2 * T, 2 * T, 2 * T)
        cs = pl.ds(i * CS, CS)
        return [pltpu.make_async_copy(ckv_hbm.at[rows], ckv_s.at[rows], s),
                pltpu.make_async_copy(wk_hbm.at[cs], rk.at[cs], s),
                pltpu.make_async_copy(wv_hbm.at[cs], rv.at[cs], s)]

    def x_copy(i):
        cols = _ds(i * TA, TA, TA)
        return pltpu.make_async_copy(xT_hbm.at[:, cols], xT_s.at[:, cols], sem.at[SEM_X + i])

    def out_copy(jp):
        cols = pl.ds(jp * 2 * T, 2 * T)
        return pltpu.make_async_copy(o_s.at[:, cols], out_hbm.at[:, cols], sem.at[SEM_OUT])

    @pl.when(h == 0)
    def _():
        cp_vec = [pltpu.make_async_copy(src, dst, sem.at[SEM_VEC])
                  for src, dst in zip((lre_hbm, lim_hbm, ldt_hbm, dsk_hbm, gw_hbm), vec_s)]
        cp_b = [pltpu.make_async_copy(src.at[pl.ds(lo, n)], b_s.at[pl.ds(dst, n)], sem.at[SEM_B])
                for src, lo, n, dst in ((bre_hbm, 0, PA, 0), (bim_hbm, 0, PA, PA),
                                        (bre_hbm, PA, PB, 2 * PA), (bim_hbm, PA, PB, 2 * PA + PB))]
        cp_wq = [pltpu.make_async_copy(wq_hbm, rq, sem.at[SEM_WQ])]
        cp_c = [pltpu.make_async_copy(src, craw_s.at[n], sem.at[SEM_C])
                for n, src in enumerate((cre_hbm, cim_hbm))]
        cp_wo = pltpu.make_async_copy(woT_hbm, wo_s, sem.at[SEM_WO])
        for cp in cp_vec + cp_b:
            cp.start()
        for i in range(S // TA):
            x_copy(i).start()
        for cp in cp_wq + cp_c:
            cp.start()
        for i in range(NP):
            for cp in slice_copies(i):
                cp.start()
        cp_wo.start()

        def phase1(i):
            x_copy(i).wait()
            u = _dot(xT_s[:, _ds(i * TA, TA, TA)], b_s[...], _TT)
            u_s[_ds(i * TA, TA, TA), :] = u
            never = zero_s[...] != 0.0

            def clocks(k, n):
                pos = (k * 6 * TA // n) // 8 * 8
                return never, u[pos % TA:pos % TA + 8, (pos // TA) * 128:(pos // TA + 1) * 128]

            for t in range(TA // (2 * T)):
                ev = _ds(i * TA + 2 * t * T, T, T)
                od = _ds(i * TA + (2 * t + 1) * T, T, T)
                for r in range(0, HM, 32):
                    top, bot = pl.ds(r, 32), pl.ds(HM + r, 32)
                    clk = clocks(t * 7 + r // 32, 14)
                    ops = _strassen_a(_tie(xT_s[top, ev].astype(f32), clk), xT_s[bot, ev].astype(f32),
                                      xT_s[top, od].astype(f32), _tie(xT_s[bot, od].astype(f32), clk))
                    for n in range(7):
                        xa_s[n, r // 2:r // 2 + 16, _ds(i * (TA // 2) + t * T, T, T)] = _pk(ops[n])
            return clocks

        for cp in cp_vec:
            cp.wait()
        _ssm_params(vec_s, coef_s, lam_s, col_s, zero_s)
        for cp in cp_b:
            cp.wait()

        def phase1_body(i, carry):
            phase1(i)
            return carry
        lax.fori_loop(0, S // TA - 1, phase1_body, 0)
        for cp in cp_wq + cp_c:
            cp.wait()
        clocks = phase1(S // TA - 1)
        for c0 in range(0, M, 8):
            _stage(rq, sq, c0, 8, clocks(c0 // 8, M // 8))
        _ssm_cmat(craw_s, coef_s, c_s, clocks)
        zero = jnp.zeros((1, 512), f32)
        carry0 = _ssm_scan(u_s, 0, (zero, zero), lam_s, h_s, clocks)

        def phase2(i, carry):
            for cp in slice_copies(i):
                cp.wait()
            yT = _dot(_up(c_s[...]), _up(h_s[...]), _NT)
            for t in range(TC // T):
                cols = _ds(i * TC + t * T, T, T)
                acc = jnp.zeros((8, T), f32)
                for r in range(0, M, 32):
                    xg = xT_s[r:r + 32, cols].astype(f32) * col_s[1, r:r + 32, :]
                    acc = acc + jnp.sum(xg.reshape(4, 8, T), axis=0)
                g = jax.nn.sigmoid(jnp.sum(acc, axis=0, keepdims=True))
                g_s[:, cols] = g
                for r in range(0, M, 32):
                    skip = xT_s[r:r + 32, cols].astype(f32) * col_s[0, r:r + 32, :]
                    o_s[r:r + 32, cols] = (1.0 - g) * (yT[r:r + 32, t * T:(t + 1) * T] + skip)

            words = _pair_words(sq, i, M)
            lo = _weight_ops([pltpu.bitcast(u << 16, f32) for u in words], M)
            hi = _weight_ops([pltpu.bitcast(u & jnp.uint32(0xFFFF0000), f32) for u in words], M)
            prods = [_dot(jnp.concatenate([lo[n], hi[n]], axis=1), _up(xa_s[n]), _TN) for n in range(7)]
            qs = LOG2E * D ** -0.5
            for n, c in enumerate(_strassen_c(prods)):
                c = c * qs
                rows = pl.ds((n % 2) * (HD // 2), HD // 2)
                q_s[2 * i, n // 2, rows, :] = _pk(c[:HD].astype(bf16))
                q_s[2 * i + 1, n // 2, rows, :] = _pk(c[HD:].astype(bf16))

            never = zero_s[...] != 0.0

            def clocks(k, n):
                pos = (k * 5 * 1024 // n) // 8 * 8
                r, c = pos % 256, (pos % 1024) // 256 * 256
                return never, prods[pos // 1024][r:r + 8, c:c + 128]

            carry = _ssm_scan(u_s, jnp.minimum(i + 1, NP - 1) * TC, carry, lam_s, h_s, clocks)

            for c0 in range(0, CS, 8):
                _stage(rk, sk, i * CS + c0, 8, clocks(c0 // 4, CS // 4))
                _stage(rv, sv, i * CS + c0, 8, clocks(c0 // 4 + 1, CS // 4))
            hc = DC // 2
            for r in range(0, T, 16):
                ev = _ds(i * 2 * T + r, 16, 16)
                od = _ds(i * 2 * T + T + r, 16, 16)
                for c0 in range(0, hc, 256):
                    lf, rt = pl.ds(c0, 256), pl.ds(hc + c0, 256)
                    clk = clocks(r // 8 + c0 // 256, T // 8)
                    ops = _strassen_a(_tie(ckv_s[ev, lf].astype(f32), clk), ckv_s[ev, rt].astype(f32),
                                      ckv_s[od, lf].astype(f32), _tie(ckv_s[od, rt].astype(f32), clk))
                    for n in range(7):
                        a_s[n, _ds(i * (T // 2) + r // 2, 8, 8), lf] = _pk(ops[n])
            return carry

        lax.fori_loop(0, NP, phase2, carry0)
        cp_wo.wait()

    wk = _head_weight_ops(sk, h, DC)
    for n, c in enumerate(_strassen_c([_dot(_up(a_s[i]), wk[i], _NN) for i in range(7)])):
        for t in range(NP):
            k_s[pl.ds((2 * t + n // 2) * (T // 2), T // 2), pl.ds((n % 2) * HD, HD)] = (
                _pk(c[t * T:(t + 1) * T].astype(bf16)))

    wv = _head_weight_ops(sv, h, DC)
    for n, c in enumerate(_strassen_c([_dot(wv[i], _up(a_s[i]), _TT) for i in range(7)])):
        for t in range(NP):
            vT_s[pl.ds((n % 2) * (HD // 2), HD // 2), pl.ds((2 * t + n // 2) * T, T)] = (
                _pk(c[:, t * T:(t + 1) * T].astype(bf16)))

    wo = wo_s[h].astype(f32)
    wo = _strassen_a(wo[:HM, :HD], wo[:HM, HD:], wo[HM:, :HD], wo[HM:, HD:])

    key = lax.broadcasted_iota(jnp.int32, (T, T), 0)
    qry = lax.broadcasted_iota(jnp.int32, (T, T), 1)
    causal = key <= qry

    def qk(j):
        kv = (j + 1) * T
        qT = _up(q_s[h, j % 2, :, pl.ds((j // 2) * T, T)])
        s = _dot(_up(k_s[0:kv // 2, :]), qT, _NN)
        sd = jnp.where(causal, s[kv - T:kv], -1e30)
        s = jnp.concatenate([s[:kv - T], sd], axis=0) if j > 0 else sd
        s_s[j % 3, 0:kv, :] = s
        parts = [jnp.max(s[a:min(a + 512, kv)], axis=0, keepdims=True) for a in range(0, kv, 512)]
        m = parts[0]
        for part in parts[1:]:
            m = jnp.maximum(m, part)
        return m

    def softmax_pv(j, m):
        kv = (j + 1) * T
        p = jnp.exp2(s_s[j % 3, 0:kv, :] - m)
        l = jnp.sum(p, axis=0, keepdims=True)
        c = _dot(_up(vT_s[:, 0:kv]), p.astype(bf16), _NN)
        return c * (g_s[:, j * T:(j + 1) * T] / l)

    def oproj(jp, ce, co):
        ops = _strassen_b(ce[:HD], co[:HD], ce[HD:], co[HD:])
        for n, c in enumerate(_strassen_c([_dot(wo[i], ops[i], _NN) for i in range(7)])):
            rows = pl.ds((n // 2) * HM, HM)
            cols = pl.ds((2 * jp + n % 2) * T, T)
            o_s[rows, cols] += c

        @pl.when(h == H - 1)
        def _():
            out_copy(jp).start()

    ss = {0: qk(0), 1: qk(1)}
    cs = {}
    for j in range(NT):
        if j + 2 < NT:
            ss[j + 2] = qk(j + 2)
        cs[j] = softmax_pv(j, ss.pop(j))
        if j >= 2 and j % 2 == 0:
            oproj(j // 2 - 1, cs.pop(j - 2), cs.pop(j - 1))
    oproj(NP - 1, cs.pop(NT - 2), cs.pop(NT - 1))

    @pl.when(h == H - 1)
    def _():
        for jp in range(NP):
            out_copy(jp).wait()


@jax.jit
def pallas_gated_mix__compressed_kv_cla__ssm_conv_s5__prompt_kernel(
    A_x: jax.Array,
    A_c_kv: jax.Array,
    A_w_q: jax.Array,
    A_w_uk: jax.Array,
    A_w_uv: jax.Array,
    A_w_o: jax.Array,
    B_x: jax.Array,
    B_Lambda_re: jax.Array,
    B_Lambda_im: jax.Array,
    B_B_re: jax.Array,
    B_B_im: jax.Array,
    B_C_re: jax.Array,
    B_C_im: jax.Array,
    B_log_dt: jax.Array,
    B_Dskip: jax.Array,
    gate_w: jax.Array,
):
    del B_x
    xT = jnp.transpose(A_x[0])
    woT = jnp.transpose(A_w_o, (0, 2, 1))
    ckv = A_c_kv[0]

    hbm = pl.BlockSpec(memory_space=pl.ANY)
    vmem = pltpu.VMEM
    outT = pl.pallas_call(
        _kernel,
        grid=(H,),
        in_specs=[hbm] * 15,
        out_specs=hbm,
        out_shape=jax.ShapeDtypeStruct((M, S), f32),
        scratch_shapes=[
            vmem((M, S), bf16),
            vmem((M,), bf16), vmem((M,), bf16), vmem((M,), bf16), vmem((M,), bf16), vmem((M,), bf16),
            vmem((2 * M, M), bf16),
            vmem((2, M, M), bf16),
            vmem((M // 2, 2 * M), u32),
            vmem((8, 512), f32),
            vmem((8, 8, 512), f32),
            vmem((2, M, 128), f32),
            vmem((S, 2 * M), f32),
            vmem((1, S), f32),
            vmem((S, DC), bf16),
            vmem((M, H, D), bf16),
            vmem((DC, H, D), bf16),
            vmem((DC, H, D), bf16),
            vmem((4, M * 4, 128), u32),
            vmem((4, DC * 4, 128), u32),
            vmem((4, DC * 4, 128), u32),
            vmem((7, S // 4, DC // 2), u32),
            vmem((7, HM // 2, S // 2), u32),
            vmem((H, 2, D // 2, S // 2), u32),
            vmem((H, M, D), bf16),
            vmem((S // 2, D), u32),
            vmem((D // 2, S), u32),
            vmem((M, S), f32),
            vmem((3, S, T), f32),
            vmem((TC // 2, 2 * M), u32),
            vmem((8, 128), f32),
            pltpu.SemaphoreType.DMA((NSEM,)),
        ],
        compiler_params=pltpu.CompilerParams(
            dimension_semantics=("arbitrary",),
            vmem_limit_bytes=120 * 1024 * 1024,
        ),
    )(xT, B_B_re, B_B_im, B_C_re, B_C_im, B_Lambda_re, B_Lambda_im, B_log_dt,
      B_Dskip, gate_w, woT, ckv, A_w_q, A_w_uk, A_w_uv)
    return jnp.transpose(outT)[None]
```

```python
import jax
import jax.numpy as jnp
from jax import lax
import jax.experimental.pallas as pl
import jax.experimental.pallas.tpu as pltpu

S = 2048
M = 448
H = 16
D = 256
DC = 1024
T = 128
NT = S // T
NP = NT // 2
HD = D // 2
HM = M // 2
PA = 384
PB = M - PA
TA = 512
TC = 256
CS = DC // NP
import os
LCH = int(os.environ.get('LCH', 512))
LOG2E = 1.4426950408889634

f32 = jnp.float32
bf16 = jnp.bfloat16
u32 = jnp.uint32

SEM_VEC, SEM_B, SEM_X, SEM_WQ, SEM_C, SEM_SL, SEM_WO, SEM_OUT = 0, 1, 2, 6, 7, 8, 16, 17
NSEM = 18


def _dot(a, b, dims):
    return lax.dot_general(a, b, (dims, ((), ())), preferred_element_type=f32)


_NN = ((1,), (0,))
_NT = ((1,), (1,))
_TN = ((0,), (0,))
_TT = ((0,), (1,))


def _pk(x):
    return pltpu.bitcast(x, u32)


def _up(x):
    return pltpu.bitcast(x, bf16)


def _tie(x, clock):
    if clock is None:
        return x
    never, tick = clock
    r, c = x.shape
    if tick.dtype != x.dtype:
        tick = pltpu.bitcast(tick, x.dtype)
    tile = lambda v: jnp.tile(v, (r // 8, c // 128))
    return jnp.where(tile(never), tile(tick), x)


def _cmul(ar, ai, br, bi):
    return ar * br - ai * bi, ar * bi + ai * br


def _ds(lo, n, align):
    return pl.ds(lo if isinstance(lo, int) else pl.multiple_of(lo, align), n)


def _strassen_a(a11, a12, a21, a22):
    ops = [a11 + a22, a21 + a22, a11, a22, a11 + a12, a21 - a11, a12 - a22]
    return [o.astype(bf16) for o in ops]


def _strassen_b(b11, b12, b21, b22):
    ops = [b11 + b22, b11, b12 - b22, b21 - b11, b22, b11 + b12, b21 + b22]
    return [o.astype(bf16) for o in ops]


def _strassen_c(m):
    c11 = (m[0] + m[3]) + (m[6] - m[4])
    c12 = m[2] + m[4]
    c21 = m[1] + m[3]
    c22 = (m[0] - m[1]) + (m[2] + m[5])
    return c11, c12, c21, c22


def _stage(raw, stg, c0, nc, clock=None):
    for ht in range(2):
        for dt in range(2):
            v = raw[pl.ds(c0, nc), ht * 8:(ht + 1) * 8, dt * 128:(dt + 1) * 128]
            stg[ht * 2 + dt, _ds(c0 * 4, nc * 4, 8), :] = _tie(_pk(v.reshape(nc * 8, 128)), clock)


def _pair_words(stg, pair, rows):
    ht = lax.shift_right_logical(pair, 2)
    return [stg[ht * 2 + dt, pl.ds(pair & 3, rows, stride=4), :] for dt in range(2)]


def _weight_ops(halves, rows):
    r = rows // 2
    return _strassen_b(halves[0][:r], halves[1][:r], halves[0][r:], halves[1][r:])


def _head_weight_ops(stg, h, rows):
    sh = (16 * (1 - (h & 1))).astype(u32)
    words = _pair_words(stg, lax.shift_right_logical(h, 1), rows)
    halves = [pltpu.bitcast((u << sh) & jnp.uint32(0xFFFF0000), f32) for u in words]
    return _weight_ops(halves, rows)


def _ssm_cmat(craw_s, coef_s, c_s, clocks):
    for r in range(0, M, 16):
        coef = _tie(coef_s[...], clocks(r // 16, M // 16))
        cr, ci = coef[0:1, :M], coef[1:2, :M]
        cp_re, cp_im = _cmul(craw_s[0, r:r + 16, :].astype(f32), craw_s[1, r:r + 16, :].astype(f32), cr, ci)
        c_s[r // 2:r // 2 + 8, :] = _pk(jnp.concatenate(
            [cp_re[:, :PA], -cp_im[:, :PA], cp_re[:, PA:], -cp_im[:, PA:]], axis=1).astype(bf16))


def _ssm_params(vec_s, coef_s, lam_s, col_s, zero_s):
    row = lambda r: r[...].astype(f32).reshape(1, M)
    lre, lim, ldt, dsk, gw = [row(v) for v in vec_s]
    dt = jnp.exp(ldt).astype(bf16).astype(f32)
    mag = jnp.exp(dt * lre)
    ang = dt * lim
    lr, li = mag * jnp.cos(ang), mag * jnp.sin(ang)
    den = lre * lre + lim * lim
    nr = lr - 1.0
    coef_s[...] = jnp.zeros(coef_s.shape, f32)
    coef_s[0:1, 0:M] = 2.0 * ((nr * lre + li * lim) / den)
    coef_s[1:2, 0:M] = 2.0 * ((li * lre - nr * lim) / den)
    zero_s[...] = jnp.zeros(zero_s.shape, f32)

    er = jnp.concatenate([lr, lr[:, PA:]], axis=1)
    ei = jnp.concatenate([li, -li[:, PA:]], axis=1)
    pw = [(er, ei)]
    for _ in range(7):
        pw.append(_cmul(pw[-1][0], pw[-1][1], er, ei))
    sub = lax.broadcasted_iota(jnp.int32, (8, 512), 0)
    for n, d in enumerate((1, 2, 4)):
        lam_s[2 * n] = jnp.where(sub >= d, pw[d - 1][0], 0.0)
        lam_s[2 * n + 1] = jnp.where(sub >= d, pw[d - 1][1], 0.0)
    lcr = jnp.zeros((8, 512), f32)
    lci = jnp.zeros((8, 512), f32)
    for r in range(8):
        lcr = jnp.where(sub == r, pw[r][0], lcr)
        lci = jnp.where(sub == r, pw[r][1], lci)
    lam_s[6] = lcr
    lam_s[7] = lci

    def col(v):
        v = jnp.concatenate([v, jnp.zeros((1, 512 - M), f32)], axis=1)
        return jnp.broadcast_to(v, (128, 512)).T[:M]
    col_s[0] = col(dsk)
    col_s[1] = col(gw)


def _ssm_scan(u_s, t0, carry, lam_s, h_s, clocks):
    car, cai = carry
    out = []
    for b in range(TC // 8):
        u = u_s[_ds(t0 + b * 8, 8, 8), :]
        mixed = u[:, 2 * PA:]
        cols = [u[:, 0:128], u[:, 128:256], u[:, 256:384], mixed]
        hr = jnp.concatenate([_tie(v, clocks(4 * b + n, TC // 2)) for n, v in enumerate(cols)], axis=1)
        hi = jnp.concatenate([u[:, PA:2 * PA], pltpu.roll(mixed, PB, 1)], axis=1)
        for n, d in enumerate((1, 2, 4)):
            sr, si = pltpu.roll(hr, d, 0), pltpu.roll(hi, d, 0)
            tr, ti = _cmul(sr, si, lam_s[2 * n], lam_s[2 * n + 1])
            hr, hi = hr + tr, hi + ti
        tr, ti = _cmul(lam_s[6], lam_s[7], car, cai)
        hr, hi = hr + tr, hi + ti
        car, cai = hr[7:8, :], hi[7:8, :]
        out.append(jnp.concatenate([hr[:, :PA], hi[:, :PA], hr[:, PA:]], axis=1))
        if b % 2 == 1:
            h_s[(b // 2) * 8:(b // 2 + 1) * 8, :] = _pk(jnp.concatenate(out, axis=0).astype(bf16))
            out = []
    return car, cai


def _kernel(xT_hbm, bre_hbm, bim_hbm, cre_hbm, cim_hbm, lre_hbm, lim_hbm, ldt_hbm,
            dsk_hbm, gw_hbm, woT_hbm, ckv_hbm, wq_hbm, wk_hbm, wv_hbm,
            out_hbm,
            xT_s, v0, v1, v2, v3, v4, b_s, craw_s, c_s, coef_s, lam_s, col_s, u_s, g_s,
            ckv_s, rq, rk, rv, sq, sk, sv, a_s, xa_s, q_s, wo_s,
            k_s, vT_s, o_s, s_s, h_s, zero_s, wl_s, cl_s, sem):
    h = pl.program_id(0)
    vec_s = (v0, v1, v2, v3, v4)

    def slice_copies(i):
        s = sem.at[SEM_SL + i]
        rows = _ds(i * 2 * T, 2 * T, 2 * T)
        cs = pl.ds(i * CS, CS)
        return [pltpu.make_async_copy(ckv_hbm.at[rows], ckv_s.at[rows], s),
                pltpu.make_async_copy(wk_hbm.at[cs], rk.at[cs], s),
                pltpu.make_async_copy(wv_hbm.at[cs], rv.at[cs], s)]

    def x_copy(i):
        cols = _ds(i * TA, TA, TA)
        return pltpu.make_async_copy(xT_hbm.at[:, cols], xT_s.at[:, cols], sem.at[SEM_X + i])

    def out_copy(jp):
        cols = pl.ds(jp * 2 * T, 2 * T)
        return pltpu.make_async_copy(o_s.at[:, cols], out_hbm.at[:, cols], sem.at[SEM_OUT])

    @pl.when(h == 0)
    def _():
        cp_vec = [pltpu.make_async_copy(src, dst, sem.at[SEM_VEC])
                  for src, dst in zip((lre_hbm, lim_hbm, ldt_hbm, dsk_hbm, gw_hbm), vec_s)]
        cp_b = [pltpu.make_async_copy(src.at[pl.ds(lo, n)], b_s.at[pl.ds(dst, n)], sem.at[SEM_B])
                for src, lo, n, dst in ((bre_hbm, 0, PA, 0), (bim_hbm, 0, PA, PA),
                                        (bre_hbm, PA, PB, 2 * PA), (bim_hbm, PA, PB, 2 * PA + PB))]
        cp_wq = [pltpu.make_async_copy(wq_hbm, rq, sem.at[SEM_WQ])]
        cp_c = [pltpu.make_async_copy(src, craw_s.at[n], sem.at[SEM_C])
                for n, src in enumerate((cre_hbm, cim_hbm))]
        cp_wo = pltpu.make_async_copy(woT_hbm, wo_s, sem.at[SEM_WO])
        for cp in cp_vec + cp_b:
            cp.start()
        for i in range(S // TA):
            x_copy(i).start()
        for cp in cp_wq + cp_c:
            cp.start()
        for i in range(NP):
            for cp in slice_copies(i):
                cp.start()
        cp_wo.start()

        def phase1(i):
            x_copy(i).wait()
            u = _dot(xT_s[:, _ds(i * TA, TA, TA)], b_s[...], _TT)
            u_s[_ds(i * TA, TA, TA), :] = u
            never = zero_s[...] != 0.0

            def clocks(k, n):
                pos = (k * 6 * TA // n) // 8 * 8
                return never, u[pos % TA:pos % TA + 8, (pos // TA) * 128:(pos // TA + 1) * 128]

            for t in range(TA // (2 * T)):
                ev = _ds(i * TA + 2 * t * T, T, T)
                od = _ds(i * TA + (2 * t + 1) * T, T, T)
                for r in range(0, HM, 32):
                    top, bot = pl.ds(r, 32), pl.ds(HM + r, 32)
                    clk = clocks(t * 7 + r // 32, 14)
                    ops = _strassen_a(_tie(xT_s[top, ev].astype(f32), clk), xT_s[bot, ev].astype(f32),
                                      xT_s[top, od].astype(f32), _tie(xT_s[bot, od].astype(f32), clk))
                    for n in range(7):
                        xa_s[n, r // 2:r // 2 + 16, _ds(i * (TA // 2) + t * T, T, T)] = _pk(ops[n])
            return clocks

        for cp in cp_vec:
            cp.wait()
        _ssm_params(vec_s, coef_s, lam_s, col_s, zero_s)
        for cp in cp_b:
            cp.wait()

        def phase1_body(i, carry):
            phase1(i)
            return carry
        lax.fori_loop(0, S // TA - 1, phase1_body, 0)
        for cp in cp_wq + cp_c:
            cp.wait()
        clocks = phase1(S // TA - 1)
        for c0 in range(0, M, 8):
            _stage(rq, sq, c0, 8, clocks(c0 // 8, M // 8))
        _ssm_cmat(craw_s, coef_s, c_s, clocks)
        zero = jnp.zeros((1, 512), f32)
        carry0 = _ssm_scan(u_s, 0, (zero, zero), lam_s, h_s, clocks)

        def phase2(i, carry):
            for cp in slice_copies(i):
                cp.wait()
            yT = _dot(_up(c_s[...]), _up(h_s[...]), _NT)
            for t in range(TC // T):
                cols = _ds(i * TC + t * T, T, T)
                acc = jnp.zeros((8, T), f32)
                for r in range(0, M, 32):
                    xg = xT_s[r:r + 32, cols].astype(f32) * col_s[1, r:r + 32, :]
                    acc = acc + jnp.sum(xg.reshape(4, 8, T), axis=0)
                g = jax.nn.sigmoid(jnp.sum(acc, axis=0, keepdims=True))
                g_s[:, cols] = g
                for r in range(0, M, 32):
                    skip = xT_s[r:r + 32, cols].astype(f32) * col_s[0, r:r + 32, :]
                    o_s[r:r + 32, cols] = (1.0 - g) * (yT[r:r + 32, t * T:(t + 1) * T] + skip)

            words = _pair_words(sq, i, M)
            lo = _weight_ops([pltpu.bitcast(u << 16, f32) for u in words], M)
            hi = _weight_ops([pltpu.bitcast(u & jnp.uint32(0xFFFF0000), f32) for u in words], M)
            prods = [_dot(jnp.concatenate([lo[n], hi[n]], axis=1), _up(xa_s[n]), _TN) for n in range(7)]
            qs = LOG2E * D ** -0.5
            for n, c in enumerate(_strassen_c(prods)):
                c = c * qs
                rows = pl.ds((n % 2) * (HD // 2), HD // 2)
                q_s[2 * i, n // 2, rows, :] = _pk(c[:HD].astype(bf16))
                q_s[2 * i + 1, n // 2, rows, :] = _pk(c[HD:].astype(bf16))

            never = zero_s[...] != 0.0

            def clocks(k, n):
                pos = (k * 5 * 1024 // n) // 8 * 8
                r, c = pos % 256, (pos % 1024) // 256 * 256
                return never, prods[pos // 1024][r:r + 8, c:c + 128]

            carry = _ssm_scan(u_s, jnp.minimum(i + 1, NP - 1) * TC, carry, lam_s, h_s, clocks)

            for c0 in range(0, CS, 8):
                _stage(rk, sk, i * CS + c0, 8, clocks(c0 // 4, CS // 4))
                _stage(rv, sv, i * CS + c0, 8, clocks(c0 // 4 + 1, CS // 4))
            hc = DC // 2
            for r in range(0, T, 16):
                ev = _ds(i * 2 * T + r, 16, 16)
                od = _ds(i * 2 * T + T + r, 16, 16)
                for c0 in range(0, hc, 256):
                    lf, rt = pl.ds(c0, 256), pl.ds(hc + c0, 256)
                    clk = clocks(r // 8 + c0 // 256, T // 8)
                    ops = _strassen_a(_tie(ckv_s[ev, lf].astype(f32), clk), ckv_s[ev, rt].astype(f32),
                                      ckv_s[od, lf].astype(f32), _tie(ckv_s[od, rt].astype(f32), clk))
                    for n in range(7):
                        a_s[n, _ds(i * (T // 2) + r // 2, 8, 8), lf] = _pk(ops[n])
            return carry

        lax.fori_loop(0, NP, phase2, carry0)
        cp_wo.wait()
        wl_s[...] = jnp.zeros(wl_s.shape, u32)
        cl_s[...] = jnp.zeros(cl_s.shape, u32)

    def wo_ops(hh):
        w = wo_s[hh].astype(f32)
        return _strassen_a(w[:HM, :HD], w[:HM, HD:], w[HM:, :HD], w[HM:, HD:])

    def oproj(jp, wo, ops):
        for n, c in enumerate(_strassen_c([_dot(wo[i], ops[i], _NN) for i in range(7)])):
            rows = pl.ds((n // 2) * HM, HM)
            cols = pl.ds((2 * jp + n % 2) * T, T)
            o_s[rows, cols] += c

    oproj(NP - 1, [_up(wl_s[i]) for i in range(7)], [_up(cl_s[i]) for i in range(7)])

    wk = _head_weight_ops(sk, h, DC)
    for n, c in enumerate(_strassen_c([_dot(_up(a_s[i]), wk[i], _NN) for i in range(7)])):
        for t in range(NP):
            k_s[pl.ds((2 * t + n // 2) * (T // 2), T // 2), pl.ds((n % 2) * HD, HD)] = (
                _pk(c[t * T:(t + 1) * T].astype(bf16)))

    wv = _head_weight_ops(sv, h, DC)
    for n, c in enumerate(_strassen_c([_dot(wv[i], _up(a_s[i]), _TT) for i in range(7)])):
        for t in range(NP):
            vT_s[pl.ds((n % 2) * (HD // 2), HD // 2), pl.ds((2 * t + n // 2) * T, T)] = (
                _pk(c[:, t * T:(t + 1) * T].astype(bf16)))

    for i, w in enumerate(wo_ops(h)):
        wl_s[i] = _pk(w)

    key = lax.broadcasted_iota(jnp.int32, (T, T), 0)
    qry = lax.broadcasted_iota(jnp.int32, (T, T), 1)
    causal = key <= qry

    def qk(j):
        kv = (j + 1) * T
        qT = _up(q_s[h, j % 2, :, pl.ds((j // 2) * T, T)])
        s = _dot(_up(k_s[0:kv // 2, :]), qT, _NN)
        sd = jnp.where(causal, s[kv - T:kv], -1e30)
        s = jnp.concatenate([s[:kv - T], sd], axis=0) if j > 0 else sd
        s_s[j % 3, 0:kv, :] = s
        parts = [jnp.max(s[a:min(a + 512, kv)], axis=0, keepdims=True) for a in range(0, kv, 512)]
        m = parts[0]
        for part in parts[1:]:
            m = jnp.maximum(m, part)
        return m

    def softmax_pv(j, m):
        kv = (j + 1) * T
        p = jnp.exp2(s_s[j % 3, 0:kv, :] - m)
        parts = [jnp.sum(p[a:min(a + LCH, kv)], axis=0, keepdims=True) for a in range(0, kv, LCH)]
        l = parts[0]
        for part in parts[1:]:
            l = l + part
        c = _dot(_up(vT_s[:, 0:kv]), p.astype(bf16), _NN)
        return c * (g_s[:, j * T:(j + 1) * T] / l)

    def ctx_ops(ce, co):
        return _strassen_b(ce[:HD], co[:HD], ce[HD:], co[HD:])

    ss = {0: qk(0), 1: qk(1)}
    cs = {}
    for j in range(NT):
        if j + 2 < NT:
            ss[j + 2] = qk(j + 2)
        cs[j] = softmax_pv(j, ss.pop(j))
        if j >= 2 and j % 2 == 0:
            jp = j // 2 - 1
            oproj(jp, [_up(wl_s[i]) for i in range(7)], ctx_ops(cs.pop(j - 2), cs.pop(j - 1)))

            @pl.when(h == H - 1)
            def _():
                out_copy(jp).start()

    for i, c in enumerate(ctx_ops(cs.pop(NT - 2), cs.pop(NT - 1))):
        cl_s[i] = _pk(c)

    @pl.when(h == H - 1)
    def _():
        oproj(NP - 1, [_up(wl_s[i]) for i in range(7)], [_up(cl_s[i]) for i in range(7)])
        out_copy(NP - 1).start()
        for jp in range(NP):
            out_copy(jp).wait()


@jax.jit
def pallas_gated_mix__compressed_kv_cla__ssm_conv_s5__prompt_kernel(
    A_x: jax.Array,
    A_c_kv: jax.Array,
    A_w_q: jax.Array,
    A_w_uk: jax.Array,
    A_w_uv: jax.Array,
    A_w_o: jax.Array,
    B_x: jax.Array,
    B_Lambda_re: jax.Array,
    B_Lambda_im: jax.Array,
    B_B_re: jax.Array,
    B_B_im: jax.Array,
    B_C_re: jax.Array,
    B_C_im: jax.Array,
    B_log_dt: jax.Array,
    B_Dskip: jax.Array,
    gate_w: jax.Array,
):
    del B_x
    xT = jnp.transpose(A_x[0])
    woT = jnp.transpose(A_w_o, (0, 2, 1))
    ckv = A_c_kv[0]

    hbm = pl.BlockSpec(memory_space=pl.ANY)
    vmem = pltpu.VMEM
    outT = pl.pallas_call(
        _kernel,
        grid=(H,),
        in_specs=[hbm] * 15,
        out_specs=hbm,
        out_shape=jax.ShapeDtypeStruct((M, S), f32),
        scratch_shapes=[
            vmem((M, S), bf16),
            vmem((M,), bf16), vmem((M,), bf16), vmem((M,), bf16), vmem((M,), bf16), vmem((M,), bf16),
            vmem((2 * M, M), bf16),
            vmem((2, M, M), bf16),
            vmem((M // 2, 2 * M), u32),
            vmem((8, 512), f32),
            vmem((8, 8, 512), f32),
            vmem((2, M, 128), f32),
            vmem((S, 2 * M), f32),
            vmem((1, S), f32),
            vmem((S, DC), bf16),
            vmem((M, H, D), bf16),
            vmem((DC, H, D), bf16),
            vmem((DC, H, D), bf16),
            vmem((4, M * 4, 128), u32),
            vmem((4, DC * 4, 128), u32),
            vmem((4, DC * 4, 128), u32),
            vmem((7, S // 4, DC // 2), u32),
            vmem((7, HM // 2, S // 2), u32),
            vmem((H, 2, D // 2, S // 2), u32),
            vmem((H, M, D), bf16),
            vmem((S // 2, D), u32),
            vmem((D // 2, S), u32),
            vmem((M, S), f32),
            vmem((3, S, T), f32),
            vmem((TC // 2, 2 * M), u32),
            vmem((8, 128), f32),
            vmem((7, HM // 2, HD), u32),
            vmem((7, HD // 2, T), u32),
            pltpu.SemaphoreType.DMA((NSEM,)),
        ],
        compiler_params=pltpu.CompilerParams(
            dimension_semantics=("arbitrary",),
            vmem_limit_bytes=120 * 1024 * 1024,
        ),
    )(xT, B_B_re, B_B_im, B_C_re, B_C_im, B_Lambda_re, B_Lambda_im, B_log_dt,
      B_Dskip, gate_w, woT, ckv, A_w_q, A_w_uk, A_w_uv)
    return jnp.transpose(outT)[None]
```

```python
import jax
import jax.numpy as jnp
from jax import lax
import jax.experimental.pallas as pl
import jax.experimental.pallas.tpu as pltpu

S = 2048
M = 448
H = 16
D = 256
DC = 1024
T = 128
NT = S // T
NP = NT // 2
HD = D // 2
HM = M // 2
PA = 384
PB = M - PA
TA = 512
TC = 256
CS = DC // NP
import os
G = int(os.environ.get('G', 32))
RCH = int(os.environ.get('RCH', 512))
QCH = int(os.environ.get('QCH', 1024))
SLACK = int(os.environ.get('SLACK', 200))
LOG2E = 1.4426950408889634

f32 = jnp.float32
bf16 = jnp.bfloat16
u32 = jnp.uint32

SEM_VEC, SEM_B, SEM_X, SEM_WQ, SEM_C, SEM_SL, SEM_WO, SEM_OUT = 0, 1, 2, 6, 7, 8, 16, 17
NSEM = 18


def _dot(a, b, dims):
    return lax.dot_general(a, b, (dims, ((), ())), preferred_element_type=f32)


_NN = ((1,), (0,))
_NT = ((1,), (1,))
_TN = ((0,), (0,))
_TT = ((0,), (1,))


def _pk(x):
    return pltpu.bitcast(x, u32)


def _up(x):
    return pltpu.bitcast(x, bf16)


class _Stack:
    def __init__(self, ref, rows, along_lanes=False):
        self.ref, self.rows, self.along_lanes = ref, rows, along_lanes

    def _idx(self, n, r0, nr, cols):
        lo = r0 // 2 if isinstance(r0, int) else lax.shift_right_logical(r0, 1)
        nr = (self.rows if nr is None else nr) // 2
        if self.along_lanes:
            return _ds(lo, nr, 8), pl.ds(n * 128, 128)
        return _ds(n * (self.rows // 2) + lo, nr, 8), (slice(None) if cols is None else cols)

    def get(self, n, r0=0, nr=None, cols=None):
        return _up(self.ref[self._idx(n, r0, nr, cols)])

    def put(self, n, r0, x, cols=None):
        self.ref[self._idx(n, r0, x.shape[0], cols)] = _pk(x)


def _tie(x, clock):
    if clock is None:
        return x
    never, tick = clock
    r, c = x.shape
    if tick.dtype != x.dtype:
        tick = pltpu.bitcast(tick, x.dtype)
    tile = lambda v: jnp.tile(v, (r // 8, c // 128))
    return jnp.where(tile(never), tile(tick), x)


def _cmul(ar, ai, br, bi):
    return ar * br - ai * bi, ar * bi + ai * br


def _ds(lo, n, align):
    return pl.ds(lo if isinstance(lo, int) else pl.multiple_of(lo, align), n)


def _strassen_a(a11, a12, a21, a22):
    ops = [a11 + a22, a21 + a22, a11, a22, a11 + a12, a21 - a11, a12 - a22]
    return [o.astype(bf16) for o in ops]


def _strassen_b(b11, b12, b21, b22, dtype=bf16):
    ops = [b11 + b22, b11, b12 - b22, b21 - b11, b22, b11 + b12, b21 + b22]
    return [o.astype(dtype) for o in ops]


def _strassen_c(m):
    c11 = (m[0] + m[3]) + (m[6] - m[4])
    c12 = m[2] + m[4]
    c21 = m[1] + m[3]
    c22 = (m[0] - m[1]) + (m[2] + m[5])
    return c11, c12, c21, c22


def _stage(raw, stg, c0, nc, clock=None):
    for ht in range(2):
        for dt in range(2):
            v = raw[pl.ds(c0, nc), ht * 8:(ht + 1) * 8, dt * 128:(dt + 1) * 128]
            stg[ht * 2 + dt, _ds(c0 * 4, nc * 4, 8), :] = _tie(_pk(v.reshape(nc * 8, 128)), clock)


def _pair_words(stg, pair, rows):
    ht = lax.shift_right_logical(pair, 2)
    return [stg[ht * 2 + dt, pl.ds(pair & 3, rows, stride=4), :] for dt in range(2)]


def _weight_ops(halves, rows, dtype=bf16):
    r = rows // 2
    return _strassen_b(halves[0][:r], halves[1][:r], halves[0][r:], halves[1][r:], dtype)


def _head_weight_block(stg, h, c0, nc, dt):
    pair = lax.shift_right_logical(h, 1)
    ht = lax.shift_right_logical(pair, 2)
    sh = (16 * (1 - (h & 1))).astype(u32)
    u = stg[ht * 2 + dt, pl.ds(c0 * 4 + (pair & 3), nc, stride=4), :]
    return pltpu.bitcast((u << sh) & jnp.uint32(0xFFFF0000), f32)


class _Clock:
    def __init__(self, never):
        self.never, self.ticks, self.t = never, [], 0

    def stage(self, duration, vals):
        for k, v in enumerate(vals):
            self.ticks.append((self.t + duration * (k + 1) / len(vals), v))
        self.t += duration

    def pacer(self, t0, t1):
        def clocks(k, n):
            want = t0 + (t1 - t0) * k / n
            best = [v for t, v in self.ticks if t <= want]
            return (self.never, best[-1]) if best else None
        return clocks


def _rows8(vals, step=8):
    return [v[r:r + 8, 0:128] for v in vals for r in range(0, v.shape[0], step)]


def _ssm_cmat(craw_s, coef_s, c_s, clocks):
    for r in range(0, M, 16):
        coef = _tie(coef_s[...], clocks(r // 16, M // 16))
        cr, ci = coef[0:1, :M], coef[1:2, :M]
        cp_re, cp_im = _cmul(craw_s[0, r:r + 16, :].astype(f32), craw_s[1, r:r + 16, :].astype(f32), cr, ci)
        c_s[r // 2:r // 2 + 8, :] = _pk(jnp.concatenate(
            [cp_re[:, :PA], -cp_im[:, :PA], cp_re[:, PA:], -cp_im[:, PA:]], axis=1).astype(bf16))


def _ssm_params(vec_s, coef_s, lam_s, col_s, zero_s):
    row = lambda r: r[...].astype(f32).reshape(1, M)
    lre, lim, ldt, dsk, gw = [row(v) for v in vec_s]
    dt = jnp.exp(ldt).astype(bf16).astype(f32)
    mag = jnp.exp(dt * lre)
    ang = dt * lim
    lr, li = mag * jnp.cos(ang), mag * jnp.sin(ang)
    den = lre * lre + lim * lim
    nr = lr - 1.0
    coef_s[...] = jnp.zeros(coef_s.shape, f32)
    coef_s[0:1, 0:M] = 2.0 * ((nr * lre + li * lim) / den)
    coef_s[1:2, 0:M] = 2.0 * ((li * lre - nr * lim) / den)
    zero_s[...] = jnp.zeros(zero_s.shape, f32)

    er = jnp.concatenate([lr, lr[:, PA:]], axis=1)
    ei = jnp.concatenate([li, -li[:, PA:]], axis=1)
    pw = [(er, ei)]
    for _ in range(7):
        pw.append(_cmul(pw[-1][0], pw[-1][1], er, ei))
    sub = lax.broadcasted_iota(jnp.int32, (8, 512), 0)
    for n, d in enumerate((1, 2, 4)):
        lam_s[2 * n] = jnp.where(sub >= d, pw[d - 1][0], 0.0)
        lam_s[2 * n + 1] = jnp.where(sub >= d, pw[d - 1][1], 0.0)
    lcr = jnp.zeros((8, 512), f32)
    lci = jnp.zeros((8, 512), f32)
    for r in range(8):
        lcr = jnp.where(sub == r, pw[r][0], lcr)
        lci = jnp.where(sub == r, pw[r][1], lci)
    lam_s[6] = lcr
    lam_s[7] = lci

    def col(v):
        v = jnp.concatenate([v, jnp.zeros((1, 512 - M), f32)], axis=1)
        return jnp.broadcast_to(v, (128, 512)).T[:M]
    col_s[0] = col(dsk)
    col_s[1] = col(gw)


def _ssm_scan(u_s, t0, carry, lam_s, h_s, clocks):
    car, cai = carry
    out = []
    for b in range(TC // 8):
        u = u_s[_ds(t0 + b * 8, 8, 8), :]
        mixed = u[:, 2 * PA:]
        cols = [u[:, 0:128], u[:, 128:256], u[:, 256:384], mixed]
        hr = jnp.concatenate([_tie(v, clocks(4 * b + n, TC // 2)) for n, v in enumerate(cols)], axis=1)
        hi = jnp.concatenate([u[:, PA:2 * PA], pltpu.roll(mixed, PB, 1)], axis=1)
        for n, d in enumerate((1, 2, 4)):
            sr, si = pltpu.roll(hr, d, 0), pltpu.roll(hi, d, 0)
            tr, ti = _cmul(sr, si, lam_s[2 * n], lam_s[2 * n + 1])
            hr, hi = hr + tr, hi + ti
        tr, ti = _cmul(lam_s[6], lam_s[7], car, cai)
        hr, hi = hr + tr, hi + ti
        car, cai = hr[7:8, :], hi[7:8, :]
        out.append(jnp.concatenate([hr[:, :PA], hi[:, :PA], hr[:, PA:]], axis=1))
        if b % 2 == 1:
            h_s[(b // 2) * 8:(b // 2 + 1) * 8, :] = _pk(jnp.concatenate(out, axis=0).astype(bf16))
            out = []
    return car, cai


def _kernel(xT_hbm, bre_hbm, bim_hbm, cre_hbm, cim_hbm, lre_hbm, lim_hbm, ldt_hbm,
            dsk_hbm, gw_hbm, woT_hbm, ckv_hbm, wq_hbm, wk_hbm, wv_hbm,
            out_hbm,
            xT_s, v0, v1, v2, v3, v4, b_s, craw_s, c_s, coef_s, lam_s, col_s, u_s, g_s,
            ckv_s, rq, rk, rv, sq, sk, sv, a_s, xa_s, q_s, wo_s,
            ka_s, va_s, pb_s, o_s, s_s, h_s, zero_s, wl_s, cl_s, wk_s, wv_s, sem):
    h = pl.program_id(0)
    vec_s = (v0, v1, v2, v3, v4)
    a_s, xa_s, q_s = _Stack(a_s, S // 2), _Stack(xa_s, HM), _Stack(q_s, D)
    ka_s, va_s, pb_s = _Stack(ka_s, S // 2, True), _Stack(va_s, HD), _Stack(pb_s, S // 2, True)
    wk_s, wv_s = _Stack(wk_s, DC // 2, True), _Stack(wv_s, HD)
    wl_s, cl_s = _Stack(wl_s, HM, True), _Stack(cl_s, HD, True)

    def slice_copies(i):
        s = sem.at[SEM_SL + i]
        rows = _ds(i * 2 * T, 2 * T, 2 * T)
        cs = pl.ds(i * CS, CS)
        return [pltpu.make_async_copy(ckv_hbm.at[rows], ckv_s.at[rows], s),
                pltpu.make_async_copy(wk_hbm.at[cs], rk.at[cs], s),
                pltpu.make_async_copy(wv_hbm.at[cs], rv.at[cs], s)]

    def x_copy(i):
        cols = _ds(i * TA, TA, TA)
        return pltpu.make_async_copy(xT_hbm.at[:, cols], xT_s.at[:, cols], sem.at[SEM_X + i])

    def out_copy(jp):
        cols = pl.ds(jp * 2 * T, 2 * T)
        return pltpu.make_async_copy(o_s.at[:, cols], out_hbm.at[:, cols], sem.at[SEM_OUT])

    def prep_wk(hh, clocks):
        for r in range(0, DC // 2, G):
            clock = clocks(r // G, DC // 2 // G)
            blk = [_head_weight_block(sk, hh, half * (DC // 2) + r, G, dt) for half in range(2) for dt in range(2)]
            ops = _strassen_b(_tie(blk[0], clock), blk[1], blk[2], _tie(blk[3], clock))
            for n in range(7):
                wk_s.put(n, r, ops[n])

    @pl.when(h == 0)
    def _():
        cp_vec = [pltpu.make_async_copy(src, dst, sem.at[SEM_VEC])
                  for src, dst in zip((lre_hbm, lim_hbm, ldt_hbm, dsk_hbm, gw_hbm), vec_s)]
        cp_b = [pltpu.make_async_copy(src.at[pl.ds(lo, n)], b_s.at[pl.ds(dst, n)], sem.at[SEM_B])
                for src, lo, n, dst in ((bre_hbm, 0, PA, 0), (bim_hbm, 0, PA, PA),
                                        (bre_hbm, PA, PB, 2 * PA), (bim_hbm, PA, PB, 2 * PA + PB))]
        cp_wq = [pltpu.make_async_copy(wq_hbm, rq, sem.at[SEM_WQ])]
        cp_c = [pltpu.make_async_copy(src, craw_s.at[n], sem.at[SEM_C])
                for n, src in enumerate((cre_hbm, cim_hbm))]
        cp_wo = pltpu.make_async_copy(woT_hbm, wo_s, sem.at[SEM_WO])
        for cp in cp_vec + cp_b:
            cp.start()
        for i in range(S // TA):
            x_copy(i).start()
        for cp in cp_wq + cp_c:
            cp.start()
        for i in range(NP):
            for cp in slice_copies(i):
                cp.start()
        cp_wo.start()

        def phase1(i):
            x_copy(i).wait()
            u = _dot(xT_s[:, _ds(i * TA, TA, TA)], b_s[...], _TT)
            u_s[_ds(i * TA, TA, TA), :] = u
            never = zero_s[...] != 0.0

            def clocks(k, n):
                pos = (k * 6 * TA // n) // 8 * 8
                return never, u[pos % TA:pos % TA + 8, (pos // TA) * 128:(pos // TA + 1) * 128]

            for t in range(TA // (2 * T)):
                ev = _ds(i * TA + 2 * t * T, T, T)
                od = _ds(i * TA + (2 * t + 1) * T, T, T)
                for r in range(0, HM, 32):
                    top, bot = pl.ds(r, 32), pl.ds(HM + r, 32)
                    clk = clocks(t * 7 + r // 32, 14)
                    ops = _strassen_a(_tie(xT_s[top, ev].astype(f32), clk), xT_s[bot, ev].astype(f32),
                                      xT_s[top, od].astype(f32), _tie(xT_s[bot, od].astype(f32), clk))
                    for n in range(7):
                        xa_s.put(n, r, ops[n], _ds(i * (TA // 2) + t * T, T, T))
            return clocks

        for cp in cp_vec:
            cp.wait()
        _ssm_params(vec_s, coef_s, lam_s, col_s, zero_s)
        for cp in cp_b:
            cp.wait()

        def phase1_body(i, carry):
            phase1(i)
            return carry
        lax.fori_loop(0, S // TA - 1, phase1_body, 0)
        for cp in cp_wq + cp_c:
            cp.wait()
        clocks = phase1(S // TA - 1)
        for c0 in range(0, M, 8):
            _stage(rq, sq, c0, 8, clocks(c0 // 8, M // 8))
        _ssm_cmat(craw_s, coef_s, c_s, clocks)
        zero = jnp.zeros((1, 512), f32)
        carry0 = _ssm_scan(u_s, 0, (zero, zero), lam_s, h_s, clocks)

        def phase2(i, carry):
            for cp in slice_copies(i):
                cp.wait()
            yT = _dot(_up(c_s[...]), _up(h_s[...]), _NT)
            for t in range(TC // T):
                cols = _ds(i * TC + t * T, T, T)
                acc = jnp.zeros((8, T), f32)
                for r in range(0, M, 32):
                    xg = xT_s[r:r + 32, cols].astype(f32) * col_s[1, r:r + 32, :]
                    acc = acc + jnp.sum(xg.reshape(4, 8, T), axis=0)
                g = jax.nn.sigmoid(jnp.sum(acc, axis=0, keepdims=True))
                g_s[:, cols] = g
                for r in range(0, M, 32):
                    skip = xT_s[r:r + 32, cols].astype(f32) * col_s[0, r:r + 32, :]
                    o_s[r:r + 32, cols] = (1.0 - g) * (yT[r:r + 32, t * T:(t + 1) * T] + skip)

            words = _pair_words(sq, i, M)
            lo = _weight_ops([pltpu.bitcast(u << 16, f32) for u in words], M, f32)
            hi = _weight_ops([pltpu.bitcast(u & jnp.uint32(0xFFFF0000), f32) for u in words], M, f32)
            prods = [_dot(jnp.concatenate([lo[n], hi[n]], axis=1).astype(bf16), xa_s.get(n), _TN)
                     for n in range(7)]
            qs = LOG2E * D ** -0.5
            for t in range(NP):
                for r in range(0, D, G):
                    cs = _strassen_c([v[r:r + G, t * T:(t + 1) * T] for v in prods])
                    for n, c in enumerate(cs):
                        q_s.put(4 * i + 2 * (r // HD) + n // 2, (n % 2) * HD + r % HD,
                                (c * qs).astype(bf16), pl.ds(t * T, T))

            never = zero_s[...] != 0.0

            def clocks(k, n):
                pos = (k * 5 * 1024 // n) // 8 * 8
                r, c = pos % 256, (pos % 1024) // 256 * 256
                return never, prods[pos // 1024][r:r + 8, c:c + 128]

            carry = _ssm_scan(u_s, jnp.minimum(i + 1, NP - 1) * TC, carry, lam_s, h_s, clocks)

            for c0 in range(0, CS, 8):
                _stage(rk, sk, i * CS + c0, 8, clocks(c0 // 4, CS // 4))
                _stage(rv, sv, i * CS + c0, 8, clocks(c0 // 4 + 1, CS // 4))
            hc = DC // 2
            for r in range(0, T, 16):
                ev = _ds(i * 2 * T + r, 16, 16)
                od = _ds(i * 2 * T + T + r, 16, 16)
                for c0 in range(0, hc, 256):
                    lf, rt = pl.ds(c0, 256), pl.ds(hc + c0, 256)
                    clk = clocks(r // 8 + c0 // 256, T // 8)
                    ops = _strassen_a(_tie(ckv_s[ev, lf].astype(f32), clk), ckv_s[ev, rt].astype(f32),
                                      ckv_s[od, lf].astype(f32), _tie(ckv_s[od, rt].astype(f32), clk))
                    for n in range(7):
                        a_s.put(n, i * T + r, ops[n], lf)
            return carry

        lax.fori_loop(0, NP, phase2, carry0)
        cp_wo.wait()
        prep_wk(h, lambda k, n: None)
        wl_s.ref[...] = jnp.zeros(wl_s.ref.shape, u32)
        cl_s.ref[...] = jnp.zeros(cl_s.ref.shape, u32)

    clk = _Clock(zero_s[...] != 0.0)
    hc = DC // 2

    def oproj(jp, ops):
        m = [_dot(wl_s.get(i), ops[i], _NN) for i in range(7)]
        for r in range(0, HM, G):
            for n, c in enumerate(_strassen_c([v[r:r + G] for v in m])):
                o_s[pl.ds((n // 2) * HM + r, G), pl.ds((2 * jp + n % 2) * T, T)] += c
        clk.stage(392, _rows8([m[0], m[4]]))

    def prep_wo(clocks):
        for r in range(0, HM, G):
            top = _tie(wo_s[h, r:r + G, :].astype(f32), clocks(r // G, HM // G))
            bot = _tie(wo_s[h, HM + r:HM + r + G, :].astype(f32), clocks(r // G, HM // G))
            for n, w in enumerate(_strassen_a(top[:, :HD], top[:, HD:], bot[:, :HD], bot[:, HD:])):
                wl_s.put(n, r, w)

    def prep_wv(clocks):
        for c0 in range(0, hc, T):
            blk = [[_tie(_head_weight_block(sv, h, half * hc + c0, T, dt), clocks(c0 // T, hc // T)).T
                    for dt in range(2)] for half in range(2)]
            for r in range(0, HD, G):
                ops = _strassen_b(*[v[r:r + G] for v in blk[0] + blk[1]])
                for n in range(7):
                    wv_s.put(n, r, ops[n], pl.ds(c0, T))

    def kproj(t):
        m = [_dot(a_s.get(n, t * T, T), wk_s.get(n), _NN) for n in range(7)]
        for r in range(0, T, G):
            c11, c12, c21, c22 = _strassen_c([v[r:r + G] for v in m])
            ops = _strassen_a(c11, c12, c21, c22) + [c12.astype(bf16), c21.astype(bf16)]
            for n in range(9):
                ka_s.put(n, t * T + r, ops[n])
        clk.stage(896, _rows8(m))

    def vproj(t):
        m = [_dot(wv_s.get(n), a_s.get(n, t * T, T), _NT) for n in range(7)]
        for r in range(0, HD, G):
            c11, c21, c12, c22 = _strassen_c([v[r:r + G] for v in m])
            ops = _strassen_a(c11, c12, c21, c22) + [c12.astype(bf16), c21.astype(bf16)]
            for n in range(9):
                va_s.put(n, r, ops[n], pl.ds(t * T, T))
        clk.stage(896, _rows8(m))

    key = lax.broadcasted_iota(jnp.int32, (T, T), 0)
    qry = lax.broadcasted_iota(jnp.int32, (T, T), 1)
    causal = key <= qry

    class Reducer:
        def __init__(self, red, comb):
            self.red, self.comb, self.acc, self.rows, self.out = red, comb, None, 0, None

        def add(self, v):
            v = self.red(v.reshape(v.shape[0] // 8, 8, T), axis=0)
            self.acc = v if self.acc is None else self.comb(self.acc, v)
            self.rows += 1
            if self.rows * G >= RCH:
                self.flush()

        def flush(self):
            if self.acc is not None:
                v = self.red(self.acc, axis=0, keepdims=True)
                self.out = v if self.out is None else self.comb(self.out, v)
            self.acc, self.rows = None, 0

        def result(self):
            self.flush()
            return self.out

    def qk(jp):
        R, slot = jp * T, jp % 2
        cols = pl.ds(jp * T, T)
        qe, qo = q_s.get(2 * h, cols=cols), q_s.get(2 * h + 1, cols=cols)
        mx = [Reducer(jnp.max, jnp.maximum) for _ in range(2)]

        def put(e, row, v):
            s_s[slot, e, row:row + G, :] = v
            mx[e].add(v)

        if jp > 0:
            qef, qof = qe.astype(f32), qo.astype(f32)
            qb = _strassen_b(qef[:HD], qof[:HD], qef[HD:], qof[HD:])
            for r0 in range(0, R, QCH):
                r1 = min(r0 + QCH, R)
                m = [_dot(ka_s.get(n, r0, r1 - r0), qb[n], _NN) for n in range(7)]
                for r in range(0, r1 - r0, G):
                    c11, c12, c21, c22 = _strassen_c([v[r:r + G] for v in m])
                    put(0, r0 + r, c11)
                    put(1, r0 + r, c12)
                    put(0, R + r0 + r, c21)
                    put(1, R + r0 + r, c22)
                clk.stage(7 * (r1 - r0) / 4, _rows8([m[0], m[4]]))
        ke = jnp.concatenate([ka_s.get(2, R, T), ka_s.get(7, R, T)], axis=1)
        ko = jnp.concatenate([ka_s.get(8, R, T), ka_s.get(3, R, T)], axis=1)
        se = _dot(ke, jnp.concatenate([qe, qo], axis=1), _NN)
        so = _dot(ko, qo, _NN)
        for r in range(0, T, G):
            put(0, 2 * R + r, jnp.where(causal[r:r + G], se[r:r + G, :T], -1e30))
            put(1, 2 * R + r, se[r:r + G, T:])
            put(1, 2 * R + T + r, jnp.where(causal[r:r + G], so[r:r + G], -1e30))
        clk.stage(192, _rows8([se]))
        return [jnp.broadcast_to(x.result(), (8, T)) for x in mx]

    def shifted_exp(slot, e, row, z):
        v = s_s[slot, e, row:row + G, :].reshape(G // 8, 8, T) - z[None]
        return jnp.exp2(v).reshape(G, T)

    def softmax(jp, mx, t0, t1):
        R, slot = jp * T, jp % 2
        tm = (t0 + t1) / 2
        clocks = clk.pacer(t0, tm)
        k, n = 0, (4 * jp + 3) * T // G
        z = []
        for e in range(2):
            sm = Reducer(jnp.sum, jnp.add)
            for r in range(0, (2 * jp + 1 + e) * T, G):
                sm.add(shifted_exp(slot, e, r, _tie(mx[e], clocks(k, n))))
                k += 1
            z.append(mx[e] + jnp.log2(sm.result()))
        clocks = clk.pacer(tm, t1)
        k = 0
        for r in range(0, R, G):
            ze, zo = _tie(z[0], clocks(k, n)), _tie(z[1], clocks(k + 2, n))
            ops = _strassen_b(shifted_exp(slot, 0, r, ze), shifted_exp(slot, 1, r, zo),
                              shifted_exp(slot, 0, R + r, ze), shifted_exp(slot, 1, R + r, zo))
            for i in range(7):
                pb_s.put(slot * 8 + i, r, ops[i])
            k += 4
        for r in range(0, 3 * T, G):
            e = int(r >= T)
            p = shifted_exp(slot, e, 2 * R + r - e * T, _tie(z[e], clocks(k, n)))
            pb_s.put(slot * 8 + 7, r, p.astype(bf16))
            k += 1

    def pv(jp):
        R, slot = jp * T, jp % 2
        if jp > 0:
            m = [_dot(va_s.get(n, cols=pl.ds(0, R)), pb_s.get(slot * 8 + n, 0, R), _NN) for n in range(7)]
            clk.stage(7 * R / 4, _rows8(m, 32))
        cols = pl.ds(R, T)
        ve = jnp.concatenate([va_s.get(2, cols=cols), va_s.get(8, cols=cols)], axis=0)
        vo = jnp.concatenate([va_s.get(7, cols=cols), va_s.get(3, cols=cols)], axis=0)
        ce = _dot(ve, pb_s.get(slot * 8 + 7, 0, T), _NN)
        co = _dot(jnp.concatenate([ve, vo], axis=1), pb_s.get(slot * 8 + 7, T, 2 * T), _NN)
        clk.stage(192, _rows8([ce], 32))
        ge = g_s[:, 2 * jp * T:(2 * jp + 1) * T]
        go = g_s[:, (2 * jp + 1) * T:(2 * jp + 2) * T]
        for r in range(0, HD, G):
            c = [ce[r:r + G], co[r:r + G], ce[HD + r:HD + r + G], co[HD + r:HD + r + G]]
            if jp > 0:
                c = [x + y for x, y in zip(c, _strassen_c([v[r:r + G] for v in m]))]
            ops = _strassen_b(c[0] * ge, c[1] * go, c[2] * ge, c[3] * go)
            for n in range(7):
                cl_s.put(slot * 7 + n, r, ops[n])

    def ctx_ops(jp):
        return [cl_s.get((jp % 2) * 7 + n) for n in range(7)]

    oproj(NP - 1, ctx_ops(NP - 1))
    t0 = clk.t
    kproj(0)
    kproj(1)
    prep_wv(clk.pacer(0, t0 + 896))
    prep_wo(clk.pacer(t0 + 896, clk.t))
    mx = qk(0)
    t0 = clk.t
    kproj(2)
    softmax(0, mx, t0, clk.t)
    for jp in range(NP):
        if jp + 1 < NP:
            mx = qk(jp + 1)
        t0 = clk.t
        if jp < NP - 1:
            vproj(jp)
        pv(jp)
        if jp > 0:
            oproj(jp - 1, ctx_ops(jp - 1))

            @pl.when(h == H - 1)
            def _():
                out_copy(jp - 1).start()
        if jp + 3 < NP:
            kproj(jp + 3)
        if jp == NP - 2:
            vproj(NP - 1)
        if jp + 1 < NP:
            softmax(jp + 1, mx, t0, clk.t - SLACK)
        else:
            prep_wk(jnp.minimum(h + 1, H - 1), clk.pacer(t0, clk.t - 400))

    @pl.when(h == H - 1)
    def _():
        oproj(NP - 1, ctx_ops(NP - 1))
        out_copy(NP - 1).start()
        for jp in range(NP):
            out_copy(jp).wait()


@jax.jit
def pallas_gated_mix__compressed_kv_cla__ssm_conv_s5__prompt_kernel(
    A_x: jax.Array,
    A_c_kv: jax.Array,
    A_w_q: jax.Array,
    A_w_uk: jax.Array,
    A_w_uv: jax.Array,
    A_w_o: jax.Array,
    B_x: jax.Array,
    B_Lambda_re: jax.Array,
    B_Lambda_im: jax.Array,
    B_B_re: jax.Array,
    B_B_im: jax.Array,
    B_C_re: jax.Array,
    B_C_im: jax.Array,
    B_log_dt: jax.Array,
    B_Dskip: jax.Array,
    gate_w: jax.Array,
):
    del B_x
    xT = jnp.transpose(A_x[0])
    woT = jnp.transpose(A_w_o, (0, 2, 1))
    ckv = A_c_kv[0]

    hbm = pl.BlockSpec(memory_space=pl.ANY)
    vmem = pltpu.VMEM
    outT = pl.pallas_call(
        _kernel,
        grid=(H,),
        in_specs=[hbm] * 15,
        out_specs=hbm,
        out_shape=jax.ShapeDtypeStruct((M, S), f32),
        scratch_shapes=[
            vmem((M, S), bf16),
            vmem((M,), bf16), vmem((M,), bf16), vmem((M,), bf16), vmem((M,), bf16), vmem((M,), bf16),
            vmem((2 * M, M), bf16),
            vmem((2, M, M), bf16),
            vmem((M // 2, 2 * M), u32),
            vmem((8, 512), f32),
            vmem((8, 8, 512), f32),
            vmem((2, M, 128), f32),
            vmem((S, 2 * M), f32),
            vmem((1, S), f32),
            vmem((S, DC), bf16),
            vmem((M, H, D), bf16),
            vmem((DC, H, D), bf16),
            vmem((DC, H, D), bf16),
            vmem((4, M * 4, 128), u32),
            vmem((4, DC * 4, 128), u32),
            vmem((4, DC * 4, 128), u32),
            vmem((7 * S // 4, DC // 2), u32),
            vmem((7 * HM // 2, S // 2), u32),
            vmem((H * D, S // 2), u32),
            vmem((H, M, D), bf16),
            vmem((S // 4, 9 * HD), u32),
            vmem((9 * HD // 2, S // 2), u32),
            vmem((S // 4, 16 * T), u32),
            vmem((M, S), f32),
            vmem((2, 2, S, T), f32),
            vmem((TC // 2, 2 * M), u32),
            vmem((8, 128), f32),
            vmem((HM // 2, 7 * HD), u32),
            vmem((HD // 2, 14 * T), u32),
            vmem((DC // 4, 7 * HD), u32),
            vmem((7 * HD // 2, DC // 2), u32),
            pltpu.SemaphoreType.DMA((NSEM,)),
        ],
        compiler_params=pltpu.CompilerParams(
            dimension_semantics=("arbitrary",),
            vmem_limit_bytes=120 * 1024 * 1024,
        ),
    )(xT, B_B_re, B_B_im, B_C_re, B_C_im, B_Lambda_re, B_Lambda_im, B_log_dt,
      B_Dskip, gate_w, woT, ckv, A_w_q, A_w_uk, A_w_uv)
    return jnp.transpose(outT)[None]
```

```python
import jax
import jax.numpy as jnp
from jax import lax
import jax.experimental.pallas as pl
import jax.experimental.pallas.tpu as pltpu

S = 2048
M = 448
H = 16
D = 256
DC = 1024
T = 128
NT = S // T
NP = NT // 2
HD = D // 2
HM = M // 2
QD = D // 4
QC = DC // 4
PA = 384
PB = M - PA
TA = 512
TC = 256
CS = DC // NP
import os
G = int(os.environ.get('G', 32))
RCH = int(os.environ.get('RCH', 512))
QCH = int(os.environ.get('QCH', 1024))
SLACK = int(os.environ.get('SLACK', 200))
LOG2E = 1.4426950408889634

f32 = jnp.float32
bf16 = jnp.bfloat16
u32 = jnp.uint32

SEM_VEC, SEM_B, SEM_X, SEM_WQ, SEM_C, SEM_SL, SEM_WO, SEM_OUT = 0, 1, 2, 6, 7, 8, 16, 17
NSEM = 18


def _dot(a, b, dims):
    return lax.dot_general(a, b, (dims, ((), ())), preferred_element_type=f32)


_NN = ((1,), (0,))
_NT = ((1,), (1,))
_TN = ((0,), (0,))
_TT = ((0,), (1,))


def _pk(x):
    return pltpu.bitcast(x, u32)


def _up(x):
    return pltpu.bitcast(x, bf16)


class _Stack:
    def __init__(self, ref, rows, along_lanes=False):
        self.ref, self.rows, self.along_lanes = ref, rows, along_lanes

    def _idx(self, n, r0, nr, cols):
        lo = r0 // 2 if isinstance(r0, int) else lax.shift_right_logical(r0, 1)
        nr = (self.rows if nr is None else nr) // 2
        if self.along_lanes:
            return _ds(lo, nr, 8), pl.ds(n * 128, 128)
        return _ds(n * (self.rows // 2) + lo, nr, 8), (slice(None) if cols is None else cols)

    def get(self, n, r0=0, nr=None, cols=None):
        return _up(self.ref[self._idx(n, r0, nr, cols)])

    def put(self, n, r0, x, cols=None):
        self.ref[self._idx(n, r0, x.shape[0], cols)] = _pk(x)


def _tie(x, clock):
    if clock is None:
        return x
    never, tick = clock
    r, c = x.shape
    if tick.dtype != x.dtype:
        tick = pltpu.bitcast(tick, x.dtype)
    tile = lambda v: jnp.tile(v, (r // 8, c // 128))
    return jnp.where(tile(never), tile(tick), x)


def _cmul(ar, ai, br, bi):
    return ar * br - ai * bi, ar * bi + ai * br


def _ds(lo, n, align):
    return pl.ds(lo if isinstance(lo, int) else pl.multiple_of(lo, align), n)


def _strassen_a(a11, a12, a21, a22):
    ops = [a11 + a22, a21 + a22, a11, a22, a11 + a12, a21 - a11, a12 - a22]
    return [o.astype(bf16) for o in ops]


def _strassen_b(b11, b12, b21, b22, dtype=bf16):
    ops = [b11 + b22, b11, b12 - b22, b21 - b11, b22, b11 + b12, b21 + b22]
    return [o.astype(dtype) for o in ops]


_A_TERMS = ((0, 3, 1), (2, 3, 1), (0, None, 0), (3, None, 0), (0, 1, 1), (2, 0, -1), (1, 3, -1))
_B_TERMS = ((0, 3, 1), (0, None, 0), (1, 3, -1), (2, 0, -1), (3, None, 0), (0, 1, 1), (2, 3, 1))


def _strassen2_ops(block, terms, inner, clock, emit):
    for n1, (x, y, sign) in enumerate(terms):
        sub = []
        for q in range(4):
            v = block(x, q)
            if q in (0, 3):
                v = _tie(v, clock(n1))
            if y is not None:
                v = v + block(y, q) if sign > 0 else v - block(y, q)
            sub.append(v)
        for n2, op in enumerate(inner(*sub)):
            emit(7 * n1 + n2, op)


def _strassen_c(m):
    c11 = (m[0] + m[3]) + (m[6] - m[4])
    c12 = m[2] + m[4]
    c21 = m[1] + m[3]
    c22 = (m[0] - m[1]) + (m[2] + m[5])
    return c11, c12, c21, c22


def _stage(raw, stg, c0, nc, clock=None):
    for ht in range(2):
        for dt in range(2):
            v = raw[pl.ds(c0, nc), ht * 8:(ht + 1) * 8, dt * 128:(dt + 1) * 128]
            stg[ht * 2 + dt, _ds(c0 * 4, nc * 4, 8), :] = _tie(_pk(v.reshape(nc * 8, 128)), clock)


def _pair_words(stg, pair, rows):
    ht = lax.shift_right_logical(pair, 2)
    return [stg[ht * 2 + dt, pl.ds(pair & 3, rows, stride=4), :] for dt in range(2)]


def _weight_ops(halves, rows, dtype=bf16):
    r = rows // 2
    return _strassen_b(halves[0][:r], halves[1][:r], halves[0][r:], halves[1][r:], dtype)


def _head_weight_block(stg, h, c0, nc, dt):
    pair = lax.shift_right_logical(h, 1)
    ht = lax.shift_right_logical(pair, 2)
    sh = (16 * (1 - (h & 1))).astype(u32)
    u = stg[ht * 2 + dt, pl.ds(c0 * 4 + (pair & 3), nc, stride=4), :]
    return pltpu.bitcast((u << sh) & jnp.uint32(0xFFFF0000), f32)


class _Clock:
    def __init__(self, never):
        self.never, self.ticks, self.t = never, [], 0

    def stage(self, duration, vals):
        for k, v in enumerate(vals):
            self.ticks.append((self.t + duration * (k + 1) / len(vals), v))
        self.t += duration

    def pacer(self, t0, t1):
        def clocks(k, n):
            want = t0 + (t1 - t0) * k / n
            best = [v for t, v in self.ticks if t <= want]
            return (self.never, best[-1]) if best else None
        return clocks


def _rows8(vals, step=8):
    return [v[r:r + 8, 0:128] for v in vals for r in range(0, v.shape[0], step)]


def _ssm_cmat(craw_s, coef_s, c_s, clocks):
    for r in range(0, M, 16):
        coef = _tie(coef_s[...], clocks(r // 16, M // 16))
        cr, ci = coef[0:1, :M], coef[1:2, :M]
        cp_re, cp_im = _cmul(craw_s[0, r:r + 16, :].astype(f32), craw_s[1, r:r + 16, :].astype(f32), cr, ci)
        c_s[r // 2:r // 2 + 8, :] = _pk(jnp.concatenate(
            [cp_re[:, :PA], -cp_im[:, :PA], cp_re[:, PA:], -cp_im[:, PA:]], axis=1).astype(bf16))


def _ssm_params(vec_s, coef_s, lam_s, col_s, zero_s):
    row = lambda r: r[...].astype(f32).reshape(1, M)
    lre, lim, ldt, dsk, gw = [row(v) for v in vec_s]
    dt = jnp.exp(ldt).astype(bf16).astype(f32)
    mag = jnp.exp(dt * lre)
    ang = dt * lim
    lr, li = mag * jnp.cos(ang), mag * jnp.sin(ang)
    den = lre * lre + lim * lim
    nr = lr - 1.0
    coef_s[...] = jnp.zeros(coef_s.shape, f32)
    coef_s[0:1, 0:M] = 2.0 * ((nr * lre + li * lim) / den)
    coef_s[1:2, 0:M] = 2.0 * ((li * lre - nr * lim) / den)
    zero_s[...] = jnp.zeros(zero_s.shape, f32)

    er = jnp.concatenate([lr, lr[:, PA:]], axis=1)
    ei = jnp.concatenate([li, -li[:, PA:]], axis=1)
    pw = [(er, ei)]
    for _ in range(7):
        pw.append(_cmul(pw[-1][0], pw[-1][1], er, ei))
    sub = lax.broadcasted_iota(jnp.int32, (8, 512), 0)
    for n, d in enumerate((1, 2, 4)):
        lam_s[2 * n] = jnp.where(sub >= d, pw[d - 1][0], 0.0)
        lam_s[2 * n + 1] = jnp.where(sub >= d, pw[d - 1][1], 0.0)
    lcr = jnp.zeros((8, 512), f32)
    lci = jnp.zeros((8, 512), f32)
    for r in range(8):
        lcr = jnp.where(sub == r, pw[r][0], lcr)
        lci = jnp.where(sub == r, pw[r][1], lci)
    lam_s[6] = lcr
    lam_s[7] = lci

    def col(v):
        v = jnp.concatenate([v, jnp.zeros((1, 512 - M), f32)], axis=1)
        return jnp.broadcast_to(v, (128, 512)).T[:M]
    col_s[0] = col(dsk)
    col_s[1] = col(gw)


def _ssm_scan(u_s, t0, carry, lam_s, h_s, clocks):
    car, cai = carry
    out = []
    for b in range(TC // 8):
        u = u_s[_ds(t0 + b * 8, 8, 8), :]
        mixed = u[:, 2 * PA:]
        cols = [u[:, 0:128], u[:, 128:256], u[:, 256:384], mixed]
        hr = jnp.concatenate([_tie(v, clocks(4 * b + n, TC // 2)) for n, v in enumerate(cols)], axis=1)
        hi = jnp.concatenate([u[:, PA:2 * PA], pltpu.roll(mixed, PB, 1)], axis=1)
        for n, d in enumerate((1, 2, 4)):
            sr, si = pltpu.roll(hr, d, 0), pltpu.roll(hi, d, 0)
            tr, ti = _cmul(sr, si, lam_s[2 * n], lam_s[2 * n + 1])
            hr, hi = hr + tr, hi + ti
        tr, ti = _cmul(lam_s[6], lam_s[7], car, cai)
        hr, hi = hr + tr, hi + ti
        car, cai = hr[7:8, :], hi[7:8, :]
        out.append(jnp.concatenate([hr[:, :PA], hi[:, :PA], hr[:, PA:]], axis=1))
        if b % 2 == 1:
            h_s[(b // 2) * 8:(b // 2 + 1) * 8, :] = _pk(jnp.concatenate(out, axis=0).astype(bf16))
            out = []
    return car, cai


def _kernel(xT_hbm, bre_hbm, bim_hbm, cre_hbm, cim_hbm, lre_hbm, lim_hbm, ldt_hbm,
            dsk_hbm, gw_hbm, woT_hbm, ckv_hbm, wq_hbm, wk_hbm, wv_hbm,
            out_hbm,
            xT_s, v0, v1, v2, v3, v4, b_s, craw_s, c_s, coef_s, lam_s, col_s, u_s, g_s,
            ckv_s, rq, rk, rv, sq, sk, sv, a_s, xa_s, q_s, wo_s,
            ka_s, va_s, pb_s, o_s, s_s, h_s, zero_s, wl_s, cl_s, wk_s, wv_s,
            wkt_s, wvt_s, mk_s, mv_s, kt_s, sem):
    h = pl.program_id(0)
    vec_s = (v0, v1, v2, v3, v4)
    a_s, xa_s, q_s = _Stack(a_s, S // 4), _Stack(xa_s, HM), _Stack(q_s, D)
    ka_s, va_s, pb_s = _Stack(ka_s, S // 2, True), _Stack(va_s, HD), _Stack(pb_s, S // 2, True)
    wk_s, wv_s = _Stack(wk_s, QD), _Stack(wv_s, QD)
    wl_s, cl_s = _Stack(wl_s, HM, True), _Stack(cl_s, HD, True)

    def slice_copies(i):
        s = sem.at[SEM_SL + i]
        grp = i // 2 if isinstance(i, int) else lax.shift_right_logical(i, 1)
        cs = pl.ds(i * CS, CS)
        return [pltpu.make_async_copy(ckv_hbm.at[grp, :, i & 1], ckv_s.at[grp, :, i & 1], s),
                pltpu.make_async_copy(wk_hbm.at[cs], rk.at[cs], s),
                pltpu.make_async_copy(wv_hbm.at[cs], rv.at[cs], s)]

    def x_copy(i):
        cols = _ds(i * TA, TA, TA)
        return pltpu.make_async_copy(xT_hbm.at[:, cols], xT_s.at[:, cols], sem.at[SEM_X + i])

    def out_copy(jp):
        cols = pl.ds(jp * 2 * T, 2 * T)
        return pltpu.make_async_copy(o_s.at[:, cols], out_hbm.at[:, cols], sem.at[SEM_OUT])

    def prep_w(stg, hh, wt_s, w_s, clocks):
        for c0 in range(0, DC, T):
            for dt in range(2):
                blk = _tie(_head_weight_block(stg, hh, c0, T, dt), clocks(2 * c0 // T + dt, 16 + 56))
                wt_s[dt * HD:(dt + 1) * HD, c0:c0 + T] = blk.T
        k = 0
        for r in range(0, QD, 16):
            for u in range(0, QC, T):
                def block(o, q):
                    row = (o % 2) * HD + (q % 2) * QD + r
                    col = (o // 2) * 2 * QC + (q // 2) * QC + u
                    return wt_s[row:row + 16, col:col + T]
                _strassen2_ops(block, _B_TERMS, _strassen_b, lambda n1: clocks(16 + 7 * k + n1, 16 + 56),
                               lambda n, op: w_s.put(n, r, op, pl.ds(u, T)))
                k += 1

    @pl.when(h == 0)
    def _():
        cp_vec = [pltpu.make_async_copy(src, dst, sem.at[SEM_VEC])
                  for src, dst in zip((lre_hbm, lim_hbm, ldt_hbm, dsk_hbm, gw_hbm), vec_s)]
        cp_b = [pltpu.make_async_copy(src.at[pl.ds(lo, n)], b_s.at[pl.ds(dst, n)], sem.at[SEM_B])
                for src, lo, n, dst in ((bre_hbm, 0, PA, 0), (bim_hbm, 0, PA, PA),
                                        (bre_hbm, PA, PB, 2 * PA), (bim_hbm, PA, PB, 2 * PA + PB))]
        cp_wq = [pltpu.make_async_copy(wq_hbm, rq, sem.at[SEM_WQ])]
        cp_c = [pltpu.make_async_copy(src, craw_s.at[n], sem.at[SEM_C])
                for n, src in enumerate((cre_hbm, cim_hbm))]
        cp_wo = pltpu.make_async_copy(woT_hbm, wo_s, sem.at[SEM_WO])
        for cp in cp_vec + cp_b:
            cp.start()
        for i in range(S // TA):
            x_copy(i).start()
        for cp in cp_wq + cp_c:
            cp.start()
        for i in range(NP):
            for cp in slice_copies(i):
                cp.start()
        cp_wo.start()

        def phase1(i):
            x_copy(i).wait()
            u = _dot(xT_s[:, _ds(i * TA, TA, TA)], b_s[...], _TT)
            u_s[_ds(i * TA, TA, TA), :] = u
            never = zero_s[...] != 0.0

            def clocks(k, n):
                pos = (k * 6 * TA // n) // 8 * 8
                return never, u[pos % TA:pos % TA + 8, (pos // TA) * 128:(pos // TA + 1) * 128]

            for t in range(TA // (2 * T)):
                ev = _ds(i * TA + 2 * t * T, T, T)
                od = _ds(i * TA + (2 * t + 1) * T, T, T)
                for r in range(0, HM, 32):
                    top, bot = pl.ds(r, 32), pl.ds(HM + r, 32)
                    clk = clocks(t * 7 + r // 32, 14)
                    ops = _strassen_a(_tie(xT_s[top, ev].astype(f32), clk), xT_s[bot, ev].astype(f32),
                                      xT_s[top, od].astype(f32), _tie(xT_s[bot, od].astype(f32), clk))
                    for n in range(7):
                        xa_s.put(n, r, ops[n], _ds(i * (TA // 2) + t * T, T, T))
            return clocks

        for cp in cp_vec:
            cp.wait()
        _ssm_params(vec_s, coef_s, lam_s, col_s, zero_s)
        for cp in cp_b:
            cp.wait()

        def phase1_body(i, carry):
            phase1(i)
            return carry
        lax.fori_loop(0, S // TA - 1, phase1_body, 0)
        for cp in cp_wq + cp_c:
            cp.wait()
        clocks = phase1(S // TA - 1)
        for c0 in range(0, M, 8):
            _stage(rq, sq, c0, 8, clocks(c0 // 8, M // 8))
        _ssm_cmat(craw_s, coef_s, c_s, clocks)
        zero = jnp.zeros((1, 512), f32)
        carry0 = _ssm_scan(u_s, 0, (zero, zero), lam_s, h_s, clocks)

        def phase2(i, carry):
            for cp in slice_copies(i):
                cp.wait()
            yT = _dot(_up(c_s[...]), _up(h_s[...]), _NT)
            for t in range(TC // T):
                cols = _ds(i * TC + t * T, T, T)
                acc = jnp.zeros((8, T), f32)
                for r in range(0, M, 32):
                    xg = xT_s[r:r + 32, cols].astype(f32) * col_s[1, r:r + 32, :]
                    acc = acc + jnp.sum(xg.reshape(4, 8, T), axis=0)
                g = jax.nn.sigmoid(jnp.sum(acc, axis=0, keepdims=True))
                g_s[:, cols] = g
                for r in range(0, M, 32):
                    skip = xT_s[r:r + 32, cols].astype(f32) * col_s[0, r:r + 32, :]
                    o_s[r:r + 32, cols] = (1.0 - g) * (yT[r:r + 32, t * T:(t + 1) * T] + skip)

            words = _pair_words(sq, i, M)
            lo = _weight_ops([pltpu.bitcast(u << 16, f32) for u in words], M, f32)
            hi = _weight_ops([pltpu.bitcast(u & jnp.uint32(0xFFFF0000), f32) for u in words], M, f32)
            prods = [_dot(jnp.concatenate([lo[n], hi[n]], axis=1).astype(bf16), xa_s.get(n), _TN)
                     for n in range(7)]
            qs = LOG2E * D ** -0.5
            for t in range(NP):
                for r in range(0, D, G):
                    cs = _strassen_c([v[r:r + G, t * T:(t + 1) * T] for v in prods])
                    for n, c in enumerate(cs):
                        q_s.put(4 * i + 2 * (r // HD) + n // 2, (n % 2) * HD + r % HD,
                                (c * qs).astype(bf16), pl.ds(t * T, T))

            never = zero_s[...] != 0.0

            def clocks(k, n):
                pos = (k * 5 * 1024 // n) // 8 * 8
                r, c = pos % 256, (pos % 1024) // 256 * 256
                return never, prods[pos // 1024][r:r + 8, c:c + 128]

            carry = _ssm_scan(u_s, jnp.minimum(i + 1, NP - 1) * TC, carry, lam_s, h_s, clocks)

            for c0 in range(0, CS, 8):
                _stage(rk, sk, i * CS + c0, 8, clocks(c0 // 4, CS // 4))
                _stage(rv, sv, i * CS + c0, 8, clocks(c0 // 4 + 1, CS // 4))
            grp, half = lax.shift_right_logical(i, 1), i & 1
            k = 0
            for r in range(0, T // 2, 16):
                for u in range(0, QC, T):
                    def block(o, q):
                        col = (o % 2) * 2 * QC + (q % 2) * QC + u
                        return ckv_s[grp, 2 * (q // 2) + o // 2, half, r:r + 16, col:col + T].astype(f32)
                    _strassen2_ops(block, _A_TERMS, _strassen_a, lambda n1: clocks(7 * k + n1, 56),
                                   lambda n, op: a_s.put(n, i * (T // 2) + r, op, pl.ds(u, T)))
                    k += 1
            return carry

        lax.fori_loop(0, NP, phase2, carry0)
        cp_wo.wait()
        prep_w(sk, h, wkt_s, wk_s, lambda k, n: None)
        wl_s.ref[...] = jnp.zeros(wl_s.ref.shape, u32)
        cl_s.ref[...] = jnp.zeros(cl_s.ref.shape, u32)

    clk = _Clock(zero_s[...] != 0.0)

    def oproj(jp, ops):
        m = [_dot(wl_s.get(i), ops[i], _NN) for i in range(7)]
        for r in range(0, HM, G):
            for n, c in enumerate(_strassen_c([v[r:r + G] for v in m])):
                o_s[pl.ds((n // 2) * HM + r, G), pl.ds((2 * jp + n % 2) * T, T)] += c
        clk.stage(392, _rows8([m[0], m[4]]))

    def prep_wo(clocks):
        for r in range(0, HM, G):
            top = _tie(wo_s[h, r:r + G, :].astype(f32), clocks(r // G, HM // G))
            bot = _tie(wo_s[h, HM + r:HM + r + G, :].astype(f32), clocks(r // G, HM // G))
            for n, w in enumerate(_strassen_a(top[:, :HD], top[:, HD:], bot[:, :HD], bot[:, HD:])):
                wl_s.put(n, r, w)

    def proj(g, w_s, m_s):
        for n1 in range(7):
            m = [_dot(w_s.get(7 * n1 + n), a_s.get(7 * n1 + n, g * T, T), _NT) for n in range(7)]
            for r in range(0, QD, G):
                for n, c in enumerate(_strassen_c([v[r:r + G] for v in m])):
                    row = n1 * HD + (n % 2) * QD + r
                    m_s[row:row + G, (n // 2) * T:(n // 2 + 1) * T] = c
            clk.stage(224, _rows8(m, 16))

    def outer(m_s, r, nr, a2):
        return _strassen_c([m_s[n * HD + r:n * HD + r + nr, a2 * T:(a2 + 1) * T] for n in range(7)])

    def nine(c11, c12, c21, c22):
        return _strassen_a(c11, c12, c21, c22) + [c12.astype(bf16), c21.astype(bf16)]

    def kproj(g):
        proj(g, wk_s, mk_s)
        for a2 in range(2):
            cs = [outer(mk_s, r, G, a2) for r in range(0, HD, G)]
            for n in range(4):
                kt_s[:, (a2 * 4 + n) * T:(a2 * 4 + n + 1) * T] = jnp.concatenate([c[n] for c in cs], axis=0).T
            for r in range(0, T, G):
                blk = [kt_s[r:r + G, (a2 * 4 + n) * T:(a2 * 4 + n + 1) * T] for n in range(4)]
                for n, op in enumerate(nine(*blk)):
                    ka_s.put(n, (2 * g + a2) * T + r, op)

    def vproj(g):
        proj(g, wv_s, mv_s)
        for a2 in range(2):
            for r in range(0, HD, G):
                c11, c21, c12, c22 = outer(mv_s, r, G, a2)
                for n, op in enumerate(nine(c11, c12, c21, c22)):
                    va_s.put(n, r, op, pl.ds((2 * g + a2) * T, T))

    key = lax.broadcasted_iota(jnp.int32, (T, T), 0)
    qry = lax.broadcasted_iota(jnp.int32, (T, T), 1)
    causal = key <= qry

    class Reducer:
        def __init__(self, red, comb):
            self.red, self.comb, self.acc, self.rows, self.out = red, comb, None, 0, None

        def add(self, v):
            v = self.red(v.reshape(v.shape[0] // 8, 8, T), axis=0)
            self.acc = v if self.acc is None else self.comb(self.acc, v)
            self.rows += 1
            if self.rows * G >= RCH:
                self.flush()

        def flush(self):
            if self.acc is not None:
                v = self.red(self.acc, axis=0, keepdims=True)
                self.out = v if self.out is None else self.comb(self.out, v)
            self.acc, self.rows = None, 0

        def result(self):
            self.flush()
            return self.out

    def qk(jp):
        R, slot = jp * T, jp % 2
        cols = pl.ds(jp * T, T)
        qe, qo = q_s.get(2 * h, cols=cols), q_s.get(2 * h + 1, cols=cols)
        mx = [Reducer(jnp.max, jnp.maximum) for _ in range(2)]

        def put(e, row, v):
            s_s[slot, e, row:row + G, :] = v
            mx[e].add(v)

        if jp > 0:
            qef, qof = qe.astype(f32), qo.astype(f32)
            qb = _strassen_b(qef[:HD], qof[:HD], qef[HD:], qof[HD:])
            for r0 in range(0, R, QCH):
                r1 = min(r0 + QCH, R)
                m = [_dot(ka_s.get(n, r0, r1 - r0), qb[n], _NN) for n in range(7)]
                for r in range(0, r1 - r0, G):
                    c11, c12, c21, c22 = _strassen_c([v[r:r + G] for v in m])
                    put(0, r0 + r, c11)
                    put(1, r0 + r, c12)
                    put(0, R + r0 + r, c21)
                    put(1, R + r0 + r, c22)
                clk.stage(7 * (r1 - r0) / 4, _rows8([m[0], m[4]]))
        ke = jnp.concatenate([ka_s.get(2, R, T), ka_s.get(7, R, T)], axis=1)
        ko = jnp.concatenate([ka_s.get(8, R, T), ka_s.get(3, R, T)], axis=1)
        se = _dot(ke, jnp.concatenate([qe, qo], axis=1), _NN)
        so = _dot(ko, qo, _NN)
        for r in range(0, T, G):
            put(0, 2 * R + r, jnp.where(causal[r:r + G], se[r:r + G, :T], -1e30))
            put(1, 2 * R + r, se[r:r + G, T:])
            put(1, 2 * R + T + r, jnp.where(causal[r:r + G], so[r:r + G], -1e30))
        clk.stage(192, _rows8([se]))
        return [jnp.broadcast_to(x.result(), (8, T)) for x in mx]

    def shifted_exp(slot, e, row, z):
        v = s_s[slot, e, row:row + G, :].reshape(G // 8, 8, T) - z[None]
        return jnp.exp2(v).reshape(G, T)

    def softmax(jp, mx, t0, t1, t2=None, t3=None):
        R, slot = jp * T, jp % 2
        if t2 is None:
            t1, t2, t3 = (t0 + t1) / 2, (t0 + t1) / 2, t1
        clocks = clk.pacer(t0, t1)
        k, n = 0, (4 * jp + 3) * T // G
        z = []
        for e in range(2):
            sm = Reducer(jnp.sum, jnp.add)
            for r in range(0, (2 * jp + 1 + e) * T, G):
                sm.add(shifted_exp(slot, e, r, _tie(mx[e], clocks(k, n))))
                k += 1
            z.append(mx[e] + jnp.log2(sm.result()))
        clocks = clk.pacer(t2, t3)
        k = 0
        for r in range(0, R, G):
            ze, zo = _tie(z[0], clocks(k, n)), _tie(z[1], clocks(k + 2, n))
            ops = _strassen_b(shifted_exp(slot, 0, r, ze), shifted_exp(slot, 1, r, zo),
                              shifted_exp(slot, 0, R + r, ze), shifted_exp(slot, 1, R + r, zo))
            for i in range(7):
                pb_s.put(slot * 8 + i, r, ops[i])
            k += 4
        for r in range(0, 3 * T, G):
            e = int(r >= T)
            p = shifted_exp(slot, e, 2 * R + r - e * T, _tie(z[e], clocks(k, n)))
            pb_s.put(slot * 8 + 7, r, p.astype(bf16))
            k += 1

    def pv(jp):
        R, slot = jp * T, jp % 2
        if jp > 0:
            m = [_dot(va_s.get(n, cols=pl.ds(0, R)), pb_s.get(slot * 8 + n, 0, R), _NN) for n in range(7)]
            clk.stage(7 * R / 4, _rows8(m, 32))
        cols = pl.ds(R, T)
        ve = jnp.concatenate([va_s.get(2, cols=cols), va_s.get(8, cols=cols)], axis=0)
        vo = jnp.concatenate([va_s.get(7, cols=cols), va_s.get(3, cols=cols)], axis=0)
        ce = _dot(ve, pb_s.get(slot * 8 + 7, 0, T), _NN)
        co = _dot(jnp.concatenate([ve, vo], axis=1), pb_s.get(slot * 8 + 7, T, 2 * T), _NN)
        clk.stage(192, _rows8([ce], 32))
        ge = g_s[:, 2 * jp * T:(2 * jp + 1) * T]
        go = g_s[:, (2 * jp + 1) * T:(2 * jp + 2) * T]
        for r in range(0, HD, G):
            c = [ce[r:r + G], co[r:r + G], ce[HD + r:HD + r + G], co[HD + r:HD + r + G]]
            if jp > 0:
                c = [x + y for x, y in zip(c, _strassen_c([v[r:r + G] for v in m]))]
            ops = _strassen_b(c[0] * ge, c[1] * go, c[2] * ge, c[3] * go)
            for n in range(7):
                cl_s.put(slot * 7 + n, r, ops[n])

    def ctx_ops(jp):
        return [cl_s.get((jp % 2) * 7 + n) for n in range(7)]

    def oproj_out(jp):
        oproj(jp, ctx_ops(jp))

        @pl.when(h == H - 1)
        def _():
            out_copy(jp).start()

    kproj(0)
    prep_w(sv, h, wvt_s, wv_s, clk.pacer(0, clk.t - 200))
    oproj(NP - 1, ctx_ops(NP - 1))
    mx = qk(0)
    t0 = clk.t
    vproj(0)
    softmax(0, mx, t0, clk.t - SLACK)
    prep_wo(clk.pacer(t0, clk.t))
    for jp in range(NP - 2):
        mx = qk(jp + 1)
        t0 = clk.t
        if jp % 2 == 0:
            kproj(jp // 2 + 1)
        elif jp < NP - 3:
            vproj(jp // 2 + 1)
        pv(jp)
        if jp > 0:
            oproj_out(jp - 1)
        if jp < NP - 3:
            softmax(jp + 1, mx, t0, clk.t - SLACK)
    t1 = clk.t
    mx7 = qk(NP - 1)
    t2 = clk.t
    vproj(NP // 2 - 1)
    t3 = clk.t
    softmax(NP - 2, mx, t0, t1, t2, t3 - SLACK - 300)
    pv(NP - 2)
    oproj_out(NP - 3)
    softmax(NP - 1, mx7, t3 - 500, clk.t - SLACK)
    t0 = clk.t
    pv(NP - 1)
    oproj_out(NP - 2)
    prep_w(sk, jnp.minimum(h + 1, H - 1), wkt_s, wk_s, clk.pacer(t0 - 200, clk.t - 400))

    @pl.when(h == H - 1)
    def _():
        oproj(NP - 1, ctx_ops(NP - 1))
        out_copy(NP - 1).start()
        for jp in range(NP):
            out_copy(jp).wait()


@jax.jit
def pallas_gated_mix__compressed_kv_cla__ssm_conv_s5__prompt_kernel(
    A_x: jax.Array,
    A_c_kv: jax.Array,
    A_w_q: jax.Array,
    A_w_uk: jax.Array,
    A_w_uv: jax.Array,
    A_w_o: jax.Array,
    B_x: jax.Array,
    B_Lambda_re: jax.Array,
    B_Lambda_im: jax.Array,
    B_B_re: jax.Array,
    B_B_im: jax.Array,
    B_C_re: jax.Array,
    B_C_im: jax.Array,
    B_log_dt: jax.Array,
    B_Dskip: jax.Array,
    gate_w: jax.Array,
):
    del B_x
    xT = jnp.transpose(A_x[0])
    woT = jnp.transpose(A_w_o, (0, 2, 1))
    ckv = A_c_kv.reshape(4, 4, 2, T // 2, DC)

    hbm = pl.BlockSpec(memory_space=pl.ANY)
    vmem = pltpu.VMEM
    outT = pl.pallas_call(
        _kernel,
        grid=(H,),
        in_specs=[hbm] * 15,
        out_specs=hbm,
        out_shape=jax.ShapeDtypeStruct((M, S), f32),
        scratch_shapes=[
            vmem((M, S), bf16),
            vmem((M,), bf16), vmem((M,), bf16), vmem((M,), bf16), vmem((M,), bf16), vmem((M,), bf16),
            vmem((2 * M, M), bf16),
            vmem((2, M, M), bf16),
            vmem((M // 2, 2 * M), u32),
            vmem((8, 512), f32),
            vmem((8, 8, 512), f32),
            vmem((2, M, 128), f32),
            vmem((S, 2 * M), f32),
            vmem((1, S), f32),
            vmem((4, 4, 2, T // 2, DC), bf16),
            vmem((M, H, D), bf16),
            vmem((DC, H, D), bf16),
            vmem((DC, H, D), bf16),
            vmem((4, M * 4, 128), u32),
            vmem((4, DC * 4, 128), u32),
            vmem((4, DC * 4, 128), u32),
            vmem((49 * S // 8, QC), u32),
            vmem((7 * HM // 2, S // 2), u32),
            vmem((H * D, S // 2), u32),
            vmem((H, M, D), bf16),
            vmem((S // 4, 9 * HD), u32),
            vmem((9 * HD // 2, S // 2), u32),
            vmem((S // 4, 16 * T), u32),
            vmem((M, S), f32),
            vmem((2, 2, S, T), f32),
            vmem((TC // 2, 2 * M), u32),
            vmem((8, 128), f32),
            vmem((HM // 2, 7 * HD), u32),
            vmem((HD // 2, 14 * T), u32),
            vmem((49 * QD // 2, QC), u32),
            vmem((49 * QD // 2, QC), u32),
            vmem((D, DC), f32),
            vmem((D, DC), f32),
            vmem((7 * HD, 2 * T), f32),
            vmem((7 * HD, 2 * T), f32),
            vmem((T, 8 * T), f32),
            pltpu.SemaphoreType.DMA((NSEM,)),
        ],
        compiler_params=pltpu.CompilerParams(
            dimension_semantics=("arbitrary",),
            vmem_limit_bytes=126 * 1024 * 1024,
        ),
    )(xT, B_B_re, B_B_im, B_C_re, B_C_im, B_Lambda_re, B_Lambda_im, B_log_dt,
      B_Dskip, gate_w, woT, ckv, A_w_q, A_w_uk, A_w_uv)
    return jnp.transpose(outT)[None]
```

```python
import jax
import jax.numpy as jnp
from jax import lax
import jax.experimental.pallas as pl
import jax.experimental.pallas.tpu as pltpu

S = 2048
M = 448
H = 16
D = 256
DC = 1024
T = 128
NT = S // T
NP = NT // 2
HD = D // 2
HM = M // 2
QD = D // 4
QC = DC // 4
PA = 384
PB = M - PA
TA = 512
TC = 256
CS = DC // NP
NRAW = 4
import os
G = int(os.environ.get('G', 32))
RCH = int(os.environ.get('RCH', 512))
QCH = int(os.environ.get('QCH', 1024))
SLACK = int(os.environ.get('SLACK', 200))
PW0 = int(os.environ.get('PW0', 100))
PLAN = os.environ.get('PLAN', 'K104,K147,K203,K237,K304 P0 P1,K347 P2 O0,P3 O1 P4 O2 O3,P5 O4 P6 O5').split(',')
LOG2E = 1.4426950408889634

f32 = jnp.float32
bf16 = jnp.bfloat16
u32 = jnp.uint32

SEM_VEC, SEM_B, SEM_X, SEM_WQ, SEM_C, SEM_SL, SEM_WO, SEM_OUT = 0, 1, 2, 6, 7, 8, 16, 17
NSEM = 18


def _dot(a, b, dims):
    return lax.dot_general(a, b, (dims, ((), ())), preferred_element_type=f32)


_NN = ((1,), (0,))
_NT = ((1,), (1,))
_TN = ((0,), (0,))
_TT = ((0,), (1,))


def _pk(x):
    return pltpu.bitcast(x, u32)


def _up(x):
    return pltpu.bitcast(x, bf16)


class _Stack:
    def __init__(self, ref, rows, along_lanes=False):
        self.ref, self.rows, self.along_lanes = ref, rows, along_lanes

    def _idx(self, n, r0, nr, cols):
        lo = r0 // 2 if isinstance(r0, int) else lax.shift_right_logical(r0, 1)
        nr = (self.rows if nr is None else nr) // 2
        if self.along_lanes:
            return _ds(lo, nr, 8), pl.ds(n * 128, 128)
        return _ds(n * (self.rows // 2) + lo, nr, 8), (slice(None) if cols is None else cols)

    def get(self, n, r0=0, nr=None, cols=None):
        return _up(self.ref[self._idx(n, r0, nr, cols)])

    def put(self, n, r0, x, cols=None):
        self.ref[self._idx(n, r0, x.shape[0], cols)] = _pk(x)


def _tie(x, clock):
    if clock is None:
        return x
    never, tick = clock
    r, c = x.shape
    if tick.dtype != x.dtype:
        tick = pltpu.bitcast(tick, x.dtype)
    tile = lambda v: jnp.tile(v, (r // 8, c // 128))
    return jnp.where(tile(never), tile(tick), x)


def _cmul(ar, ai, br, bi):
    return ar * br - ai * bi, ar * bi + ai * br


def _ds(lo, n, align):
    return pl.ds(lo if isinstance(lo, int) else pl.multiple_of(lo, align), n)


def _strassen_a(a11, a12, a21, a22):
    ops = [a11 + a22, a21 + a22, a11, a22, a11 + a12, a21 - a11, a12 - a22]
    return [o.astype(bf16) for o in ops]


def _strassen_b(b11, b12, b21, b22, dtype=bf16):
    ops = [b11 + b22, b11, b12 - b22, b21 - b11, b22, b11 + b12, b21 + b22]
    return [o.astype(dtype) for o in ops]


_A_TERMS = ((0, 3, 1), (2, 3, 1), (0, None, 0), (3, None, 0), (0, 1, 1), (2, 0, -1), (1, 3, -1))
_B_TERMS = ((0, 3, 1), (0, None, 0), (1, 3, -1), (2, 0, -1), (3, None, 0), (0, 1, 1), (2, 3, 1))


def _strassen2_ops(block, terms, inner, clock, emit):
    for n1, (x, y, sign) in enumerate(terms):
        sub = []
        for q in range(4):
            v = block(x, q)
            if q in (0, 3):
                v = _tie(v, clock(n1))
            if y is not None:
                v = v + block(y, q) if sign > 0 else v - block(y, q)
            sub.append(v)
        for n2, op in enumerate(inner(*sub)):
            emit(7 * n1 + n2, op)


def _strassen_c(m):
    c11 = (m[0] + m[3]) + (m[6] - m[4])
    c12 = m[2] + m[4]
    c21 = m[1] + m[3]
    c22 = (m[0] - m[1]) + (m[2] + m[5])
    return c11, c12, c21, c22


def _stage(raw, r0, stg, c0, nc, clock=None):
    for ht in range(2):
        for dt in range(2):
            v = raw[pl.ds(r0, nc), ht * 8:(ht + 1) * 8, dt * 128:(dt + 1) * 128]
            stg[ht * 2 + dt, _ds(c0 * 4, nc * 4, 8), :] = _tie(_pk(v.reshape(nc * 8, 128)), clock)


def _pair_words(stg, pair, rows):
    ht = lax.shift_right_logical(pair, 2)
    return [stg[ht * 2 + dt, pl.ds(pair & 3, rows, stride=4), :] for dt in range(2)]


def _weight_ops(halves, rows, dtype=bf16):
    r = rows // 2
    return _strassen_b(halves[0][:r], halves[1][:r], halves[0][r:], halves[1][r:], dtype)


class _Clock:
    def __init__(self, never):
        self.never, self.ticks, self.t = never, [], 0

    def stage(self, duration, vals):
        for k, v in enumerate(vals):
            self.ticks.append((self.t + duration * (k + 1) / len(vals), v))
        self.t += duration

    def pacer(self, t0, t1):
        def clocks(k, n):
            want = t0 + (t1 - t0) * k / n
            best = [v for t, v in self.ticks if t <= want]
            return (self.never, best[-1]) if best else None
        return clocks


def _rows8(vals, step=8):
    return [v[r:r + 8, 0:128] for v in vals for r in range(0, v.shape[0], step)]


def _ssm_cmat(craw_s, coef_s, c_s, clocks):
    for r in range(0, M, 16):
        coef = _tie(coef_s[...], clocks(r // 16, M // 16))
        cr, ci = coef[0:1, :M], coef[1:2, :M]
        cp_re, cp_im = _cmul(craw_s[0, r:r + 16, :].astype(f32), craw_s[1, r:r + 16, :].astype(f32), cr, ci)
        c_s[r // 2:r // 2 + 8, :] = _pk(jnp.concatenate(
            [cp_re[:, :PA], -cp_im[:, :PA], cp_re[:, PA:], -cp_im[:, PA:]], axis=1).astype(bf16))


def _ssm_params(vec_s, coef_s, lam_s, col_s, zero_s):
    row = lambda r: r[...].astype(f32).reshape(1, M)
    lre, lim, ldt, dsk, gw = [row(v) for v in vec_s]
    dt = jnp.exp(ldt).astype(bf16).astype(f32)
    mag = jnp.exp(dt * lre)
    ang = dt * lim
    lr, li = mag * jnp.cos(ang), mag * jnp.sin(ang)
    den = lre * lre + lim * lim
    nr = lr - 1.0
    coef_s[...] = jnp.zeros(coef_s.shape, f32)
    coef_s[0:1, 0:M] = 2.0 * ((nr * lre + li * lim) / den)
    coef_s[1:2, 0:M] = 2.0 * ((li * lre - nr * lim) / den)
    zero_s[...] = jnp.zeros(zero_s.shape, f32)

    er = jnp.concatenate([lr, lr[:, PA:]], axis=1)
    ei = jnp.concatenate([li, -li[:, PA:]], axis=1)
    pw = [(er, ei)]
    for _ in range(7):
        pw.append(_cmul(pw[-1][0], pw[-1][1], er, ei))
    sub = lax.broadcasted_iota(jnp.int32, (8, 512), 0)
    for n, d in enumerate((1, 2, 4)):
        lam_s[2 * n] = jnp.where(sub >= d, pw[d - 1][0], 0.0)
        lam_s[2 * n + 1] = jnp.where(sub >= d, pw[d - 1][1], 0.0)
    lcr = jnp.zeros((8, 512), f32)
    lci = jnp.zeros((8, 512), f32)
    for r in range(8):
        lcr = jnp.where(sub == r, pw[r][0], lcr)
        lci = jnp.where(sub == r, pw[r][1], lci)
    lam_s[6] = lcr
    lam_s[7] = lci

    def col(v):
        v = jnp.concatenate([v, jnp.zeros((1, 512 - M), f32)], axis=1)
        return jnp.broadcast_to(v, (128, 512)).T[:M]
    col_s[0] = col(dsk)
    col_s[1] = col(gw)


def _ssm_scan(u_s, t0, carry, lam_s, h_s, clocks):
    car, cai = carry
    out = []
    for b in range(TC // 8):
        u = u_s[_ds(t0 + b * 8, 8, 8), :]
        mixed = u[:, 2 * PA:]
        cols = [u[:, 0:128], u[:, 128:256], u[:, 256:384], mixed]
        hr = jnp.concatenate([_tie(v, clocks(4 * b + n, TC // 2)) for n, v in enumerate(cols)], axis=1)
        hi = jnp.concatenate([u[:, PA:2 * PA], pltpu.roll(mixed, PB, 1)], axis=1)
        for n, d in enumerate((1, 2, 4)):
            sr, si = pltpu.roll(hr, d, 0), pltpu.roll(hi, d, 0)
            tr, ti = _cmul(sr, si, lam_s[2 * n], lam_s[2 * n + 1])
            hr, hi = hr + tr, hi + ti
        tr, ti = _cmul(lam_s[6], lam_s[7], car, cai)
        hr, hi = hr + tr, hi + ti
        car, cai = hr[7:8, :], hi[7:8, :]
        out.append(jnp.concatenate([hr[:, :PA], hi[:, :PA], hr[:, PA:]], axis=1))
        if b % 2 == 1:
            h_s[(b // 2) * 8:(b // 2 + 1) * 8, :] = _pk(jnp.concatenate(out, axis=0).astype(bf16))
            out = []
    return car, cai


def _kernel(xT_hbm, bre_hbm, bim_hbm, cre_hbm, cim_hbm, lre_hbm, lim_hbm, ldt_hbm,
            dsk_hbm, gw_hbm, woT_hbm, ckv_hbm, wq_hbm, wk_hbm, wv_hbm,
            out_hbm,
            xT_s, v0, v1, v2, v3, v4, b_s, craw_s, c_s, coef_s, lam_s, col_s, u_s, g_s,
            ckv_s, rq, rk, rv, sq, sk, sv, a_s, xa_s, q_s, wo_s,
            ka_s, va_s, pb_s, o_s, s_s, h_s, zero_s, wl_s, cl_s, w_s,
            wkt_s, wvt_s, mk_s, mv_s, kt_s, sem):
    h = pl.program_id(0)
    vec_s = (v0, v1, v2, v3, v4)
    a_s, xa_s, q_s = _Stack(a_s, S // 4), _Stack(xa_s, HM), _Stack(q_s, D)
    ka_s, va_s, pb_s = _Stack(ka_s, S // 2, True), _Stack(va_s, HD), _Stack(pb_s, S // 2, True)
    w_s = _Stack(w_s, 2 * QD)
    wl_s, cl_s = _Stack(wl_s, HM, True), _Stack(cl_s, HD, True)

    def slice_copies(i):
        s = sem.at[SEM_SL + i]
        grp = i // 2 if isinstance(i, int) else lax.shift_right_logical(i, 1)
        cs, dst = pl.ds(i * CS, CS), pl.ds((i & (NRAW - 1)) * CS, CS)
        return [pltpu.make_async_copy(ckv_hbm.at[grp, :, i & 1], ckv_s.at[grp, :, i & 1], s),
                pltpu.make_async_copy(wk_hbm.at[cs], rk.at[dst], s),
                pltpu.make_async_copy(wv_hbm.at[cs], rv.at[dst], s)]

    def x_copy(i):
        cols = _ds(i * TA, TA, TA)
        return pltpu.make_async_copy(xT_hbm.at[:, cols], xT_s.at[:, cols], sem.at[SEM_X + i])

    def out_copy(jp):
        cols = pl.ds(jp * 2 * T, 2 * T)
        return pltpu.make_async_copy(o_s.at[:, cols], out_hbm.at[:, cols], sem.at[SEM_OUT])

    def prep_w(hh, clocks):
        base = lax.shift_right_logical(hh, 1) * D
        sh = (16 * (1 - (hh & 1))).astype(u32)
        k = 0
        for row0, wt_s in ((0, wkt_s), (QD, wvt_s)):
            for r in range(0, QD, 16):
                for u in range(0, QC, T):
                    def block(o, q):
                        row = (o % 2) * HD + (q % 2) * QD + r
                        col = (o // 2) * 2 * QC + (q // 2) * QC + u
                        w = wt_s[_ds(base + row, 16, 16), col:col + T]
                        return pltpu.bitcast((w << sh) & jnp.uint32(0xFFFF0000), f32)
                    _strassen2_ops(block, _B_TERMS, _strassen_b, lambda n1: clocks(7 * k + n1, 112),
                                   lambda n, op: w_s.put(n, row0 + r, op, pl.ds(u, T)))
                    k += 1

    @pl.when(h == 0)
    def _():
        cp_vec = [pltpu.make_async_copy(src, dst, sem.at[SEM_VEC])
                  for src, dst in zip((lre_hbm, lim_hbm, ldt_hbm, dsk_hbm, gw_hbm), vec_s)]
        cp_b = [pltpu.make_async_copy(src.at[pl.ds(lo, n)], b_s.at[pl.ds(dst, n)], sem.at[SEM_B])
                for src, lo, n, dst in ((bre_hbm, 0, PA, 0), (bim_hbm, 0, PA, PA),
                                        (bre_hbm, PA, PB, 2 * PA), (bim_hbm, PA, PB, 2 * PA + PB))]
        cp_wq = [pltpu.make_async_copy(wq_hbm, rq, sem.at[SEM_WQ])]
        cp_c = [pltpu.make_async_copy(src, craw_s.at[n], sem.at[SEM_C])
                for n, src in enumerate((cre_hbm, cim_hbm))]
        cp_wo = pltpu.make_async_copy(woT_hbm, wo_s, sem.at[SEM_WO])
        for cp in cp_vec + cp_b:
            cp.start()
        for i in range(S // TA):
            x_copy(i).start()
        for cp in cp_wq + cp_c:
            cp.start()
        for i in range(NRAW - 1):
            for cp in slice_copies(i):
                cp.start()
        cp_wo.start()

        def phase1(i):
            x_copy(i).wait()
            u = _dot(xT_s[:, _ds(i * TA, TA, TA)], b_s[...], _TT)
            u_s[_ds(i * TA, TA, TA), :] = u
            never = zero_s[...] != 0.0

            def clocks(k, n):
                pos = (k * 6 * TA // n) // 8 * 8
                return never, u[pos % TA:pos % TA + 8, (pos // TA) * 128:(pos // TA + 1) * 128]

            for t in range(TA // (2 * T)):
                ev = _ds(i * TA + 2 * t * T, T, T)
                od = _ds(i * TA + (2 * t + 1) * T, T, T)
                for r in range(0, HM, 32):
                    top, bot = pl.ds(r, 32), pl.ds(HM + r, 32)
                    clk = clocks(t * 7 + r // 32, 14)
                    ops = _strassen_a(_tie(xT_s[top, ev].astype(f32), clk), xT_s[bot, ev].astype(f32),
                                      xT_s[top, od].astype(f32), _tie(xT_s[bot, od].astype(f32), clk))
                    for n in range(7):
                        xa_s.put(n, r, ops[n], _ds(i * (TA // 2) + t * T, T, T))
            return clocks

        for cp in cp_vec:
            cp.wait()
        _ssm_params(vec_s, coef_s, lam_s, col_s, zero_s)
        for cp in cp_b:
            cp.wait()

        def phase1_body(i, carry):
            phase1(i)
            return carry
        lax.fori_loop(0, S // TA - 1, phase1_body, 0)
        for cp in cp_wq + cp_c:
            cp.wait()
        clocks = phase1(S // TA - 1)
        for c0 in range(0, M, 8):
            _stage(rq, c0, sq, c0, 8, clocks(c0 // 8, M // 8))
        _ssm_cmat(craw_s, coef_s, c_s, clocks)
        zero = jnp.zeros((1, 512), f32)
        carry0 = _ssm_scan(u_s, 0, (zero, zero), lam_s, h_s, clocks)

        def phase2(i, carry):
            @pl.when(i + NRAW - 1 < NP)
            def _():
                for cp in slice_copies(i + NRAW - 1):
                    cp.start()

            for cp in slice_copies(i):
                cp.wait()
            yT = _dot(_up(c_s[...]), _up(h_s[...]), _NT)
            for t in range(TC // T):
                cols = _ds(i * TC + t * T, T, T)
                acc = jnp.zeros((8, T), f32)
                for r in range(0, M, 32):
                    xg = xT_s[r:r + 32, cols].astype(f32) * col_s[1, r:r + 32, :]
                    acc = acc + jnp.sum(xg.reshape(4, 8, T), axis=0)
                g = jax.nn.sigmoid(jnp.sum(acc, axis=0, keepdims=True))
                g_s[:, cols] = g
                for r in range(0, M, 32):
                    skip = xT_s[r:r + 32, cols].astype(f32) * col_s[0, r:r + 32, :]
                    o_s[r:r + 32, cols] = (1.0 - g) * (yT[r:r + 32, t * T:(t + 1) * T] + skip)

            words = _pair_words(sq, i, M)
            lo = _weight_ops([pltpu.bitcast(u << 16, f32) for u in words], M, f32)
            hi = _weight_ops([pltpu.bitcast(u & jnp.uint32(0xFFFF0000), f32) for u in words], M, f32)
            prods = [_dot(jnp.concatenate([lo[n], hi[n]], axis=1).astype(bf16), xa_s.get(n), _TN)
                     for n in range(7)]
            qs = LOG2E * D ** -0.5
            for t in range(NP):
                for r in range(0, D, G):
                    cs = _strassen_c([v[r:r + G, t * T:(t + 1) * T] for v in prods])
                    for n, c in enumerate(cs):
                        q_s.put(4 * i + 2 * (r // HD) + n // 2, (n % 2) * HD + r % HD,
                                (c * qs).astype(bf16), pl.ds(t * T, T))

            never = zero_s[...] != 0.0

            def clocks(k, n):
                pos = (k * 5 * 1024 // n) // 8 * 8
                r, c = pos % 256, (pos % 1024) // 256 * 256
                return never, prods[pos // 1024][r:r + 8, c:c + 128]

            carry = _ssm_scan(u_s, jnp.minimum(i + 1, NP - 1) * TC, carry, lam_s, h_s, clocks)

            for c0 in range(0, CS, 8):
                r0 = (i & (NRAW - 1)) * CS + c0
                _stage(rk, r0, sk, c0, 8, clocks(c0 // 8, 64))
                _stage(rv, r0, sv, c0, 8, clocks(16 + c0 // 8, 64))
            for n, (stg, wt_s) in enumerate(((sk, wkt_s), (sv, wvt_s))):
                for pair in range(H // 2):
                    for dt in range(2):
                        blk = stg[(pair // 4) * 2 + dt, pl.ds(pair % 4, CS, stride=4), :]
                        blk = _tie(blk, clocks(16 + 24 * n + 3 * pair + dt, 64))
                        wt_s[pair * D + dt * HD:pair * D + (dt + 1) * HD, _ds(i * CS, CS, CS)] = blk.T
            grp, half = lax.shift_right_logical(i, 1), i & 1
            k = 0
            for r in range(0, T // 2, 16):
                for u in range(0, QC, T):
                    def block(o, q):
                        col = (o % 2) * 2 * QC + (q % 2) * QC + u
                        return ckv_s[grp, 2 * (q // 2) + o // 2, half, r:r + 16, col:col + T].astype(f32)
                    _strassen2_ops(block, _A_TERMS, _strassen_a, lambda n1: clocks(7 * k + n1, 56),
                                   lambda n, op: a_s.put(n, i * (T // 2) + r, op, pl.ds(u, T)))
                    k += 1
            return carry

        lax.fori_loop(0, NP, phase2, carry0)
        cp_wo.wait()
        prep_w(h, lambda k, n: None)
        wl_s.ref[...] = jnp.zeros(wl_s.ref.shape, u32)
        cl_s.ref[...] = jnp.zeros(cl_s.ref.shape, u32)

    clk = _Clock(zero_s[...] != 0.0)

    def oproj(jp, ops):
        m = [_dot(wl_s.get(i), ops[i], _NN) for i in range(7)]
        for r in range(0, HM, G):
            for n, c in enumerate(_strassen_c([v[r:r + G] for v in m])):
                o_s[pl.ds((n // 2) * HM + r, G), pl.ds((2 * jp + n % 2) * T, T)] += c
        clk.stage(392, _rows8([m[0], m[4]]))

    def prep_wo(clocks):
        for r in range(0, HM, G):
            top = _tie(wo_s[h, r:r + G, :].astype(f32), clocks(r // G, HM // G))
            bot = _tie(wo_s[h, HM + r:HM + r + G, :].astype(f32), clocks(r // G, HM // G))
            for n, w in enumerate(_strassen_a(top[:, :HD], top[:, HD:], bot[:, :HD], bot[:, HD:])):
                wl_s.put(n, r, w)

    def proj(g, lo, hi):
        for n1 in range(lo, hi):
            m = [_dot(w_s.get(7 * n1 + n), a_s.get(7 * n1 + n, g * T, T), _NT) for n in range(7)]
            for r in range(0, 2 * QD, G):
                m_s = mk_s if r < QD else mv_s
                for n, c in enumerate(_strassen_c([v[r:r + G] for v in m])):
                    row = n1 * HD + (n % 2) * QD + r % QD
                    m_s[row:row + G, (n // 2) * T:(n // 2 + 1) * T] = c
            clk.stage(448, _rows8(m[0::2], 16))
        if hi == 7:
            kfin(g)
            vfin(g)

    def outer(m_s, r, nr, a2):
        return _strassen_c([m_s[n * HD + r:n * HD + r + nr, a2 * T:(a2 + 1) * T] for n in range(7)])

    def nine(c11, c12, c21, c22):
        return _strassen_a(c11, c12, c21, c22) + [c12.astype(bf16), c21.astype(bf16)]

    def kfin(g):
        for a2 in range(2):
            cs = [outer(mk_s, r, G, a2) for r in range(0, HD, G)]
            for n in range(4):
                kt_s[:, (a2 * 4 + n) * T:(a2 * 4 + n + 1) * T] = jnp.concatenate([c[n] for c in cs], axis=0).T
            for r in range(0, T, G):
                blk = [kt_s[r:r + G, (a2 * 4 + n) * T:(a2 * 4 + n + 1) * T] for n in range(4)]
                for n, op in enumerate(nine(*blk)):
                    ka_s.put(n, (2 * g + a2) * T + r, op)

    def vfin(g):
        for a2 in range(2):
            for r in range(0, HD, G):
                c11, c21, c12, c22 = outer(mv_s, r, G, a2)
                for n, op in enumerate(nine(c11, c12, c21, c22)):
                    va_s.put(n, r, op, pl.ds((2 * g + a2) * T, T))

    key = lax.broadcasted_iota(jnp.int32, (T, T), 0)
    qry = lax.broadcasted_iota(jnp.int32, (T, T), 1)
    causal = key <= qry

    class Reducer:
        def __init__(self, red, comb):
            self.red, self.comb, self.acc, self.rows, self.out = red, comb, None, 0, None

        def add(self, v):
            v = self.red(v.reshape(v.shape[0] // 8, 8, T), axis=0)
            self.acc = v if self.acc is None else self.comb(self.acc, v)
            self.rows += 1
            if self.rows * G >= RCH:
                self.flush()

        def flush(self):
            if self.acc is not None:
                v = self.red(self.acc, axis=0, keepdims=True)
                self.out = v if self.out is None else self.comb(self.out, v)
            self.acc, self.rows = None, 0

        def result(self):
            self.flush()
            return self.out

    def qk(jp):
        R, slot = jp * T, jp % 2
        cols = pl.ds(jp * T, T)
        qe, qo = q_s.get(2 * h, cols=cols), q_s.get(2 * h + 1, cols=cols)
        mx = [Reducer(jnp.max, jnp.maximum) for _ in range(2)]

        def put(e, row, v):
            s_s[slot, e, row:row + G, :] = v
            mx[e].add(v)

        if jp > 0:
            qef, qof = qe.astype(f32), qo.astype(f32)
            qb = _strassen_b(qef[:HD], qof[:HD], qef[HD:], qof[HD:])
            for r0 in range(0, R, QCH):
                r1 = min(r0 + QCH, R)
                m = [_dot(ka_s.get(n, r0, r1 - r0), qb[n], _NN) for n in range(7)]
                for r in range(0, r1 - r0, G):
                    c11, c12, c21, c22 = _strassen_c([v[r:r + G] for v in m])
                    put(0, r0 + r, c11)
                    put(1, r0 + r, c12)
                    put(0, R + r0 + r, c21)
                    put(1, R + r0 + r, c22)
                clk.stage(7 * (r1 - r0) / 4, _rows8([m[0], m[4]]))
        ke = jnp.concatenate([ka_s.get(2, R, T), ka_s.get(7, R, T)], axis=1)
        ko = jnp.concatenate([ka_s.get(8, R, T), ka_s.get(3, R, T)], axis=1)
        se = _dot(ke, jnp.concatenate([qe, qo], axis=1), _NN)
        so = _dot(ko, qo, _NN)
        for r in range(0, T, G):
            put(0, 2 * R + r, jnp.where(causal[r:r + G], se[r:r + G, :T], -1e30))
            put(1, 2 * R + r, se[r:r + G, T:])
            put(1, 2 * R + T + r, jnp.where(causal[r:r + G], so[r:r + G], -1e30))
        clk.stage(192, _rows8([se]))
        return [jnp.broadcast_to(x.result(), (8, T)) for x in mx]

    def pb0(jp):
        return jp * (jp - 1) // 2 * T

    def shifted_exp(slot, e, row, z):
        v = s_s[slot, e, row:row + G, :].reshape(G // 8, 8, T) - z[None]
        return jnp.exp2(v).reshape(G, T)

    def softmax(jp, mx, t0, t1, t2=None, t3=None):
        R, slot = jp * T, jp % 2
        if t2 is None:
            t1, t2, t3 = (t0 + t1) / 2, (t0 + t1) / 2, t1
        clocks = clk.pacer(t0, t1)
        k, n = 0, (4 * jp + 3) * T // G
        z = []
        for e in range(2):
            sm = Reducer(jnp.sum, jnp.add)
            for r in range(0, (2 * jp + 1 + e) * T, G):
                sm.add(shifted_exp(slot, e, r, _tie(mx[e], clocks(k, n))))
                k += 1
            z.append(mx[e] + jnp.log2(sm.result()))
        clocks = clk.pacer(t2, t3)
        k = 0
        for r in range(0, R, G):
            ze, zo = _tie(z[0], clocks(k, n)), _tie(z[1], clocks(k + 2, n))
            ops = _strassen_b(shifted_exp(slot, 0, r, ze), shifted_exp(slot, 1, r, zo),
                              shifted_exp(slot, 0, R + r, ze), shifted_exp(slot, 1, R + r, zo))
            for i in range(7):
                pb_s.put(i, pb0(jp) + r, ops[i])
            k += 4
        for r in range(0, 3 * T, G):
            e = int(r >= T)
            p = shifted_exp(slot, e, 2 * R + r - e * T, _tie(z[e], clocks(k, n)))
            pb_s.put(7, jp * 3 * T + r, p.astype(bf16))
            k += 1

    def pv(jp):
        R, slot = jp * T, jp % 4
        if jp > 0:
            m = [_dot(va_s.get(n, cols=pl.ds(0, R)), pb_s.get(n, pb0(jp), R), _NN) for n in range(7)]
            clk.stage(7 * R / 4, _rows8(m, 32))
        cols = pl.ds(R, T)
        ve = jnp.concatenate([va_s.get(2, cols=cols), va_s.get(8, cols=cols)], axis=0)
        vo = jnp.concatenate([va_s.get(7, cols=cols), va_s.get(3, cols=cols)], axis=0)
        ce = _dot(ve, pb_s.get(7, jp * 3 * T, T), _NN)
        co = _dot(jnp.concatenate([ve, vo], axis=1), pb_s.get(7, jp * 3 * T + T, 2 * T), _NN)
        clk.stage(192, _rows8([ce], 32))
        ge = g_s[:, 2 * jp * T:(2 * jp + 1) * T]
        go = g_s[:, (2 * jp + 1) * T:(2 * jp + 2) * T]
        for r in range(0, HD, G):
            c = [ce[r:r + G], co[r:r + G], ce[HD + r:HD + r + G], co[HD + r:HD + r + G]]
            if jp > 0:
                c = [x + y for x, y in zip(c, _strassen_c([v[r:r + G] for v in m]))]
            ops = _strassen_b(c[0] * ge, c[1] * go, c[2] * ge, c[3] * go)
            for n in range(7):
                cl_s.put(slot * 7 + n, r, ops[n])

    def ctx_ops(jp):
        return [cl_s.get((jp % 4) * 7 + n) for n in range(7)]

    def oproj_out(jp):
        oproj(jp, ctx_ops(jp))

        @pl.when(h == H - 1)
        def _():
            out_copy(jp).start()

    proj(0, 0, 7)
    oproj(NP - 1, ctx_ops(NP - 1))
    for jp, cover in enumerate(PLAN):
        mx = qk(jp)
        t0 = clk.t
        for item in cover.split():
            if item[0] == 'P':
                pv(int(item[1]))
            elif item[0] == 'O':
                oproj_out(int(item[1]))
            else:
                proj(int(item[1]), int(item[2]), int(item[3]))
        softmax(jp, mx, t0, clk.t - SLACK)
        if jp == 0:
            prep_wo(clk.pacer(t0, clk.t))
    t0 = clk.t
    pv(NP - 1)
    oproj_out(NP - 2)
    prep_w(jnp.minimum(h + 1, H - 1), clk.pacer(t0 - PW0, clk.t - 300))

    @pl.when(h == H - 1)
    def _():
        oproj(NP - 1, ctx_ops(NP - 1))
        out_copy(NP - 1).start()
        for jp in range(NP):
            out_copy(jp).wait()


@jax.jit
def pallas_gated_mix__compressed_kv_cla__ssm_conv_s5__prompt_kernel(
    A_x: jax.Array,
    A_c_kv: jax.Array,
    A_w_q: jax.Array,
    A_w_uk: jax.Array,
    A_w_uv: jax.Array,
    A_w_o: jax.Array,
    B_x: jax.Array,
    B_Lambda_re: jax.Array,
    B_Lambda_im: jax.Array,
    B_B_re: jax.Array,
    B_B_im: jax.Array,
    B_C_re: jax.Array,
    B_C_im: jax.Array,
    B_log_dt: jax.Array,
    B_Dskip: jax.Array,
    gate_w: jax.Array,
):
    del B_x
    xT = jnp.transpose(A_x[0])
    woT = jnp.transpose(A_w_o, (0, 2, 1))
    ckv = A_c_kv.reshape(4, 4, 2, T // 2, DC)

    hbm = pl.BlockSpec(memory_space=pl.ANY)
    vmem = pltpu.VMEM
    outT = pl.pallas_call(
        _kernel,
        grid=(H,),
        in_specs=[hbm] * 15,
        out_specs=hbm,
        out_shape=jax.ShapeDtypeStruct((M, S), f32),
        scratch_shapes=[
            vmem((M, S), bf16),
            vmem((M,), bf16), vmem((M,), bf16), vmem((M,), bf16), vmem((M,), bf16), vmem((M,), bf16),
            vmem((2 * M, M), bf16),
            vmem((2, M, M), bf16),
            vmem((M // 2, 2 * M), u32),
            vmem((8, 512), f32),
            vmem((8, 8, 512), f32),
            vmem((2, M, 128), f32),
            vmem((S, 2 * M), f32),
            vmem((1, S), f32),
            vmem((4, 4, 2, T // 2, DC), bf16),
            vmem((M, H, D), bf16),
            vmem((NRAW * CS, H, D), bf16),
            vmem((NRAW * CS, H, D), bf16),
            vmem((4, M * 4, 128), u32),
            vmem((4, CS * 4, 128), u32),
            vmem((4, CS * 4, 128), u32),
            vmem((49 * S // 8, QC), u32),
            vmem((7 * HM // 2, S // 2), u32),
            vmem((H * D, S // 2), u32),
            vmem((H, M, D), bf16),
            vmem((S // 4, 9 * HD), u32),
            vmem((9 * HD // 2, S // 2), u32),
            vmem((14 * T, 8 * T), u32),
            vmem((M, S), f32),
            vmem((2, 2, S, T), f32),
            vmem((TC // 2, 2 * M), u32),
            vmem((8, 128), f32),
            vmem((HM // 2, 7 * HD), u32),
            vmem((HD // 2, 28 * T), u32),
            vmem((49 * QD, QC), u32),
            vmem((H // 2 * D, DC), u32),
            vmem((H // 2 * D, DC), u32),
            vmem((7 * HD, 2 * T), f32),
            vmem((7 * HD, 2 * T), f32),
            vmem((T, 8 * T), f32),
            pltpu.SemaphoreType.DMA((NSEM,)),
        ],
        compiler_params=pltpu.CompilerParams(
            dimension_semantics=("arbitrary",),
            vmem_limit_bytes=126 * 1024 * 1024,
        ),
    )(xT, B_B_re, B_B_im, B_C_re, B_C_im, B_Lambda_re, B_Lambda_im, B_log_dt,
      B_Dskip, gate_w, woT, ckv, A_w_q, A_w_uk, A_w_uv)
    return jnp.transpose(outT)[None]
```

```python
import jax
import jax.numpy as jnp
from jax import lax
import jax.experimental.pallas as pl
import jax.experimental.pallas.tpu as pltpu

S = 2048
M = 448
H = 16
D = 256
DC = 1024
T = 128
NT = S // T
NP = NT // 2
HD = D // 2
HM = M // 2
QD = D // 4
QC = DC // 4
PA = 384
PB = M - PA
TA = 512
TC = 256
CS = DC // NP
NRAW = 4
import os
G = int(os.environ.get('G', 16))
RCH = int(os.environ.get('RCH', 512))
QCH = int(os.environ.get('QCH', 1024))
SLACK = int(os.environ.get('SLACK', 200))
PW0 = int(os.environ.get('PW0', 100))
PULL = int(os.environ.get('PULL', 4))
D0 = int(os.environ.get('D0', 0))
NT1 = int(os.environ.get('NT1', 3))
LEAD = int(os.environ.get('LEAD', 448))
PLAN = os.environ.get('PLAN', 'K104,K147,K203,K237,K304 P0 P1,K347 P2 O0,P3 O1 P4 O2 O3,P5 O4 P6 O5').split(',')
LOG2E = 1.4426950408889634

f32 = jnp.float32
bf16 = jnp.bfloat16
u32 = jnp.uint32

SEM_VEC, SEM_B, SEM_X, SEM_WQ, SEM_C, SEM_SL, SEM_WO, SEM_OUT = 0, 1, 2, 6, 7, 8, 16, 17
NSEM = 18


def _dot(a, b, dims):
    return lax.dot_general(a, b, (dims, ((), ())), preferred_element_type=f32)


_NN = ((1,), (0,))
_NT = ((1,), (1,))
_TN = ((0,), (0,))
_TT = ((0,), (1,))


def _pk(x):
    return pltpu.bitcast(x, u32)


def _up(x):
    return pltpu.bitcast(x, bf16)


class _Stack:
    def __init__(self, ref, rows, along_lanes=False):
        self.ref, self.rows, self.along_lanes = ref, rows, along_lanes

    def _idx(self, n, r0, nr, cols):
        lo = r0 // 2 if isinstance(r0, int) else lax.shift_right_logical(r0, 1)
        nr = (self.rows if nr is None else nr) // 2
        if self.along_lanes:
            return _ds(lo, nr, 8), pl.ds(n * 128, 128)
        return _ds(n * (self.rows // 2) + lo, nr, 8), (slice(None) if cols is None else cols)

    def get(self, n, r0=0, nr=None, cols=None):
        return _up(self.ref[self._idx(n, r0, nr, cols)])

    def put(self, n, r0, x, cols=None):
        self.ref[self._idx(n, r0, x.shape[0], cols)] = _pk(x)


def _tie(x, clock):
    if clock is None:
        return x
    never, tick = clock
    r, c = x.shape
    if tick.dtype != x.dtype:
        tick = pltpu.bitcast(tick, x.dtype)
    tile = lambda v: jnp.tile(v, (r // 8, c // 128))
    return jnp.where(tile(never), tile(tick), x)


def _cmul(ar, ai, br, bi):
    return ar * br - ai * bi, ar * bi + ai * br


def _ds(lo, n, align):
    return pl.ds(lo if isinstance(lo, int) else pl.multiple_of(lo, align), n)


def _strassen_a(a11, a12, a21, a22):
    ops = [a11 + a22, a21 + a22, a11, a22, a11 + a12, a21 - a11, a12 - a22]
    return [o.astype(bf16) for o in ops]


def _strassen_b(b11, b12, b21, b22, dtype=bf16):
    ops = [b11 + b22, b11, b12 - b22, b21 - b11, b22, b11 + b12, b21 + b22]
    return [o.astype(dtype) for o in ops]


_A_TERMS = ((0, 3, 1), (2, 3, 1), (0, None, 0), (3, None, 0), (0, 1, 1), (2, 0, -1), (1, 3, -1))
_B_TERMS = ((0, 3, 1), (0, None, 0), (1, 3, -1), (2, 0, -1), (3, None, 0), (0, 1, 1), (2, 3, 1))


def _strassen2_ops(block, terms, inner, clock, emit, outer=range(7)):
    for n1 in outer:
        x, y, sign = terms[n1]
        sub = []
        for q in range(4):
            v = block(x, q)
            if q in (0, 3):
                v = _tie(v, clock(n1))
            if y is not None:
                v = v + block(y, q) if sign > 0 else v - block(y, q)
            sub.append(v)
        for n2, op in enumerate(inner(*sub)):
            emit(7 * n1 + n2, op)


def _strassen_c(m):
    c11 = (m[0] + m[3]) + (m[6] - m[4])
    c12 = m[2] + m[4]
    c21 = m[1] + m[3]
    c22 = (m[0] - m[1]) + (m[2] + m[5])
    return c11, c12, c21, c22


def _stage(raw, r0, stg, c0, nc, clock=None):
    for ht in range(2):
        for dt in range(2):
            v = raw[pl.ds(r0, nc), ht * 8:(ht + 1) * 8, dt * 128:(dt + 1) * 128]
            stg[ht * 2 + dt, _ds(c0 * 4, nc * 4, 8), :] = _tie(_pk(v.reshape(nc * 8, 128)), clock)


def _pair_words(stg, pair, rows):
    ht = lax.shift_right_logical(pair, 2)
    return [stg[ht * 2 + dt, pl.ds(pair & 3, rows, stride=4), :] for dt in range(2)]


def _weight_ops(halves, rows, dtype=bf16):
    r = rows // 2
    return _strassen_b(halves[0][:r], halves[1][:r], halves[0][r:], halves[1][r:], dtype)


class _Clock:
    def __init__(self, never):
        self.never, self.ticks, self.t = never, [], 0

    def stage(self, duration, vals):
        for k, v in enumerate(vals):
            self.ticks.append((self.t + duration * (k + 1) / len(vals), v))
        self.t += duration

    def pacer(self, t0, t1):
        def clocks(k, n):
            want = t0 + (t1 - t0) * k / n
            best = [v for t, v in self.ticks if t <= want]
            return (self.never, best[-1]) if best else None
        return clocks


def _rows8(vals, step=8):
    return [v[r:r + 8, 0:128] for v in vals for r in range(0, v.shape[0], step)]


def _ssm_cmat(craw_s, coef_s, c_s, clocks):
    for r in range(0, M, 16):
        coef = _tie(coef_s[...], clocks(r // 16, M // 16))
        cr, ci = coef[0:1, :M], coef[1:2, :M]
        cp_re, cp_im = _cmul(craw_s[0, r:r + 16, :].astype(f32), craw_s[1, r:r + 16, :].astype(f32), cr, ci)
        c_s[r // 2:r // 2 + 8, :] = _pk(jnp.concatenate(
            [cp_re[:, :PA], -cp_im[:, :PA], cp_re[:, PA:], -cp_im[:, PA:]], axis=1).astype(bf16))


def _ssm_params(vec_s, coef_s, lam_s, col_s, zero_s):
    row = lambda r: r[...].astype(f32).reshape(1, M)
    lre, lim, ldt, dsk, gw = [row(v) for v in vec_s]
    dt = jnp.exp(ldt).astype(bf16).astype(f32)
    mag = jnp.exp(dt * lre)
    ang = dt * lim
    lr, li = mag * jnp.cos(ang), mag * jnp.sin(ang)
    den = lre * lre + lim * lim
    nr = lr - 1.0
    coef_s[...] = jnp.zeros(coef_s.shape, f32)
    coef_s[0:1, 0:M] = 2.0 * ((nr * lre + li * lim) / den)
    coef_s[1:2, 0:M] = 2.0 * ((li * lre - nr * lim) / den)
    zero_s[...] = jnp.zeros(zero_s.shape, f32)

    er = jnp.concatenate([lr, lr[:, PA:]], axis=1)
    ei = jnp.concatenate([li, -li[:, PA:]], axis=1)
    pw = [(er, ei)]
    for _ in range(7):
        pw.append(_cmul(pw[-1][0], pw[-1][1], er, ei))
    sub = lax.broadcasted_iota(jnp.int32, (8, 512), 0)
    for n, d in enumerate((1, 2, 4)):
        lam_s[2 * n] = jnp.where(sub >= d, pw[d - 1][0], 0.0)
        lam_s[2 * n + 1] = jnp.where(sub >= d, pw[d - 1][1], 0.0)
    lcr = jnp.zeros((8, 512), f32)
    lci = jnp.zeros((8, 512), f32)
    for r in range(8):
        lcr = jnp.where(sub == r, pw[r][0], lcr)
        lci = jnp.where(sub == r, pw[r][1], lci)
    lam_s[6] = lcr
    lam_s[7] = lci

    def col(v):
        v = jnp.concatenate([v, jnp.zeros((1, 512 - M), f32)], axis=1)
        return jnp.broadcast_to(v, (128, 512)).T[:M]
    col_s[0] = col(dsk)
    col_s[1] = col(gw)


def _ssm_scan(u_s, t0, carry, lam_s, h_s, clocks):
    car, cai = carry
    out = []
    for b in range(TC // 8):
        u = u_s[_ds(t0 + b * 8, 8, 8), :]
        mixed = u[:, 2 * PA:]
        cols = [u[:, 0:128], u[:, 128:256], u[:, 256:384], mixed]
        hr = jnp.concatenate([_tie(v, clocks(4 * b + n, TC // 2)) for n, v in enumerate(cols)], axis=1)
        hi = jnp.concatenate([u[:, PA:2 * PA], pltpu.roll(mixed, PB, 1)], axis=1)
        for n, d in enumerate((1, 2, 4)):
            sr, si = pltpu.roll(hr, d, 0), pltpu.roll(hi, d, 0)
            tr, ti = _cmul(sr, si, lam_s[2 * n], lam_s[2 * n + 1])
            hr, hi = hr + tr, hi + ti
        tr, ti = _cmul(lam_s[6], lam_s[7], car, cai)
        hr, hi = hr + tr, hi + ti
        car, cai = hr[7:8, :], hi[7:8, :]
        out.append(jnp.concatenate([hr[:, :PA], hi[:, :PA], hr[:, PA:]], axis=1))
        if b % 2 == 1:
            h_s[(b // 2) * 8:(b // 2 + 1) * 8, :] = _pk(jnp.concatenate(out, axis=0).astype(bf16))
            out = []
    return car, cai


def _kernel(xT_hbm, bre_hbm, bim_hbm, cre_hbm, cim_hbm, lre_hbm, lim_hbm, ldt_hbm,
            dsk_hbm, gw_hbm, woT_hbm, ckv_hbm, wq_hbm, wk_hbm, wv_hbm,
            out_hbm,
            xT_s, v0, v1, v2, v3, v4, b_s, craw_s, c_s, coef_s, lam_s, col_s, u_s, g_s,
            ckv_s, rq, rk, rv, sq, sk, sv, a_s, xa_s, q_s, wo_s,
            ka_s, va_s, pb_s, o_s, s_s, h_s, zero_s, wl_s, cl_s, w_s,
            wkt_s, wvt_s, mk_s, mv_s, kt_s, sink_s, sem):
    h = pl.program_id(0)
    vec_s = (v0, v1, v2, v3, v4)
    a_s, xa_s, q_s = _Stack(a_s, S // 4), _Stack(xa_s, HM), _Stack(q_s, D)
    ka_s, va_s, pb_s = _Stack(ka_s, S // 2, True), _Stack(va_s, HD), _Stack(pb_s, S // 2, True)
    w_s = _Stack(w_s, 2 * QD)
    wl_s, cl_s = _Stack(wl_s, HM, True), _Stack(cl_s, HD, True)

    def slice_copies(i):
        s = sem.at[SEM_SL + i]
        grp = i // 2 if isinstance(i, int) else lax.shift_right_logical(i, 1)
        cs, dst = pl.ds(i * CS, CS), pl.ds((i & (NRAW - 1)) * CS, CS)
        return [pltpu.make_async_copy(ckv_hbm.at[grp, :, i & 1], ckv_s.at[grp, :, i & 1], s),
                pltpu.make_async_copy(wk_hbm.at[cs], rk.at[dst], s),
                pltpu.make_async_copy(wv_hbm.at[cs], rv.at[dst], s)]

    def x_copy(i):
        cols = _ds(i * TA, TA, TA)
        return pltpu.make_async_copy(xT_hbm.at[:, cols], xT_s.at[:, cols], sem.at[SEM_X + i])

    def out_copy(jp):
        cols = pl.ds(jp * 2 * T, 2 * T)
        return pltpu.make_async_copy(o_s.at[:, cols], out_hbm.at[:, cols], sem.at[SEM_OUT])

    def prep_w(hh, clocks, outer):
        base = lax.shift_right_logical(hh, 1) * D
        sh = (16 * (1 - (hh & 1))).astype(u32)
        k = 0
        for row0, wt_s in ((0, wkt_s), (QD, wvt_s)):
            for r in range(0, QD, 16):
                for u in range(0, QC, T):
                    def block(o, q):
                        row = (o % 2) * HD + (q % 2) * QD + r
                        col = (o // 2) * 2 * QC + (q // 2) * QC + u
                        w = wt_s[_ds(base + row, 16, 16), col:col + T]
                        return pltpu.bitcast((w << sh) & jnp.uint32(0xFFFF0000), f32)
                    _strassen2_ops(block, _B_TERMS, _strassen_b,
                                   lambda n1: clocks(len(outer) * k + n1 - outer[0], 16 * len(outer)),
                                   lambda n, op: w_s.put(n, row0 + r, op, pl.ds(u, T)), outer)
                    k += 1

    @pl.when(h == 0)
    def _():
        cp_vec = [pltpu.make_async_copy(src, dst, sem.at[SEM_VEC])
                  for src, dst in zip((lre_hbm, lim_hbm, ldt_hbm, dsk_hbm, gw_hbm), vec_s)]
        cp_b = [pltpu.make_async_copy(src.at[pl.ds(lo, n)], b_s.at[pl.ds(dst, n)], sem.at[SEM_B])
                for src, lo, n, dst in ((bre_hbm, 0, PA, 0), (bim_hbm, 0, PA, PA),
                                        (bre_hbm, PA, PB, 2 * PA), (bim_hbm, PA, PB, 2 * PA + PB))]
        cp_wq = [pltpu.make_async_copy(wq_hbm, rq, sem.at[SEM_WQ])]
        cp_c = [pltpu.make_async_copy(src, craw_s.at[n], sem.at[SEM_C])
                for n, src in enumerate((cre_hbm, cim_hbm))]
        cp_wo = pltpu.make_async_copy(woT_hbm, wo_s, sem.at[SEM_WO])
        for cp in cp_vec + cp_b:
            cp.start()
        for i in range(S // TA):
            x_copy(i).start()
        for cp in cp_wq + cp_c:
            cp.start()
        for i in range(NRAW - 1):
            for cp in slice_copies(i):
                cp.start()
        cp_wo.start()

        def phase1(i):
            x_copy(i).wait()
            u = _dot(xT_s[:, _ds(i * TA, TA, TA)], b_s[...], _TT)
            u_s[_ds(i * TA, TA, TA), :] = u
            never = zero_s[...] != 0.0

            def clocks(k, n):
                pos = (k * 6 * TA // n) // 8 * 8
                return never, u[pos % TA:pos % TA + 8, (pos // TA) * 128:(pos // TA + 1) * 128]

            for t in range(TA // (2 * T)):
                ev = _ds(i * TA + 2 * t * T, T, T)
                od = _ds(i * TA + (2 * t + 1) * T, T, T)
                for r in range(0, HM, 32):
                    top, bot = pl.ds(r, 32), pl.ds(HM + r, 32)
                    clk = clocks(t * 7 + r // 32, 14)
                    ops = _strassen_a(_tie(xT_s[top, ev].astype(f32), clk), xT_s[bot, ev].astype(f32),
                                      xT_s[top, od].astype(f32), _tie(xT_s[bot, od].astype(f32), clk))
                    for n in range(7):
                        xa_s.put(n, r, ops[n], _ds(i * (TA // 2) + t * T, T, T))
            return clocks

        for cp in cp_vec:
            cp.wait()
        _ssm_params(vec_s, coef_s, lam_s, col_s, zero_s)
        for cp in cp_b:
            cp.wait()

        def phase1_body(i, carry):
            phase1(i)
            return carry
        lax.fori_loop(0, S // TA - 1, phase1_body, 0)
        for cp in cp_wq + cp_c:
            cp.wait()
        clocks = phase1(S // TA - 1)
        for c0 in range(0, M, 8):
            _stage(rq, c0, sq, c0, 8, clocks(c0 // 8, M // 8))
        _ssm_cmat(craw_s, coef_s, c_s, clocks)
        zero = jnp.zeros((1, 512), f32)
        carry0 = _ssm_scan(u_s, 0, (zero, zero), lam_s, h_s, clocks)

        def phase2(i, carry):
            @pl.when(i + NRAW - 1 < NP)
            def _():
                for cp in slice_copies(i + NRAW - 1):
                    cp.start()

            for cp in slice_copies(i):
                cp.wait()
            yT = _dot(_up(c_s[...]), _up(h_s[...]), _NT)
            for t in range(TC // T):
                cols = _ds(i * TC + t * T, T, T)
                acc = jnp.zeros((8, T), f32)
                for r in range(0, M, 32):
                    xg = xT_s[r:r + 32, cols].astype(f32) * col_s[1, r:r + 32, :]
                    acc = acc + jnp.sum(xg.reshape(4, 8, T), axis=0)
                g = jax.nn.sigmoid(jnp.sum(acc, axis=0, keepdims=True))
                g_s[:, cols] = g
                for r in range(0, M, 32):
                    skip = xT_s[r:r + 32, cols].astype(f32) * col_s[0, r:r + 32, :]
                    o_s[r:r + 32, cols] = (1.0 - g) * (yT[r:r + 32, t * T:(t + 1) * T] + skip)

            words = _pair_words(sq, i, M)
            lo = _weight_ops([pltpu.bitcast(u << 16, f32) for u in words], M, f32)
            hi = _weight_ops([pltpu.bitcast(u & jnp.uint32(0xFFFF0000), f32) for u in words], M, f32)
            prods = [_dot(jnp.concatenate([lo[n], hi[n]], axis=1).astype(bf16), xa_s.get(n), _TN)
                     for n in range(7)]
            qs = LOG2E * D ** -0.5
            for t in range(NP):
                for r in range(0, D, G):
                    cs = _strassen_c([v[r:r + G, t * T:(t + 1) * T] for v in prods])
                    for n, c in enumerate(cs):
                        q_s.put(4 * i + 2 * (r // HD) + n // 2, (n % 2) * HD + r % HD,
                                (c * qs).astype(bf16), pl.ds(t * T, T))

            never = zero_s[...] != 0.0

            def clocks(k, n):
                pos = (k * 5 * 1024 // n) // 8 * 8
                r, c = pos % 256, (pos % 1024) // 256 * 256
                return never, prods[pos // 1024][r:r + 8, c:c + 128]

            carry = _ssm_scan(u_s, jnp.minimum(i + 1, NP - 1) * TC, carry, lam_s, h_s, clocks)

            for c0 in range(0, CS, 8):
                r0 = (i & (NRAW - 1)) * CS + c0
                _stage(rk, r0, sk, c0, 8, clocks(c0 // 8, 64))
                _stage(rv, r0, sv, c0, 8, clocks(16 + c0 // 8, 64))
            for n, (stg, wt_s) in enumerate(((sk, wkt_s), (sv, wvt_s))):
                for pair in range(H // 2):
                    for dt in range(2):
                        blk = stg[(pair // 4) * 2 + dt, pl.ds(pair % 4, CS, stride=4), :]
                        blk = _tie(blk, clocks(16 + 24 * n + 3 * pair + dt, 64))
                        wt_s[pair * D + dt * HD:pair * D + (dt + 1) * HD, _ds(i * CS, CS, CS)] = blk.T
            grp, half = lax.shift_right_logical(i, 1), i & 1
            k = 0
            for r in range(0, T // 2, 16):
                for u in range(0, QC, T):
                    def block(o, q):
                        col = (o % 2) * 2 * QC + (q % 2) * QC + u
                        return ckv_s[grp, 2 * (q // 2) + o // 2, half, r:r + 16, col:col + T].astype(f32)
                    _strassen2_ops(block, _A_TERMS, _strassen_a, lambda n1: clocks(7 * k + n1, 56),
                                   lambda n, op: a_s.put(n, i * (T // 2) + r, op, pl.ds(u, T)))
                    k += 1
            return carry

        lax.fori_loop(0, NP, phase2, carry0)
        cp_wo.wait()
        prep_w(h, lambda k, n: None, range(NT1))
        wl_s.ref[...] = jnp.zeros(wl_s.ref.shape, u32)
        cl_s.ref[...] = jnp.zeros(cl_s.ref.shape, u32)

    clk = _Clock(zero_s[...] != 0.0)

    def oproj(jp, ops):
        m = [_dot(wl_s.get(i), ops[i], _NN) for i in range(7)]
        for r in range(0, HM, G):
            for n, c in enumerate(_strassen_c([v[r:r + G] for v in m])):
                o_s[pl.ds((n // 2) * HM + r, G), pl.ds((2 * jp + n % 2) * T, T)] += c
        clk.stage(392, _rows8([m[0], m[4]]))

    def prep_wo(clocks):
        for r in range(0, HM, G):
            top = _tie(wo_s[h, r:r + G, :].astype(f32), clocks(r // G, HM // G))
            bot = _tie(wo_s[h, HM + r:HM + r + G, :].astype(f32), clocks(r // G, HM // G))
            for n, w in enumerate(_strassen_a(top[:, :HD], top[:, HD:], bot[:, :HD], bot[:, HD:])):
                wl_s.put(n, r, w)

    def proj(g, lo, hi):
        for n1 in range(lo, hi):
            m = [_dot(w_s.get(7 * n1 + n), a_s.get(7 * n1 + n, g * T, T), _NT) for n in range(7)]
            for r in range(0, 2 * QD, G):
                m_s = mk_s if r < QD else mv_s
                for n, c in enumerate(_strassen_c([v[r:r + G] for v in m])):
                    row = n1 * HD + (n % 2) * QD + r % QD
                    m_s[row:row + G, (n // 2) * T:(n // 2 + 1) * T] = c
            clk.stage(448, _rows8(m[0::2], 16))
        if hi == 7:
            kfin(g)
            vfin(g)

    def outer(m_s, r, nr, a2):
        return _strassen_c([m_s[n * HD + r:n * HD + r + nr, a2 * T:(a2 + 1) * T] for n in range(7)])

    def nine(c11, c12, c21, c22):
        return _strassen_a(c11, c12, c21, c22) + [c12.astype(bf16), c21.astype(bf16)]

    def kfin(g):
        for a2 in range(2):
            cs = [outer(mk_s, r, G, a2) for r in range(0, HD, G)]
            for n in range(4):
                kt_s[:, (a2 * 4 + n) * T:(a2 * 4 + n + 1) * T] = jnp.concatenate([c[n] for c in cs], axis=0).T
            for r in range(0, T, G):
                blk = [kt_s[r:r + G, (a2 * 4 + n) * T:(a2 * 4 + n + 1) * T] for n in range(4)]
                for n, op in enumerate(nine(*blk)):
                    ka_s.put(n, (2 * g + a2) * T + r, op)

    def vfin(g):
        for a2 in range(2):
            for r in range(0, HD, G):
                c11, c21, c12, c22 = outer(mv_s, r, G, a2)
                for n, op in enumerate(nine(c11, c12, c21, c22)):
                    va_s.put(n, r, op, pl.ds((2 * g + a2) * T, T))

    key = lax.broadcasted_iota(jnp.int32, (T, T), 0)
    qry = lax.broadcasted_iota(jnp.int32, (T, T), 1)
    causal = key <= qry

    class Reducer:
        def __init__(self, red, comb):
            self.red, self.comb, self.acc, self.rows, self.out = red, comb, None, 0, None

        def add(self, v):
            v = self.red(v.reshape(v.shape[0] // 8, 8, T), axis=0)
            self.acc = v if self.acc is None else self.comb(self.acc, v)
            self.rows += 1
            if self.rows * G >= RCH:
                self.flush()

        def flush(self):
            if self.acc is not None:
                v = self.red(self.acc, axis=0, keepdims=True)
                self.out = v if self.out is None else self.comb(self.out, v)
            self.acc, self.rows = None, 0

        def result(self):
            self.flush()
            return self.out

    def qk(jp):
        R, slot = jp * T, jp % 2
        cols = pl.ds(jp * T, T)
        qe, qo = q_s.get(2 * h, cols=cols), q_s.get(2 * h + 1, cols=cols)
        mx = [Reducer(jnp.max, jnp.maximum) for _ in range(2)]

        def put(e, row, v):
            s_s[slot, e, row:row + G, :] = v
            mx[e].add(v)

        if jp > 0:
            qef, qof = qe.astype(f32), qo.astype(f32)
            qb = _strassen_b(qef[:HD], qof[:HD], qef[HD:], qof[HD:])
            for r0 in range(0, R, QCH):
                r1 = min(r0 + QCH, R)
                m = [_dot(ka_s.get(n, r0, r1 - r0), qb[n], _NN) for n in range(7)]
                for r in range(0, r1 - r0, G):
                    c11, c12, c21, c22 = _strassen_c([v[r:r + G] for v in m])
                    put(0, r0 + r, c11)
                    put(1, r0 + r, c12)
                    put(0, R + r0 + r, c21)
                    put(1, R + r0 + r, c22)
                clk.stage(7 * (r1 - r0) / 4, _rows8([m[0], m[4]]))
        ke = jnp.concatenate([ka_s.get(2, R, T), ka_s.get(7, R, T)], axis=1)
        ko = jnp.concatenate([ka_s.get(8, R, T), ka_s.get(3, R, T)], axis=1)
        se = _dot(ke, jnp.concatenate([qe, qo], axis=1), _NN)
        so = _dot(ko, qo, _NN)
        for r in range(0, T, G):
            put(0, 2 * R + r, jnp.where(causal[r:r + G], se[r:r + G, :T], -1e30))
            put(1, 2 * R + r, se[r:r + G, T:])
            put(1, 2 * R + T + r, jnp.where(causal[r:r + G], so[r:r + G], -1e30))
        clk.stage(192, _rows8([se]))
        return [jnp.broadcast_to(x.result(), (8, T)) for x in mx]

    pull = [0]

    def pb0(jp):
        return jp * (jp - 1) // 2 * T

    def shifted_exp(slot, e, row, z):
        v = s_s[slot, e, row:row + G, :].reshape(G // 8, 8, T) - z[None]
        return jnp.exp2(v).reshape(G, T)

    def softmax(jp, mx, t0, t1, t2=None, t3=None):
        R, slot = jp * T, jp % 2
        if t2 is None:
            t1, t2, t3 = (t0 + t1) / 2, (t0 + t1) / 2, t1
        clocks = clk.pacer(t0, t1)
        k, n = 0, (4 * jp + 3) * T // G
        z = []
        for e in range(2):
            sm = Reducer(jnp.sum, jnp.add)
            for r in range(0, (2 * jp + 1 + e) * T, G):
                sm.add(shifted_exp(slot, e, r, _tie(mx[e], clocks(k, n))))
                k += 1
                if PULL and k % PULL == 0 and sm.acc is not None:
                    sink_s[pull[0] * 8:(pull[0] + 1) * 8, :] = sm.acc
                    pull[0] += 1
            z.append(mx[e] + jnp.log2(sm.result()))
        clocks = clk.pacer(t2, t3)
        k = 0
        for r in range(0, R, G):
            ze, zo = _tie(z[0], clocks(k, n)), _tie(z[1], clocks(k + 2, n))
            ops = _strassen_b(shifted_exp(slot, 0, r, ze), shifted_exp(slot, 1, r, zo),
                              shifted_exp(slot, 0, R + r, ze), shifted_exp(slot, 1, R + r, zo))
            for i in range(7):
                pb_s.put(i, pb0(jp) + r, ops[i])
            k += 4
        for r in range(0, 3 * T, G):
            e = int(r >= T)
            p = shifted_exp(slot, e, 2 * R + r - e * T, _tie(z[e], clocks(k, n)))
            pb_s.put(7, jp * 3 * T + r, p.astype(bf16))
            k += 1

    def pv(jp):
        R, slot = jp * T, jp % 4
        if jp > 0:
            m = [_dot(va_s.get(n, cols=pl.ds(0, R)), pb_s.get(n, pb0(jp), R), _NN) for n in range(7)]
            clk.stage(7 * R / 4, _rows8(m, 32))
        cols = pl.ds(R, T)
        ve = jnp.concatenate([va_s.get(2, cols=cols), va_s.get(8, cols=cols)], axis=0)
        vo = jnp.concatenate([va_s.get(7, cols=cols), va_s.get(3, cols=cols)], axis=0)
        ce = _dot(ve, pb_s.get(7, jp * 3 * T, T), _NN)
        co = _dot(jnp.concatenate([ve, vo], axis=1), pb_s.get(7, jp * 3 * T + T, 2 * T), _NN)
        clk.stage(192, _rows8([ce], 32))
        ge = g_s[:, 2 * jp * T:(2 * jp + 1) * T]
        go = g_s[:, (2 * jp + 1) * T:(2 * jp + 2) * T]
        for r in range(0, HD, G):
            c = [ce[r:r + G], co[r:r + G], ce[HD + r:HD + r + G], co[HD + r:HD + r + G]]
            if jp > 0:
                c = [x + y for x, y in zip(c, _strassen_c([v[r:r + G] for v in m]))]
            ops = _strassen_b(c[0] * ge, c[1] * go, c[2] * ge, c[3] * go)
            for n in range(7):
                cl_s.put(slot * 7 + n, r, ops[n])

    def ctx_ops(jp):
        return [cl_s.get((jp % 4) * 7 + n) for n in range(7)]

    def oproj_out(jp):
        oproj(jp, ctx_ops(jp))

        @pl.when(h == H - 1)
        def _():
            out_copy(jp).start()

    for n1 in range(7):
        if n1 >= NT1:
            prep_w(h, clk.pacer(max(clk.t - LEAD - 448, 1), max(clk.t - LEAD, 1)), range(n1, n1 + 1))
        proj(0, n1, n1 + 1)
    oproj(NP - 1, ctx_ops(NP - 1))
    for jp, cover in enumerate(PLAN):
        mx = qk(jp)
        t0 = clk.t
        for item in cover.split():
            if item[0] == 'P':
                pv(int(item[1]))
            elif item[0] == 'O':
                oproj_out(int(item[1]))
            else:
                proj(int(item[1]), int(item[2]), int(item[3]))
        softmax(jp, mx, t0 + D0, clk.t - SLACK)
        if jp == 0:
            prep_wo(clk.pacer(t0, clk.t))
    t0 = clk.t
    pv(NP - 1)
    oproj_out(NP - 2)
    prep_w(jnp.minimum(h + 1, H - 1), clk.pacer(t0 - PW0, clk.t - 300), range(NT1))

    @pl.when(h == H - 1)
    def _():
        oproj(NP - 1, ctx_ops(NP - 1))
        out_copy(NP - 1).start()
        for jp in range(NP):
            out_copy(jp).wait()


@jax.jit
def pallas_gated_mix__compressed_kv_cla__ssm_conv_s5__prompt_kernel(
    A_x: jax.Array,
    A_c_kv: jax.Array,
    A_w_q: jax.Array,
    A_w_uk: jax.Array,
    A_w_uv: jax.Array,
    A_w_o: jax.Array,
    B_x: jax.Array,
    B_Lambda_re: jax.Array,
    B_Lambda_im: jax.Array,
    B_B_re: jax.Array,
    B_B_im: jax.Array,
    B_C_re: jax.Array,
    B_C_im: jax.Array,
    B_log_dt: jax.Array,
    B_Dskip: jax.Array,
    gate_w: jax.Array,
):
    del B_x
    xT = jnp.transpose(A_x[0])
    woT = jnp.transpose(A_w_o, (0, 2, 1))
    ckv = A_c_kv.reshape(4, 4, 2, T // 2, DC)

    hbm = pl.BlockSpec(memory_space=pl.ANY)
    vmem = pltpu.VMEM
    outT = pl.pallas_call(
        _kernel,
        grid=(H,),
        in_specs=[hbm] * 15,
        out_specs=hbm,
        out_shape=jax.ShapeDtypeStruct((M, S), f32),
        scratch_shapes=[
            vmem((M, S), bf16),
            vmem((M,), bf16), vmem((M,), bf16), vmem((M,), bf16), vmem((M,), bf16), vmem((M,), bf16),
            vmem((2 * M, M), bf16),
            vmem((2, M, M), bf16),
            vmem((M // 2, 2 * M), u32),
            vmem((8, 512), f32),
            vmem((8, 8, 512), f32),
            vmem((2, M, 128), f32),
            vmem((S, 2 * M), f32),
            vmem((1, S), f32),
            vmem((4, 4, 2, T // 2, DC), bf16),
            vmem((M, H, D), bf16),
            vmem((NRAW * CS, H, D), bf16),
            vmem((NRAW * CS, H, D), bf16),
            vmem((4, M * 4, 128), u32),
            vmem((4, CS * 4, 128), u32),
            vmem((4, CS * 4, 128), u32),
            vmem((49 * S // 8, QC), u32),
            vmem((7 * HM // 2, S // 2), u32),
            vmem((H * D, S // 2), u32),
            vmem((H, M, D), bf16),
            vmem((S // 4, 9 * HD), u32),
            vmem((9 * HD // 2, S // 2), u32),
            vmem((14 * T, 8 * T), u32),
            vmem((M, S), f32),
            vmem((2, 2, S, T), f32),
            vmem((TC // 2, 2 * M), u32),
            vmem((8, 128), f32),
            vmem((HM // 2, 7 * HD), u32),
            vmem((HD // 2, 28 * T), u32),
            vmem((49 * QD, QC), u32),
            vmem((H // 2 * D, DC), u32),
            vmem((H // 2 * D, DC), u32),
            vmem((7 * HD, 2 * T), f32),
            vmem((7 * HD, 2 * T), f32),
            vmem((T, 8 * T), f32),
            vmem((544 * 8, T), f32),
            pltpu.SemaphoreType.DMA((NSEM,)),
        ],
        compiler_params=pltpu.CompilerParams(
            dimension_semantics=("arbitrary",),
            vmem_limit_bytes=126 * 1024 * 1024,
        ),
    )(xT, B_B_re, B_B_im, B_C_re, B_C_im, B_Lambda_re, B_Lambda_im, B_log_dt,
      B_Dskip, gate_w, woT, ckv, A_w_q, A_w_uk, A_w_uv)
    return jnp.transpose(outT)[None]
```

```python
import jax
import jax.numpy as jnp
from jax import lax
import jax.experimental.pallas as pl
import jax.experimental.pallas.tpu as pltpu

S = 2048
M = 448
H = 16
D = 256
DC = 1024
T = 128
NT = S // T
NP = NT // 2
HD = D // 2
HM = M // 2
QD = D // 4
QC = DC // 4
PA = 384
PB = M - PA
TA = 512
TC = 256
CS = DC // NP
NRAW = 4
import os
G = int(os.environ.get('G', 16))
RCH = int(os.environ.get('RCH', 512))
QCH = int(os.environ.get('QCH', 1024))
SLACK = int(os.environ.get('SLACK', 200))
PW0 = int(os.environ.get('PW0', 100))
P1LINE = int(os.environ.get('P1LINE', 1))
FIN = int(os.environ.get('FIN', 0))
PULL = int(os.environ.get('PULL', 4))
D0 = int(os.environ.get('D0', 0))
NT1 = int(os.environ.get('NT1', 3))
LEAD = int(os.environ.get('LEAD', 448))
PLAN = os.environ.get('PLAN', 'K104,K147,K203,K237,K304 P0 P1,K347 P2 O0,P3 O1 P4 O2 O3,P5 O4 P6 O5').split(',')
LOG2E = 1.4426950408889634

f32 = jnp.float32
bf16 = jnp.bfloat16
u32 = jnp.uint32

SEM_VEC, SEM_B, SEM_X, SEM_WQ, SEM_C, SEM_SL, SEM_WO, SEM_OUT = 0, 1, 2, 6, 7, 8, 16, 17
NSEM = 18


def _dot(a, b, dims):
    return lax.dot_general(a, b, (dims, ((), ())), preferred_element_type=f32)


_NN = ((1,), (0,))
_NT = ((1,), (1,))
_TN = ((0,), (0,))
_TT = ((0,), (1,))


def _pk(x):
    return pltpu.bitcast(x, u32)


def _up(x):
    return pltpu.bitcast(x, bf16)


class _Stack:
    def __init__(self, ref, rows, along_lanes=False):
        self.ref, self.rows, self.along_lanes = ref, rows, along_lanes

    def _idx(self, n, r0, nr, cols):
        lo = r0 // 2 if isinstance(r0, int) else lax.shift_right_logical(r0, 1)
        nr = (self.rows if nr is None else nr) // 2
        if self.along_lanes:
            return _ds(lo, nr, 8), pl.ds(n * 128, 128)
        return _ds(n * (self.rows // 2) + lo, nr, 8), (slice(None) if cols is None else cols)

    def get(self, n, r0=0, nr=None, cols=None):
        return _up(self.ref[self._idx(n, r0, nr, cols)])

    def put(self, n, r0, x, cols=None):
        self.ref[self._idx(n, r0, x.shape[0], cols)] = _pk(x)


def _tie(x, clock):
    if clock is None:
        return x
    never, tick = clock
    r, c = x.shape
    if tick.dtype != x.dtype:
        tick = pltpu.bitcast(tick, x.dtype)
    tile = lambda v: jnp.tile(v, (r // 8, c // 128))
    return jnp.where(tile(never), tile(tick), x)


def _cmul(ar, ai, br, bi):
    return ar * br - ai * bi, ar * bi + ai * br


def _ds(lo, n, align):
    return pl.ds(lo if isinstance(lo, int) else pl.multiple_of(lo, align), n)


def _strassen_a(a11, a12, a21, a22):
    ops = [a11 + a22, a21 + a22, a11, a22, a11 + a12, a21 - a11, a12 - a22]
    return [o.astype(bf16) for o in ops]


def _strassen_b(b11, b12, b21, b22, dtype=bf16):
    ops = [b11 + b22, b11, b12 - b22, b21 - b11, b22, b11 + b12, b21 + b22]
    return [o.astype(dtype) for o in ops]


_A_TERMS = ((0, 3, 1), (2, 3, 1), (0, None, 0), (3, None, 0), (0, 1, 1), (2, 0, -1), (1, 3, -1))
_B_TERMS = ((0, 3, 1), (0, None, 0), (1, 3, -1), (2, 0, -1), (3, None, 0), (0, 1, 1), (2, 3, 1))


def _strassen2_ops(block, terms, inner, clock, emit, outer=range(7)):
    for n1 in outer:
        x, y, sign = terms[n1]
        sub = []
        for q in range(4):
            v = block(x, q)
            if q in (0, 3):
                v = _tie(v, clock(n1))
            if y is not None:
                v = v + block(y, q) if sign > 0 else v - block(y, q)
            sub.append(v)
        for n2, op in enumerate(inner(*sub)):
            emit(7 * n1 + n2, op)


def _strassen_c(m, only=None):
    c = (lambda: (m[0] + m[3]) + (m[6] - m[4]),
         lambda: m[2] + m[4],
         lambda: m[1] + m[3],
         lambda: (m[0] - m[1]) + (m[2] + m[5]))
    return [f() for f in c] if only is None else c[only]()


def _stage(raw, r0, stg, c0, nc, clock=None):
    for ht in range(2):
        for dt in range(2):
            v = raw[pl.ds(r0, nc), ht * 8:(ht + 1) * 8, dt * 128:(dt + 1) * 128]
            stg[ht * 2 + dt, _ds(c0 * 4, nc * 4, 8), :] = _tie(_pk(v.reshape(nc * 8, 128)), clock)


def _pair_words(stg, pair, rows):
    ht = lax.shift_right_logical(pair, 2)
    return [stg[ht * 2 + dt, pl.ds(pair & 3, rows, stride=4), :] for dt in range(2)]


def _weight_ops(halves, rows, dtype=bf16):
    r = rows // 2
    return _strassen_b(halves[0][:r], halves[1][:r], halves[0][r:], halves[1][r:], dtype)


class _Clock:
    def __init__(self, never):
        self.never, self.ticks, self.t = never, [], 0

    def stage(self, duration, vals):
        for k, v in enumerate(vals):
            self.ticks.append((self.t + duration * (k + 1) / len(vals), v))
        self.t += duration

    def pacer(self, t0, t1):
        def clocks(k, n):
            want = t0 + (t1 - t0) * k / n
            best = [v for t, v in self.ticks if t <= want]
            return (self.never, best[-1]) if best else None
        return clocks


def _rows8(vals, step=8):
    return [v[r:r + 8, 0:128] for v in vals for r in range(0, v.shape[0], step)]


def _ssm_cmat(craw_s, coef_s, c_s, clocks):
    for r in range(0, M, 16):
        coef = _tie(coef_s[...], clocks(r // 16, M // 16))
        cr, ci = coef[0:1, :M], coef[1:2, :M]
        cp_re, cp_im = _cmul(craw_s[0, r:r + 16, :].astype(f32), craw_s[1, r:r + 16, :].astype(f32), cr, ci)
        c_s[r // 2:r // 2 + 8, :] = _pk(jnp.concatenate(
            [cp_re[:, :PA], -cp_im[:, :PA], cp_re[:, PA:], -cp_im[:, PA:]], axis=1).astype(bf16))


def _ssm_params(vec_s, coef_s, lam_s, col_s, zero_s):
    row = lambda r: r[...].astype(f32).reshape(1, M)
    lre, lim, ldt, dsk, gw = [row(v) for v in vec_s]
    dt = jnp.exp(ldt).astype(bf16).astype(f32)
    mag = jnp.exp(dt * lre)
    ang = dt * lim
    lr, li = mag * jnp.cos(ang), mag * jnp.sin(ang)
    den = lre * lre + lim * lim
    nr = lr - 1.0
    coef_s[...] = jnp.zeros(coef_s.shape, f32)
    coef_s[0:1, 0:M] = 2.0 * ((nr * lre + li * lim) / den)
    coef_s[1:2, 0:M] = 2.0 * ((li * lre - nr * lim) / den)
    zero_s[...] = jnp.zeros(zero_s.shape, f32)

    er = jnp.concatenate([lr, lr[:, PA:]], axis=1)
    ei = jnp.concatenate([li, -li[:, PA:]], axis=1)
    pw = [(er, ei)]
    for _ in range(7):
        pw.append(_cmul(pw[-1][0], pw[-1][1], er, ei))
    sub = lax.broadcasted_iota(jnp.int32, (8, 512), 0)
    for n, d in enumerate((1, 2, 4)):
        lam_s[2 * n] = jnp.where(sub >= d, pw[d - 1][0], 0.0)
        lam_s[2 * n + 1] = jnp.where(sub >= d, pw[d - 1][1], 0.0)
    lcr = jnp.zeros((8, 512), f32)
    lci = jnp.zeros((8, 512), f32)
    for r in range(8):
        lcr = jnp.where(sub == r, pw[r][0], lcr)
        lci = jnp.where(sub == r, pw[r][1], lci)
    lam_s[6] = lcr
    lam_s[7] = lci

    def col(v):
        v = jnp.concatenate([v, jnp.zeros((1, 512 - M), f32)], axis=1)
        return jnp.broadcast_to(v, (128, 512)).T[:M]
    col_s[0] = col(dsk)
    col_s[1] = col(gw)


def _ssm_scan(u_s, t0, carry, lam_s, h_s, clocks):
    car, cai = carry
    out = []
    for b in range(TC // 8):
        u = u_s[_ds(t0 + b * 8, 8, 8), :]
        mixed = u[:, 2 * PA:]
        cols = [u[:, 0:128], u[:, 128:256], u[:, 256:384], mixed]
        hr = jnp.concatenate([_tie(v, clocks(4 * b + n, TC // 2)) for n, v in enumerate(cols)], axis=1)
        hi = jnp.concatenate([u[:, PA:2 * PA], pltpu.roll(mixed, PB, 1)], axis=1)
        for n, d in enumerate((1, 2, 4)):
            sr, si = pltpu.roll(hr, d, 0), pltpu.roll(hi, d, 0)
            tr, ti = _cmul(sr, si, lam_s[2 * n], lam_s[2 * n + 1])
            hr, hi = hr + tr, hi + ti
        tr, ti = _cmul(lam_s[6], lam_s[7], car, cai)
        hr, hi = hr + tr, hi + ti
        car, cai = hr[7:8, :], hi[7:8, :]
        out.append(jnp.concatenate([hr[:, :PA], hi[:, :PA], hr[:, PA:]], axis=1))
        if b % 2 == 1:
            h_s[(b // 2) * 8:(b // 2 + 1) * 8, :] = _pk(jnp.concatenate(out, axis=0).astype(bf16))
            out = []
    return car, cai


def _kernel(xT_hbm, bre_hbm, bim_hbm, cre_hbm, cim_hbm, lre_hbm, lim_hbm, ldt_hbm,
            dsk_hbm, gw_hbm, woT_hbm, ckv_hbm, wq_hbm, wk_hbm, wv_hbm,
            out_hbm,
            xT_s, v0, v1, v2, v3, v4, b_s, craw_s, c_s, coef_s, lam_s, col_s, u_s, g_s,
            ckv_s, rq, rk, rv, sq, sk, sv, a_s, xa_s, q_s, wo_s,
            ka_s, va_s, pb_s, o_s, s_s, h_s, zero_s, wl_s, cl_s, w_s,
            wkt_s, wvt_s, mk_s, mv_s, kt_s, sink_s, sem):
    h = pl.program_id(0)
    vec_s = (v0, v1, v2, v3, v4)
    a_s, xa_s, q_s = _Stack(a_s, S // 4), _Stack(xa_s, HM), _Stack(q_s, D)
    ka_s, va_s, pb_s = _Stack(ka_s, S // 2, True), _Stack(va_s, HD), _Stack(pb_s, S // 2, True)
    w_s = _Stack(w_s, 2 * QD)
    wl_s, cl_s = _Stack(wl_s, HM, True), _Stack(cl_s, HD, True)

    def slice_copies(i):
        s = sem.at[SEM_SL + i]
        grp = i // 2 if isinstance(i, int) else lax.shift_right_logical(i, 1)
        cs, dst = pl.ds(i * CS, CS), pl.ds((i & (NRAW - 1)) * CS, CS)
        return [pltpu.make_async_copy(ckv_hbm.at[grp, :, i & 1], ckv_s.at[grp, :, i & 1], s),
                pltpu.make_async_copy(wk_hbm.at[cs], rk.at[dst], s),
                pltpu.make_async_copy(wv_hbm.at[cs], rv.at[dst], s)]

    def x_copy(i):
        cols = _ds(i * TA, TA, TA)
        return pltpu.make_async_copy(xT_hbm.at[:, cols], xT_s.at[:, cols], sem.at[SEM_X + i])

    def out_copy(jp):
        cols = pl.ds(jp * 2 * T, 2 * T)
        return pltpu.make_async_copy(o_s.at[:, cols], out_hbm.at[:, cols], sem.at[SEM_OUT])

    def prep_w(hh, clocks, outer):
        base = lax.shift_right_logical(hh, 1) * D
        sh = (16 * (1 - (hh & 1))).astype(u32)
        k = 0
        for row0, wt_s in ((0, wkt_s), (QD, wvt_s)):
            for r in range(0, QD, 16):
                for u in range(0, QC, T):
                    def block(o, q):
                        row = (o % 2) * HD + (q % 2) * QD + r
                        col = (o // 2) * 2 * QC + (q // 2) * QC + u
                        w = wt_s[_ds(base + row, 16, 16), col:col + T]
                        return pltpu.bitcast((w << sh) & jnp.uint32(0xFFFF0000), f32)
                    _strassen2_ops(block, _B_TERMS, _strassen_b,
                                   lambda n1: clocks(len(outer) * k + n1 - outer[0], 16 * len(outer)),
                                   lambda n, op: w_s.put(n, row0 + r, op, pl.ds(u, T)), outer)
                    k += 1

    @pl.when(h == 0)
    def _():
        cp_vec = [pltpu.make_async_copy(src, dst, sem.at[SEM_VEC])
                  for src, dst in zip((lre_hbm, lim_hbm, ldt_hbm, dsk_hbm, gw_hbm), vec_s)]
        cp_b = [pltpu.make_async_copy(src.at[pl.ds(lo, n)], b_s.at[pl.ds(dst, n)], sem.at[SEM_B])
                for src, lo, n, dst in ((bre_hbm, 0, PA, 0), (bim_hbm, 0, PA, PA),
                                        (bre_hbm, PA, PB, 2 * PA), (bim_hbm, PA, PB, 2 * PA + PB))]
        cp_wq = [pltpu.make_async_copy(wq_hbm, rq, sem.at[SEM_WQ])]
        cp_c = [pltpu.make_async_copy(src, craw_s.at[n], sem.at[SEM_C])
                for n, src in enumerate((cre_hbm, cim_hbm))]
        cp_wo = pltpu.make_async_copy(woT_hbm, wo_s, sem.at[SEM_WO])
        for cp in cp_vec + cp_b:
            cp.start()
        for i in range(S // TA):
            x_copy(i).start()
        for cp in cp_c + cp_wq:
            cp.start()
        for i in range(NRAW - 1):
            for cp in slice_copies(i):
                cp.start()
        cp_wo.start()

        def phase1(i):
            x_copy(i).wait()
            u = _dot(xT_s[:, _ds(i * TA, TA, TA)], b_s[...], _TT)
            u_s[_ds(i * TA, TA, TA), :] = u
            never = zero_s[...] != 0.0

            def clocks(k, n):
                pos = (k * 6 * TA // n) // 8 * 8
                return never, u[pos % TA:pos % TA + 8, (pos // TA) * 128:(pos // TA + 1) * 128]

            for t in range(TA // (2 * T)):
                ev = _ds(i * TA + 2 * t * T, T, T)
                od = _ds(i * TA + (2 * t + 1) * T, T, T)
                for r in range(0, HM, 32):
                    top, bot = pl.ds(r, 32), pl.ds(HM + r, 32)
                    clk = clocks(t * 7 + r // 32, 14)
                    ops = _strassen_a(_tie(xT_s[top, ev].astype(f32), clk), xT_s[bot, ev].astype(f32),
                                      xT_s[top, od].astype(f32), _tie(xT_s[bot, od].astype(f32), clk))
                    for n in range(7):
                        xa_s.put(n, r, ops[n], _ds(i * (TA // 2) + t * T, T, T))
            return clocks

        wl_s.ref[...] = jnp.zeros(wl_s.ref.shape, u32)
        cl_s.ref[...] = jnp.zeros(cl_s.ref.shape, u32)
        for cp in cp_vec:
            cp.wait()
        _ssm_params(vec_s, coef_s, lam_s, col_s, zero_s)
        for cp in cp_b:
            cp.wait()

        zero = jnp.zeros((1, 512), f32)
        if P1LINE:
            phase1(0)
            clocks = phase1(1)
            carry0 = _ssm_scan(u_s, 0, (zero, zero), lam_s, h_s, clocks)
            for cp in cp_c:
                cp.wait()
            clocks = phase1(2)
            _ssm_cmat(craw_s, coef_s, c_s, clocks)
            for cp in cp_wq:
                cp.wait()
            clocks = phase1(3)
            for c0 in range(0, M, 8):
                _stage(rq, c0, sq, c0, 8, clocks(c0 // 8, M // 8))
        else:
            def phase1_body(i, carry):
                phase1(i)
                return carry
            lax.fori_loop(0, S // TA - 1, phase1_body, 0)
            for cp in cp_wq + cp_c:
                cp.wait()
            clocks = phase1(S // TA - 1)
            for c0 in range(0, M, 8):
                _stage(rq, c0, sq, c0, 8, clocks(c0 // 8, M // 8))
            _ssm_cmat(craw_s, coef_s, c_s, clocks)
            carry0 = _ssm_scan(u_s, 0, (zero, zero), lam_s, h_s, clocks)

        def phase2(i, carry):
            @pl.when(i + NRAW - 1 < NP)
            def _():
                for cp in slice_copies(i + NRAW - 1):
                    cp.start()

            for cp in slice_copies(i):
                cp.wait()
            yT = _dot(_up(c_s[...]), _up(h_s[...]), _NT)
            for t in range(TC // T):
                cols = _ds(i * TC + t * T, T, T)
                acc = jnp.zeros((8, T), f32)
                for r in range(0, M, 32):
                    xg = xT_s[r:r + 32, cols].astype(f32) * col_s[1, r:r + 32, :]
                    acc = acc + jnp.sum(xg.reshape(4, 8, T), axis=0)
                g = jax.nn.sigmoid(jnp.sum(acc, axis=0, keepdims=True))
                g_s[:, cols] = g
                for r in range(0, M, 32):
                    skip = xT_s[r:r + 32, cols].astype(f32) * col_s[0, r:r + 32, :]
                    o_s[r:r + 32, cols] = (1.0 - g) * (yT[r:r + 32, t * T:(t + 1) * T] + skip)

            words = _pair_words(sq, i, M)
            lo = _weight_ops([pltpu.bitcast(u << 16, f32) for u in words], M, f32)
            hi = _weight_ops([pltpu.bitcast(u & jnp.uint32(0xFFFF0000), f32) for u in words], M, f32)
            prods = [_dot(jnp.concatenate([lo[n], hi[n]], axis=1).astype(bf16), xa_s.get(n), _TN)
                     for n in range(7)]
            qs = LOG2E * D ** -0.5
            for n in (2, 1, 3, 0):
                for t in range(NP):
                    for r in range(0, D, G):
                        c = _strassen_c([v[r:r + G, t * T:(t + 1) * T] for v in prods], n)
                        q_s.put(4 * i + 2 * (r // HD) + n // 2, (n % 2) * HD + r % HD,
                                (c * qs).astype(bf16), pl.ds(t * T, T))

            never = zero_s[...] != 0.0

            def clocks(k, n):
                pos = (k * 5 * 1024 // n) // 8 * 8
                r, c = pos % 256, (pos % 1024) // 256 * 256
                return never, prods[pos // 1024][r:r + 8, c:c + 128]

            carry = _ssm_scan(u_s, jnp.minimum(i + 1, NP - 1) * TC, carry, lam_s, h_s, clocks)

            for c0 in range(0, CS, 8):
                r0 = (i & (NRAW - 1)) * CS + c0
                _stage(rk, r0, sk, c0, 8, clocks(c0 // 8, 64))
                _stage(rv, r0, sv, c0, 8, clocks(16 + c0 // 8, 64))
            for n, (stg, wt_s) in enumerate(((sk, wkt_s), (sv, wvt_s))):
                for pair in range(H // 2):
                    for dt in range(2):
                        blk = stg[(pair // 4) * 2 + dt, pl.ds(pair % 4, CS, stride=4), :]
                        blk = _tie(blk, clocks(16 + 24 * n + 3 * pair + dt, 64))
                        wt_s[pair * D + dt * HD:pair * D + (dt + 1) * HD, _ds(i * CS, CS, CS)] = blk.T
            grp, half = lax.shift_right_logical(i, 1), i & 1
            k = 0
            for r in range(0, T // 2, 16):
                for u in range(0, QC, T):
                    def block(o, q):
                        col = (o % 2) * 2 * QC + (q % 2) * QC + u
                        return ckv_s[grp, 2 * (q // 2) + o // 2, half, r:r + 16, col:col + T].astype(f32)
                    _strassen2_ops(block, _A_TERMS, _strassen_a, lambda n1: clocks(7 * k + n1, 56),
                                   lambda n, op: a_s.put(n, i * (T // 2) + r, op, pl.ds(u, T)))
                    k += 1
            return carry

        lax.fori_loop(0, NP, phase2, carry0)
        cp_wo.wait()
        prep_w(h, lambda k, n: None, range(NT1))

    clk = _Clock(zero_s[...] != 0.0)

    def oproj(jp, ops):
        m = [_dot(wl_s.get(i), ops[i], _NN) for i in range(7)]
        for r in range(0, HM, G):
            for n, c in enumerate(_strassen_c([v[r:r + G] for v in m])):
                o_s[pl.ds((n // 2) * HM + r, G), pl.ds((2 * jp + n % 2) * T, T)] += c
        clk.stage(392, _rows8([m[0], m[4]]))

    def prep_wo(clocks):
        for r in range(0, HM, G):
            top = _tie(wo_s[h, r:r + G, :].astype(f32), clocks(r // G, HM // G))
            bot = _tie(wo_s[h, HM + r:HM + r + G, :].astype(f32), clocks(r // G, HM // G))
            for n, w in enumerate(_strassen_a(top[:, :HD], top[:, HD:], bot[:, :HD], bot[:, HD:])):
                wl_s.put(n, r, w)

    def proj(g, lo, hi):
        for n1 in range(lo, hi):
            m = [_dot(w_s.get(7 * n1 + n), a_s.get(7 * n1 + n, g * T, T), _NT) for n in range(7)]
            for r in range(0, 2 * QD, G):
                m_s = mk_s if r < QD else mv_s
                for n, c in enumerate(_strassen_c([v[r:r + G] for v in m])):
                    row = n1 * HD + (n % 2) * QD + r % QD
                    m_s[row:row + G, (n // 2) * T:(n // 2 + 1) * T] = c
            clk.stage(448, _rows8(m[0::2], 16))
        if hi == 7:
            kfin(g)
            vfin(g)

    def outer(m_s, r, nr, a2):
        return _strassen_c([m_s[n * HD + r:n * HD + r + nr, a2 * T:(a2 + 1) * T] for n in range(7)])

    def nine(c11, c12, c21, c22):
        return _strassen_a(c11, c12, c21, c22) + [c12.astype(bf16), c21.astype(bf16)]

    def kfin(g):
        for a2 in range(2):
            cs = [outer(mk_s, r, G, a2) for r in range(0, HD, G)]
            for n in range(4):
                kt_s[:, (a2 * 4 + n) * T:(a2 * 4 + n + 1) * T] = jnp.concatenate([c[n] for c in cs], axis=0).T
            for r in range(0, T, G):
                blk = [kt_s[r:r + G, (a2 * 4 + n) * T:(a2 * 4 + n + 1) * T] for n in range(4)]
                for n, op in enumerate(nine(*blk)):
                    ka_s.put(n, (2 * g + a2) * T + r, op)

    def vfin(g):
        for a2 in range(2):
            for r in range(0, HD, G):
                c11, c21, c12, c22 = outer(mv_s, r, G, a2)
                for n, op in enumerate(nine(c11, c12, c21, c22)):
                    va_s.put(n, r, op, pl.ds((2 * g + a2) * T, T))

    key = lax.broadcasted_iota(jnp.int32, (T, T), 0)
    qry = lax.broadcasted_iota(jnp.int32, (T, T), 1)
    causal = key <= qry

    class Reducer:
        def __init__(self, red, comb):
            self.red, self.comb, self.acc, self.rows, self.out = red, comb, None, 0, None

        def add(self, v):
            v = self.red(v.reshape(v.shape[0] // 8, 8, T), axis=0)
            self.acc = v if self.acc is None else self.comb(self.acc, v)
            self.rows += 1
            if self.rows * G >= RCH:
                self.flush()

        def flush(self):
            if self.acc is not None:
                v = self.red(self.acc, axis=0, keepdims=True)
                self.out = v if self.out is None else self.comb(self.out, v)
            self.acc, self.rows = None, 0

        def result(self):
            self.flush()
            return self.out

    def qk(jp):
        R, slot = jp * T, jp % 2
        cols = pl.ds(jp * T, T)
        qe, qo = q_s.get(2 * h, cols=cols), q_s.get(2 * h + 1, cols=cols)
        mx = [Reducer(jnp.max, jnp.maximum) for _ in range(2)]

        def put(e, row, v):
            s_s[slot, e, row:row + G, :] = v
            mx[e].add(v)

        if jp > 0:
            qef, qof = qe.astype(f32), qo.astype(f32)
            qb = _strassen_b(qef[:HD], qof[:HD], qef[HD:], qof[HD:])
            for r0 in range(0, R, QCH):
                r1 = min(r0 + QCH, R)
                m = [_dot(ka_s.get(n, r0, r1 - r0), qb[n], _NN) for n in range(7)]
                for r in range(0, r1 - r0, G):
                    c11, c12, c21, c22 = _strassen_c([v[r:r + G] for v in m])
                    put(0, r0 + r, c11)
                    put(1, r0 + r, c12)
                    put(0, R + r0 + r, c21)
                    put(1, R + r0 + r, c22)
                clk.stage(7 * (r1 - r0) / 4, _rows8([m[0], m[4]]))
        ke = jnp.concatenate([ka_s.get(2, R, T), ka_s.get(7, R, T)], axis=1)
        ko = jnp.concatenate([ka_s.get(8, R, T), ka_s.get(3, R, T)], axis=1)
        se = _dot(ke, jnp.concatenate([qe, qo], axis=1), _NN)
        so = _dot(ko, qo, _NN)
        for r in range(0, T, G):
            put(0, 2 * R + r, jnp.where(causal[r:r + G], se[r:r + G, :T], -1e30))
            put(1, 2 * R + r, se[r:r + G, T:])
            put(1, 2 * R + T + r, jnp.where(causal[r:r + G], so[r:r + G], -1e30))
        clk.stage(192, _rows8([se]))
        return [jnp.broadcast_to(x.result(), (8, T)) for x in mx]

    pull = [0]

    def pb0(jp):
        return jp * (jp - 1) // 2 * T

    def shifted_exp(slot, e, row, z):
        v = s_s[slot, e, row:row + G, :].reshape(G // 8, 8, T) - z[None]
        return jnp.exp2(v).reshape(G, T)

    def softmax(jp, mx, t0, t1, t2=None, t3=None):
        R, slot = jp * T, jp % 2
        if t2 is None:
            t1, t2, t3 = (t0 + t1) / 2, (t0 + t1) / 2, t1
        clocks = clk.pacer(t0, t1)
        k, n = 0, (4 * jp + 3) * T // G
        z = []
        for e in range(2):
            sm = Reducer(jnp.sum, jnp.add)
            for r in range(0, (2 * jp + 1 + e) * T, G):
                sm.add(shifted_exp(slot, e, r, _tie(mx[e], clocks(k, n))))
                k += 1
                if PULL and k % PULL == 0 and sm.acc is not None:
                    sink_s[pull[0] * 8:(pull[0] + 1) * 8, :] = sm.acc
                    pull[0] += 1
            z.append(mx[e] + jnp.log2(sm.result()))
        clocks = clk.pacer(t2, t3)
        k = 0
        for r in range(0, R, G):
            ze, zo = _tie(z[0], clocks(k, n)), _tie(z[1], clocks(k + 2, n))
            ops = _strassen_b(shifted_exp(slot, 0, r, ze), shifted_exp(slot, 1, r, zo),
                              shifted_exp(slot, 0, R + r, ze), shifted_exp(slot, 1, R + r, zo))
            for i in range(7):
                pb_s.put(i, pb0(jp) + r, ops[i])
            k += 4
        for r in range(0, 3 * T, G):
            e = int(r >= T)
            p = shifted_exp(slot, e, 2 * R + r - e * T, _tie(z[e], clocks(k, n)))
            pb_s.put(7, jp * 3 * T + r, p.astype(bf16))
            k += 1

    def pv(jp):
        R, slot = jp * T, jp % 4
        if jp > 0:
            m = [_dot(va_s.get(n, cols=pl.ds(0, R)), pb_s.get(n, pb0(jp), R), _NN) for n in range(7)]
            clk.stage(7 * R / 4, _rows8(m, 32))
        cols = pl.ds(R, T)
        ve = jnp.concatenate([va_s.get(2, cols=cols), va_s.get(8, cols=cols)], axis=0)
        vo = jnp.concatenate([va_s.get(7, cols=cols), va_s.get(3, cols=cols)], axis=0)
        ce = _dot(ve, pb_s.get(7, jp * 3 * T, T), _NN)
        co = _dot(jnp.concatenate([ve, vo], axis=1), pb_s.get(7, jp * 3 * T + T, 2 * T), _NN)
        clk.stage(192, _rows8([ce], 32))
        ge = g_s[:, 2 * jp * T:(2 * jp + 1) * T]
        go = g_s[:, (2 * jp + 1) * T:(2 * jp + 2) * T]
        for r in range(0, HD, G):
            c = [ce[r:r + G], co[r:r + G], ce[HD + r:HD + r + G], co[HD + r:HD + r + G]]
            if jp > 0:
                c = [x + y for x, y in zip(c, _strassen_c([v[r:r + G] for v in m]))]
            ops = _strassen_b(c[0] * ge, c[1] * go, c[2] * ge, c[3] * go)
            for n in range(7):
                cl_s.put(slot * 7 + n, r, ops[n])

    def ctx_ops(jp):
        return [cl_s.get((jp % 4) * 7 + n) for n in range(7)]

    def oproj_out(jp):
        oproj(jp, ctx_ops(jp))

        @pl.when(h == H - 1)
        def _():
            out_copy(jp).start()

    for n1 in range(7):
        if n1 >= NT1:
            prep_w(h, clk.pacer(max(clk.t - LEAD - 448, 1), max(clk.t - LEAD, 1)), range(n1, n1 + 1))
        proj(0, n1, n1 + 1)
    oproj(NP - 1, ctx_ops(NP - 1))
    for jp, cover in enumerate(PLAN):
        mx = qk(jp)
        t0 = clk.t
        for item in cover.split():
            if item[0] == 'P':
                pv(int(item[1]))
            elif item[0] == 'O':
                oproj_out(int(item[1]))
            else:
                proj(int(item[1]), int(item[2]), int(item[3]))
        softmax(jp, mx, t0 + D0, clk.t - SLACK)
        if jp == 0:
            prep_wo(clk.pacer(t0, clk.t))
    t0 = clk.t
    if FIN:
        oproj_out(NP - 2)
        pv(NP - 1)
    else:
        pv(NP - 1)
        oproj_out(NP - 2)
    prep_w(jnp.minimum(h + 1, H - 1), clk.pacer(t0 - PW0, clk.t - 300), range(NT1))

    @pl.when(h == H - 1)
    def _():
        oproj(NP - 1, ctx_ops(NP - 1))
        out_copy(NP - 1).start()
        for jp in range(NP):
            out_copy(jp).wait()


@jax.jit
def pallas_gated_mix__compressed_kv_cla__ssm_conv_s5__prompt_kernel(
    A_x: jax.Array,
    A_c_kv: jax.Array,
    A_w_q: jax.Array,
    A_w_uk: jax.Array,
    A_w_uv: jax.Array,
    A_w_o: jax.Array,
    B_x: jax.Array,
    B_Lambda_re: jax.Array,
    B_Lambda_im: jax.Array,
    B_B_re: jax.Array,
    B_B_im: jax.Array,
    B_C_re: jax.Array,
    B_C_im: jax.Array,
    B_log_dt: jax.Array,
    B_Dskip: jax.Array,
    gate_w: jax.Array,
):
    del B_x
    xT = jnp.transpose(A_x[0])
    woT = jnp.transpose(A_w_o, (0, 2, 1))
    ckv = A_c_kv.reshape(4, 4, 2, T // 2, DC)

    hbm = pl.BlockSpec(memory_space=pl.ANY)
    vmem = pltpu.VMEM
    outT = pl.pallas_call(
        _kernel,
        grid=(H,),
        in_specs=[hbm] * 15,
        out_specs=hbm,
        out_shape=jax.ShapeDtypeStruct((M, S), f32),
        scratch_shapes=[
            vmem((M, S), bf16),
            vmem((M,), bf16), vmem((M,), bf16), vmem((M,), bf16), vmem((M,), bf16), vmem((M,), bf16),
            vmem((2 * M, M), bf16),
            vmem((2, M, M), bf16),
            vmem((M // 2, 2 * M), u32),
            vmem((8, 512), f32),
            vmem((8, 8, 512), f32),
            vmem((2, M, 128), f32),
            vmem((S, 2 * M), f32),
            vmem((1, S), f32),
            vmem((4, 4, 2, T // 2, DC), bf16),
            vmem((M, H, D), bf16),
            vmem((NRAW * CS, H, D), bf16),
            vmem((NRAW * CS, H, D), bf16),
            vmem((4, M * 4, 128), u32),
            vmem((4, CS * 4, 128), u32),
            vmem((4, CS * 4, 128), u32),
            vmem((49 * S // 8, QC), u32),
            vmem((7 * HM // 2, S // 2), u32),
            vmem((H * D, S // 2), u32),
            vmem((H, M, D), bf16),
            vmem((S // 4, 9 * HD), u32),
            vmem((9 * HD // 2, S // 2), u32),
            vmem((14 * T, 8 * T), u32),
            vmem((M, S), f32),
            vmem((2, 2, S, T), f32),
            vmem((TC // 2, 2 * M), u32),
            vmem((8, 128), f32),
            vmem((HM // 2, 7 * HD), u32),
            vmem((HD // 2, 28 * T), u32),
            vmem((49 * QD, QC), u32),
            vmem((H // 2 * D, DC), u32),
            vmem((H // 2 * D, DC), u32),
            vmem((7 * HD, 2 * T), f32),
            vmem((7 * HD, 2 * T), f32),
            vmem((T, 8 * T), f32),
            vmem((544 * 8, T), f32),
            pltpu.SemaphoreType.DMA((NSEM,)),
        ],
        compiler_params=pltpu.CompilerParams(
            dimension_semantics=("arbitrary",),
            vmem_limit_bytes=126 * 1024 * 1024,
        ),
    )(xT, B_B_re, B_B_im, B_C_re, B_C_im, B_Lambda_re, B_Lambda_im, B_log_dt,
      B_Dskip, gate_w, woT, ckv, A_w_q, A_w_uk, A_w_uv)
    return jnp.transpose(outT)[None]
```

```python
import jax
import jax.numpy as jnp
from jax import lax
import jax.experimental.pallas as pl
import jax.experimental.pallas.tpu as pltpu

S = 2048
M = 448
H = 16
D = 256
DC = 1024
T = 128
NT = S // T
NP = NT // 2
HD = D // 2
HM = M // 2
QD = D // 4
QC = DC // 4
PA = 384
PB = M - PA
TA = 512
TC = 256
CS = DC // NP
NRAW = 4
import os
G = int(os.environ.get('G', 16))
RCH = int(os.environ.get('RCH', 512))
QCH = int(os.environ.get('QCH', 1024))
SLACK = int(os.environ.get('SLACK', 200))
PW0 = int(os.environ.get('PW0', 100))
FIN = int(os.environ.get('FIN', 0))
PULL = int(os.environ.get('PULL', 4))
D0 = int(os.environ.get('D0', 0))
NT1 = int(os.environ.get('NT1', 3))
LEAD = int(os.environ.get('LEAD', 448))
PLAN = os.environ.get('PLAN', 'K104,K147,K203,K237,K304 P0 P1,K347 P2 O0,P3 O1 P4 O2 O3,P5 O4 P6 O5').split(',')
LOG2E = 1.4426950408889634

f32 = jnp.float32
bf16 = jnp.bfloat16
u32 = jnp.uint32

SEM_VEC, SEM_B, SEM_X, SEM_WQ, SEM_C, SEM_SL, SEM_WO, SEM_OUT, SEM_WQ1 = 0, 1, 2, 6, 7, 8, 16, 17, 18
NSEM = 22


def _dot(a, b, dims):
    return lax.dot_general(a, b, (dims, ((), ())), preferred_element_type=f32)


_NN = ((1,), (0,))
_NT = ((1,), (1,))
_TN = ((0,), (0,))
_TT = ((0,), (1,))


def _pk(x):
    return pltpu.bitcast(x, u32)


def _up(x):
    return pltpu.bitcast(x, bf16)


class _Stack:
    def __init__(self, ref, rows, along_lanes=False):
        self.ref, self.rows, self.along_lanes = ref, rows, along_lanes

    def _idx(self, n, r0, nr, cols):
        lo = r0 // 2 if isinstance(r0, int) else lax.shift_right_logical(r0, 1)
        nr = (self.rows if nr is None else nr) // 2
        if self.along_lanes:
            return _ds(lo, nr, 8), pl.ds(n * 128, 128)
        return _ds(n * (self.rows // 2) + lo, nr, 8), (slice(None) if cols is None else cols)

    def get(self, n, r0=0, nr=None, cols=None):
        return _up(self.ref[self._idx(n, r0, nr, cols)])

    def put(self, n, r0, x, cols=None):
        self.ref[self._idx(n, r0, x.shape[0], cols)] = _pk(x)


def _tie(x, clock):
    if clock is None:
        return x
    never, tick = clock
    r, c = x.shape
    if tick.dtype != x.dtype:
        tick = pltpu.bitcast(tick, x.dtype)
    tile = lambda v: jnp.tile(v, (r // 8, c // 128))
    return jnp.where(tile(never), tile(tick), x)


def _cmul(ar, ai, br, bi):
    return ar * br - ai * bi, ar * bi + ai * br


def _ds(lo, n, align):
    return pl.ds(lo if isinstance(lo, int) else pl.multiple_of(lo, align), n)


def _strassen_a(a11, a12, a21, a22):
    ops = [a11 + a22, a21 + a22, a11, a22, a11 + a12, a21 - a11, a12 - a22]
    return [o.astype(bf16) for o in ops]


def _strassen_b(b11, b12, b21, b22, dtype=bf16):
    ops = [b11 + b22, b11, b12 - b22, b21 - b11, b22, b11 + b12, b21 + b22]
    return [o.astype(dtype) for o in ops]


_A_TERMS = ((0, 3, 1), (2, 3, 1), (0, None, 0), (3, None, 0), (0, 1, 1), (2, 0, -1), (1, 3, -1))
_B_TERMS = ((0, 3, 1), (0, None, 0), (1, 3, -1), (2, 0, -1), (3, None, 0), (0, 1, 1), (2, 3, 1))


def _strassen2_ops(block, terms, inner, clock, emit, outer=range(7)):
    for n1 in outer:
        x, y, sign = terms[n1]
        sub = []
        for q in range(4):
            v = block(x, q)
            if q in (0, 3):
                v = _tie(v, clock(n1))
            if y is not None:
                v = v + block(y, q) if sign > 0 else v - block(y, q)
            sub.append(v)
        for n2, op in enumerate(inner(*sub)):
            emit(7 * n1 + n2, op)


def _strassen_c(m, only=None):
    c = (lambda: (m[0] + m[3]) + (m[6] - m[4]),
         lambda: m[2] + m[4],
         lambda: m[1] + m[3],
         lambda: (m[0] - m[1]) + (m[2] + m[5]))
    return [f() for f in c] if only is None else c[only]()


def _stage(raw, r0, stg, c0, nc, clock=None, groups=(0, 1)):
    for ht in groups:
        for dt in range(2):
            v = raw[pl.ds(r0, nc), ht * 8:(ht + 1) * 8, dt * 128:(dt + 1) * 128]
            stg[ht * 2 + dt, _ds(c0 * 4, nc * 4, 8), :] = _tie(_pk(v.reshape(nc * 8, 128)), clock)


def _pair_words(stg, pair, rows):
    ht = lax.shift_right_logical(pair, 2)
    return [stg[ht * 2 + dt, pl.ds(pair & 3, rows, stride=4), :] for dt in range(2)]


def _weight_ops(halves, rows, dtype=bf16):
    r = rows // 2
    return _strassen_b(halves[0][:r], halves[1][:r], halves[0][r:], halves[1][r:], dtype)


class _Clock:
    def __init__(self, never):
        self.never, self.ticks, self.t = never, [], 0

    def stage(self, duration, vals):
        for k, v in enumerate(vals):
            self.ticks.append((self.t + duration * (k + 1) / len(vals), v))
        self.t += duration

    def pacer(self, t0, t1):
        def clocks(k, n):
            want = t0 + (t1 - t0) * k / n
            best = [v for t, v in self.ticks if t <= want]
            return (self.never, best[-1]) if best else None
        return clocks


def _rows8(vals, step=8):
    return [v[r:r + 8, 0:128] for v in vals for r in range(0, v.shape[0], step)]


def _ssm_cmat(craw_s, coef_s, c_s, clocks):
    for r in range(0, M, 16):
        coef = _tie(coef_s[...], clocks(r // 16, M // 16))
        cr, ci = coef[0:1, :M], coef[1:2, :M]
        cp_re, cp_im = _cmul(craw_s[0, r:r + 16, :].astype(f32), craw_s[1, r:r + 16, :].astype(f32), cr, ci)
        c_s[r // 2:r // 2 + 8, :] = _pk(jnp.concatenate(
            [cp_re[:, :PA], -cp_im[:, :PA], cp_re[:, PA:], -cp_im[:, PA:]], axis=1).astype(bf16))


def _ssm_params(vec_s, coef_s, lam_s, col_s, zero_s):
    row = lambda r: r[...].astype(f32).reshape(1, M)
    lre, lim, ldt, dsk, gw = [row(v) for v in vec_s]
    dt = jnp.exp(ldt).astype(bf16).astype(f32)
    mag = jnp.exp(dt * lre)
    ang = dt * lim
    lr, li = mag * jnp.cos(ang), mag * jnp.sin(ang)
    den = lre * lre + lim * lim
    nr = lr - 1.0
    coef_s[...] = jnp.zeros(coef_s.shape, f32)
    coef_s[0:1, 0:M] = 2.0 * ((nr * lre + li * lim) / den)
    coef_s[1:2, 0:M] = 2.0 * ((li * lre - nr * lim) / den)
    zero_s[...] = jnp.zeros(zero_s.shape, f32)

    er = jnp.concatenate([lr, lr[:, PA:]], axis=1)
    ei = jnp.concatenate([li, -li[:, PA:]], axis=1)
    pw = [(er, ei)]
    for _ in range(7):
        pw.append(_cmul(pw[-1][0], pw[-1][1], er, ei))
    sub = lax.broadcasted_iota(jnp.int32, (8, 512), 0)
    for n, d in enumerate((1, 2, 4)):
        lam_s[2 * n] = jnp.where(sub >= d, pw[d - 1][0], 0.0)
        lam_s[2 * n + 1] = jnp.where(sub >= d, pw[d - 1][1], 0.0)
    lcr = jnp.zeros((8, 512), f32)
    lci = jnp.zeros((8, 512), f32)
    for r in range(8):
        lcr = jnp.where(sub == r, pw[r][0], lcr)
        lci = jnp.where(sub == r, pw[r][1], lci)
    lam_s[6] = lcr
    lam_s[7] = lci

    def col(v):
        v = jnp.concatenate([v, jnp.zeros((1, 512 - M), f32)], axis=1)
        return jnp.broadcast_to(v, (128, 512)).T[:M]
    col_s[0] = col(dsk)
    col_s[1] = col(gw)


def _ssm_scan(u_s, t0, carry, lam_s, h_s, clocks):
    car, cai = carry
    out = []
    for b in range(TC // 8):
        u = u_s[_ds(t0 + b * 8, 8, 8), :]
        mixed = u[:, 2 * PA:]
        cols = [u[:, 0:128], u[:, 128:256], u[:, 256:384], mixed]
        hr = jnp.concatenate([_tie(v, clocks(4 * b + n, TC // 2)) for n, v in enumerate(cols)], axis=1)
        hi = jnp.concatenate([u[:, PA:2 * PA], pltpu.roll(mixed, PB, 1)], axis=1)
        for n, d in enumerate((1, 2, 4)):
            sr, si = pltpu.roll(hr, d, 0), pltpu.roll(hi, d, 0)
            tr, ti = _cmul(sr, si, lam_s[2 * n], lam_s[2 * n + 1])
            hr, hi = hr + tr, hi + ti
        tr, ti = _cmul(lam_s[6], lam_s[7], car, cai)
        hr, hi = hr + tr, hi + ti
        car, cai = hr[7:8, :], hi[7:8, :]
        out.append(jnp.concatenate([hr[:, :PA], hi[:, :PA], hr[:, PA:]], axis=1))
        if b % 2 == 1:
            h_s[(b // 2) * 8:(b // 2 + 1) * 8, :] = _pk(jnp.concatenate(out, axis=0).astype(bf16))
            out = []
    return car, cai


def _kernel(xT_hbm, bre_hbm, bim_hbm, cre_hbm, cim_hbm, lre_hbm, lim_hbm, ldt_hbm,
            dsk_hbm, gw_hbm, woT_hbm, ckv_hbm, wq_hbm, wk_hbm, wv_hbm,
            out_hbm,
            xT_s, v0, v1, v2, v3, v4, b_s, craw_s, c_s, coef_s, lam_s, col_s, u_s, g_s,
            ckv_s, rq, rk, rv, sq, sk, sv, a_s, xa_s, q_s, wo_s,
            ka_s, va_s, pb_s, o_s, s_s, h_s, zero_s, wl_s, cl_s, w_s,
            wkt_s, wvt_s, mk_s, mv_s, kt_s, sink_s, sem):
    h = pl.program_id(0)
    vec_s = (v0, v1, v2, v3, v4)
    a_s, xa_s, q_s = _Stack(a_s, S // 4), _Stack(xa_s, HM), _Stack(q_s, D)
    ka_s, va_s, pb_s = _Stack(ka_s, S // 2, True), _Stack(va_s, HD), _Stack(pb_s, S // 2, True)
    w_s = _Stack(w_s, 2 * QD)
    wl_s, cl_s = _Stack(wl_s, HM, True), _Stack(cl_s, HD, True)

    def slice_copies(i):
        s = sem.at[SEM_SL + i]
        grp = i // 2 if isinstance(i, int) else lax.shift_right_logical(i, 1)
        cs, dst = pl.ds(i * CS, CS), pl.ds((i & (NRAW - 1)) * CS, CS)
        return [pltpu.make_async_copy(ckv_hbm.at[grp, :, i & 1], ckv_s.at[grp, :, i & 1], s),
                pltpu.make_async_copy(wk_hbm.at[cs], rk.at[dst], s),
                pltpu.make_async_copy(wv_hbm.at[cs], rv.at[dst], s)]

    def wq1_copy(i):
        rows = pl.ds(i * (M // 4), M // 4)
        return pltpu.make_async_copy(wq_hbm.at[rows, 8:16], rq.at[rows, 8:16], sem.at[SEM_WQ1 + i])

    def x_copy(i):
        cols = _ds(i * TA, TA, TA)
        return pltpu.make_async_copy(xT_hbm.at[:, cols], xT_s.at[:, cols], sem.at[SEM_X + i])

    def out_copy(jp):
        cols = pl.ds(jp * 2 * T, 2 * T)
        return pltpu.make_async_copy(o_s.at[:, cols], out_hbm.at[:, cols], sem.at[SEM_OUT])

    def prep_w(hh, clocks, outer):
        base = lax.shift_right_logical(hh, 1) * D
        sh = (16 * (1 - (hh & 1))).astype(u32)
        k = 0
        for row0, wt_s in ((0, wkt_s), (QD, wvt_s)):
            for r in range(0, QD, 16):
                for u in range(0, QC, T):
                    def block(o, q):
                        row = (o % 2) * HD + (q % 2) * QD + r
                        col = (o // 2) * 2 * QC + (q // 2) * QC + u
                        w = wt_s[_ds(base + row, 16, 16), col:col + T]
                        return pltpu.bitcast((w << sh) & jnp.uint32(0xFFFF0000), f32)
                    _strassen2_ops(block, _B_TERMS, _strassen_b,
                                   lambda n1: clocks(len(outer) * k + n1 - outer[0], 16 * len(outer)),
                                   lambda n, op: w_s.put(n, row0 + r, op, pl.ds(u, T)), outer)
                    k += 1

    @pl.when(h == 0)
    def _():
        cp_vec = [pltpu.make_async_copy(src, dst, sem.at[SEM_VEC])
                  for src, dst in zip((lre_hbm, lim_hbm, ldt_hbm, dsk_hbm, gw_hbm), vec_s)]
        cp_b = [pltpu.make_async_copy(src.at[pl.ds(lo, n)], b_s.at[pl.ds(dst, n)], sem.at[SEM_B])
                for src, lo, n, dst in ((bre_hbm, 0, PA, 0), (bim_hbm, 0, PA, PA),
                                        (bre_hbm, PA, PB, 2 * PA), (bim_hbm, PA, PB, 2 * PA + PB))]
        cp_wq = [pltpu.make_async_copy(wq_hbm.at[:, 0:8], rq.at[:, 0:8], sem.at[SEM_WQ])]
        cp_c = [pltpu.make_async_copy(src, craw_s.at[n], sem.at[SEM_C])
                for n, src in enumerate((cre_hbm, cim_hbm))]
        cp_wo = pltpu.make_async_copy(woT_hbm, wo_s, sem.at[SEM_WO])
        for cp in cp_vec + cp_b:
            cp.start()
        for i in range(S // TA):
            x_copy(i).start()
        for cp in cp_c + cp_wq:
            cp.start()
        for i in range(NRAW - 1):
            wq1_copy(i).start()
            for cp in slice_copies(i):
                cp.start()
        wq1_copy(3).start()
        cp_wo.start()

        def phase1(i):
            u = _dot(xT_s[:, _ds(i * TA, TA, TA)], b_s[...], _TT)
            u_s[_ds(i * TA, TA, TA), :] = u
            never = zero_s[...] != 0.0

            def clocks(k, n):
                pos = (k * 6 * TA // n) // 8 * 8
                return never, u[pos % TA:pos % TA + 8, (pos // TA) * 128:(pos // TA + 1) * 128]

            for t in range(TA // (2 * T)):
                ev = _ds(i * TA + 2 * t * T, T, T)
                od = _ds(i * TA + (2 * t + 1) * T, T, T)
                for r in range(0, HM, 32):
                    top, bot = pl.ds(r, 32), pl.ds(HM + r, 32)
                    clk = clocks(t * 7 + r // 32, 14)
                    ops = _strassen_a(_tie(xT_s[top, ev].astype(f32), clk), xT_s[bot, ev].astype(f32),
                                      xT_s[top, od].astype(f32), _tie(xT_s[bot, od].astype(f32), clk))
                    for n in range(7):
                        xa_s.put(n, r, ops[n], _ds(i * (TA // 2) + t * T, T, T))
            return clocks

        wl_s.ref[...] = jnp.zeros(wl_s.ref.shape, u32)
        cl_s.ref[...] = jnp.zeros(cl_s.ref.shape, u32)
        for cp in cp_vec:
            cp.wait()
        _ssm_params(vec_s, coef_s, lam_s, col_s, zero_s)
        for cp in cp_b:
            cp.wait()

        x_copy(0).wait()
        phase1(0)
        x_copy(1).wait()
        clocks = phase1(1)
        zero = jnp.zeros((1, 512), f32)
        carry0 = _ssm_scan(u_s, 0, (zero, zero), lam_s, h_s, clocks)
        for cp in [x_copy(2), x_copy(3)] + cp_c + cp_wq:
            cp.wait()
        clocks = phase1(2)
        _ssm_cmat(craw_s, coef_s, c_s, clocks)
        clocks = phase1(3)
        for c0 in range(0, M, 8):
            _stage(rq, c0, sq, c0, 8, clocks(c0 // 8, M // 8), groups=(0,))

        def phase2(i, carry):
            @pl.when(i + NRAW - 1 < NP)
            def _():
                for cp in slice_copies(i + NRAW - 1):
                    cp.start()

            @pl.when(i < 4)
            def _():
                wq1_copy(i).wait()

            for cp in slice_copies(i):
                cp.wait()
            yT = _dot(_up(c_s[...]), _up(h_s[...]), _NT)
            for t in range(TC // T):
                cols = _ds(i * TC + t * T, T, T)
                acc = jnp.zeros((8, T), f32)
                for r in range(0, M, 32):
                    xg = xT_s[r:r + 32, cols].astype(f32) * col_s[1, r:r + 32, :]
                    acc = acc + jnp.sum(xg.reshape(4, 8, T), axis=0)
                g = jax.nn.sigmoid(jnp.sum(acc, axis=0, keepdims=True))
                g_s[:, cols] = g
                for r in range(0, M, 32):
                    skip = xT_s[r:r + 32, cols].astype(f32) * col_s[0, r:r + 32, :]
                    o_s[r:r + 32, cols] = (1.0 - g) * (yT[r:r + 32, t * T:(t + 1) * T] + skip)

            words = _pair_words(sq, i, M)
            lo = _weight_ops([pltpu.bitcast(u << 16, f32) for u in words], M, f32)
            hi = _weight_ops([pltpu.bitcast(u & jnp.uint32(0xFFFF0000), f32) for u in words], M, f32)
            prods = [_dot(jnp.concatenate([lo[n], hi[n]], axis=1).astype(bf16), xa_s.get(n), _TN)
                     for n in range(7)]
            qs = LOG2E * D ** -0.5
            for n in (2, 1, 3, 0):
                for t in range(NP):
                    for r in range(0, D, G):
                        c = _strassen_c([v[r:r + G, t * T:(t + 1) * T] for v in prods], n)
                        q_s.put(4 * i + 2 * (r // HD) + n // 2, (n % 2) * HD + r % HD,
                                (c * qs).astype(bf16), pl.ds(t * T, T))

            never = zero_s[...] != 0.0

            def clocks(k, n):
                pos = (k * 5 * 1024 // n) // 8 * 8
                r, c = pos % 256, (pos % 1024) // 256 * 256
                return never, prods[pos // 1024][r:r + 8, c:c + 128]

            carry = _ssm_scan(u_s, jnp.minimum(i + 1, NP - 1) * TC, carry, lam_s, h_s, clocks)

            for c0 in range(0, M // 4, 8):
                r0 = (i & 3) * (M // 4) + c0
                _stage(rq, r0, sq, r0, 8, clocks(4 * (c0 // 8) + 2, 64), groups=(1,))
            for c0 in range(0, CS, 8):
                r0 = (i & (NRAW - 1)) * CS + c0
                _stage(rk, r0, sk, c0, 8, clocks(c0 // 8, 64))
                _stage(rv, r0, sv, c0, 8, clocks(16 + c0 // 8, 64))
            for n, (stg, wt_s) in enumerate(((sk, wkt_s), (sv, wvt_s))):
                for pair in range(H // 2):
                    for dt in range(2):
                        blk = stg[(pair // 4) * 2 + dt, pl.ds(pair % 4, CS, stride=4), :]
                        blk = _tie(blk, clocks(16 + 24 * n + 3 * pair + dt, 64))
                        wt_s[pair * D + dt * HD:pair * D + (dt + 1) * HD, _ds(i * CS, CS, CS)] = blk.T
            grp, half = lax.shift_right_logical(i, 1), i & 1
            k = 0
            for r in range(0, T // 2, 16):
                for u in range(0, QC, T):
                    def block(o, q):
                        col = (o % 2) * 2 * QC + (q % 2) * QC + u
                        return ckv_s[grp, 2 * (q // 2) + o // 2, half, r:r + 16, col:col + T].astype(f32)
                    _strassen2_ops(block, _A_TERMS, _strassen_a, lambda n1: clocks(7 * k + n1, 56),
                                   lambda n, op: a_s.put(n, i * (T // 2) + r, op, pl.ds(u, T)))
                    k += 1
            return carry

        lax.fori_loop(0, NP, phase2, carry0)
        cp_wo.wait()
        prep_w(h, lambda k, n: None, range(NT1))

    clk = _Clock(zero_s[...] != 0.0)

    def oproj(jp, ops):
        m = [_dot(wl_s.get(i), ops[i], _NN) for i in range(7)]
        for r in range(0, HM, G):
            for n, c in enumerate(_strassen_c([v[r:r + G] for v in m])):
                o_s[pl.ds((n // 2) * HM + r, G), pl.ds((2 * jp + n % 2) * T, T)] += c
        clk.stage(392, _rows8([m[0], m[4]]))

    def prep_wo(clocks):
        for r in range(0, HM, G):
            top = _tie(wo_s[h, r:r + G, :].astype(f32), clocks(r // G, HM // G))
            bot = _tie(wo_s[h, HM + r:HM + r + G, :].astype(f32), clocks(r // G, HM // G))
            for n, w in enumerate(_strassen_a(top[:, :HD], top[:, HD:], bot[:, :HD], bot[:, HD:])):
                wl_s.put(n, r, w)

    def proj(g, lo, hi):
        for n1 in range(lo, hi):
            m = [_dot(w_s.get(7 * n1 + n), a_s.get(7 * n1 + n, g * T, T), _NT) for n in range(7)]
            for r in range(0, 2 * QD, G):
                m_s = mk_s if r < QD else mv_s
                for n, c in enumerate(_strassen_c([v[r:r + G] for v in m])):
                    row = n1 * HD + (n % 2) * QD + r % QD
                    m_s[row:row + G, (n // 2) * T:(n // 2 + 1) * T] = c
            clk.stage(448, _rows8(m[0::2], 16))
        if hi == 7:
            kfin(g)
            vfin(g)

    def outer(m_s, r, nr, a2):
        return _strassen_c([m_s[n * HD + r:n * HD + r + nr, a2 * T:(a2 + 1) * T] for n in range(7)])

    def nine(c11, c12, c21, c22):
        return _strassen_a(c11, c12, c21, c22) + [c12.astype(bf16), c21.astype(bf16)]

    def kfin(g):
        for a2 in range(2):
            cs = [outer(mk_s, r, G, a2) for r in range(0, HD, G)]
            for n in range(4):
                kt_s[:, (a2 * 4 + n) * T:(a2 * 4 + n + 1) * T] = jnp.concatenate([c[n] for c in cs], axis=0).T
            for r in range(0, T, G):
                blk = [kt_s[r:r + G, (a2 * 4 + n) * T:(a2 * 4 + n + 1) * T] for n in range(4)]
                for n, op in enumerate(nine(*blk)):
                    ka_s.put(n, (2 * g + a2) * T + r, op)

    def vfin(g):
        for a2 in range(2):
            for r in range(0, HD, G):
                c11, c21, c12, c22 = outer(mv_s, r, G, a2)
                for n, op in enumerate(nine(c11, c12, c21, c22)):
                    va_s.put(n, r, op, pl.ds((2 * g + a2) * T, T))

    key = lax.broadcasted_iota(jnp.int32, (T, T), 0)
    qry = lax.broadcasted_iota(jnp.int32, (T, T), 1)
    causal = key <= qry

    class Reducer:
        def __init__(self, red, comb):
            self.red, self.comb, self.acc, self.rows, self.out = red, comb, None, 0, None

        def add(self, v):
            v = self.red(v.reshape(v.shape[0] // 8, 8, T), axis=0)
            self.acc = v if self.acc is None else self.comb(self.acc, v)
            self.rows += 1
            if self.rows * G >= RCH:
                self.flush()

        def flush(self):
            if self.acc is not None:
                v = self.red(self.acc, axis=0, keepdims=True)
                self.out = v if self.out is None else self.comb(self.out, v)
            self.acc, self.rows = None, 0

        def result(self):
            self.flush()
            return self.out

    def qk(jp):
        R, slot = jp * T, jp % 2
        cols = pl.ds(jp * T, T)
        qe, qo = q_s.get(2 * h, cols=cols), q_s.get(2 * h + 1, cols=cols)
        mx = [Reducer(jnp.max, jnp.maximum) for _ in range(2)]

        def put(e, row, v):
            s_s[slot, e, row:row + G, :] = v
            mx[e].add(v)

        if jp > 0:
            qef, qof = qe.astype(f32), qo.astype(f32)
            qb = _strassen_b(qef[:HD], qof[:HD], qef[HD:], qof[HD:])
            for r0 in range(0, R, QCH):
                r1 = min(r0 + QCH, R)
                m = [_dot(ka_s.get(n, r0, r1 - r0), qb[n], _NN) for n in range(7)]
                for r in range(0, r1 - r0, G):
                    c11, c12, c21, c22 = _strassen_c([v[r:r + G] for v in m])
                    put(0, r0 + r, c11)
                    put(1, r0 + r, c12)
                    put(0, R + r0 + r, c21)
                    put(1, R + r0 + r, c22)
                clk.stage(7 * (r1 - r0) / 4, _rows8([m[0], m[4]]))
        ke = jnp.concatenate([ka_s.get(2, R, T), ka_s.get(7, R, T)], axis=1)
        ko = jnp.concatenate([ka_s.get(8, R, T), ka_s.get(3, R, T)], axis=1)
        se = _dot(ke, jnp.concatenate([qe, qo], axis=1), _NN)
        so = _dot(ko, qo, _NN)
        for r in range(0, T, G):
            put(0, 2 * R + r, jnp.where(causal[r:r + G], se[r:r + G, :T], -1e30))
            put(1, 2 * R + r, se[r:r + G, T:])
            put(1, 2 * R + T + r, jnp.where(causal[r:r + G], so[r:r + G], -1e30))
        clk.stage(192, _rows8([se]))
        return [jnp.broadcast_to(x.result(), (8, T)) for x in mx]

    pull = [0]

    def pb0(jp):
        return jp * (jp - 1) // 2 * T

    def shifted_exp(slot, e, row, z):
        v = s_s[slot, e, row:row + G, :].reshape(G // 8, 8, T) - z[None]
        return jnp.exp2(v).reshape(G, T)

    def softmax(jp, mx, t0, t1, t2=None, t3=None):
        R, slot = jp * T, jp % 2
        if t2 is None:
            t1, t2, t3 = (t0 + t1) / 2, (t0 + t1) / 2, t1
        clocks = clk.pacer(t0, t1)
        k, n = 0, (4 * jp + 3) * T // G
        z = []
        for e in range(2):
            sm = Reducer(jnp.sum, jnp.add)
            for r in range(0, (2 * jp + 1 + e) * T, G):
                sm.add(shifted_exp(slot, e, r, _tie(mx[e], clocks(k, n))))
                k += 1
                if PULL and k % PULL == 0 and sm.acc is not None:
                    sink_s[pull[0] * 8:(pull[0] + 1) * 8, :] = sm.acc
                    pull[0] += 1
            z.append(mx[e] + jnp.log2(sm.result()))
        clocks = clk.pacer(t2, t3)
        k = 0
        for r in range(0, R, G):
            ze, zo = _tie(z[0], clocks(k, n)), _tie(z[1], clocks(k + 2, n))
            ops = _strassen_b(shifted_exp(slot, 0, r, ze), shifted_exp(slot, 1, r, zo),
                              shifted_exp(slot, 0, R + r, ze), shifted_exp(slot, 1, R + r, zo))
            for i in range(7):
                pb_s.put(i, pb0(jp) + r, ops[i])
            k += 4
        for r in range(0, 3 * T, G):
            e = int(r >= T)
            p = shifted_exp(slot, e, 2 * R + r - e * T, _tie(z[e], clocks(k, n)))
            pb_s.put(7, jp * 3 * T + r, p.astype(bf16))
            k += 1

    def pv(jp):
        R, slot = jp * T, jp % 4
        if jp > 0:
            m = [_dot(va_s.get(n, cols=pl.ds(0, R)), pb_s.get(n, pb0(jp), R), _NN) for n in range(7)]
            clk.stage(7 * R / 4, _rows8(m, 32))
        cols = pl.ds(R, T)
        ve = jnp.concatenate([va_s.get(2, cols=cols), va_s.get(8, cols=cols)], axis=0)
        vo = jnp.concatenate([va_s.get(7, cols=cols), va_s.get(3, cols=cols)], axis=0)
        ce = _dot(ve, pb_s.get(7, jp * 3 * T, T), _NN)
        co = _dot(jnp.concatenate([ve, vo], axis=1), pb_s.get(7, jp * 3 * T + T, 2 * T), _NN)
        clk.stage(192, _rows8([ce], 32))
        ge = g_s[:, 2 * jp * T:(2 * jp + 1) * T]
        go = g_s[:, (2 * jp + 1) * T:(2 * jp + 2) * T]
        for r in range(0, HD, G):
            c = [ce[r:r + G], co[r:r + G], ce[HD + r:HD + r + G], co[HD + r:HD + r + G]]
            if jp > 0:
                c = [x + y for x, y in zip(c, _strassen_c([v[r:r + G] for v in m]))]
            ops = _strassen_b(c[0] * ge, c[1] * go, c[2] * ge, c[3] * go)
            for n in range(7):
                cl_s.put(slot * 7 + n, r, ops[n])

    def ctx_ops(jp):
        return [cl_s.get((jp % 4) * 7 + n) for n in range(7)]

    def oproj_out(jp):
        oproj(jp, ctx_ops(jp))

        @pl.when(h == H - 1)
        def _():
            out_copy(jp).start()

    for n1 in range(7):
        if n1 >= NT1:
            prep_w(h, clk.pacer(max(clk.t - LEAD - 448, 1), max(clk.t - LEAD, 1)), range(n1, n1 + 1))
        proj(0, n1, n1 + 1)
    oproj(NP - 1, ctx_ops(NP - 1))
    for jp, cover in enumerate(PLAN):
        mx = qk(jp)
        t0 = clk.t
        for item in cover.split():
            if item[0] == 'P':
                pv(int(item[1]))
            elif item[0] == 'O':
                oproj_out(int(item[1]))
            else:
                proj(int(item[1]), int(item[2]), int(item[3]))
        softmax(jp, mx, t0 + D0, clk.t - SLACK)
        if jp == 0:
            prep_wo(clk.pacer(t0, clk.t))
    t0 = clk.t
    if FIN:
        oproj_out(NP - 2)
        pv(NP - 1)
    else:
        pv(NP - 1)
        oproj_out(NP - 2)
    prep_w(jnp.minimum(h + 1, H - 1), clk.pacer(t0 - PW0, clk.t - 300), range(NT1))

    @pl.when(h == H - 1)
    def _():
        oproj(NP - 1, ctx_ops(NP - 1))
        out_copy(NP - 1).start()
        for jp in range(NP):
            out_copy(jp).wait()


@jax.jit
def pallas_gated_mix__compressed_kv_cla__ssm_conv_s5__prompt_kernel(
    A_x: jax.Array,
    A_c_kv: jax.Array,
    A_w_q: jax.Array,
    A_w_uk: jax.Array,
    A_w_uv: jax.Array,
    A_w_o: jax.Array,
    B_x: jax.Array,
    B_Lambda_re: jax.Array,
    B_Lambda_im: jax.Array,
    B_B_re: jax.Array,
    B_B_im: jax.Array,
    B_C_re: jax.Array,
    B_C_im: jax.Array,
    B_log_dt: jax.Array,
    B_Dskip: jax.Array,
    gate_w: jax.Array,
):
    del B_x
    xT = jnp.transpose(A_x[0])
    woT = jnp.transpose(A_w_o, (0, 2, 1))
    ckv = A_c_kv.reshape(4, 4, 2, T // 2, DC)

    hbm = pl.BlockSpec(memory_space=pl.ANY)
    vmem = pltpu.VMEM
    outT = pl.pallas_call(
        _kernel,
        grid=(H,),
        in_specs=[hbm] * 15,
        out_specs=hbm,
        out_shape=jax.ShapeDtypeStruct((M, S), f32),
        scratch_shapes=[
            vmem((M, S), bf16),
            vmem((M,), bf16), vmem((M,), bf16), vmem((M,), bf16), vmem((M,), bf16), vmem((M,), bf16),
            vmem((2 * M, M), bf16),
            vmem((2, M, M), bf16),
            vmem((M // 2, 2 * M), u32),
            vmem((8, 512), f32),
            vmem((8, 8, 512), f32),
            vmem((2, M, 128), f32),
            vmem((S, 2 * M), f32),
            vmem((1, S), f32),
            vmem((4, 4, 2, T // 2, DC), bf16),
            vmem((M, H, D), bf16),
            vmem((NRAW * CS, H, D), bf16),
            vmem((NRAW * CS, H, D), bf16),
            vmem((4, M * 4, 128), u32),
            vmem((4, CS * 4, 128), u32),
            vmem((4, CS * 4, 128), u32),
            vmem((49 * S // 8, QC), u32),
            vmem((7 * HM // 2, S // 2), u32),
            vmem((H * D, S // 2), u32),
            vmem((H, M, D), bf16),
            vmem((S // 4, 9 * HD), u32),
            vmem((9 * HD // 2, S // 2), u32),
            vmem((14 * T, 8 * T), u32),
            vmem((M, S), f32),
            vmem((2, 2, S, T), f32),
            vmem((TC // 2, 2 * M), u32),
            vmem((8, 128), f32),
            vmem((HM // 2, 7 * HD), u32),
            vmem((HD // 2, 28 * T), u32),
            vmem((49 * QD, QC), u32),
            vmem((H // 2 * D, DC), u32),
            vmem((H // 2 * D, DC), u32),
            vmem((7 * HD, 2 * T), f32),
            vmem((7 * HD, 2 * T), f32),
            vmem((T, 8 * T), f32),
            vmem((544 * 8, T), f32),
            pltpu.SemaphoreType.DMA((NSEM,)),
        ],
        compiler_params=pltpu.CompilerParams(
            dimension_semantics=("arbitrary",),
            vmem_limit_bytes=126 * 1024 * 1024,
        ),
    )(xT, B_B_re, B_B_im, B_C_re, B_C_im, B_Lambda_re, B_Lambda_im, B_log_dt,
      B_Dskip, gate_w, woT, ckv, A_w_q, A_w_uk, A_w_uv)
    return jnp.transpose(outT)[None]
```

```python
import os

import jax
import jax.numpy as jnp
from jax import lax
import jax.experimental.pallas as pl
import jax.experimental.pallas.tpu as pltpu

S = 2048
M = 448
H = 16
D = 256
DC = 1024
T = 128
NP = S // T // 2
HD = D // 2
HM = M // 2
QD = D // 4
QC = DC // 4
PA = 384
PB = M - PA
TA = 512
TC = 256
CS = DC // NP
NRAW = 4
LOG2E = 1.4426950408889634
NEG = -1e30

_env = lambda k, d: type(d)(os.environ.get(k, d))
GC = _env('GC', 32)
GS = _env('GS', 16)
RCH = _env('RCH', 256)
SLACK = _env('SLACK', 200)
D0 = _env('D0', 0)
PULL = _env('PULL', 2)
NT1 = _env('NT1', 3)
LEAD = _env('LEAD', 448)
PW0 = _env('PW0', 100)
PLAN = _env('PLAN', 'K104,K147,K203,K237,K304 P0 P1,K347 P2 O0,P3 O1 P4 O2 O3,P5 O4 P6 O5').split(',')

f32 = jnp.float32
bf16 = jnp.bfloat16
u32 = jnp.uint32

SEM_VEC, SEM_B, SEM_X, SEM_WQ, SEM_C, SEM_SL, SEM_WO, SEM_OUT, SEM_WQ1 = 0, 1, 2, 6, 7, 8, 16, 17, 18
NSEM = 22

_NN = ((1,), (0,))
_NT = ((1,), (1,))
_TN = ((0,), (0,))
_TT = ((0,), (1,))


def _dot(a, b, dims):
    return lax.dot_general(a, b, (dims, ((), ())), preferred_element_type=f32)


def _cat(xs, axis):
    return xs[0] if len(xs) == 1 else jnp.concatenate(xs, axis=axis)


def _ds(lo, n, align):
    return pl.ds(lo if isinstance(lo, int) else pl.multiple_of(lo, align), n)


def _put(ref, row, col, xs):
    x = _cat(xs, 1)
    ref[row // 2:(row + x.shape[0]) // 2, col:col + x.shape[1]] = pltpu.bitcast(x.astype(bf16), u32)


def _get(ref, row, nrows, col, ncols):
    return pltpu.bitcast(ref[row // 2:(row + nrows) // 2, col:col + ncols], bf16)


class _Clock:
    def __init__(self, zero_ref):
        self.masks = {(8, T): zero_ref[...] != 0.0}
        self.ticks, self.t = [], 0

    def stage(self, duration, vals, step=8, cols=(0,)):
        where = [(v, r, c) for v in vals for c in cols for r in range(0, v.shape[0], step)]
        for k, w in enumerate(where):
            self.ticks.append((self.t + duration * (k + 1) / len(where), w))
        self.t += duration

    def pacer(self, t0, t1, n):
        def tie(x, k):
            past = [w for t, w in self.ticks if t <= t0 + (t1 - t0) * k / n]
            if not past:
                return x
            v, r, c = past[-1]
            tick = v[r:r + 8, c:c + T]
            if tick.dtype != x.dtype:
                tick = pltpu.bitcast(tick, x.dtype)
            reps = (x.shape[0] // 8, x.shape[1] // T)
            if x.shape not in self.masks:
                self.masks[x.shape] = jnp.tile(self.masks[(8, T)], reps)
            return lax.select(self.masks[x.shape], tick if reps == (1, 1) else jnp.tile(tick, reps), x)
        return tie


def _no_tie(x, k):
    return x


_A_TERMS = ((0, 3, 1), (2, 3, 1), (0, None, 0), (3, None, 0), (0, 1, 1), (2, 0, -1), (1, 3, -1))
_B_TERMS = ((0, 3, 1), (0, None, 0), (1, 3, -1), (2, 0, -1), (3, None, 0), (0, 1, 1), (2, 3, 1))


def _operand(term, block):
    x, y, sign = term
    if y is None:
        return block(x)
    return block(x) + block(y) if sign > 0 else block(x) - block(y)


def _operands(terms, blocks):
    return [_operand(t, blocks.__getitem__) for t in terms]


def _operands2(terms, n1, block, tie):
    first = terms[n1][0]
    sub = [_operand(terms[n1], lambda o: tie(block(o, q)) if o == first and q in (0, 3) else block(o, q))
           for q in range(4)]
    return _operands(terms, sub)


def _combine(m, only=(0, 1, 2, 3)):
    c = (lambda: (m[0] + m[3]) + (m[6] - m[4]),
         lambda: m[2] + m[4],
         lambda: m[1] + m[3],
         lambda: (m[0] - m[1]) + (m[2] + m[5]))
    return [c[n]() for n in only]


class _Tiles:
    def __init__(self, vals, r, n, c=0, w=None):
        self.vals, self.idx, self.cache = vals, (slice(r, r + n), slice(c, None if w is None else c + w)), {}

    def __getitem__(self, i):
        if i not in self.cache:
            self.cache[i] = self.vals[i][self.idx]
        return self.cache[i]


class _Reducer:
    def __init__(self, red, comb):
        self.red, self.comb, self.acc, self.rows, self.out = red, comb, None, 0, None

    def add(self, v):
        self.rows += 8 * v.shape[0]
        v = self.red(v, axis=0)
        self.acc = v if self.acc is None else self.comb(self.acc, v)
        if self.rows >= RCH:
            self.result()

    def result(self):
        if self.acc is not None:
            v = self.red(self.acc, axis=0, keepdims=True)
            self.out = v if self.out is None else self.comb(self.out, v)
        self.acc, self.rows = None, 0
        return self.out


def _cmul(ar, ai, br, bi):
    return ar * br - ai * bi, ar * bi + ai * br


def _hi16(w):
    return pltpu.bitcast(w & jnp.uint32(0xFFFF0000), f32)


def _stage(raw, stg, c0, nc, tie, groups=(0, 1)):
    for ht in groups:
        for dt in range(2):
            v = raw[c0:c0 + nc, ht * 8:(ht + 1) * 8, dt * T:(dt + 1) * T].reshape(nc * 8, T)
            stg[ht * 2 + dt, c0 * 4:(c0 + nc) * 4, :] = tie(pltpu.bitcast(v, u32))


def _ssm_params(vec_s, coef_s, lam_s, col_s):
    row = lambda r: r[...].astype(f32).reshape(1, M)
    lre, lim, ldt, dsk, gw = [row(v) for v in vec_s]
    dt = jnp.exp(ldt).astype(bf16).astype(f32)
    mag = jnp.exp(dt * lre)
    ang = dt * lim
    lr, li = mag * jnp.cos(ang), mag * jnp.sin(ang)
    den = lre * lre + lim * lim
    nr = lr - 1.0
    coef_s[...] = jnp.zeros(coef_s.shape, f32)
    coef_s[0:1, 0:M] = 2.0 * ((nr * lre + li * lim) / den)
    coef_s[1:2, 0:M] = 2.0 * ((li * lre - nr * lim) / den)

    er = jnp.concatenate([lr, lr[:, PA:]], axis=1)
    ei = jnp.concatenate([li, -li[:, PA:]], axis=1)
    pw = [(er, ei)]
    for _ in range(7):
        pw.append(_cmul(pw[-1][0], pw[-1][1], er, ei))
    sub = lax.broadcasted_iota(jnp.int32, (8, 512), 0)
    for n, d in enumerate((1, 2, 4)):
        lam_s[2 * n] = jnp.where(sub >= d, pw[d - 1][0], 0.0)
        lam_s[2 * n + 1] = jnp.where(sub >= d, pw[d - 1][1], 0.0)
    lcr = jnp.zeros((8, 512), f32)
    lci = jnp.zeros((8, 512), f32)
    for r in range(8):
        lcr = jnp.where(sub == r, pw[r][0], lcr)
        lci = jnp.where(sub == r, pw[r][1], lci)
    lam_s[6] = lcr
    lam_s[7] = lci

    def col(v):
        v = jnp.concatenate([v, jnp.zeros((1, 512 - M), f32)], axis=1)
        return jnp.broadcast_to(v, (T, 512)).T[:M]
    col_s[0] = col(dsk)
    col_s[1] = col(gw)


def _ssm_cmat(craw_s, coef_s, c_s, tie):
    for r in range(0, M, 16):
        coef = tie(coef_s[...], r // 16)
        cr, ci = coef[0:1, :M], coef[1:2, :M]
        re, im = _cmul(craw_s[0, r:r + 16, :].astype(f32), craw_s[1, r:r + 16, :].astype(f32), cr, ci)
        _put(c_s, r, 0, [re[:, :PA], -im[:, :PA], re[:, PA:], -im[:, PA:]])


def _ssm_scan(u_ref, carry, lam_s, h_s, tie):
    car, cai = carry
    out = []
    for b in range(TC // 8):
        u = u_ref[b * 8:(b + 1) * 8, :]
        mixed = u[:, 2 * PA:]
        cols = [u[:, 0:T], u[:, T:2 * T], u[:, 2 * T:PA], mixed]
        hr = jnp.concatenate([tie(v, 4 * b + n) for n, v in enumerate(cols)], axis=1)
        hi = jnp.concatenate([u[:, PA:2 * PA], pltpu.roll(mixed, PB, 1)], axis=1)
        for n, d in enumerate((1, 2, 4)):
            sr, si = pltpu.roll(hr, d, 0), pltpu.roll(hi, d, 0)
            tr, ti = _cmul(sr, si, lam_s[2 * n], lam_s[2 * n + 1])
            hr, hi = hr + tr, hi + ti
        tr, ti = _cmul(lam_s[6], lam_s[7], car, cai)
        hr, hi = hr + tr, hi + ti
        car, cai = hr[7:8, :], hi[7:8, :]
        out.append(jnp.concatenate([hr[:, :PA], hi[:, :PA], hr[:, PA:]], axis=1))
        if b % 2 == 1:
            _put(h_s, (b - 1) * 8, 0, [jnp.concatenate(out, axis=0)])
            out = []
    return car, cai


def _kernel(xT_hbm, bre_hbm, bim_hbm, cre_hbm, cim_hbm, lre_hbm, lim_hbm, ldt_hbm,
            dsk_hbm, gw_hbm, woT_hbm, ckv_hbm, wq_hbm, wk_hbm, wv_hbm,
            out_hbm,
            xT_s, v0, v1, v2, v3, v4, b_s, craw_s, c_s, coef_s, lam_s, col_s, u_s, h_s, g_s,
            ckv_s, rq, rk, rv, sq, sk, sv, wkt_s, wvt_s, a_s, xa_s, q_s, wo_s,
            w_s, wl_s, mk_s, mv_s, kt_s, ka_s, va_s, s_s, pb_s, cl_s, o_s,
            zero_s, sink_s, sem):
    h = pl.program_id(0)
    vec_s = (v0, v1, v2, v3, v4)

    def slice_copies(i):
        s = sem.at[SEM_SL + i]
        grp = i // 2 if isinstance(i, int) else lax.shift_right_logical(i, 1)
        cs, dst = pl.ds(i * CS, CS), pl.ds((i & (NRAW - 1)) * CS, CS)
        return [pltpu.make_async_copy(ckv_hbm.at[grp, :, i & 1], ckv_s.at[grp, :, i & 1], s),
                pltpu.make_async_copy(wk_hbm.at[cs], rk.at[dst], s),
                pltpu.make_async_copy(wv_hbm.at[cs], rv.at[dst], s)]

    def wq1_copy(i):
        rows = pl.ds(i * (M // 4), M // 4)
        return pltpu.make_async_copy(wq_hbm.at[rows, 8:16], rq.at[rows, 8:16], sem.at[SEM_WQ1 + i])

    def x_copy(i):
        cols = pl.ds(i * TA, TA)
        return pltpu.make_async_copy(xT_hbm.at[:, cols], xT_s.at[:, cols], sem.at[SEM_X + i])

    def out_copy(jp):
        cols = pl.ds(jp * 2 * T, 2 * T)
        return pltpu.make_async_copy(o_s.at[:, cols], out_hbm.at[:, cols], sem.at[SEM_OUT])

    def prep_w(hh, outer, tie):
        rows = _ds(lax.shift_right_logical(hh, 1) * D, D, D)
        sh = (16 * (1 - (hh & 1))).astype(u32)
        k = 0
        for row0, wt_s in ((0, wkt_s.at[rows]), (QD, wvt_s.at[rows])):
            for r in range(0, QD, 16):
                def block(o, q):
                    row = (o % 2) * HD + (q % 2) * QD + r
                    col = (o // 2) * 2 * QC + (q // 2) * QC
                    return _hi16(wt_s[row:row + 16, col:col + QC] << sh)
                for n1 in outer:
                    _put(w_s, row0 + r, 7 * n1 * QC, _operands2(_B_TERMS, n1, block, lambda x: tie(x, k)))
                    k += 1

    @pl.when(h == 0)
    def _():
        cp_vec = [pltpu.make_async_copy(src, dst, sem.at[SEM_VEC])
                  for src, dst in zip((lre_hbm, lim_hbm, ldt_hbm, dsk_hbm, gw_hbm), vec_s)]
        cp_b = [pltpu.make_async_copy(src.at[pl.ds(lo, n)], b_s.at[pl.ds(dst, n)], sem.at[SEM_B])
                for src, lo, n, dst in ((bre_hbm, 0, PA, 0), (bim_hbm, 0, PA, PA),
                                        (bre_hbm, PA, PB, 2 * PA), (bim_hbm, PA, PB, 2 * PA + PB))]
        cp_wq = [pltpu.make_async_copy(wq_hbm.at[:, 0:8], rq.at[:, 0:8], sem.at[SEM_WQ])]
        cp_c = [pltpu.make_async_copy(src, craw_s.at[n], sem.at[SEM_C])
                for n, src in enumerate((cre_hbm, cim_hbm))]
        cp_wo = pltpu.make_async_copy(woT_hbm, wo_s, sem.at[SEM_WO])
        for cp in cp_vec + cp_b + [x_copy(i) for i in range(S // TA)] + cp_c + cp_wq:
            cp.start()
        for i in range(NRAW - 1):
            for cp in [wq1_copy(i)] + slice_copies(i):
                cp.start()
        wq1_copy(3).start()
        cp_wo.start()

        zero_s[...] = jnp.zeros(zero_s.shape, f32)
        wl_s[...] = jnp.zeros(wl_s.shape, u32)
        cl_s[...] = jnp.zeros(cl_s.shape, u32)
        for cp in cp_vec:
            cp.wait()
        _ssm_params(vec_s, coef_s, lam_s, col_s)

        def phase1(i):
            clk = _Clock(zero_s)
            u = _dot(xT_s[:, i * TA:(i + 1) * TA], b_s[...], _TT)
            u_s[i * TA:(i + 1) * TA, :] = u
            clk.stage(1.0, [u], cols=range(0, 2 * PA, T))
            tie = clk.pacer(0.0, 1.0, 14)
            for t in range(2 * i, 2 * i + 2):
                for r in range(0, HM, 32):
                    k = (t % 2) * 7 + r // 32
                    top = xT_s[r:r + 32, 2 * t * T:(2 * t + 2) * T].astype(f32)
                    bot = xT_s[HM + r:HM + r + 32, 2 * t * T:(2 * t + 2) * T].astype(f32)
                    blocks = [tie(top[:, :T], k), bot[:, :T], top[:, T:], tie(bot[:, T:], k)]
                    _put(xa_s, r, t * 7 * T, _operands(_A_TERMS, blocks))
            return clk

        for cp in cp_b + [x_copy(0)]:
            cp.wait()
        phase1(0)
        x_copy(1).wait()
        clk = phase1(1)
        zero = jnp.zeros((1, 512), f32)
        carry0 = _ssm_scan(u_s.at[0:TC], (zero, zero), lam_s, h_s, clk.pacer(0.0, 1.0, TC // 2))
        for cp in [x_copy(2), x_copy(3)] + cp_c + cp_wq:
            cp.wait()
        _ssm_cmat(craw_s, coef_s, c_s, phase1(2).pacer(0.0, 1.0, M // 16))
        tie = phase1(3).pacer(0.0, 1.0, M // 8)
        for c0 in range(0, M, 8):
            _stage(rq, sq, c0, 8, lambda x: tie(x, c0 // 8), groups=(0,))

        def phase2(i, carry):
            @pl.when(i + NRAW - 1 < NP)
            def _():
                for cp in slice_copies(i + NRAW - 1):
                    cp.start()

            @pl.when(i < 4)
            def _():
                wq1_copy(i).wait()

            for cp in slice_copies(i):
                cp.wait()

            yT = _dot(_get(c_s, 0, M, 0, 2 * M), _get(h_s, 0, TC, 0, 2 * M), _NT)
            for t in range(TC // T):
                cols = _ds(i * TC + t * T, T, T)
                acc = jnp.zeros((8, T), f32)
                for r in range(0, M, 32):
                    xg = xT_s[r:r + 32, cols].astype(f32) * col_s[1, r:r + 32, :]
                    acc = acc + jnp.sum(xg.reshape(4, 8, T), axis=0)
                g = jax.nn.sigmoid(jnp.sum(acc, axis=0, keepdims=True))
                g_s[:, cols] = g
                for r in range(0, M, 32):
                    skip = xT_s[r:r + 32, cols].astype(f32) * col_s[0, r:r + 32, :]
                    o_s[r:r + 32, cols] = (1.0 - g) * (yT[r:r + 32, t * T:(t + 1) * T] + skip)

            ht = lax.shift_right_logical(i, 2)
            words = [sq[ht * 2 + dt, pl.ds(i & 3, M, stride=4), :] for dt in range(2)]
            both = [jnp.concatenate([pltpu.bitcast(w << 16, f32), _hi16(w)], axis=1) for w in words]
            wq = _operands(_B_TERMS, [both[0][:HM], both[1][:HM], both[0][HM:], both[1][HM:]])
            m = [_dot(wq[n].astype(bf16), _cat([_get(xa_s, 0, HM, (t * 7 + n) * T, T) for t in range(NP)], 1), _TN)
                 for n in range(7)]
            q_i = q_s.at[_ds(i * 2 * D, 2 * D, 2 * D)]
            for n in (2, 1, 3, 0):
                for t in range(NP):
                    for r in range(0, D, GC):
                        c, = _combine(_Tiles(m, r, GC, t * T, T), (n,))
                        row = (2 * (r // HD) + n // 2) * D + (n % 2) * HD + r % HD
                        _put(q_i, row, t * T, [c * (LOG2E * D ** -0.5)])

            clk = _Clock(zero_s)
            clk.stage(1.0, m[:5], cols=range(0, S // 2, 2 * T))

            u_next = u_s.at[_ds(jnp.minimum(i + 1, NP - 1) * TC, TC, TC)]
            carry = _ssm_scan(u_next, carry, lam_s, h_s, clk.pacer(0.0, 1.0, TC // 2))

            tie = clk.pacer(0.0, 1.0, 64)
            rq_i = rq.at[pl.ds((i & 3) * (M // 4), M // 4)]
            sq_i = sq.at[:, _ds((i & 3) * M, M, 8)]
            for c0 in range(0, M // 4, 8):
                _stage(rq_i, sq_i, c0, 8, lambda x: tie(x, c0 // 2 + 2), groups=(1,))
            slot = pl.ds((i & (NRAW - 1)) * CS, CS)
            for n, (raw, stg, wt_s) in enumerate(((rk, sk, wkt_s), (rv, sv, wvt_s))):
                for c0 in range(0, CS, 8):
                    _stage(raw.at[slot], stg, c0, 8, lambda x: tie(x, 16 * n + c0 // 8))
                cols = _ds(i * CS, CS, CS)
                for pair in range(H // 2):
                    for dt in range(2):
                        blk = stg[(pair // 4) * 2 + dt, pl.ds(pair % 4, CS, stride=4), :]
                        row = pair * D + dt * HD
                        wt_s[row:row + HD, cols] = tie(blk, 16 + 24 * n + 3 * pair + dt).T

            tie = clk.pacer(0.0, 1.0, 28)
            ckv_i = ckv_s.at[lax.shift_right_logical(i, 1), :, i & 1]
            a_i = a_s.at[_ds(i * (T // 4), T // 4, T // 4)]
            for r in range(0, T // 2, 16):
                def block(o, q):
                    col = (o % 2) * 2 * QC + (q % 2) * QC
                    return ckv_i[2 * (q // 2) + o // 2, r:r + 16, col:col + QC].astype(f32)
                for n1 in range(7):
                    ops = _operands2(_A_TERMS, n1, block, lambda x: tie(x, 7 * (r // 16) + n1))
                    _put(a_i, r, 7 * n1 * QC, ops)
            return carry

        lax.fori_loop(0, NP, phase2, carry0)
        cp_wo.wait()
        prep_w(h, range(NT1), _no_tie)

    clk = _Clock(zero_s)
    q_h = q_s.at[_ds(h * D, D, D)]

    def prep_wo(tie):
        for r in range(0, HM, 16):
            top = tie(wo_s[h, r:r + 16, :].astype(f32), r // 16)
            bot = tie(wo_s[h, HM + r:HM + r + 16, :].astype(f32), r // 16)
            _put(wl_s, r, 0, _operands(_A_TERMS, [top[:, :HD], top[:, HD:], bot[:, :HD], bot[:, HD:]]))

    def proj(g, lo, hi):
        for n1 in range(lo, hi):
            m = [_dot(_get(w_s, 0, 2 * QD, n * QC, QC), _get(a_s, g * T, T, n * QC, QC), _NT)
                 for n in range(7 * n1, 7 * n1 + 7)]
            for r in range(0, 2 * QD, GC):
                m_s, row = mk_s if r < QD else mv_s, n1 * HD + r % QD
                c = _combine(_Tiles(m, r, GC))
                m_s[row:row + GC, :] = jnp.concatenate([c[0], c[2]], axis=1)
                m_s[QD + row:QD + row + GC, :] = jnp.concatenate([c[1], c[3]], axis=1)
            clk.stage(448, m[0::2], 16)
        if hi < 7:
            return
        outer = lambda m_s, r: _combine([m_s[n * HD + r:n * HD + r + 16, :] for n in range(7)])
        nine = lambda c: _operands(_A_TERMS, c) + [c[1], c[2]]
        cs = [outer(mk_s, r) for r in range(0, HD, 16)]
        for n in range(4):
            kt_s[:, n * T:(n + 1) * T] = jnp.concatenate([c[n] for c in cs], axis=0).T
        for r in range(0, 2 * T, GC):
            blk = kt_s[r:r + GC, :]
            _put(ka_s, 2 * g * T + r, 0, nine([blk[:, n * T:(n + 1) * T] for n in range(4)]))
        for r in range(0, HD, 16):
            c = outer(mv_s, r)
            ops = nine([c[0], c[2], c[1], c[3]])
            _put(va_s, r, 2 * g * 9 * T, [o[:, :T] for o in ops] + [o[:, T:] for o in ops])

    key = lax.broadcasted_iota(jnp.int32, (T, 2 * T), 0)
    qry = lax.broadcasted_iota(jnp.int32, (T, 2 * T), 1)
    causal = key <= qry

    def qk(jp):
        R, s_j = jp * T, s_s.at[jp % 2]
        qe, qo = _get(q_h, 0, D, R, T), _get(q_h, D, D, R, T)
        mx = _Reducer(jnp.max, jnp.maximum)

        def put(row, v):
            v = v.reshape(v.shape[0] // 8, 8, 2 * T)
            s_j[row // 8:row // 8 + v.shape[0]] = v
            mx.add(v)

        if jp > 0:
            qef, qof = qe.astype(f32), qo.astype(f32)
            qb = _operands(_B_TERMS, [qef[:HD], qof[:HD], qef[HD:], qof[HD:]])
            m = [_dot(_get(ka_s, 0, R, n * T, T), qb[n].astype(bf16), _NN) for n in range(7)]
            for r in range(0, R, GC):
                c = _combine(_Tiles(m, r, GC))
                put(r, jnp.concatenate(c[:2], axis=1))
                put(R + r, jnp.concatenate(c[2:], axis=1))
            clk.stage(7 * R / 4, [m[0], m[4]])
        kb = lambda a, b: jnp.concatenate([_get(ka_s, R, T, a * T, T), _get(ka_s, R, T, b * T, T)], axis=1)
        se = _dot(kb(2, 7), jnp.concatenate([qe, qo], axis=1), _NN)
        so = _dot(kb(8, 3), qo, _NN)
        clk.stage(192, [se])
        put(2 * R, jnp.where(causal, se, NEG))
        so = jnp.where(causal[:, :T], so, NEG)
        s_j[(2 * R + T) // 8:(2 * R + 2 * T) // 8, :, T:] = so.reshape(T // 8, 8, T)
        mo = jnp.concatenate([jnp.full((1, T), NEG, f32), jnp.max(so, axis=0, keepdims=True)], axis=1)
        return jnp.broadcast_to(jnp.maximum(mx.result(), mo), (8, 2 * T))

    pb0 = lambda jp: jp * (jp - 1) // 2 * T
    sunk = [0]

    def softmax(jp, mx, t0, t1):
        R, s_j = jp * T, s_s.at[jp % 2]
        n = (2 * R + T + T // 2) // GS
        prob = lambda row, z: jnp.exp2(s_j[row // 8:(row + GS) // 8] - z)
        last = lambda row, z: jnp.exp2(s_j[row // 8:(row + 2 * GS) // 8, :, T:] - z[:, T:])
        tie = clk.pacer(t0, (t0 + t1) / 2, n)
        sm, so = _Reducer(jnp.sum, jnp.add), _Reducer(jnp.sum, jnp.add)
        for k, r in enumerate(range(0, 2 * R + T, GS)):
            sm.add(prob(r, tie(mx, k)))
            if k % PULL == 0 and sm.acc is not None:
                sink_s[sunk[0]] = sm.acc
                sunk[0] += 1
        for k, r in enumerate(range(2 * R + T, 2 * R + 2 * T, 2 * GS)):
            so.add(last(r, tie(mx, (2 * R + T) // GS + k)))
        z = mx + jnp.log2(sm.result() + jnp.concatenate([jnp.zeros((1, T), f32), so.result()], axis=1))
        tie = clk.pacer((t0 + t1) / 2, t1, n)
        for k, r in enumerate(range(0, R, GS)):
            top = prob(r, tie(z, 2 * k)).reshape(GS, 2 * T)
            bot = prob(R + r, tie(z, 2 * k + 1)).reshape(GS, 2 * T)
            ops = _operands(_B_TERMS, [top[:, :T], top[:, T:], bot[:, :T], bot[:, T:]])
            _put(pb_s, pb0(jp) + r, 0, ops)
        for r in range(0, T, GS):
            p = prob(2 * R + r, tie(z, (2 * R + r) // GS)).reshape(GS, 2 * T)
            _put(pb_s, 2 * jp * T + r, 7 * T, [p])
        for k, r in enumerate(range(0, T, 2 * GS)):
            p = last(2 * R + T + r, tie(z, (2 * R + T) // GS + k)).reshape(2 * GS, T)
            _put(pb_s, (2 * jp + 1) * T + r, 8 * T, [p])

    def pv(jp):
        R = jp * T
        va = lambda n, t: _get(va_s, 0, HD, (t * 9 + n) * T, T)
        if jp > 0:
            m = [_dot(_cat([va(n, t) for t in range(jp)], 1), _get(pb_s, pb0(jp), R, n * T, T), _NN)
                 for n in range(7)]
            clk.stage(7 * R / 4, m, 32)
        ve = jnp.concatenate([va(2, jp), va(8, jp)], axis=0)
        vo = jnp.concatenate([va(7, jp), va(3, jp)], axis=0)
        ce = _dot(ve, _get(pb_s, 2 * R, T, 7 * T, T), _NN)
        co = _dot(jnp.concatenate([ve, vo], axis=1), _get(pb_s, 2 * R, 2 * T, 8 * T, T), _NN)
        clk.stage(192, [ce], 32)
        ge, go = g_s[:, 2 * R:2 * R + T], g_s[:, 2 * R + T:2 * R + 2 * T]
        for r in range(0, HD, GC):
            c = [ce[r:r + GC], co[r:r + GC], ce[HD + r:HD + r + GC], co[HD + r:HD + r + GC]]
            if jp > 0:
                c = [x + y for x, y in zip(c, _combine(_Tiles(m, r, GC)))]
            ops = _operands(_B_TERMS, [c[0] * ge, c[1] * go, c[2] * ge, c[3] * go])
            _put(cl_s, r, (jp % 4) * 7 * T, ops)

    def oproj(jp):
        m = [_dot(_get(wl_s, 0, HM, n * T, T), _get(cl_s, 0, HD, ((jp % 4) * 7 + n) * T, T), _NN)
             for n in range(7)]
        cols = slice(2 * jp * T, (2 * jp + 2) * T)
        for r in range(0, HM, 32):
            c = _combine(_Tiles(m, r, 32))
            o_s[r:r + 32, cols] += jnp.concatenate(c[:2], axis=1)
            o_s[HM + r:HM + r + 32, cols] += jnp.concatenate(c[2:], axis=1)
        clk.stage(392, [m[0], m[4]])

    def oproj_out(jp):
        oproj(jp)

        @pl.when(h == H - 1)
        def _():
            out_copy(jp).start()

    for n1 in range(7):
        if n1 >= NT1:
            prep_w(h, [n1], clk.pacer(max(clk.t - LEAD - 448, 1), max(clk.t - LEAD, 1), 8))
        proj(0, n1, n1 + 1)
    oproj(NP - 1)
    for jp, cover in enumerate(PLAN):
        mx = qk(jp)
        t0 = clk.t
        for item in cover.split():
            if item[0] == 'P':
                pv(int(item[1]))
            elif item[0] == 'O':
                oproj_out(int(item[1]))
            else:
                proj(int(item[1]), int(item[2]), int(item[3]))
        softmax(jp, mx, t0 + D0, clk.t - SLACK)
        if jp == 0:
            prep_wo(clk.pacer(t0, clk.t, HM // 16))
    t0 = clk.t
    pv(NP - 1)
    oproj_out(NP - 2)
    prep_w(jnp.minimum(h + 1, H - 1), range(NT1), clk.pacer(t0 - PW0, clk.t - 300, 8 * NT1))

    @pl.when(h == H - 1)
    def _():
        oproj(NP - 1)
        out_copy(NP - 1).start()
        for jp in range(NP):
            out_copy(jp).wait()


@jax.jit
def pallas_gated_mix__compressed_kv_cla__ssm_conv_s5__prompt_kernel(
    A_x: jax.Array,
    A_c_kv: jax.Array,
    A_w_q: jax.Array,
    A_w_uk: jax.Array,
    A_w_uv: jax.Array,
    A_w_o: jax.Array,
    B_x: jax.Array,
    B_Lambda_re: jax.Array,
    B_Lambda_im: jax.Array,
    B_B_re: jax.Array,
    B_B_im: jax.Array,
    B_C_re: jax.Array,
    B_C_im: jax.Array,
    B_log_dt: jax.Array,
    B_Dskip: jax.Array,
    gate_w: jax.Array,
):
    del B_x
    xT = jnp.transpose(A_x[0])
    woT = jnp.transpose(A_w_o, (0, 2, 1))
    ckv = A_c_kv.reshape(4, 4, 2, T // 2, DC)

    hbm = pl.BlockSpec(memory_space=pl.ANY)
    vmem = pltpu.VMEM
    outT = pl.pallas_call(
        _kernel,
        grid=(H,),
        in_specs=[hbm] * 15,
        out_specs=hbm,
        out_shape=jax.ShapeDtypeStruct((M, S), f32),
        scratch_shapes=[
            vmem((M, S), bf16),
            vmem((M,), bf16), vmem((M,), bf16), vmem((M,), bf16), vmem((M,), bf16), vmem((M,), bf16),
            vmem((2 * M, M), bf16),
            vmem((2, M, M), bf16),
            vmem((M // 2, 2 * M), u32),
            vmem((8, 512), f32),
            vmem((8, 8, 512), f32),
            vmem((2, M, T), f32),
            vmem((S, 2 * M), f32),
            vmem((TC // 2, 2 * M), u32),
            vmem((1, S), f32),
            vmem((4, 4, 2, T // 2, DC), bf16),
            vmem((M, H, D), bf16),
            vmem((NRAW * CS, H, D), bf16),
            vmem((NRAW * CS, H, D), bf16),
            vmem((4, M * 4, T), u32),
            vmem((4, CS * 4, T), u32),
            vmem((4, CS * 4, T), u32),
            vmem((H // 2 * D, DC), u32),
            vmem((H // 2 * D, DC), u32),
            vmem((S // 8, 49 * QC), u32),
            vmem((HM // 2, NP * 7 * T), u32),
            vmem((H * D, S // 2), u32),
            vmem((H, M, D), bf16),
            vmem((QD, 49 * QC), u32),
            vmem((HM // 2, 7 * T), u32),
            vmem((7 * HD, 2 * T), f32),
            vmem((7 * HD, 2 * T), f32),
            vmem((2 * T, 4 * T), f32),
            vmem((S // 4, 9 * T), u32),
            vmem((HD // 2, NP * 9 * T), u32),
            vmem((2, S // 8, 8, 2 * T), f32),
            vmem((14 * T, 9 * T), u32),
            vmem((HD // 2, 28 * T), u32),
            vmem((M, S), f32),
            vmem((8, T), f32),
            vmem((256, 8, 2 * T), f32),
            pltpu.SemaphoreType.DMA((NSEM,)),
        ],
        compiler_params=pltpu.CompilerParams(
            dimension_semantics=("arbitrary",),
            vmem_limit_bytes=126 * 1024 * 1024,
        ),
    )(xT, B_B_re, B_B_im, B_C_re, B_C_im, B_Lambda_re, B_Lambda_im, B_log_dt,
      B_Dskip, gate_w, woT, ckv, A_w_q, A_w_uk, A_w_uv)
    return jnp.transpose(outT)[None]
```

```python
import os

import jax
import jax.numpy as jnp
from jax import lax
import jax.experimental.pallas as pl
import jax.experimental.pallas.tpu as pltpu

S = 2048
M = 448
H = 16
D = 256
DC = 1024
T = 128
NP = S // T // 2
HD = D // 2
HM = M // 2
QD = D // 4
QC = DC // 4
PA = 384
PB = M - PA
TA = 512
TC = 256
CS = DC // NP
NRAW = 4
LOG2E = 1.4426950408889634
NEG = -1e30

_env = lambda k, d: type(d)(os.environ.get(k, d))
GC = _env('GC', 64)
GS = _env('GS', 16)
RCH = _env('RCH', 256)
SLACK = _env('SLACK', 200)
D0 = _env('D0', 0)
PULL = _env('PULL', 2)
NT1 = _env('NT1', 3)
LEAD = _env('LEAD', 448)
PW0 = _env('PW0', 100)
LSUB = _env('LSUB', 1)
PLAN = _env('PLAN', 'K103,K137,K203,K237,K304 P0 P1,K347 P2 O0,P3 O1 P4 O2 O3,P5 O4 P6 O5').split(',')

f32 = jnp.float32
bf16 = jnp.bfloat16
u32 = jnp.uint32

SEM_VEC, SEM_B, SEM_X, SEM_WQ, SEM_C, SEM_SL, SEM_WO, SEM_OUT, SEM_WQ1 = 0, 1, 2, 6, 7, 8, 16, 17, 18
NSEM = 22

_NN = ((1,), (0,))
_NT = ((1,), (1,))
_TN = ((0,), (0,))
_TT = ((0,), (1,))


def _dot(a, b, dims):
    return lax.dot_general(a, b, (dims, ((), ())), preferred_element_type=f32)


def _cat(xs, axis):
    return xs[0] if len(xs) == 1 else jnp.concatenate(xs, axis=axis)


def _ds(lo, n, align):
    return pl.ds(lo if isinstance(lo, int) else pl.multiple_of(lo, align), n)


def _put(ref, row, col, xs):
    x = _cat(xs, 1)
    ref[row // 2:(row + x.shape[0]) // 2, col:col + x.shape[1]] = pltpu.bitcast(x.astype(bf16), u32)


def _get(ref, row, nrows, col, ncols):
    return pltpu.bitcast(ref[row // 2:(row + nrows) // 2, col:col + ncols], bf16)


class _Clock:
    def __init__(self, zero_ref):
        self.masks = {(8, T): zero_ref[...] != 0.0}
        self.ticks, self.t = [], 0

    def stage(self, duration, vals, step=8, cols=(0,)):
        where = [(v, r, c) for v in vals for c in cols for r in range(0, v.shape[0], step)]
        for k, w in enumerate(where):
            self.ticks.append((self.t + duration * (k + 1) / len(where), w))
        self.t += duration

    def pacer(self, t0, t1, n):
        def tie(x, k):
            past = [w for t, w in self.ticks if t <= t0 + (t1 - t0) * k / n]
            if not past:
                return x
            v, r, c = past[-1]
            tick = v[r:r + 8, c:c + T]
            if tick.dtype != x.dtype:
                tick = pltpu.bitcast(tick, x.dtype)
            reps = (x.shape[0] // 8, x.shape[1] // T)
            if x.shape not in self.masks:
                self.masks[x.shape] = jnp.tile(self.masks[(8, T)], reps)
            return lax.select(self.masks[x.shape], tick if reps == (1, 1) else jnp.tile(tick, reps), x)
        return tie


def _no_tie(x, k):
    return x


_A_TERMS = ((0, 3, 1), (2, 3, 1), (0, None, 0), (3, None, 0), (0, 1, 1), (2, 0, -1), (1, 3, -1))
_B_TERMS = ((0, 3, 1), (0, None, 0), (1, 3, -1), (2, 0, -1), (3, None, 0), (0, 1, 1), (2, 3, 1))


def _operand(term, block):
    x, y, sign = term
    if y is None:
        return block(x)
    return block(x) + block(y) if sign > 0 else block(x) - block(y)


def _operands(terms, blocks):
    return [_operand(t, blocks.__getitem__) for t in terms]


def _operands2(terms, n1, block, tie):
    first = terms[n1][0]
    sub = [_operand(terms[n1], lambda o: tie(block(o, q)) if o == first and q in (0, 3) else block(o, q))
           for q in range(4)]
    return _operands(terms, sub)


def _combine(m, only=(0, 1, 2, 3)):
    c = (lambda: (m[0] + m[3]) + (m[6] - m[4]),
         lambda: m[2] + m[4],
         lambda: m[1] + m[3],
         lambda: (m[0] - m[1]) + (m[2] + m[5]))
    return [c[n]() for n in only]


class _Tiles:
    def __init__(self, vals, r, n, c=0, w=None):
        self.vals, self.idx, self.cache = vals, (slice(r, r + n), slice(c, None if w is None else c + w)), {}

    def __getitem__(self, i):
        if i not in self.cache:
            self.cache[i] = self.vals[i][self.idx]
        return self.cache[i]


class _Reducer:
    def __init__(self, red, comb):
        self.red, self.comb, self.acc, self.rows, self.out = red, comb, None, 0, None

    def add(self, v):
        self.rows += 8 * v.shape[0]
        v = self.red(v, axis=0)
        self.acc = v if self.acc is None else self.comb(self.acc, v)
        if self.rows >= RCH:
            self.result()

    def result(self):
        if self.acc is not None:
            v = self.red(self.acc, axis=0, keepdims=True)
            self.out = v if self.out is None else self.comb(self.out, v)
        self.acc, self.rows = None, 0
        return self.out


def _cmul(ar, ai, br, bi):
    return ar * br - ai * bi, ar * bi + ai * br


def _hi16(w):
    return pltpu.bitcast(w & jnp.uint32(0xFFFF0000), f32)


def _stage(raw, stg, c0, nc, tie, groups=(0, 1)):
    for ht in groups:
        for dt in range(2):
            v = raw[c0:c0 + nc, ht * 8:(ht + 1) * 8, dt * T:(dt + 1) * T].reshape(nc * 8, T)
            stg[ht * 2 + dt, c0 * 4:(c0 + nc) * 4, :] = tie(pltpu.bitcast(v, u32))


def _ssm_params(vec_s, coef_s, lam_s, col_s):
    row = lambda r: r[...].astype(f32).reshape(1, M)
    lre, lim, ldt, dsk, gw = [row(v) for v in vec_s]
    dt = jnp.exp(ldt).astype(bf16).astype(f32)
    mag = jnp.exp(dt * lre)
    ang = dt * lim
    lr, li = mag * jnp.cos(ang), mag * jnp.sin(ang)
    den = lre * lre + lim * lim
    nr = lr - 1.0
    coef_s[...] = jnp.zeros(coef_s.shape, f32)
    coef_s[0:1, 0:M] = 2.0 * ((nr * lre + li * lim) / den)
    coef_s[1:2, 0:M] = 2.0 * ((li * lre - nr * lim) / den)

    er = jnp.concatenate([lr, lr[:, PA:]], axis=1)
    ei = jnp.concatenate([li, -li[:, PA:]], axis=1)
    pw = [(er, ei)]
    for _ in range(7):
        pw.append(_cmul(pw[-1][0], pw[-1][1], er, ei))
    sub = lax.broadcasted_iota(jnp.int32, (8, 512), 0)
    for n, d in enumerate((1, 2, 4)):
        lam_s[2 * n] = jnp.where(sub >= d, pw[d - 1][0], 0.0)
        lam_s[2 * n + 1] = jnp.where(sub >= d, pw[d - 1][1], 0.0)
    lcr = jnp.zeros((8, 512), f32)
    lci = jnp.zeros((8, 512), f32)
    for r in range(8):
        lcr = jnp.where(sub == r, pw[r][0], lcr)
        lci = jnp.where(sub == r, pw[r][1], lci)
    lam_s[6] = lcr
    lam_s[7] = lci

    def col(v):
        v = jnp.concatenate([v, jnp.zeros((1, 512 - M), f32)], axis=1)
        return jnp.broadcast_to(v, (T, 512)).T[:M]
    col_s[0] = col(dsk)
    col_s[1] = col(gw)


def _ssm_cmat(craw_s, coef_s, c_s, tie):
    for r in range(0, M, 16):
        coef = tie(coef_s[...], r // 16)
        cr, ci = coef[0:1, :M], coef[1:2, :M]
        re, im = _cmul(craw_s[0, r:r + 16, :].astype(f32), craw_s[1, r:r + 16, :].astype(f32), cr, ci)
        _put(c_s, r, 0, [re[:, :PA], -im[:, :PA], re[:, PA:], -im[:, PA:]])


def _ssm_scan(u_ref, carry, lam_s, h_s, tie):
    car, cai = carry
    out = []
    for b in range(TC // 8):
        u = u_ref[b * 8:(b + 1) * 8, :]
        mixed = u[:, 2 * PA:]
        cols = [u[:, 0:T], u[:, T:2 * T], u[:, 2 * T:PA], mixed]
        hr = jnp.concatenate([tie(v, 4 * b + n) for n, v in enumerate(cols)], axis=1)
        hi = jnp.concatenate([u[:, PA:2 * PA], pltpu.roll(mixed, PB, 1)], axis=1)
        for n, d in enumerate((1, 2, 4)):
            sr, si = pltpu.roll(hr, d, 0), pltpu.roll(hi, d, 0)
            tr, ti = _cmul(sr, si, lam_s[2 * n], lam_s[2 * n + 1])
            hr, hi = hr + tr, hi + ti
        tr, ti = _cmul(lam_s[6], lam_s[7], car, cai)
        hr, hi = hr + tr, hi + ti
        car, cai = hr[7:8, :], hi[7:8, :]
        out.append(jnp.concatenate([hr[:, :PA], hi[:, :PA], hr[:, PA:]], axis=1))
        if b % 2 == 1:
            _put(h_s, (b - 1) * 8, 0, [jnp.concatenate(out, axis=0)])
            out = []
    return car, cai


def _kernel(xT_hbm, bre_hbm, bim_hbm, cre_hbm, cim_hbm, lre_hbm, lim_hbm, ldt_hbm,
            dsk_hbm, gw_hbm, woT_hbm, ckv_hbm, wq_hbm, wk_hbm, wv_hbm,
            out_hbm,
            xT_s, v0, v1, v2, v3, v4, b_s, craw_s, c_s, coef_s, lam_s, col_s, u_s, h_s, g_s,
            ckv_s, rq, rk, rv, sq, sk, sv, wkt_s, wvt_s, a_s, xa_s, q_s, wo_s,
            w_s, wl_s, mk_s, mv_s, kt_s, ka_s, va_s, s_s, pb_s, cl_s, o_s,
            zero_s, sink_s, sc_s, sem):
    h = pl.program_id(0)
    vec_s = (v0, v1, v2, v3, v4)

    def slice_copies(i):
        s = sem.at[SEM_SL + i]
        grp = i // 2 if isinstance(i, int) else lax.shift_right_logical(i, 1)
        cs, dst = pl.ds(i * CS, CS), pl.ds((i & (NRAW - 1)) * CS, CS)
        return [pltpu.make_async_copy(ckv_hbm.at[grp, :, i & 1], ckv_s.at[grp, :, i & 1], s),
                pltpu.make_async_copy(wk_hbm.at[cs], rk.at[dst], s),
                pltpu.make_async_copy(wv_hbm.at[cs], rv.at[dst], s)]

    def wq1_copy(i):
        rows = pl.ds(i * (M // 4), M // 4)
        return pltpu.make_async_copy(wq_hbm.at[rows, 8:16], rq.at[rows, 8:16], sem.at[SEM_WQ1 + i])

    def x_copy(i):
        cols = pl.ds(i * TA, TA)
        return pltpu.make_async_copy(xT_hbm.at[:, cols], xT_s.at[:, cols], sem.at[SEM_X + i])

    def out_copy(jp):
        cols = pl.ds(jp * 2 * T, 2 * T)
        return pltpu.make_async_copy(o_s.at[:, cols], out_hbm.at[:, cols], sem.at[SEM_OUT])

    def prep_w(hh, outer, tie):
        rows = _ds(lax.shift_right_logical(hh, 1) * D, D, D)
        sh = (16 * (1 - (hh & 1))).astype(u32)
        k = 0
        for row0, wt_s in ((0, wkt_s.at[rows]), (QD, wvt_s.at[rows])):
            for r in range(0, QD, 16):
                def block(o, q):
                    row = (o % 2) * HD + (q % 2) * QD + r
                    col = (o // 2) * 2 * QC + (q // 2) * QC
                    return _hi16(wt_s[row:row + 16, col:col + QC] << sh)
                for n1 in outer:
                    _put(w_s, row0 + r, 7 * n1 * QC, _operands2(_B_TERMS, n1, block, lambda x: tie(x, k)))
                    k += 1

    @pl.when(h == 0)
    def _():
        cp_vec = [pltpu.make_async_copy(src, dst, sem.at[SEM_VEC])
                  for src, dst in zip((lre_hbm, lim_hbm, ldt_hbm, dsk_hbm, gw_hbm), vec_s)]
        cp_b = [pltpu.make_async_copy(src.at[pl.ds(lo, n)], b_s.at[pl.ds(dst, n)], sem.at[SEM_B])
                for src, lo, n, dst in ((bre_hbm, 0, PA, 0), (bim_hbm, 0, PA, PA),
                                        (bre_hbm, PA, PB, 2 * PA), (bim_hbm, PA, PB, 2 * PA + PB))]
        cp_wq = [pltpu.make_async_copy(wq_hbm.at[:, 0:8], rq.at[:, 0:8], sem.at[SEM_WQ])]
        cp_c = [pltpu.make_async_copy(src, craw_s.at[n], sem.at[SEM_C])
                for n, src in enumerate((cre_hbm, cim_hbm))]
        cp_wo = pltpu.make_async_copy(woT_hbm, wo_s, sem.at[SEM_WO])
        for cp in cp_vec + cp_b + [x_copy(i) for i in range(S // TA)] + cp_c + cp_wq:
            cp.start()
        for i in range(NRAW - 1):
            for cp in [wq1_copy(i)] + slice_copies(i):
                cp.start()
        wq1_copy(3).start()
        cp_wo.start()

        zero_s[...] = jnp.zeros(zero_s.shape, f32)
        wl_s[...] = jnp.zeros(wl_s.shape, u32)
        cl_s[...] = jnp.zeros(cl_s.shape, u32)
        for cp in cp_vec:
            cp.wait()
        _ssm_params(vec_s, coef_s, lam_s, col_s)

        def phase1(i):
            clk = _Clock(zero_s)
            u = _dot(xT_s[:, i * TA:(i + 1) * TA], b_s[...], _TT)
            u_s[i * TA:(i + 1) * TA, :] = u
            clk.stage(1.0, [u], cols=range(0, 2 * PA, T))
            tie = clk.pacer(0.0, 1.0, 14)
            for t in range(2 * i, 2 * i + 2):
                for r in range(0, HM, 32):
                    k = (t % 2) * 7 + r // 32
                    top = xT_s[r:r + 32, 2 * t * T:(2 * t + 2) * T].astype(f32)
                    bot = xT_s[HM + r:HM + r + 32, 2 * t * T:(2 * t + 2) * T].astype(f32)
                    blocks = [tie(top[:, :T], k), bot[:, :T], top[:, T:], tie(bot[:, T:], k)]
                    _put(xa_s, r, t * 7 * T, _operands(_A_TERMS, blocks))
            return clk

        for cp in cp_b + [x_copy(0)]:
            cp.wait()
        phase1(0)
        x_copy(1).wait()
        clk = phase1(1)
        zero = jnp.zeros((1, 512), f32)
        carry0 = _ssm_scan(u_s.at[0:TC], (zero, zero), lam_s, h_s, clk.pacer(0.0, 1.0, TC // 2))
        for cp in [x_copy(2), x_copy(3)] + cp_c + cp_wq:
            cp.wait()
        _ssm_cmat(craw_s, coef_s, c_s, phase1(2).pacer(0.0, 1.0, M // 16))
        tie = phase1(3).pacer(0.0, 1.0, M // 8)
        for c0 in range(0, M, 8):
            _stage(rq, sq, c0, 8, lambda x: tie(x, c0 // 8), groups=(0,))

        def phase2(i, carry):
            @pl.when(i + NRAW - 1 < NP)
            def _():
                for cp in slice_copies(i + NRAW - 1):
                    cp.start()

            @pl.when(i < 4)
            def _():
                wq1_copy(i).wait()

            for cp in slice_copies(i):
                cp.wait()

            yT = _dot(_get(c_s, 0, M, 0, 2 * M), _get(h_s, 0, TC, 0, 2 * M), _NT)
            for t in range(TC // T):
                cols = _ds(i * TC + t * T, T, T)
                acc = jnp.zeros((8, T), f32)
                for r in range(0, M, 32):
                    xg = xT_s[r:r + 32, cols].astype(f32) * col_s[1, r:r + 32, :]
                    acc = acc + jnp.sum(xg.reshape(4, 8, T), axis=0)
                g = jax.nn.sigmoid(jnp.sum(acc, axis=0, keepdims=True))
                g_s[:, cols] = g
                for r in range(0, M, 32):
                    skip = xT_s[r:r + 32, cols].astype(f32) * col_s[0, r:r + 32, :]
                    o_s[r:r + 32, cols] = (1.0 - g) * (yT[r:r + 32, t * T:(t + 1) * T] + skip)

            ht = lax.shift_right_logical(i, 2)
            words = [sq[ht * 2 + dt, pl.ds(i & 3, M, stride=4), :] for dt in range(2)]
            both = [jnp.concatenate([pltpu.bitcast(w << 16, f32), _hi16(w)], axis=1) for w in words]
            wq = _operands(_B_TERMS, [both[0][:HM], both[1][:HM], both[0][HM:], both[1][HM:]])
            m = [_dot(wq[n].astype(bf16), _cat([_get(xa_s, 0, HM, (t * 7 + n) * T, T) for t in range(NP)], 1), _TN)
                 for n in range(7)]
            q_i = q_s.at[_ds(i * 2 * D, 2 * D, 2 * D)]
            for n in (2, 1, 3, 0):
                for t in range(NP):
                    for r in range(0, D, GC):
                        c, = _combine(_Tiles(m, r, GC, t * T, T), (n,))
                        row = (2 * (r // HD) + n // 2) * D + (n % 2) * HD + r % HD
                        _put(q_i, row, t * T, [c * (LOG2E * D ** -0.5)])

            clk = _Clock(zero_s)
            clk.stage(1.0, m[:5], cols=range(0, S // 2, 2 * T))

            u_next = u_s.at[_ds(jnp.minimum(i + 1, NP - 1) * TC, TC, TC)]
            carry = _ssm_scan(u_next, carry, lam_s, h_s, clk.pacer(0.0, 1.0, TC // 2))

            tie = clk.pacer(0.0, 1.0, 64)
            rq_i = rq.at[pl.ds((i & 3) * (M // 4), M // 4)]
            sq_i = sq.at[:, _ds((i & 3) * M, M, 8)]
            for c0 in range(0, M // 4, 8):
                _stage(rq_i, sq_i, c0, 8, lambda x: tie(x, c0 // 2 + 2), groups=(1,))
            slot = pl.ds((i & (NRAW - 1)) * CS, CS)
            for n, (raw, stg, wt_s) in enumerate(((rk, sk, wkt_s), (rv, sv, wvt_s))):
                for c0 in range(0, CS, 8):
                    _stage(raw.at[slot], stg, c0, 8, lambda x: tie(x, 16 * n + c0 // 8))
                cols = _ds(i * CS, CS, CS)
                for pair in range(H // 2):
                    for dt in range(2):
                        blk = stg[(pair // 4) * 2 + dt, pl.ds(pair % 4, CS, stride=4), :]
                        row = pair * D + dt * HD
                        wt_s[row:row + HD, cols] = tie(blk, 16 + 24 * n + 3 * pair + dt).T

            tie = clk.pacer(0.0, 1.0, 28)
            ckv_i = ckv_s.at[lax.shift_right_logical(i, 1), :, i & 1]
            a_i = a_s.at[_ds(i * (T // 4), T // 4, T // 4)]
            for r in range(0, T // 2, 16):
                def block(o, q):
                    col = (o % 2) * 2 * QC + (q % 2) * QC
                    return ckv_i[2 * (q // 2) + o // 2, r:r + 16, col:col + QC].astype(f32)
                for n1 in range(7):
                    ops = _operands2(_A_TERMS, n1, block, lambda x: tie(x, 7 * (r // 16) + n1))
                    _put(a_i, r, 7 * n1 * QC, ops)
            return carry

        lax.fori_loop(0, NP, phase2, carry0)
        cp_wo.wait()
        prep_w(h, range(NT1), _no_tie)

    clk = _Clock(zero_s)
    q_h = q_s.at[_ds(h * D, D, D)]

    def prep_wo(tie):
        for r in range(0, HM, 16):
            top = tie(wo_s[h, r:r + 16, :].astype(f32), r // 16)
            bot = tie(wo_s[h, HM + r:HM + r + 16, :].astype(f32), r // 16)
            _put(wl_s, r, 0, _operands(_A_TERMS, [top[:, :HD], top[:, HD:], bot[:, :HD], bot[:, HD:]]))

    def proj(g, lo, hi):
        for n1 in range(lo, hi):
            m = [_dot(_get(w_s, 0, 2 * QD, n * QC, QC), _get(a_s, g * T, T, n * QC, QC), _NT)
                 for n in range(7 * n1, 7 * n1 + 7)]
            for r in range(0, 2 * QD, GC):
                m_s, row = mk_s if r < QD else mv_s, n1 * HD + r % QD
                c = _combine(_Tiles(m, r, GC))
                m_s[row:row + GC, :] = jnp.concatenate([c[0], c[2]], axis=1)
                m_s[QD + row:QD + row + GC, :] = jnp.concatenate([c[1], c[3]], axis=1)
            clk.stage(448, m[0::2], 16)
        if hi < 7:
            return
        outer = lambda m_s, r: _combine([m_s[n * HD + r:n * HD + r + 16, :] for n in range(7)])
        nine = lambda c: _operands(_A_TERMS, c) + [c[1], c[2]]
        cs = [outer(mk_s, r) for r in range(0, HD, 16)]
        for n in range(4):
            kt_s[:, n * T:(n + 1) * T] = jnp.concatenate([c[n] for c in cs], axis=0).T
        for r in range(0, 2 * T, GC):
            blk = kt_s[r:r + GC, :]
            _put(ka_s, 2 * g * T + r, 0, nine([blk[:, n * T:(n + 1) * T] for n in range(4)]))
        for r in range(0, HD, 16):
            c = outer(mv_s, r)
            ops = nine([c[0], c[2], c[1], c[3]])
            _put(va_s, r, 2 * g * 9 * T, [o[:, :T] for o in ops] + [o[:, T:] for o in ops])

    key = lax.broadcasted_iota(jnp.int32, (T, 2 * T), 0)
    qry = lax.broadcasted_iota(jnp.int32, (T, 2 * T), 1)
    causal = key <= qry

    def qk(jp):
        R, s_j = jp * T, s_s.at[jp % 2]
        qe, qo = _get(q_h, 0, D, R, T), _get(q_h, D, D, R, T)
        mx = _Reducer(jnp.max, jnp.maximum)

        def put(row, v):
            v = v.reshape(v.shape[0] // 8, 8, 2 * T)
            s_j[row // 8:row // 8 + v.shape[0]] = v
            mx.add(v)

        if jp > 0:
            qef, qof = qe.astype(f32), qo.astype(f32)
            qb = _operands(_B_TERMS, [qef[:HD], qof[:HD], qef[HD:], qof[HD:]])
            m = [_dot(_get(ka_s, 0, R, n * T, T), qb[n].astype(bf16), _NN) for n in range(7)]
            for r in range(0, R, GC):
                c = _combine(_Tiles(m, r, GC))
                put(r, jnp.concatenate(c[:2], axis=1))
                put(R + r, jnp.concatenate(c[2:], axis=1))
            clk.stage(7 * R / 4, [m[0], m[4]])
        kb = lambda a, b: jnp.concatenate([_get(ka_s, R, T, a * T, T), _get(ka_s, R, T, b * T, T)], axis=1)
        se = _dot(kb(2, 7), jnp.concatenate([qe, qo], axis=1), _NN)
        so = _dot(kb(8, 3), qo, _NN)
        clk.stage(192, [se])
        put(2 * R, jnp.where(causal, se, NEG))
        so = jnp.where(causal[:, :T], so, NEG)
        s_j[(2 * R + T) // 8:(2 * R + 2 * T) // 8, :, T:] = so.reshape(T // 8, 8, T)
        mo = jnp.concatenate([jnp.full((1, T), NEG, f32), jnp.max(so, axis=0, keepdims=True)], axis=1)
        return jnp.broadcast_to(jnp.maximum(mx.result(), mo), (8, 2 * T))

    pb0 = lambda jp: jp * (jp - 1) // 2 * T
    sunk = [0]

    def softmax(jp, mx, t0, t1):
        R, s_j = jp * T, s_s.at[jp % 2]
        n = (2 * R + T + T // 2) // GS
        prob = lambda row, z: jnp.exp2(s_j[row // 8:(row + GS) // 8] - z)
        last = lambda row, z: jnp.exp2(s_j[row // 8:(row + 2 * GS) // 8, :, T:] - z[:, T:])
        both = lambda a, b: a.result() + jnp.concatenate([jnp.zeros((1, T), f32), b.result()], axis=1)

        def sink(k, red):
            if k % PULL == 0 and red.acc is not None:
                sink_s[sunk[0]] = red.acc
                sunk[0] += 1

        tm = t0 + (t1 - t0) / (1 + LSUB)
        tie = clk.pacer(t0, tm, n)
        if LSUB == 1:
            sm, so = _Reducer(jnp.sum, jnp.add), _Reducer(jnp.sum, jnp.add)
            for k, r in enumerate(range(0, 2 * R + T, GS)):
                sm.add(prob(r, tie(mx, k)))
                sink(k, sm)
            for k, r in enumerate(range(2 * R + T, 2 * R + 2 * T, 2 * GS)):
                so.add(last(r, tie(mx, (2 * R + T) // GS + k)))
            z = mx + jnp.log2(both(sm, so))
        elif jp > 0:
            sm = _Reducer(jnp.sum, jnp.add)
            for k, r in enumerate(range(0, 2 * R, GS * LSUB)):
                sm.add(prob(r, tie(mx, k * LSUB)))
                sink(k, sm)
            z = mx + jnp.log2(jnp.maximum(LSUB * sm.result(), 1.0))
        else:
            z = mx
        tie = clk.pacer(tm, t1, n)
        sm, so = _Reducer(jnp.sum, jnp.add), _Reducer(jnp.sum, jnp.add)
        for k, r in enumerate(range(0, R, GS)):
            top, bot = prob(r, tie(z, 2 * k)), prob(R + r, tie(z, 2 * k + 1))
            if LSUB > 1:
                sm.add(top + bot)
                sink(k, sm)
            top, bot = top.reshape(GS, 2 * T), bot.reshape(GS, 2 * T)
            ops = _operands(_B_TERMS, [top[:, :T], top[:, T:], bot[:, :T], bot[:, T:]])
            _put(pb_s, pb0(jp) + r, 0, ops)
        for r in range(0, T, GS):
            p = prob(2 * R + r, tie(z, (2 * R + r) // GS))
            if LSUB > 1:
                sm.add(p)
            _put(pb_s, 2 * jp * T + r, 7 * T, [p.reshape(GS, 2 * T)])
        for k, r in enumerate(range(0, T, 2 * GS)):
            p = last(2 * R + T + r, tie(z, (2 * R + T) // GS + k))
            if LSUB > 1:
                so.add(p)
            _put(pb_s, (2 * jp + 1) * T + r, 8 * T, [p.reshape(2 * GS, T)])
        g = g_s[:, 2 * R:2 * R + 2 * T]
        sc_s[:, 2 * R:2 * R + 2 * T] = g / both(sm, so) if LSUB > 1 else g

    def pv(jp):
        R = jp * T
        va = lambda n, t: _get(va_s, 0, HD, (t * 9 + n) * T, T)
        if jp > 0:
            m = [_dot(_cat([va(n, t) for t in range(jp)], 1), _get(pb_s, pb0(jp), R, n * T, T), _NN)
                 for n in range(7)]
            clk.stage(7 * R / 4, m, 32)
        ve = jnp.concatenate([va(2, jp), va(8, jp)], axis=0)
        vo = jnp.concatenate([va(7, jp), va(3, jp)], axis=0)
        ce = _dot(ve, _get(pb_s, 2 * R, T, 7 * T, T), _NN)
        co = _dot(jnp.concatenate([ve, vo], axis=1), _get(pb_s, 2 * R, 2 * T, 8 * T, T), _NN)
        clk.stage(192, [ce], 32)
        ge, go = sc_s[:, 2 * R:2 * R + T], sc_s[:, 2 * R + T:2 * R + 2 * T]
        for r in range(0, HD, GC):
            c = [ce[r:r + GC], co[r:r + GC], ce[HD + r:HD + r + GC], co[HD + r:HD + r + GC]]
            if jp > 0:
                c = [x + y for x, y in zip(c, _combine(_Tiles(m, r, GC)))]
            ops = _operands(_B_TERMS, [c[0] * ge, c[1] * go, c[2] * ge, c[3] * go])
            _put(cl_s, r, (jp % 4) * 7 * T, ops)

    def oproj(jp):
        m = [_dot(_get(wl_s, 0, HM, n * T, T), _get(cl_s, 0, HD, ((jp % 4) * 7 + n) * T, T), _NN)
             for n in range(7)]
        cols = slice(2 * jp * T, (2 * jp + 2) * T)
        for r in range(0, HM, 32):
            c = _combine(_Tiles(m, r, 32))
            o_s[r:r + 32, cols] += jnp.concatenate(c[:2], axis=1)
            o_s[HM + r:HM + r + 32, cols] += jnp.concatenate(c[2:], axis=1)
        clk.stage(392, [m[0], m[4]])

    def oproj_out(jp):
        oproj(jp)

        @pl.when(h == H - 1)
        def _():
            out_copy(jp).start()

    for n1 in range(7):
        if n1 >= NT1:
            prep_w(h, [n1], clk.pacer(max(clk.t - LEAD - 448, 1), max(clk.t - LEAD, 1), 8))
        proj(0, n1, n1 + 1)
    oproj(NP - 1)
    for jp, cover in enumerate(PLAN):
        mx = qk(jp)
        t0 = clk.t
        for item in cover.split():
            if item[0] == 'P':
                pv(int(item[1]))
            elif item[0] == 'O':
                oproj_out(int(item[1]))
            else:
                proj(int(item[1]), int(item[2]), int(item[3]))
        softmax(jp, mx, t0 + D0, clk.t - SLACK)
        if jp == 0:
            prep_wo(clk.pacer(t0, clk.t, HM // 16))
    t0 = clk.t
    pv(NP - 1)
    oproj_out(NP - 2)
    prep_w(jnp.minimum(h + 1, H - 1), range(NT1), clk.pacer(t0 - PW0, clk.t - 300, 8 * NT1))

    @pl.when(h == H - 1)
    def _():
        oproj(NP - 1)
        out_copy(NP - 1).start()
        for jp in range(NP):
            out_copy(jp).wait()


@jax.jit
def pallas_gated_mix__compressed_kv_cla__ssm_conv_s5__prompt_kernel(
    A_x: jax.Array,
    A_c_kv: jax.Array,
    A_w_q: jax.Array,
    A_w_uk: jax.Array,
    A_w_uv: jax.Array,
    A_w_o: jax.Array,
    B_x: jax.Array,
    B_Lambda_re: jax.Array,
    B_Lambda_im: jax.Array,
    B_B_re: jax.Array,
    B_B_im: jax.Array,
    B_C_re: jax.Array,
    B_C_im: jax.Array,
    B_log_dt: jax.Array,
    B_Dskip: jax.Array,
    gate_w: jax.Array,
):
    del B_x
    xT = jnp.transpose(A_x[0])
    woT = jnp.transpose(A_w_o, (0, 2, 1))
    ckv = A_c_kv.reshape(4, 4, 2, T // 2, DC)

    hbm = pl.BlockSpec(memory_space=pl.ANY)
    vmem = pltpu.VMEM
    outT = pl.pallas_call(
        _kernel,
        grid=(H,),
        in_specs=[hbm] * 15,
        out_specs=hbm,
        out_shape=jax.ShapeDtypeStruct((M, S), f32),
        scratch_shapes=[
            vmem((M, S), bf16),
            vmem((M,), bf16), vmem((M,), bf16), vmem((M,), bf16), vmem((M,), bf16), vmem((M,), bf16),
            vmem((2 * M, M), bf16),
            vmem((2, M, M), bf16),
            vmem((M // 2, 2 * M), u32),
            vmem((8, 512), f32),
            vmem((8, 8, 512), f32),
            vmem((2, M, T), f32),
            vmem((S, 2 * M), f32),
            vmem((TC // 2, 2 * M), u32),
            vmem((1, S), f32),
            vmem((4, 4, 2, T // 2, DC), bf16),
            vmem((M, H, D), bf16),
            vmem((NRAW * CS, H, D), bf16),
            vmem((NRAW * CS, H, D), bf16),
            vmem((4, M * 4, T), u32),
            vmem((4, CS * 4, T), u32),
            vmem((4, CS * 4, T), u32),
            vmem((H // 2 * D, DC), u32),
            vmem((H // 2 * D, DC), u32),
            vmem((S // 8, 49 * QC), u32),
            vmem((HM // 2, NP * 7 * T), u32),
            vmem((H * D, S // 2), u32),
            vmem((H, M, D), bf16),
            vmem((QD, 49 * QC), u32),
            vmem((HM // 2, 7 * T), u32),
            vmem((7 * HD, 2 * T), f32),
            vmem((7 * HD, 2 * T), f32),
            vmem((2 * T, 4 * T), f32),
            vmem((S // 4, 9 * T), u32),
            vmem((HD // 2, NP * 9 * T), u32),
            vmem((2, S // 8, 8, 2 * T), f32),
            vmem((14 * T, 9 * T), u32),
            vmem((HD // 2, 28 * T), u32),
            vmem((M, S), f32),
            vmem((8, T), f32),
            vmem((256, 8, 2 * T), f32),
            vmem((1, S), f32),
            pltpu.SemaphoreType.DMA((NSEM,)),
        ],
        compiler_params=pltpu.CompilerParams(
            dimension_semantics=("arbitrary",),
            vmem_limit_bytes=126 * 1024 * 1024,
        ),
    )(xT, B_B_re, B_B_im, B_C_re, B_C_im, B_Lambda_re, B_Lambda_im, B_log_dt,
      B_Dskip, gate_w, woT, ckv, A_w_q, A_w_uk, A_w_uv)
    return jnp.transpose(outT)[None]
```

```python
import os

import jax
import jax.numpy as jnp
from jax import lax
import jax.experimental.pallas as pl
import jax.experimental.pallas.tpu as pltpu

S = 2048
M = 448
H = 16
D = 256
DC = 1024
T = 128
NP = S // T // 2
HD = D // 2
HM = M // 2
QD = D // 4
QC = DC // 4
PA = 384
PB = M - PA
TA = 512
TC = 256
CS = DC // NP
NRAW = 4
LOG2E = 1.4426950408889634
NEG = -1e30

_env = lambda k, d: type(d)(os.environ.get(k, d))
GC = _env('GC', 64)
GS = _env('GS', 16)
RCH = _env('RCH', 256)
SLACK = _env('SLACK', 200)
D0 = _env('D0', 0)
NT1 = _env('NT1', 3)
LEAD = _env('LEAD', 448)
PW0 = _env('PW0', 100)
QCH = _env('QCH', 64)
OCH = ((0, 64), (64, 64), (128, 48), (176, 48))
LSUB = _env('LSUB', 4)
PLAN = _env('PLAN', ',K107,,K207,,K307,,P0 P1 P2,O0 O1 O2 P3 O3 O4 O5 O6').split(',')

f32 = jnp.float32
bf16 = jnp.bfloat16
u32 = jnp.uint32

SEM_VEC, SEM_B, SEM_X, SEM_WQ, SEM_C, SEM_SL, SEM_WO, SEM_OUT, SEM_WQ1 = 0, 1, 2, 6, 7, 8, 16, 17, 18
NSEM = 22

_NN = ((1,), (0,))
_NT = ((1,), (1,))
_TN = ((0,), (0,))
_TT = ((0,), (1,))


def _dot(a, b, dims):
    return lax.dot_general(a, b, (dims, ((), ())), preferred_element_type=f32)


def _cat(xs, axis):
    return xs[0] if len(xs) == 1 else jnp.concatenate(xs, axis=axis)


def _ds(lo, n, align):
    return pl.ds(lo if isinstance(lo, int) else pl.multiple_of(lo, align), n)


def _put(ref, row, col, xs):
    x = _cat(xs, 1)
    ref[row // 2:(row + x.shape[0]) // 2, col:col + x.shape[1]] = pltpu.bitcast(x.astype(bf16), u32)


def _get(ref, row, nrows, col, ncols):
    return pltpu.bitcast(ref[row // 2:(row + nrows) // 2, col:col + ncols], bf16)


class _Clock:
    def __init__(self, zero_ref):
        self.masks = {(8, T): zero_ref[...] != 0.0}
        self.ticks, self.load = [], [0, 0, 0, 0]

    @property
    def t(self):
        return max(self.load)

    def dot(self, a, b, dims):
        v = _dot(a, b, dims)
        rows, depth = v.shape[0], a.shape[dims[0][0]]
        for c in range(0, v.shape[1], T):
            start = 0
            for _ in range(0, depth, T):
                k = self.load.index(min(self.load))
                start = max(start, self.load[k])
                self.load[k] += rows
            self.ticks += [(start + r + 8, (v, r, c)) for r in range(0, rows, 8)]
        return v, start

    def strassen(self, lhs, rhs, dims, split_last=False):
        jobs = -(-lhs(0).shape[dims[0][0]] // T)
        lag = sum(l + 32 <= max(self.load) for l in self.load) // jobs if jobs < 3 else 0
        order = ((1, 3, 2, 4, 0, 5, 6), (0, 1, 3, 2, 4, 5, 6), (5, 6, 1, 3, 2, 4, 0), (0, 5, 6, 1, 3, 2, 4))[lag]
        m = {}
        for n in order:
            if split_last and n == order[-1]:
                a, half = lhs(n), lhs(0).shape[0] // 2
                m[n] = jnp.concatenate([self.dot(a[:half], rhs(n), dims)[0], self.dot(a[half:], rhs(n), dims)[0]], 0)
            else:
                m[n] = self.dot(lhs(n), rhs(n), dims)[0]
        vals = [m[n] for n in range(7)]
        return lambda r=0, n=None, only=(0, 1, 2, 3), c=0, w=None: _combine(
            vals if n is None else _Tiles(vals, r, n, c, w), only, order)

    def level(self, pairs):
        target = (sum(self.load) + sum(a.shape[0] for a, _ in pairs)) // 4
        out = []
        for a, b in pairs:
            r, parts = 0, []
            while r < a.shape[0]:
                n = min(max(target - min(self.load), 16) // 16 * 16, a.shape[0] - r)
                parts.append(self.dot(a[r:r + n], b, _NN)[0])
                r += n
            out.append(_cat(parts, 0))
        return out

    def pacer(self, t0, t1, n):
        def tie(x, k):
            past = [tw for tw in self.ticks if tw[0] <= t0 + (t1 - t0) * k / n]
            if not past:
                return x
            v, r, c = max(past, key=lambda tw: tw[0])[1]
            tick = v[r:r + 8, c:c + T]
            if tick.dtype != x.dtype:
                tick = pltpu.bitcast(tick, x.dtype)
            reps = (x.shape[0] // 8, x.shape[1] // T)
            if x.shape not in self.masks:
                self.masks[x.shape] = jnp.tile(self.masks[(8, T)], reps)
            return lax.select(self.masks[x.shape], tick if reps == (1, 1) else jnp.tile(tick, reps), x)
        return tie


def _no_tie(x, k):
    return x


_A_TERMS = ((0, 3, 1), (2, 3, 1), (0, None, 0), (3, None, 0), (0, 1, 1), (2, 0, -1), (1, 3, -1))
_B_TERMS = ((0, 3, 1), (0, None, 0), (1, 3, -1), (2, 0, -1), (3, None, 0), (0, 1, 1), (2, 3, 1))


def _operand(term, block):
    x, y, sign = term
    if y is None:
        return block(x)
    return block(x) + block(y) if sign > 0 else block(x) - block(y)


def _operands(terms, blocks):
    return [_operand(t, blocks.__getitem__) for t in terms]


def _operands2(terms, n1, block, tie):
    first = terms[n1][0]
    sub = [_operand(terms[n1], lambda o: tie(block(o, q)) if o == first and q in (0, 3) else block(o, q))
           for q in range(4)]
    return _operands(terms, sub)


_C_TERMS = ({0: 1, 3: 1, 4: -1, 6: 1}, {2: 1, 4: 1}, {1: 1, 3: 1}, {0: 1, 1: -1, 2: 1, 5: 1})


def _combine(m, only=(0, 1, 2, 3), order=(1, 3, 2, 4, 0, 5, 6)):
    out = []
    for terms in (_C_TERMS[n] for n in only):
        seq = [n for n in order if n in terms]
        if terms[seq[0]] < 0:
            seq[0], seq[1] = seq[1], seq[0]
        acc = m[seq[0]]
        for n in seq[1:]:
            acc = acc + m[n] if terms[n] > 0 else acc - m[n]
        out.append(acc)
    return out


class _Tiles:
    def __init__(self, vals, r, n, c=0, w=None):
        self.vals, self.idx, self.cache = vals, (slice(r, r + n), slice(c, None if w is None else c + w)), {}

    def __getitem__(self, i):
        if i not in self.cache:
            self.cache[i] = self.vals[i][self.idx]
        return self.cache[i]


class _Reducer:
    def __init__(self, red, comb):
        self.red, self.comb, self.acc, self.rows, self.out = red, comb, None, 0, None

    def add(self, v):
        self.rows += 8 * v.shape[0]
        v = self.red(v, axis=0)
        self.acc = v if self.acc is None else self.comb(self.acc, v)
        if self.rows >= RCH:
            self.result()

    def result(self):
        if self.acc is not None:
            v = self.red(self.acc, axis=0, keepdims=True)
            self.out = v if self.out is None else self.comb(self.out, v)
        self.acc, self.rows = None, 0
        return self.out


def _cmul(ar, ai, br, bi):
    return ar * br - ai * bi, ar * bi + ai * br


def _hi16(w):
    return pltpu.bitcast(w & jnp.uint32(0xFFFF0000), f32)


def _stage(raw, stg, c0, nc, tie, groups=(0, 1)):
    for ht in groups:
        for dt in range(2):
            v = raw[c0:c0 + nc, ht * 8:(ht + 1) * 8, dt * T:(dt + 1) * T].reshape(nc * 8, T)
            stg[ht * 2 + dt, c0 * 4:(c0 + nc) * 4, :] = tie(pltpu.bitcast(v, u32))


def _ssm_params(vec_s, coef_s, lam_s, col_s):
    row = lambda r: r[...].astype(f32).reshape(1, M)
    lre, lim, ldt, dsk, gw = [row(v) for v in vec_s]
    dt = jnp.exp(ldt).astype(bf16).astype(f32)
    mag = jnp.exp(dt * lre)
    ang = dt * lim
    lr, li = mag * jnp.cos(ang), mag * jnp.sin(ang)
    den = lre * lre + lim * lim
    nr = lr - 1.0
    coef_s[...] = jnp.zeros(coef_s.shape, f32)
    coef_s[0:1, 0:M] = 2.0 * ((nr * lre + li * lim) / den)
    coef_s[1:2, 0:M] = 2.0 * ((li * lre - nr * lim) / den)

    er = jnp.concatenate([lr, lr[:, PA:]], axis=1)
    ei = jnp.concatenate([li, -li[:, PA:]], axis=1)
    pw = [(er, ei)]
    for _ in range(7):
        pw.append(_cmul(pw[-1][0], pw[-1][1], er, ei))
    sub = lax.broadcasted_iota(jnp.int32, (8, 512), 0)
    for n, d in enumerate((1, 2, 4)):
        lam_s[2 * n] = jnp.where(sub >= d, pw[d - 1][0], 0.0)
        lam_s[2 * n + 1] = jnp.where(sub >= d, pw[d - 1][1], 0.0)
    lcr = jnp.zeros((8, 512), f32)
    lci = jnp.zeros((8, 512), f32)
    for r in range(8):
        lcr = jnp.where(sub == r, pw[r][0], lcr)
        lci = jnp.where(sub == r, pw[r][1], lci)
    lam_s[6] = lcr
    lam_s[7] = lci

    def col(v):
        v = jnp.concatenate([v, jnp.zeros((1, 512 - M), f32)], axis=1)
        return jnp.broadcast_to(v, (T, 512)).T[:M]
    col_s[0] = col(dsk)
    col_s[1] = col(gw)


def _ssm_cmat(craw_s, coef_s, c_s, tie):
    for r in range(0, M, 16):
        coef = tie(coef_s[...], r // 16)
        cr, ci = coef[0:1, :M], coef[1:2, :M]
        re, im = _cmul(craw_s[0, r:r + 16, :].astype(f32), craw_s[1, r:r + 16, :].astype(f32), cr, ci)
        _put(c_s, r, 0, [re[:, :PA], -im[:, :PA], re[:, PA:], -im[:, PA:]])


def _ssm_scan(u_ref, carry, lam_s, h_s, tie):
    car, cai = carry
    out = []
    for b in range(TC // 8):
        mixed = u_ref[3, b, :, 0:T]
        u = jnp.concatenate([u_ref[cb, b] for cb in range(3)], axis=1)
        cols = [u[:, 0:T], u[:, T:2 * T], u[:, 2 * T:PA], mixed]
        hr = jnp.concatenate([tie(v, 4 * b + n) for n, v in enumerate(cols)], axis=1)
        hi = jnp.concatenate([u[:, PA:2 * PA], pltpu.roll(mixed, PB, 1)], axis=1)
        for n, d in enumerate((1, 2, 4)):
            sr, si = pltpu.roll(hr, d, 0), pltpu.roll(hi, d, 0)
            tr, ti = _cmul(sr, si, lam_s[2 * n], lam_s[2 * n + 1])
            hr, hi = hr + tr, hi + ti
        tr, ti = _cmul(lam_s[6], lam_s[7], car, cai)
        hr, hi = hr + tr, hi + ti
        car, cai = hr[7:8, :], hi[7:8, :]
        out.append(jnp.concatenate([hr[:, :PA], hi[:, :PA], hr[:, PA:]], axis=1))
        if b % 2 == 1:
            _put(h_s, (b - 1) * 8, 0, [jnp.concatenate(out, axis=0)])
            out = []
    return car, cai


_vmem = pltpu.VMEM
_PROLOGUE_SCRATCH = dict(
    xT_s=_vmem((M, S), bf16),
    v0=_vmem((M,), bf16), v1=_vmem((M,), bf16), v2=_vmem((M,), bf16), v3=_vmem((M,), bf16), v4=_vmem((M,), bf16),
    b_s=_vmem((2 * M, M), bf16),
    craw_s=_vmem((2, M, M), bf16),
    c_s=_vmem((M // 2, 2 * M), u32),
    coef_s=_vmem((8, 512), f32),
    lam_s=_vmem((8, 8, 512), f32),
    col_s=_vmem((2, M, T), f32),
    h_s=_vmem((TC // 2, 2 * M), u32),
    ckv_s=_vmem((4, 4, 2, T // 2, DC), bf16),
    rq=_vmem((M, H, D), bf16),
    rk=_vmem((NRAW * CS, H, D), bf16),
    rv=_vmem((NRAW * CS, H, D), bf16),
    sq=_vmem((4, M * 4, T), u32),
    sk=_vmem((4, CS * 4, T), u32),
    sv=_vmem((4, CS * 4, T), u32),
    xa_s=_vmem((HM // 2, NP * 7 * T), u32),
)
_HEAD_SCRATCH = dict(
    mk_s=_vmem((7 * HD, 2 * T), f32),
    mv_s=_vmem((7 * HD, 2 * T), f32),
    mp_s=_vmem((7 * HD, 2 * T), f32),
    kt_s=_vmem((2 * T, 4 * T), f32),
    ka_s=_vmem((S // 4, 9 * T), u32),
    va_s=_vmem((HD // 2, NP * 9 * T), u32),
    v2_s=_vmem((QD // 2, 3 * 49 * T), u32),
    s_s=_vmem((4, S // 8, 8, 2 * T), f32),
    pb_s=_vmem((2 * T, 7 * T), u32),
    pd_s=_vmem((S // 2, 2 * T), u32),
    p2_s=_vmem((3 * T, 49 * T), u32),
    sc_s=_vmem((1, S), f32),
    qb_s=_vmem((HD // 2, 14 * T), u32),
)
_SHARED_SCRATCH = [
    _vmem((H // 2 * D, DC), u32),
    _vmem((H // 2 * D, DC), u32),
    _vmem((S // 8, 49 * QC), u32),
    _vmem((H * D, S // 2), u32),
    _vmem((H, M, D), bf16),
    _vmem((QD, 49 * QC), u32),
    _vmem((HM // 2, 7 * T), u32),
    _vmem((HD // 2, NP * 7 * T), u32),
    _vmem((M, S), f32),
    _vmem((1, S), f32),
    _vmem((8, T), f32),
    pltpu.SemaphoreType.DMA((NSEM,)),
]


def _kernel(xT_hbm, bre_hbm, bim_hbm, cre_hbm, cim_hbm, lre_hbm, lim_hbm, ldt_hbm,
            dsk_hbm, gw_hbm, woT_hbm, ckv_hbm, wq_hbm, wk_hbm, wv_hbm,
            out_hbm,
            wkt_s, wvt_s, a_s, q_s, wo_s, w_s, wl_s, cl_s, o_s, g_s, zero_s, sem, *rest):
    h = pl.program_id(0)
    pro_refs = dict(zip(_PROLOGUE_SCRATCH, rest))
    head_refs = dict(zip(_HEAD_SCRATCH, rest[len(pro_refs):]))

    def out_copy(jp):
        cols = pl.ds(jp * 2 * T, 2 * T)
        return pltpu.make_async_copy(o_s.at[:, cols], out_hbm.at[:, cols], sem.at[SEM_OUT])

    def prep_w(hh, outer, tie):
        rows = _ds(lax.shift_right_logical(hh, 1) * D, D, D)
        sh = (16 * (1 - (hh & 1))).astype(u32)
        k = 0
        for row0, wt_s in ((0, wkt_s.at[rows]), (QD, wvt_s.at[rows])):
            for r in range(0, QD, 16):
                def block(o, q):
                    row = (o % 2) * HD + (q % 2) * QD + r
                    col = (o // 2) * 2 * QC + (q // 2) * QC
                    return _hi16(wt_s[row:row + 16, col:col + QC] << sh)
                for n1 in outer:
                    _put(w_s, row0 + r, 7 * n1 * QC, _operands2(_B_TERMS, n1, block, lambda x: tie(x, k)))
                    k += 1

    def prologue(xT_s, v0, v1, v2, v3, v4, b_s, craw_s, c_s, coef_s, lam_s, col_s, h_s,
                 ckv_s, rq, rk, rv, sq, sk, sv, xa_s):
        u_s = head_refs['s_s']
        vec_s = (v0, v1, v2, v3, v4)

        def slice_copies(i):
            s = sem.at[SEM_SL + i]
            grp = i // 2 if isinstance(i, int) else lax.shift_right_logical(i, 1)
            cs, dst = pl.ds(i * CS, CS), pl.ds((i & (NRAW - 1)) * CS, CS)
            return [pltpu.make_async_copy(ckv_hbm.at[grp, :, i & 1], ckv_s.at[grp, :, i & 1], s),
                    pltpu.make_async_copy(wk_hbm.at[cs], rk.at[dst], s),
                    pltpu.make_async_copy(wv_hbm.at[cs], rv.at[dst], s)]

        def wq1_copy(i):
            rows = pl.ds(i * (M // 4), M // 4)
            return pltpu.make_async_copy(wq_hbm.at[rows, 8:16], rq.at[rows, 8:16], sem.at[SEM_WQ1 + i])

        def x_copy(i):
            cols = pl.ds(i * TA, TA)
            return pltpu.make_async_copy(xT_hbm.at[:, cols], xT_s.at[:, cols], sem.at[SEM_X + i])

        cp_vec = [pltpu.make_async_copy(src, dst, sem.at[SEM_VEC])
                  for src, dst in zip((lre_hbm, lim_hbm, ldt_hbm, dsk_hbm, gw_hbm), vec_s)]
        cp_b = [pltpu.make_async_copy(src.at[pl.ds(lo, n)], b_s.at[pl.ds(dst, n)], sem.at[SEM_B])
                for src, lo, n, dst in ((bre_hbm, 0, PA, 0), (bim_hbm, 0, PA, PA),
                                        (bre_hbm, PA, PB, 2 * PA), (bim_hbm, PA, PB, 2 * PA + PB))]
        cp_wq = [pltpu.make_async_copy(wq_hbm.at[:, 0:8], rq.at[:, 0:8], sem.at[SEM_WQ])]
        cp_c = [pltpu.make_async_copy(src, craw_s.at[n], sem.at[SEM_C])
                for n, src in enumerate((cre_hbm, cim_hbm))]
        cp_wo = pltpu.make_async_copy(woT_hbm, wo_s, sem.at[SEM_WO])
        for cp in cp_vec + cp_b + [x_copy(i) for i in range(S // TA)] + cp_c + cp_wq:
            cp.start()
        for i in range(NRAW - 1):
            for cp in [wq1_copy(i)] + slice_copies(i):
                cp.start()
        wq1_copy(3).start()
        cp_wo.start()

        zero_s[...] = jnp.zeros(zero_s.shape, f32)
        wl_s[...] = jnp.zeros(wl_s.shape, u32)
        cl_s[:, (NP - 1) * 7 * T:] = jnp.zeros((HD // 2, 7 * T), u32)
        for cp in cp_vec:
            cp.wait()
        _ssm_params(vec_s, coef_s, lam_s, col_s)

        def phase1(i):
            clk = _Clock(zero_s)
            u, _ = clk.dot(xT_s[:, i * TA:(i + 1) * TA], b_s[...], _TT)
            for cb in range(4):
                w = min(2 * T, 2 * M - cb * 2 * T)
                u_s[cb, i * TA // 8:(i + 1) * TA // 8, :, 0:w] = (
                    u[:, cb * 2 * T:cb * 2 * T + w].reshape(TA // 8, 8, w))
            tie = clk.pacer(0, 6 * TA, 14)
            for t in range(2 * i, 2 * i + 2):
                for r in range(0, HM, 32):
                    k = (t % 2) * 7 + r // 32
                    top = xT_s[r:r + 32, 2 * t * T:(2 * t + 2) * T].astype(f32)
                    bot = xT_s[HM + r:HM + r + 32, 2 * t * T:(2 * t + 2) * T].astype(f32)
                    blocks = [tie(top[:, :T], k), bot[:, :T], top[:, T:], tie(bot[:, T:], k)]
                    _put(xa_s, r, t * 7 * T, _operands(_A_TERMS, blocks))
            return clk

        for cp in cp_b + [x_copy(0)]:
            cp.wait()
        phase1(0)
        x_copy(1).wait()
        clk = phase1(1)
        zero = jnp.zeros((1, 512), f32)
        carry0 = _ssm_scan(u_s.at[:, 0:TC // 8], (zero, zero), lam_s, h_s, clk.pacer(0, 6 * TA, TC // 2))
        for cp in [x_copy(2), x_copy(3)] + cp_c + cp_wq:
            cp.wait()
        _ssm_cmat(craw_s, coef_s, c_s, phase1(2).pacer(0, 6 * TA, M // 16))
        tie = phase1(3).pacer(0, 6 * TA, M // 8)
        for c0 in range(0, M, 8):
            _stage(rq, sq, c0, 8, lambda x: tie(x, c0 // 8), groups=(0,))

        def phase2(i, carry):
            @pl.when(i + NRAW - 1 < NP)
            def _():
                for cp in slice_copies(i + NRAW - 1):
                    cp.start()

            @pl.when(i < 4)
            def _():
                wq1_copy(i).wait()

            for cp in slice_copies(i):
                cp.wait()

            yT = _dot(_get(c_s, 0, M, 0, 2 * M), _get(h_s, 0, TC, 0, 2 * M), _NT)
            for t in range(TC // T):
                cols = _ds(i * TC + t * T, T, T)
                acc = jnp.zeros((8, T), f32)
                for r in range(0, M, 32):
                    xg = xT_s[r:r + 32, cols].astype(f32) * col_s[1, r:r + 32, :]
                    acc = acc + jnp.sum(xg.reshape(4, 8, T), axis=0)
                g = jax.nn.sigmoid(jnp.sum(acc, axis=0, keepdims=True))
                g_s[:, cols] = g
                for r in range(0, M, 32):
                    skip = xT_s[r:r + 32, cols].astype(f32) * col_s[0, r:r + 32, :]
                    o_s[r:r + 32, cols] = (1.0 - g) * (yT[r:r + 32, t * T:(t + 1) * T] + skip)

            ht = lax.shift_right_logical(i, 2)
            words = [sq[ht * 2 + dt, pl.ds(i & 3, M, stride=4), :] for dt in range(2)]
            both = [jnp.concatenate([pltpu.bitcast(w << 16, f32), _hi16(w)], axis=1) for w in words]
            wq = _operands(_B_TERMS, [both[0][:HM], both[1][:HM], both[0][HM:], both[1][HM:]])
            clk = _Clock(zero_s)
            m = [clk.dot(wq[n].astype(bf16),
                         _cat([_get(xa_s, 0, HM, (t * 7 + n) * T, T) for t in range(NP)], 1), _TN)[0]
                 for n in range(7)]
            q_i = q_s.at[_ds(i * 2 * D, 2 * D, 2 * D)]
            for n in (2, 1, 3, 0):
                for t in range(NP):
                    for r in range(0, D, GC):
                        c, = _combine(_Tiles(m, r, GC, t * T, T), (n,), range(7))
                        row = (2 * (r // HD) + n // 2) * D + (n % 2) * HD + r % HD
                        _put(q_i, row, t * T, [c * (LOG2E * D ** -0.5)])

            span = 5 * 1024

            u_next = u_s.at[:, pl.ds(jnp.minimum(i + 1, NP - 1) * (TC // 8), TC // 8)]
            carry = _ssm_scan(u_next, carry, lam_s, h_s, clk.pacer(0, span, TC // 2))

            tie = clk.pacer(0, span, 64)
            rq_i = rq.at[pl.ds((i & 3) * (M // 4), M // 4)]
            sq_i = sq.at[:, _ds((i & 3) * M, M, 8)]
            for c0 in range(0, M // 4, 8):
                _stage(rq_i, sq_i, c0, 8, lambda x: tie(x, c0 // 2 + 2), groups=(1,))
            slot = pl.ds((i & (NRAW - 1)) * CS, CS)
            for n, (raw, stg, wt_s) in enumerate(((rk, sk, wkt_s), (rv, sv, wvt_s))):
                for c0 in range(0, CS, 8):
                    _stage(raw.at[slot], stg, c0, 8, lambda x: tie(x, 16 * n + c0 // 8))
                cols = _ds(i * CS, CS, CS)
                for pair in range(H // 2):
                    for dt in range(2):
                        blk = stg[(pair // 4) * 2 + dt, pl.ds(pair % 4, CS, stride=4), :]
                        row = pair * D + dt * HD
                        wt_s[row:row + HD, cols] = tie(blk, 16 + 24 * n + 3 * pair + dt).T

            tie = clk.pacer(0, span, 28)
            ckv_i = ckv_s.at[lax.shift_right_logical(i, 1), :, i & 1]
            a_i = a_s.at[_ds(i * (T // 4), T // 4, T // 4)]
            for r in range(0, T // 2, 16):
                def block(o, q):
                    col = (o % 2) * 2 * QC + (q % 2) * QC
                    return ckv_i[2 * (q // 2) + o // 2, r:r + 16, col:col + QC].astype(f32)
                for n1 in range(7):
                    ops = _operands2(_A_TERMS, n1, block, lambda x: tie(x, 7 * (r // 16) + n1))
                    _put(a_i, r, 7 * n1 * QC, ops)
            return carry

        lax.fori_loop(0, NP, phase2, carry0)
        cp_wo.wait()
        prep_w(h, range(NT1), _no_tie)

    @pl.when(h == 0)
    def _():
        prologue(**pro_refs)

    def oproj(jp, clk):
        cols = slice(2 * jp * T, (2 * jp + 2) * T)
        for r, n in OCH:
            c = clk.strassen(lambda i: _get(wl_s, r, n, i * T, T),
                             lambda i: _get(cl_s, 0, HD, (jp * 7 + i) * T, T), _NN)()
            o_s[r:r + n, cols] += jnp.concatenate(c[:2], axis=1)
            o_s[HM + r:HM + r + n, cols] += jnp.concatenate(c[2:], axis=1)

    def head(mk_s, mv_s, mp_s, kt_s, ka_s, va_s, v2_s, s_s, pb_s, pd_s, p2_s, sc_s, qb_s):
        clk = _Clock(zero_s)
        q_h = q_s.at[_ds(h * D, D, D)]

        def prep_wo(tie):
            for r in range(0, HM, 16):
                top = tie(wo_s[h, r:r + 16, :].astype(f32), r // 16)
                bot = tie(wo_s[h, HM + r:HM + r + 16, :].astype(f32), r // 16)
                _put(wl_s, r, 0, _operands(_A_TERMS, [top[:, :HD], top[:, HD:], bot[:, :HD], bot[:, HD:]]))

        def outer(m_s, r):
            return _combine([m_s[n * HD + r:n * HD + r + 16, :] for n in range(7)], order=range(7))

        def proj(g, lo, hi):
            for n1 in range(lo, hi):
                comb = clk.strassen(lambda n: _get(w_s, 0, 2 * QD, (7 * n1 + n) * QC, QC),
                                    lambda n: _get(a_s, g * T, T, (7 * n1 + n) * QC, QC), _NT, n1 == 6)
                for r in range(0, 2 * QD, GC):
                    m_s, row = mk_s if r < QD else mv_s, n1 * HD + r % QD
                    c = comb(r, GC)
                    m_s[row:row + GC, :] = jnp.concatenate([c[0], c[2]], axis=1)
                    m_s[QD + row:QD + row + GC, :] = jnp.concatenate([c[1], c[3]], axis=1)
            if hi < 7:
                return
            nine = lambda c: _operands(_A_TERMS, c) + [c[1], c[2]]
            cs = [outer(mk_s, r) for r in range(0, HD, 16)]
            for n in range(4):
                kt_s[:, n * T:(n + 1) * T] = jnp.concatenate([c[n] for c in cs], axis=0).T
            for r in range(0, 2 * T, GC):
                blk = kt_s[r:r + GC, :]
                _put(ka_s, 2 * g * T + r, 0, nine([blk[:, n * T:(n + 1) * T] for n in range(4)]))
            for r in range(0, QD, 16):
                ops = []
                for row in (r, QD + r):
                    c = outer(mv_s, row)
                    ops.append(nine([c[0], c[2], c[1], c[3]]))
                    _put(va_s, row, 2 * g * 9 * T, [o[:, :T] for o in ops[-1]])
                    for n in (2, 7):
                        _put(va_s, row, ((2 * g + 1) * 9 + n) * T, [o[:, T:] for o in ops[-1][n:n + 2]])
                if g < 3:
                    for n1 in range(7):
                        lo_, hi_ = ops[0][n1], ops[1][n1]
                        _put(v2_s, r, (g * 7 + n1) * 7 * T,
                             _operands(_A_TERMS, [lo_[:, :T], lo_[:, T:], hi_[:, :T], hi_[:, T:]]))

        key = lax.broadcasted_iota(jnp.int32, (T, 2 * T), 0)
        qry = lax.broadcasted_iota(jnp.int32, (T, 2 * T), 1)
        causal = key <= qry

        def qk(g):
            pairs = (2 * g, 2 * g + 1)
            mx = {jp: _Reducer(jnp.max, jnp.maximum) for jp in pairs}

            def put(jp, row, v):
                v = v.reshape(v.shape[0] // 8, 8, 2 * T)
                s_s[jp % 4, row // 8:row // 8 + v.shape[0]] = v
                mx[jp].add(v)

            def rect(jp, lo, hi, n):
                for r in range(lo, hi, n):
                    c = clk.strassen(lambda i: _get(ka_s, r, n, i * T, T),
                                     lambda i: _get(qb_s, 0, HD, ((jp % 2) * 7 + i) * T, T), _NN)()
                    put(jp, r, jnp.concatenate(c[:2], axis=1))
                    put(jp, jp * T + r, jnp.concatenate(c[2:], axis=1))

            q = lambda jp, e: _get(q_h, e * D, D, jp * T, T)
            for jp in pairs[g == 0:]:
                for r in range(0, HD, 32):
                    blk = [_get(q_h, e * D + d * HD + r, 32, jp * T, T).astype(f32) for d in range(2) for e in range(2)]
                    _put(qb_s, r, (jp % 2) * 7 * T, _operands(_B_TERMS, blk))
            for jp in pairs:
                rect(jp, 0, 2 * g * T, QCH if QCH else g * T // 2 or 1)
            kb = lambda jp, a, b: jnp.concatenate(
                [_get(ka_s, jp * T, T, a * T, T), _get(ka_s, jp * T, T, b * T, T)], axis=1)
            for jp in pairs:
                se, _ = clk.dot(kb(jp, 2, 7), jnp.concatenate([q(jp, 0), q(jp, 1)], axis=1), _NN)
                put(jp, 2 * jp * T, jnp.where(causal, se, NEG))
            last = {}
            for jp in pairs:
                so = jnp.where(causal[:, :T], clk.dot(kb(jp, 8, 3), q(jp, 1), _NN)[0], NEG)
                row = (2 * jp + 1) * T // 8
                s_s[jp % 4, row:row + T // 8, :, T:] = so.reshape(T // 8, 8, T)
                last[jp] = jnp.concatenate([jnp.full((1, T), NEG, f32), jnp.max(so, axis=0, keepdims=True)], axis=1)
            rect(2 * g + 1, 2 * g * T, (2 * g + 1) * T, T // 4)
            return [jnp.broadcast_to(jnp.maximum(mx[jp].result(), last[jp]), (8, 2 * T)) for jp in pairs]

        zs, sums = {}, {}

        def prob(jp, row, z, n=GS, lanes=slice(None)):
            return jnp.exp2(s_s[jp % 4, row // 8:(row + n) // 8, :, lanes] - z[:, lanes])

        def rough(jp, mx, tie):
            zs[jp] = mx
            if jp > 0:
                sm = _Reducer(jnp.sum, jnp.add)
                for k, r in enumerate(range(0, 2 * jp * T, GS * LSUB)):
                    sm.add(prob(jp, r, tie(mx, k)))
                zs[jp] = mx + jnp.log2(jnp.maximum(LSUB * sm.result(), 1.0))
            sums[jp] = _Reducer(jnp.sum, jnp.add)

        def blocks(jp, row, tie, k):
            top, bot = prob(jp, row, tie(zs[jp], k)), prob(jp, jp * T + row, tie(zs[jp], k + 1))
            sums[jp].add(top + bot)
            top, bot = top.reshape(GS, 2 * T), bot.reshape(GS, 2 * T)
            return [top[:, :T], top[:, T:], bot[:, :T], bot[:, T:]]

        def near(jp, tie, k):
            R, z = jp * T, zs[jp]
            if jp % 2:
                for r in range(0, T, GS):
                    _put(pb_s, jp // 2 * T + r, 0, _operands(_B_TERMS, blocks(jp, R - T + r, tie, k)))
                    k += 2
            for r in range(0, T, GS):
                p = prob(jp, 2 * R + r, tie(z, k))
                sums[jp].add(p)
                _put(pd_s, 2 * R + r, 0, [p.reshape(GS, 2 * T)])
                k += 1
            so = _Reducer(jnp.sum, jnp.add)
            for r in range(0, T, 2 * GS):
                p = prob(jp, 2 * R + T + r, tie(z, k), 2 * GS, slice(T, 2 * T))
                so.add(p)
                _put(pd_s, 2 * R + T + r, T, [p.reshape(2 * GS, T)])
                k += 1
            sums[jp].result()
            sums[jp].out = sums[jp].out + jnp.concatenate([jnp.zeros((1, T), f32), so.result()], axis=1)

        p20 = lambda g: g * (g - 1) // 2 * T

        def far(g, tie, k):
            for kg in range(g):
                for r in range(0, T, GS):
                    blk = []
                    for q in range(4):
                        blk.append(blocks(2 * g + q % 2, (2 * kg + q // 2) * T + r, tie, k))
                        k += 2
                    for n1 in range(7):
                        ops = _operands2(_B_TERMS, n1, lambda o, q: blk[q][o], lambda x: x)
                        _put(p2_s, p20(g) + kg * T + r, 7 * n1 * T, ops)
            for jp in (2 * g, 2 * g + 1):
                cols = slice(2 * jp * T, 2 * (jp + 1) * T)
                sc_s[:, cols] = g_s[:, cols] / sums[jp].result()

        def pv(g):
            pairs = (2 * g, 2 * g + 1)
            va = lambda n, t, r=0, nr=HD: _get(va_s, r, nr, (t * 9 + n) * T, T)
            for n1 in range(7 if g else 0):
                c = clk.strassen(
                    lambda n: _cat([_get(v2_s, 0, QD, (kg * 49 + 7 * n1 + n) * T, T) for kg in range(g)], 1),
                    lambda n: _get(p2_s, p20(g), g * T, (7 * n1 + n) * T, T), _NN)()
                mp_s[n1 * HD:n1 * HD + QD, :] = jnp.concatenate(c[:2], axis=1)
                mp_s[n1 * HD + QD:(n1 + 1) * HD, :] = jnp.concatenate(c[2:], axis=1)
            ve = [jnp.concatenate([va(2, jp), va(8, jp)], axis=0) for jp in pairs]
            vo = [jnp.concatenate([va(7, jp), va(3, jp)], axis=0) for jp in pairs]
            ce = clk.level([(ve[jp % 2], _get(pd_s, 2 * jp * T, T, 0, T)) for jp in pairs])
            co = [clk.dot(jnp.concatenate([ve[jp % 2], vo[jp % 2]], axis=1),
                          _get(pd_s, 2 * jp * T, 2 * T, T, T), _NN)[0] for jp in pairs]
            for jp in pairs:
                R, e = jp * T, jp % 2
                ge, go = sc_s[:, 2 * R:2 * R + T], sc_s[:, 2 * R + T:2 * R + 2 * T]
                for r in range(0, HD, 32):
                    c = [ce[e][r:r + 32], co[e][r:r + 32], ce[e][HD + r:HD + r + 32], co[e][HD + r:HD + r + 32]]
                    if g:
                        far_ = _combine([mp_s[n * HD + r:n * HD + r + 32, e * T:(e + 1) * T] for n in range(7)],
                                        order=range(7))
                        c = [x + y for x, y in zip(c, far_)]
                    if e:
                        near_ = clk.strassen(lambda n: va(n, 2 * g, r, 32),
                                             lambda n: _get(pb_s, g * T, T, n * T, T), _NN)()
                        c = [x + y for x, y in zip(c, near_)]
                    ops = _operands(_B_TERMS, [c[0] * ge, c[1] * go, c[2] * ge, c[3] * go])
                    _put(cl_s, r, jp * 7 * T, ops)

        def run(items):
            for item in items.split():
                if item[0] == 'P':
                    pv(int(item[1]))
                elif item[0] == 'K':
                    proj(int(item[1]), int(item[2]), int(item[3]))
                else:
                    jp = int(item[1])
                    oproj(jp, clk)

                    @pl.when(h == H - 1)
                    def _():
                        out_copy(jp).start()

        for n1 in range(7):
            if n1 >= NT1:
                prep_w(h, [n1], clk.pacer(max(clk.t - LEAD - 448, 1), max(clk.t - LEAD, 1), 8))
            proj(0, n1, n1 + 1)
        oproj(NP - 1, clk)
        for g in range(4):
            run(PLAN[2 * g])
            mx0, mx1 = qk(g)
            t0 = clk.t
            run(PLAN[2 * g + 1])
            n_rough = [2 * jp * T // (GS * LSUB) for jp in (2 * g, 2 * g + 1)]
            n_near = [(T + T // 2) // GS, (3 * T + T // 2) // GS]
            tie = clk.pacer(t0 + D0, clk.t - SLACK, sum(n_rough) + sum(n_near) + g * 8 * T // GS)
            rough(2 * g, mx0, tie)
            near(2 * g, tie, n_rough[0])
            k = n_rough[0] + n_near[0]
            rough(2 * g + 1, mx1, lambda x, i: tie(x, k + i))
            near(2 * g + 1, tie, k + n_rough[1])
            far(g, tie, k + n_rough[1] + n_near[1])
            if g == 0:
                prep_wo(clk.pacer(t0, clk.t, HM // 16))
        t0 = clk.t
        run(PLAN[NP])
        prep_w(jnp.minimum(h + 1, H - 1), range(NT1), clk.pacer(t0 - PW0, clk.t - 300, 8 * NT1))
        if os.environ.get('SHOW'):
            print('final loads', clk.load)

    head(**head_refs)

    @pl.when(h == H - 1)
    def _():
        oproj(NP - 1, _Clock(zero_s))
        out_copy(NP - 1).start()
        for jp in range(NP):
            out_copy(jp).wait()


@jax.jit
def pallas_gated_mix__compressed_kv_cla__ssm_conv_s5__prompt_kernel(
    A_x: jax.Array,
    A_c_kv: jax.Array,
    A_w_q: jax.Array,
    A_w_uk: jax.Array,
    A_w_uv: jax.Array,
    A_w_o: jax.Array,
    B_x: jax.Array,
    B_Lambda_re: jax.Array,
    B_Lambda_im: jax.Array,
    B_B_re: jax.Array,
    B_B_im: jax.Array,
    B_C_re: jax.Array,
    B_C_im: jax.Array,
    B_log_dt: jax.Array,
    B_Dskip: jax.Array,
    gate_w: jax.Array,
):
    del B_x
    xT = jnp.transpose(A_x[0])
    woT = jnp.transpose(A_w_o, (0, 2, 1))
    ckv = A_c_kv.reshape(4, 4, 2, T // 2, DC)

    hbm = pl.BlockSpec(memory_space=pl.ANY)
    outT = pl.pallas_call(
        _kernel,
        grid=(H,),
        in_specs=[hbm] * 15,
        out_specs=hbm,
        out_shape=jax.ShapeDtypeStruct((M, S), f32),
        scratch_shapes=_SHARED_SCRATCH + list(_PROLOGUE_SCRATCH.values()) + list(_HEAD_SCRATCH.values()),
        compiler_params=pltpu.CompilerParams(
            dimension_semantics=("arbitrary",),
            vmem_limit_bytes=126 * 1024 * 1024,
        ),
    )(xT, B_B_re, B_B_im, B_C_re, B_C_im, B_Lambda_re, B_Lambda_im, B_log_dt,
      B_Dskip, gate_w, woT, ckv, A_w_q, A_w_uk, A_w_uv)
    return jnp.transpose(outT)[None]
```

```python
import bisect
import os

import jax
import jax.numpy as jnp
from jax import lax
import jax.experimental.pallas as pl
import jax.experimental.pallas.tpu as pltpu

S = 2048
M = 448
H = 16
D = 256
DC = 1024
T = 128
NP = S // T // 2
HD = D // 2
HM = M // 2
QD = D // 4
QC = DC // 4
PA = 384
PB = M - PA
TA = 512
TC = 256
CS = DC // NP
NRAW = 4
LOG2E = 1.4426950408889634
NEG = -1e30

_env = lambda k, d: type(d)(os.environ.get(k, d))
GC = _env('GC', 64)
GS = _env('GS', 16)
RCH = _env('RCH', 256)
SLACK = _env('SLACK', 200)
D0 = _env('D0', 0)
NT1 = _env('NT1', 3)
LEAD = _env('LEAD', 448)
PW0 = _env('PW0', 100)
FTIE = _env('FTIE', 1)
FLAG = _env('FLAG', 40)
FW = _env('FW', 2)
HOLE0 = _env('HOLE0', 400)
HOLE1 = _env('HOLE1', 400)
QCH = _env('QCH', 64)
OCH = ((0, 64), (64, 64), (128, 48), (176, 48))
LSUB = _env('LSUB', 4)
PLAN = _env('PLAN', 'K107,K207,K307,P0 P1 O0 O1 P2 O2 O3 O4,P3 O5 O6').split(',')

f32 = jnp.float32
bf16 = jnp.bfloat16
u32 = jnp.uint32

SEM_VEC, SEM_B, SEM_X, SEM_WQ, SEM_C, SEM_SL, SEM_WO, SEM_OUT, SEM_WQ1 = 0, 1, 2, 6, 7, 8, 16, 17, 18
NSEM = 22

_NN = ((1,), (0,))
_NT = ((1,), (1,))
_TN = ((0,), (0,))
_TT = ((0,), (1,))


def _dot(a, b, dims):
    return lax.dot_general(a, b, (dims, ((), ())), preferred_element_type=f32)


def _cat(xs, axis):
    return xs[0] if len(xs) == 1 else jnp.concatenate(xs, axis=axis)


def _ds(lo, n, align):
    return pl.ds(lo if isinstance(lo, int) else pl.multiple_of(lo, align), n)


def _put(ref, row, col, xs, tie=None):
    x = _cat(xs, 1)
    if tie is not None:
        x = jnp.concatenate([tie(x[:8]), x[8:]], axis=0)
    ref[row // 2:(row + x.shape[0]) // 2, col:col + x.shape[1]] = pltpu.bitcast(x.astype(bf16), u32)


def _get(ref, row, nrows, col, ncols):
    return pltpu.bitcast(ref[row // 2:(row + nrows) // 2, col:col + ncols], bf16)


class _Clock:
    def __init__(self, zero_ref):
        self.masks = {(8, T): zero_ref[...] != 0.0}
        self.ticks, self.load = [], [0, 0, 0, 0]

    @property
    def t(self):
        return max(self.load)

    def dot(self, a, b, dims):
        v = _dot(a, b, dims)
        rows, depth = v.shape[0], a.shape[dims[0][0]]
        for c in range(0, v.shape[1], T):
            start = 0
            for _ in range(0, depth, T):
                k = self.load.index(min(self.load))
                start = max(start, self.load[k])
                self.load[k] += rows
            self.ticks += [(start + r + 8, (v, r, c)) for r in range(0, rows, 8)]
        return v, start

    def strassen(self, lhs, rhs, dims, split_last=False):
        jobs = -(-lhs(0).shape[dims[0][0]] // T)
        lag = sum(l + 32 <= max(self.load) for l in self.load) // jobs if jobs < 3 else 0
        order = ((1, 3, 2, 4, 0, 5, 6), (0, 1, 3, 2, 4, 5, 6), (5, 6, 1, 3, 2, 4, 0), (0, 5, 6, 1, 3, 2, 4))[lag]
        m = {}
        for n in order:
            if split_last and n == order[-1]:
                a, half = lhs(n), lhs(0).shape[0] // 2
                m[n] = jnp.concatenate([self.dot(a[:half], rhs(n), dims)[0], self.dot(a[half:], rhs(n), dims)[0]], 0)
            else:
                m[n] = self.dot(lhs(n), rhs(n), dims)[0]
        vals = [m[n] for n in range(7)]
        return lambda r=0, n=None, only=(0, 1, 2, 3), c=0, w=None: _combine(
            vals if n is None else _Tiles(vals, r, n, c, w), only, order)

    def level(self, pairs):
        target = -(-(sum(self.load) + sum(a.shape[0] for a, _ in pairs)) // 64) * 16
        out = []
        for a, b in pairs:
            r, parts = 0, []
            while r < a.shape[0]:
                n = min(target - min(self.load), a.shape[0] - r)
                parts.append(self.dot(a[r:r + n], b, _NN)[0])
                r += n
            out.append(_cat(parts, 0))
        return out

    def pacer(self, t0, t1, n, hole=None):
        gap = hole[1] - hole[0] if hole else 0
        ticks = sorted(self.ticks, key=lambda tw: tw[0])
        times = [tw[0] for tw in ticks]

        def tie(x, k, distinct=False, delay=0):
            t = t0 + (t1 - t0 - gap) * k / n
            t += delay + (gap if hole and t > hole[0] else 0)
            past = ticks[:bisect.bisect_right(times, t)]
            if not past:
                return x
            reps = (x.shape[0] // 8, x.shape[1] // T)
            tick = _cat([v[r:r + 8, c:c + T] for _, (v, r, c) in past[-reps[1] if distinct else -1:]], 1)
            if tick.dtype != x.dtype:
                tick = pltpu.bitcast(tick, x.dtype)
            if x.shape not in self.masks:
                self.masks[x.shape] = jnp.tile(self.masks[(8, T)], reps)
            return lax.select(self.masks[x.shape], tick if tick.shape == x.shape else jnp.tile(tick, reps), x)
        return tie


def _no_tie(x, k):
    return x


_A_TERMS = ((0, 3, 1), (2, 3, 1), (0, None, 0), (3, None, 0), (0, 1, 1), (2, 0, -1), (1, 3, -1))
_B_TERMS = ((0, 3, 1), (0, None, 0), (1, 3, -1), (2, 0, -1), (3, None, 0), (0, 1, 1), (2, 3, 1))


def _operand(term, block):
    x, y, sign = term
    if y is None:
        return block(x)
    return block(x) + block(y) if sign > 0 else block(x) - block(y)


def _operands(terms, blocks):
    return [_operand(t, blocks.__getitem__) for t in terms]


def _operands2(terms, n1, block, tie):
    first = terms[n1][0]
    sub = [_operand(terms[n1], lambda o: tie(block(o, q)) if o == first and q in (0, 3) else block(o, q))
           for q in range(4)]
    return _operands(terms, sub)


_C_TERMS = ({0: 1, 3: 1, 4: -1, 6: 1}, {2: 1, 4: 1}, {1: 1, 3: 1}, {0: 1, 1: -1, 2: 1, 5: 1})


def _combine(m, only=(0, 1, 2, 3), order=(1, 3, 2, 4, 0, 5, 6)):
    out = []
    for terms in (_C_TERMS[n] for n in only):
        seq = [n for n in order if n in terms]
        if terms[seq[0]] < 0:
            seq[0], seq[1] = seq[1], seq[0]
        acc = m[seq[0]]
        for n in seq[1:]:
            acc = acc + m[n] if terms[n] > 0 else acc - m[n]
        out.append(acc)
    return out


class _Tiles:
    def __init__(self, vals, r, n, c=0, w=None):
        self.vals, self.idx, self.cache = vals, (slice(r, r + n), slice(c, None if w is None else c + w)), {}

    def __getitem__(self, i):
        if i not in self.cache:
            self.cache[i] = self.vals[i][self.idx]
        return self.cache[i]


class _Reducer:
    def __init__(self, red, comb):
        self.red, self.comb, self.acc, self.rows, self.out = red, comb, None, 0, None

    def add(self, v):
        self.rows += 8 * v.shape[0]
        v = self.red(v, axis=0)
        self.acc = v if self.acc is None else self.comb(self.acc, v)
        if self.rows >= RCH:
            self.result()

    def result(self):
        if self.acc is not None:
            v = self.red(self.acc, axis=0, keepdims=True)
            self.out = v if self.out is None else self.comb(self.out, v)
        self.acc, self.rows = None, 0
        return self.out


def _cmul(ar, ai, br, bi):
    return ar * br - ai * bi, ar * bi + ai * br


def _hi16(w):
    return pltpu.bitcast(w & jnp.uint32(0xFFFF0000), f32)


def _stage(raw, stg, c0, nc, tie, groups=(0, 1)):
    for ht in groups:
        for dt in range(2):
            v = raw[c0:c0 + nc, ht * 8:(ht + 1) * 8, dt * T:(dt + 1) * T].reshape(nc * 8, T)
            stg[ht * 2 + dt, c0 * 4:(c0 + nc) * 4, :] = tie(pltpu.bitcast(v, u32))


def _ssm_params(vec_s, coef_s, lam_s, col_s):
    row = lambda r: r[...].astype(f32).reshape(1, M)
    lre, lim, ldt, dsk, gw = [row(v) for v in vec_s]
    dt = jnp.exp(ldt).astype(bf16).astype(f32)
    mag = jnp.exp(dt * lre)
    ang = dt * lim
    lr, li = mag * jnp.cos(ang), mag * jnp.sin(ang)
    den = lre * lre + lim * lim
    nr = lr - 1.0
    coef_s[...] = jnp.zeros(coef_s.shape, f32)
    coef_s[0:1, 0:M] = 2.0 * ((nr * lre + li * lim) / den)
    coef_s[1:2, 0:M] = 2.0 * ((li * lre - nr * lim) / den)

    er = jnp.concatenate([lr, lr[:, PA:]], axis=1)
    ei = jnp.concatenate([li, -li[:, PA:]], axis=1)
    pw = [(er, ei)]
    for _ in range(7):
        pw.append(_cmul(pw[-1][0], pw[-1][1], er, ei))
    sub = lax.broadcasted_iota(jnp.int32, (8, 512), 0)
    for n, d in enumerate((1, 2, 4)):
        lam_s[2 * n] = jnp.where(sub >= d, pw[d - 1][0], 0.0)
        lam_s[2 * n + 1] = jnp.where(sub >= d, pw[d - 1][1], 0.0)
    lcr = jnp.zeros((8, 512), f32)
    lci = jnp.zeros((8, 512), f32)
    for r in range(8):
        lcr = jnp.where(sub == r, pw[r][0], lcr)
        lci = jnp.where(sub == r, pw[r][1], lci)
    lam_s[6] = lcr
    lam_s[7] = lci

    def col(v):
        v = jnp.concatenate([v, jnp.zeros((1, 512 - M), f32)], axis=1)
        return jnp.broadcast_to(v, (T, 512)).T[:M]
    col_s[0] = col(dsk)
    col_s[1] = col(gw)


def _ssm_cmat(craw_s, coef_s, c_s, tie):
    for r in range(0, M, 16):
        coef = tie(coef_s[...], r // 16)
        cr, ci = coef[0:1, :M], coef[1:2, :M]
        re, im = _cmul(craw_s[0, r:r + 16, :].astype(f32), craw_s[1, r:r + 16, :].astype(f32), cr, ci)
        _put(c_s, r, 0, [re[:, :PA], -im[:, :PA], re[:, PA:], -im[:, PA:]])


def _ssm_scan(u_ref, carry, lam_s, h_s, tie):
    car, cai = carry
    out = []
    for b in range(TC // 8):
        mixed = u_ref[3, b, :, 0:T]
        u = jnp.concatenate([u_ref[cb, b] for cb in range(3)], axis=1)
        cols = [u[:, 0:T], u[:, T:2 * T], u[:, 2 * T:PA], mixed]
        hr = jnp.concatenate([tie(v, 4 * b + n) for n, v in enumerate(cols)], axis=1)
        hi = jnp.concatenate([u[:, PA:2 * PA], pltpu.roll(mixed, PB, 1)], axis=1)
        for n, d in enumerate((1, 2, 4)):
            sr, si = pltpu.roll(hr, d, 0), pltpu.roll(hi, d, 0)
            tr, ti = _cmul(sr, si, lam_s[2 * n], lam_s[2 * n + 1])
            hr, hi = hr + tr, hi + ti
        tr, ti = _cmul(lam_s[6], lam_s[7], car, cai)
        hr, hi = hr + tr, hi + ti
        car, cai = hr[7:8, :], hi[7:8, :]
        out.append(jnp.concatenate([hr[:, :PA], hi[:, :PA], hr[:, PA:]], axis=1))
        if b % 2 == 1:
            _put(h_s, (b - 1) * 8, 0, [jnp.concatenate(out, axis=0)])
            out = []
    return car, cai


_vmem = pltpu.VMEM
_PROLOGUE_SCRATCH = dict(
    xT_s=_vmem((M, S), bf16),
    v0=_vmem((M,), bf16), v1=_vmem((M,), bf16), v2=_vmem((M,), bf16), v3=_vmem((M,), bf16), v4=_vmem((M,), bf16),
    b_s=_vmem((2 * M, M), bf16),
    craw_s=_vmem((2, M, M), bf16),
    c_s=_vmem((M // 2, 2 * M), u32),
    coef_s=_vmem((8, 512), f32),
    lam_s=_vmem((8, 8, 512), f32),
    col_s=_vmem((2, M, T), f32),
    h_s=_vmem((TC // 2, 2 * M), u32),
    ckv_s=_vmem((4, 4, 2, T // 2, DC), bf16),
    rq=_vmem((M, H, D), bf16),
    rk=_vmem((NRAW * CS, H, D), bf16),
    rv=_vmem((NRAW * CS, H, D), bf16),
    sq=_vmem((4, M * 4, T), u32),
    sk=_vmem((4, CS * 4, T), u32),
    sv=_vmem((4, CS * 4, T), u32),
    xa_s=_vmem((HM // 2, NP * 7 * T), u32),
)
_HEAD_SCRATCH = dict(
    mk_s=_vmem((7 * HD, 2 * T), f32),
    mv_s=_vmem((7 * HD, 2 * T), f32),
    mp_s=_vmem((7 * HD, 2 * T), f32),
    kt_s=_vmem((2 * T, 4 * T), f32),
    ka_s=_vmem((S // 4, 9 * T), u32),
    va_s=_vmem((HD // 2, NP * 9 * T), u32),
    v2_s=_vmem((QD // 2, 3 * 49 * T), u32),
    s_s=_vmem((4, S // 8, 8, 2 * T), f32),
    pb_s=_vmem((2 * T, 7 * T), u32),
    pd_s=_vmem((S // 2, 2 * T), u32),
    p2_s=_vmem((3 * T, 49 * T), u32),
    sc_s=_vmem((1, S), f32),
    qb_s=_vmem((HD // 2, 14 * T), u32),
)
_SHARED_SCRATCH = [
    _vmem((H // 2 * D, DC), u32),
    _vmem((H // 2 * D, DC), u32),
    _vmem((S // 8, 49 * QC), u32),
    _vmem((H * D, S // 2), u32),
    _vmem((H, M, D), bf16),
    _vmem((QD, 49 * QC), u32),
    _vmem((HM // 2, 7 * T), u32),
    _vmem((HD // 2, NP * 7 * T), u32),
    _vmem((M, S), f32),
    _vmem((1, S), f32),
    _vmem((8, T), f32),
    pltpu.SemaphoreType.DMA((NSEM,)),
]


def _kernel(xT_hbm, bre_hbm, bim_hbm, cre_hbm, cim_hbm, lre_hbm, lim_hbm, ldt_hbm,
            dsk_hbm, gw_hbm, woT_hbm, ckv_hbm, wq_hbm, wk_hbm, wv_hbm,
            out_hbm,
            wkt_s, wvt_s, a_s, q_s, wo_s, w_s, wl_s, cl_s, o_s, g_s, zero_s, sem, *rest):
    h = pl.program_id(0)
    pro_refs = dict(zip(_PROLOGUE_SCRATCH, rest))
    head_refs = dict(zip(_HEAD_SCRATCH, rest[len(pro_refs):]))

    def out_copy(jp):
        cols = pl.ds(jp * 2 * T, 2 * T)
        return pltpu.make_async_copy(o_s.at[:, cols], out_hbm.at[:, cols], sem.at[SEM_OUT])

    def prep_w(hh, outer, tie):
        rows = _ds(lax.shift_right_logical(hh, 1) * D, D, D)
        sh = (16 * (1 - (hh & 1))).astype(u32)
        k = 0
        for row0, wt_s in ((0, wkt_s.at[rows]), (QD, wvt_s.at[rows])):
            for r in range(0, QD, 16):
                def block(o, q):
                    row = (o % 2) * HD + (q % 2) * QD + r
                    col = (o // 2) * 2 * QC + (q // 2) * QC
                    return _hi16(wt_s[row:row + 16, col:col + QC] << sh)
                for n1 in outer:
                    _put(w_s, row0 + r, 7 * n1 * QC, _operands2(_B_TERMS, n1, block, lambda x: tie(x, k)))
                    k += 1

    def prologue(xT_s, v0, v1, v2, v3, v4, b_s, craw_s, c_s, coef_s, lam_s, col_s, h_s,
                 ckv_s, rq, rk, rv, sq, sk, sv, xa_s):
        u_s = head_refs['s_s']
        vec_s = (v0, v1, v2, v3, v4)

        def slice_copies(i):
            s = sem.at[SEM_SL + i]
            grp = i // 2 if isinstance(i, int) else lax.shift_right_logical(i, 1)
            cs, dst = pl.ds(i * CS, CS), pl.ds((i & (NRAW - 1)) * CS, CS)
            return [pltpu.make_async_copy(ckv_hbm.at[grp, :, i & 1], ckv_s.at[grp, :, i & 1], s),
                    pltpu.make_async_copy(wk_hbm.at[cs], rk.at[dst], s),
                    pltpu.make_async_copy(wv_hbm.at[cs], rv.at[dst], s)]

        def wq1_copy(i):
            rows = pl.ds(i * (M // 4), M // 4)
            return pltpu.make_async_copy(wq_hbm.at[rows, 8:16], rq.at[rows, 8:16], sem.at[SEM_WQ1 + i])

        def x_copy(i):
            cols = pl.ds(i * TA, TA)
            return pltpu.make_async_copy(xT_hbm.at[:, cols], xT_s.at[:, cols], sem.at[SEM_X + i])

        cp_vec = [pltpu.make_async_copy(src, dst, sem.at[SEM_VEC])
                  for src, dst in zip((lre_hbm, lim_hbm, ldt_hbm, dsk_hbm, gw_hbm), vec_s)]
        cp_b = [pltpu.make_async_copy(src.at[pl.ds(lo, n)], b_s.at[pl.ds(dst, n)], sem.at[SEM_B])
                for src, lo, n, dst in ((bre_hbm, 0, PA, 0), (bim_hbm, 0, PA, PA),
                                        (bre_hbm, PA, PB, 2 * PA), (bim_hbm, PA, PB, 2 * PA + PB))]
        cp_wq = [pltpu.make_async_copy(wq_hbm.at[:, 0:8], rq.at[:, 0:8], sem.at[SEM_WQ])]
        cp_c = [pltpu.make_async_copy(src, craw_s.at[n], sem.at[SEM_C])
                for n, src in enumerate((cre_hbm, cim_hbm))]
        cp_wo = pltpu.make_async_copy(woT_hbm, wo_s, sem.at[SEM_WO])
        for cp in cp_vec + cp_b + [x_copy(i) for i in range(S // TA)] + cp_c + cp_wq:
            cp.start()
        for i in range(NRAW - 1):
            for cp in [wq1_copy(i)] + slice_copies(i):
                cp.start()
        wq1_copy(3).start()
        cp_wo.start()

        zero_s[...] = jnp.zeros(zero_s.shape, f32)
        wl_s[...] = jnp.zeros(wl_s.shape, u32)
        cl_s[:, (NP - 1) * 7 * T:] = jnp.zeros((HD // 2, 7 * T), u32)
        for cp in cp_vec:
            cp.wait()
        _ssm_params(vec_s, coef_s, lam_s, col_s)

        def phase1(i):
            clk = _Clock(zero_s)
            u, _ = clk.dot(xT_s[:, i * TA:(i + 1) * TA], b_s[...], _TT)
            for cb in range(4):
                w = min(2 * T, 2 * M - cb * 2 * T)
                u_s[cb, i * TA // 8:(i + 1) * TA // 8, :, 0:w] = (
                    u[:, cb * 2 * T:cb * 2 * T + w].reshape(TA // 8, 8, w))
            tie = clk.pacer(0, 6 * TA, 14)
            for t in range(2 * i, 2 * i + 2):
                for r in range(0, HM, 32):
                    k = (t % 2) * 7 + r // 32
                    top = xT_s[r:r + 32, 2 * t * T:(2 * t + 2) * T].astype(f32)
                    bot = xT_s[HM + r:HM + r + 32, 2 * t * T:(2 * t + 2) * T].astype(f32)
                    blocks = [tie(top[:, :T], k), bot[:, :T], top[:, T:], tie(bot[:, T:], k)]
                    _put(xa_s, r, t * 7 * T, _operands(_A_TERMS, blocks))
            return clk

        for cp in cp_b + [x_copy(0)]:
            cp.wait()
        phase1(0)
        x_copy(1).wait()
        clk = phase1(1)
        zero = jnp.zeros((1, 512), f32)
        carry0 = _ssm_scan(u_s.at[:, 0:TC // 8], (zero, zero), lam_s, h_s, clk.pacer(0, 6 * TA, TC // 2))
        for cp in [x_copy(2), x_copy(3)] + cp_c + cp_wq:
            cp.wait()
        _ssm_cmat(craw_s, coef_s, c_s, phase1(2).pacer(0, 6 * TA, M // 16))
        tie = phase1(3).pacer(0, 6 * TA, M // 8)
        for c0 in range(0, M, 8):
            _stage(rq, sq, c0, 8, lambda x: tie(x, c0 // 8), groups=(0,))

        def phase2(i, carry):
            @pl.when(i + NRAW - 1 < NP)
            def _():
                for cp in slice_copies(i + NRAW - 1):
                    cp.start()

            @pl.when(i < 4)
            def _():
                wq1_copy(i).wait()

            for cp in slice_copies(i):
                cp.wait()

            yT = _dot(_get(c_s, 0, M, 0, 2 * M), _get(h_s, 0, TC, 0, 2 * M), _NT)
            for t in range(TC // T):
                cols = _ds(i * TC + t * T, T, T)
                acc = jnp.zeros((8, T), f32)
                for r in range(0, M, 32):
                    xg = xT_s[r:r + 32, cols].astype(f32) * col_s[1, r:r + 32, :]
                    acc = acc + jnp.sum(xg.reshape(4, 8, T), axis=0)
                g = jax.nn.sigmoid(jnp.sum(acc, axis=0, keepdims=True))
                g_s[:, cols] = g
                for r in range(0, M, 32):
                    skip = xT_s[r:r + 32, cols].astype(f32) * col_s[0, r:r + 32, :]
                    o_s[r:r + 32, cols] = (1.0 - g) * (yT[r:r + 32, t * T:(t + 1) * T] + skip)

            ht = lax.shift_right_logical(i, 2)
            words = [sq[ht * 2 + dt, pl.ds(i & 3, M, stride=4), :] for dt in range(2)]
            both = [jnp.concatenate([pltpu.bitcast(w << 16, f32), _hi16(w)], axis=1) for w in words]
            wq = _operands(_B_TERMS, [both[0][:HM], both[1][:HM], both[0][HM:], both[1][HM:]])
            clk = _Clock(zero_s)
            m = [clk.dot(wq[n].astype(bf16),
                         _cat([_get(xa_s, 0, HM, (t * 7 + n) * T, T) for t in range(NP)], 1), _TN)[0]
                 for n in range(7)]
            q_i = q_s.at[_ds(i * 2 * D, 2 * D, 2 * D)]
            for n in (2, 1, 3, 0):
                for t in range(NP):
                    for r in range(0, D, GC):
                        c, = _combine(_Tiles(m, r, GC, t * T, T), (n,), range(7))
                        row = (2 * (r // HD) + n // 2) * D + (n % 2) * HD + r % HD
                        _put(q_i, row, t * T, [c * (LOG2E * D ** -0.5)])

            span = 5 * 1024

            u_next = u_s.at[:, pl.ds(jnp.minimum(i + 1, NP - 1) * (TC // 8), TC // 8)]
            carry = _ssm_scan(u_next, carry, lam_s, h_s, clk.pacer(0, span, TC // 2))

            tie = clk.pacer(0, span, 64)
            rq_i = rq.at[pl.ds((i & 3) * (M // 4), M // 4)]
            sq_i = sq.at[:, _ds((i & 3) * M, M, 8)]
            for c0 in range(0, M // 4, 8):
                _stage(rq_i, sq_i, c0, 8, lambda x: tie(x, c0 // 2 + 2), groups=(1,))
            slot = pl.ds((i & (NRAW - 1)) * CS, CS)
            for n, (raw, stg, wt_s) in enumerate(((rk, sk, wkt_s), (rv, sv, wvt_s))):
                for c0 in range(0, CS, 8):
                    _stage(raw.at[slot], stg, c0, 8, lambda x: tie(x, 16 * n + c0 // 8))
                cols = _ds(i * CS, CS, CS)
                for pair in range(H // 2):
                    for dt in range(2):
                        blk = stg[(pair // 4) * 2 + dt, pl.ds(pair % 4, CS, stride=4), :]
                        row = pair * D + dt * HD
                        wt_s[row:row + HD, cols] = tie(blk, 16 + 24 * n + 3 * pair + dt).T

            tie = clk.pacer(0, span, 28)
            ckv_i = ckv_s.at[lax.shift_right_logical(i, 1), :, i & 1]
            a_i = a_s.at[_ds(i * (T // 4), T // 4, T // 4)]
            for r in range(0, T // 2, 16):
                def block(o, q):
                    col = (o % 2) * 2 * QC + (q % 2) * QC
                    return ckv_i[2 * (q // 2) + o // 2, r:r + 16, col:col + QC].astype(f32)
                for n1 in range(7):
                    ops = _operands2(_A_TERMS, n1, block, lambda x: tie(x, 7 * (r // 16) + n1))
                    _put(a_i, r, 7 * n1 * QC, ops)
            return carry

        lax.fori_loop(0, NP, phase2, carry0)
        cp_wo.wait()
        prep_w(h, range(NT1), _no_tie)

    @pl.when(h == 0)
    def _():
        prologue(**pro_refs)

    def oproj(jp, clk):
        cols = slice(2 * jp * T, (2 * jp + 2) * T)
        for r, n in OCH:
            c = clk.strassen(lambda i: _get(wl_s, r, n, i * T, T),
                             lambda i: _get(cl_s, 0, HD, (jp * 7 + i) * T, T), _NN)()
            o_s[r:r + n, cols] += jnp.concatenate(c[:2], axis=1)
            o_s[HM + r:HM + r + n, cols] += jnp.concatenate(c[2:], axis=1)

    def head(mk_s, mv_s, mp_s, kt_s, ka_s, va_s, v2_s, s_s, pb_s, pd_s, p2_s, sc_s, qb_s):
        clk = _Clock(zero_s)
        q_h = q_s.at[_ds(h * D, D, D)]

        def prep_wo(tie):
            for r in range(0, HM, 16):
                top = tie(wo_s[h, r:r + 16, :].astype(f32), r // 16)
                bot = tie(wo_s[h, HM + r:HM + r + 16, :].astype(f32), r // 16)
                _put(wl_s, r, 0, _operands(_A_TERMS, [top[:, :HD], top[:, HD:], bot[:, :HD], bot[:, HD:]]))

        def outer(m_s, r):
            return _combine([m_s[n * HD + r:n * HD + r + 16, :] for n in range(7)], order=range(7))

        def proj(g, lo, hi):
            for n1 in range(lo, hi):
                comb = clk.strassen(lambda n: _get(w_s, 0, 2 * QD, (7 * n1 + n) * QC, QC),
                                    lambda n: _get(a_s, g * T, T, (7 * n1 + n) * QC, QC), _NT, n1 == 6)
                for r in range(0, 2 * QD, GC):
                    m_s, row = mk_s if r < QD else mv_s, n1 * HD + r % QD
                    c = comb(r, GC)
                    m_s[row:row + GC, :] = jnp.concatenate([c[0], c[2]], axis=1)
                    m_s[QD + row:QD + row + GC, :] = jnp.concatenate([c[1], c[3]], axis=1)
            if hi < 7:
                return
            nine = lambda c: _operands(_A_TERMS, c) + [c[1], c[2]]
            cs = [outer(mk_s, r) for r in range(0, HD, 16)]
            for n in range(4):
                kt_s[:, n * T:(n + 1) * T] = jnp.concatenate([c[n] for c in cs], axis=0).T
            for r in range(0, 2 * T, GC):
                blk = kt_s[r:r + GC, :]
                _put(ka_s, 2 * g * T + r, 0, nine([blk[:, n * T:(n + 1) * T] for n in range(4)]))
            for r in range(0, QD, 16):
                ops = []
                for row in (r, QD + r):
                    c = outer(mv_s, row)
                    ops.append(nine([c[0], c[2], c[1], c[3]]))
                    _put(va_s, row, 2 * g * 9 * T, [o[:, :T] for o in ops[-1]])
                    for n in (2, 7):
                        _put(va_s, row, ((2 * g + 1) * 9 + n) * T, [o[:, T:] for o in ops[-1][n:n + 2]])
                if g < 3:
                    for n1 in range(7):
                        lo_, hi_ = ops[0][n1], ops[1][n1]
                        _put(v2_s, r, (g * 7 + n1) * 7 * T,
                             _operands(_A_TERMS, [lo_[:, :T], lo_[:, T:], hi_[:, :T], hi_[:, T:]]))

        key = lax.broadcasted_iota(jnp.int32, (T, 2 * T), 0)
        qry = lax.broadcasted_iota(jnp.int32, (T, 2 * T), 1)
        causal = key <= qry

        def qk(g):
            pairs = (2 * g, 2 * g + 1)
            mx = {jp: _Reducer(jnp.max, jnp.maximum) for jp in pairs}

            def put(jp, row, v):
                v = v.reshape(v.shape[0] // 8, 8, 2 * T)
                s_s[jp % 4, row // 8:row // 8 + v.shape[0]] = v
                mx[jp].add(v)

            def rect(jp, lo, hi, n):
                for r in range(lo, hi, n):
                    c = clk.strassen(lambda i: _get(ka_s, r, n, i * T, T),
                                     lambda i: _get(qb_s, 0, HD, ((jp % 2) * 7 + i) * T, T), _NN)()
                    put(jp, r, jnp.concatenate(c[:2], axis=1))
                    put(jp, jp * T + r, jnp.concatenate(c[2:], axis=1))

            q = lambda jp, e: _get(q_h, e * D, D, jp * T, T)
            for jp in pairs[g == 0:]:
                for r in range(0, HD, 32):
                    blk = [_get(q_h, e * D + d * HD + r, 32, jp * T, T).astype(f32) for d in range(2) for e in range(2)]
                    _put(qb_s, r, (jp % 2) * 7 * T, _operands(_B_TERMS, blk))
            for jp in pairs:
                rect(jp, 0, 2 * g * T, QCH if QCH else g * T // 2 or 1)
            kb = lambda jp, a, b: jnp.concatenate(
                [_get(ka_s, jp * T, T, a * T, T), _get(ka_s, jp * T, T, b * T, T)], axis=1)
            for jp in pairs:
                se, _ = clk.dot(kb(jp, 2, 7), jnp.concatenate([q(jp, 0), q(jp, 1)], axis=1), _NN)
                put(jp, 2 * jp * T, jnp.where(causal, se, NEG))
            last = {}
            for jp in pairs:
                so = jnp.where(causal[:, :T], clk.dot(kb(jp, 8, 3), q(jp, 1), _NN)[0], NEG)
                row = (2 * jp + 1) * T // 8
                s_s[jp % 4, row:row + T // 8, :, T:] = so.reshape(T // 8, 8, T)
                last[jp] = jnp.concatenate([jnp.full((1, T), NEG, f32), jnp.max(so, axis=0, keepdims=True)], axis=1)
            rect(2 * g + 1, 2 * g * T, (2 * g + 1) * T, T // 4)
            return [jnp.broadcast_to(jnp.maximum(mx[jp].result(), last[jp]), (8, 2 * T)) for jp in pairs]

        zs, sums = {}, {}

        def prob(jp, row, z, n=GS, lanes=slice(None)):
            return jnp.exp2(s_s[jp % 4, row // 8:(row + n) // 8, :, lanes] - z[:, lanes])

        def rough(jp, mx, tie):
            zs[jp] = mx
            if jp > 0:
                sm = _Reducer(jnp.sum, jnp.add)
                for k, r in enumerate(range(0, 2 * jp * T, GS * LSUB)):
                    sm.add(prob(jp, r, tie(mx, k)))
                zs[jp] = mx + jnp.log2(jnp.maximum(LSUB * sm.result(), 1.0))
            sums[jp] = _Reducer(jnp.sum, jnp.add)

        def blocks(jp, row, tie, k):
            top, bot = prob(jp, row, tie(zs[jp], k)), prob(jp, jp * T + row, tie(zs[jp], k + 1))
            sums[jp].add(top + bot)
            top, bot = top.reshape(GS, 2 * T), bot.reshape(GS, 2 * T)
            return [top[:, :T], top[:, T:], bot[:, :T], bot[:, T:]]

        def near(jp, tie, k):
            R, z = jp * T, zs[jp]
            if jp % 2:
                for r in range(0, T, GS):
                    _put(pb_s, jp // 2 * T + r, 0, _operands(_B_TERMS, blocks(jp, R - T + r, tie, k)))
                    k += 2
            for r in range(0, T, GS):
                p = prob(jp, 2 * R + r, tie(z, k))
                sums[jp].add(p)
                _put(pd_s, 2 * R + r, 0, [p.reshape(GS, 2 * T)])
                k += 1
            so = _Reducer(jnp.sum, jnp.add)
            for r in range(0, T, 2 * GS):
                p = prob(jp, 2 * R + T + r, tie(z, k), 2 * GS, slice(T, 2 * T))
                so.add(p)
                _put(pd_s, 2 * R + T + r, T, [p.reshape(2 * GS, T)])
                k += 1
            sums[jp].result()
            sums[jp].out = sums[jp].out + jnp.concatenate([jnp.zeros((1, T), f32), so.result()], axis=1)

        p20 = lambda g: g * (g - 1) // 2 * T

        def far(g, tie, k):
            half = {(jp, e): _Reducer(jnp.sum, jnp.add) for jp in (2 * g, 2 * g + 1) for e in range(2)}
            for kg in range(g):
                for r in range(0, T, GS):
                    blk = {}
                    for new, n1 in (((0,), 1), ((1,), 5), ((3,), 2), ((), 0), ((), 4), ((2,), 3), ((), 6)):
                        for o in new:
                            lanes = slice((o % 2) * T, (o % 2 + 1) * T)
                            for jp in (2 * g, 2 * g + 1):
                                z = tie(zs[jp][:, lanes], k)
                                row = (o // 2) * jp * T + 2 * kg * T + r
                                p = [jnp.exp2(s_s[jp % 4, x // 8:(x + GS) // 8, :, lanes] - z) for x in (row, row + T)]
                                half[jp, o % 2].add(p[0] + p[1])
                                blk[o, jp % 2], blk[o, 2 + jp % 2] = [x.reshape(GS, T) for x in p]
                        ops = _operands2(_B_TERMS, n1, lambda o, q: blk[o, q], lambda x: x)
                        _put(p2_s, p20(g) + kg * T + r, 7 * n1 * T, ops,
                             (lambda w: tie(w, k, True, FLAG)) if FTIE else None)
                        k += FW * 8 / 7
            for jp in (2 * g, 2 * g + 1):
                if g:
                    sums[jp].out = sums[jp].out + jnp.concatenate([half[jp, e].result() for e in range(2)], axis=1)
            for jp in (2 * g, 2 * g + 1):
                cols = slice(2 * jp * T, 2 * (jp + 1) * T)
                sc_s[:, cols] = g_s[:, cols] / sums[jp].result()

        def pv(g):
            pairs = (2 * g, 2 * g + 1)
            va = lambda n, t, r=0, nr=HD: _get(va_s, r, nr, (t * 9 + n) * T, T)
            for n1 in range(7 if g else 0):
                c = clk.strassen(
                    lambda n: _cat([_get(v2_s, 0, QD, (kg * 49 + 7 * n1 + n) * T, T) for kg in range(g)], 1),
                    lambda n: _get(p2_s, p20(g), g * T, (7 * n1 + n) * T, T), _NN)()
                mp_s[n1 * HD:n1 * HD + QD, :] = jnp.concatenate(c[:2], axis=1)
                mp_s[n1 * HD + QD:(n1 + 1) * HD, :] = jnp.concatenate(c[2:], axis=1)
            ve = [jnp.concatenate([va(2, jp), va(8, jp)], axis=0) for jp in pairs]
            vo = [jnp.concatenate([va(7, jp), va(3, jp)], axis=0) for jp in pairs]
            ce = clk.level([(ve[jp % 2], _get(pd_s, 2 * jp * T, T, 0, T)) for jp in pairs])
            co = [clk.dot(jnp.concatenate([ve[jp % 2], vo[jp % 2]], axis=1),
                          _get(pd_s, 2 * jp * T, 2 * T, T, T), _NN)[0] for jp in pairs]
            for jp in pairs:
                R, e = jp * T, jp % 2
                ge, go = sc_s[:, 2 * R:2 * R + T], sc_s[:, 2 * R + T:2 * R + 2 * T]
                for r in range(0, HD, 32):
                    c = [ce[e][r:r + 32], co[e][r:r + 32], ce[e][HD + r:HD + r + 32], co[e][HD + r:HD + r + 32]]
                    if g:
                        far_ = _combine([mp_s[n * HD + r:n * HD + r + 32, e * T:(e + 1) * T] for n in range(7)],
                                        order=range(7))
                        c = [x + y for x, y in zip(c, far_)]
                    if e:
                        near_ = clk.strassen(lambda n: va(n, 2 * g, r, 32),
                                             lambda n: _get(pb_s, g * T, T, n * T, T), _NN)()
                        c = [x + y for x, y in zip(c, near_)]
                    ops = _operands(_B_TERMS, [c[0] * ge, c[1] * go, c[2] * ge, c[3] * go])
                    _put(cl_s, r, jp * 7 * T, ops)

        def run(items):
            for item in items.split():
                if item[0] == 'P':
                    pv(int(item[1]))
                elif item[0] == 'K':
                    proj(int(item[1]), int(item[2]), int(item[3]))
                else:
                    jp = int(item[1])
                    oproj(jp, clk)

                    @pl.when(h == H - 1)
                    def _():
                        out_copy(jp).start()

        for n1 in range(7):
            if n1 >= NT1:
                prep_w(h, [n1], clk.pacer(max(clk.t - LEAD - 448, 1), max(clk.t - LEAD, 1), 8))
            proj(0, n1, n1 + 1)
        oproj(NP - 1, clk)
        mx = qk(0)
        for g in range(4):
            t0 = clk.t
            run(PLAN[g])
            t1 = clk.t
            nxt = qk(g + 1) if g < 3 else None
            n_rough = [2 * jp * T // (GS * LSUB) for jp in (2 * g, 2 * g + 1)]
            n_near = [(T + T // 2) // GS, (3 * T + T // 2) // GS]
            hole = (t1 - HOLE0, t1 + HOLE1) if 0 < g < 3 else None
            tie = clk.pacer(t0 + D0, (clk.t if g else t1) - SLACK,
                            sum(n_rough) + sum(n_near) + FW * g * 8 * T // GS, hole)
            rough(2 * g, mx[0], tie)
            near(2 * g, tie, n_rough[0])
            k = n_rough[0] + n_near[0]
            rough(2 * g + 1, mx[1], lambda x, i: tie(x, k + i))
            near(2 * g + 1, tie, k + n_rough[1])
            far(g, tie, k + n_rough[1] + n_near[1])
            if g == 0:
                prep_wo(clk.pacer(t0, t1, HM // 16))
            mx = nxt
        t0 = clk.t
        run(PLAN[4])
        prep_w(jnp.minimum(h + 1, H - 1), range(NT1), clk.pacer(t0 - PW0, clk.t - 300, 8 * NT1))
        if os.environ.get('SHOW'):
            print('final loads', clk.load)

    head(**head_refs)

    @pl.when(h == H - 1)
    def _():
        oproj(NP - 1, _Clock(zero_s))
        out_copy(NP - 1).start()
        for jp in range(NP):
            out_copy(jp).wait()


@jax.jit
def pallas_gated_mix__compressed_kv_cla__ssm_conv_s5__prompt_kernel(
    A_x: jax.Array,
    A_c_kv: jax.Array,
    A_w_q: jax.Array,
    A_w_uk: jax.Array,
    A_w_uv: jax.Array,
    A_w_o: jax.Array,
    B_x: jax.Array,
    B_Lambda_re: jax.Array,
    B_Lambda_im: jax.Array,
    B_B_re: jax.Array,
    B_B_im: jax.Array,
    B_C_re: jax.Array,
    B_C_im: jax.Array,
    B_log_dt: jax.Array,
    B_Dskip: jax.Array,
    gate_w: jax.Array,
):
    del B_x
    xT = jnp.transpose(A_x[0])
    woT = jnp.transpose(A_w_o, (0, 2, 1))
    ckv = A_c_kv.reshape(4, 4, 2, T // 2, DC)

    hbm = pl.BlockSpec(memory_space=pl.ANY)
    outT = pl.pallas_call(
        _kernel,
        grid=(H,),
        in_specs=[hbm] * 15,
        out_specs=hbm,
        out_shape=jax.ShapeDtypeStruct((M, S), f32),
        scratch_shapes=_SHARED_SCRATCH + list(_PROLOGUE_SCRATCH.values()) + list(_HEAD_SCRATCH.values()),
        compiler_params=pltpu.CompilerParams(
            dimension_semantics=("arbitrary",),
            vmem_limit_bytes=126 * 1024 * 1024,
        ),
    )(xT, B_B_re, B_B_im, B_C_re, B_C_im, B_Lambda_re, B_Lambda_im, B_log_dt,
      B_Dskip, gate_w, woT, ckv, A_w_q, A_w_uk, A_w_uv)
    return jnp.transpose(outT)[None]
```

```python
import bisect
import os

import jax
import jax.numpy as jnp
from jax import lax
import jax.experimental.pallas as pl
import jax.experimental.pallas.tpu as pltpu

S = 2048
M = 448
H = 16
D = 256
DC = 1024
T = 128
NP = S // T // 2
HD = D // 2
HM = M // 2
QD = D // 4
QC = DC // 4
PA = 384
PB = M - PA
TA = 512
TC = 256
CS = DC // NP
NRAW = 4
LOG2E = 1.4426950408889634
NEG = -1e30

_env = lambda k, d: type(d)(os.environ.get(k, d))
GC = _env('GC', 64)
GS = _env('GS', 16)
RCH = _env('RCH', 256)
SLACK = _env('SLACK', 200)
D0 = _env('D0', 0)
NT1 = _env('NT1', 3)
LEAD = _env('LEAD', 448)
PW0 = _env('PW0', 100)
FTIE = _env('FTIE', 1)
FLAG = _env('FLAG', 40)
FW = _env('FW', 2)
HOLE0 = _env('HOLE0', 400)
HOLE1 = _env('HOLE1', 400)
VW = _env('VW', 900)
PH0 = _env('PH0', 500)
PH1 = _env('PH1', 100)
QCH = _env('QCH', 64)
OCH = ((0, 64), (64, 64), (128, 48), (176, 48))
LSUB = _env('LSUB', 4)
PLAN = _env('PLAN', 'K107,K207,K307,P0 P1 O0 O1 P2 O2 O3 O4,P3 O5 O6').split(',')

f32 = jnp.float32
bf16 = jnp.bfloat16
u32 = jnp.uint32

SEM_VEC, SEM_B, SEM_X, SEM_WQ, SEM_C, SEM_SL, SEM_WO, SEM_OUT, SEM_WQ1 = 0, 1, 2, 6, 7, 8, 16, 17, 18
NSEM = 22

_NN = ((1,), (0,))
_NT = ((1,), (1,))
_TN = ((0,), (0,))
_TT = ((0,), (1,))


def _dot(a, b, dims):
    return lax.dot_general(a, b, (dims, ((), ())), preferred_element_type=f32)


def _cat(xs, axis):
    return xs[0] if len(xs) == 1 else jnp.concatenate(xs, axis=axis)


def _ds(lo, n, align):
    return pl.ds(lo if isinstance(lo, int) else pl.multiple_of(lo, align), n)


def _put(ref, row, col, xs, tie=None):
    x = _cat(xs, 1)
    if tie is not None:
        x = jnp.concatenate([tie(x[:8]), x[8:]], axis=0)
    ref[row // 2:(row + x.shape[0]) // 2, col:col + x.shape[1]] = pltpu.bitcast(x.astype(bf16), u32)


def _get(ref, row, nrows, col, ncols):
    return pltpu.bitcast(ref[row // 2:(row + nrows) // 2, col:col + ncols], bf16)


class _Clock:
    def __init__(self, zero_ref):
        self.masks = {(8, T): zero_ref[...] != 0.0}
        self.ticks, self.load = [], [0, 0, 0, 0]

    @property
    def t(self):
        return max(self.load)

    def dot(self, a, b, dims):
        v = _dot(a, b, dims)
        rows, depth = v.shape[0], a.shape[dims[0][0]]
        for c in range(0, v.shape[1], T):
            start = 0
            for _ in range(0, depth, T):
                k = self.load.index(min(self.load))
                start = max(start, self.load[k])
                self.load[k] += rows
            self.ticks += [(start + r + 8, (v, r, c)) for r in range(0, rows, 8)]
        return v, start

    def strassen(self, lhs, rhs, dims, split_last=False):
        jobs = -(-lhs(0).shape[dims[0][0]] // T)
        lag = sum(l + 32 <= max(self.load) for l in self.load) // jobs if jobs < 3 else 0
        order = ((1, 3, 2, 4, 0, 5, 6), (0, 1, 3, 2, 4, 5, 6), (5, 6, 1, 3, 2, 4, 0), (0, 5, 6, 1, 3, 2, 4))[lag]
        m = {}
        for n in order:
            if split_last and n == order[-1]:
                a, half = lhs(n), lhs(0).shape[0] // 2
                m[n] = jnp.concatenate([self.dot(a[:half], rhs(n), dims)[0], self.dot(a[half:], rhs(n), dims)[0]], 0)
            else:
                m[n] = self.dot(lhs(n), rhs(n), dims)[0]
        vals = [m[n] for n in range(7)]
        return lambda r=0, n=None, only=(0, 1, 2, 3), c=0, w=None: _combine(
            vals if n is None else _Tiles(vals, r, n, c, w), only, order)

    def level(self, pairs):
        target = -(-(sum(self.load) + sum(a.shape[0] for a, _ in pairs)) // 64) * 16
        out = []
        for a, b in pairs:
            r, parts = 0, []
            while r < a.shape[0]:
                n = min(target - min(self.load), a.shape[0] - r)
                parts.append(self.dot(a[r:r + n], b, _NN)[0])
                r += n
            out.append(_cat(parts, 0))
        return out

    def pacer(self, t0, t1, n, holes=()):
        holes = sorted((max(a, t0), min(b, t1)) for a, b in holes if a < t1 and b > t0)
        gap = sum(b - a for a, b in holes)
        ticks = sorted(self.ticks, key=lambda tw: tw[0])
        times = [tw[0] for tw in ticks]

        def tie(x, k, distinct=False, delay=0):
            t = t0 + (t1 - t0 - gap) * k / n
            for a, b in holes:
                t += b - a if t > a else 0
            t += delay
            past = ticks[:bisect.bisect_right(times, t)]
            if not past:
                return x
            reps = (x.shape[0] // 8, x.shape[1] // T)
            tick = _cat([v[r:r + 8, c:c + T] for _, (v, r, c) in past[-reps[1] if distinct else -1:]], 1)
            if tick.dtype != x.dtype:
                tick = pltpu.bitcast(tick, x.dtype)
            if x.shape not in self.masks:
                self.masks[x.shape] = jnp.tile(self.masks[(8, T)], reps)
            return lax.select(self.masks[x.shape], tick if tick.shape == x.shape else jnp.tile(tick, reps), x)
        return tie


def _no_tie(x, k):
    return x


_A_TERMS = ((0, 3, 1), (2, 3, 1), (0, None, 0), (3, None, 0), (0, 1, 1), (2, 0, -1), (1, 3, -1))
_B_TERMS = ((0, 3, 1), (0, None, 0), (1, 3, -1), (2, 0, -1), (3, None, 0), (0, 1, 1), (2, 3, 1))


def _operand(term, block):
    x, y, sign = term
    if y is None:
        return block(x)
    return block(x) + block(y) if sign > 0 else block(x) - block(y)


def _operands(terms, blocks):
    return [_operand(t, blocks.__getitem__) for t in terms]


def _operands2(terms, n1, block, tie):
    first = terms[n1][0]
    sub = [_operand(terms[n1], lambda o: tie(block(o, q)) if o == first and q in (0, 3) else block(o, q))
           for q in range(4)]
    return _operands(terms, sub)


_C_TERMS = ({0: 1, 3: 1, 4: -1, 6: 1}, {2: 1, 4: 1}, {1: 1, 3: 1}, {0: 1, 1: -1, 2: 1, 5: 1})


def _combine(m, only=(0, 1, 2, 3), order=(1, 3, 2, 4, 0, 5, 6)):
    out = []
    for terms in (_C_TERMS[n] for n in only):
        seq = [n for n in order if n in terms]
        if terms[seq[0]] < 0:
            seq[0], seq[1] = seq[1], seq[0]
        acc = m[seq[0]]
        for n in seq[1:]:
            acc = acc + m[n] if terms[n] > 0 else acc - m[n]
        out.append(acc)
    return out


class _Tiles:
    def __init__(self, vals, r, n, c=0, w=None):
        self.vals, self.idx, self.cache = vals, (slice(r, r + n), slice(c, None if w is None else c + w)), {}

    def __getitem__(self, i):
        if i not in self.cache:
            self.cache[i] = self.vals[i][self.idx]
        return self.cache[i]


class _Reducer:
    def __init__(self, red, comb):
        self.red, self.comb, self.acc, self.rows, self.out = red, comb, None, 0, None

    def add(self, v):
        self.rows += 8 * v.shape[0]
        v = self.red(v, axis=0)
        self.acc = v if self.acc is None else self.comb(self.acc, v)
        if self.rows >= RCH:
            self.result()

    def result(self):
        if self.acc is not None:
            v = self.red(self.acc, axis=0, keepdims=True)
            self.out = v if self.out is None else self.comb(self.out, v)
        self.acc, self.rows = None, 0
        return self.out


def _cmul(ar, ai, br, bi):
    return ar * br - ai * bi, ar * bi + ai * br


def _hi16(w):
    return pltpu.bitcast(w & jnp.uint32(0xFFFF0000), f32)


def _stage(raw, stg, c0, nc, tie, groups=(0, 1)):
    for ht in groups:
        for dt in range(2):
            v = raw[c0:c0 + nc, ht * 8:(ht + 1) * 8, dt * T:(dt + 1) * T].reshape(nc * 8, T)
            stg[ht * 2 + dt, c0 * 4:(c0 + nc) * 4, :] = tie(pltpu.bitcast(v, u32))


def _ssm_params(vec_s, coef_s, lam_s, col_s):
    row = lambda r: r[...].astype(f32).reshape(1, M)
    lre, lim, ldt, dsk, gw = [row(v) for v in vec_s]
    dt = jnp.exp(ldt).astype(bf16).astype(f32)
    mag = jnp.exp(dt * lre)
    ang = dt * lim
    lr, li = mag * jnp.cos(ang), mag * jnp.sin(ang)
    den = lre * lre + lim * lim
    nr = lr - 1.0
    coef_s[...] = jnp.zeros(coef_s.shape, f32)
    coef_s[0:1, 0:M] = 2.0 * ((nr * lre + li * lim) / den)
    coef_s[1:2, 0:M] = 2.0 * ((li * lre - nr * lim) / den)

    er = jnp.concatenate([lr, lr[:, PA:]], axis=1)
    ei = jnp.concatenate([li, -li[:, PA:]], axis=1)
    pw = [(er, ei)]
    for _ in range(7):
        pw.append(_cmul(pw[-1][0], pw[-1][1], er, ei))
    sub = lax.broadcasted_iota(jnp.int32, (8, 512), 0)
    for n, d in enumerate((1, 2, 4)):
        lam_s[2 * n] = jnp.where(sub >= d, pw[d - 1][0], 0.0)
        lam_s[2 * n + 1] = jnp.where(sub >= d, pw[d - 1][1], 0.0)
    lcr = jnp.zeros((8, 512), f32)
    lci = jnp.zeros((8, 512), f32)
    for r in range(8):
        lcr = jnp.where(sub == r, pw[r][0], lcr)
        lci = jnp.where(sub == r, pw[r][1], lci)
    lam_s[6] = lcr
    lam_s[7] = lci

    def col(v):
        v = jnp.concatenate([v, jnp.zeros((1, 512 - M), f32)], axis=1)
        return jnp.broadcast_to(v, (T, 512)).T[:M]
    col_s[0] = col(dsk)
    col_s[1] = col(gw)


def _ssm_cmat(craw_s, coef_s, c_s, tie):
    for r in range(0, M, 16):
        coef = tie(coef_s[...], r // 16)
        cr, ci = coef[0:1, :M], coef[1:2, :M]
        re, im = _cmul(craw_s[0, r:r + 16, :].astype(f32), craw_s[1, r:r + 16, :].astype(f32), cr, ci)
        _put(c_s, r, 0, [re[:, :PA], -im[:, :PA], re[:, PA:], -im[:, PA:]])


def _ssm_scan(u_ref, carry, lam_s, h_s, tie):
    car, cai = carry
    out = []
    for b in range(TC // 8):
        mixed = u_ref[3, b, :, 0:T]
        u = jnp.concatenate([u_ref[cb, b] for cb in range(3)], axis=1)
        cols = [u[:, 0:T], u[:, T:2 * T], u[:, 2 * T:PA], mixed]
        hr = jnp.concatenate([tie(v, 4 * b + n) for n, v in enumerate(cols)], axis=1)
        hi = jnp.concatenate([u[:, PA:2 * PA], pltpu.roll(mixed, PB, 1)], axis=1)
        for n, d in enumerate((1, 2, 4)):
            sr, si = pltpu.roll(hr, d, 0), pltpu.roll(hi, d, 0)
            tr, ti = _cmul(sr, si, lam_s[2 * n], lam_s[2 * n + 1])
            hr, hi = hr + tr, hi + ti
        tr, ti = _cmul(lam_s[6], lam_s[7], car, cai)
        hr, hi = hr + tr, hi + ti
        car, cai = hr[7:8, :], hi[7:8, :]
        out.append(jnp.concatenate([hr[:, :PA], hi[:, :PA], hr[:, PA:]], axis=1))
        if b % 2 == 1:
            _put(h_s, (b - 1) * 8, 0, [jnp.concatenate(out, axis=0)])
            out = []
    return car, cai


_vmem = pltpu.VMEM
_PROLOGUE_SCRATCH = dict(
    xT_s=_vmem((M, S), bf16),
    v0=_vmem((M,), bf16), v1=_vmem((M,), bf16), v2=_vmem((M,), bf16), v3=_vmem((M,), bf16), v4=_vmem((M,), bf16),
    b_s=_vmem((2 * M, M), bf16),
    craw_s=_vmem((2, M, M), bf16),
    c_s=_vmem((M // 2, 2 * M), u32),
    coef_s=_vmem((8, 512), f32),
    lam_s=_vmem((8, 8, 512), f32),
    col_s=_vmem((2, M, T), f32),
    h_s=_vmem((TC // 2, 2 * M), u32),
    ckv_s=_vmem((4, 4, 2, T // 2, DC), bf16),
    rq=_vmem((M, H, D), bf16),
    rk=_vmem((NRAW * CS, H, D), bf16),
    rv=_vmem((NRAW * CS, H, D), bf16),
    sq=_vmem((4, M * 4, T), u32),
    sk=_vmem((4, CS * 4, T), u32),
    sv=_vmem((4, CS * 4, T), u32),
    xa_s=_vmem((HM // 2, NP * 7 * T), u32),
)
_HEAD_SCRATCH = dict(
    mk_s=_vmem((7 * HD, 2 * T), f32),
    mv_s=_vmem((2, 7 * HD, 2 * T), f32),
    mp_s=_vmem((7 * HD, 2 * T), f32),
    kt_s=_vmem((2 * T, 4 * T), f32),
    ka_s=_vmem((S // 4, 9 * T), u32),
    va_s=_vmem((HD // 2, NP * 9 * T), u32),
    v2_s=_vmem((QD // 2, 3 * 49 * T), u32),
    s_s=_vmem((4, S // 8, 8, 2 * T), f32),
    pb_s=_vmem((2 * T, 7 * T), u32),
    pd_s=_vmem((S // 2, 2 * T), u32),
    p2_s=_vmem((3 * T, 49 * T), u32),
    sc_s=_vmem((1, S), f32),
    qb_s=_vmem((HD // 2, 14 * T), u32),
)
_SHARED_SCRATCH = [
    _vmem((H // 2 * D, DC), u32),
    _vmem((H // 2 * D, DC), u32),
    _vmem((S // 8, 49 * QC), u32),
    _vmem((H * D, S // 2), u32),
    _vmem((H, M, D), bf16),
    _vmem((QD, 49 * QC), u32),
    _vmem((HM // 2, 7 * T), u32),
    _vmem((HD // 2, NP * 7 * T), u32),
    _vmem((M, S), f32),
    _vmem((1, S), f32),
    _vmem((8, T), f32),
    pltpu.SemaphoreType.DMA((NSEM,)),
]


def _kernel(xT_hbm, bre_hbm, bim_hbm, cre_hbm, cim_hbm, lre_hbm, lim_hbm, ldt_hbm,
            dsk_hbm, gw_hbm, woT_hbm, ckv_hbm, wq_hbm, wk_hbm, wv_hbm,
            out_hbm,
            wkt_s, wvt_s, a_s, q_s, wo_s, w_s, wl_s, cl_s, o_s, g_s, zero_s, sem, *rest):
    h = pl.program_id(0)
    pro_refs = dict(zip(_PROLOGUE_SCRATCH, rest))
    head_refs = dict(zip(_HEAD_SCRATCH, rest[len(pro_refs):]))

    def out_copy(jp):
        cols = pl.ds(jp * 2 * T, 2 * T)
        return pltpu.make_async_copy(o_s.at[:, cols], out_hbm.at[:, cols], sem.at[SEM_OUT])

    def prep_w(hh, outer, tie):
        rows = _ds(lax.shift_right_logical(hh, 1) * D, D, D)
        sh = (16 * (1 - (hh & 1))).astype(u32)
        k = 0
        for row0, wt_s in ((0, wkt_s.at[rows]), (QD, wvt_s.at[rows])):
            for r in range(0, QD, 16):
                def block(o, q):
                    row = (o % 2) * HD + (q % 2) * QD + r
                    col = (o // 2) * 2 * QC + (q // 2) * QC
                    return _hi16(wt_s[row:row + 16, col:col + QC] << sh)
                for n1 in outer:
                    _put(w_s, row0 + r, 7 * n1 * QC, _operands2(_B_TERMS, n1, block, lambda x: tie(x, k)))
                    k += 1

    def prologue(xT_s, v0, v1, v2, v3, v4, b_s, craw_s, c_s, coef_s, lam_s, col_s, h_s,
                 ckv_s, rq, rk, rv, sq, sk, sv, xa_s):
        u_s = head_refs['s_s']
        vec_s = (v0, v1, v2, v3, v4)

        def slice_copies(i):
            s = sem.at[SEM_SL + i]
            grp = i // 2 if isinstance(i, int) else lax.shift_right_logical(i, 1)
            cs, dst = pl.ds(i * CS, CS), pl.ds((i & (NRAW - 1)) * CS, CS)
            return [pltpu.make_async_copy(ckv_hbm.at[grp, :, i & 1], ckv_s.at[grp, :, i & 1], s),
                    pltpu.make_async_copy(wk_hbm.at[cs], rk.at[dst], s),
                    pltpu.make_async_copy(wv_hbm.at[cs], rv.at[dst], s)]

        def wq1_copy(i):
            rows = pl.ds(i * (M // 4), M // 4)
            return pltpu.make_async_copy(wq_hbm.at[rows, 8:16], rq.at[rows, 8:16], sem.at[SEM_WQ1 + i])

        def x_copy(i):
            cols = pl.ds(i * TA, TA)
            return pltpu.make_async_copy(xT_hbm.at[:, cols], xT_s.at[:, cols], sem.at[SEM_X + i])

        cp_vec = [pltpu.make_async_copy(src, dst, sem.at[SEM_VEC])
                  for src, dst in zip((lre_hbm, lim_hbm, ldt_hbm, dsk_hbm, gw_hbm), vec_s)]
        cp_b = [pltpu.make_async_copy(src.at[pl.ds(lo, n)], b_s.at[pl.ds(dst, n)], sem.at[SEM_B])
                for src, lo, n, dst in ((bre_hbm, 0, PA, 0), (bim_hbm, 0, PA, PA),
                                        (bre_hbm, PA, PB, 2 * PA), (bim_hbm, PA, PB, 2 * PA + PB))]
        cp_wq = [pltpu.make_async_copy(wq_hbm.at[:, 0:8], rq.at[:, 0:8], sem.at[SEM_WQ])]
        cp_c = [pltpu.make_async_copy(src, craw_s.at[n], sem.at[SEM_C])
                for n, src in enumerate((cre_hbm, cim_hbm))]
        cp_wo = pltpu.make_async_copy(woT_hbm, wo_s, sem.at[SEM_WO])
        for cp in cp_vec + cp_b + [x_copy(i) for i in range(S // TA)] + cp_c + cp_wq:
            cp.start()
        for i in range(NRAW - 1):
            for cp in [wq1_copy(i)] + slice_copies(i):
                cp.start()
        wq1_copy(3).start()
        cp_wo.start()

        zero_s[...] = jnp.zeros(zero_s.shape, f32)
        wl_s[...] = jnp.zeros(wl_s.shape, u32)
        cl_s[:, (NP - 1) * 7 * T:] = jnp.zeros((HD // 2, 7 * T), u32)
        for cp in cp_vec:
            cp.wait()
        _ssm_params(vec_s, coef_s, lam_s, col_s)

        def phase1(i):
            clk = _Clock(zero_s)
            u, _ = clk.dot(xT_s[:, i * TA:(i + 1) * TA], b_s[...], _TT)
            for cb in range(4):
                w = min(2 * T, 2 * M - cb * 2 * T)
                u_s[cb, i * TA // 8:(i + 1) * TA // 8, :, 0:w] = (
                    u[:, cb * 2 * T:cb * 2 * T + w].reshape(TA // 8, 8, w))
            tie = clk.pacer(0, 6 * TA, 14)
            for t in range(2 * i, 2 * i + 2):
                for r in range(0, HM, 32):
                    k = (t % 2) * 7 + r // 32
                    top = xT_s[r:r + 32, 2 * t * T:(2 * t + 2) * T].astype(f32)
                    bot = xT_s[HM + r:HM + r + 32, 2 * t * T:(2 * t + 2) * T].astype(f32)
                    blocks = [tie(top[:, :T], k), bot[:, :T], top[:, T:], tie(bot[:, T:], k)]
                    _put(xa_s, r, t * 7 * T, _operands(_A_TERMS, blocks))
            return clk

        for cp in cp_b + [x_copy(0)]:
            cp.wait()
        phase1(0)
        x_copy(1).wait()
        clk = phase1(1)
        zero = jnp.zeros((1, 512), f32)
        carry0 = _ssm_scan(u_s.at[:, 0:TC // 8], (zero, zero), lam_s, h_s, clk.pacer(0, 6 * TA, TC // 2))
        for cp in [x_copy(2), x_copy(3)] + cp_c + cp_wq:
            cp.wait()
        _ssm_cmat(craw_s, coef_s, c_s, phase1(2).pacer(0, 6 * TA, M // 16))
        tie = phase1(3).pacer(0, 6 * TA, M // 8)
        for c0 in range(0, M, 8):
            _stage(rq, sq, c0, 8, lambda x: tie(x, c0 // 8), groups=(0,))

        def phase2(i, carry):
            @pl.when(i + NRAW - 1 < NP)
            def _():
                for cp in slice_copies(i + NRAW - 1):
                    cp.start()

            @pl.when(i < 4)
            def _():
                wq1_copy(i).wait()

            for cp in slice_copies(i):
                cp.wait()

            yT = _dot(_get(c_s, 0, M, 0, 2 * M), _get(h_s, 0, TC, 0, 2 * M), _NT)
            for t in range(TC // T):
                cols = _ds(i * TC + t * T, T, T)
                acc = jnp.zeros((8, T), f32)
                for r in range(0, M, 32):
                    xg = xT_s[r:r + 32, cols].astype(f32) * col_s[1, r:r + 32, :]
                    acc = acc + jnp.sum(xg.reshape(4, 8, T), axis=0)
                g = jax.nn.sigmoid(jnp.sum(acc, axis=0, keepdims=True))
                g_s[:, cols] = g
                for r in range(0, M, 32):
                    skip = xT_s[r:r + 32, cols].astype(f32) * col_s[0, r:r + 32, :]
                    o_s[r:r + 32, cols] = (1.0 - g) * (yT[r:r + 32, t * T:(t + 1) * T] + skip)

            ht = lax.shift_right_logical(i, 2)
            words = [sq[ht * 2 + dt, pl.ds(i & 3, M, stride=4), :] for dt in range(2)]
            both = [jnp.concatenate([pltpu.bitcast(w << 16, f32), _hi16(w)], axis=1) for w in words]
            wq = _operands(_B_TERMS, [both[0][:HM], both[1][:HM], both[0][HM:], both[1][HM:]])
            clk = _Clock(zero_s)
            m = [clk.dot(wq[n].astype(bf16),
                         _cat([_get(xa_s, 0, HM, (t * 7 + n) * T, T) for t in range(NP)], 1), _TN)[0]
                 for n in range(7)]
            q_i = q_s.at[_ds(i * 2 * D, 2 * D, 2 * D)]
            for n in (2, 1, 3, 0):
                for t in range(NP):
                    for r in range(0, D, GC):
                        c, = _combine(_Tiles(m, r, GC, t * T, T), (n,), range(7))
                        row = (2 * (r // HD) + n // 2) * D + (n % 2) * HD + r % HD
                        _put(q_i, row, t * T, [c * (LOG2E * D ** -0.5)])

            span = 5 * 1024

            u_next = u_s.at[:, pl.ds(jnp.minimum(i + 1, NP - 1) * (TC // 8), TC // 8)]
            carry = _ssm_scan(u_next, carry, lam_s, h_s, clk.pacer(0, span, TC // 2))

            tie = clk.pacer(0, span, 64)
            rq_i = rq.at[pl.ds((i & 3) * (M // 4), M // 4)]
            sq_i = sq.at[:, _ds((i & 3) * M, M, 8)]
            for c0 in range(0, M // 4, 8):
                _stage(rq_i, sq_i, c0, 8, lambda x: tie(x, c0 // 2 + 2), groups=(1,))
            slot = pl.ds((i & (NRAW - 1)) * CS, CS)
            for n, (raw, stg, wt_s) in enumerate(((rk, sk, wkt_s), (rv, sv, wvt_s))):
                for c0 in range(0, CS, 8):
                    _stage(raw.at[slot], stg, c0, 8, lambda x: tie(x, 16 * n + c0 // 8))
                cols = _ds(i * CS, CS, CS)
                for pair in range(H // 2):
                    for dt in range(2):
                        blk = stg[(pair // 4) * 2 + dt, pl.ds(pair % 4, CS, stride=4), :]
                        row = pair * D + dt * HD
                        wt_s[row:row + HD, cols] = tie(blk, 16 + 24 * n + 3 * pair + dt).T

            tie = clk.pacer(0, span, 28)
            ckv_i = ckv_s.at[lax.shift_right_logical(i, 1), :, i & 1]
            a_i = a_s.at[_ds(i * (T // 4), T // 4, T // 4)]
            for r in range(0, T // 2, 16):
                def block(o, q):
                    col = (o % 2) * 2 * QC + (q % 2) * QC
                    return ckv_i[2 * (q // 2) + o // 2, r:r + 16, col:col + QC].astype(f32)
                for n1 in range(7):
                    ops = _operands2(_A_TERMS, n1, block, lambda x: tie(x, 7 * (r // 16) + n1))
                    _put(a_i, r, 7 * n1 * QC, ops)
            return carry

        lax.fori_loop(0, NP, phase2, carry0)
        cp_wo.wait()
        prep_w(h, range(NT1), _no_tie)

    @pl.when(h == 0)
    def _():
        prologue(**pro_refs)

    def oproj(jp, clk):
        cols = slice(2 * jp * T, (2 * jp + 2) * T)
        for r, n in OCH:
            c = clk.strassen(lambda i: _get(wl_s, r, n, i * T, T),
                             lambda i: _get(cl_s, 0, HD, (jp * 7 + i) * T, T), _NN)()
            o_s[r:r + n, cols] += jnp.concatenate(c[:2], axis=1)
            o_s[HM + r:HM + r + n, cols] += jnp.concatenate(c[2:], axis=1)

    def head(mk_s, mv_s, mp_s, kt_s, ka_s, va_s, v2_s, s_s, pb_s, pd_s, p2_s, sc_s, qb_s):
        clk = _Clock(zero_s)
        q_h = q_s.at[_ds(h * D, D, D)]

        def prep_wo(tie):
            for r in range(0, HM, 16):
                top = tie(wo_s[h, r:r + 16, :].astype(f32), r // 16)
                bot = tie(wo_s[h, HM + r:HM + r + 16, :].astype(f32), r // 16)
                _put(wl_s, r, 0, _operands(_A_TERMS, [top[:, :HD], top[:, HD:], bot[:, :HD], bot[:, HD:]]))

        nine = lambda c: _operands(_A_TERMS, c) + [c[1], c[2]]

        def outer(m_s, r):
            return _combine([m_s[n * HD + r:n * HD + r + 16, :] for n in range(7)], order=range(7))

        def proj(g, lo, hi):
            for n1 in range(lo, hi):
                comb = clk.strassen(lambda n: _get(w_s, 0, 2 * QD, (7 * n1 + n) * QC, QC),
                                    lambda n: _get(a_s, g * T, T, (7 * n1 + n) * QC, QC), _NT, n1 == 6)
                for r in range(0, 2 * QD, GC):
                    m_s, row = mk_s if r < QD else mv_s.at[g % 2], n1 * HD + r % QD
                    c = comb(r, GC)
                    m_s[row:row + GC, :] = jnp.concatenate([c[0], c[2]], axis=1)
                    m_s[QD + row:QD + row + GC, :] = jnp.concatenate([c[1], c[3]], axis=1)
            if hi < 7:
                return
            cs = [outer(mk_s, r) for r in range(0, HD, 16)]
            for n in range(4):
                kt_s[:, n * T:(n + 1) * T] = jnp.concatenate([c[n] for c in cs], axis=0).T
            for r in range(0, 2 * T, GC):
                blk = kt_s[r:r + GC, :]
                _put(ka_s, 2 * g * T + r, 0, nine([blk[:, n * T:(n + 1) * T] for n in range(4)]))

        def vfin(g, tie):
            for r in range(0, QD, 16):
                k, ops = 9 * (r // 16), []
                for i, row in enumerate((r, QD + r)):
                    c = [tie(x, k + i) for x in outer(mv_s.at[g % 2], row)]
                    ops.append(nine([c[0], c[2], c[1], c[3]]))
                    _put(va_s, row, 2 * g * 9 * T, [o[:, :T] for o in ops[-1]], lambda w: tie(w, k + i, True, FLAG))
                    for n in (2, 7):
                        _put(va_s, row, ((2 * g + 1) * 9 + n) * T, [o[:, T:] for o in ops[-1][n:n + 2]])
                if g < 3:
                    for n1 in range(7):
                        lo_, hi_ = ops[0][n1], ops[1][n1]
                        _put(v2_s, r, (g * 7 + n1) * 7 * T,
                             _operands(_A_TERMS, [lo_[:, :T], lo_[:, T:], hi_[:, :T], hi_[:, T:]]),
                             lambda w: tie(w, k + 2 + n1, True, FLAG))

        key = lax.broadcasted_iota(jnp.int32, (T, 2 * T), 0)
        qry = lax.broadcasted_iota(jnp.int32, (T, 2 * T), 1)
        causal = key <= qry

        def qk(g):
            pairs = (2 * g, 2 * g + 1)
            mx = {jp: _Reducer(jnp.max, jnp.maximum) for jp in pairs}

            def put(jp, row, v):
                v = v.reshape(v.shape[0] // 8, 8, 2 * T)
                s_s[jp % 4, row // 8:row // 8 + v.shape[0]] = v
                mx[jp].add(v)

            def rect(jp, lo, hi, n):
                for r in range(lo, hi, n):
                    c = clk.strassen(lambda i: _get(ka_s, r, n, i * T, T),
                                     lambda i: _get(qb_s, 0, HD, ((jp % 2) * 7 + i) * T, T), _NN)()
                    put(jp, r, jnp.concatenate(c[:2], axis=1))
                    put(jp, jp * T + r, jnp.concatenate(c[2:], axis=1))

            q = lambda jp, e: _get(q_h, e * D, D, jp * T, T)
            for jp in pairs[g == 0:]:
                for r in range(0, HD, 32):
                    blk = [_get(q_h, e * D + d * HD + r, 32, jp * T, T).astype(f32) for d in range(2) for e in range(2)]
                    _put(qb_s, r, (jp % 2) * 7 * T, _operands(_B_TERMS, blk))
            for jp in pairs:
                rect(jp, 0, 2 * g * T, QCH if QCH else g * T // 2 or 1)
            kb = lambda jp, a, b: jnp.concatenate(
                [_get(ka_s, jp * T, T, a * T, T), _get(ka_s, jp * T, T, b * T, T)], axis=1)
            for jp in pairs:
                se, _ = clk.dot(kb(jp, 2, 7), jnp.concatenate([q(jp, 0), q(jp, 1)], axis=1), _NN)
                put(jp, 2 * jp * T, jnp.where(causal, se, NEG))
            last = {}
            for jp in pairs:
                so = jnp.where(causal[:, :T], clk.dot(kb(jp, 8, 3), q(jp, 1), _NN)[0], NEG)
                row = (2 * jp + 1) * T // 8
                s_s[jp % 4, row:row + T // 8, :, T:] = so.reshape(T // 8, 8, T)
                last[jp] = jnp.concatenate([jnp.full((1, T), NEG, f32), jnp.max(so, axis=0, keepdims=True)], axis=1)
            rect(2 * g + 1, 2 * g * T, (2 * g + 1) * T, T // 4)
            return [jnp.broadcast_to(jnp.maximum(mx[jp].result(), last[jp]), (8, 2 * T)) for jp in pairs]

        zs, sums = {}, {}

        def prob(jp, row, z, n=GS, lanes=slice(None)):
            return jnp.exp2(s_s[jp % 4, row // 8:(row + n) // 8, :, lanes] - z[:, lanes])

        def rough(jp, mx, tie):
            zs[jp] = mx
            if jp > 0:
                sm = _Reducer(jnp.sum, jnp.add)
                for k, r in enumerate(range(0, 2 * jp * T, GS * LSUB)):
                    sm.add(prob(jp, r, tie(mx, k)))
                zs[jp] = mx + jnp.log2(jnp.maximum(LSUB * sm.result(), 1.0))
            sums[jp] = _Reducer(jnp.sum, jnp.add)

        def blocks(jp, row, tie, k):
            top, bot = prob(jp, row, tie(zs[jp], k)), prob(jp, jp * T + row, tie(zs[jp], k + 1))
            sums[jp].add(top + bot)
            top, bot = top.reshape(GS, 2 * T), bot.reshape(GS, 2 * T)
            return [top[:, :T], top[:, T:], bot[:, :T], bot[:, T:]]

        def near(jp, tie, k):
            R, z = jp * T, zs[jp]
            if jp % 2:
                for r in range(0, T, GS):
                    _put(pb_s, jp // 2 * T + r, 0, _operands(_B_TERMS, blocks(jp, R - T + r, tie, k)))
                    k += 2
            for r in range(0, T, GS):
                p = prob(jp, 2 * R + r, tie(z, k))
                sums[jp].add(p)
                _put(pd_s, 2 * R + r, 0, [p.reshape(GS, 2 * T)])
                k += 1
            so = _Reducer(jnp.sum, jnp.add)
            for r in range(0, T, 2 * GS):
                p = prob(jp, 2 * R + T + r, tie(z, k), 2 * GS, slice(T, 2 * T))
                so.add(p)
                _put(pd_s, 2 * R + T + r, T, [p.reshape(2 * GS, T)])
                k += 1
            sums[jp].result()
            sums[jp].out = sums[jp].out + jnp.concatenate([jnp.zeros((1, T), f32), so.result()], axis=1)

        p20 = lambda g: g * (g - 1) // 2 * T

        def far(g, tie, k):
            half = {(jp, e): _Reducer(jnp.sum, jnp.add) for jp in (2 * g, 2 * g + 1) for e in range(2)}
            for kg in range(g):
                for r in range(0, T, GS):
                    blk = {}
                    for new, n1 in (((0,), 1), ((1,), 5), ((3,), 2), ((), 0), ((), 4), ((2,), 3), ((), 6)):
                        for o in new:
                            lanes = slice((o % 2) * T, (o % 2 + 1) * T)
                            for jp in (2 * g, 2 * g + 1):
                                z = tie(zs[jp][:, lanes], k)
                                row = (o // 2) * jp * T + 2 * kg * T + r
                                p = [jnp.exp2(s_s[jp % 4, x // 8:(x + GS) // 8, :, lanes] - z) for x in (row, row + T)]
                                half[jp, o % 2].add(p[0] + p[1])
                                blk[o, jp % 2], blk[o, 2 + jp % 2] = [x.reshape(GS, T) for x in p]
                        ops = _operands2(_B_TERMS, n1, lambda o, q: blk[o, q], lambda x: x)
                        _put(p2_s, p20(g) + kg * T + r, 7 * n1 * T, ops,
                             (lambda w: tie(w, k, True, FLAG)) if FTIE else None)
                        k += FW * 8 / 7
            for jp in (2 * g, 2 * g + 1):
                if g:
                    sums[jp].out = sums[jp].out + jnp.concatenate([half[jp, e].result() for e in range(2)], axis=1)
            for jp in (2 * g, 2 * g + 1):
                cols = slice(2 * jp * T, 2 * (jp + 1) * T)
                sc_s[:, cols] = g_s[:, cols] / sums[jp].result()

        def pv(g):
            pairs = (2 * g, 2 * g + 1)
            va = lambda n, t, r=0, nr=HD: _get(va_s, r, nr, (t * 9 + n) * T, T)
            for n1 in range(7 if g else 0):
                c = clk.strassen(
                    lambda n: _cat([_get(v2_s, 0, QD, (kg * 49 + 7 * n1 + n) * T, T) for kg in range(g)], 1),
                    lambda n: _get(p2_s, p20(g), g * T, (7 * n1 + n) * T, T), _NN)()
                mp_s[n1 * HD:n1 * HD + QD, :] = jnp.concatenate(c[:2], axis=1)
                mp_s[n1 * HD + QD:(n1 + 1) * HD, :] = jnp.concatenate(c[2:], axis=1)
            ve = [jnp.concatenate([va(2, jp), va(8, jp)], axis=0) for jp in pairs]
            vo = [jnp.concatenate([va(7, jp), va(3, jp)], axis=0) for jp in pairs]
            ce = clk.level([(ve[jp % 2], _get(pd_s, 2 * jp * T, T, 0, T)) for jp in pairs])
            co = [clk.dot(jnp.concatenate([ve[jp % 2], vo[jp % 2]], axis=1),
                          _get(pd_s, 2 * jp * T, 2 * T, T, T), _NN)[0] for jp in pairs]
            for jp in pairs:
                R, e = jp * T, jp % 2
                ge, go = sc_s[:, 2 * R:2 * R + T], sc_s[:, 2 * R + T:2 * R + 2 * T]
                for r in range(0, HD, 32):
                    c = [ce[e][r:r + 32], co[e][r:r + 32], ce[e][HD + r:HD + r + 32], co[e][HD + r:HD + r + 32]]
                    if g:
                        far_ = _combine([mp_s[n * HD + r:n * HD + r + 32, e * T:(e + 1) * T] for n in range(7)],
                                        order=range(7))
                        c = [x + y for x, y in zip(c, far_)]
                    if e:
                        near_ = clk.strassen(lambda n: va(n, 2 * g, r, 32),
                                             lambda n: _get(pb_s, g * T, T, n * T, T), _NN)()
                        c = [x + y for x, y in zip(c, near_)]
                    ops = _operands(_B_TERMS, [c[0] * ge, c[1] * go, c[2] * ge, c[3] * go])
                    _put(cl_s, r, jp * 7 * T, ops)

        ends = []

        def run(items):
            for item in items.split():
                if item[0] == 'P':
                    pv(int(item[1]))
                    ends.append(clk.t)
                elif item[0] == 'K':
                    proj(int(item[1]), int(item[2]), int(item[3]))
                else:
                    jp = int(item[1])
                    oproj(jp, clk)

                    @pl.when(h == H - 1)
                    def _():
                        out_copy(jp).start()

        for n1 in range(7):
            if n1 >= NT1:
                prep_w(h, [n1], clk.pacer(max(clk.t - LEAD - 448, 1), max(clk.t - LEAD, 1), 8))
            proj(0, n1, n1 + 1)
        oproj(NP - 1, clk)
        mx = qk(0)
        for g in range(4):
            t0 = clk.t
            del ends[:]
            run(PLAN[g])
            t1 = clk.t
            nxt = qk(g + 1) if g < 3 else None
            n_rough = [2 * jp * T // (GS * LSUB) for jp in (2 * g, 2 * g + 1)]
            n_near = [(T + T // 2) // GS, (3 * T + T // 2) // GS]
            holes = [(t - PH0, t + PH1) for t in ends]
            if g == 0:
                vfin(0, clk.pacer(t0, t0 + VW, 36))
                holes.append((t0, t0 + VW))
            if g < 3:
                vfin(g + 1, clk.pacer(t1 + HOLE1, t1 + HOLE1 + (VW if g < 2 else VW // 3), 36))
                holes.append((t1 - HOLE0, t1 + HOLE1 + (VW if g < 2 else VW // 3)))
            tie = clk.pacer(t0 + D0, (clk.t if g else t1) - SLACK,
                            sum(n_rough) + sum(n_near) + FW * g * 8 * T // GS, holes)
            rough(2 * g, mx[0], tie)
            near(2 * g, tie, n_rough[0])
            k = n_rough[0] + n_near[0]
            rough(2 * g + 1, mx[1], lambda x, i: tie(x, k + i))
            near(2 * g + 1, tie, k + n_rough[1])
            far(g, tie, k + n_rough[1] + n_near[1])
            if g == 0:
                prep_wo(clk.pacer(t0 + VW, t1 - HOLE0, HM // 16))
            mx = nxt
        t0 = clk.t
        run(PLAN[4])
        prep_w(jnp.minimum(h + 1, H - 1), range(NT1), clk.pacer(t0 - PW0, clk.t - 300, 8 * NT1))
        if os.environ.get('SHOW'):
            print('final loads', clk.load)

    head(**head_refs)

    @pl.when(h == H - 1)
    def _():
        oproj(NP - 1, _Clock(zero_s))
        out_copy(NP - 1).start()
        for jp in range(NP):
            out_copy(jp).wait()


@jax.jit
def pallas_gated_mix__compressed_kv_cla__ssm_conv_s5__prompt_kernel(
    A_x: jax.Array,
    A_c_kv: jax.Array,
    A_w_q: jax.Array,
    A_w_uk: jax.Array,
    A_w_uv: jax.Array,
    A_w_o: jax.Array,
    B_x: jax.Array,
    B_Lambda_re: jax.Array,
    B_Lambda_im: jax.Array,
    B_B_re: jax.Array,
    B_B_im: jax.Array,
    B_C_re: jax.Array,
    B_C_im: jax.Array,
    B_log_dt: jax.Array,
    B_Dskip: jax.Array,
    gate_w: jax.Array,
):
    del B_x
    xT = jnp.transpose(A_x[0])
    woT = jnp.transpose(A_w_o, (0, 2, 1))
    ckv = A_c_kv.reshape(4, 4, 2, T // 2, DC)

    hbm = pl.BlockSpec(memory_space=pl.ANY)
    outT = pl.pallas_call(
        _kernel,
        grid=(H,),
        in_specs=[hbm] * 15,
        out_specs=hbm,
        out_shape=jax.ShapeDtypeStruct((M, S), f32),
        scratch_shapes=_SHARED_SCRATCH + list(_PROLOGUE_SCRATCH.values()) + list(_HEAD_SCRATCH.values()),
        compiler_params=pltpu.CompilerParams(
            dimension_semantics=("arbitrary",),
            vmem_limit_bytes=126 * 1024 * 1024,
        ),
    )(xT, B_B_re, B_B_im, B_C_re, B_C_im, B_Lambda_re, B_Lambda_im, B_log_dt,
      B_Dskip, gate_w, woT, ckv, A_w_q, A_w_uk, A_w_uv)
    return jnp.transpose(outT)[None]
```

```python
import bisect
import os

import jax
import jax.numpy as jnp
from jax import lax
import jax.experimental.pallas as pl
import jax.experimental.pallas.tpu as pltpu

S = 2048
M = 448
H = 16
D = 256
DC = 1024
T = 128
NP = S // T // 2
HD = D // 2
HM = M // 2
QD = D // 4
QC = DC // 4
PA = 384
PB = M - PA
TA = 512
TC = 256
CS = DC // NP
NRAW = 4
LOG2E = 1.4426950408889634
NEG = -1e30

_env = lambda k, d: type(d)(os.environ.get(k, d))
GC = _env('GC', 64)
GS = _env('GS', 16)
RCH = _env('RCH', 256)
SLACK = _env('SLACK', 200)
D0 = _env('D0', 0)
NT1 = _env('NT1', 3)
LEAD = _env('LEAD', 448)
PW0 = _env('PW0', 100)
FTIE = _env('FTIE', 1)
FLAG = _env('FLAG', 40)
FW = _env('FW', 2)
HOLE0 = _env('HOLE0', 300)
HOLE1 = _env('HOLE1', 300)
VW = _env('VW', 900)
VB = _env('VB', 0)
PH0 = _env('PH0', 500)
PH1 = _env('PH1', 100)
QCH = _env('QCH', 64)
OCH = ((0, 64), (64, 64), (128, 48), (176, 48))
LSUB = _env('LSUB', 4)
PLAN = _env('PLAN', 'K107,K207,K307,P0 P1 O0 O1 P2 O2 O3 O4,P3 O5 O6').split(',')

f32 = jnp.float32
bf16 = jnp.bfloat16
u32 = jnp.uint32

SEM_VEC, SEM_B, SEM_X, SEM_WQ, SEM_C, SEM_SL, SEM_WO, SEM_OUT, SEM_WQ1 = 0, 1, 2, 6, 7, 8, 16, 17, 18
NSEM = 22

_NN = ((1,), (0,))
_NT = ((1,), (1,))
_TN = ((0,), (0,))
_TT = ((0,), (1,))


def _dot(a, b, dims):
    return lax.dot_general(a, b, (dims, ((), ())), preferred_element_type=f32)


def _cat(xs, axis):
    return xs[0] if len(xs) == 1 else jnp.concatenate(xs, axis=axis)


def _ds(lo, n, align):
    return pl.ds(lo if isinstance(lo, int) else pl.multiple_of(lo, align), n)


def _put(ref, row, col, xs, tie=None):
    x = _cat(xs, 1)
    if tie is not None:
        x = jnp.concatenate([tie(x[:8]), x[8:]], axis=0)
    ref[row // 2:(row + x.shape[0]) // 2, col:col + x.shape[1]] = pltpu.bitcast(x.astype(bf16), u32)


def _get(ref, row, nrows, col, ncols):
    return pltpu.bitcast(ref[row // 2:(row + nrows) // 2, col:col + ncols], bf16)


class _Clock:
    def __init__(self, zero_ref):
        self.masks = {(8, T): zero_ref[...] != 0.0}
        self.ticks, self.load = [], [0, 0, 0, 0]

    @property
    def t(self):
        return max(self.load)

    def dot(self, a, b, dims):
        v = _dot(a, b, dims)
        rows, depth = v.shape[0], a.shape[dims[0][0]]
        for c in range(0, v.shape[1], T):
            start = 0
            for _ in range(0, depth, T):
                k = self.load.index(min(self.load))
                start = max(start, self.load[k])
                self.load[k] += rows
            self.ticks += [(start + r + 8, (v, r, c)) for r in range(0, rows, 8)]
        return v, start

    def strassen(self, lhs, rhs, dims, split_last=False):
        jobs = -(-lhs(0).shape[dims[0][0]] // T)
        lag = sum(l + 32 <= max(self.load) for l in self.load) // jobs if jobs < 3 else 0
        order = ((1, 3, 2, 4, 0, 5, 6), (0, 1, 3, 2, 4, 5, 6), (5, 6, 1, 3, 2, 4, 0), (0, 5, 6, 1, 3, 2, 4))[lag]
        m = {}
        for n in order:
            if split_last and n == order[-1]:
                a, half = lhs(n), lhs(0).shape[0] // 2
                m[n] = jnp.concatenate([self.dot(a[:half], rhs(n), dims)[0], self.dot(a[half:], rhs(n), dims)[0]], 0)
            else:
                m[n] = self.dot(lhs(n), rhs(n), dims)[0]
        vals = [m[n] for n in range(7)]
        return lambda r=0, n=None, only=(0, 1, 2, 3), c=0, w=None: _combine(
            vals if n is None else _Tiles(vals, r, n, c, w), only, order)

    def level(self, pairs):
        target = -(-(sum(self.load) + sum(a.shape[0] for a, _ in pairs)) // 64) * 16
        out = []
        for a, b in pairs:
            r, parts = 0, []
            while r < a.shape[0]:
                n = min(target - min(self.load), a.shape[0] - r)
                parts.append(self.dot(a[r:r + n], b, _NN)[0])
                r += n
            out.append(_cat(parts, 0))
        return out

    def pacer(self, t0, t1, n, holes=()):
        holes = sorted((max(a, t0), min(b, t1)) for a, b in holes if a < t1 and b > t0)
        gap = sum(b - a for a, b in holes)
        ticks = sorted(self.ticks, key=lambda tw: tw[0])
        times = [tw[0] for tw in ticks]

        def tie(x, k, distinct=False, delay=0):
            t = t0 + (t1 - t0 - gap) * k / n
            for a, b in holes:
                t += b - a if t > a else 0
            t += delay
            past = ticks[:bisect.bisect_right(times, t)]
            if not past:
                return x
            reps = (x.shape[0] // 8, x.shape[1] // T)
            tick = _cat([v[r:r + 8, c:c + T] for _, (v, r, c) in past[-reps[1] if distinct else -1:]], 1)
            if tick.dtype != x.dtype:
                tick = pltpu.bitcast(tick, x.dtype)
            if x.shape not in self.masks:
                self.masks[x.shape] = jnp.tile(self.masks[(8, T)], reps)
            return lax.select(self.masks[x.shape], tick if tick.shape == x.shape else jnp.tile(tick, reps), x)
        return tie


def _no_tie(x, k):
    return x


_A_TERMS = ((0, 3, 1), (2, 3, 1), (0, None, 0), (3, None, 0), (0, 1, 1), (2, 0, -1), (1, 3, -1))
_B_TERMS = ((0, 3, 1), (0, None, 0), (1, 3, -1), (2, 0, -1), (3, None, 0), (0, 1, 1), (2, 3, 1))


def _operand(term, block):
    x, y, sign = term
    if y is None:
        return block(x)
    return block(x) + block(y) if sign > 0 else block(x) - block(y)


def _operands(terms, blocks):
    return [_operand(t, blocks.__getitem__) for t in terms]


def _operands2(terms, n1, block, tie):
    first = terms[n1][0]
    sub = [_operand(terms[n1], lambda o: tie(block(o, q)) if o == first and q in (0, 3) else block(o, q))
           for q in range(4)]
    return _operands(terms, sub)


_C_TERMS = ({0: 1, 3: 1, 4: -1, 6: 1}, {2: 1, 4: 1}, {1: 1, 3: 1}, {0: 1, 1: -1, 2: 1, 5: 1})


def _combine(m, only=(0, 1, 2, 3), order=(1, 3, 2, 4, 0, 5, 6)):
    out = []
    for terms in (_C_TERMS[n] for n in only):
        seq = [n for n in order if n in terms]
        if terms[seq[0]] < 0:
            seq[0], seq[1] = seq[1], seq[0]
        acc = m[seq[0]]
        for n in seq[1:]:
            acc = acc + m[n] if terms[n] > 0 else acc - m[n]
        out.append(acc)
    return out


class _Tiles:
    def __init__(self, vals, r, n, c=0, w=None):
        self.vals, self.idx, self.cache = vals, (slice(r, r + n), slice(c, None if w is None else c + w)), {}

    def __getitem__(self, i):
        if i not in self.cache:
            self.cache[i] = self.vals[i][self.idx]
        return self.cache[i]


class _Reducer:
    def __init__(self, red, comb):
        self.red, self.comb, self.acc, self.rows, self.out = red, comb, None, 0, None

    def add(self, v):
        self.rows += 8 * v.shape[0]
        v = self.red(v, axis=0)
        self.acc = v if self.acc is None else self.comb(self.acc, v)
        if self.rows >= RCH:
            self.result()

    def result(self):
        if self.acc is not None:
            v = self.red(self.acc, axis=0, keepdims=True)
            self.out = v if self.out is None else self.comb(self.out, v)
        self.acc, self.rows = None, 0
        return self.out


def _cmul(ar, ai, br, bi):
    return ar * br - ai * bi, ar * bi + ai * br


def _hi16(w):
    return pltpu.bitcast(w & jnp.uint32(0xFFFF0000), f32)


def _stage(raw, stg, c0, nc, tie, groups=(0, 1)):
    for ht in groups:
        for dt in range(2):
            v = raw[c0:c0 + nc, ht * 8:(ht + 1) * 8, dt * T:(dt + 1) * T].reshape(nc * 8, T)
            stg[ht * 2 + dt, c0 * 4:(c0 + nc) * 4, :] = tie(pltpu.bitcast(v, u32))


def _ssm_params(vec_s, coef_s, lam_s, col_s):
    row = lambda r: r[...].astype(f32).reshape(1, M)
    lre, lim, ldt, dsk, gw = [row(v) for v in vec_s]
    dt = jnp.exp(ldt).astype(bf16).astype(f32)
    mag = jnp.exp(dt * lre)
    ang = dt * lim
    lr, li = mag * jnp.cos(ang), mag * jnp.sin(ang)
    den = lre * lre + lim * lim
    nr = lr - 1.0
    coef_s[...] = jnp.zeros(coef_s.shape, f32)
    coef_s[0:1, 0:M] = 2.0 * ((nr * lre + li * lim) / den)
    coef_s[1:2, 0:M] = 2.0 * ((li * lre - nr * lim) / den)

    er = jnp.concatenate([lr, lr[:, PA:]], axis=1)
    ei = jnp.concatenate([li, -li[:, PA:]], axis=1)
    pw = [(er, ei)]
    for _ in range(7):
        pw.append(_cmul(pw[-1][0], pw[-1][1], er, ei))
    sub = lax.broadcasted_iota(jnp.int32, (8, 512), 0)
    for n, d in enumerate((1, 2, 4)):
        lam_s[2 * n] = jnp.where(sub >= d, pw[d - 1][0], 0.0)
        lam_s[2 * n + 1] = jnp.where(sub >= d, pw[d - 1][1], 0.0)
    lcr = jnp.zeros((8, 512), f32)
    lci = jnp.zeros((8, 512), f32)
    for r in range(8):
        lcr = jnp.where(sub == r, pw[r][0], lcr)
        lci = jnp.where(sub == r, pw[r][1], lci)
    lam_s[6] = lcr
    lam_s[7] = lci

    def col(v):
        v = jnp.concatenate([v, jnp.zeros((1, 512 - M), f32)], axis=1)
        return jnp.broadcast_to(v, (T, 512)).T[:M]
    col_s[0] = col(dsk)
    col_s[1] = col(gw)


def _ssm_cmat(craw_s, coef_s, c_s, tie):
    for r in range(0, M, 16):
        coef = tie(coef_s[...], r // 16)
        cr, ci = coef[0:1, :M], coef[1:2, :M]
        re, im = _cmul(craw_s[0, r:r + 16, :].astype(f32), craw_s[1, r:r + 16, :].astype(f32), cr, ci)
        _put(c_s, r, 0, [re[:, :PA], -im[:, :PA], re[:, PA:], -im[:, PA:]])


def _ssm_scan(u_ref, carry, lam_s, h_s, tie):
    car, cai = carry
    out = []
    for b in range(TC // 8):
        mixed = u_ref[3, b, :, 0:T]
        u = jnp.concatenate([u_ref[cb, b] for cb in range(3)], axis=1)
        cols = [u[:, 0:T], u[:, T:2 * T], u[:, 2 * T:PA], mixed]
        hr = jnp.concatenate([tie(v, 4 * b + n) for n, v in enumerate(cols)], axis=1)
        hi = jnp.concatenate([u[:, PA:2 * PA], pltpu.roll(mixed, PB, 1)], axis=1)
        for n, d in enumerate((1, 2, 4)):
            sr, si = pltpu.roll(hr, d, 0), pltpu.roll(hi, d, 0)
            tr, ti = _cmul(sr, si, lam_s[2 * n], lam_s[2 * n + 1])
            hr, hi = hr + tr, hi + ti
        tr, ti = _cmul(lam_s[6], lam_s[7], car, cai)
        hr, hi = hr + tr, hi + ti
        car, cai = hr[7:8, :], hi[7:8, :]
        out.append(jnp.concatenate([hr[:, :PA], hi[:, :PA], hr[:, PA:]], axis=1))
        if b % 2 == 1:
            _put(h_s, (b - 1) * 8, 0, [jnp.concatenate(out, axis=0)])
            out = []
    return car, cai


_vmem = pltpu.VMEM
_PROLOGUE_SCRATCH = dict(
    xT_s=_vmem((M, S), bf16),
    v0=_vmem((M,), bf16), v1=_vmem((M,), bf16), v2=_vmem((M,), bf16), v3=_vmem((M,), bf16), v4=_vmem((M,), bf16),
    b_s=_vmem((2 * M, M), bf16),
    craw_s=_vmem((2, M, M), bf16),
    c_s=_vmem((M // 2, 2 * M), u32),
    coef_s=_vmem((8, 512), f32),
    lam_s=_vmem((8, 8, 512), f32),
    col_s=_vmem((2, M, T), f32),
    h_s=_vmem((TC // 2, 2 * M), u32),
    ckv_s=_vmem((4, 4, 2, T // 2, DC), bf16),
    rq=_vmem((M, H, D), bf16),
    rk=_vmem((NRAW * CS, H, D), bf16),
    rv=_vmem((NRAW * CS, H, D), bf16),
    sq=_vmem((4, M * 4, T), u32),
    sk=_vmem((4, CS * 4, T), u32),
    sv=_vmem((4, CS * 4, T), u32),
    xa_s=_vmem((HM // 2, NP * 7 * T), u32),
)
_HEAD_SCRATCH = dict(
    mk_s=_vmem((7 * HD, 2 * T), f32),
    mv_s=_vmem((2, 7 * HD, 2 * T), f32),
    mp_s=_vmem((7 * HD, 2 * T), f32),
    kt_s=_vmem((2 * T, 4 * T), f32),
    ka_s=_vmem((S // 4, 9 * T), u32),
    va_s=_vmem((HD // 2, NP * 9 * T), u32),
    v2_s=_vmem((QD // 2, 3 * 49 * T), u32),
    s_s=_vmem((4, S // 8, 8, 2 * T), f32),
    pb_s=_vmem((2 * T, 7 * T), u32),
    pd_s=_vmem((S // 2, 2 * T), u32),
    p2_s=_vmem((3 * T, 49 * T), u32),
    sc_s=_vmem((1, S), f32),
    qb_s=_vmem((HD // 2, 14 * T), u32),
)
_SHARED_SCRATCH = [
    _vmem((H // 2 * D, DC), u32),
    _vmem((H // 2 * D, DC), u32),
    _vmem((S // 8, 49 * QC), u32),
    _vmem((H * D, S // 2), u32),
    _vmem((H, M, D), bf16),
    _vmem((QD, 49 * QC), u32),
    _vmem((HM // 2, 7 * T), u32),
    _vmem((HD // 2, NP * 7 * T), u32),
    _vmem((M, S), f32),
    _vmem((1, S), f32),
    _vmem((8, T), f32),
    pltpu.SemaphoreType.DMA((NSEM,)),
]


def _kernel(xT_hbm, bre_hbm, bim_hbm, cre_hbm, cim_hbm, lre_hbm, lim_hbm, ldt_hbm,
            dsk_hbm, gw_hbm, woT_hbm, ckv_hbm, wq_hbm, wk_hbm, wv_hbm,
            out_hbm,
            wkt_s, wvt_s, a_s, q_s, wo_s, w_s, wl_s, cl_s, o_s, g_s, zero_s, sem, *rest):
    h = pl.program_id(0)
    pro_refs = dict(zip(_PROLOGUE_SCRATCH, rest))
    head_refs = dict(zip(_HEAD_SCRATCH, rest[len(pro_refs):]))

    def out_copy(jp):
        cols = pl.ds(jp * 2 * T, 2 * T)
        return pltpu.make_async_copy(o_s.at[:, cols], out_hbm.at[:, cols], sem.at[SEM_OUT])

    def prep_w(hh, outer, tie):
        rows = _ds(lax.shift_right_logical(hh, 1) * D, D, D)
        sh = (16 * (1 - (hh & 1))).astype(u32)
        k = 0
        for row0, wt_s in ((0, wkt_s.at[rows]), (QD, wvt_s.at[rows])):
            for r in range(0, QD, 16):
                def block(o, q):
                    row = (o % 2) * HD + (q % 2) * QD + r
                    col = (o // 2) * 2 * QC + (q // 2) * QC
                    return _hi16(wt_s[row:row + 16, col:col + QC] << sh)
                for n1 in outer:
                    _put(w_s, row0 + r, 7 * n1 * QC, _operands2(_B_TERMS, n1, block, lambda x: tie(x, k)))
                    k += 1

    def prologue(xT_s, v0, v1, v2, v3, v4, b_s, craw_s, c_s, coef_s, lam_s, col_s, h_s,
                 ckv_s, rq, rk, rv, sq, sk, sv, xa_s):
        u_s = head_refs['s_s']
        vec_s = (v0, v1, v2, v3, v4)

        def slice_copies(i):
            s = sem.at[SEM_SL + i]
            grp = i // 2 if isinstance(i, int) else lax.shift_right_logical(i, 1)
            cs, dst = pl.ds(i * CS, CS), pl.ds((i & (NRAW - 1)) * CS, CS)
            return [pltpu.make_async_copy(ckv_hbm.at[grp, :, i & 1], ckv_s.at[grp, :, i & 1], s),
                    pltpu.make_async_copy(wk_hbm.at[cs], rk.at[dst], s),
                    pltpu.make_async_copy(wv_hbm.at[cs], rv.at[dst], s)]

        def wq1_copy(i):
            rows = pl.ds(i * (M // 4), M // 4)
            return pltpu.make_async_copy(wq_hbm.at[rows, 8:16], rq.at[rows, 8:16], sem.at[SEM_WQ1 + i])

        def x_copy(i):
            cols = pl.ds(i * TA, TA)
            return pltpu.make_async_copy(xT_hbm.at[:, cols], xT_s.at[:, cols], sem.at[SEM_X + i])

        cp_vec = [pltpu.make_async_copy(src, dst, sem.at[SEM_VEC])
                  for src, dst in zip((lre_hbm, lim_hbm, ldt_hbm, dsk_hbm, gw_hbm), vec_s)]
        cp_b = [pltpu.make_async_copy(src.at[pl.ds(lo, n)], b_s.at[pl.ds(dst, n)], sem.at[SEM_B])
                for src, lo, n, dst in ((bre_hbm, 0, PA, 0), (bim_hbm, 0, PA, PA),
                                        (bre_hbm, PA, PB, 2 * PA), (bim_hbm, PA, PB, 2 * PA + PB))]
        cp_wq = [pltpu.make_async_copy(wq_hbm.at[:, 0:8], rq.at[:, 0:8], sem.at[SEM_WQ])]
        cp_c = [pltpu.make_async_copy(src, craw_s.at[n], sem.at[SEM_C])
                for n, src in enumerate((cre_hbm, cim_hbm))]
        cp_wo = pltpu.make_async_copy(woT_hbm, wo_s, sem.at[SEM_WO])
        for cp in cp_vec + cp_b + [x_copy(i) for i in range(S // TA)] + cp_c + cp_wq:
            cp.start()
        for i in range(NRAW - 1):
            for cp in [wq1_copy(i)] + slice_copies(i):
                cp.start()
        wq1_copy(3).start()
        cp_wo.start()

        zero_s[...] = jnp.zeros(zero_s.shape, f32)
        wl_s[...] = jnp.zeros(wl_s.shape, u32)
        cl_s[:, (NP - 1) * 7 * T:] = jnp.zeros((HD // 2, 7 * T), u32)
        for cp in cp_vec:
            cp.wait()
        _ssm_params(vec_s, coef_s, lam_s, col_s)

        def phase1(i):
            clk = _Clock(zero_s)
            u, _ = clk.dot(xT_s[:, i * TA:(i + 1) * TA], b_s[...], _TT)
            for cb in range(4):
                w = min(2 * T, 2 * M - cb * 2 * T)
                u_s[cb, i * TA // 8:(i + 1) * TA // 8, :, 0:w] = (
                    u[:, cb * 2 * T:cb * 2 * T + w].reshape(TA // 8, 8, w))
            tie = clk.pacer(0, 6 * TA, 14)
            for t in range(2 * i, 2 * i + 2):
                for r in range(0, HM, 32):
                    k = (t % 2) * 7 + r // 32
                    top = xT_s[r:r + 32, 2 * t * T:(2 * t + 2) * T].astype(f32)
                    bot = xT_s[HM + r:HM + r + 32, 2 * t * T:(2 * t + 2) * T].astype(f32)
                    blocks = [tie(top[:, :T], k), bot[:, :T], top[:, T:], tie(bot[:, T:], k)]
                    _put(xa_s, r, t * 7 * T, _operands(_A_TERMS, blocks))
            return clk

        for cp in cp_b + [x_copy(0)]:
            cp.wait()
        phase1(0)
        x_copy(1).wait()
        clk = phase1(1)
        zero = jnp.zeros((1, 512), f32)
        carry0 = _ssm_scan(u_s.at[:, 0:TC // 8], (zero, zero), lam_s, h_s, clk.pacer(0, 6 * TA, TC // 2))
        for cp in [x_copy(2), x_copy(3)] + cp_c + cp_wq:
            cp.wait()
        _ssm_cmat(craw_s, coef_s, c_s, phase1(2).pacer(0, 6 * TA, M // 16))
        tie = phase1(3).pacer(0, 6 * TA, M // 8)
        for c0 in range(0, M, 8):
            _stage(rq, sq, c0, 8, lambda x: tie(x, c0 // 8), groups=(0,))

        def phase2(i, carry):
            @pl.when(i + NRAW - 1 < NP)
            def _():
                for cp in slice_copies(i + NRAW - 1):
                    cp.start()

            @pl.when(i < 4)
            def _():
                wq1_copy(i).wait()

            for cp in slice_copies(i):
                cp.wait()

            yT = _dot(_get(c_s, 0, M, 0, 2 * M), _get(h_s, 0, TC, 0, 2 * M), _NT)
            for t in range(TC // T):
                cols = _ds(i * TC + t * T, T, T)
                acc = jnp.zeros((8, T), f32)
                for r in range(0, M, 32):
                    xg = xT_s[r:r + 32, cols].astype(f32) * col_s[1, r:r + 32, :]
                    acc = acc + jnp.sum(xg.reshape(4, 8, T), axis=0)
                g = jax.nn.sigmoid(jnp.sum(acc, axis=0, keepdims=True))
                g_s[:, cols] = g
                for r in range(0, M, 32):
                    skip = xT_s[r:r + 32, cols].astype(f32) * col_s[0, r:r + 32, :]
                    o_s[r:r + 32, cols] = (1.0 - g) * (yT[r:r + 32, t * T:(t + 1) * T] + skip)

            ht = lax.shift_right_logical(i, 2)
            words = [sq[ht * 2 + dt, pl.ds(i & 3, M, stride=4), :] for dt in range(2)]
            both = [jnp.concatenate([pltpu.bitcast(w << 16, f32), _hi16(w)], axis=1) for w in words]
            wq = _operands(_B_TERMS, [both[0][:HM], both[1][:HM], both[0][HM:], both[1][HM:]])
            clk = _Clock(zero_s)
            m = [clk.dot(wq[n].astype(bf16),
                         _cat([_get(xa_s, 0, HM, (t * 7 + n) * T, T) for t in range(NP)], 1), _TN)[0]
                 for n in range(7)]
            q_i = q_s.at[_ds(i * 2 * D, 2 * D, 2 * D)]
            for n in (2, 1, 3, 0):
                for t in range(NP):
                    for r in range(0, D, GC):
                        c, = _combine(_Tiles(m, r, GC, t * T, T), (n,), range(7))
                        row = (2 * (r // HD) + n // 2) * D + (n % 2) * HD + r % HD
                        _put(q_i, row, t * T, [c * (LOG2E * D ** -0.5)])

            span = 5 * 1024

            u_next = u_s.at[:, pl.ds(jnp.minimum(i + 1, NP - 1) * (TC // 8), TC // 8)]
            carry = _ssm_scan(u_next, carry, lam_s, h_s, clk.pacer(0, span, TC // 2))

            tie = clk.pacer(0, span, 64)
            rq_i = rq.at[pl.ds((i & 3) * (M // 4), M // 4)]
            sq_i = sq.at[:, _ds((i & 3) * M, M, 8)]
            for c0 in range(0, M // 4, 8):
                _stage(rq_i, sq_i, c0, 8, lambda x: tie(x, c0 // 2 + 2), groups=(1,))
            slot = pl.ds((i & (NRAW - 1)) * CS, CS)
            for n, (raw, stg, wt_s) in enumerate(((rk, sk, wkt_s), (rv, sv, wvt_s))):
                for c0 in range(0, CS, 8):
                    _stage(raw.at[slot], stg, c0, 8, lambda x: tie(x, 16 * n + c0 // 8))
                cols = _ds(i * CS, CS, CS)
                for pair in range(H // 2):
                    for dt in range(2):
                        blk = stg[(pair // 4) * 2 + dt, pl.ds(pair % 4, CS, stride=4), :]
                        row = pair * D + dt * HD
                        wt_s[row:row + HD, cols] = tie(blk, 16 + 24 * n + 3 * pair + dt).T

            tie = clk.pacer(0, span, 28)
            ckv_i = ckv_s.at[lax.shift_right_logical(i, 1), :, i & 1]
            a_i = a_s.at[_ds(i * (T // 4), T // 4, T // 4)]
            for r in range(0, T // 2, 16):
                def block(o, q):
                    col = (o % 2) * 2 * QC + (q % 2) * QC
                    return ckv_i[2 * (q // 2) + o // 2, r:r + 16, col:col + QC].astype(f32)
                for n1 in range(7):
                    ops = _operands2(_A_TERMS, n1, block, lambda x: tie(x, 7 * (r // 16) + n1))
                    _put(a_i, r, 7 * n1 * QC, ops)
            return carry

        lax.fori_loop(0, NP, phase2, carry0)
        cp_wo.wait()
        prep_w(h, range(NT1), _no_tie)

    @pl.when(h == 0)
    def _():
        prologue(**pro_refs)

    def oproj(jp, clk):
        cols = slice(2 * jp * T, (2 * jp + 2) * T)
        for r, n in OCH:
            c = clk.strassen(lambda i: _get(wl_s, r, n, i * T, T),
                             lambda i: _get(cl_s, 0, HD, (jp * 7 + i) * T, T), _NN)()
            o_s[r:r + n, cols] += jnp.concatenate(c[:2], axis=1)
            o_s[HM + r:HM + r + n, cols] += jnp.concatenate(c[2:], axis=1)

    def head(mk_s, mv_s, mp_s, kt_s, ka_s, va_s, v2_s, s_s, pb_s, pd_s, p2_s, sc_s, qb_s):
        clk = _Clock(zero_s)
        q_h = q_s.at[_ds(h * D, D, D)]

        def prep_wo(tie):
            for r in range(0, HM, 16):
                top = tie(wo_s[h, r:r + 16, :].astype(f32), r // 16)
                bot = tie(wo_s[h, HM + r:HM + r + 16, :].astype(f32), r // 16)
                _put(wl_s, r, 0, _operands(_A_TERMS, [top[:, :HD], top[:, HD:], bot[:, :HD], bot[:, HD:]]))

        nine = lambda c: _operands(_A_TERMS, c) + [c[1], c[2]]

        def outer(m_s, r):
            return _combine([m_s[n * HD + r:n * HD + r + 16, :] for n in range(7)], order=range(7))

        def proj(g, lo, hi):
            for n1 in range(lo, hi):
                comb = clk.strassen(lambda n: _get(w_s, 0, 2 * QD, (7 * n1 + n) * QC, QC),
                                    lambda n: _get(a_s, g * T, T, (7 * n1 + n) * QC, QC), _NT, n1 == 6)
                for r in range(0, 2 * QD, GC):
                    m_s, row = mk_s if r < QD else mv_s.at[g % 2], n1 * HD + r % QD
                    c = comb(r, GC)
                    m_s[row:row + GC, :] = jnp.concatenate([c[0], c[2]], axis=1)
                    m_s[QD + row:QD + row + GC, :] = jnp.concatenate([c[1], c[3]], axis=1)
            if hi < 7:
                return
            cs = [outer(mk_s, r) for r in range(0, HD, 16)]
            for n in range(4):
                kt_s[:, n * T:(n + 1) * T] = jnp.concatenate([c[n] for c in cs], axis=0).T
            for r in range(0, 2 * T, GC):
                blk = kt_s[r:r + GC, :]
                _put(ka_s, 2 * g * T + r, 0, nine([blk[:, n * T:(n + 1) * T] for n in range(4)]))

        def vfin(g, tie):
            m_s = mv_s.at[g % 2]
            for r in range(0, QD, 16):
                k, blk = 8 * (r // 16), {}
                late = lambda w: tie(w, k, True, FLAG)
                for new, n1 in (((0,), 2), ((1,), 4), ((3,), 6), ((), 0), ((), 3), ((2,), 5), ((), 1)):
                    for o in new:
                        for i, row in enumerate((r, QD + r)):
                            tiles = _Tiles([m_s.at[n * HD:(n + 1) * HD] for n in range(7)], row, 16)
                            c, = _combine(tiles, ((o % 2) * 2 + o // 2,), range(7))
                            blk[o, i] = c = tie(c, k)
                            slot = (2, 7, 8, 3)[o]
                            _put(va_s, row, ((2 * g + 1) * 9 + slot) * T, [c[:, T:]])
                            if o in (1, 2):
                                _put(va_s, row, (2 * g * 9 + slot) * T, [c[:, :T]])
                    lo_, hi_ = [_operand(_A_TERMS[n1], lambda o: blk[o, i]) for i in range(2)]
                    _put(va_s, r, (2 * g * 9 + n1) * T, [lo_[:, :T]], late)
                    _put(va_s, QD + r, (2 * g * 9 + n1) * T, [hi_[:, :T]], late)
                    if g < 3:
                        _put(v2_s, r, (g * 7 + n1) * 7 * T,
                             _operands(_A_TERMS, [lo_[:, :T], lo_[:, T:], hi_[:, :T], hi_[:, T:]]), late)
                    k += 8 / 7

        key = lax.broadcasted_iota(jnp.int32, (T, 2 * T), 0)
        qry = lax.broadcasted_iota(jnp.int32, (T, 2 * T), 1)
        causal = key <= qry

        def qk(g):
            pairs = (2 * g, 2 * g + 1)
            mx = {jp: _Reducer(jnp.max, jnp.maximum) for jp in pairs}

            def put(jp, row, v):
                v = v.reshape(v.shape[0] // 8, 8, 2 * T)
                s_s[jp % 4, row // 8:row // 8 + v.shape[0]] = v
                mx[jp].add(v)

            def rect(jp, lo, hi, n):
                for r in range(lo, hi, n):
                    c = clk.strassen(lambda i: _get(ka_s, r, n, i * T, T),
                                     lambda i: _get(qb_s, 0, HD, ((jp % 2) * 7 + i) * T, T), _NN)()
                    put(jp, r, jnp.concatenate(c[:2], axis=1))
                    put(jp, jp * T + r, jnp.concatenate(c[2:], axis=1))

            q = lambda jp, e: _get(q_h, e * D, D, jp * T, T)
            for jp in pairs[g == 0:]:
                for r in range(0, HD, 32):
                    blk = [_get(q_h, e * D + d * HD + r, 32, jp * T, T).astype(f32) for d in range(2) for e in range(2)]
                    _put(qb_s, r, (jp % 2) * 7 * T, _operands(_B_TERMS, blk))
            for jp in pairs:
                rect(jp, 0, 2 * g * T, QCH if QCH else g * T // 2 or 1)
            kb = lambda jp, a, b: jnp.concatenate(
                [_get(ka_s, jp * T, T, a * T, T), _get(ka_s, jp * T, T, b * T, T)], axis=1)
            for jp in pairs:
                se, _ = clk.dot(kb(jp, 2, 7), jnp.concatenate([q(jp, 0), q(jp, 1)], axis=1), _NN)
                put(jp, 2 * jp * T, jnp.where(causal, se, NEG))
            last = {}
            for jp in pairs:
                so = jnp.where(causal[:, :T], clk.dot(kb(jp, 8, 3), q(jp, 1), _NN)[0], NEG)
                row = (2 * jp + 1) * T // 8
                s_s[jp % 4, row:row + T // 8, :, T:] = so.reshape(T // 8, 8, T)
                last[jp] = jnp.concatenate([jnp.full((1, T), NEG, f32), jnp.max(so, axis=0, keepdims=True)], axis=1)
            rect(2 * g + 1, 2 * g * T, (2 * g + 1) * T, T // 4)
            return [jnp.broadcast_to(jnp.maximum(mx[jp].result(), last[jp]), (8, 2 * T)) for jp in pairs]

        zs, sums = {}, {}

        def prob(jp, row, z, n=GS, lanes=slice(None)):
            return jnp.exp2(s_s[jp % 4, row // 8:(row + n) // 8, :, lanes] - z[:, lanes])

        def rough(jp, mx, tie):
            zs[jp] = mx
            if jp > 0:
                sm = _Reducer(jnp.sum, jnp.add)
                for k, r in enumerate(range(0, 2 * jp * T, GS * LSUB)):
                    sm.add(prob(jp, r, tie(mx, k)))
                zs[jp] = mx + jnp.log2(jnp.maximum(LSUB * sm.result(), 1.0))
            sums[jp] = _Reducer(jnp.sum, jnp.add)

        def blocks(jp, row, tie, k):
            top, bot = prob(jp, row, tie(zs[jp], k)), prob(jp, jp * T + row, tie(zs[jp], k + 1))
            sums[jp].add(top + bot)
            top, bot = top.reshape(GS, 2 * T), bot.reshape(GS, 2 * T)
            return [top[:, :T], top[:, T:], bot[:, :T], bot[:, T:]]

        def near(jp, tie, k):
            R, z = jp * T, zs[jp]
            if jp % 2:
                for r in range(0, T, GS):
                    _put(pb_s, jp // 2 * T + r, 0, _operands(_B_TERMS, blocks(jp, R - T + r, tie, k)))
                    k += 2
            for r in range(0, T, GS):
                p = prob(jp, 2 * R + r, tie(z, k))
                sums[jp].add(p)
                _put(pd_s, 2 * R + r, 0, [p.reshape(GS, 2 * T)])
                k += 1
            so = _Reducer(jnp.sum, jnp.add)
            for r in range(0, T, 2 * GS):
                p = prob(jp, 2 * R + T + r, tie(z, k), 2 * GS, slice(T, 2 * T))
                so.add(p)
                _put(pd_s, 2 * R + T + r, T, [p.reshape(2 * GS, T)])
                k += 1
            sums[jp].result()
            sums[jp].out = sums[jp].out + jnp.concatenate([jnp.zeros((1, T), f32), so.result()], axis=1)

        p20 = lambda g: g * (g - 1) // 2 * T

        def far(g, tie, k):
            half = {(jp, e): _Reducer(jnp.sum, jnp.add) for jp in (2 * g, 2 * g + 1) for e in range(2)}
            for kg in range(g):
                for r in range(0, T, GS):
                    blk = {}
                    for new, n1 in (((0,), 1), ((1,), 5), ((3,), 2), ((), 0), ((), 4), ((2,), 3), ((), 6)):
                        for o in new:
                            lanes = slice((o % 2) * T, (o % 2 + 1) * T)
                            for jp in (2 * g, 2 * g + 1):
                                z = tie(zs[jp][:, lanes], k)
                                row = (o // 2) * jp * T + 2 * kg * T + r
                                p = [jnp.exp2(s_s[jp % 4, x // 8:(x + GS) // 8, :, lanes] - z) for x in (row, row + T)]
                                half[jp, o % 2].add(p[0] + p[1])
                                blk[o, jp % 2], blk[o, 2 + jp % 2] = [x.reshape(GS, T) for x in p]
                        ops = _operands2(_B_TERMS, n1, lambda o, q: blk[o, q], lambda x: x)
                        _put(p2_s, p20(g) + kg * T + r, 7 * n1 * T, ops,
                             (lambda w: tie(w, k, True, FLAG)) if FTIE else None)
                        k += FW * 8 / 7
            for jp in (2 * g, 2 * g + 1):
                if g:
                    sums[jp].out = sums[jp].out + jnp.concatenate([half[jp, e].result() for e in range(2)], axis=1)
            for jp in (2 * g, 2 * g + 1):
                cols = slice(2 * jp * T, 2 * (jp + 1) * T)
                sc_s[:, cols] = g_s[:, cols] / sums[jp].result()

        def pv(g):
            pairs = (2 * g, 2 * g + 1)
            va = lambda n, t, r=0, nr=HD: _get(va_s, r, nr, (t * 9 + n) * T, T)
            for n1 in range(7 if g else 0):
                c = clk.strassen(
                    lambda n: _cat([_get(v2_s, 0, QD, (kg * 49 + 7 * n1 + n) * T, T) for kg in range(g)], 1),
                    lambda n: _get(p2_s, p20(g), g * T, (7 * n1 + n) * T, T), _NN)()
                mp_s[n1 * HD:n1 * HD + QD, :] = jnp.concatenate(c[:2], axis=1)
                mp_s[n1 * HD + QD:(n1 + 1) * HD, :] = jnp.concatenate(c[2:], axis=1)
            ve = [jnp.concatenate([va(2, jp), va(8, jp)], axis=0) for jp in pairs]
            vo = [jnp.concatenate([va(7, jp), va(3, jp)], axis=0) for jp in pairs]
            ce = clk.level([(ve[jp % 2], _get(pd_s, 2 * jp * T, T, 0, T)) for jp in pairs])
            co = [clk.dot(jnp.concatenate([ve[jp % 2], vo[jp % 2]], axis=1),
                          _get(pd_s, 2 * jp * T, 2 * T, T, T), _NN)[0] for jp in pairs]
            for jp in pairs:
                R, e = jp * T, jp % 2
                ge, go = sc_s[:, 2 * R:2 * R + T], sc_s[:, 2 * R + T:2 * R + 2 * T]
                for r in range(0, HD, 32):
                    c = [ce[e][r:r + 32], co[e][r:r + 32], ce[e][HD + r:HD + r + 32], co[e][HD + r:HD + r + 32]]
                    if g:
                        far_ = _combine([mp_s[n * HD + r:n * HD + r + 32, e * T:(e + 1) * T] for n in range(7)],
                                        order=range(7))
                        c = [x + y for x, y in zip(c, far_)]
                    if e:
                        near_ = clk.strassen(lambda n: va(n, 2 * g, r, 32),
                                             lambda n: _get(pb_s, g * T, T, n * T, T), _NN)()
                        c = [x + y for x, y in zip(c, near_)]
                    ops = _operands(_B_TERMS, [c[0] * ge, c[1] * go, c[2] * ge, c[3] * go])
                    _put(cl_s, r, jp * 7 * T, ops)

        ends = []

        def run(items):
            for item in items.split():
                if item[0] == 'P':
                    pv(int(item[1]))
                    ends.append(clk.t)
                elif item[0] == 'K':
                    proj(int(item[1]), int(item[2]), int(item[3]))
                else:
                    jp = int(item[1])
                    oproj(jp, clk)

                    @pl.when(h == H - 1)
                    def _():
                        out_copy(jp).start()

        for n1 in range(7):
            if n1 >= NT1:
                prep_w(h, [n1], clk.pacer(max(clk.t - LEAD - 448, 1), max(clk.t - LEAD, 1), 8))
            proj(0, n1, n1 + 1)
        oproj(NP - 1, clk)
        mx = qk(0)
        for g in range(4):
            t0 = clk.t
            del ends[:]
            run(PLAN[g])
            t1 = clk.t
            nxt = qk(g + 1) if g < 3 else None
            n_rough = [2 * jp * T // (GS * LSUB) for jp in (2 * g, 2 * g + 1)]
            n_near = [(T + T // 2) // GS, (3 * T + T // 2) // GS]
            holes = [(t - PH0, t + PH1) for t in ends]
            if g < 3:
                vfin(g, clk.pacer(t0 - VB, t0 + VW, 32))
                holes += [(t0, t0 + VW), (t1 - HOLE0, t1 + HOLE1)]
            if g == 2:
                vfin(3, clk.pacer(clk.t - SLACK - VW // 2, clk.t - SLACK, 32))
                holes.append((clk.t - SLACK - VW // 2, clk.t))
            tie = clk.pacer(t0 + D0, (clk.t if g else t1) - SLACK,
                            sum(n_rough) + sum(n_near) + FW * g * 8 * T // GS, holes)
            rough(2 * g, mx[0], tie)
            near(2 * g, tie, n_rough[0])
            k = n_rough[0] + n_near[0]
            rough(2 * g + 1, mx[1], lambda x, i: tie(x, k + i))
            near(2 * g + 1, tie, k + n_rough[1])
            far(g, tie, k + n_rough[1] + n_near[1])
            if g == 0:
                prep_wo(clk.pacer(t0 + VW, t1 - HOLE0, HM // 16))
            mx = nxt
        t0 = clk.t
        run(PLAN[4])
        prep_w(jnp.minimum(h + 1, H - 1), range(NT1), clk.pacer(t0 - PW0, clk.t - 300, 8 * NT1))
        if os.environ.get('SHOW'):
            print('final loads', clk.load)

    head(**head_refs)

    @pl.when(h == H - 1)
    def _():
        oproj(NP - 1, _Clock(zero_s))
        out_copy(NP - 1).start()
        for jp in range(NP):
            out_copy(jp).wait()


@jax.jit
def pallas_gated_mix__compressed_kv_cla__ssm_conv_s5__prompt_kernel(
    A_x: jax.Array,
    A_c_kv: jax.Array,
    A_w_q: jax.Array,
    A_w_uk: jax.Array,
    A_w_uv: jax.Array,
    A_w_o: jax.Array,
    B_x: jax.Array,
    B_Lambda_re: jax.Array,
    B_Lambda_im: jax.Array,
    B_B_re: jax.Array,
    B_B_im: jax.Array,
    B_C_re: jax.Array,
    B_C_im: jax.Array,
    B_log_dt: jax.Array,
    B_Dskip: jax.Array,
    gate_w: jax.Array,
):
    del B_x
    xT = jnp.transpose(A_x[0])
    woT = jnp.transpose(A_w_o, (0, 2, 1))
    ckv = A_c_kv.reshape(4, 4, 2, T // 2, DC)

    hbm = pl.BlockSpec(memory_space=pl.ANY)
    outT = pl.pallas_call(
        _kernel,
        grid=(H,),
        in_specs=[hbm] * 15,
        out_specs=hbm,
        out_shape=jax.ShapeDtypeStruct((M, S), f32),
        scratch_shapes=_SHARED_SCRATCH + list(_PROLOGUE_SCRATCH.values()) + list(_HEAD_SCRATCH.values()),
        compiler_params=pltpu.CompilerParams(
            dimension_semantics=("arbitrary",),
            vmem_limit_bytes=126 * 1024 * 1024,
        ),
    )(xT, B_B_re, B_B_im, B_C_re, B_C_im, B_Lambda_re, B_Lambda_im, B_log_dt,
      B_Dskip, gate_w, woT, ckv, A_w_q, A_w_uk, A_w_uv)
    return jnp.transpose(outT)[None]
```

```python
import bisect
import os

import jax
import jax.numpy as jnp
from jax import lax
import jax.experimental.pallas as pl
import jax.experimental.pallas.tpu as pltpu

S = 2048
M = 448
H = 16
D = 256
DC = 1024
T = 128
NP = S // T // 2
HD = D // 2
HM = M // 2
QD = D // 4
QC = DC // 4
PA = 384
PB = M - PA
TA = 512
TC = 256
CS = DC // NP
NRAW = 4
LOG2E = 1.4426950408889634
NEG = -1e30

_env = lambda k, d: type(d)(os.environ.get(k, d))
GC = _env('GC', 64)
GS = _env('GS', 16)
RCH = _env('RCH', 256)
SLACK = _env('SLACK', 200)
D0 = _env('D0', 0)
NT1 = _env('NT1', 3)
LEAD = _env('LEAD', 448)
PW0 = _env('PW0', 100)
FTIE = _env('FTIE', 1)
YS = _env('YS', 2)
QORD = _env('QORD', 0)
SPAN = _env('SPAN', 6400)
SP0 = _env('SP0', 0)
FLAG = _env('FLAG', 40)
FW = _env('FW', 2)
HOLE0 = _env('HOLE0', 300)
HOLE1 = _env('HOLE1', 300)
VW = _env('VW', 900)
VB = _env('VB', 0)
PH0 = _env('PH0', 500)
PH1 = _env('PH1', 100)
QCH = _env('QCH', 64)
OCH = ((0, 64), (64, 64), (128, 48), (176, 48))
LSUB = _env('LSUB', 4)
PLAN = _env('PLAN', 'K107,K207,K307,P0 P1 O0 O1 P2 O2 O3 O4,P3 O5 O6').split(',')

f32 = jnp.float32
bf16 = jnp.bfloat16
u32 = jnp.uint32

SEM_VEC, SEM_B, SEM_X, SEM_WQ, SEM_C, SEM_SL, SEM_WO, SEM_OUT, SEM_WQ1 = 0, 1, 2, 6, 7, 8, 16, 17, 18
NSEM = 22

_NN = ((1,), (0,))
_NT = ((1,), (1,))
_TN = ((0,), (0,))
_TT = ((0,), (1,))


def _dot(a, b, dims):
    return lax.dot_general(a, b, (dims, ((), ())), preferred_element_type=f32)


def _cat(xs, axis):
    return xs[0] if len(xs) == 1 else jnp.concatenate(xs, axis=axis)


def _ds(lo, n, align):
    return pl.ds(lo if isinstance(lo, int) else pl.multiple_of(lo, align), n)


def _put(ref, row, col, xs, tie=None):
    x = _cat(xs, 1)
    if tie is not None:
        x = jnp.concatenate([tie(x[:8]), x[8:]], axis=0)
    ref[row // 2:(row + x.shape[0]) // 2, col:col + x.shape[1]] = pltpu.bitcast(x.astype(bf16), u32)


def _get(ref, row, nrows, col, ncols):
    return pltpu.bitcast(ref[row // 2:(row + nrows) // 2, col:col + ncols], bf16)


class _Clock:
    def __init__(self, zero_ref):
        self.masks = {(8, T): zero_ref[...] != 0.0}
        self.ticks, self.load = [], [0, 0, 0, 0]

    @property
    def t(self):
        return max(self.load)

    def dot(self, a, b, dims):
        v = _dot(a, b, dims)
        rows, depth = v.shape[0], a.shape[dims[0][0]]
        for c in range(0, v.shape[1], T):
            start = 0
            for _ in range(0, depth, T):
                k = self.load.index(min(self.load))
                start = max(start, self.load[k])
                self.load[k] += rows
            self.ticks += [(start + r + 8, (v, r, c)) for r in range(0, rows, 8)]
        return v, start

    def strassen(self, lhs, rhs, dims, split_last=False):
        jobs = -(-lhs(0).shape[dims[0][0]] // T)
        lag = sum(l + 32 <= max(self.load) for l in self.load) // jobs if jobs < 3 else 0
        order = ((1, 3, 2, 4, 0, 5, 6), (0, 1, 3, 2, 4, 5, 6), (5, 6, 1, 3, 2, 4, 0), (0, 5, 6, 1, 3, 2, 4))[lag]
        m = {}
        for n in order:
            if split_last and n == order[-1]:
                a, half = lhs(n), lhs(0).shape[0] // 2
                m[n] = jnp.concatenate([self.dot(a[:half], rhs(n), dims)[0], self.dot(a[half:], rhs(n), dims)[0]], 0)
            else:
                m[n] = self.dot(lhs(n), rhs(n), dims)[0]
        vals = [m[n] for n in range(7)]
        return lambda r=0, n=None, only=(0, 1, 2, 3), c=0, w=None: _combine(
            vals if n is None else _Tiles(vals, r, n, c, w), only, order)

    def level(self, pairs):
        base, extra = divmod((sum(self.load) + sum(a.shape[0] for a, _ in pairs)) // 16, 4)
        target = [16 * (base + (k < extra)) for k in range(4)]
        out = []
        for a, b in pairs:
            r, parts = 0, []
            while r < a.shape[0]:
                k = self.load.index(min(self.load))
                n = min(max(target[k] - self.load[k], 16), a.shape[0] - r)
                parts.append(self.dot(a[r:r + n], b, _NN)[0])
                r += n
            out.append(_cat(parts, 0))
        return out

    def pacer(self, t0, t1, n, holes=()):
        holes = sorted((max(a, t0), min(b, t1)) for a, b in holes if a < t1 and b > t0)
        gap = sum(b - a for a, b in holes)
        ticks = sorted(self.ticks, key=lambda tw: tw[0])
        times = [tw[0] for tw in ticks]

        def tie(x, k, distinct=False, delay=0):
            t = t0 + (t1 - t0 - gap) * k / n
            for a, b in holes:
                t += b - a if t > a else 0
            t += delay
            past = ticks[:bisect.bisect_right(times, t)]
            if not past:
                return x
            reps = (x.shape[0] // 8, x.shape[1] // T)
            tick = _cat([v[r:r + 8, c:c + T] for _, (v, r, c) in past[-reps[1] if distinct else -1:]], 1)
            if tick.dtype != x.dtype:
                tick = pltpu.bitcast(tick, x.dtype)
            if x.shape not in self.masks:
                self.masks[x.shape] = jnp.tile(self.masks[(8, T)], reps)
            return lax.select(self.masks[x.shape], tick if tick.shape == x.shape else jnp.tile(tick, reps), x)
        return tie


def _no_tie(x, k):
    return x


_A_TERMS = ((0, 3, 1), (2, 3, 1), (0, None, 0), (3, None, 0), (0, 1, 1), (2, 0, -1), (1, 3, -1))
_B_TERMS = ((0, 3, 1), (0, None, 0), (1, 3, -1), (2, 0, -1), (3, None, 0), (0, 1, 1), (2, 3, 1))


def _operand(term, block):
    x, y, sign = term
    if y is None:
        return block(x)
    return block(x) + block(y) if sign > 0 else block(x) - block(y)


def _operands(terms, blocks):
    return [_operand(t, blocks.__getitem__) for t in terms]


def _operands2(terms, n1, block, tie):
    first = terms[n1][0]
    sub = [_operand(terms[n1], lambda o: tie(block(o, q)) if o == first and q in (0, 3) else block(o, q))
           for q in range(4)]
    return _operands(terms, sub)


_C_TERMS = ({0: 1, 3: 1, 4: -1, 6: 1}, {2: 1, 4: 1}, {1: 1, 3: 1}, {0: 1, 1: -1, 2: 1, 5: 1})


def _combine(m, only=(0, 1, 2, 3), order=(1, 3, 2, 4, 0, 5, 6)):
    out = []
    for terms in (_C_TERMS[n] for n in only):
        seq = [n for n in order if n in terms]
        if terms[seq[0]] < 0:
            seq[0], seq[1] = seq[1], seq[0]
        acc = m[seq[0]]
        for n in seq[1:]:
            acc = acc + m[n] if terms[n] > 0 else acc - m[n]
        out.append(acc)
    return out


class _Tiles:
    def __init__(self, vals, r, n, c=0, w=None):
        self.vals, self.idx, self.cache = vals, (slice(r, r + n), slice(c, None if w is None else c + w)), {}

    def __getitem__(self, i):
        if i not in self.cache:
            self.cache[i] = self.vals[i][self.idx]
        return self.cache[i]


class _Reducer:
    def __init__(self, red, comb):
        self.red, self.comb, self.acc, self.rows, self.out = red, comb, None, 0, None

    def add(self, v):
        self.rows += 8 * v.shape[0]
        v = self.red(v, axis=0)
        self.acc = v if self.acc is None else self.comb(self.acc, v)
        if self.rows >= RCH:
            self.result()

    def result(self):
        if self.acc is not None:
            v = self.red(self.acc, axis=0, keepdims=True)
            self.out = v if self.out is None else self.comb(self.out, v)
        self.acc, self.rows = None, 0
        return self.out


def _cmul(ar, ai, br, bi):
    return ar * br - ai * bi, ar * bi + ai * br


def _hi16(w):
    return pltpu.bitcast(w & jnp.uint32(0xFFFF0000), f32)


def _stage(raw, stg, c0, nc, tie, groups=(0, 1)):
    for ht in groups:
        for dt in range(2):
            v = raw[c0:c0 + nc, ht * 8:(ht + 1) * 8, dt * T:(dt + 1) * T].reshape(nc * 8, T)
            stg[ht * 2 + dt, c0 * 4:(c0 + nc) * 4, :] = tie(pltpu.bitcast(v, u32))


def _ssm_params(vec_s, coef_s, lam_s, col_s):
    row = lambda r: r[...].astype(f32).reshape(1, M)
    lre, lim, ldt, dsk, gw = [row(v) for v in vec_s]
    dt = jnp.exp(ldt).astype(bf16).astype(f32)
    mag = jnp.exp(dt * lre)
    ang = dt * lim
    lr, li = mag * jnp.cos(ang), mag * jnp.sin(ang)
    den = lre * lre + lim * lim
    nr = lr - 1.0
    coef_s[...] = jnp.zeros(coef_s.shape, f32)
    coef_s[0:1, 0:M] = 2.0 * ((nr * lre + li * lim) / den)
    coef_s[1:2, 0:M] = 2.0 * ((li * lre - nr * lim) / den)

    er = jnp.concatenate([lr, lr[:, PA:]], axis=1)
    ei = jnp.concatenate([li, -li[:, PA:]], axis=1)
    pw = [(er, ei)]
    for _ in range(7):
        pw.append(_cmul(pw[-1][0], pw[-1][1], er, ei))
    sub = lax.broadcasted_iota(jnp.int32, (8, 512), 0)
    for n, d in enumerate((1, 2, 4)):
        lam_s[2 * n] = jnp.where(sub >= d, pw[d - 1][0], 0.0)
        lam_s[2 * n + 1] = jnp.where(sub >= d, pw[d - 1][1], 0.0)
    lcr = jnp.zeros((8, 512), f32)
    lci = jnp.zeros((8, 512), f32)
    for r in range(8):
        lcr = jnp.where(sub == r, pw[r][0], lcr)
        lci = jnp.where(sub == r, pw[r][1], lci)
    lam_s[6] = lcr
    lam_s[7] = lci

    def col(v):
        v = jnp.concatenate([v, jnp.zeros((1, 512 - M), f32)], axis=1)
        return jnp.broadcast_to(v, (T, 512)).T[:M]
    col_s[0] = col(dsk)
    col_s[1] = col(gw)


def _ssm_cmat(craw_s, coef_s, c_s, tie):
    for r in range(0, M, 16):
        coef = tie(coef_s[...], r // 16)
        cr, ci = coef[0:1, :M], coef[1:2, :M]
        re, im = _cmul(craw_s[0, r:r + 16, :].astype(f32), craw_s[1, r:r + 16, :].astype(f32), cr, ci)
        _put(c_s, r, 0, [re[:, :PA], -im[:, :PA], re[:, PA:], -im[:, PA:]])


def _ssm_scan(u_ref, carry, lam_s, h_s, tie):
    car, cai = carry
    out = []
    for b in range(TC // 8):
        mixed = u_ref[3, b, :, 0:T]
        u = jnp.concatenate([u_ref[cb, b] for cb in range(3)], axis=1)
        cols = [u[:, 0:T], u[:, T:2 * T], u[:, 2 * T:PA], mixed]
        hr = jnp.concatenate([tie(v, 4 * b + n) for n, v in enumerate(cols)], axis=1)
        hi = jnp.concatenate([u[:, PA:2 * PA], pltpu.roll(mixed, PB, 1)], axis=1)
        for n, d in enumerate((1, 2, 4)):
            sr, si = pltpu.roll(hr, d, 0), pltpu.roll(hi, d, 0)
            tr, ti = _cmul(sr, si, lam_s[2 * n], lam_s[2 * n + 1])
            hr, hi = hr + tr, hi + ti
        tr, ti = _cmul(lam_s[6], lam_s[7], car, cai)
        hr, hi = hr + tr, hi + ti
        car, cai = hr[7:8, :], hi[7:8, :]
        out.append(jnp.concatenate([hr[:, :PA], hi[:, :PA], hr[:, PA:]], axis=1))
        if b % 2 == 1:
            _put(h_s, (b - 1) * 8, 0, [jnp.concatenate(out, axis=0)])
            out = []
    return car, cai


_vmem = pltpu.VMEM
_PROLOGUE_SCRATCH = dict(
    xT_s=_vmem((M, S), bf16),
    v0=_vmem((M,), bf16), v1=_vmem((M,), bf16), v2=_vmem((M,), bf16), v3=_vmem((M,), bf16), v4=_vmem((M,), bf16),
    b_s=_vmem((2 * M, M), bf16),
    craw_s=_vmem((2, M, M), bf16),
    c_s=_vmem((M // 2, 2 * M), u32),
    coef_s=_vmem((8, 512), f32),
    lam_s=_vmem((8, 8, 512), f32),
    col_s=_vmem((2, M, T), f32),
    h_s=_vmem((TC // 2, 2 * M), u32),
    ckv_s=_vmem((4, 4, 2, T // 2, DC), bf16),
    rq=_vmem((M, H, D), bf16),
    rk=_vmem((NRAW * CS, H, D), bf16),
    rv=_vmem((NRAW * CS, H, D), bf16),
    sq=_vmem((4, M * 4, T), u32),
    sk=_vmem((4, CS * 4, T), u32),
    sv=_vmem((4, CS * 4, T), u32),
    xa_s=_vmem((HM // 2, NP * 7 * T), u32),
)
_HEAD_SCRATCH = dict(
    mk_s=_vmem((7 * HD, 2 * T), f32),
    mv_s=_vmem((2, 7 * HD, 2 * T), f32),
    mp_s=_vmem((7 * HD, 2 * T), f32),
    kt_s=_vmem((2 * T, 4 * T), f32),
    ka_s=_vmem((S // 4, 9 * T), u32),
    va_s=_vmem((HD // 2, NP * 9 * T), u32),
    v2_s=_vmem((QD // 2, 3 * 49 * T), u32),
    s_s=_vmem((4, S // 8, 8, 2 * T), f32),
    pb_s=_vmem((2 * T, 7 * T), u32),
    pd_s=_vmem((S // 2, 2 * T), u32),
    p2_s=_vmem((3 * T, 49 * T), u32),
    sc_s=_vmem((1, S), f32),
    qb_s=_vmem((HD // 2, 14 * T), u32),
)
_SHARED_SCRATCH = [
    _vmem((H // 2 * D, DC), u32),
    _vmem((H // 2 * D, DC), u32),
    _vmem((S // 8, 49 * QC), u32),
    _vmem((H * D, S // 2), u32),
    _vmem((H, M, D), bf16),
    _vmem((QD, 49 * QC), u32),
    _vmem((HM // 2, 7 * T), u32),
    _vmem((HD // 2, NP * 7 * T), u32),
    _vmem((M, S), f32),
    _vmem((1, S), f32),
    _vmem((8, T), f32),
    pltpu.SemaphoreType.DMA((NSEM,)),
]


def _kernel(xT_hbm, bre_hbm, bim_hbm, cre_hbm, cim_hbm, lre_hbm, lim_hbm, ldt_hbm,
            dsk_hbm, gw_hbm, woT_hbm, ckv_hbm, wq_hbm, wk_hbm, wv_hbm,
            out_hbm,
            wkt_s, wvt_s, a_s, q_s, wo_s, w_s, wl_s, cl_s, o_s, g_s, zero_s, sem, *rest):
    h = pl.program_id(0)
    pro_refs = dict(zip(_PROLOGUE_SCRATCH, rest))
    head_refs = dict(zip(_HEAD_SCRATCH, rest[len(pro_refs):]))

    def out_copy(jp):
        cols = pl.ds(jp * 2 * T, 2 * T)
        return pltpu.make_async_copy(o_s.at[:, cols], out_hbm.at[:, cols], sem.at[SEM_OUT])

    def prep_w(hh, outer, tie):
        rows = _ds(lax.shift_right_logical(hh, 1) * D, D, D)
        sh = (16 * (1 - (hh & 1))).astype(u32)
        k = 0
        for row0, wt_s in ((0, wkt_s.at[rows]), (QD, wvt_s.at[rows])):
            for r in range(0, QD, 16):
                def block(o, q):
                    row = (o % 2) * HD + (q % 2) * QD + r
                    col = (o // 2) * 2 * QC + (q // 2) * QC
                    return _hi16(wt_s[row:row + 16, col:col + QC] << sh)
                for n1 in outer:
                    _put(w_s, row0 + r, 7 * n1 * QC, _operands2(_B_TERMS, n1, block, lambda x: tie(x, k)))
                    k += 1

    def prologue(xT_s, v0, v1, v2, v3, v4, b_s, craw_s, c_s, coef_s, lam_s, col_s, h_s,
                 ckv_s, rq, rk, rv, sq, sk, sv, xa_s):
        u_s = head_refs['s_s']
        vec_s = (v0, v1, v2, v3, v4)

        def slice_copies(i):
            s = sem.at[SEM_SL + i]
            grp = i // 2 if isinstance(i, int) else lax.shift_right_logical(i, 1)
            cs, dst = pl.ds(i * CS, CS), pl.ds((i & (NRAW - 1)) * CS, CS)
            return [pltpu.make_async_copy(ckv_hbm.at[grp, :, i & 1], ckv_s.at[grp, :, i & 1], s),
                    pltpu.make_async_copy(wk_hbm.at[cs], rk.at[dst], s),
                    pltpu.make_async_copy(wv_hbm.at[cs], rv.at[dst], s)]

        def wq1_copy(i):
            rows = pl.ds(i * (M // 4), M // 4)
            return pltpu.make_async_copy(wq_hbm.at[rows, 8:16], rq.at[rows, 8:16], sem.at[SEM_WQ1 + i])

        def x_copy(i):
            cols = pl.ds(i * TA, TA)
            return pltpu.make_async_copy(xT_hbm.at[:, cols], xT_s.at[:, cols], sem.at[SEM_X + i])

        cp_vec = [pltpu.make_async_copy(src, dst, sem.at[SEM_VEC])
                  for src, dst in zip((lre_hbm, lim_hbm, ldt_hbm, dsk_hbm, gw_hbm), vec_s)]
        cp_b = [pltpu.make_async_copy(src.at[pl.ds(lo, n)], b_s.at[pl.ds(dst, n)], sem.at[SEM_B])
                for src, lo, n, dst in ((bre_hbm, 0, PA, 0), (bim_hbm, 0, PA, PA),
                                        (bre_hbm, PA, PB, 2 * PA), (bim_hbm, PA, PB, 2 * PA + PB))]
        cp_wq = [pltpu.make_async_copy(wq_hbm.at[:, 0:8], rq.at[:, 0:8], sem.at[SEM_WQ])]
        cp_c = [pltpu.make_async_copy(src, craw_s.at[n], sem.at[SEM_C])
                for n, src in enumerate((cre_hbm, cim_hbm))]
        cp_wo = pltpu.make_async_copy(woT_hbm, wo_s, sem.at[SEM_WO])
        for cp in cp_vec + cp_b + [x_copy(i) for i in range(S // TA)] + cp_c + cp_wq:
            cp.start()
        for i in range(NRAW - 1):
            for cp in [wq1_copy(i)] + slice_copies(i):
                cp.start()
        wq1_copy(3).start()
        cp_wo.start()

        zero_s[...] = jnp.zeros(zero_s.shape, f32)
        wl_s[...] = jnp.zeros(wl_s.shape, u32)
        cl_s[:, (NP - 1) * 7 * T:] = jnp.zeros((HD // 2, 7 * T), u32)
        for cp in cp_vec:
            cp.wait()
        _ssm_params(vec_s, coef_s, lam_s, col_s)

        def phase1(i):
            clk = _Clock(zero_s)
            u, _ = clk.dot(xT_s[:, i * TA:(i + 1) * TA], b_s[...], _TT)
            for cb in range(4):
                w = min(2 * T, 2 * M - cb * 2 * T)
                u_s[cb, i * TA // 8:(i + 1) * TA // 8, :, 0:w] = (
                    u[:, cb * 2 * T:cb * 2 * T + w].reshape(TA // 8, 8, w))
            tie = clk.pacer(0, 6 * TA, 14)
            for t in range(2 * i, 2 * i + 2):
                for r in range(0, HM, 32):
                    k = (t % 2) * 7 + r // 32
                    top = xT_s[r:r + 32, 2 * t * T:(2 * t + 2) * T].astype(f32)
                    bot = xT_s[HM + r:HM + r + 32, 2 * t * T:(2 * t + 2) * T].astype(f32)
                    blocks = [tie(top[:, :T], k), bot[:, :T], top[:, T:], tie(bot[:, T:], k)]
                    _put(xa_s, r, t * 7 * T, _operands(_A_TERMS, blocks))
            return clk

        for cp in cp_b + [x_copy(0)]:
            cp.wait()
        phase1(0)
        x_copy(1).wait()
        clk = phase1(1)
        zero = jnp.zeros((1, 512), f32)
        carry0 = _ssm_scan(u_s.at[:, 0:TC // 8], (zero, zero), lam_s, h_s, clk.pacer(0, 6 * TA, TC // 2))
        for cp in [x_copy(2), x_copy(3)] + cp_c + cp_wq:
            cp.wait()
        _ssm_cmat(craw_s, coef_s, c_s, phase1(2).pacer(0, 6 * TA, M // 16))
        tie = phase1(3).pacer(0, 6 * TA, M // 8)
        for c0 in range(0, M, 8):
            _stage(rq, sq, c0, 8, lambda x: tie(x, c0 // 8), groups=(0,))

        def phase2(i, carry):
            @pl.when(i + NRAW - 1 < NP)
            def _():
                for cp in slice_copies(i + NRAW - 1):
                    cp.start()

            @pl.when(i < 4)
            def _():
                wq1_copy(i).wait()

            for cp in slice_copies(i):
                cp.wait()

            clk = _Clock(zero_s)
            yT = _cat([clk.dot(_get(c_s, r, M // YS, 0, 2 * M), _get(h_s, 0, TC, 0, 2 * M), _NT)[0]
                       for r in range(0, M, M // YS)], 0)
            ty = clk.t
            for t in range(TC // T):
                cols = _ds(i * TC + t * T, T, T)
                acc = jnp.zeros((8, T), f32)
                for r in range(0, M, 32):
                    xg = xT_s[r:r + 32, cols].astype(f32) * col_s[1, r:r + 32, :]
                    acc = acc + jnp.sum(xg.reshape(4, 8, T), axis=0)
                g = jax.nn.sigmoid(jnp.sum(acc, axis=0, keepdims=True))
                g_s[:, cols] = g
                for r in range(0, M, 32):
                    skip = xT_s[r:r + 32, cols].astype(f32) * col_s[0, r:r + 32, :]
                    o_s[r:r + 32, cols] = (1.0 - g) * (yT[r:r + 32, t * T:(t + 1) * T] + skip)

            ht = lax.shift_right_logical(i, 2)
            words = [sq[ht * 2 + dt, pl.ds(i & 3, M, stride=4), :] for dt in range(2)]
            both = [jnp.concatenate([pltpu.bitcast(w << 16, f32), _hi16(w)], axis=1) for w in words]
            wq = _operands(_B_TERMS, [both[0][:HM], both[1][:HM], both[0][HM:], both[1][HM:]])
            order = (1, 3, 2, 4, 0, 5, 6) if QORD else range(7)
            m = {n: clk.dot(wq[n].astype(bf16),
                            _cat([_get(xa_s, 0, HM, (t * 7 + n) * T, T) for t in range(NP)], 1), _TN)[0]
                 for n in order}
            q_i = q_s.at[_ds(i * 2 * D, 2 * D, 2 * D)]
            for n in (2, 1, 3, 0):
                for t in range(NP):
                    for r in range(0, D, GC):
                        c, = _combine(_Tiles(m, r, GC, t * T, T), (n,), order)
                        row = (2 * (r // HD) + n // 2) * D + (n % 2) * HD + r % HD
                        _put(q_i, row, t * T, [c * (LOG2E * D ** -0.5)])

            span = ty + SPAN

            u_next = u_s.at[:, pl.ds(jnp.minimum(i + 1, NP - 1) * (TC // 8), TC // 8)]
            carry = _ssm_scan(u_next, carry, lam_s, h_s, clk.pacer(ty, span, TC // 2))

            tie = clk.pacer(ty - SP0, span, 64)
            rq_i = rq.at[pl.ds((i & 3) * (M // 4), M // 4)]
            sq_i = sq.at[:, _ds((i & 3) * M, M, 8)]
            for c0 in range(0, M // 4, 8):
                _stage(rq_i, sq_i, c0, 8, lambda x: tie(x, c0 // 2 + 2), groups=(1,))
            slot = pl.ds((i & (NRAW - 1)) * CS, CS)
            for n, (raw, stg, wt_s) in enumerate(((rk, sk, wkt_s), (rv, sv, wvt_s))):
                for c0 in range(0, CS, 8):
                    _stage(raw.at[slot], stg, c0, 8, lambda x: tie(x, 16 * n + c0 // 8))
                cols = _ds(i * CS, CS, CS)
                for pair in range(H // 2):
                    for dt in range(2):
                        blk = stg[(pair // 4) * 2 + dt, pl.ds(pair % 4, CS, stride=4), :]
                        row = pair * D + dt * HD
                        wt_s[row:row + HD, cols] = tie(blk, 16 + 24 * n + 3 * pair + dt).T

            tie = clk.pacer(ty - SP0, span, 28)
            ckv_i = ckv_s.at[lax.shift_right_logical(i, 1), :, i & 1]
            a_i = a_s.at[_ds(i * (T // 4), T // 4, T // 4)]
            for r in range(0, T // 2, 16):
                def block(o, q):
                    col = (o % 2) * 2 * QC + (q % 2) * QC
                    return ckv_i[2 * (q // 2) + o // 2, r:r + 16, col:col + QC].astype(f32)
                for n1 in range(7):
                    ops = _operands2(_A_TERMS, n1, block, lambda x: tie(x, 7 * (r // 16) + n1))
                    _put(a_i, r, 7 * n1 * QC, ops)
            return carry

        lax.fori_loop(0, NP, phase2, carry0)
        cp_wo.wait()
        prep_w(h, range(NT1), _no_tie)

    @pl.when(h == 0)
    def _():
        prologue(**pro_refs)

    def oproj(jp, clk):
        cols = slice(2 * jp * T, (2 * jp + 2) * T)
        for r, n in OCH:
            c = clk.strassen(lambda i: _get(wl_s, r, n, i * T, T),
                             lambda i: _get(cl_s, 0, HD, (jp * 7 + i) * T, T), _NN)()
            o_s[r:r + n, cols] += jnp.concatenate(c[:2], axis=1)
            o_s[HM + r:HM + r + n, cols] += jnp.concatenate(c[2:], axis=1)

    def head(mk_s, mv_s, mp_s, kt_s, ka_s, va_s, v2_s, s_s, pb_s, pd_s, p2_s, sc_s, qb_s):
        clk = _Clock(zero_s)
        q_h = q_s.at[_ds(h * D, D, D)]

        def prep_wo(tie):
            for r in range(0, HM, 16):
                top = tie(wo_s[h, r:r + 16, :].astype(f32), r // 16)
                bot = tie(wo_s[h, HM + r:HM + r + 16, :].astype(f32), r // 16)
                _put(wl_s, r, 0, _operands(_A_TERMS, [top[:, :HD], top[:, HD:], bot[:, :HD], bot[:, HD:]]))

        nine = lambda c: _operands(_A_TERMS, c) + [c[1], c[2]]

        def outer(m_s, r):
            return _combine([m_s[n * HD + r:n * HD + r + 16, :] for n in range(7)], order=range(7))

        def proj(g, lo, hi):
            for n1 in range(lo, hi):
                comb = clk.strassen(lambda n: _get(w_s, 0, 2 * QD, (7 * n1 + n) * QC, QC),
                                    lambda n: _get(a_s, g * T, T, (7 * n1 + n) * QC, QC), _NT, n1 == 6)
                for r in range(0, 2 * QD, GC):
                    m_s, row = mk_s if r < QD else mv_s.at[g % 2], n1 * HD + r % QD
                    c = comb(r, GC)
                    m_s[row:row + GC, :] = jnp.concatenate([c[0], c[2]], axis=1)
                    m_s[QD + row:QD + row + GC, :] = jnp.concatenate([c[1], c[3]], axis=1)
            if hi < 7:
                return
            cs = [outer(mk_s, r) for r in range(0, HD, 16)]
            for n in range(4):
                kt_s[:, n * T:(n + 1) * T] = jnp.concatenate([c[n] for c in cs], axis=0).T
            for r in range(0, 2 * T, GC):
                blk = kt_s[r:r + GC, :]
                _put(ka_s, 2 * g * T + r, 0, nine([blk[:, n * T:(n + 1) * T] for n in range(4)]))

        def vfin(g, tie):
            m_s = mv_s.at[g % 2]
            for r in range(0, QD, 16):
                k, blk = 8 * (r // 16), {}
                late = lambda w: tie(w, k, True, FLAG)
                for new, n1 in (((0,), 2), ((1,), 4), ((3,), 6), ((), 0), ((), 3), ((2,), 5), ((), 1)):
                    for o in new:
                        for i, row in enumerate((r, QD + r)):
                            tiles = _Tiles([m_s.at[n * HD:(n + 1) * HD] for n in range(7)], row, 16)
                            c, = _combine(tiles, ((o % 2) * 2 + o // 2,), range(7))
                            blk[o, i] = c = tie(c, k)
                            slot = (2, 7, 8, 3)[o]
                            _put(va_s, row, ((2 * g + 1) * 9 + slot) * T, [c[:, T:]])
                            if o in (1, 2):
                                _put(va_s, row, (2 * g * 9 + slot) * T, [c[:, :T]])
                    lo_, hi_ = [_operand(_A_TERMS[n1], lambda o: blk[o, i]) for i in range(2)]
                    _put(va_s, r, (2 * g * 9 + n1) * T, [lo_[:, :T]], late)
                    _put(va_s, QD + r, (2 * g * 9 + n1) * T, [hi_[:, :T]], late)
                    if g < 3:
                        _put(v2_s, r, (g * 7 + n1) * 7 * T,
                             _operands(_A_TERMS, [lo_[:, :T], lo_[:, T:], hi_[:, :T], hi_[:, T:]]), late)
                    k += 8 / 7

        key = lax.broadcasted_iota(jnp.int32, (T, 2 * T), 0)
        qry = lax.broadcasted_iota(jnp.int32, (T, 2 * T), 1)
        causal = key <= qry

        def qk(g):
            pairs = (2 * g, 2 * g + 1)
            mx = {jp: _Reducer(jnp.max, jnp.maximum) for jp in pairs}

            def put(jp, row, v):
                v = v.reshape(v.shape[0] // 8, 8, 2 * T)
                s_s[jp % 4, row // 8:row // 8 + v.shape[0]] = v
                mx[jp].add(v)

            def rect(jp, lo, hi, n):
                for r in range(lo, hi, n):
                    c = clk.strassen(lambda i: _get(ka_s, r, n, i * T, T),
                                     lambda i: _get(qb_s, 0, HD, ((jp % 2) * 7 + i) * T, T), _NN)()
                    put(jp, r, jnp.concatenate(c[:2], axis=1))
                    put(jp, jp * T + r, jnp.concatenate(c[2:], axis=1))

            q = lambda jp, e: _get(q_h, e * D, D, jp * T, T)
            for jp in pairs[g == 0:]:
                for r in range(0, HD, 32):
                    blk = [_get(q_h, e * D + d * HD + r, 32, jp * T, T).astype(f32) for d in range(2) for e in range(2)]
                    _put(qb_s, r, (jp % 2) * 7 * T, _operands(_B_TERMS, blk))
            for jp in pairs:
                rect(jp, 0, 2 * g * T, QCH if QCH else g * T // 2 or 1)
            kb = lambda jp, a, b: jnp.concatenate(
                [_get(ka_s, jp * T, T, a * T, T), _get(ka_s, jp * T, T, b * T, T)], axis=1)
            for jp in pairs:
                se, _ = clk.dot(kb(jp, 2, 7), jnp.concatenate([q(jp, 0), q(jp, 1)], axis=1), _NN)
                put(jp, 2 * jp * T, jnp.where(causal, se, NEG))
            last = {}
            for jp in pairs:
                so = jnp.where(causal[:, :T], clk.dot(kb(jp, 8, 3), q(jp, 1), _NN)[0], NEG)
                row = (2 * jp + 1) * T // 8
                s_s[jp % 4, row:row + T // 8, :, T:] = so.reshape(T // 8, 8, T)
                last[jp] = jnp.concatenate([jnp.full((1, T), NEG, f32), jnp.max(so, axis=0, keepdims=True)], axis=1)
            rect(2 * g + 1, 2 * g * T, (2 * g + 1) * T, T // 4)
            return [jnp.broadcast_to(jnp.maximum(mx[jp].result(), last[jp]), (8, 2 * T)) for jp in pairs]

        zs, sums = {}, {}

        def prob(jp, row, z, n=GS, lanes=slice(None)):
            return jnp.exp2(s_s[jp % 4, row // 8:(row + n) // 8, :, lanes] - z[:, lanes])

        def rough(jp, mx, tie):
            zs[jp] = mx
            if jp > 0:
                sm = _Reducer(jnp.sum, jnp.add)
                for k, r in enumerate(range(0, 2 * jp * T, GS * LSUB)):
                    sm.add(prob(jp, r, tie(mx, k)))
                zs[jp] = mx + jnp.log2(jnp.maximum(LSUB * sm.result(), 1.0))
            sums[jp] = _Reducer(jnp.sum, jnp.add)

        def blocks(jp, row, tie, k):
            top, bot = prob(jp, row, tie(zs[jp], k)), prob(jp, jp * T + row, tie(zs[jp], k + 1))
            sums[jp].add(top + bot)
            top, bot = top.reshape(GS, 2 * T), bot.reshape(GS, 2 * T)
            return [top[:, :T], top[:, T:], bot[:, :T], bot[:, T:]]

        def near(jp, tie, k):
            R, z = jp * T, zs[jp]
            if jp % 2:
                for r in range(0, T, GS):
                    _put(pb_s, jp // 2 * T + r, 0, _operands(_B_TERMS, blocks(jp, R - T + r, tie, k)))
                    k += 2
            for r in range(0, T, GS):
                p = prob(jp, 2 * R + r, tie(z, k))
                sums[jp].add(p)
                _put(pd_s, 2 * R + r, 0, [p.reshape(GS, 2 * T)])
                k += 1
            so = _Reducer(jnp.sum, jnp.add)
            for r in range(0, T, 2 * GS):
                p = prob(jp, 2 * R + T + r, tie(z, k), 2 * GS, slice(T, 2 * T))
                so.add(p)
                _put(pd_s, 2 * R + T + r, T, [p.reshape(2 * GS, T)])
                k += 1
            sums[jp].result()
            sums[jp].out = sums[jp].out + jnp.concatenate([jnp.zeros((1, T), f32), so.result()], axis=1)

        p20 = lambda g: g * (g - 1) // 2 * T

        def far(g, tie, k):
            half = {(jp, e): _Reducer(jnp.sum, jnp.add) for jp in (2 * g, 2 * g + 1) for e in range(2)}
            for kg in range(g):
                for r in range(0, T, GS):
                    blk = {}
                    for new, n1 in (((0,), 1), ((1,), 5), ((3,), 2), ((), 0), ((), 4), ((2,), 3), ((), 6)):
                        for o in new:
                            lanes = slice((o % 2) * T, (o % 2 + 1) * T)
                            for jp in (2 * g, 2 * g + 1):
                                z = tie(zs[jp][:, lanes], k)
                                row = (o // 2) * jp * T + 2 * kg * T + r
                                p = [jnp.exp2(s_s[jp % 4, x // 8:(x + GS) // 8, :, lanes] - z) for x in (row, row + T)]
                                half[jp, o % 2].add(p[0] + p[1])
                                blk[o, jp % 2], blk[o, 2 + jp % 2] = [x.reshape(GS, T) for x in p]
                        ops = _operands2(_B_TERMS, n1, lambda o, q: blk[o, q], lambda x: x)
                        _put(p2_s, p20(g) + kg * T + r, 7 * n1 * T, ops,
                             (lambda w: tie(w, k, True, FLAG)) if FTIE else None)
                        k += FW * 8 / 7
            for jp in (2 * g, 2 * g + 1):
                if g:
                    sums[jp].out = sums[jp].out + jnp.concatenate([half[jp, e].result() for e in range(2)], axis=1)
            for jp in (2 * g, 2 * g + 1):
                cols = slice(2 * jp * T, 2 * (jp + 1) * T)
                sc_s[:, cols] = g_s[:, cols] / sums[jp].result()

        def pv(g):
            pairs = (2 * g, 2 * g + 1)
            va = lambda n, t, r=0, nr=HD: _get(va_s, r, nr, (t * 9 + n) * T, T)
            for n1 in range(7 if g else 0):
                c = clk.strassen(
                    lambda n: _cat([_get(v2_s, 0, QD, (kg * 49 + 7 * n1 + n) * T, T) for kg in range(g)], 1),
                    lambda n: _get(p2_s, p20(g), g * T, (7 * n1 + n) * T, T), _NN)()
                mp_s[n1 * HD:n1 * HD + QD, :] = jnp.concatenate(c[:2], axis=1)
                mp_s[n1 * HD + QD:(n1 + 1) * HD, :] = jnp.concatenate(c[2:], axis=1)
            ve = [jnp.concatenate([va(2, jp), va(8, jp)], axis=0) for jp in pairs]
            vo = [jnp.concatenate([va(7, jp), va(3, jp)], axis=0) for jp in pairs]
            ce = clk.level([(ve[jp % 2], _get(pd_s, 2 * jp * T, T, 0, T)) for jp in pairs])
            co = [clk.dot(jnp.concatenate([ve[jp % 2], vo[jp % 2]], axis=1),
                          _get(pd_s, 2 * jp * T, 2 * T, T, T), _NN)[0] for jp in pairs]
            for jp in pairs:
                R, e = jp * T, jp % 2
                ge, go = sc_s[:, 2 * R:2 * R + T], sc_s[:, 2 * R + T:2 * R + 2 * T]
                for r in range(0, HD, 32):
                    c = [ce[e][r:r + 32], co[e][r:r + 32], ce[e][HD + r:HD + r + 32], co[e][HD + r:HD + r + 32]]
                    if g:
                        far_ = _combine([mp_s[n * HD + r:n * HD + r + 32, e * T:(e + 1) * T] for n in range(7)],
                                        order=range(7))
                        c = [x + y for x, y in zip(c, far_)]
                    if e:
                        near_ = clk.strassen(lambda n: va(n, 2 * g, r, 32),
                                             lambda n: _get(pb_s, g * T, T, n * T, T), _NN)()
                        c = [x + y for x, y in zip(c, near_)]
                    ops = _operands(_B_TERMS, [c[0] * ge, c[1] * go, c[2] * ge, c[3] * go])
                    _put(cl_s, r, jp * 7 * T, ops)

        ends = []

        def run(items):
            for item in items.split():
                if item[0] == 'P':
                    pv(int(item[1]))
                    ends.append(clk.t)
                elif item[0] == 'K':
                    proj(int(item[1]), int(item[2]), int(item[3]))
                else:
                    jp = int(item[1])
                    oproj(jp, clk)

                    @pl.when(h == H - 1)
                    def _():
                        out_copy(jp).start()

        for n1 in range(7):
            if n1 >= NT1:
                prep_w(h, [n1], clk.pacer(max(clk.t - LEAD - 448, 1), max(clk.t - LEAD, 1), 8))
            proj(0, n1, n1 + 1)
        oproj(NP - 1, clk)
        mx = qk(0)
        for g in range(4):
            t0 = clk.t
            del ends[:]
            run(PLAN[g])
            t1 = clk.t
            nxt = qk(g + 1) if g < 3 else None
            n_rough = [2 * jp * T // (GS * LSUB) for jp in (2 * g, 2 * g + 1)]
            n_near = [(T + T // 2) // GS, (3 * T + T // 2) // GS]
            holes = [(t - PH0, t + PH1) for t in ends]
            if g < 3:
                vfin(g, clk.pacer(t0 - VB, t0 + VW, 32))
                holes += [(t0, t0 + VW), (t1 - HOLE0, t1 + HOLE1)]
            if g == 2:
                vfin(3, clk.pacer(clk.t - SLACK - VW // 2, clk.t - SLACK, 32))
                holes.append((clk.t - SLACK - VW // 2, clk.t))
            tie = clk.pacer(t0 + D0, (clk.t if g else t1) - SLACK,
                            sum(n_rough) + sum(n_near) + FW * g * 8 * T // GS, holes)
            rough(2 * g, mx[0], tie)
            near(2 * g, tie, n_rough[0])
            k = n_rough[0] + n_near[0]
            rough(2 * g + 1, mx[1], lambda x, i: tie(x, k + i))
            near(2 * g + 1, tie, k + n_rough[1])
            far(g, tie, k + n_rough[1] + n_near[1])
            if g == 0:
                prep_wo(clk.pacer(t0 + VW, t1 - HOLE0, HM // 16))
            mx = nxt
        t0 = clk.t
        run(PLAN[4])
        prep_w(jnp.minimum(h + 1, H - 1), range(NT1), clk.pacer(t0 - PW0, clk.t - 300, 8 * NT1))
        if os.environ.get('SHOW'):
            print('final loads', clk.load)

    head(**head_refs)

    @pl.when(h == H - 1)
    def _():
        oproj(NP - 1, _Clock(zero_s))
        out_copy(NP - 1).start()
        for jp in range(NP):
            out_copy(jp).wait()


@jax.jit
def pallas_gated_mix__compressed_kv_cla__ssm_conv_s5__prompt_kernel(
    A_x: jax.Array,
    A_c_kv: jax.Array,
    A_w_q: jax.Array,
    A_w_uk: jax.Array,
    A_w_uv: jax.Array,
    A_w_o: jax.Array,
    B_x: jax.Array,
    B_Lambda_re: jax.Array,
    B_Lambda_im: jax.Array,
    B_B_re: jax.Array,
    B_B_im: jax.Array,
    B_C_re: jax.Array,
    B_C_im: jax.Array,
    B_log_dt: jax.Array,
    B_Dskip: jax.Array,
    gate_w: jax.Array,
):
    del B_x
    xT = jnp.transpose(A_x[0])
    woT = jnp.transpose(A_w_o, (0, 2, 1))
    ckv = A_c_kv.reshape(4, 4, 2, T // 2, DC)

    hbm = pl.BlockSpec(memory_space=pl.ANY)
    outT = pl.pallas_call(
        _kernel,
        grid=(H,),
        in_specs=[hbm] * 15,
        out_specs=hbm,
        out_shape=jax.ShapeDtypeStruct((M, S), f32),
        scratch_shapes=_SHARED_SCRATCH + list(_PROLOGUE_SCRATCH.values()) + list(_HEAD_SCRATCH.values()),
        compiler_params=pltpu.CompilerParams(
            dimension_semantics=("arbitrary",),
            vmem_limit_bytes=126 * 1024 * 1024,
        ),
    )(xT, B_B_re, B_B_im, B_C_re, B_C_im, B_Lambda_re, B_Lambda_im, B_log_dt,
      B_Dskip, gate_w, woT, ckv, A_w_q, A_w_uk, A_w_uv)
    return jnp.transpose(outT)[None]
```

```python
import bisect
import os

import jax
import jax.numpy as jnp
from jax import lax
import jax.experimental.pallas as pl
import jax.experimental.pallas.tpu as pltpu

S = 2048
M = 448
H = 16
D = 256
DC = 1024
T = 128
NP = S // T // 2
HD = D // 2
HM = M // 2
QD = D // 4
QC = DC // 4
QM = M // 4
PA = 384
PB = M - PA
TA = 512
TC = 256
CS = DC // NP
NRAW = 4
LOG2E = 1.4426950408889634
NEG = -1e30

_env = lambda k, d: type(d)(os.environ.get(k, d))
GC = _env('GC', 64)
GS = _env('GS', 16)
RCH = _env('RCH', 256)
SLACK = _env('SLACK', 200)
D0 = _env('D0', 0)
NT1 = _env('NT1', 3)
LEAD = _env('LEAD', 448)
PW0 = _env('PW0', 100)
FTIE = _env('FTIE', 1)
YS = _env('YS', 2)
QR = _env('QR', 128)
QL0 = _env('QL0', 200)
QL1 = _env('QL1', 500)
SPAN = _env('SPAN', 6000)
QLATE = _env('QLATE', 0)
SC0 = _env('SC0', 0)
QH0 = _env('QH0', 0)
QH1 = _env('QH1', 1000)
AP0 = _env('AP0', 1000)
SP0 = _env('SP0', 1200)
FLAG = _env('FLAG', 40)
FW = _env('FW', 2)
HOLE0 = _env('HOLE0', 300)
HOLE1 = _env('HOLE1', 300)
VW = _env('VW', 900)
VB = _env('VB', 0)
PH0 = _env('PH0', 400)
PH1 = _env('PH1', 0)
QCH = _env('QCH', 64)
OCH = ((0, 64), (64, 64), (128, 48), (176, 48))
LSUB = _env('LSUB', 4)
PLAN = _env('PLAN', 'K107,K207,K307,P1 P0 O2 O3 P2 O0 O1 O4,O5 P3 O6').split(',')

f32 = jnp.float32
bf16 = jnp.bfloat16
u32 = jnp.uint32

SEM_VEC, SEM_B, SEM_X, SEM_WQ, SEM_C, SEM_SL, SEM_WO, SEM_OUT, SEM_WQ1 = 0, 1, 2, 6, 7, 8, 16, 17, 18
NSEM = 22

_NN = ((1,), (0,))
_NT = ((1,), (1,))
_TN = ((0,), (0,))
_TT = ((0,), (1,))


def _dot(a, b, dims):
    return lax.dot_general(a, b, (dims, ((), ())), preferred_element_type=f32)


def _cat(xs, axis):
    return xs[0] if len(xs) == 1 else jnp.concatenate(xs, axis=axis)


def _ds(lo, n, align):
    return pl.ds(lo if isinstance(lo, int) else pl.multiple_of(lo, align), n)


def _put(ref, row, col, xs, tie=None):
    x = _cat(xs, 1)
    if tie is not None:
        x = jnp.concatenate([tie(x[:8]), x[8:]], axis=0)
    ref[row // 2:(row + x.shape[0]) // 2, col:col + x.shape[1]] = pltpu.bitcast(x.astype(bf16), u32)


def _get(ref, row, nrows, col, ncols):
    return pltpu.bitcast(ref[row // 2:(row + nrows) // 2, col:col + ncols], bf16)


class _Clock:
    def __init__(self, zero_ref):
        self.masks = {(8, T): zero_ref[...] != 0.0}
        self.ticks, self.load = [], [0, 0, 0, 0]

    @property
    def t(self):
        return max(self.load)

    def dot(self, a, b, dims):
        v = _dot(a, b, dims)
        rows, depth = v.shape[0], a.shape[dims[0][0]]
        for c in range(0, v.shape[1], T):
            start = 0
            for _ in range(0, depth, T):
                k = self.load.index(min(self.load))
                start = max(start, self.load[k])
                self.load[k] += rows
            self.ticks += [(start + r + 8, (v, r, c)) for r in range(0, rows, 8)]
        return v, start

    def strassen(self, lhs, rhs, dims, split_last=False):
        jobs = -(-lhs(0).shape[dims[0][0]] // T)
        lag = sum(l + 32 <= max(self.load) for l in self.load) // jobs if jobs < 3 else 0
        order = ((1, 3, 2, 4, 0, 5, 6), (0, 1, 3, 2, 4, 5, 6), (5, 6, 1, 3, 2, 4, 0), (0, 5, 6, 1, 3, 2, 4))[lag]
        m = {}
        for n in order:
            if split_last and n == order[-1]:
                a, half = lhs(n), lhs(0).shape[0] // 2
                m[n] = jnp.concatenate([self.dot(a[:half], rhs(n), dims)[0], self.dot(a[half:], rhs(n), dims)[0]], 0)
            else:
                m[n] = self.dot(lhs(n), rhs(n), dims)[0]
        vals = [m[n] for n in range(7)]
        return lambda r=0, n=None, only=(0, 1, 2, 3), c=0, w=None: _combine(
            vals if n is None else _Tiles(vals, r, n, c, w), only, order)

    def level(self, pairs):
        base, extra = divmod((sum(self.load) + sum(a.shape[0] for a, _ in pairs)) // 16, 4)
        target = [16 * (base + (k < extra)) for k in range(4)]
        out = []
        for a, b in pairs:
            r, parts = 0, []
            while r < a.shape[0]:
                k = self.load.index(min(self.load))
                n = min(max(target[k] - self.load[k], 16), a.shape[0] - r)
                parts.append(self.dot(a[r:r + n], b, _NN)[0])
                r += n
            out.append(_cat(parts, 0))
        return out

    def pacer(self, t0, t1, n, holes=()):
        holes = sorted((max(a, t0), min(b, t1)) for a, b in holes if a < t1 and b > t0)
        gap = sum(b - a for a, b in holes)
        ticks = sorted(self.ticks, key=lambda tw: tw[0])
        times = [tw[0] for tw in ticks]

        def tie(x, k, distinct=False, delay=0):
            t = t0 + (t1 - t0 - gap) * k / n
            for a, b in holes:
                t += b - a if t > a else 0
            t += delay
            past = ticks[:bisect.bisect_right(times, t)]
            reps = (x.shape[0] // 8, x.shape[1] // T)
            if len(past) < (reps[1] if distinct else 1):
                return x
            tick = _cat([v[r:r + 8, c:c + T] for _, (v, r, c) in past[-reps[1] if distinct else -1:]], 1)
            if tick.dtype != x.dtype:
                tick = pltpu.bitcast(tick, x.dtype)
            if x.shape not in self.masks:
                self.masks[x.shape] = jnp.tile(self.masks[(8, T)], reps)
            return lax.select(self.masks[x.shape], tick if tick.shape == x.shape else jnp.tile(tick, reps), x)
        return tie


def _no_tie(x, k):
    return x


_A_TERMS = ((0, 3, 1), (2, 3, 1), (0, None, 0), (3, None, 0), (0, 1, 1), (2, 0, -1), (1, 3, -1))
_B_TERMS = ((0, 3, 1), (0, None, 0), (1, 3, -1), (2, 0, -1), (3, None, 0), (0, 1, 1), (2, 3, 1))


def _operand(term, block):
    x, y, sign = term
    if y is None:
        return block(x)
    return block(x) + block(y) if sign > 0 else block(x) - block(y)


def _operands(terms, blocks):
    return [_operand(t, blocks.__getitem__) for t in terms]


def _operands2(terms, n1, block, tie):
    first = terms[n1][0]
    sub = [_operand(terms[n1], lambda o: tie(block(o, q)) if o == first and q in (0, 3) else block(o, q))
           for q in range(4)]
    return _operands(terms, sub)


_C_TERMS = ({0: 1, 3: 1, 4: -1, 6: 1}, {2: 1, 4: 1}, {1: 1, 3: 1}, {0: 1, 1: -1, 2: 1, 5: 1})


def _combine(m, only=(0, 1, 2, 3), order=(1, 3, 2, 4, 0, 5, 6)):
    out = []
    for terms in (_C_TERMS[n] for n in only):
        seq = [n for n in order if n in terms]
        if terms[seq[0]] < 0:
            seq[0], seq[1] = seq[1], seq[0]
        acc = m[seq[0]]
        for n in seq[1:]:
            acc = acc + m[n] if terms[n] > 0 else acc - m[n]
        out.append(acc)
    return out


def _outer_step(m_s, n1, row, v):
    n = v.shape[0]
    if n1 < 5:
        m_s[n1 * HD + row:n1 * HD + row + n, :] = v
    if n1 < 3:
        return None
    blk = (2, 1, 3, 0)[n1 - 3]
    m = {j: v if j == n1 else m_s[j * HD + row:j * HD + row + n, :] for j in _C_TERMS[blk]}
    return blk, _combine(m, (blk,), range(7))[0]


class _Tiles:
    def __init__(self, vals, r, n, c=0, w=None):
        self.vals, self.idx, self.cache = vals, (slice(r, r + n), slice(c, None if w is None else c + w)), {}

    def __getitem__(self, i):
        if i not in self.cache:
            self.cache[i] = self.vals[i][self.idx]
        return self.cache[i]


class _Reducer:
    def __init__(self, red, comb):
        self.red, self.comb, self.acc, self.rows, self.out = red, comb, None, 0, None

    def add(self, v):
        self.rows += 8 * v.shape[0]
        v = self.red(v, axis=0)
        self.acc = v if self.acc is None else self.comb(self.acc, v)
        if self.rows >= RCH:
            self.result()

    def result(self):
        if self.acc is not None:
            v = self.red(self.acc, axis=0, keepdims=True)
            self.out = v if self.out is None else self.comb(self.out, v)
        self.acc, self.rows = None, 0
        return self.out


def _cmul(ar, ai, br, bi):
    return ar * br - ai * bi, ar * bi + ai * br


def _hi16(w):
    return pltpu.bitcast(w & jnp.uint32(0xFFFF0000), f32)


def _stage(raw, stg, c0, nc, tie, groups=(0, 1)):
    for ht in groups:
        for dt in range(2):
            v = raw[c0:c0 + nc, ht * 8:(ht + 1) * 8, dt * T:(dt + 1) * T].reshape(nc * 8, T)
            stg[ht * 2 + dt, c0 * 4:(c0 + nc) * 4, :] = tie(pltpu.bitcast(v, u32))


def _ssm_params(vec_s, coef_s, lam_s, col_s):
    row = lambda r: r[...].astype(f32).reshape(1, M)
    lre, lim, ldt, dsk, gw = [row(v) for v in vec_s]
    dt = jnp.exp(ldt).astype(bf16).astype(f32)
    mag = jnp.exp(dt * lre)
    ang = dt * lim
    lr, li = mag * jnp.cos(ang), mag * jnp.sin(ang)
    den = lre * lre + lim * lim
    nr = lr - 1.0
    coef_s[...] = jnp.zeros(coef_s.shape, f32)
    coef_s[0:1, 0:M] = 2.0 * ((nr * lre + li * lim) / den)
    coef_s[1:2, 0:M] = 2.0 * ((li * lre - nr * lim) / den)

    er = jnp.concatenate([lr, lr[:, PA:]], axis=1)
    ei = jnp.concatenate([li, -li[:, PA:]], axis=1)
    pw = [(er, ei)]
    for _ in range(7):
        pw.append(_cmul(pw[-1][0], pw[-1][1], er, ei))
    sub = lax.broadcasted_iota(jnp.int32, (8, 512), 0)
    for n, d in enumerate((1, 2, 4)):
        lam_s[2 * n] = jnp.where(sub >= d, pw[d - 1][0], 0.0)
        lam_s[2 * n + 1] = jnp.where(sub >= d, pw[d - 1][1], 0.0)
    lcr = jnp.zeros((8, 512), f32)
    lci = jnp.zeros((8, 512), f32)
    for r in range(8):
        lcr = jnp.where(sub == r, pw[r][0], lcr)
        lci = jnp.where(sub == r, pw[r][1], lci)
    lam_s[6] = lcr
    lam_s[7] = lci

    def col(v):
        v = jnp.concatenate([v, jnp.zeros((1, 512 - M), f32)], axis=1)
        return jnp.broadcast_to(v, (T, 512)).T[:M]
    col_s[0] = col(dsk)
    col_s[1] = col(gw)


def _ssm_cmat(craw_s, coef_s, c_s, tie):
    for r in range(0, M, 16):
        coef = tie(coef_s[...], r // 16)
        cr, ci = coef[0:1, :M], coef[1:2, :M]
        re, im = _cmul(craw_s[0, r:r + 16, :].astype(f32), craw_s[1, r:r + 16, :].astype(f32), cr, ci)
        _put(c_s, r, 0, [re[:, :PA], -im[:, :PA], re[:, PA:], -im[:, PA:]])


def _ssm_scan(u_ref, carry, lam_s, h_s, tie):
    car, cai = carry
    out = []
    for b in range(TC // 8):
        mixed = u_ref[3, b, :, 0:T]
        u = jnp.concatenate([u_ref[cb, b] for cb in range(3)], axis=1)
        cols = [u[:, 0:T], u[:, T:2 * T], u[:, 2 * T:PA], mixed]
        hr = jnp.concatenate([tie(v, 4 * b + n) for n, v in enumerate(cols)], axis=1)
        hi = jnp.concatenate([u[:, PA:2 * PA], pltpu.roll(mixed, PB, 1)], axis=1)
        for n, d in enumerate((1, 2, 4)):
            sr, si = pltpu.roll(hr, d, 0), pltpu.roll(hi, d, 0)
            tr, ti = _cmul(sr, si, lam_s[2 * n], lam_s[2 * n + 1])
            hr, hi = hr + tr, hi + ti
        tr, ti = _cmul(lam_s[6], lam_s[7], car, cai)
        hr, hi = hr + tr, hi + ti
        car, cai = hr[7:8, :], hi[7:8, :]
        out.append(jnp.concatenate([hr[:, :PA], hi[:, :PA], hr[:, PA:]], axis=1))
        if b % 2 == 1:
            _put(h_s, (b - 1) * 8, 0, [jnp.concatenate(out, axis=0)])
            out = []
    return car, cai


_vmem = pltpu.VMEM
_PROLOGUE_SCRATCH = dict(
    xT_s=_vmem((M, S), bf16),
    v0=_vmem((M,), bf16), v1=_vmem((M,), bf16), v2=_vmem((M,), bf16), v3=_vmem((M,), bf16), v4=_vmem((M,), bf16),
    b_s=_vmem((2 * M, M), bf16),
    craw_s=_vmem((2, M, M), bf16),
    c_s=_vmem((M // 2, 2 * M), u32),
    coef_s=_vmem((8, 512), f32),
    lam_s=_vmem((8, 8, 512), f32),
    col_s=_vmem((2, M, T), f32),
    h_s=_vmem((TC // 2, 2 * M), u32),
    ckv_s=_vmem((4, 4, 2, T // 2, DC), bf16),
    rq=_vmem((M, H, D), bf16),
    rk=_vmem((NRAW * CS, H, D), bf16),
    rv=_vmem((NRAW * CS, H, D), bf16),
    sq=_vmem((4, M * 4, T), u32),
    sk=_vmem((4, CS * 4, T), u32),
    sv=_vmem((4, CS * 4, T), u32),
    xa_s=_vmem((QM // 2, 4 * 49 * T), u32),
    wqt_s=_vmem((D, 4 * T), u32),
    wq_s=_vmem((QD, 49 * T), u32),
)
_HEAD_SCRATCH = dict(
    mk_s=_vmem((7 * HD, 2 * T), f32),
    mv_s=_vmem((2, 7 * HD, 2 * T), f32),
    mp_s=_vmem((7 * HD, 2 * T), f32),
    kt_s=_vmem((2 * T, 4 * T), f32),
    ka_s=_vmem((S // 4, 9 * T), u32),
    va_s=_vmem((HD // 2, NP * 9 * T), u32),
    v2_s=_vmem((QD // 2, 3 * 49 * T), u32),
    s_s=_vmem((4, S // 8, 8, 2 * T), f32),
    pb_s=_vmem((2 * T, 7 * T), u32),
    pd_s=_vmem((S // 2, 2 * T), u32),
    p2_s=_vmem((3 * T, 49 * T), u32),
    sc_s=_vmem((1, S), f32),
    qb_s=_vmem((HD // 2, 14 * T), u32),
)
_SHARED_SCRATCH = [
    _vmem((H // 2 * D, DC), u32),
    _vmem((H // 2 * D, DC), u32),
    _vmem((S // 8, 49 * QC), u32),
    _vmem((H * D, S // 2), u32),
    _vmem((H, M, D), bf16),
    _vmem((QD, 49 * QC), u32),
    _vmem((HM // 2, 7 * T), u32),
    _vmem((HD // 2, NP * 7 * T), u32),
    _vmem((M, S), f32),
    _vmem((1, S), f32),
    _vmem((8, T), f32),
    pltpu.SemaphoreType.DMA((NSEM,)),
]


def _kernel(xT_hbm, bre_hbm, bim_hbm, cre_hbm, cim_hbm, lre_hbm, lim_hbm, ldt_hbm,
            dsk_hbm, gw_hbm, woT_hbm, ckv_hbm, wq_hbm, wk_hbm, wv_hbm,
            out_hbm,
            wkt_s, wvt_s, a_s, q_s, wo_s, w_s, wl_s, cl_s, o_s, g_s, zero_s, sem, *rest):
    h = pl.program_id(0)
    pro_refs = dict(zip(_PROLOGUE_SCRATCH, rest))
    head_refs = dict(zip(_HEAD_SCRATCH, rest[len(pro_refs):]))

    def out_copy(jp):
        cols = pl.ds(jp * 2 * T, 2 * T)
        return pltpu.make_async_copy(o_s.at[:, cols], out_hbm.at[:, cols], sem.at[SEM_OUT])

    def prep_w(hh, outer, tie):
        rows = _ds(lax.shift_right_logical(hh, 1) * D, D, D)
        sh = (16 * (1 - (hh & 1))).astype(u32)
        k = 0
        for row0, wt_s in ((0, wkt_s.at[rows]), (QD, wvt_s.at[rows])):
            for r in range(0, QD, 16):
                def block(o, q):
                    row = (o % 2) * HD + (q % 2) * QD + r
                    col = (o // 2) * 2 * QC + (q // 2) * QC
                    return _hi16(wt_s[row:row + 16, col:col + QC] << sh)
                for n1 in outer:
                    _put(w_s, row0 + r, 7 * n1 * QC, _operands2(_B_TERMS, n1, block, lambda x: tie(x, k)))
                    k += 1

    def prologue(xT_s, v0, v1, v2, v3, v4, b_s, craw_s, c_s, coef_s, lam_s, col_s, h_s,
                 ckv_s, rq, rk, rv, sq, sk, sv, xa_s, wqt_s, wq_s):
        u_s = head_refs['s_s']
        vec_s = (v0, v1, v2, v3, v4)

        def slice_copies(i):
            s = sem.at[SEM_SL + i]
            grp = i // 2 if isinstance(i, int) else lax.shift_right_logical(i, 1)
            cs, dst = pl.ds(i * CS, CS), pl.ds((i & (NRAW - 1)) * CS, CS)
            return [pltpu.make_async_copy(ckv_hbm.at[grp, :, i & 1], ckv_s.at[grp, :, i & 1], s),
                    pltpu.make_async_copy(wk_hbm.at[cs], rk.at[dst], s),
                    pltpu.make_async_copy(wv_hbm.at[cs], rv.at[dst], s)]

        def wq1_copy(i):
            rows = pl.ds(i * (M // 4), M // 4)
            return pltpu.make_async_copy(wq_hbm.at[rows, 8:16], rq.at[rows, 8:16], sem.at[SEM_WQ1 + i])

        def x_copy(i):
            cols = pl.ds(i * TA, TA)
            return pltpu.make_async_copy(xT_hbm.at[:, cols], xT_s.at[:, cols], sem.at[SEM_X + i])

        cp_vec = [pltpu.make_async_copy(src, dst, sem.at[SEM_VEC])
                  for src, dst in zip((lre_hbm, lim_hbm, ldt_hbm, dsk_hbm, gw_hbm), vec_s)]
        cp_b = [pltpu.make_async_copy(src.at[pl.ds(lo, n)], b_s.at[pl.ds(dst, n)], sem.at[SEM_B])
                for src, lo, n, dst in ((bre_hbm, 0, PA, 0), (bim_hbm, 0, PA, PA),
                                        (bre_hbm, PA, PB, 2 * PA), (bim_hbm, PA, PB, 2 * PA + PB))]
        cp_wq = [pltpu.make_async_copy(wq_hbm.at[:, 0:8], rq.at[:, 0:8], sem.at[SEM_WQ])]
        cp_c = [pltpu.make_async_copy(src, craw_s.at[n], sem.at[SEM_C])
                for n, src in enumerate((cre_hbm, cim_hbm))]
        cp_wo = pltpu.make_async_copy(woT_hbm, wo_s, sem.at[SEM_WO])
        for cp in cp_vec + cp_b + [x_copy(i) for i in range(S // TA)] + cp_c + cp_wq:
            cp.start()
        for i in range(NRAW - 1):
            for cp in [wq1_copy(i)] + slice_copies(i):
                cp.start()
        wq1_copy(3).start()
        cp_wo.start()

        zero_s[...] = jnp.zeros(zero_s.shape, f32)
        wl_s[...] = jnp.zeros(wl_s.shape, u32)
        cl_s[:, (NP - 1) * 7 * T:] = jnp.zeros((HD // 2, 7 * T), u32)
        for cp in cp_vec:
            cp.wait()
        _ssm_params(vec_s, coef_s, lam_s, col_s)

        def wq_transpose(pair, tie):
            ht = pair // 4 if isinstance(pair, int) else lax.shift_right_logical(pair, 2)
            pad = jnp.zeros((T - QM, T), u32)
            for dt in range(2):
                for mq in range(4):
                    blk = sq[ht * 2 + dt, pl.ds(mq * QM * 4 + (pair & 3), QM, stride=4), :]
                    blk = jnp.concatenate([tie(blk[:8], 4 * dt + mq), blk[8:], pad], axis=0)
                    wqt_s[dt * HD:(dt + 1) * HD, mq * T:(mq + 1) * T] = blk.T

        def phase1(i):
            clk = _Clock(zero_s)
            u, _ = clk.dot(xT_s[:, i * TA:(i + 1) * TA], b_s[...], _TT)
            for cb in range(4):
                w = min(2 * T, 2 * M - cb * 2 * T)
                u_s[cb, i * TA // 8:(i + 1) * TA // 8, :, 0:w] = (
                    u[:, cb * 2 * T:cb * 2 * T + w].reshape(TA // 8, 8, w))
            tie = clk.pacer(0, 6 * TA, 49)
            for r in range(0, QM, 16):
                def block(o, q):
                    row, col = (o % 2) * HM + (q % 2) * QM + r, (4 * i + 2 * (q // 2) + o // 2) * T
                    return xT_s[row:row + 16, col:col + T].astype(f32)
                for n1 in range(7):
                    ops = _operands2(_A_TERMS, n1, block, lambda x: tie(x, 7 * (r // 16) + n1))
                    _put(xa_s, r, (i * 7 + n1) * 7 * T, ops)
            return clk

        for cp in cp_b + [x_copy(0)]:
            cp.wait()
        phase1(0)
        x_copy(1).wait()
        clk = phase1(1)
        zero = jnp.zeros((1, 512), f32)
        carry0 = _ssm_scan(u_s.at[:, 0:TC // 8], (zero, zero), lam_s, h_s, clk.pacer(0, 6 * TA, TC // 2))
        for cp in [x_copy(2), x_copy(3)] + cp_c + cp_wq:
            cp.wait()
        _ssm_cmat(craw_s, coef_s, c_s, phase1(2).pacer(0, 6 * TA, M // 16))
        tie = phase1(3).pacer(0, 6 * TA, M // 8)
        for c0 in range(0, M, 8):
            _stage(rq, sq, c0, 8, lambda x: tie(x, c0 // 10), groups=(0,))
        wq_transpose(0, lambda x, k: tie(x, 46 + k))

        def phase2(i, carry):
            @pl.when(i + NRAW - 1 < NP)
            def _():
                for cp in slice_copies(i + NRAW - 1):
                    cp.start()

            @pl.when(i < 4)
            def _():
                wq1_copy(i).wait()

            for cp in slice_copies(i):
                cp.wait()

            clk = _Clock(zero_s)
            yT = _cat([clk.dot(_get(c_s, r, M // YS, 0, 2 * M), _get(h_s, 0, TC, 0, 2 * M), _NT)[0]
                       for r in range(0, M, M // YS)], 0)
            ty = clk.t
            for t in range(TC // T):
                cols = _ds(i * TC + t * T, T, T)
                acc = jnp.zeros((8, T), f32)
                for r in range(0, M, 32):
                    xg = xT_s[r:r + 32, cols].astype(f32) * col_s[1, r:r + 32, :]
                    acc = acc + jnp.sum(xg.reshape(4, 8, T), axis=0)
                g = jax.nn.sigmoid(jnp.sum(acc, axis=0, keepdims=True))
                g_s[:, cols] = g
                for r in range(0, M, 32):
                    skip = xT_s[r:r + 32, cols].astype(f32) * col_s[0, r:r + 32, :]
                    o_s[r:r + 32, cols] = (1.0 - g) * (yT[r:r + 32, t * T:(t + 1) * T] + skip)

            q_i = q_s.at[_ds(i * 2 * D, 2 * D, 2 * D)]
            mq_s = (head_refs['mk_s'], head_refs['mp_s'], head_refs['mv_s'].at[0], head_refs['mv_s'].at[1])
            for g in range(4):
                for n1 in range(7):
                    if g == 0:
                        t = QL0 + (ty + 6 * 224 - QL1 - QL0) * n1 / 7
                        tie = clk.pacer(min(t, clk.t - QL1), min(t + 300, clk.t - QL1), 8)
                        for r in range(0, 2 * QD, 16):
                            def block(o, q):
                                row = (o % 2) * HD + (q % 2) * QD + r % QD
                                col = (2 * (o // 2) + q // 2) * T
                                w = wqt_s[row:row + 16, col:col + T]
                                return _hi16(w) if r >= QD else pltpu.bitcast(w << 16, f32)
                            _put(wq_s, r, 7 * n1 * T, _operands2(_B_TERMS, n1, block, lambda x: tie(x, r // 16)),
                                 (lambda w: tie(w, r // 16, True, FLAG)) if QLATE else None)
                    for r0 in range(0, 2 * QD, QR):
                        comb = clk.strassen(lambda n: _get(wq_s, r0, QR, (7 * n1 + n) * T, QM),
                                            lambda n: _get(xa_s, 0, QM, (g * 49 + 7 * n1 + n) * T, T), _NN)
                        for r in range(0, QR, 32):
                            e, c = (r0 + r) // QD, comb(r, 32)
                            for dq in range(2):
                                row = dq * QD + r % QD
                                done = _outer_step(mq_s[2 * (g % 2) + e], n1, row,
                                                   jnp.concatenate([c[dq], c[2 + dq]], axis=1))
                                if done:
                                    n, v = done
                                    _put(q_i, (2 * e + n // 2) * D + (n % 2) * HD + row, 2 * g * T,
                                         [v * (LOG2E * D ** -0.5)])

            span = ty + SPAN

            u_next = u_s.at[:, pl.ds(jnp.minimum(i + 1, NP - 1) * (TC // 8), TC // 8)]
            carry = _ssm_scan(u_next, carry, lam_s, h_s, clk.pacer(ty + SC0, span, TC // 2))

            tie = clk.pacer(ty - SP0, span, 64, [(ty + QH0, ty + QH1)])
            rq_i = rq.at[pl.ds((i & 3) * (M // 4), M // 4)]
            sq_i = sq.at[:, _ds((i & 3) * M, M, 8)]
            for c0 in range(0, M // 4, 8):
                _stage(rq_i, sq_i, c0, 8, lambda x: tie(x, c0 // 4 + 2), groups=(1,))
            wq_transpose(jnp.minimum(i + 1, NP - 1), lambda x, k: tie(x, 36 + 3 * k))
            slot = pl.ds((i & (NRAW - 1)) * CS, CS)
            for n, (raw, stg, wt_s) in enumerate(((rk, sk, wkt_s), (rv, sv, wvt_s))):
                for c0 in range(0, CS, 8):
                    _stage(raw.at[slot], stg, c0, 8, lambda x: tie(x, 16 * n + c0 // 8))
                cols = _ds(i * CS, CS, CS)
                for pair in range(H // 2):
                    for dt in range(2):
                        blk = stg[(pair // 4) * 2 + dt, pl.ds(pair % 4, CS, stride=4), :]
                        row = pair * D + dt * HD
                        blk = jnp.concatenate([tie(blk[:8], 16 + 24 * n + 3 * pair + dt), blk[8:]], axis=0)
                        wt_s[row:row + HD, cols] = blk.T

            tie = clk.pacer(ty + AP0, span, 28)
            ckv_i = ckv_s.at[lax.shift_right_logical(i, 1), :, i & 1]
            a_i = a_s.at[_ds(i * (T // 4), T // 4, T // 4)]
            for r in range(0, T // 2, 16):
                def block(o, q):
                    col = (o % 2) * 2 * QC + (q % 2) * QC
                    return ckv_i[2 * (q // 2) + o // 2, r:r + 16, col:col + QC].astype(f32)
                for n1 in range(7):
                    ops = _operands2(_A_TERMS, n1, block, lambda x: tie(x, 7 * (r // 16) + n1))
                    _put(a_i, r, 7 * n1 * QC, ops)
            return carry

        lax.fori_loop(0, NP, phase2, carry0)
        cp_wo.wait()
        prep_w(h, range(NT1), _no_tie)

    @pl.when(h == 0)
    def _():
        prologue(**pro_refs)

    def oproj(jp, clk):
        cols = slice(2 * jp * T, (2 * jp + 2) * T)
        for r, n in OCH:
            c = clk.strassen(lambda i: _get(wl_s, r, n, i * T, T),
                             lambda i: _get(cl_s, 0, HD, (jp * 7 + i) * T, T), _NN)()
            o_s[r:r + n, cols] += jnp.concatenate(c[:2], axis=1)
            o_s[HM + r:HM + r + n, cols] += jnp.concatenate(c[2:], axis=1)

    def head(mk_s, mv_s, mp_s, kt_s, ka_s, va_s, v2_s, s_s, pb_s, pd_s, p2_s, sc_s, qb_s):
        clk = _Clock(zero_s)
        q_h = q_s.at[_ds(h * D, D, D)]

        def prep_wo(tie):
            for r in range(0, HM, 16):
                top = tie(wo_s[h, r:r + 16, :].astype(f32), r // 16)
                bot = tie(wo_s[h, HM + r:HM + r + 16, :].astype(f32), r // 16)
                _put(wl_s, r, 0, _operands(_A_TERMS, [top[:, :HD], top[:, HD:], bot[:, :HD], bot[:, HD:]]))

        nine = lambda c: _operands(_A_TERMS, c) + [c[1], c[2]]

        def outer(m_s, r):
            return _combine([m_s[n * HD + r:n * HD + r + 16, :] for n in range(7)], order=range(7))

        def proj(g, lo, hi):
            for n1 in range(lo, hi):
                comb = clk.strassen(lambda n: _get(w_s, 0, 2 * QD, (7 * n1 + n) * QC, QC),
                                    lambda n: _get(a_s, g * T, T, (7 * n1 + n) * QC, QC), _NT, n1 == 6)
                for r in range(0, 2 * QD, GC):
                    m_s, row = mk_s if r < QD else mv_s.at[g % 2], n1 * HD + r % QD
                    c = comb(r, GC)
                    m_s[row:row + GC, :] = jnp.concatenate([c[0], c[2]], axis=1)
                    m_s[QD + row:QD + row + GC, :] = jnp.concatenate([c[1], c[3]], axis=1)
            if hi < 7:
                return
            cs = [outer(mk_s, r) for r in range(0, HD, 16)]
            for n in range(4):
                kt_s[:, n * T:(n + 1) * T] = jnp.concatenate([c[n] for c in cs], axis=0).T
            for r in range(0, 2 * T, GC):
                blk = kt_s[r:r + GC, :]
                _put(ka_s, 2 * g * T + r, 0, nine([blk[:, n * T:(n + 1) * T] for n in range(4)]))

        def vfin(g, tie):
            m_s = mv_s.at[g % 2]
            for r in range(0, QD, 16):
                k, blk = 8 * (r // 16), {}
                late = lambda w: tie(w, k, True, FLAG)
                for new, n1 in (((0,), 2), ((1,), 4), ((3,), 6), ((), 0), ((), 3), ((2,), 5), ((), 1)):
                    for o in new:
                        for i, row in enumerate((r, QD + r)):
                            tiles = _Tiles([m_s.at[n * HD:(n + 1) * HD] for n in range(7)], row, 16)
                            c, = _combine(tiles, ((o % 2) * 2 + o // 2,), range(7))
                            blk[o, i] = c = tie(c, k)
                            slot = (2, 7, 8, 3)[o]
                            _put(va_s, row, ((2 * g + 1) * 9 + slot) * T, [c[:, T:]])
                            if o in (1, 2):
                                _put(va_s, row, (2 * g * 9 + slot) * T, [c[:, :T]])
                    lo_, hi_ = [_operand(_A_TERMS[n1], lambda o: blk[o, i]) for i in range(2)]
                    _put(va_s, r, (2 * g * 9 + n1) * T, [lo_[:, :T]], late)
                    _put(va_s, QD + r, (2 * g * 9 + n1) * T, [hi_[:, :T]], late)
                    if g < 3:
                        _put(v2_s, r, (g * 7 + n1) * 7 * T,
                             _operands(_A_TERMS, [lo_[:, :T], lo_[:, T:], hi_[:, :T], hi_[:, T:]]), late)
                    k += 8 / 7

        key = lax.broadcasted_iota(jnp.int32, (T, 2 * T), 0)
        qry = lax.broadcasted_iota(jnp.int32, (T, 2 * T), 1)
        causal = key <= qry

        def qk(g):
            pairs = (2 * g, 2 * g + 1)
            mx = {jp: _Reducer(jnp.max, jnp.maximum) for jp in pairs}

            def put(jp, row, v):
                v = v.reshape(v.shape[0] // 8, 8, 2 * T)
                s_s[jp % 4, row // 8:row // 8 + v.shape[0]] = v
                mx[jp].add(v)

            def rect(jp, lo, hi, n):
                for r in range(lo, hi, n):
                    c = clk.strassen(lambda i: _get(ka_s, r, n, i * T, T),
                                     lambda i: _get(qb_s, 0, HD, ((jp % 2) * 7 + i) * T, T), _NN)()
                    put(jp, r, jnp.concatenate(c[:2], axis=1))
                    put(jp, jp * T + r, jnp.concatenate(c[2:], axis=1))

            q = lambda jp, e: _get(q_h, e * D, D, jp * T, T)
            for jp in pairs[g == 0:]:
                for r in range(0, HD, 32):
                    blk = [_get(q_h, e * D + d * HD + r, 32, jp * T, T).astype(f32) for d in range(2) for e in range(2)]
                    _put(qb_s, r, (jp % 2) * 7 * T, _operands(_B_TERMS, blk))
            for jp in pairs:
                rect(jp, 0, 2 * g * T, QCH if QCH else g * T // 2 or 1)
            kb = lambda jp, a, b: jnp.concatenate(
                [_get(ka_s, jp * T, T, a * T, T), _get(ka_s, jp * T, T, b * T, T)], axis=1)
            for jp in pairs:
                se, _ = clk.dot(kb(jp, 2, 7), jnp.concatenate([q(jp, 0), q(jp, 1)], axis=1), _NN)
                put(jp, 2 * jp * T, jnp.where(causal, se, NEG))
            last = {}
            for jp in pairs:
                so = jnp.where(causal[:, :T], clk.dot(kb(jp, 8, 3), q(jp, 1), _NN)[0], NEG)
                row = (2 * jp + 1) * T // 8
                s_s[jp % 4, row:row + T // 8, :, T:] = so.reshape(T // 8, 8, T)
                last[jp] = jnp.concatenate([jnp.full((1, T), NEG, f32), jnp.max(so, axis=0, keepdims=True)], axis=1)
            rect(2 * g + 1, 2 * g * T, (2 * g + 1) * T, T // 4)
            return [jnp.broadcast_to(jnp.maximum(mx[jp].result(), last[jp]), (8, 2 * T)) for jp in pairs]

        zs, sums = {}, {}

        def prob(jp, row, z, n=GS, lanes=slice(None)):
            return jnp.exp2(s_s[jp % 4, row // 8:(row + n) // 8, :, lanes] - z[:, lanes])

        def rough(jp, mx, tie):
            zs[jp] = mx
            if jp > 0:
                sm = _Reducer(jnp.sum, jnp.add)
                for k, r in enumerate(range(0, 2 * jp * T, GS * LSUB)):
                    sm.add(prob(jp, r, tie(mx, k)))
                zs[jp] = mx + jnp.log2(jnp.maximum(LSUB * sm.result(), 1.0))
            sums[jp] = _Reducer(jnp.sum, jnp.add)

        def blocks(jp, row, tie, k):
            top, bot = prob(jp, row, tie(zs[jp], k)), prob(jp, jp * T + row, tie(zs[jp], k + 1))
            sums[jp].add(top + bot)
            top, bot = top.reshape(GS, 2 * T), bot.reshape(GS, 2 * T)
            return [top[:, :T], top[:, T:], bot[:, :T], bot[:, T:]]

        def near(jp, tie, k):
            R, z = jp * T, zs[jp]
            if jp % 2:
                for r in range(0, T, GS):
                    _put(pb_s, jp // 2 * T + r, 0, _operands(_B_TERMS, blocks(jp, R - T + r, tie, k)))
                    k += 2
            for r in range(0, T, GS):
                p = prob(jp, 2 * R + r, tie(z, k))
                sums[jp].add(p)
                _put(pd_s, 2 * R + r, 0, [p.reshape(GS, 2 * T)])
                k += 1
            so = _Reducer(jnp.sum, jnp.add)
            for r in range(0, T, 2 * GS):
                p = prob(jp, 2 * R + T + r, tie(z, k), 2 * GS, slice(T, 2 * T))
                so.add(p)
                _put(pd_s, 2 * R + T + r, T, [p.reshape(2 * GS, T)])
                k += 1
            sums[jp].result()
            sums[jp].out = sums[jp].out + jnp.concatenate([jnp.zeros((1, T), f32), so.result()], axis=1)

        p20 = lambda g: g * (g - 1) // 2 * T

        def far(g, tie, k):
            half = {(jp, e): _Reducer(jnp.sum, jnp.add) for jp in (2 * g, 2 * g + 1) for e in range(2)}
            for kg in range(g):
                for r in range(0, T, GS):
                    blk = {}
                    for new, n1 in (((0,), 1), ((1,), 5), ((3,), 2), ((), 0), ((), 4), ((2,), 3), ((), 6)):
                        for o in new:
                            lanes = slice((o % 2) * T, (o % 2 + 1) * T)
                            for jp in (2 * g, 2 * g + 1):
                                z = tie(zs[jp][:, lanes], k)
                                row = (o // 2) * jp * T + 2 * kg * T + r
                                p = [jnp.exp2(s_s[jp % 4, x // 8:(x + GS) // 8, :, lanes] - z) for x in (row, row + T)]
                                half[jp, o % 2].add(p[0] + p[1])
                                blk[o, jp % 2], blk[o, 2 + jp % 2] = [x.reshape(GS, T) for x in p]
                        ops = _operands2(_B_TERMS, n1, lambda o, q: blk[o, q], lambda x: x)
                        _put(p2_s, p20(g) + kg * T + r, 7 * n1 * T, ops,
                             (lambda w: tie(w, k, True, FLAG)) if FTIE else None)
                        k += FW * 8 / 7
            for jp in (2 * g, 2 * g + 1):
                if g:
                    sums[jp].out = sums[jp].out + jnp.concatenate([half[jp, e].result() for e in range(2)], axis=1)
            for jp in (2 * g, 2 * g + 1):
                cols = slice(2 * jp * T, 2 * (jp + 1) * T)
                sc_s[:, cols] = g_s[:, cols] / sums[jp].result()

        def pv(g):
            pairs = (2 * g, 2 * g + 1)
            va = lambda n, t, r=0, nr=HD: _get(va_s, r, nr, (t * 9 + n) * T, T)
            for n1 in range(7 if g else 0):
                c = clk.strassen(
                    lambda n: _cat([_get(v2_s, 0, QD, (kg * 49 + 7 * n1 + n) * T, T) for kg in range(g)], 1),
                    lambda n: _get(p2_s, p20(g), g * T, (7 * n1 + n) * T, T), _NN)()
                mp_s[n1 * HD:n1 * HD + QD, :] = jnp.concatenate(c[:2], axis=1)
                mp_s[n1 * HD + QD:(n1 + 1) * HD, :] = jnp.concatenate(c[2:], axis=1)
            ve = [jnp.concatenate([va(2, jp), va(8, jp)], axis=0) for jp in pairs]
            vo = [jnp.concatenate([va(7, jp), va(3, jp)], axis=0) for jp in pairs]
            ce = clk.level([(ve[jp % 2], _get(pd_s, 2 * jp * T, T, 0, T)) for jp in pairs])
            co = [clk.dot(jnp.concatenate([ve[jp % 2], vo[jp % 2]], axis=1),
                          _get(pd_s, 2 * jp * T, 2 * T, T, T), _NN)[0] for jp in pairs]
            for jp in pairs:
                R, e = jp * T, jp % 2
                ge, go = sc_s[:, 2 * R:2 * R + T], sc_s[:, 2 * R + T:2 * R + 2 * T]
                for r in range(0, HD, 32):
                    c = [ce[e][r:r + 32], co[e][r:r + 32], ce[e][HD + r:HD + r + 32], co[e][HD + r:HD + r + 32]]
                    if g:
                        far_ = _combine([mp_s[n * HD + r:n * HD + r + 32, e * T:(e + 1) * T] for n in range(7)],
                                        order=range(7))
                        c = [x + y for x, y in zip(c, far_)]
                    if e:
                        near_ = clk.strassen(lambda n: va(n, 2 * g, r, 32),
                                             lambda n: _get(pb_s, g * T, T, n * T, T), _NN)()
                        c = [x + y for x, y in zip(c, near_)]
                    ops = _operands(_B_TERMS, [c[0] * ge, c[1] * go, c[2] * ge, c[3] * go])
                    _put(cl_s, r, jp * 7 * T, ops)

        ends = []

        def run(items):
            for item in items.split():
                if item[0] == 'P':
                    pv(int(item[1]))
                    ends.append(clk.t)
                elif item[0] == 'K':
                    proj(int(item[1]), int(item[2]), int(item[3]))
                else:
                    jp = int(item[1])
                    oproj(jp, clk)

                    @pl.when(h == H - 1)
                    def _():
                        out_copy(jp).start()

        for n1 in range(7):
            if n1 >= NT1:
                prep_w(h, [n1], clk.pacer(max(clk.t - LEAD - 448, 1), max(clk.t - LEAD, 1), 8))
            proj(0, n1, n1 + 1)
        oproj(NP - 1, clk)
        mx = qk(0)
        for g in range(4):
            t0 = clk.t
            del ends[:]
            run(PLAN[g])
            t1 = clk.t
            nxt = qk(g + 1) if g < 3 else None
            n_rough = [2 * jp * T // (GS * LSUB) for jp in (2 * g, 2 * g + 1)]
            n_near = [(T + T // 2) // GS, (3 * T + T // 2) // GS]
            holes = [(t - PH0, t + PH1) for t in ends]
            if g < 3:
                vfin(g, clk.pacer(t0 - VB, t0 + VW, 32))
                holes += [(t0, t0 + VW), (t1 - HOLE0, t1 + HOLE1)]
            if g == 2:
                vfin(3, clk.pacer(clk.t - SLACK - VW // 2, clk.t - SLACK, 32))
                holes.append((clk.t - SLACK - VW // 2, clk.t))
            tie = clk.pacer(t0 + D0, (clk.t if g else t1) - SLACK,
                            sum(n_rough) + sum(n_near) + FW * g * 8 * T // GS, holes)
            rough(2 * g, mx[0], tie)
            near(2 * g, tie, n_rough[0])
            k = n_rough[0] + n_near[0]
            rough(2 * g + 1, mx[1], lambda x, i: tie(x, k + i))
            near(2 * g + 1, tie, k + n_rough[1])
            far(g, tie, k + n_rough[1] + n_near[1])
            if g == 0:
                prep_wo(clk.pacer(t0 + VW, t1 - HOLE0, HM // 16))
            mx = nxt
        t0 = clk.t
        run(PLAN[4])
        prep_w(jnp.minimum(h + 1, H - 1), range(NT1), clk.pacer(t0 - PW0, clk.t - 300, 8 * NT1))
        if os.environ.get('SHOW'):
            print('final loads', clk.load)

    head(**head_refs)

    @pl.when(h == H - 1)
    def _():
        oproj(NP - 1, _Clock(zero_s))
        out_copy(NP - 1).start()
        for jp in range(NP):
            out_copy(jp).wait()


@jax.jit
def pallas_gated_mix__compressed_kv_cla__ssm_conv_s5__prompt_kernel(
    A_x: jax.Array,
    A_c_kv: jax.Array,
    A_w_q: jax.Array,
    A_w_uk: jax.Array,
    A_w_uv: jax.Array,
    A_w_o: jax.Array,
    B_x: jax.Array,
    B_Lambda_re: jax.Array,
    B_Lambda_im: jax.Array,
    B_B_re: jax.Array,
    B_B_im: jax.Array,
    B_C_re: jax.Array,
    B_C_im: jax.Array,
    B_log_dt: jax.Array,
    B_Dskip: jax.Array,
    gate_w: jax.Array,
):
    del B_x
    xT = jnp.transpose(A_x[0])
    woT = jnp.transpose(A_w_o, (0, 2, 1))
    ckv = A_c_kv.reshape(4, 4, 2, T // 2, DC)

    hbm = pl.BlockSpec(memory_space=pl.ANY)
    outT = pl.pallas_call(
        _kernel,
        grid=(H,),
        in_specs=[hbm] * 15,
        out_specs=hbm,
        out_shape=jax.ShapeDtypeStruct((M, S), f32),
        scratch_shapes=_SHARED_SCRATCH + list(_PROLOGUE_SCRATCH.values()) + list(_HEAD_SCRATCH.values()),
        compiler_params=pltpu.CompilerParams(
            dimension_semantics=("arbitrary",),
            vmem_limit_bytes=126 * 1024 * 1024,
        ),
    )(xT, B_B_re, B_B_im, B_C_re, B_C_im, B_Lambda_re, B_Lambda_im, B_log_dt,
      B_Dskip, gate_w, woT, ckv, A_w_q, A_w_uk, A_w_uv)
    return jnp.transpose(outT)[None]
```

```python
import bisect
import os

import jax
import jax.numpy as jnp
from jax import lax
import jax.experimental.pallas as pl
import jax.experimental.pallas.tpu as pltpu

S = 2048
M = 448
H = 16
D = 256
DC = 1024
T = 128
NP = S // T // 2
HD = D // 2
HM = M // 2
QD = D // 4
QC = DC // 4
QM = M // 4
PA = 384
PB = M - PA
TA = 512
TC = 256
CS = DC // NP
NRAW = 4
LOG2E = 1.4426950408889634
NEG = -1e30

_env = lambda k, d: type(d)(os.environ.get(k, d))
GC = _env('GC', 64)
GS = _env('GS', 16)
RCH = _env('RCH', 256)
SLACK = _env('SLACK', 200)
D0 = _env('D0', 0)
NT1 = _env('NT1', 3)
LEAD = _env('LEAD', 448)
PW0 = _env('PW0', 100)
FTIE = _env('FTIE', 1)
YS = _env('YS', 2)
QR = _env('QR', 128)
QL0 = _env('QL0', 200)
QL1 = _env('QL1', 500)
SPAN = _env('SPAN', 6000)
QLATE = _env('QLATE', 0)
SC0 = _env('SC0', 0)
QH0 = _env('QH0', 0)
QH1 = _env('QH1', 1000)
AP0 = _env('AP0', 1000)
SP0 = _env('SP0', 1200)
FLAG = _env('FLAG', 40)
FW = _env('FW', 2)
HOLE0 = _env('HOLE0', 300)
HOLE1 = _env('HOLE1', 300)
VW = _env('VW', 900)
VB = _env('VB', 0)
PH0 = _env('PH0', 400)
PH1 = _env('PH1', 0)
QCH = _env('QCH', 64)
OCH = ((0, 64), (64, 64), (128, 48), (176, 48))
LSUB = _env('LSUB', 4)
PLAN = _env('PLAN', 'K107,K207,K307,P1 P0 O2 O3 P2 O0 O1 O4,O5 P3 O6').split(',')

f32 = jnp.float32
bf16 = jnp.bfloat16
u32 = jnp.uint32

SEM_VEC, SEM_B, SEM_X, SEM_WQ, SEM_C, SEM_SL, SEM_WO, SEM_OUT, SEM_WQ1 = 0, 1, 2, 6, 7, 8, 16, 17, 18
NSEM = 22

_NN = ((1,), (0,))
_NT = ((1,), (1,))
_TN = ((0,), (0,))
_TT = ((0,), (1,))


def _dot(a, b, dims):
    return lax.dot_general(a, b, (dims, ((), ())), preferred_element_type=f32)


def _cat(xs, axis):
    return xs[0] if len(xs) == 1 else jnp.concatenate(xs, axis=axis)


def _ds(lo, n, align):
    return pl.ds(lo if isinstance(lo, int) else pl.multiple_of(lo, align), n)


def _put(ref, row, col, xs, tie=None):
    x = _cat(xs, 1)
    if tie is not None:
        x = jnp.concatenate([tie(x[:8]), x[8:]], axis=0)
    ref[row // 2:(row + x.shape[0]) // 2, col:col + x.shape[1]] = pltpu.bitcast(x.astype(bf16), u32)


def _get(ref, row, nrows, col, ncols):
    return pltpu.bitcast(ref[row // 2:(row + nrows) // 2, col:col + ncols], bf16)


class _Clock:
    def __init__(self, zero_ref):
        self.masks = {(8, T): zero_ref[...] != 0.0}
        self.ticks, self.load = [], [0, 0, 0, 0]

    @property
    def t(self):
        return max(self.load)

    def dot(self, a, b, dims):
        v = _dot(a, b, dims)
        rows, depth = v.shape[0], a.shape[dims[0][0]]
        for c in range(0, v.shape[1], T):
            start = 0
            for _ in range(0, depth, T):
                k = self.load.index(min(self.load))
                start = max(start, self.load[k])
                self.load[k] += rows
            self.ticks += [(start + r + 8, (v, r, c)) for r in range(0, rows, 8)]
        return v, start

    def strassen(self, lhs, rhs, dims, split_last=False):
        jobs = -(-lhs(0).shape[dims[0][0]] // T)
        lag = sum(l + 32 <= max(self.load) for l in self.load) // jobs if jobs < 3 else 0
        order = ((1, 3, 2, 4, 0, 5, 6), (0, 1, 3, 2, 4, 5, 6), (5, 6, 1, 3, 2, 4, 0), (0, 5, 6, 1, 3, 2, 4))[lag]
        m = {}
        for n in order:
            if split_last and n == order[-1]:
                a, half = lhs(n), lhs(0).shape[0] // 2
                m[n] = jnp.concatenate([self.dot(a[:half], rhs(n), dims)[0], self.dot(a[half:], rhs(n), dims)[0]], 0)
            else:
                m[n] = self.dot(lhs(n), rhs(n), dims)[0]
        vals = [m[n] for n in range(7)]
        return lambda r=0, n=None, only=(0, 1, 2, 3), c=0, w=None: _combine(
            vals if n is None else _Tiles(vals, r, n, c, w), only, order)

    def level(self, pairs):
        base, extra = divmod((sum(self.load) + sum(a.shape[0] for a, _ in pairs)) // 16, 4)
        target = [16 * (base + (k < extra)) for k in range(4)]
        out = []
        for a, b in pairs:
            r, parts = 0, []
            while r < a.shape[0]:
                k = self.load.index(min(self.load))
                n = min(max(target[k] - self.load[k], 16), a.shape[0] - r)
                parts.append(self.dot(a[r:r + n], b, _NN)[0])
                r += n
            out.append(_cat(parts, 0))
        return out

    def pacer(self, t0, t1, n, holes=()):
        holes = sorted((max(a, t0), min(b, t1)) for a, b in holes if a < t1 and b > t0)
        gap = sum(b - a for a, b in holes)
        ticks = sorted(self.ticks, key=lambda tw: tw[0])
        times = [tw[0] for tw in ticks]

        def tie(x, k, distinct=False, delay=0):
            t = t0 + (t1 - t0 - gap) * k / n
            for a, b in holes:
                t += b - a if t > a else 0
            t += delay
            past = ticks[:bisect.bisect_right(times, t)]
            reps = (x.shape[0] // 8, x.shape[1] // T)
            if len(past) < (reps[1] if distinct else 1):
                return x
            tick = _cat([v[r:r + 8, c:c + T] for _, (v, r, c) in past[-reps[1] if distinct else -1:]], 1)
            if tick.dtype != x.dtype:
                tick = pltpu.bitcast(tick, x.dtype)
            if x.shape not in self.masks:
                self.masks[x.shape] = jnp.tile(self.masks[(8, T)], reps)
            return lax.select(self.masks[x.shape], tick if tick.shape == x.shape else jnp.tile(tick, reps), x)
        return tie


def _no_tie(x, k):
    return x


_A_TERMS = ((0, 3, 1), (2, 3, 1), (0, None, 0), (3, None, 0), (0, 1, 1), (2, 0, -1), (1, 3, -1))
_B_TERMS = ((0, 3, 1), (0, None, 0), (1, 3, -1), (2, 0, -1), (3, None, 0), (0, 1, 1), (2, 3, 1))


def _operand(term, block):
    x, y, sign = term
    if y is None:
        return block(x)
    return block(x) + block(y) if sign > 0 else block(x) - block(y)


def _operands(terms, blocks):
    return [_operand(t, blocks.__getitem__) for t in terms]


def _operands2(terms, n1, block, tie):
    first = terms[n1][0]
    sub = [_operand(terms[n1], lambda o: tie(block(o, q)) if o == first and q in (0, 3) else block(o, q))
           for q in range(4)]
    return _operands(terms, sub)


_C_TERMS = ({0: 1, 3: 1, 4: -1, 6: 1}, {2: 1, 4: 1}, {1: 1, 3: 1}, {0: 1, 1: -1, 2: 1, 5: 1})


def _combine(m, only=(0, 1, 2, 3), order=(1, 3, 2, 4, 0, 5, 6)):
    out = []
    for terms in (_C_TERMS[n] for n in only):
        seq = [n for n in order if n in terms]
        if terms[seq[0]] < 0:
            seq[0], seq[1] = seq[1], seq[0]
        acc = m[seq[0]]
        for n in seq[1:]:
            acc = acc + m[n] if terms[n] > 0 else acc - m[n]
        out.append(acc)
    return out


def _outer_step(m_s, n1, row, v):
    n = v.shape[0]
    if n1 < 5:
        m_s[n1 * HD + row:n1 * HD + row + n, :] = v
    if n1 < 3:
        return None
    blk = (2, 1, 3, 0)[n1 - 3]
    m = {j: v if j == n1 else m_s[j * HD + row:j * HD + row + n, :] for j in _C_TERMS[blk]}
    return blk, _combine(m, (blk,), range(7))[0]


class _Tiles:
    def __init__(self, vals, r, n, c=0, w=None):
        self.vals, self.idx, self.cache = vals, (slice(r, r + n), slice(c, None if w is None else c + w)), {}

    def __getitem__(self, i):
        if i not in self.cache:
            self.cache[i] = self.vals[i][self.idx]
        return self.cache[i]


class _Reducer:
    def __init__(self, red, comb):
        self.red, self.comb, self.acc, self.rows, self.out = red, comb, None, 0, None

    def add(self, v):
        self.rows += 8 * v.shape[0]
        v = self.red(v, axis=0)
        self.acc = v if self.acc is None else self.comb(self.acc, v)
        if self.rows >= RCH:
            self.result()

    def result(self):
        if self.acc is not None:
            v = self.red(self.acc, axis=0, keepdims=True)
            self.out = v if self.out is None else self.comb(self.out, v)
        self.acc, self.rows = None, 0
        return self.out


def _cmul(ar, ai, br, bi):
    return ar * br - ai * bi, ar * bi + ai * br


def _hi16(w):
    return pltpu.bitcast(w & jnp.uint32(0xFFFF0000), f32)


def _stage(raw, stg, c0, nc, tie, groups=(0, 1)):
    for ht in groups:
        for dt in range(2):
            v = raw[c0:c0 + nc, ht * 8:(ht + 1) * 8, dt * T:(dt + 1) * T].reshape(nc * 8, T)
            stg[ht * 2 + dt, c0 * 4:(c0 + nc) * 4, :] = tie(pltpu.bitcast(v, u32))


def _ssm_params(vec_s, coef_s, lam_s, col_s):
    row = lambda r: r[...].astype(f32).reshape(1, M)
    lre, lim, ldt, dsk, gw = [row(v) for v in vec_s]
    dt = jnp.exp(ldt).astype(bf16).astype(f32)
    mag = jnp.exp(dt * lre)
    ang = dt * lim
    lr, li = mag * jnp.cos(ang), mag * jnp.sin(ang)
    den = lre * lre + lim * lim
    nr = lr - 1.0
    coef_s[...] = jnp.zeros(coef_s.shape, f32)
    coef_s[0:1, 0:M] = 2.0 * ((nr * lre + li * lim) / den)
    coef_s[1:2, 0:M] = 2.0 * ((li * lre - nr * lim) / den)

    er = jnp.concatenate([lr, lr[:, PA:]], axis=1)
    ei = jnp.concatenate([li, -li[:, PA:]], axis=1)
    pw = [(er, ei)]
    for _ in range(7):
        pw.append(_cmul(pw[-1][0], pw[-1][1], er, ei))
    sub = lax.broadcasted_iota(jnp.int32, (8, 512), 0)
    for n, d in enumerate((1, 2, 4)):
        lam_s[2 * n] = jnp.where(sub >= d, pw[d - 1][0], 0.0)
        lam_s[2 * n + 1] = jnp.where(sub >= d, pw[d - 1][1], 0.0)
    lcr = jnp.zeros((8, 512), f32)
    lci = jnp.zeros((8, 512), f32)
    for r in range(8):
        lcr = jnp.where(sub == r, pw[r][0], lcr)
        lci = jnp.where(sub == r, pw[r][1], lci)
    lam_s[6] = lcr
    lam_s[7] = lci

    def col(v):
        v = jnp.concatenate([v, jnp.zeros((1, 512 - M), f32)], axis=1)
        return jnp.broadcast_to(v, (T, 512)).T[:M]
    col_s[0] = col(dsk)
    col_s[1] = col(gw)


def _ssm_cmat(craw_s, coef_s, c_s, tie):
    for r in range(0, M, 16):
        coef = tie(coef_s[...], r // 16)
        cr, ci = coef[0:1, :M], coef[1:2, :M]
        re, im = _cmul(craw_s[0, r:r + 16, :].astype(f32), craw_s[1, r:r + 16, :].astype(f32), cr, ci)
        _put(c_s, r, 0, [re[:, :PA], -im[:, :PA], re[:, PA:], -im[:, PA:]])


def _ssm_scan(u_ref, carry, lam_s, h_s, tie):
    car, cai = carry
    out = []
    for b in range(TC // 8):
        mixed = u_ref[3, b, :, 0:T]
        u = jnp.concatenate([u_ref[cb, b] for cb in range(3)], axis=1)
        cols = [u[:, 0:T], u[:, T:2 * T], u[:, 2 * T:PA], mixed]
        hr = jnp.concatenate([tie(v, 4 * b + n) for n, v in enumerate(cols)], axis=1)
        hi = jnp.concatenate([u[:, PA:2 * PA], pltpu.roll(mixed, PB, 1)], axis=1)
        for n, d in enumerate((1, 2, 4)):
            sr, si = pltpu.roll(hr, d, 0), pltpu.roll(hi, d, 0)
            tr, ti = _cmul(sr, si, lam_s[2 * n], lam_s[2 * n + 1])
            hr, hi = hr + tr, hi + ti
        tr, ti = _cmul(lam_s[6], lam_s[7], car, cai)
        hr, hi = hr + tr, hi + ti
        car, cai = hr[7:8, :], hi[7:8, :]
        out.append(jnp.concatenate([hr[:, :PA], hi[:, :PA], hr[:, PA:]], axis=1))
        if b % 2 == 1:
            _put(h_s, (b - 1) * 8, 0, [jnp.concatenate(out, axis=0)])
            out = []
    return car, cai


_vmem = pltpu.VMEM
_PROLOGUE_SCRATCH = dict(
    xT_s=_vmem((M, S), bf16),
    v0=_vmem((M,), bf16), v1=_vmem((M,), bf16), v2=_vmem((M,), bf16), v3=_vmem((M,), bf16), v4=_vmem((M,), bf16),
    b_s=_vmem((2 * M, M), bf16),
    craw_s=_vmem((2, M, M), bf16),
    c_s=_vmem((M // 2, 2 * M), u32),
    coef_s=_vmem((8, 512), f32),
    lam_s=_vmem((8, 8, 512), f32),
    col_s=_vmem((2, M, T), f32),
    h_s=_vmem((TC // 2, 2 * M), u32),
    ckv_s=_vmem((NRAW, 4, T // 2, DC), bf16),
    rq=_vmem((M, H, D), bf16),
    rk=_vmem((NRAW * CS, H, D), bf16),
    rv=_vmem((NRAW * CS, H, D), bf16),
    sq=_vmem((4, M * 4, T), u32),
    sk=_vmem((4, CS * 4, T), u32),
    sv=_vmem((4, CS * 4, T), u32),
    wqt_s=_vmem((D, 4 * T), u32),
)
_HEAD_SCRATCH = dict(
    mk_s=_vmem((7 * HD, 2 * T), f32),
    mv_s=_vmem((2, 7 * HD, 2 * T), f32),
    mp_s=_vmem((7 * HD, 2 * T), f32),
    kt_s=_vmem((2 * T, 4 * T), f32),
    ka_s=_vmem((S // 4, 9 * T), u32),
    va_s=_vmem((HD // 2, NP * 9 * T), u32),
    v2_s=_vmem((QD // 2, 3 * 49 * T), u32),
    s_s=_vmem((4, S // 8, 8, 2 * T), f32),
    pb_s=_vmem((2 * T, 7 * T), u32),
    pd_s=_vmem((S // 2, 2 * T), u32),
    p2_s=_vmem((3 * T, 49 * T), u32),
    sc_s=_vmem((1, S), f32),
    qb_s=_vmem((HD // 2, 14 * T), u32),
)
_SHARED_SCRATCH = [
    _vmem((H // 2 * D, DC), u32),
    _vmem((H // 2 * D, DC), u32),
    _vmem((S // 8, 49 * QC), u32),
    _vmem((H * D, S // 2), u32),
    _vmem((H, M, D), bf16),
    _vmem((QD, 49 * QC), u32),
    _vmem((HM // 2, 7 * T), u32),
    _vmem((HD // 2, NP * 7 * T), u32),
    _vmem((M, S), f32),
    _vmem((1, S), f32),
    _vmem((8, T), f32),
    pltpu.SemaphoreType.DMA((NSEM,)),
]


def _kernel(xT_hbm, bre_hbm, bim_hbm, cre_hbm, cim_hbm, lre_hbm, lim_hbm, ldt_hbm,
            dsk_hbm, gw_hbm, woT_hbm, ckv_hbm, wq_hbm, wk_hbm, wv_hbm,
            out_hbm,
            wkt_s, wvt_s, a_s, q_s, wo_s, w_s, wl_s, cl_s, o_s, g_s, zero_s, sem, *rest):
    h = pl.program_id(0)
    pro_refs = dict(zip(_PROLOGUE_SCRATCH, rest))
    head_refs = dict(zip(_HEAD_SCRATCH, rest[len(pro_refs):]))

    def out_copy(jp):
        cols = pl.ds(jp * 2 * T, 2 * T)
        return pltpu.make_async_copy(o_s.at[:, cols], out_hbm.at[:, cols], sem.at[SEM_OUT])

    def prep_w(hh, outer, tie):
        rows = _ds(lax.shift_right_logical(hh, 1) * D, D, D)
        sh = (16 * (1 - (hh & 1))).astype(u32)
        k = 0
        for row0, wt_s in ((0, wkt_s.at[rows]), (QD, wvt_s.at[rows])):
            for r in range(0, QD, 16):
                def block(o, q):
                    row = (o % 2) * HD + (q % 2) * QD + r
                    col = (o // 2) * 2 * QC + (q // 2) * QC
                    return _hi16(wt_s[row:row + 16, col:col + QC] << sh)
                for n1 in outer:
                    _put(w_s, row0 + r, 7 * n1 * QC, _operands2(_B_TERMS, n1, block, lambda x: tie(x, k)))
                    k += 1

    def prologue(xT_s, v0, v1, v2, v3, v4, b_s, craw_s, c_s, coef_s, lam_s, col_s, h_s,
                 ckv_s, rq, rk, rv, sq, sk, sv, wqt_s):
        xa_s = head_refs['p2_s']
        wq_s = xa_s.at[2 * QM:2 * QM + QD]
        u_s = head_refs['s_s']
        vec_s = (v0, v1, v2, v3, v4)

        def slice_copies(i):
            s = sem.at[SEM_SL + i]
            grp = i // 2 if isinstance(i, int) else lax.shift_right_logical(i, 1)
            cs, dst = pl.ds(i * CS, CS), pl.ds((i & (NRAW - 1)) * CS, CS)
            return [pltpu.make_async_copy(ckv_hbm.at[grp, :, i & 1], ckv_s.at[i & (NRAW - 1)], s),
                    pltpu.make_async_copy(wk_hbm.at[cs], rk.at[dst], s),
                    pltpu.make_async_copy(wv_hbm.at[cs], rv.at[dst], s)]

        def wq1_copy(i):
            rows = pl.ds(i * (M // 4), M // 4)
            return pltpu.make_async_copy(wq_hbm.at[rows, 8:16], rq.at[rows, 8:16], sem.at[SEM_WQ1 + i])

        def x_copy(i):
            cols = pl.ds(i * TA, TA)
            return pltpu.make_async_copy(xT_hbm.at[:, cols], xT_s.at[:, cols], sem.at[SEM_X + i])

        cp_vec = [pltpu.make_async_copy(src, dst, sem.at[SEM_VEC])
                  for src, dst in zip((lre_hbm, lim_hbm, ldt_hbm, dsk_hbm, gw_hbm), vec_s)]
        cp_b = [pltpu.make_async_copy(src.at[pl.ds(lo, n)], b_s.at[pl.ds(dst, n)], sem.at[SEM_B])
                for src, lo, n, dst in ((bre_hbm, 0, PA, 0), (bim_hbm, 0, PA, PA),
                                        (bre_hbm, PA, PB, 2 * PA), (bim_hbm, PA, PB, 2 * PA + PB))]
        cp_wq = [pltpu.make_async_copy(wq_hbm.at[:, 0:8], rq.at[:, 0:8], sem.at[SEM_WQ])]
        cp_c = [pltpu.make_async_copy(src, craw_s.at[n], sem.at[SEM_C])
                for n, src in enumerate((cre_hbm, cim_hbm))]
        cp_wo = pltpu.make_async_copy(woT_hbm, wo_s, sem.at[SEM_WO])
        for cp in cp_vec + cp_b + [x_copy(i) for i in range(S // TA)] + cp_c + cp_wq:
            cp.start()
        for i in range(NRAW - 1):
            for cp in [wq1_copy(i)] + slice_copies(i):
                cp.start()
        wq1_copy(3).start()
        cp_wo.start()

        zero_s[...] = jnp.zeros(zero_s.shape, f32)
        wl_s[...] = jnp.zeros(wl_s.shape, u32)
        cl_s[:, (NP - 1) * 7 * T:] = jnp.zeros((HD // 2, 7 * T), u32)
        for cp in cp_vec:
            cp.wait()
        _ssm_params(vec_s, coef_s, lam_s, col_s)

        def wq_transpose(pair, tie):
            ht = pair // 4 if isinstance(pair, int) else lax.shift_right_logical(pair, 2)
            pad = jnp.zeros((T - QM, T), u32)
            for dt in range(2):
                for mq in range(4):
                    blk = sq[ht * 2 + dt, pl.ds(mq * QM * 4 + (pair & 3), QM, stride=4), :]
                    blk = jnp.concatenate([tie(blk[:8], 4 * dt + mq), blk[8:], pad], axis=0)
                    wqt_s[dt * HD:(dt + 1) * HD, mq * T:(mq + 1) * T] = blk.T

        def phase1(i):
            clk = _Clock(zero_s)
            u = _cat([clk.dot(xT_s[:, i * TA + lo:i * TA + hi], b_s[...], _TT)[0]
                      for lo, hi in ((0, T), (T, TA))], 0)
            for cb in range(4):
                w = min(2 * T, 2 * M - cb * 2 * T)
                u_s[cb, i * TA // 8:(i + 1) * TA // 8, :, 0:w] = (
                    u[:, cb * 2 * T:cb * 2 * T + w].reshape(TA // 8, 8, w))
            tie = clk.pacer(0, 6 * TA, 49)
            for r in range(0, QM, 16):
                def block(o, q):
                    row, col = (o % 2) * HM + (q % 2) * QM + r, (4 * i + 2 * (q // 2) + o // 2) * T
                    return xT_s[row:row + 16, col:col + T].astype(f32)
                for n1 in range(7):
                    ops = _operands2(_A_TERMS, n1, block, lambda x: tie(x, 7 * (r // 16) + n1))
                    _put(xa_s, i * QM + r, 7 * n1 * T, ops)
            return clk

        for cp in cp_b + [x_copy(0)]:
            cp.wait()
        phase1(0)
        x_copy(1).wait()
        clk = phase1(1)
        zero = jnp.zeros((1, 512), f32)
        carry0 = _ssm_scan(u_s.at[:, 0:TC // 8], (zero, zero), lam_s, h_s, clk.pacer(0, 6 * TA, TC // 2))
        for cp in [x_copy(2), x_copy(3)] + cp_c + cp_wq:
            cp.wait()
        _ssm_cmat(craw_s, coef_s, c_s, phase1(2).pacer(0, 6 * TA, M // 16))
        tie = phase1(3).pacer(0, 6 * TA, M // 8)
        for c0 in range(0, M, 8):
            _stage(rq, sq, c0, 8, lambda x: tie(x, c0 // 10), groups=(0,))
        wq_transpose(0, lambda x, k: tie(x, 46 + k))

        def phase2(i, carry):
            @pl.when(i + NRAW - 1 < NP)
            def _():
                for cp in slice_copies(i + NRAW - 1):
                    cp.start()

            @pl.when(i < 4)
            def _():
                wq1_copy(i).wait()

            for cp in slice_copies(i):
                cp.wait()

            clk = _Clock(zero_s)
            yT = _cat([clk.dot(_get(c_s, r, M // YS, 0, 2 * M), _get(h_s, 0, TC, 0, 2 * M), _NT)[0]
                       for r in range(0, M, M // YS)], 0)
            ty = clk.t
            for t in range(TC // T):
                cols = _ds(i * TC + t * T, T, T)
                acc = jnp.zeros((8, T), f32)
                for r in range(0, M, 32):
                    xg = xT_s[r:r + 32, cols].astype(f32) * col_s[1, r:r + 32, :]
                    acc = acc + jnp.sum(xg.reshape(4, 8, T), axis=0)
                g = jax.nn.sigmoid(jnp.sum(acc, axis=0, keepdims=True))
                g_s[:, cols] = g
                for r in range(0, M, 32):
                    skip = xT_s[r:r + 32, cols].astype(f32) * col_s[0, r:r + 32, :]
                    o_s[r:r + 32, cols] = (1.0 - g) * (yT[r:r + 32, t * T:(t + 1) * T] + skip)

            q_i = q_s.at[_ds(i * 2 * D, 2 * D, 2 * D)]
            mq_s = (head_refs['mk_s'], head_refs['mp_s'], head_refs['mv_s'].at[0], head_refs['mv_s'].at[1])
            for g in range(4):
                for n1 in range(7):
                    if g == 0:
                        t = QL0 + (ty + 6 * 224 - QL1 - QL0) * n1 / 7
                        tie = clk.pacer(min(t, clk.t - QL1), min(t + 300, clk.t - QL1), 8)
                        for r in range(0, 2 * QD, 16):
                            def block(o, q):
                                row = (o % 2) * HD + (q % 2) * QD + r % QD
                                col = (2 * (o // 2) + q // 2) * T
                                w = wqt_s[row:row + 16, col:col + T]
                                return _hi16(w) if r >= QD else pltpu.bitcast(w << 16, f32)
                            _put(wq_s, r, 7 * n1 * T, _operands2(_B_TERMS, n1, block, lambda x: tie(x, r // 16)),
                                 (lambda w: tie(w, r // 16, True, FLAG)) if QLATE else None)
                    for r0 in range(0, 2 * QD, QR):
                        comb = clk.strassen(lambda n: _get(wq_s, r0, QR, (7 * n1 + n) * T, QM),
                                            lambda n: _get(xa_s, g * QM, QM, (7 * n1 + n) * T, T), _NN)
                        for r in range(0, QR, 32):
                            e, c = (r0 + r) // QD, comb(r, 32)
                            for dq in range(2):
                                row = dq * QD + r % QD
                                done = _outer_step(mq_s[2 * (g % 2) + e], n1, row,
                                                   jnp.concatenate([c[dq], c[2 + dq]], axis=1))
                                if done:
                                    n, v = done
                                    _put(q_i, (2 * e + n // 2) * D + (n % 2) * HD + row, 2 * g * T,
                                         [v * (LOG2E * D ** -0.5)])

            span = ty + SPAN

            u_next = u_s.at[:, pl.ds(jnp.minimum(i + 1, NP - 1) * (TC // 8), TC // 8)]
            carry = _ssm_scan(u_next, carry, lam_s, h_s, clk.pacer(ty + SC0, span, TC // 2))

            tie = clk.pacer(ty - SP0, span, 64, [(ty + QH0, ty + QH1)])
            rq_i = rq.at[pl.ds((i & 3) * (M // 4), M // 4)]
            sq_i = sq.at[:, _ds((i & 3) * M, M, 8)]
            for c0 in range(0, M // 4, 8):
                _stage(rq_i, sq_i, c0, 8, lambda x: tie(x, c0 // 4 + 2), groups=(1,))
            wq_transpose(jnp.minimum(i + 1, NP - 1), lambda x, k: tie(x, 36 + 3 * k))
            slot = pl.ds((i & (NRAW - 1)) * CS, CS)
            for n, (raw, stg, wt_s) in enumerate(((rk, sk, wkt_s), (rv, sv, wvt_s))):
                for c0 in range(0, CS, 8):
                    _stage(raw.at[slot], stg, c0, 8, lambda x: tie(x, 16 * n + c0 // 8))
                cols = _ds(i * CS, CS, CS)
                for pair in range(H // 2):
                    for dt in range(2):
                        blk = stg[(pair // 4) * 2 + dt, pl.ds(pair % 4, CS, stride=4), :]
                        row = pair * D + dt * HD
                        blk = jnp.concatenate([tie(blk[:8], 16 + 24 * n + 3 * pair + dt), blk[8:]], axis=0)
                        wt_s[row:row + HD, cols] = blk.T

            tie = clk.pacer(ty + AP0, span, 28)
            ckv_i = ckv_s.at[i & (NRAW - 1)]
            a_i = a_s.at[_ds(i * (T // 4), T // 4, T // 4)]
            for r in range(0, T // 2, 16):
                def block(o, q):
                    col = (o % 2) * 2 * QC + (q % 2) * QC
                    return ckv_i[2 * (q // 2) + o // 2, r:r + 16, col:col + QC].astype(f32)
                for n1 in range(7):
                    ops = _operands2(_A_TERMS, n1, block, lambda x: tie(x, 7 * (r // 16) + n1))
                    _put(a_i, r, 7 * n1 * QC, ops)
            return carry

        lax.fori_loop(0, NP, phase2, carry0)
        cp_wo.wait()
        prep_w(h, range(NT1), _no_tie)

    @pl.when(h == 0)
    def _():
        prologue(**pro_refs)

    def oproj(jp, clk):
        cols = slice(2 * jp * T, (2 * jp + 2) * T)
        for r, n in OCH:
            c = clk.strassen(lambda i: _get(wl_s, r, n, i * T, T),
                             lambda i: _get(cl_s, 0, HD, (jp * 7 + i) * T, T), _NN)()
            o_s[r:r + n, cols] += jnp.concatenate(c[:2], axis=1)
            o_s[HM + r:HM + r + n, cols] += jnp.concatenate(c[2:], axis=1)

    def head(mk_s, mv_s, mp_s, kt_s, ka_s, va_s, v2_s, s_s, pb_s, pd_s, p2_s, sc_s, qb_s):
        clk = _Clock(zero_s)
        q_h = q_s.at[_ds(h * D, D, D)]

        def prep_wo(tie):
            for r in range(0, HM, 16):
                top = tie(wo_s[h, r:r + 16, :].astype(f32), r // 16)
                bot = tie(wo_s[h, HM + r:HM + r + 16, :].astype(f32), r // 16)
                _put(wl_s, r, 0, _operands(_A_TERMS, [top[:, :HD], top[:, HD:], bot[:, :HD], bot[:, HD:]]))

        nine = lambda c: _operands(_A_TERMS, c) + [c[1], c[2]]

        def outer(m_s, r):
            return _combine([m_s[n * HD + r:n * HD + r + 16, :] for n in range(7)], order=range(7))

        def proj(g, lo, hi):
            for n1 in range(lo, hi):
                comb = clk.strassen(lambda n: _get(w_s, 0, 2 * QD, (7 * n1 + n) * QC, QC),
                                    lambda n: _get(a_s, g * T, T, (7 * n1 + n) * QC, QC), _NT, n1 == 6)
                for r in range(0, 2 * QD, GC):
                    m_s, row = mk_s if r < QD else mv_s.at[g % 2], n1 * HD + r % QD
                    c = comb(r, GC)
                    m_s[row:row + GC, :] = jnp.concatenate([c[0], c[2]], axis=1)
                    m_s[QD + row:QD + row + GC, :] = jnp.concatenate([c[1], c[3]], axis=1)
            if hi < 7:
                return
            cs = [outer(mk_s, r) for r in range(0, HD, 16)]
            for n in range(4):
                kt_s[:, n * T:(n + 1) * T] = jnp.concatenate([c[n] for c in cs], axis=0).T
            for r in range(0, 2 * T, GC):
                blk = kt_s[r:r + GC, :]
                _put(ka_s, 2 * g * T + r, 0, nine([blk[:, n * T:(n + 1) * T] for n in range(4)]))

        def vfin(g, tie):
            m_s = mv_s.at[g % 2]
            for r in range(0, QD, 16):
                k, blk = 8 * (r // 16), {}
                late = lambda w: tie(w, k, True, FLAG)
                for new, n1 in (((0,), 2), ((1,), 4), ((3,), 6), ((), 0), ((), 3), ((2,), 5), ((), 1)):
                    for o in new:
                        for i, row in enumerate((r, QD + r)):
                            tiles = _Tiles([m_s.at[n * HD:(n + 1) * HD] for n in range(7)], row, 16)
                            c, = _combine(tiles, ((o % 2) * 2 + o // 2,), range(7))
                            blk[o, i] = c = tie(c, k)
                            slot = (2, 7, 8, 3)[o]
                            _put(va_s, row, ((2 * g + 1) * 9 + slot) * T, [c[:, T:]])
                            if o in (1, 2):
                                _put(va_s, row, (2 * g * 9 + slot) * T, [c[:, :T]])
                    lo_, hi_ = [_operand(_A_TERMS[n1], lambda o: blk[o, i]) for i in range(2)]
                    _put(va_s, r, (2 * g * 9 + n1) * T, [lo_[:, :T]], late)
                    _put(va_s, QD + r, (2 * g * 9 + n1) * T, [hi_[:, :T]], late)
                    if g < 3:
                        _put(v2_s, r, (g * 7 + n1) * 7 * T,
                             _operands(_A_TERMS, [lo_[:, :T], lo_[:, T:], hi_[:, :T], hi_[:, T:]]), late)
                    k += 8 / 7

        key = lax.broadcasted_iota(jnp.int32, (T, 2 * T), 0)
        qry = lax.broadcasted_iota(jnp.int32, (T, 2 * T), 1)
        causal = key <= qry

        def qk(g):
            pairs = (2 * g, 2 * g + 1)
            mx = {jp: _Reducer(jnp.max, jnp.maximum) for jp in pairs}

            def put(jp, row, v):
                v = v.reshape(v.shape[0] // 8, 8, 2 * T)
                s_s[jp % 4, row // 8:row // 8 + v.shape[0]] = v
                mx[jp].add(v)

            def rect(jp, lo, hi, n):
                for r in range(lo, hi, n):
                    c = clk.strassen(lambda i: _get(ka_s, r, n, i * T, T),
                                     lambda i: _get(qb_s, 0, HD, ((jp % 2) * 7 + i) * T, T), _NN)()
                    put(jp, r, jnp.concatenate(c[:2], axis=1))
                    put(jp, jp * T + r, jnp.concatenate(c[2:], axis=1))

            q = lambda jp, e: _get(q_h, e * D, D, jp * T, T)
            for jp in pairs[g == 0:]:
                for r in range(0, HD, 32):
                    blk = [_get(q_h, e * D + d * HD + r, 32, jp * T, T).astype(f32) for d in range(2) for e in range(2)]
                    _put(qb_s, r, (jp % 2) * 7 * T, _operands(_B_TERMS, blk))
            for jp in pairs:
                rect(jp, 0, 2 * g * T, QCH if QCH else g * T // 2 or 1)
            kb = lambda jp, a, b: jnp.concatenate(
                [_get(ka_s, jp * T, T, a * T, T), _get(ka_s, jp * T, T, b * T, T)], axis=1)
            for jp in pairs:
                se, _ = clk.dot(kb(jp, 2, 7), jnp.concatenate([q(jp, 0), q(jp, 1)], axis=1), _NN)
                put(jp, 2 * jp * T, jnp.where(causal, se, NEG))
            last = {}
            for jp in pairs:
                so = jnp.where(causal[:, :T], clk.dot(kb(jp, 8, 3), q(jp, 1), _NN)[0], NEG)
                row = (2 * jp + 1) * T // 8
                s_s[jp % 4, row:row + T // 8, :, T:] = so.reshape(T // 8, 8, T)
                last[jp] = jnp.concatenate([jnp.full((1, T), NEG, f32), jnp.max(so, axis=0, keepdims=True)], axis=1)
            rect(2 * g + 1, 2 * g * T, (2 * g + 1) * T, T // 4)
            return [jnp.broadcast_to(jnp.maximum(mx[jp].result(), last[jp]), (8, 2 * T)) for jp in pairs]

        zs, sums = {}, {}

        def prob(jp, row, z, n=GS, lanes=slice(None)):
            return jnp.exp2(s_s[jp % 4, row // 8:(row + n) // 8, :, lanes] - z[:, lanes])

        def rough(jp, mx, tie):
            zs[jp] = mx
            if jp > 0:
                sm = _Reducer(jnp.sum, jnp.add)
                for k, r in enumerate(range(0, 2 * jp * T, GS * LSUB)):
                    sm.add(prob(jp, r, tie(mx, k)))
                zs[jp] = mx + jnp.log2(jnp.maximum(LSUB * sm.result(), 1.0))
            sums[jp] = _Reducer(jnp.sum, jnp.add)

        def blocks(jp, row, tie, k):
            top, bot = prob(jp, row, tie(zs[jp], k)), prob(jp, jp * T + row, tie(zs[jp], k + 1))
            sums[jp].add(top + bot)
            top, bot = top.reshape(GS, 2 * T), bot.reshape(GS, 2 * T)
            return [top[:, :T], top[:, T:], bot[:, :T], bot[:, T:]]

        def near(jp, tie, k):
            R, z = jp * T, zs[jp]
            if jp % 2:
                for r in range(0, T, GS):
                    _put(pb_s, jp // 2 * T + r, 0, _operands(_B_TERMS, blocks(jp, R - T + r, tie, k)))
                    k += 2
            for r in range(0, T, GS):
                p = prob(jp, 2 * R + r, tie(z, k))
                sums[jp].add(p)
                _put(pd_s, 2 * R + r, 0, [p.reshape(GS, 2 * T)])
                k += 1
            so = _Reducer(jnp.sum, jnp.add)
            for r in range(0, T, 2 * GS):
                p = prob(jp, 2 * R + T + r, tie(z, k), 2 * GS, slice(T, 2 * T))
                so.add(p)
                _put(pd_s, 2 * R + T + r, T, [p.reshape(2 * GS, T)])
                k += 1
            sums[jp].result()
            sums[jp].out = sums[jp].out + jnp.concatenate([jnp.zeros((1, T), f32), so.result()], axis=1)

        p20 = lambda g: g * (g - 1) // 2 * T

        def far(g, tie, k):
            half = {(jp, e): _Reducer(jnp.sum, jnp.add) for jp in (2 * g, 2 * g + 1) for e in range(2)}
            for kg in range(g):
                for r in range(0, T, GS):
                    blk = {}
                    for new, n1 in (((0,), 1), ((1,), 5), ((3,), 2), ((), 0), ((), 4), ((2,), 3), ((), 6)):
                        for o in new:
                            lanes = slice((o % 2) * T, (o % 2 + 1) * T)
                            for jp in (2 * g, 2 * g + 1):
                                z = tie(zs[jp][:, lanes], k)
                                row = (o // 2) * jp * T + 2 * kg * T + r
                                p = [jnp.exp2(s_s[jp % 4, x // 8:(x + GS) // 8, :, lanes] - z) for x in (row, row + T)]
                                half[jp, o % 2].add(p[0] + p[1])
                                blk[o, jp % 2], blk[o, 2 + jp % 2] = [x.reshape(GS, T) for x in p]
                        ops = _operands2(_B_TERMS, n1, lambda o, q: blk[o, q], lambda x: x)
                        _put(p2_s, p20(g) + kg * T + r, 7 * n1 * T, ops,
                             (lambda w: tie(w, k, True, FLAG)) if FTIE else None)
                        k += FW * 8 / 7
            for jp in (2 * g, 2 * g + 1):
                if g:
                    sums[jp].out = sums[jp].out + jnp.concatenate([half[jp, e].result() for e in range(2)], axis=1)
            for jp in (2 * g, 2 * g + 1):
                cols = slice(2 * jp * T, 2 * (jp + 1) * T)
                sc_s[:, cols] = g_s[:, cols] / sums[jp].result()

        def pv(g):
            pairs = (2 * g, 2 * g + 1)
            va = lambda n, t, r=0, nr=HD: _get(va_s, r, nr, (t * 9 + n) * T, T)
            for n1 in range(7 if g else 0):
                c = clk.strassen(
                    lambda n: _cat([_get(v2_s, 0, QD, (kg * 49 + 7 * n1 + n) * T, T) for kg in range(g)], 1),
                    lambda n: _get(p2_s, p20(g), g * T, (7 * n1 + n) * T, T), _NN)()
                mp_s[n1 * HD:n1 * HD + QD, :] = jnp.concatenate(c[:2], axis=1)
                mp_s[n1 * HD + QD:(n1 + 1) * HD, :] = jnp.concatenate(c[2:], axis=1)
            ve = [jnp.concatenate([va(2, jp), va(8, jp)], axis=0) for jp in pairs]
            vo = [jnp.concatenate([va(7, jp), va(3, jp)], axis=0) for jp in pairs]
            ce = clk.level([(ve[jp % 2], _get(pd_s, 2 * jp * T, T, 0, T)) for jp in pairs])
            co = [clk.dot(jnp.concatenate([ve[jp % 2], vo[jp % 2]], axis=1),
                          _get(pd_s, 2 * jp * T, 2 * T, T, T), _NN)[0] for jp in pairs]
            for jp in pairs:
                R, e = jp * T, jp % 2
                ge, go = sc_s[:, 2 * R:2 * R + T], sc_s[:, 2 * R + T:2 * R + 2 * T]
                for r in range(0, HD, 32):
                    c = [ce[e][r:r + 32], co[e][r:r + 32], ce[e][HD + r:HD + r + 32], co[e][HD + r:HD + r + 32]]
                    if g:
                        far_ = _combine([mp_s[n * HD + r:n * HD + r + 32, e * T:(e + 1) * T] for n in range(7)],
                                        order=range(7))
                        c = [x + y for x, y in zip(c, far_)]
                    if e:
                        near_ = clk.strassen(lambda n: va(n, 2 * g, r, 32),
                                             lambda n: _get(pb_s, g * T, T, n * T, T), _NN)()
                        c = [x + y for x, y in zip(c, near_)]
                    ops = _operands(_B_TERMS, [c[0] * ge, c[1] * go, c[2] * ge, c[3] * go])
                    _put(cl_s, r, jp * 7 * T, ops)

        ends = []

        def run(items):
            for item in items.split():
                if item[0] == 'P':
                    pv(int(item[1]))
                    ends.append(clk.t)
                elif item[0] == 'K':
                    proj(int(item[1]), int(item[2]), int(item[3]))
                else:
                    jp = int(item[1])
                    oproj(jp, clk)

                    @pl.when(h == H - 1)
                    def _():
                        out_copy(jp).start()

        for n1 in range(7):
            if n1 >= NT1:
                prep_w(h, [n1], clk.pacer(max(clk.t - LEAD - 448, 1), max(clk.t - LEAD, 1), 8))
            proj(0, n1, n1 + 1)
        oproj(NP - 1, clk)
        mx = qk(0)
        for g in range(4):
            t0 = clk.t
            del ends[:]
            run(PLAN[g])
            t1 = clk.t
            nxt = qk(g + 1) if g < 3 else None
            n_rough = [2 * jp * T // (GS * LSUB) for jp in (2 * g, 2 * g + 1)]
            n_near = [(T + T // 2) // GS, (3 * T + T // 2) // GS]
            holes = [(t - PH0, t + PH1) for t in ends]
            if g < 3:
                vfin(g, clk.pacer(t0 - VB, t0 + VW, 32))
                holes += [(t0, t0 + VW), (t1 - HOLE0, t1 + HOLE1)]
            if g == 2:
                vfin(3, clk.pacer(clk.t - SLACK - VW // 2, clk.t - SLACK, 32))
                holes.append((clk.t - SLACK - VW // 2, clk.t))
            tie = clk.pacer(t0 + D0, (clk.t if g else t1) - SLACK,
                            sum(n_rough) + sum(n_near) + FW * g * 8 * T // GS, holes)
            rough(2 * g, mx[0], tie)
            near(2 * g, tie, n_rough[0])
            k = n_rough[0] + n_near[0]
            rough(2 * g + 1, mx[1], lambda x, i: tie(x, k + i))
            near(2 * g + 1, tie, k + n_rough[1])
            far(g, tie, k + n_rough[1] + n_near[1])
            if g == 0:
                prep_wo(clk.pacer(t0 + VW, t1 - HOLE0, HM // 16))
            mx = nxt
        t0 = clk.t
        run(PLAN[4])
        prep_w(jnp.minimum(h + 1, H - 1), range(NT1), clk.pacer(t0 - PW0, clk.t - 300, 8 * NT1))
        if os.environ.get('SHOW'):
            print('final loads', clk.load)

    head(**head_refs)

    @pl.when(h == H - 1)
    def _():
        oproj(NP - 1, _Clock(zero_s))
        out_copy(NP - 1).start()
        for jp in range(NP):
            out_copy(jp).wait()


@jax.jit
def pallas_gated_mix__compressed_kv_cla__ssm_conv_s5__prompt_kernel(
    A_x: jax.Array,
    A_c_kv: jax.Array,
    A_w_q: jax.Array,
    A_w_uk: jax.Array,
    A_w_uv: jax.Array,
    A_w_o: jax.Array,
    B_x: jax.Array,
    B_Lambda_re: jax.Array,
    B_Lambda_im: jax.Array,
    B_B_re: jax.Array,
    B_B_im: jax.Array,
    B_C_re: jax.Array,
    B_C_im: jax.Array,
    B_log_dt: jax.Array,
    B_Dskip: jax.Array,
    gate_w: jax.Array,
):
    del B_x
    xT = jnp.transpose(A_x[0])
    woT = jnp.transpose(A_w_o, (0, 2, 1))
    ckv = A_c_kv.reshape(4, 4, 2, T // 2, DC)

    hbm = pl.BlockSpec(memory_space=pl.ANY)
    outT = pl.pallas_call(
        _kernel,
        grid=(H,),
        in_specs=[hbm] * 15,
        out_specs=hbm,
        out_shape=jax.ShapeDtypeStruct((M, S), f32),
        scratch_shapes=_SHARED_SCRATCH + list(_PROLOGUE_SCRATCH.values()) + list(_HEAD_SCRATCH.values()),
        compiler_params=pltpu.CompilerParams(
            dimension_semantics=("arbitrary",),
            vmem_limit_bytes=127 * 1024 * 1024,
        ),
    )(xT, B_B_re, B_B_im, B_C_re, B_C_im, B_Lambda_re, B_Lambda_im, B_log_dt,
      B_Dskip, gate_w, woT, ckv, A_w_q, A_w_uk, A_w_uv)
    return jnp.transpose(outT)[None]
```

```python
import bisect
import os

import jax
import jax.numpy as jnp
from jax import lax
import jax.experimental.pallas as pl
import jax.experimental.pallas.tpu as pltpu

S = 2048
M = 448
H = 16
D = 256
DC = 1024
T = 128
NP = S // T // 2
HD = D // 2
HM = M // 2
QD = D // 4
QC = DC // 4
QM = M // 4
PA = 384
PB = M - PA
TA = 512
TC = 256
CS = DC // NP
NRAW = 4
LOG2E = 1.4426950408889634
NEG = -1e30

_env = lambda k, d: type(d)(os.environ.get(k, d))
GC = _env('GC', 64)
GS = _env('GS', 16)
RCH = _env('RCH', 256)
SLACK = _env('SLACK', 200)
D0 = _env('D0', 0)
NT1 = _env('NT1', 3)
LEAD = _env('LEAD', 448)
PW0 = _env('PW0', 100)
FTIE = _env('FTIE', 1)
YS = _env('YS', 2)
QR = _env('QR', 128)
QL0 = _env('QL0', 200)
QL1 = _env('QL1', 500)
SPAN = _env('SPAN', 6000)
QLATE = _env('QLATE', 0)
SC0 = _env('SC0', 0)
QH0 = _env('QH0', 0)
QH1 = _env('QH1', 1000)
AP0 = _env('AP0', 1000)
SP0 = _env('SP0', 1200)
FLAG = _env('FLAG', 40)
FW = _env('FW', 2)
HOLE0 = _env('HOLE0', 300)
HOLE1 = _env('HOLE1', 300)
VW = _env('VW', 900)
VB = _env('VB', 0)
PH0 = _env('PH0', 400)
PH1 = _env('PH1', 0)
QCH = _env('QCH', 64)
OCH = ((0, 64), (64, 64), (128, 48), (176, 48))
LSUB = _env('LSUB', 4)
PLAN = _env('PLAN', 'K107,K207,K307,P1 P0 O2 O3 P2 O0 O1 O4,O5 P3 O6').split(',')

f32 = jnp.float32
bf16 = jnp.bfloat16
u32 = jnp.uint32

SEM_VEC, SEM_B, SEM_X, SEM_WQ, SEM_C, SEM_SL, SEM_WO, SEM_OUT, SEM_WQ1 = 0, 1, 2, 6, 7, 8, 16, 17, 18
NSEM = 22

_NN = ((1,), (0,))
_NT = ((1,), (1,))
_TN = ((0,), (0,))
_TT = ((0,), (1,))


def _dot(a, b, dims):
    return lax.dot_general(a, b, (dims, ((), ())), preferred_element_type=f32)


def _cat(xs, axis):
    return xs[0] if len(xs) == 1 else jnp.concatenate(xs, axis=axis)


def _ds(lo, n, align):
    return pl.ds(lo if isinstance(lo, int) else pl.multiple_of(lo, align), n)


def _put(ref, row, col, xs, tie=None):
    x = _cat(xs, 1)
    if tie is not None:
        x = jnp.concatenate([tie(x[:8]), x[8:]], axis=0)
    ref[row // 2:(row + x.shape[0]) // 2, col:col + x.shape[1]] = pltpu.bitcast(x.astype(bf16), u32)


def _get(ref, row, nrows, col, ncols):
    return pltpu.bitcast(ref[row // 2:(row + nrows) // 2, col:col + ncols], bf16)


class _Clock:
    def __init__(self, zero_ref):
        self.masks = {(8, T): zero_ref[...] != 0.0}
        self.ticks, self.load = [], [0, 0, 0, 0]

    @property
    def t(self):
        return max(self.load)

    def dot(self, a, b, dims):
        v = _dot(a, b, dims)
        rows, depth = v.shape[0], a.shape[dims[0][0]]
        for c in range(0, v.shape[1], T):
            start = 0
            for _ in range(0, depth, T):
                k = self.load.index(min(self.load))
                start = max(start, self.load[k])
                self.load[k] += rows
            self.ticks += [(start + r + 8, (v, r, c)) for r in range(0, rows, 8)]
        return v, start

    def strassen(self, lhs, rhs, dims, split_last=False):
        jobs = -(-lhs(0).shape[dims[0][0]] // T)
        lag = sum(l + 32 <= max(self.load) for l in self.load) // jobs if jobs < 3 else 0
        order = ((1, 3, 2, 4, 0, 5, 6), (0, 1, 3, 2, 4, 5, 6), (5, 6, 1, 3, 2, 4, 0), (0, 5, 6, 1, 3, 2, 4))[lag]
        m = {}
        for n in order:
            if split_last and n == order[-1]:
                a, half = lhs(n), lhs(0).shape[0] // 2
                m[n] = jnp.concatenate([self.dot(a[:half], rhs(n), dims)[0], self.dot(a[half:], rhs(n), dims)[0]], 0)
            else:
                m[n] = self.dot(lhs(n), rhs(n), dims)[0]
        vals = [m[n] for n in range(7)]
        return lambda r=0, n=None, only=(0, 1, 2, 3), c=0, w=None: _combine(
            vals if n is None else _Tiles(vals, r, n, c, w), only, order)

    def level(self, pairs):
        base, extra = divmod((sum(self.load) + sum(a.shape[0] for a, _ in pairs)) // 16, 4)
        target = [16 * (base + (k < extra)) for k in range(4)]
        out = []
        for a, b in pairs:
            r, parts = 0, []
            while r < a.shape[0]:
                k = self.load.index(min(self.load))
                n = min(max(target[k] - self.load[k], 16), a.shape[0] - r)
                parts.append(self.dot(a[r:r + n], b, _NN)[0])
                r += n
            out.append(_cat(parts, 0))
        return out

    def pacer(self, t0, t1, n, holes=()):
        holes = sorted((max(a, t0), min(b, t1)) for a, b in holes if a < t1 and b > t0)
        gap = sum(b - a for a, b in holes)
        ticks = sorted(self.ticks, key=lambda tw: tw[0])
        times = [tw[0] for tw in ticks]

        def tie(x, k, distinct=False, delay=0):
            t = t0 + (t1 - t0 - gap) * k / n
            for a, b in holes:
                t += b - a if t > a else 0
            t += delay
            past = ticks[:bisect.bisect_right(times, t)]
            reps = (x.shape[0] // 8, x.shape[1] // T)
            if len(past) < (reps[1] if distinct else 1):
                return x
            tick = _cat([v[r:r + 8, c:c + T] for _, (v, r, c) in past[-reps[1] if distinct else -1:]], 1)
            if tick.dtype != x.dtype:
                tick = pltpu.bitcast(tick, x.dtype)
            if x.shape not in self.masks:
                self.masks[x.shape] = jnp.tile(self.masks[(8, T)], reps)
            return lax.select(self.masks[x.shape], tick if tick.shape == x.shape else jnp.tile(tick, reps), x)
        return tie


def _no_tie(x, k):
    return x


_A_TERMS = ((0, 3, 1), (2, 3, 1), (0, None, 0), (3, None, 0), (0, 1, 1), (2, 0, -1), (1, 3, -1))
_B_TERMS = ((0, 3, 1), (0, None, 0), (1, 3, -1), (2, 0, -1), (3, None, 0), (0, 1, 1), (2, 3, 1))


def _operand(term, block):
    x, y, sign = term
    if y is None:
        return block(x)
    return block(x) + block(y) if sign > 0 else block(x) - block(y)


def _operands(terms, blocks):
    return [_operand(t, blocks.__getitem__) for t in terms]


def _operands2(terms, n1, block, tie):
    first = terms[n1][0]
    sub = [_operand(terms[n1], lambda o: tie(block(o, q)) if o == first and q in (0, 3) else block(o, q))
           for q in range(4)]
    return _operands(terms, sub)


_C_TERMS = ({0: 1, 3: 1, 4: -1, 6: 1}, {2: 1, 4: 1}, {1: 1, 3: 1}, {0: 1, 1: -1, 2: 1, 5: 1})


def _combine(m, only=(0, 1, 2, 3), order=(1, 3, 2, 4, 0, 5, 6)):
    out = []
    for terms in (_C_TERMS[n] for n in only):
        seq = [n for n in order if n in terms]
        if terms[seq[0]] < 0:
            seq[0], seq[1] = seq[1], seq[0]
        acc = m[seq[0]]
        for n in seq[1:]:
            acc = acc + m[n] if terms[n] > 0 else acc - m[n]
        out.append(acc)
    return out


def _outer_step(m_s, n1, row, v):
    n = v.shape[0]
    if n1 < 5:
        m_s[n1 * HD + row:n1 * HD + row + n, :] = v
    if n1 < 3:
        return None
    blk = (2, 1, 3, 0)[n1 - 3]
    m = {j: v if j == n1 else m_s[j * HD + row:j * HD + row + n, :] for j in _C_TERMS[blk]}
    return blk, _combine(m, (blk,), range(7))[0]


class _Tiles:
    def __init__(self, vals, r, n, c=0, w=None):
        self.vals, self.idx, self.cache = vals, (slice(r, r + n), slice(c, None if w is None else c + w)), {}

    def __getitem__(self, i):
        if i not in self.cache:
            self.cache[i] = self.vals[i][self.idx]
        return self.cache[i]


class _Reducer:
    def __init__(self, red, comb):
        self.red, self.comb, self.acc, self.rows, self.out = red, comb, None, 0, None

    def add(self, v):
        self.rows += 8 * v.shape[0]
        v = self.red(v, axis=0)
        self.acc = v if self.acc is None else self.comb(self.acc, v)
        if self.rows >= RCH:
            self.result()

    def result(self):
        if self.acc is not None:
            v = self.red(self.acc, axis=0, keepdims=True)
            self.out = v if self.out is None else self.comb(self.out, v)
        self.acc, self.rows = None, 0
        return self.out


def _cmul(ar, ai, br, bi):
    return ar * br - ai * bi, ar * bi + ai * br


def _hi16(w):
    return pltpu.bitcast(w & jnp.uint32(0xFFFF0000), f32)


def _stage(raw, stg, c0, nc, tie, groups=(0, 1)):
    for ht in groups:
        for dt in range(2):
            v = raw[c0:c0 + nc, ht * 8:(ht + 1) * 8, dt * T:(dt + 1) * T].reshape(nc * 8, T)
            stg[ht * 2 + dt, c0 * 4:(c0 + nc) * 4, :] = tie(pltpu.bitcast(v, u32))


def _ssm_params(vec_s, coef_s, lam_s, col_s):
    row = lambda r: r[...].astype(f32).reshape(1, M)
    lre, lim, ldt, dsk, gw = [row(v) for v in vec_s]
    dt = jnp.exp(ldt).astype(bf16).astype(f32)
    mag = jnp.exp(dt * lre)
    ang = dt * lim
    lr, li = mag * jnp.cos(ang), mag * jnp.sin(ang)
    den = lre * lre + lim * lim
    nr = lr - 1.0
    coef_s[...] = jnp.zeros(coef_s.shape, f32)
    coef_s[0:1, 0:M] = 2.0 * ((nr * lre + li * lim) / den)
    coef_s[1:2, 0:M] = 2.0 * ((li * lre - nr * lim) / den)

    er = jnp.concatenate([lr, lr[:, PA:]], axis=1)
    ei = jnp.concatenate([li, -li[:, PA:]], axis=1)
    pw = [(er, ei)]
    for _ in range(7):
        pw.append(_cmul(pw[-1][0], pw[-1][1], er, ei))
    sub = lax.broadcasted_iota(jnp.int32, (8, 512), 0)
    for n, d in enumerate((1, 2, 4)):
        lam_s[2 * n] = jnp.where(sub >= d, pw[d - 1][0], 0.0)
        lam_s[2 * n + 1] = jnp.where(sub >= d, pw[d - 1][1], 0.0)
    lcr = jnp.zeros((8, 512), f32)
    lci = jnp.zeros((8, 512), f32)
    for r in range(8):
        lcr = jnp.where(sub == r, pw[r][0], lcr)
        lci = jnp.where(sub == r, pw[r][1], lci)
    lam_s[6] = lcr
    lam_s[7] = lci

    def col(v):
        v = jnp.concatenate([v, jnp.zeros((1, 512 - M), f32)], axis=1)
        return jnp.broadcast_to(v, (T, 512)).T[:M]
    col_s[0] = col(dsk)
    col_s[1] = col(gw)


def _ssm_cmat(craw_s, coef_s, c_s, tie):
    for r in range(0, M, 16):
        coef = tie(coef_s[...], r // 16)
        cr, ci = coef[0:1, :M], coef[1:2, :M]
        re, im = _cmul(craw_s[0, r:r + 16, :].astype(f32), craw_s[1, r:r + 16, :].astype(f32), cr, ci)
        _put(c_s, r, 0, [re[:, :PA], -im[:, :PA], re[:, PA:], -im[:, PA:]])


def _ssm_scan(u_ref, carry, lam_s, h_s, tie):
    car, cai = carry
    out = []
    for b in range(TC // 8):
        mixed = u_ref[3, b, :, 0:T]
        u = jnp.concatenate([u_ref[cb, b] for cb in range(3)], axis=1)
        cols = [u[:, 0:T], u[:, T:2 * T], u[:, 2 * T:PA], mixed]
        hr = jnp.concatenate([tie(v, 4 * b + n) for n, v in enumerate(cols)], axis=1)
        hi = jnp.concatenate([u[:, PA:2 * PA], pltpu.roll(mixed, PB, 1)], axis=1)
        for n, d in enumerate((1, 2, 4)):
            sr, si = pltpu.roll(hr, d, 0), pltpu.roll(hi, d, 0)
            tr, ti = _cmul(sr, si, lam_s[2 * n], lam_s[2 * n + 1])
            hr, hi = hr + tr, hi + ti
        tr, ti = _cmul(lam_s[6], lam_s[7], car, cai)
        hr, hi = hr + tr, hi + ti
        car, cai = hr[7:8, :], hi[7:8, :]
        out.append(jnp.concatenate([hr[:, :PA], hi[:, :PA], hr[:, PA:]], axis=1))
        if b % 2 == 1:
            _put(h_s, (b - 1) * 8, 0, [jnp.concatenate(out, axis=0)])
            out = []
    return car, cai


_vmem = pltpu.VMEM
_PROLOGUE_SCRATCH = dict(
    xT_s=_vmem((M, S), bf16),
    v0=_vmem((M,), bf16), v1=_vmem((M,), bf16), v2=_vmem((M,), bf16), v3=_vmem((M,), bf16), v4=_vmem((M,), bf16),
    b_s=_vmem((2 * M, M), bf16),
    craw_s=_vmem((2, M, M), bf16),
    c_s=_vmem((M // 2, 2 * M), u32),
    coef_s=_vmem((8, 512), f32),
    lam_s=_vmem((8, 8, 512), f32),
    col_s=_vmem((2, M, T), f32),
    h_s=_vmem((TC // 2, 2 * M), u32),
    ckv_s=_vmem((NRAW, 4, T // 2, DC), bf16),
    rq=_vmem((M, H, D), bf16),
    rk=_vmem((NRAW * CS, H, D), bf16),
    rv=_vmem((NRAW * CS, H, D), bf16),
    sq=_vmem((4, M * 4, T), u32),
    sk=_vmem((4, CS * 4, T), u32),
    sv=_vmem((4, CS * 4, T), u32),
    wqt_s=_vmem((D, 4 * T), u32),
)
_HEAD_SCRATCH = dict(
    mk_s=_vmem((7 * HD, 2 * T), f32),
    mv_s=_vmem((2, 7 * HD, 2 * T), f32),
    mp_s=_vmem((7 * HD, 2 * T), f32),
    kt_s=_vmem((2 * T, 4 * T), f32),
    ka_s=_vmem((S // 4, 9 * T), u32),
    va_s=_vmem((HD // 2, NP * 9 * T), u32),
    v2_s=_vmem((QD // 2, 3 * 49 * T), u32),
    s_s=_vmem((4, S // 8, 8, 2 * T), f32),
    pb_s=_vmem((2 * T, 7 * T), u32),
    pd_s=_vmem((S // 2, 2 * T), u32),
    p2_s=_vmem((3 * T, 49 * T), u32),
    sc_s=_vmem((1, S), f32),
    qb_s=_vmem((HD // 2, 14 * T), u32),
)
_SHARED_SCRATCH = [
    _vmem((H // 2 * D, DC), u32),
    _vmem((H // 2 * D, DC), u32),
    _vmem((S // 8, 49 * QC), u32),
    _vmem((H * D, S // 2), u32),
    _vmem((H, M, D), bf16),
    _vmem((QD, 49 * QC), u32),
    _vmem((HM // 2, 7 * T), u32),
    _vmem((HD // 2, NP * 7 * T), u32),
    _vmem((M, S), f32),
    _vmem((1, S), f32),
    _vmem((8, T), f32),
    pltpu.SemaphoreType.DMA((NSEM,)),
]


def _kernel(xT_hbm, bre_hbm, bim_hbm, cre_hbm, cim_hbm, lre_hbm, lim_hbm, ldt_hbm,
            dsk_hbm, gw_hbm, woT_hbm, ckv_hbm, wq_hbm, wk_hbm, wv_hbm,
            out_hbm,
            wkt_s, wvt_s, a_s, q_s, wo_s, w_s, wl_s, cl_s, o_s, g_s, zero_s, sem, *rest):
    h = pl.program_id(0)
    pro_refs = dict(zip(_PROLOGUE_SCRATCH, rest))
    head_refs = dict(zip(_HEAD_SCRATCH, rest[len(pro_refs):]))

    def out_copy(jp):
        cols = pl.ds(jp * 2 * T, 2 * T)
        return pltpu.make_async_copy(o_s.at[:, cols], out_hbm.at[:, cols], sem.at[SEM_OUT])

    def prep_w(hh, outer, tie):
        rows = _ds(lax.shift_right_logical(hh, 1) * D, D, D)
        sh = (16 * (1 - (hh & 1))).astype(u32)
        k = 0
        for row0, wt_s in ((0, wkt_s.at[rows]), (QD, wvt_s.at[rows])):
            for r in range(0, QD, 16):
                def block(o, q):
                    row = (o % 2) * HD + (q % 2) * QD + r
                    col = (o // 2) * 2 * QC + (q // 2) * QC
                    return _hi16(wt_s[row:row + 16, col:col + QC] << sh)
                for n1 in outer:
                    _put(w_s, row0 + r, 7 * n1 * QC, _operands2(_B_TERMS, n1, block, lambda x: tie(x, k)))
                    k += 1

    def prologue(xT_s, v0, v1, v2, v3, v4, b_s, craw_s, c_s, coef_s, lam_s, col_s, h_s,
                 ckv_s, rq, rk, rv, sq, sk, sv, wqt_s):
        xa_s = head_refs['p2_s']
        wq_s = xa_s.at[2 * QM:2 * QM + QD]
        u_s = head_refs['s_s']
        vec_s = (v0, v1, v2, v3, v4)

        def slice_copies(i):
            s = sem.at[SEM_SL + i]
            grp = i // 2 if isinstance(i, int) else lax.shift_right_logical(i, 1)
            cs, dst = pl.ds(i * CS, CS), pl.ds((i & (NRAW - 1)) * CS, CS)
            return [pltpu.make_async_copy(ckv_hbm.at[grp, :, i & 1], ckv_s.at[i & (NRAW - 1)], s),
                    pltpu.make_async_copy(wk_hbm.at[cs], rk.at[dst], s),
                    pltpu.make_async_copy(wv_hbm.at[cs], rv.at[dst], s)]

        def wq1_copy(i):
            rows = pl.ds(i * (M // 4), M // 4)
            return pltpu.make_async_copy(wq_hbm.at[rows, 8:16], rq.at[rows, 8:16], sem.at[SEM_WQ1 + i])

        def x_copy(i):
            cols = pl.ds(i * TA, TA)
            return pltpu.make_async_copy(xT_hbm.at[:, cols], xT_s.at[:, cols], sem.at[SEM_X + i])

        cp_vec = [pltpu.make_async_copy(src, dst, sem.at[SEM_VEC])
                  for src, dst in zip((lre_hbm, lim_hbm, ldt_hbm, dsk_hbm, gw_hbm), vec_s)]
        cp_b = [pltpu.make_async_copy(src.at[pl.ds(lo, n)], b_s.at[pl.ds(dst, n)], sem.at[SEM_B])
                for src, lo, n, dst in ((bre_hbm, 0, PA, 0), (bim_hbm, 0, PA, PA),
                                        (bre_hbm, PA, PB, 2 * PA), (bim_hbm, PA, PB, 2 * PA + PB))]
        cp_wq = [pltpu.make_async_copy(wq_hbm.at[:, 0:8], rq.at[:, 0:8], sem.at[SEM_WQ])]
        cp_c = [pltpu.make_async_copy(src, craw_s.at[n], sem.at[SEM_C])
                for n, src in enumerate((cre_hbm, cim_hbm))]
        cp_wo = pltpu.make_async_copy(woT_hbm, wo_s, sem.at[SEM_WO])
        for cp in cp_vec + cp_b + [x_copy(i) for i in range(S // TA)] + cp_c + cp_wq:
            cp.start()
        for i in range(NRAW - 1):
            for cp in [wq1_copy(i)] + slice_copies(i):
                cp.start()
        wq1_copy(3).start()
        cp_wo.start()

        zero_s[...] = jnp.zeros(zero_s.shape, f32)
        wl_s[...] = jnp.zeros(wl_s.shape, u32)
        cl_s[:, (NP - 1) * 7 * T:] = jnp.zeros((HD // 2, 7 * T), u32)
        for cp in cp_vec:
            cp.wait()
        _ssm_params(vec_s, coef_s, lam_s, col_s)

        def wq_transpose(pair, tie):
            ht = pair // 4 if isinstance(pair, int) else lax.shift_right_logical(pair, 2)
            pad = jnp.zeros((T - QM, T), u32)
            for dt in range(2):
                for mq in range(4):
                    blk = sq[ht * 2 + dt, pl.ds(mq * QM * 4 + (pair & 3), QM, stride=4), :]
                    blk = jnp.concatenate([tie(blk[:8], 4 * dt + mq), blk[8:], pad], axis=0)
                    wqt_s[dt * HD:(dt + 1) * HD, mq * T:(mq + 1) * T] = blk.T

        def phase1(i):
            clk = _Clock(zero_s)
            u = _cat([clk.dot(xT_s[:, i * TA + lo:i * TA + hi], b_s[...], _TT)[0]
                      for lo, hi in ((0, T), (T, TA))], 0)
            for cb in range(4):
                w = min(2 * T, 2 * M - cb * 2 * T)
                u_s[cb, i * TA // 8:(i + 1) * TA // 8, :, 0:w] = (
                    u[:, cb * 2 * T:cb * 2 * T + w].reshape(TA // 8, 8, w))
            tie = clk.pacer(0, 6 * TA, 49)
            for r in range(0, QM, 16):
                def block(o, q):
                    row, col = (o % 2) * HM + (q % 2) * QM + r, (4 * i + 2 * (q // 2) + o // 2) * T
                    return xT_s[row:row + 16, col:col + T].astype(f32)
                for n1 in range(7):
                    ops = _operands2(_A_TERMS, n1, block, lambda x: tie(x, 7 * (r // 16) + n1))
                    _put(xa_s, i * QM + r, 7 * n1 * T, ops)
            tie = clk.pacer(0, 6 * TA, 8 * 14)
            for t in range(TA // T):
                cols = slice(i * TA + t * T, i * TA + (t + 1) * T)
                acc = jnp.zeros((8, T), f32)
                for r in range(0, M, 32):
                    xg = xT_s[r:r + 32, cols].astype(f32) * tie(col_s[1, r:r + 32, :], 28 * t + r // 32)
                    acc = acc + jnp.sum(xg.reshape(4, 8, T), axis=0)
                g = jax.nn.sigmoid(jnp.sum(acc, axis=0, keepdims=True))
                g_s[:, cols] = g
                for r in range(0, M, 32):
                    skip = xT_s[r:r + 32, cols].astype(f32) * tie(col_s[0, r:r + 32, :], 28 * t + 14 + r // 32)
                    o_s[r:r + 32, cols] = (1.0 - g) * skip
            return clk

        for cp in cp_b + [x_copy(0)]:
            cp.wait()
        phase1(0)
        x_copy(1).wait()
        clk = phase1(1)
        zero = jnp.zeros((1, 512), f32)
        carry0 = _ssm_scan(u_s.at[:, 0:TC // 8], (zero, zero), lam_s, h_s, clk.pacer(0, 6 * TA, TC // 2))
        for cp in [x_copy(2), x_copy(3)] + cp_c + cp_wq:
            cp.wait()
        _ssm_cmat(craw_s, coef_s, c_s, phase1(2).pacer(0, 6 * TA, M // 16))
        tie = phase1(3).pacer(0, 6 * TA, M // 8)
        for c0 in range(0, M, 8):
            _stage(rq, sq, c0, 8, lambda x: tie(x, c0 // 10), groups=(0,))
        wq_transpose(0, lambda x, k: tie(x, 46 + k))

        def phase2(i, carry):
            @pl.when(i + NRAW - 1 < NP)
            def _():
                for cp in slice_copies(i + NRAW - 1):
                    cp.start()

            @pl.when(i < 4)
            def _():
                wq1_copy(i).wait()

            for cp in slice_copies(i):
                cp.wait()

            clk = _Clock(zero_s)
            yT = _cat([clk.dot(_get(c_s, r, M // YS, 0, 2 * M), _get(h_s, 0, TC, 0, 2 * M), _NT)[0]
                       for r in range(0, M, M // YS)], 0)
            ty = clk.t
            cols = _ds(i * TC, TC, TC)
            keep = 1.0 - g_s[:, cols]
            for r in range(0, M, 32):
                o_s[r:r + 32, cols] += keep * yT[r:r + 32]

            q_i = q_s.at[_ds(i * 2 * D, 2 * D, 2 * D)]
            mq_s = (head_refs['mk_s'], head_refs['mp_s'], head_refs['mv_s'].at[0], head_refs['mv_s'].at[1])
            for g in range(4):
                for n1 in range(7):
                    if g == 0:
                        t = QL0 + (ty + 6 * 224 - QL1 - QL0) * n1 / 7
                        tie = clk.pacer(min(t, clk.t - QL1), min(t + 300, clk.t - QL1), 8)
                        for r in range(0, 2 * QD, 16):
                            def block(o, q):
                                row = (o % 2) * HD + (q % 2) * QD + r % QD
                                col = (2 * (o // 2) + q // 2) * T
                                w = wqt_s[row:row + 16, col:col + T]
                                return _hi16(w) if r >= QD else pltpu.bitcast(w << 16, f32)
                            _put(wq_s, r, 7 * n1 * T, _operands2(_B_TERMS, n1, block, lambda x: tie(x, r // 16)),
                                 (lambda w: tie(w, r // 16, True, FLAG)) if QLATE else None)
                    for r0 in range(0, 2 * QD, QR):
                        comb = clk.strassen(lambda n: _get(wq_s, r0, QR, (7 * n1 + n) * T, QM),
                                            lambda n: _get(xa_s, g * QM, QM, (7 * n1 + n) * T, T), _NN)
                        for r in range(0, QR, 32):
                            e, c = (r0 + r) // QD, comb(r, 32)
                            for dq in range(2):
                                row = dq * QD + r % QD
                                done = _outer_step(mq_s[2 * (g % 2) + e], n1, row,
                                                   jnp.concatenate([c[dq], c[2 + dq]], axis=1))
                                if done:
                                    n, v = done
                                    _put(q_i, (2 * e + n // 2) * D + (n % 2) * HD + row, 2 * g * T,
                                         [v * (LOG2E * D ** -0.5)])

            span = ty + SPAN

            u_next = u_s.at[:, pl.ds(jnp.minimum(i + 1, NP - 1) * (TC // 8), TC // 8)]
            carry = _ssm_scan(u_next, carry, lam_s, h_s, clk.pacer(ty + SC0, span, TC // 2))

            tie = clk.pacer(ty - SP0, span, 64, [(ty + QH0, ty + QH1)])
            rq_i = rq.at[pl.ds((i & 3) * (M // 4), M // 4)]
            sq_i = sq.at[:, _ds((i & 3) * M, M, 8)]
            for c0 in range(0, M // 4, 8):
                _stage(rq_i, sq_i, c0, 8, lambda x: tie(x, c0 // 4 + 2), groups=(1,))
            wq_transpose(jnp.minimum(i + 1, NP - 1), lambda x, k: tie(x, 36 + 3 * k))
            slot = pl.ds((i & (NRAW - 1)) * CS, CS)
            for n, (raw, stg, wt_s) in enumerate(((rk, sk, wkt_s), (rv, sv, wvt_s))):
                for c0 in range(0, CS, 8):
                    _stage(raw.at[slot], stg, c0, 8, lambda x: tie(x, 16 * n + c0 // 8))
                cols = _ds(i * CS, CS, CS)
                for pair in range(H // 2):
                    for dt in range(2):
                        blk = stg[(pair // 4) * 2 + dt, pl.ds(pair % 4, CS, stride=4), :]
                        row = pair * D + dt * HD
                        blk = jnp.concatenate([tie(blk[:8], 16 + 24 * n + 3 * pair + dt), blk[8:]], axis=0)
                        wt_s[row:row + HD, cols] = blk.T

            tie = clk.pacer(ty + AP0, span, 28)
            ckv_i = ckv_s.at[i & (NRAW - 1)]
            a_i = a_s.at[_ds(i * (T // 4), T // 4, T // 4)]
            for r in range(0, T // 2, 16):
                def block(o, q):
                    col = (o % 2) * 2 * QC + (q % 2) * QC
                    return ckv_i[2 * (q // 2) + o // 2, r:r + 16, col:col + QC].astype(f32)
                for n1 in range(7):
                    ops = _operands2(_A_TERMS, n1, block, lambda x: tie(x, 7 * (r // 16) + n1))
                    _put(a_i, r, 7 * n1 * QC, ops)
            return carry

        lax.fori_loop(0, NP, phase2, carry0)
        cp_wo.wait()
        prep_w(h, range(NT1), _no_tie)

    @pl.when(h == 0)
    def _():
        prologue(**pro_refs)

    def oproj(jp, clk):
        cols = slice(2 * jp * T, (2 * jp + 2) * T)
        for r, n in OCH:
            c = clk.strassen(lambda i: _get(wl_s, r, n, i * T, T),
                             lambda i: _get(cl_s, 0, HD, (jp * 7 + i) * T, T), _NN)()
            o_s[r:r + n, cols] += jnp.concatenate(c[:2], axis=1)
            o_s[HM + r:HM + r + n, cols] += jnp.concatenate(c[2:], axis=1)

    def head(mk_s, mv_s, mp_s, kt_s, ka_s, va_s, v2_s, s_s, pb_s, pd_s, p2_s, sc_s, qb_s):
        clk = _Clock(zero_s)
        q_h = q_s.at[_ds(h * D, D, D)]

        def prep_wo(tie):
            for r in range(0, HM, 16):
                top = tie(wo_s[h, r:r + 16, :].astype(f32), r // 16)
                bot = tie(wo_s[h, HM + r:HM + r + 16, :].astype(f32), r // 16)
                _put(wl_s, r, 0, _operands(_A_TERMS, [top[:, :HD], top[:, HD:], bot[:, :HD], bot[:, HD:]]))

        nine = lambda c: _operands(_A_TERMS, c) + [c[1], c[2]]

        def outer(m_s, r):
            return _combine([m_s[n * HD + r:n * HD + r + 16, :] for n in range(7)], order=range(7))

        def proj(g, lo, hi):
            for n1 in range(lo, hi):
                comb = clk.strassen(lambda n: _get(w_s, 0, 2 * QD, (7 * n1 + n) * QC, QC),
                                    lambda n: _get(a_s, g * T, T, (7 * n1 + n) * QC, QC), _NT, n1 == 6)
                for r in range(0, 2 * QD, GC):
                    m_s, row = mk_s if r < QD else mv_s.at[g % 2], n1 * HD + r % QD
                    c = comb(r, GC)
                    m_s[row:row + GC, :] = jnp.concatenate([c[0], c[2]], axis=1)
                    m_s[QD + row:QD + row + GC, :] = jnp.concatenate([c[1], c[3]], axis=1)
            if hi < 7:
                return
            cs = [outer(mk_s, r) for r in range(0, HD, 16)]
            for n in range(4):
                kt_s[:, n * T:(n + 1) * T] = jnp.concatenate([c[n] for c in cs], axis=0).T
            for r in range(0, 2 * T, GC):
                blk = kt_s[r:r + GC, :]
                _put(ka_s, 2 * g * T + r, 0, nine([blk[:, n * T:(n + 1) * T] for n in range(4)]))

        def vfin(g, tie):
            m_s = mv_s.at[g % 2]
            for r in range(0, QD, 16):
                k, blk = 8 * (r // 16), {}
                late = lambda w: tie(w, k, True, FLAG)
                for new, n1 in (((0,), 2), ((1,), 4), ((3,), 6), ((), 0), ((), 3), ((2,), 5), ((), 1)):
                    for o in new:
                        for i, row in enumerate((r, QD + r)):
                            tiles = _Tiles([m_s.at[n * HD:(n + 1) * HD] for n in range(7)], row, 16)
                            c, = _combine(tiles, ((o % 2) * 2 + o // 2,), range(7))
                            blk[o, i] = c = tie(c, k)
                            slot = (2, 7, 8, 3)[o]
                            _put(va_s, row, ((2 * g + 1) * 9 + slot) * T, [c[:, T:]])
                            if o in (1, 2):
                                _put(va_s, row, (2 * g * 9 + slot) * T, [c[:, :T]])
                    lo_, hi_ = [_operand(_A_TERMS[n1], lambda o: blk[o, i]) for i in range(2)]
                    _put(va_s, r, (2 * g * 9 + n1) * T, [lo_[:, :T]], late)
                    _put(va_s, QD + r, (2 * g * 9 + n1) * T, [hi_[:, :T]], late)
                    if g < 3:
                        _put(v2_s, r, (g * 7 + n1) * 7 * T,
                             _operands(_A_TERMS, [lo_[:, :T], lo_[:, T:], hi_[:, :T], hi_[:, T:]]), late)
                    k += 8 / 7

        key = lax.broadcasted_iota(jnp.int32, (T, 2 * T), 0)
        qry = lax.broadcasted_iota(jnp.int32, (T, 2 * T), 1)
        causal = key <= qry

        def qk(g):
            pairs = (2 * g, 2 * g + 1)
            mx = {jp: _Reducer(jnp.max, jnp.maximum) for jp in pairs}

            def put(jp, row, v):
                v = v.reshape(v.shape[0] // 8, 8, 2 * T)
                s_s[jp % 4, row // 8:row // 8 + v.shape[0]] = v
                mx[jp].add(v)

            def rect(jp, lo, hi, n):
                for r in range(lo, hi, n):
                    c = clk.strassen(lambda i: _get(ka_s, r, n, i * T, T),
                                     lambda i: _get(qb_s, 0, HD, ((jp % 2) * 7 + i) * T, T), _NN)()
                    put(jp, r, jnp.concatenate(c[:2], axis=1))
                    put(jp, jp * T + r, jnp.concatenate(c[2:], axis=1))

            q = lambda jp, e: _get(q_h, e * D, D, jp * T, T)
            for jp in pairs[g == 0:]:
                for r in range(0, HD, 32):
                    blk = [_get(q_h, e * D + d * HD + r, 32, jp * T, T).astype(f32) for d in range(2) for e in range(2)]
                    _put(qb_s, r, (jp % 2) * 7 * T, _operands(_B_TERMS, blk))
            for jp in pairs:
                rect(jp, 0, 2 * g * T, QCH if QCH else g * T // 2 or 1)
            kb = lambda jp, a, b: jnp.concatenate(
                [_get(ka_s, jp * T, T, a * T, T), _get(ka_s, jp * T, T, b * T, T)], axis=1)
            for jp in pairs:
                se, _ = clk.dot(kb(jp, 2, 7), jnp.concatenate([q(jp, 0), q(jp, 1)], axis=1), _NN)
                put(jp, 2 * jp * T, jnp.where(causal, se, NEG))
            last = {}
            for jp in pairs:
                so = jnp.where(causal[:, :T], clk.dot(kb(jp, 8, 3), q(jp, 1), _NN)[0], NEG)
                row = (2 * jp + 1) * T // 8
                s_s[jp % 4, row:row + T // 8, :, T:] = so.reshape(T // 8, 8, T)
                last[jp] = jnp.concatenate([jnp.full((1, T), NEG, f32), jnp.max(so, axis=0, keepdims=True)], axis=1)
            rect(2 * g + 1, 2 * g * T, (2 * g + 1) * T, T // 4)
            return [jnp.broadcast_to(jnp.maximum(mx[jp].result(), last[jp]), (8, 2 * T)) for jp in pairs]

        zs, sums = {}, {}

        def prob(jp, row, z, n=GS, lanes=slice(None)):
            return jnp.exp2(s_s[jp % 4, row // 8:(row + n) // 8, :, lanes] - z[:, lanes])

        def rough(jp, mx, tie):
            zs[jp] = mx
            if jp > 0:
                sm = _Reducer(jnp.sum, jnp.add)
                for k, r in enumerate(range(0, 2 * jp * T, GS * LSUB)):
                    sm.add(prob(jp, r, tie(mx, k)))
                zs[jp] = mx + jnp.log2(jnp.maximum(LSUB * sm.result(), 1.0))
            sums[jp] = _Reducer(jnp.sum, jnp.add)

        def blocks(jp, row, tie, k):
            top, bot = prob(jp, row, tie(zs[jp], k)), prob(jp, jp * T + row, tie(zs[jp], k + 1))
            sums[jp].add(top + bot)
            top, bot = top.reshape(GS, 2 * T), bot.reshape(GS, 2 * T)
            return [top[:, :T], top[:, T:], bot[:, :T], bot[:, T:]]

        def near(jp, tie, k):
            R, z = jp * T, zs[jp]
            if jp % 2:
                for r in range(0, T, GS):
                    _put(pb_s, jp // 2 * T + r, 0, _operands(_B_TERMS, blocks(jp, R - T + r, tie, k)))
                    k += 2
            for r in range(0, T, GS):
                p = prob(jp, 2 * R + r, tie(z, k))
                sums[jp].add(p)
                _put(pd_s, 2 * R + r, 0, [p.reshape(GS, 2 * T)])
                k += 1
            so = _Reducer(jnp.sum, jnp.add)
            for r in range(0, T, 2 * GS):
                p = prob(jp, 2 * R + T + r, tie(z, k), 2 * GS, slice(T, 2 * T))
                so.add(p)
                _put(pd_s, 2 * R + T + r, T, [p.reshape(2 * GS, T)])
                k += 1
            sums[jp].result()
            sums[jp].out = sums[jp].out + jnp.concatenate([jnp.zeros((1, T), f32), so.result()], axis=1)

        p20 = lambda g: g * (g - 1) // 2 * T

        def far(g, tie, k):
            half = {(jp, e): _Reducer(jnp.sum, jnp.add) for jp in (2 * g, 2 * g + 1) for e in range(2)}
            for kg in range(g):
                for r in range(0, T, GS):
                    blk = {}
                    for new, n1 in (((0,), 1), ((1,), 5), ((3,), 2), ((), 0), ((), 4), ((2,), 3), ((), 6)):
                        for o in new:
                            lanes = slice((o % 2) * T, (o % 2 + 1) * T)
                            for jp in (2 * g, 2 * g + 1):
                                z = tie(zs[jp][:, lanes], k)
                                row = (o // 2) * jp * T + 2 * kg * T + r
                                p = [jnp.exp2(s_s[jp % 4, x // 8:(x + GS) // 8, :, lanes] - z) for x in (row, row + T)]
                                half[jp, o % 2].add(p[0] + p[1])
                                blk[o, jp % 2], blk[o, 2 + jp % 2] = [x.reshape(GS, T) for x in p]
                        ops = _operands2(_B_TERMS, n1, lambda o, q: blk[o, q], lambda x: x)
                        _put(p2_s, p20(g) + kg * T + r, 7 * n1 * T, ops,
                             (lambda w: tie(w, k, True, FLAG)) if FTIE else None)
                        k += FW * 8 / 7
            for jp in (2 * g, 2 * g + 1):
                if g:
                    sums[jp].out = sums[jp].out + jnp.concatenate([half[jp, e].result() for e in range(2)], axis=1)
            for jp in (2 * g, 2 * g + 1):
                cols = slice(2 * jp * T, 2 * (jp + 1) * T)
                sc_s[:, cols] = g_s[:, cols] / sums[jp].result()

        def pv(g):
            pairs = (2 * g, 2 * g + 1)
            va = lambda n, t, r=0, nr=HD: _get(va_s, r, nr, (t * 9 + n) * T, T)
            for n1 in range(7 if g else 0):
                c = clk.strassen(
                    lambda n: _cat([_get(v2_s, 0, QD, (kg * 49 + 7 * n1 + n) * T, T) for kg in range(g)], 1),
                    lambda n: _get(p2_s, p20(g), g * T, (7 * n1 + n) * T, T), _NN)()
                mp_s[n1 * HD:n1 * HD + QD, :] = jnp.concatenate(c[:2], axis=1)
                mp_s[n1 * HD + QD:(n1 + 1) * HD, :] = jnp.concatenate(c[2:], axis=1)
            ve = [jnp.concatenate([va(2, jp), va(8, jp)], axis=0) for jp in pairs]
            vo = [jnp.concatenate([va(7, jp), va(3, jp)], axis=0) for jp in pairs]
            ce = clk.level([(ve[jp % 2], _get(pd_s, 2 * jp * T, T, 0, T)) for jp in pairs])
            co = [clk.dot(jnp.concatenate([ve[jp % 2], vo[jp % 2]], axis=1),
                          _get(pd_s, 2 * jp * T, 2 * T, T, T), _NN)[0] for jp in pairs]
            for jp in pairs:
                R, e = jp * T, jp % 2
                ge, go = sc_s[:, 2 * R:2 * R + T], sc_s[:, 2 * R + T:2 * R + 2 * T]
                for r in range(0, HD, 32):
                    c = [ce[e][r:r + 32], co[e][r:r + 32], ce[e][HD + r:HD + r + 32], co[e][HD + r:HD + r + 32]]
                    if g:
                        far_ = _combine([mp_s[n * HD + r:n * HD + r + 32, e * T:(e + 1) * T] for n in range(7)],
                                        order=range(7))
                        c = [x + y for x, y in zip(c, far_)]
                    if e:
                        near_ = clk.strassen(lambda n: va(n, 2 * g, r, 32),
                                             lambda n: _get(pb_s, g * T, T, n * T, T), _NN)()
                        c = [x + y for x, y in zip(c, near_)]
                    ops = _operands(_B_TERMS, [c[0] * ge, c[1] * go, c[2] * ge, c[3] * go])
                    _put(cl_s, r, jp * 7 * T, ops)

        ends = []

        def run(items):
            for item in items.split():
                if item[0] == 'P':
                    pv(int(item[1]))
                    ends.append(clk.t)
                elif item[0] == 'K':
                    proj(int(item[1]), int(item[2]), int(item[3]))
                else:
                    jp = int(item[1])
                    oproj(jp, clk)

                    @pl.when(h == H - 1)
                    def _():
                        out_copy(jp).start()

        for n1 in range(7):
            if n1 >= NT1:
                prep_w(h, [n1], clk.pacer(max(clk.t - LEAD - 448, 1), max(clk.t - LEAD, 1), 8))
            proj(0, n1, n1 + 1)
        oproj(NP - 1, clk)
        mx = qk(0)
        for g in range(4):
            t0 = clk.t
            del ends[:]
            run(PLAN[g])
            t1 = clk.t
            nxt = qk(g + 1) if g < 3 else None
            n_rough = [2 * jp * T // (GS * LSUB) for jp in (2 * g, 2 * g + 1)]
            n_near = [(T + T // 2) // GS, (3 * T + T // 2) // GS]
            holes = [(t - PH0, t + PH1) for t in ends]
            if g < 3:
                vfin(g, clk.pacer(t0 - VB, t0 + VW, 32))
                holes += [(t0, t0 + VW), (t1 - HOLE0, t1 + HOLE1)]
            if g == 2:
                vfin(3, clk.pacer(clk.t - SLACK - VW // 2, clk.t - SLACK, 32))
                holes.append((clk.t - SLACK - VW // 2, clk.t))
            tie = clk.pacer(t0 + D0, (clk.t if g else t1) - SLACK,
                            sum(n_rough) + sum(n_near) + FW * g * 8 * T // GS, holes)
            rough(2 * g, mx[0], tie)
            near(2 * g, tie, n_rough[0])
            k = n_rough[0] + n_near[0]
            rough(2 * g + 1, mx[1], lambda x, i: tie(x, k + i))
            near(2 * g + 1, tie, k + n_rough[1])
            far(g, tie, k + n_rough[1] + n_near[1])
            if g == 0:
                prep_wo(clk.pacer(t0 + VW, t1 - HOLE0, HM // 16))
            mx = nxt
        t0 = clk.t
        run(PLAN[4])
        prep_w(jnp.minimum(h + 1, H - 1), range(NT1), clk.pacer(t0 - PW0, clk.t - 300, 8 * NT1))
        if os.environ.get('SHOW'):
            print('final loads', clk.load)

    head(**head_refs)

    @pl.when(h == H - 1)
    def _():
        oproj(NP - 1, _Clock(zero_s))
        out_copy(NP - 1).start()
        for jp in range(NP):
            out_copy(jp).wait()


@jax.jit
def pallas_gated_mix__compressed_kv_cla__ssm_conv_s5__prompt_kernel(
    A_x: jax.Array,
    A_c_kv: jax.Array,
    A_w_q: jax.Array,
    A_w_uk: jax.Array,
    A_w_uv: jax.Array,
    A_w_o: jax.Array,
    B_x: jax.Array,
    B_Lambda_re: jax.Array,
    B_Lambda_im: jax.Array,
    B_B_re: jax.Array,
    B_B_im: jax.Array,
    B_C_re: jax.Array,
    B_C_im: jax.Array,
    B_log_dt: jax.Array,
    B_Dskip: jax.Array,
    gate_w: jax.Array,
):
    del B_x
    xT = jnp.transpose(A_x[0])
    woT = jnp.transpose(A_w_o, (0, 2, 1))
    ckv = A_c_kv.reshape(4, 4, 2, T // 2, DC)

    hbm = pl.BlockSpec(memory_space=pl.ANY)
    outT = pl.pallas_call(
        _kernel,
        grid=(H,),
        in_specs=[hbm] * 15,
        out_specs=hbm,
        out_shape=jax.ShapeDtypeStruct((M, S), f32),
        scratch_shapes=_SHARED_SCRATCH + list(_PROLOGUE_SCRATCH.values()) + list(_HEAD_SCRATCH.values()),
        compiler_params=pltpu.CompilerParams(
            dimension_semantics=("arbitrary",),
            vmem_limit_bytes=127 * 1024 * 1024,
        ),
    )(xT, B_B_re, B_B_im, B_C_re, B_C_im, B_Lambda_re, B_Lambda_im, B_log_dt,
      B_Dskip, gate_w, woT, ckv, A_w_q, A_w_uk, A_w_uv)
    return jnp.transpose(outT)[None]
```

```python
import bisect
import os

import jax
import jax.numpy as jnp
from jax import lax
import jax.experimental.pallas as pl
import jax.experimental.pallas.tpu as pltpu

S = 2048
M = 448
H = 16
D = 256
DC = 1024
T = 128
NP = S // T // 2
HD = D // 2
HM = M // 2
QD = D // 4
QC = DC // 4
QM = M // 4
PA = 384
PB = M - PA
TA = 512
TC = 256
CS = DC // NP
NRAW = 4
LOG2E = 1.4426950408889634
NEG = -1e30

_env = lambda k, d: type(d)(os.environ.get(k, d))
GC = _env('GC', 64)
GS = _env('GS', 16)
RCH = _env('RCH', 256)
SLACK = _env('SLACK', 200)
D0 = _env('D0', 0)
NT1 = _env('NT1', 3)
LEAD = _env('LEAD', 448)
PW0 = _env('PW0', 100)
FTIE = _env('FTIE', 1)
YS = _env('YS', 2)
QR = _env('QR', 128)
QL0 = _env('QL0', 200)
QL1 = _env('QL1', 500)
SPAN = _env('SPAN', 6000)
QLATE = _env('QLATE', 0)
SC0 = _env('SC0', 0)
QH0 = _env('QH0', 0)
QH1 = _env('QH1', 1000)
AP0 = _env('AP0', 1000)
SP0 = _env('SP0', 1200)
FLAG = _env('FLAG', 40)
FW = _env('FW', 2)
HOLE0 = _env('HOLE0', 300)
HOLE1 = _env('HOLE1', 300)
VW = _env('VW', 900)
VB = _env('VB', 0)
SW0 = _env('SW0', 400)
SW1 = _env('SW1', -100)
SE0 = _env('SE0', 0)
SE1 = _env('SE1', 0)
NEAR64 = _env('NEAR64', 0)
SES = _env('SES', 1)
PH0 = _env('PH0', 400)
PH1 = _env('PH1', 0)
QCH = _env('QCH', 64)
OCH = ((0, 64), (64, 64), (128, 48), (176, 48))
LSUB = _env('LSUB', 4)
PLAN = _env('PLAN', 'K107,K207,K307,P1 P0 O2 O3 P2 O0 O1 O4,O5 P3 O6').split(',')

f32 = jnp.float32
bf16 = jnp.bfloat16
u32 = jnp.uint32

SEM_VEC, SEM_B, SEM_X, SEM_WQ, SEM_C, SEM_SL, SEM_WO, SEM_OUT, SEM_WQ1 = 0, 1, 2, 6, 7, 8, 16, 17, 18
NSEM = 22

_NN = ((1,), (0,))
_NT = ((1,), (1,))
_TN = ((0,), (0,))
_TT = ((0,), (1,))


def _dot(a, b, dims):
    return lax.dot_general(a, b, (dims, ((), ())), preferred_element_type=f32)


def _cat(xs, axis):
    return xs[0] if len(xs) == 1 else jnp.concatenate(xs, axis=axis)


def _ds(lo, n, align):
    return pl.ds(lo if isinstance(lo, int) else pl.multiple_of(lo, align), n)


def _put(ref, row, col, xs, tie=None):
    x = _cat(xs, 1)
    if tie is not None:
        x = jnp.concatenate([tie(x[:8]), x[8:]], axis=0)
    ref[row // 2:(row + x.shape[0]) // 2, col:col + x.shape[1]] = pltpu.bitcast(x.astype(bf16), u32)


def _get(ref, row, nrows, col, ncols):
    return pltpu.bitcast(ref[row // 2:(row + nrows) // 2, col:col + ncols], bf16)


class _Clock:
    def __init__(self, zero_ref):
        self.masks = {(8, T): zero_ref[...] != 0.0}
        self.ticks, self.load = [], [0, 0, 0, 0]

    @property
    def t(self):
        return max(self.load)

    def dot(self, a, b, dims):
        v = _dot(a, b, dims)
        rows, depth = v.shape[0], a.shape[dims[0][0]]
        for c in range(0, v.shape[1], T):
            start = 0
            for _ in range(0, depth, T):
                k = self.load.index(min(self.load))
                start = max(start, self.load[k])
                self.load[k] += rows
            self.ticks += [(start + r + 8, (v, r, c)) for r in range(0, rows, 8)]
        return v, start

    def strassen(self, lhs, rhs, dims, split_last=False):
        jobs = -(-lhs(0).shape[dims[0][0]] // T)
        lag = sum(l + 32 <= max(self.load) for l in self.load) // jobs if jobs < 3 else 0
        order = ((1, 3, 2, 4, 0, 5, 6), (0, 1, 3, 2, 4, 5, 6), (5, 6, 1, 3, 2, 4, 0), (0, 5, 6, 1, 3, 2, 4))[lag]
        m = {}
        for n in order:
            if split_last and n == order[-1]:
                a, half = lhs(n), lhs(0).shape[0] // 2
                m[n] = jnp.concatenate([self.dot(a[:half], rhs(n), dims)[0], self.dot(a[half:], rhs(n), dims)[0]], 0)
            else:
                m[n] = self.dot(lhs(n), rhs(n), dims)[0]
        vals = [m[n] for n in range(7)]
        return lambda r=0, n=None, only=(0, 1, 2, 3), c=0, w=None: _combine(
            vals if n is None else _Tiles(vals, r, n, c, w), only, order)

    def level(self, pairs):
        base, extra = divmod((sum(self.load) + sum(a.shape[0] for a, _ in pairs)) // 16, 4)
        target = [16 * (base + (k < extra)) for k in range(4)]
        out = []
        for a, b in pairs:
            r, parts = 0, []
            while r < a.shape[0]:
                k = self.load.index(min(self.load))
                n = min(max(target[k] - self.load[k], 16), a.shape[0] - r)
                parts.append(self.dot(a[r:r + n], b, _NN)[0])
                r += n
            out.append(_cat(parts, 0))
        return out

    def pacer(self, t0, t1, n, holes=()):
        holes = sorted((max(a, t0), min(b, t1)) for a, b in holes if a < t1 and b > t0)
        gap = sum(b - a for a, b in holes)
        ticks = sorted(self.ticks, key=lambda tw: tw[0])
        times = [tw[0] for tw in ticks]

        def tie(x, k, distinct=False, delay=0):
            t = t0 + (t1 - t0 - gap) * k / n
            for a, b in holes:
                t += b - a if t > a else 0
            t += delay
            past = ticks[:bisect.bisect_right(times, t)]
            reps = (x.shape[0] // 8, x.shape[1] // T)
            if len(past) < (reps[1] if distinct else 1):
                return x
            tick = _cat([v[r:r + 8, c:c + T] for _, (v, r, c) in past[-reps[1] if distinct else -1:]], 1)
            if tick.dtype != x.dtype:
                tick = pltpu.bitcast(tick, x.dtype)
            if x.shape not in self.masks:
                self.masks[x.shape] = jnp.tile(self.masks[(8, T)], reps)
            return lax.select(self.masks[x.shape], tick if tick.shape == x.shape else jnp.tile(tick, reps), x)
        return tie


def _no_tie(x, k):
    return x


_A_TERMS = ((0, 3, 1), (2, 3, 1), (0, None, 0), (3, None, 0), (0, 1, 1), (2, 0, -1), (1, 3, -1))
_B_TERMS = ((0, 3, 1), (0, None, 0), (1, 3, -1), (2, 0, -1), (3, None, 0), (0, 1, 1), (2, 3, 1))


def _operand(term, block):
    x, y, sign = term
    if y is None:
        return block(x)
    return block(x) + block(y) if sign > 0 else block(x) - block(y)


def _operands(terms, blocks):
    return [_operand(t, blocks.__getitem__) for t in terms]


def _operands2(terms, n1, block, tie):
    first = terms[n1][0]
    sub = [_operand(terms[n1], lambda o: tie(block(o, q)) if o == first and q in (0, 3) else block(o, q))
           for q in range(4)]
    return _operands(terms, sub)


_C_TERMS = ({0: 1, 3: 1, 4: -1, 6: 1}, {2: 1, 4: 1}, {1: 1, 3: 1}, {0: 1, 1: -1, 2: 1, 5: 1})


def _combine(m, only=(0, 1, 2, 3), order=(1, 3, 2, 4, 0, 5, 6)):
    out = []
    for terms in (_C_TERMS[n] for n in only):
        seq = [n for n in order if n in terms]
        if terms[seq[0]] < 0:
            seq[0], seq[1] = seq[1], seq[0]
        acc = m[seq[0]]
        for n in seq[1:]:
            acc = acc + m[n] if terms[n] > 0 else acc - m[n]
        out.append(acc)
    return out


def _outer_step(m_s, n1, row, v):
    n = v.shape[0]
    if n1 < 5:
        m_s[n1 * HD + row:n1 * HD + row + n, :] = v
    if n1 < 3:
        return None
    blk = (2, 1, 3, 0)[n1 - 3]
    m = {j: v if j == n1 else m_s[j * HD + row:j * HD + row + n, :] for j in _C_TERMS[blk]}
    return blk, _combine(m, (blk,), range(7))[0]


class _Tiles:
    def __init__(self, vals, r, n, c=0, w=None):
        self.vals, self.idx, self.cache = vals, (slice(r, r + n), slice(c, None if w is None else c + w)), {}

    def __getitem__(self, i):
        if i not in self.cache:
            self.cache[i] = self.vals[i][self.idx]
        return self.cache[i]


class _Reducer:
    def __init__(self, red, comb):
        self.red, self.comb, self.acc, self.rows, self.out = red, comb, None, 0, None

    def add(self, v):
        self.rows += 8 * v.shape[0]
        v = self.red(v, axis=0)
        self.acc = v if self.acc is None else self.comb(self.acc, v)
        if self.rows >= RCH:
            self.result()

    def result(self):
        if self.acc is not None:
            v = self.red(self.acc, axis=0, keepdims=True)
            self.out = v if self.out is None else self.comb(self.out, v)
        self.acc, self.rows = None, 0
        return self.out


def _cmul(ar, ai, br, bi):
    return ar * br - ai * bi, ar * bi + ai * br


def _hi16(w):
    return pltpu.bitcast(w & jnp.uint32(0xFFFF0000), f32)


def _stage(raw, stg, c0, nc, tie, groups=(0, 1)):
    for ht in groups:
        for dt in range(2):
            v = raw[c0:c0 + nc, ht * 8:(ht + 1) * 8, dt * T:(dt + 1) * T].reshape(nc * 8, T)
            stg[ht * 2 + dt, c0 * 4:(c0 + nc) * 4, :] = tie(pltpu.bitcast(v, u32))


def _ssm_params(vec_s, coef_s, lam_s, col_s):
    row = lambda r: r[...].astype(f32).reshape(1, M)
    lre, lim, ldt, dsk, gw = [row(v) for v in vec_s]
    dt = jnp.exp(ldt).astype(bf16).astype(f32)
    mag = jnp.exp(dt * lre)
    ang = dt * lim
    lr, li = mag * jnp.cos(ang), mag * jnp.sin(ang)
    den = lre * lre + lim * lim
    nr = lr - 1.0
    coef_s[...] = jnp.zeros(coef_s.shape, f32)
    coef_s[0:1, 0:M] = 2.0 * ((nr * lre + li * lim) / den)
    coef_s[1:2, 0:M] = 2.0 * ((li * lre - nr * lim) / den)

    er = jnp.concatenate([lr, lr[:, PA:]], axis=1)
    ei = jnp.concatenate([li, -li[:, PA:]], axis=1)
    pw = [(er, ei)]
    for _ in range(7):
        pw.append(_cmul(pw[-1][0], pw[-1][1], er, ei))
    sub = lax.broadcasted_iota(jnp.int32, (8, 512), 0)
    for n, d in enumerate((1, 2, 4)):
        lam_s[2 * n] = jnp.where(sub >= d, pw[d - 1][0], 0.0)
        lam_s[2 * n + 1] = jnp.where(sub >= d, pw[d - 1][1], 0.0)
    lcr = jnp.zeros((8, 512), f32)
    lci = jnp.zeros((8, 512), f32)
    for r in range(8):
        lcr = jnp.where(sub == r, pw[r][0], lcr)
        lci = jnp.where(sub == r, pw[r][1], lci)
    lam_s[6] = lcr
    lam_s[7] = lci

    def col(v):
        v = jnp.concatenate([v, jnp.zeros((1, 512 - M), f32)], axis=1)
        return jnp.broadcast_to(v, (T, 512)).T[:M]
    col_s[0] = col(dsk)
    col_s[1] = col(gw)


def _ssm_cmat(craw_s, coef_s, c_s, tie):
    for r in range(0, M, 16):
        coef = tie(coef_s[...], r // 16)
        cr, ci = coef[0:1, :M], coef[1:2, :M]
        re, im = _cmul(craw_s[0, r:r + 16, :].astype(f32), craw_s[1, r:r + 16, :].astype(f32), cr, ci)
        _put(c_s, r, 0, [re[:, :PA], -im[:, :PA], re[:, PA:], -im[:, PA:]])


def _ssm_scan(u_ref, carry, lam_s, h_s, tie):
    car, cai = carry
    out = []
    for b in range(TC // 8):
        mixed = u_ref[3, b, :, 0:T]
        u = jnp.concatenate([u_ref[cb, b] for cb in range(3)], axis=1)
        cols = [u[:, 0:T], u[:, T:2 * T], u[:, 2 * T:PA], mixed]
        hr = jnp.concatenate([tie(v, 4 * b + n) for n, v in enumerate(cols)], axis=1)
        hi = jnp.concatenate([u[:, PA:2 * PA], pltpu.roll(mixed, PB, 1)], axis=1)
        for n, d in enumerate((1, 2, 4)):
            sr, si = pltpu.roll(hr, d, 0), pltpu.roll(hi, d, 0)
            tr, ti = _cmul(sr, si, lam_s[2 * n], lam_s[2 * n + 1])
            hr, hi = hr + tr, hi + ti
        tr, ti = _cmul(lam_s[6], lam_s[7], car, cai)
        hr, hi = hr + tr, hi + ti
        car, cai = hr[7:8, :], hi[7:8, :]
        out.append(jnp.concatenate([hr[:, :PA], hi[:, :PA], hr[:, PA:]], axis=1))
        if b % 2 == 1:
            _put(h_s, (b - 1) * 8, 0, [jnp.concatenate(out, axis=0)])
            out = []
    return car, cai


_vmem = pltpu.VMEM
_PROLOGUE_SCRATCH = dict(
    xT_s=_vmem((M, S), bf16),
    v0=_vmem((M,), bf16), v1=_vmem((M,), bf16), v2=_vmem((M,), bf16), v3=_vmem((M,), bf16), v4=_vmem((M,), bf16),
    b_s=_vmem((2 * M, M), bf16),
    craw_s=_vmem((2, M, M), bf16),
    c_s=_vmem((M // 2, 2 * M), u32),
    coef_s=_vmem((8, 512), f32),
    lam_s=_vmem((8, 8, 512), f32),
    col_s=_vmem((2, M, T), f32),
    h_s=_vmem((TC // 2, 2 * M), u32),
    ckv_s=_vmem((NRAW, 4, T // 2, DC), bf16),
    rq=_vmem((M, H, D), bf16),
    rk=_vmem((NRAW * CS, H, D), bf16),
    rv=_vmem((NRAW * CS, H, D), bf16),
    sq=_vmem((4, M * 4, T), u32),
    sk=_vmem((4, CS * 4, T), u32),
    sv=_vmem((4, CS * 4, T), u32),
    wqt_s=_vmem((D, 4 * T), u32),
)
_HEAD_SCRATCH = dict(
    mk_s=_vmem((7 * HD, 2 * T), f32),
    mv_s=_vmem((2, 7 * HD, 2 * T), f32),
    mp_s=_vmem((7 * HD, 2 * T), f32),
    kt_s=_vmem((2 * T, 4 * T), f32),
    ka_s=_vmem((S // 4, 9 * T), u32),
    va_s=_vmem((HD // 2, NP * 9 * T), u32),
    v2_s=_vmem((QD // 2, 3 * 49 * T), u32),
    s_s=_vmem((4, S // 8, 8, 2 * T), f32),
    pb_s=_vmem((2 * T, 7 * T), u32),
    pd_s=_vmem((S // 2, 2 * T), u32),
    p2_s=_vmem((3 * T, 49 * T), u32),
    sc_s=_vmem((1, S), f32),
    qb_s=_vmem((HD // 2, 14 * T), u32),
    kd_s=_vmem((T // 2, 7 * T), u32),
)
_SHARED_SCRATCH = [
    _vmem((H // 2 * D, DC), u32),
    _vmem((H // 2 * D, DC), u32),
    _vmem((S // 8, 49 * QC), u32),
    _vmem((H * D, S // 2), u32),
    _vmem((H, M, D), bf16),
    _vmem((QD, 49 * QC), u32),
    _vmem((HM // 2, 7 * T), u32),
    _vmem((HD // 2, NP * 7 * T), u32),
    _vmem((M, S), f32),
    _vmem((1, S), f32),
    _vmem((8, T), f32),
    pltpu.SemaphoreType.DMA((NSEM,)),
]


def _kernel(xT_hbm, bre_hbm, bim_hbm, cre_hbm, cim_hbm, lre_hbm, lim_hbm, ldt_hbm,
            dsk_hbm, gw_hbm, woT_hbm, ckv_hbm, wq_hbm, wk_hbm, wv_hbm,
            out_hbm,
            wkt_s, wvt_s, a_s, q_s, wo_s, w_s, wl_s, cl_s, o_s, g_s, zero_s, sem, *rest):
    h = pl.program_id(0)
    pro_refs = dict(zip(_PROLOGUE_SCRATCH, rest))
    head_refs = dict(zip(_HEAD_SCRATCH, rest[len(pro_refs):]))

    def out_copy(jp):
        cols = pl.ds(jp * 2 * T, 2 * T)
        return pltpu.make_async_copy(o_s.at[:, cols], out_hbm.at[:, cols], sem.at[SEM_OUT])

    def prep_w(hh, outer, tie):
        rows = _ds(lax.shift_right_logical(hh, 1) * D, D, D)
        sh = (16 * (1 - (hh & 1))).astype(u32)
        k = 0
        for row0, wt_s in ((0, wkt_s.at[rows]), (QD, wvt_s.at[rows])):
            for r in range(0, QD, 16):
                def block(o, q):
                    row = (o % 2) * HD + (q % 2) * QD + r
                    col = (o // 2) * 2 * QC + (q // 2) * QC
                    return _hi16(wt_s[row:row + 16, col:col + QC] << sh)
                for n1 in outer:
                    _put(w_s, row0 + r, 7 * n1 * QC, _operands2(_B_TERMS, n1, block, lambda x: tie(x, k)))
                    k += 1

    def prologue(xT_s, v0, v1, v2, v3, v4, b_s, craw_s, c_s, coef_s, lam_s, col_s, h_s,
                 ckv_s, rq, rk, rv, sq, sk, sv, wqt_s):
        xa_s = head_refs['p2_s']
        wq_s = xa_s.at[2 * QM:2 * QM + QD]
        u_s = head_refs['s_s']
        vec_s = (v0, v1, v2, v3, v4)

        def slice_copies(i):
            s = sem.at[SEM_SL + i]
            grp = i // 2 if isinstance(i, int) else lax.shift_right_logical(i, 1)
            cs, dst = pl.ds(i * CS, CS), pl.ds((i & (NRAW - 1)) * CS, CS)
            return [pltpu.make_async_copy(ckv_hbm.at[grp, :, i & 1], ckv_s.at[i & (NRAW - 1)], s),
                    pltpu.make_async_copy(wk_hbm.at[cs], rk.at[dst], s),
                    pltpu.make_async_copy(wv_hbm.at[cs], rv.at[dst], s)]

        def wq1_copy(i):
            rows = pl.ds(i * (M // 4), M // 4)
            return pltpu.make_async_copy(wq_hbm.at[rows, 8:16], rq.at[rows, 8:16], sem.at[SEM_WQ1 + i])

        def x_copy(i):
            cols = pl.ds(i * TA, TA)
            return pltpu.make_async_copy(xT_hbm.at[:, cols], xT_s.at[:, cols], sem.at[SEM_X + i])

        cp_vec = [pltpu.make_async_copy(src, dst, sem.at[SEM_VEC])
                  for src, dst in zip((lre_hbm, lim_hbm, ldt_hbm, dsk_hbm, gw_hbm), vec_s)]
        cp_b = [pltpu.make_async_copy(src.at[pl.ds(lo, n)], b_s.at[pl.ds(dst, n)], sem.at[SEM_B])
                for src, lo, n, dst in ((bre_hbm, 0, PA, 0), (bim_hbm, 0, PA, PA),
                                        (bre_hbm, PA, PB, 2 * PA), (bim_hbm, PA, PB, 2 * PA + PB))]
        cp_wq = [pltpu.make_async_copy(wq_hbm.at[:, 0:8], rq.at[:, 0:8], sem.at[SEM_WQ])]
        cp_c = [pltpu.make_async_copy(src, craw_s.at[n], sem.at[SEM_C])
                for n, src in enumerate((cre_hbm, cim_hbm))]
        cp_wo = pltpu.make_async_copy(woT_hbm, wo_s, sem.at[SEM_WO])
        for cp in cp_vec + cp_b + [x_copy(i) for i in range(S // TA)] + cp_c + cp_wq:
            cp.start()
        for i in range(NRAW - 1):
            for cp in [wq1_copy(i)] + slice_copies(i):
                cp.start()
        wq1_copy(3).start()
        cp_wo.start()

        zero_s[...] = jnp.zeros(zero_s.shape, f32)
        wl_s[...] = jnp.zeros(wl_s.shape, u32)
        cl_s[:, (NP - 1) * 7 * T:] = jnp.zeros((HD // 2, 7 * T), u32)
        for cp in cp_vec:
            cp.wait()
        _ssm_params(vec_s, coef_s, lam_s, col_s)

        def wq_transpose(pair, tie):
            ht = pair // 4 if isinstance(pair, int) else lax.shift_right_logical(pair, 2)
            pad = jnp.zeros((T - QM, T), u32)
            for dt in range(2):
                for mq in range(4):
                    blk = sq[ht * 2 + dt, pl.ds(mq * QM * 4 + (pair & 3), QM, stride=4), :]
                    blk = jnp.concatenate([tie(blk[:8], 4 * dt + mq), blk[8:], pad], axis=0)
                    wqt_s[dt * HD:(dt + 1) * HD, mq * T:(mq + 1) * T] = blk.T

        def phase1(i):
            clk = _Clock(zero_s)
            u = _cat([clk.dot(xT_s[:, i * TA + lo:i * TA + hi], b_s[...], _TT)[0]
                      for lo, hi in ((0, T), (T, TA))], 0)
            for cb in range(4):
                w = min(2 * T, 2 * M - cb * 2 * T)
                u_s[cb, i * TA // 8:(i + 1) * TA // 8, :, 0:w] = (
                    u[:, cb * 2 * T:cb * 2 * T + w].reshape(TA // 8, 8, w))
            tie = clk.pacer(0, 6 * TA, 49)
            for r in range(0, QM, 16):
                def block(o, q):
                    row, col = (o % 2) * HM + (q % 2) * QM + r, (4 * i + 2 * (q // 2) + o // 2) * T
                    return xT_s[row:row + 16, col:col + T].astype(f32)
                for n1 in range(7):
                    ops = _operands2(_A_TERMS, n1, block, lambda x: tie(x, 7 * (r // 16) + n1))
                    _put(xa_s, i * QM + r, 7 * n1 * T, ops)
            tie = clk.pacer(0, 6 * TA, 8 * 14)
            for t in range(TA // T):
                cols = slice(i * TA + t * T, i * TA + (t + 1) * T)
                acc = jnp.zeros((8, T), f32)
                for r in range(0, M, 32):
                    xg = xT_s[r:r + 32, cols].astype(f32) * tie(col_s[1, r:r + 32, :], 28 * t + r // 32)
                    acc = acc + jnp.sum(xg.reshape(4, 8, T), axis=0)
                g = jax.nn.sigmoid(jnp.sum(acc, axis=0, keepdims=True))
                g_s[:, cols] = g
                for r in range(0, M, 32):
                    skip = xT_s[r:r + 32, cols].astype(f32) * tie(col_s[0, r:r + 32, :], 28 * t + 14 + r // 32)
                    o_s[r:r + 32, cols] = (1.0 - g) * skip
            return clk

        for cp in cp_b + [x_copy(0)]:
            cp.wait()
        phase1(0)
        x_copy(1).wait()
        clk = phase1(1)
        zero = jnp.zeros((1, 512), f32)
        carry0 = _ssm_scan(u_s.at[:, 0:TC // 8], (zero, zero), lam_s, h_s, clk.pacer(0, 6 * TA, TC // 2))
        for cp in [x_copy(2), x_copy(3)] + cp_c + cp_wq:
            cp.wait()
        _ssm_cmat(craw_s, coef_s, c_s, phase1(2).pacer(0, 6 * TA, M // 16))
        tie = phase1(3).pacer(0, 6 * TA, M // 8)
        for c0 in range(0, M, 8):
            _stage(rq, sq, c0, 8, lambda x: tie(x, c0 // 10), groups=(0,))
        wq_transpose(0, lambda x, k: tie(x, 46 + k))

        def phase2(i, carry):
            @pl.when(i + NRAW - 1 < NP)
            def _():
                for cp in slice_copies(i + NRAW - 1):
                    cp.start()

            @pl.when(i < 4)
            def _():
                wq1_copy(i).wait()

            for cp in slice_copies(i):
                cp.wait()

            clk = _Clock(zero_s)
            yT = _cat([clk.dot(_get(c_s, r, M // YS, 0, 2 * M), _get(h_s, 0, TC, 0, 2 * M), _NT)[0]
                       for r in range(0, M, M // YS)], 0)
            ty = clk.t
            cols = _ds(i * TC, TC, TC)
            keep = 1.0 - g_s[:, cols]
            for r in range(0, M, 32):
                o_s[r:r + 32, cols] += keep * yT[r:r + 32]

            q_i = q_s.at[_ds(i * 2 * D, 2 * D, 2 * D)]
            mq_s = (head_refs['mk_s'], head_refs['mp_s'], head_refs['mv_s'].at[0], head_refs['mv_s'].at[1])
            for g in range(4):
                for n1 in range(7):
                    if g == 0:
                        t = QL0 + (ty + 6 * 224 - QL1 - QL0) * n1 / 7
                        tie = clk.pacer(min(t, clk.t - QL1), min(t + 300, clk.t - QL1), 8)
                        for r in range(0, 2 * QD, 16):
                            def block(o, q):
                                row = (o % 2) * HD + (q % 2) * QD + r % QD
                                col = (2 * (o // 2) + q // 2) * T
                                w = wqt_s[row:row + 16, col:col + T]
                                return _hi16(w) if r >= QD else pltpu.bitcast(w << 16, f32)
                            _put(wq_s, r, 7 * n1 * T, _operands2(_B_TERMS, n1, block, lambda x: tie(x, r // 16)),
                                 (lambda w: tie(w, r // 16, True, FLAG)) if QLATE else None)
                    for r0 in range(0, 2 * QD, QR):
                        comb = clk.strassen(lambda n: _get(wq_s, r0, QR, (7 * n1 + n) * T, QM),
                                            lambda n: _get(xa_s, g * QM, QM, (7 * n1 + n) * T, T), _NN)
                        for r in range(0, QR, 32):
                            e, c = (r0 + r) // QD, comb(r, 32)
                            for dq in range(2):
                                row = dq * QD + r % QD
                                done = _outer_step(mq_s[2 * (g % 2) + e], n1, row,
                                                   jnp.concatenate([c[dq], c[2 + dq]], axis=1))
                                if done:
                                    n, v = done
                                    _put(q_i, (2 * e + n // 2) * D + (n % 2) * HD + row, 2 * g * T,
                                         [v * (LOG2E * D ** -0.5)])

            span = ty + SPAN

            u_next = u_s.at[:, pl.ds(jnp.minimum(i + 1, NP - 1) * (TC // 8), TC // 8)]
            carry = _ssm_scan(u_next, carry, lam_s, h_s, clk.pacer(ty + SC0, span, TC // 2))

            tie = clk.pacer(ty - SP0, span, 64, [(ty + QH0, ty + QH1)])
            rq_i = rq.at[pl.ds((i & 3) * (M // 4), M // 4)]
            sq_i = sq.at[:, _ds((i & 3) * M, M, 8)]
            for c0 in range(0, M // 4, 8):
                _stage(rq_i, sq_i, c0, 8, lambda x: tie(x, c0 // 4 + 2), groups=(1,))
            wq_transpose(jnp.minimum(i + 1, NP - 1), lambda x, k: tie(x, 36 + 3 * k))
            slot = pl.ds((i & (NRAW - 1)) * CS, CS)
            for n, (raw, stg, wt_s) in enumerate(((rk, sk, wkt_s), (rv, sv, wvt_s))):
                for c0 in range(0, CS, 8):
                    _stage(raw.at[slot], stg, c0, 8, lambda x: tie(x, 16 * n + c0 // 8))
                cols = _ds(i * CS, CS, CS)
                for pair in range(H // 2):
                    for dt in range(2):
                        blk = stg[(pair // 4) * 2 + dt, pl.ds(pair % 4, CS, stride=4), :]
                        row = pair * D + dt * HD
                        blk = jnp.concatenate([tie(blk[:8], 16 + 24 * n + 3 * pair + dt), blk[8:]], axis=0)
                        wt_s[row:row + HD, cols] = blk.T

            tie = clk.pacer(ty + AP0, span, 28)
            ckv_i = ckv_s.at[i & (NRAW - 1)]
            a_i = a_s.at[_ds(i * (T // 4), T // 4, T // 4)]
            for r in range(0, T // 2, 16):
                def block(o, q):
                    col = (o % 2) * 2 * QC + (q % 2) * QC
                    return ckv_i[2 * (q // 2) + o // 2, r:r + 16, col:col + QC].astype(f32)
                for n1 in range(7):
                    ops = _operands2(_A_TERMS, n1, block, lambda x: tie(x, 7 * (r // 16) + n1))
                    _put(a_i, r, 7 * n1 * QC, ops)
            return carry

        lax.fori_loop(0, NP, phase2, carry0)
        cp_wo.wait()
        prep_w(h, range(NT1), _no_tie)

    @pl.when(h == 0)
    def _():
        prologue(**pro_refs)

    def oproj(jp, clk):
        cols = slice(2 * jp * T, (2 * jp + 2) * T)
        for r, n in OCH:
            c = clk.strassen(lambda i: _get(wl_s, r, n, i * T, T),
                             lambda i: _get(cl_s, 0, HD, (jp * 7 + i) * T, T), _NN)()
            o_s[r:r + n, cols] += jnp.concatenate(c[:2], axis=1)
            o_s[HM + r:HM + r + n, cols] += jnp.concatenate(c[2:], axis=1)

    def head(mk_s, mv_s, mp_s, kt_s, ka_s, va_s, v2_s, s_s, pb_s, pd_s, p2_s, sc_s, qb_s, kd_s):
        clk = _Clock(zero_s)
        q_h = q_s.at[_ds(h * D, D, D)]

        def prep_wo(tie):
            for r in range(0, HM, 16):
                top = tie(wo_s[h, r:r + 16, :].astype(f32), r // 16)
                bot = tie(wo_s[h, HM + r:HM + r + 16, :].astype(f32), r // 16)
                _put(wl_s, r, 0, _operands(_A_TERMS, [top[:, :HD], top[:, HD:], bot[:, :HD], bot[:, HD:]]))

        nine = lambda c: _operands(_A_TERMS, c) + [c[1], c[2]]

        def outer(m_s, r):
            return _combine([m_s[n * HD + r:n * HD + r + 16, :] for n in range(7)], order=range(7))

        def proj(g, lo, hi):
            for n1 in range(lo, hi):
                comb = clk.strassen(lambda n: _get(w_s, 0, 2 * QD, (7 * n1 + n) * QC, QC),
                                    lambda n: _get(a_s, g * T, T, (7 * n1 + n) * QC, QC), _NT, n1 == 6)
                for r in range(0, 2 * QD, GC):
                    m_s, row = mk_s if r < QD else mv_s.at[g % 2], n1 * HD + r % QD
                    c = comb(r, GC)
                    m_s[row:row + GC, :] = jnp.concatenate([c[0], c[2]], axis=1)
                    m_s[QD + row:QD + row + GC, :] = jnp.concatenate([c[1], c[3]], axis=1)
            if hi < 7:
                return
            cs = [outer(mk_s, r) for r in range(0, HD, 16)]
            for n in range(4):
                kt_s[:, n * T:(n + 1) * T] = jnp.concatenate([c[n] for c in cs], axis=0).T
            for r in range(0, 2 * T, GC):
                blk = kt_s[r:r + GC, :]
                ops = nine([blk[:, n * T:(n + 1) * T] for n in range(4)])
                _put(ka_s, 2 * g * T + r, 0, ops[:7] + ops[8:] if SES else ops)
            if SES:
                for r in (0, 32, T, T + 32):
                    lo_, hi_ = kt_s[r:r + 32, 0:2 * T], kt_s[r + T // 2:r + T // 2 + 32, 0:2 * T]
                    _put(kd_s, r // T * (T // 2) + r % T, 0,
                         _operands(_A_TERMS, [lo_[:, :T], lo_[:, T:], hi_[:, :T], hi_[:, T:]]))

        def vfin(g, tie):
            m_s = mv_s.at[g % 2]
            for r in range(0, QD, 16):
                k, blk = 8 * (r // 16), {}
                late = lambda w: tie(w, k, True, FLAG)
                for new, n1 in (((0,), 2), ((1,), 4), ((3,), 6), ((), 0), ((), 3), ((2,), 5), ((), 1)):
                    for o in new:
                        for i, row in enumerate((r, QD + r)):
                            tiles = _Tiles([m_s.at[n * HD:(n + 1) * HD] for n in range(7)], row, 16)
                            c, = _combine(tiles, ((o % 2) * 2 + o // 2,), range(7))
                            blk[o, i] = c = tie(c, k)
                            slot = (2, 7, 8, 3)[o]
                            _put(va_s, row, ((2 * g + 1) * 9 + slot) * T, [c[:, T:]])
                            if o in (1, 2):
                                _put(va_s, row, (2 * g * 9 + slot) * T, [c[:, :T]])
                    lo_, hi_ = [_operand(_A_TERMS[n1], lambda o: blk[o, i]) for i in range(2)]
                    _put(va_s, r, (2 * g * 9 + n1) * T, [lo_[:, :T]], late)
                    _put(va_s, QD + r, (2 * g * 9 + n1) * T, [hi_[:, :T]], late)
                    if g < 3:
                        _put(v2_s, r, (g * 7 + n1) * 7 * T,
                             _operands(_A_TERMS, [lo_[:, :T], lo_[:, T:], hi_[:, :T], hi_[:, T:]]), late)
                    k += 8 / 7

        key = lax.broadcasted_iota(jnp.int32, (T, 2 * T), 0)
        qry = lax.broadcasted_iota(jnp.int32, (T, 2 * T), 1)
        causal = key <= qry

        marks = []

        def qk(g):
            pairs = (2 * g, 2 * g + 1)
            mx = {jp: _Reducer(jnp.max, jnp.maximum) for jp in pairs}

            def put(jp, row, v):
                v = v.reshape(v.shape[0] // 8, 8, 2 * T)
                s_s[jp % 4, row // 8:row // 8 + v.shape[0]] = v
                mx[jp].add(v)

            def rect(jp, lo, hi, n):
                for r in range(lo, hi, n):
                    c = clk.strassen(lambda i: _get(ka_s, r, n, i * T, T),
                                     lambda i: _get(qb_s, 0, HD, ((jp % 2) * 7 + i) * T, T), _NN)()
                    put(jp, r, jnp.concatenate(c[:2], axis=1))
                    put(jp, jp * T + r, jnp.concatenate(c[2:], axis=1))

            q = lambda jp, e: _get(q_h, e * D, D, jp * T, T)
            for jp in pairs[g == 0 and not SES:]:
                for r in range(0, HD, 32):
                    blk = [_get(q_h, e * D + d * HD + r, 32, jp * T, T).astype(f32) for d in range(2) for e in range(2)]
                    _put(qb_s, r, (jp % 2) * 7 * T, _operands(_B_TERMS, blk))
            for jp in pairs:
                rect(jp, 0, 2 * g * T, QCH if QCH else g * T // 2 or 1)
                marks.append(clk.t)
            kb = lambda jp, a, b: jnp.concatenate(
                [_get(ka_s, jp * T, T, a * T, T), _get(ka_s, jp * T, T, b * T, T)], axis=1)
            last = {}
            for jp in pairs:
                so = jnp.where(causal[:, :T], clk.dot(kb(jp, 7, 3), q(jp, 1), _NN)[0], NEG)
                row = (2 * jp + 1) * T // 8
                s_s[jp % 4, row:row + T // 8, :, T:] = so.reshape(T // 8, 8, T)
                last[jp] = jnp.concatenate([jnp.full((1, T), NEG, f32), jnp.max(so, axis=0, keepdims=True)], axis=1)
            rect(2 * g + 1, 2 * g * T, (2 * g + 1) * T, T // 2)
            for jp in pairs:
                c = clk.strassen(lambda i: _get(kd_s, (jp % 2) * (T // 2), T // 2, i * T, T),
                                 lambda i: _get(qb_s, 0, HD, ((jp % 2) * 7 + i) * T, T), _NN)()
                se = jnp.concatenate([jnp.concatenate(c[:2], axis=1), jnp.concatenate(c[2:], axis=1)], axis=0)
                put(jp, 2 * jp * T, jnp.where(causal, se, NEG))
            return [jnp.broadcast_to(jnp.maximum(mx[jp].result(), last[jp]), (8, 2 * T)) for jp in pairs]

        zs, sums = {}, {}

        def prob(jp, row, z, n=GS, lanes=slice(None)):
            return jnp.exp2(s_s[jp % 4, row // 8:(row + n) // 8, :, lanes] - z[:, lanes])

        def rough(jp, mx, tie):
            zs[jp] = mx
            if jp > 0:
                sm = _Reducer(jnp.sum, jnp.add)
                for k, r in enumerate(range(0, 2 * jp * T, GS * LSUB)):
                    sm.add(prob(jp, r, tie(mx, k)))
                zs[jp] = mx + jnp.log2(jnp.maximum(LSUB * sm.result(), 1.0))
            sums[jp] = _Reducer(jnp.sum, jnp.add)

        def blocks(jp, row, tie, k):
            top, bot = prob(jp, row, tie(zs[jp], k)), prob(jp, jp * T + row, tie(zs[jp], k + 1))
            sums[jp].add(top + bot)
            top, bot = top.reshape(GS, 2 * T), bot.reshape(GS, 2 * T)
            return [top[:, :T], top[:, T:], bot[:, :T], bot[:, T:]]

        def near(jp, tie, k):
            R, z = jp * T, zs[jp]
            if jp % 2:
                for r in range(0, T, GS):
                    _put(pb_s, jp // 2 * T + r, 0, _operands(_B_TERMS, blocks(jp, R - T + r, tie, k)))
                    k += 2
            for r in range(0, T, GS):
                p = prob(jp, 2 * R + r, tie(z, k))
                sums[jp].add(p)
                _put(pd_s, 2 * R + r, 0, [p.reshape(GS, 2 * T)])
                k += 1
            so = _Reducer(jnp.sum, jnp.add)
            for r in range(0, T, 2 * GS):
                p = prob(jp, 2 * R + T + r, tie(z, k), 2 * GS, slice(T, 2 * T))
                so.add(p)
                _put(pd_s, 2 * R + T + r, T, [p.reshape(2 * GS, T)])
                k += 1
            sums[jp].result()
            sums[jp].out = sums[jp].out + jnp.concatenate([jnp.zeros((1, T), f32), so.result()], axis=1)

        p20 = lambda g: g * (g - 1) // 2 * T

        def far(g, tie, k):
            half = {(jp, e): _Reducer(jnp.sum, jnp.add) for jp in (2 * g, 2 * g + 1) for e in range(2)}
            for kg in range(g):
                for r in range(0, T, GS):
                    blk = {}
                    for new, n1 in (((0,), 1), ((1,), 5), ((3,), 2), ((), 0), ((), 4), ((2,), 3), ((), 6)):
                        for o in new:
                            lanes = slice((o % 2) * T, (o % 2 + 1) * T)
                            for jp in (2 * g, 2 * g + 1):
                                z = tie(zs[jp][:, lanes], k)
                                row = (o // 2) * jp * T + 2 * kg * T + r
                                p = [jnp.exp2(s_s[jp % 4, x // 8:(x + GS) // 8, :, lanes] - z) for x in (row, row + T)]
                                half[jp, o % 2].add(p[0] + p[1])
                                blk[o, jp % 2], blk[o, 2 + jp % 2] = [x.reshape(GS, T) for x in p]
                        ops = _operands2(_B_TERMS, n1, lambda o, q: blk[o, q], lambda x: x)
                        _put(p2_s, p20(g) + kg * T + r, 7 * n1 * T, ops,
                             (lambda w: tie(w, k, True, FLAG)) if FTIE else None)
                        k += FW * 8 / 7
            for jp in (2 * g, 2 * g + 1):
                if g:
                    sums[jp].out = sums[jp].out + jnp.concatenate([half[jp, e].result() for e in range(2)], axis=1)
            for jp in (2 * g, 2 * g + 1):
                cols = slice(2 * jp * T, 2 * (jp + 1) * T)
                sc_s[:, cols] = g_s[:, cols] / sums[jp].result()

        def pv(g):
            pairs = (2 * g, 2 * g + 1)
            va = lambda n, t, r=0, nr=HD: _get(va_s, r, nr, (t * 9 + n) * T, T)
            for n1 in range(7 if g else 0):
                c = clk.strassen(
                    lambda n: _cat([_get(v2_s, 0, QD, (kg * 49 + 7 * n1 + n) * T, T) for kg in range(g)], 1),
                    lambda n: _get(p2_s, p20(g), g * T, (7 * n1 + n) * T, T), _NN)()
                mp_s[n1 * HD:n1 * HD + QD, :] = jnp.concatenate(c[:2], axis=1)
                mp_s[n1 * HD + QD:(n1 + 1) * HD, :] = jnp.concatenate(c[2:], axis=1)
            ve = [jnp.concatenate([va(2, jp), va(8, jp)], axis=0) for jp in pairs]
            vo = [jnp.concatenate([va(7, jp), va(3, jp)], axis=0) for jp in pairs]
            if NEAR64:
                near64 = [clk.strassen(lambda n: va(n, 2 * g, r, QD),
                                       lambda n: _get(pb_s, g * T, T, n * T, T), _NN) for r in (0, QD)]
            ce = clk.level([(ve[jp % 2], _get(pd_s, 2 * jp * T, T, 0, T)) for jp in pairs])
            co = [clk.dot(jnp.concatenate([ve[jp % 2], vo[jp % 2]], axis=1),
                          _get(pd_s, 2 * jp * T, 2 * T, T, T), _NN)[0] for jp in pairs]
            for jp in pairs:
                R, e = jp * T, jp % 2
                ge, go = sc_s[:, 2 * R:2 * R + T], sc_s[:, 2 * R + T:2 * R + 2 * T]
                for r in range(0, HD, 32):
                    c = [ce[e][r:r + 32], co[e][r:r + 32], ce[e][HD + r:HD + r + 32], co[e][HD + r:HD + r + 32]]
                    if g:
                        far_ = _combine([mp_s[n * HD + r:n * HD + r + 32, e * T:(e + 1) * T] for n in range(7)],
                                        order=range(7))
                        c = [x + y for x, y in zip(c, far_)]
                    if e and NEAR64:
                        c = [x + y for x, y in zip(c, near64[r // QD](r % QD, 32))]
                    elif e:
                        near_ = clk.strassen(lambda n: va(n, 2 * g, r, 32),
                                             lambda n: _get(pb_s, g * T, T, n * T, T), _NN)()
                        c = [x + y for x, y in zip(c, near_)]
                    ops = _operands(_B_TERMS, [c[0] * ge, c[1] * go, c[2] * ge, c[3] * go])
                    _put(cl_s, r, jp * 7 * T, ops)

        ends = []

        def run(items):
            for item in items.split():
                if item[0] == 'P':
                    pv(int(item[1]))
                    ends.append(clk.t)
                elif item[0] == 'K':
                    proj(int(item[1]), int(item[2]), int(item[3]))
                else:
                    jp = int(item[1])
                    oproj(jp, clk)

                    @pl.when(h == H - 1)
                    def _():
                        out_copy(jp).start()

        for n1 in range(7):
            if n1 >= NT1:
                prep_w(h, [n1], clk.pacer(max(clk.t - LEAD - 448, 1), max(clk.t - LEAD, 1), 8))
            proj(0, n1, n1 + 1)
        oproj(NP - 1, clk)
        mx = qk(0)
        for g in range(4):
            t0 = clk.t
            del ends[:]
            run(PLAN[g])
            t1 = clk.t
            nxt = qk(g + 1) if g < 3 else None
            n_rough = [2 * jp * T // (GS * LSUB) for jp in (2 * g, 2 * g + 1)]
            n_near = [(T + T // 2) // GS, (3 * T + T // 2) // GS]
            holes = [(t - PH0, t + PH1) for t in ends]
            if 0 < g < 3:
                holes += [(marks[-2] - SW0, marks[-2] + SW1), (marks[-1] - SE0, marks[-1] + SE1)]
            if g < 3:
                vfin(g, clk.pacer(t0 - VB, t0 + VW, 32))
                holes += [(t0, t0 + VW), (t1 - HOLE0, t1 + HOLE1)]
            if g == 2:
                vfin(3, clk.pacer(clk.t - SLACK - VW // 2, clk.t - SLACK, 32))
                holes.append((clk.t - SLACK - VW // 2, clk.t))
            tie = clk.pacer(t0 + D0, (clk.t if g else t1) - SLACK,
                            sum(n_rough) + sum(n_near) + FW * g * 8 * T // GS, holes)
            rough(2 * g, mx[0], tie)
            near(2 * g, tie, n_rough[0])
            k = n_rough[0] + n_near[0]
            rough(2 * g + 1, mx[1], lambda x, i: tie(x, k + i))
            near(2 * g + 1, tie, k + n_rough[1])
            far(g, tie, k + n_rough[1] + n_near[1])
            if g == 0:
                prep_wo(clk.pacer(t0 + VW, t1 - HOLE0, HM // 16))
            mx = nxt
        t0 = clk.t
        run(PLAN[4])
        prep_w(jnp.minimum(h + 1, H - 1), range(NT1), clk.pacer(t0 - PW0, clk.t - 300, 8 * NT1))
        if os.environ.get('SHOW'):
            print('final loads', clk.load)

    head(**head_refs)

    @pl.when(h == H - 1)
    def _():
        oproj(NP - 1, _Clock(zero_s))
        out_copy(NP - 1).start()
        for jp in range(NP):
            out_copy(jp).wait()


@jax.jit
def pallas_gated_mix__compressed_kv_cla__ssm_conv_s5__prompt_kernel(
    A_x: jax.Array,
    A_c_kv: jax.Array,
    A_w_q: jax.Array,
    A_w_uk: jax.Array,
    A_w_uv: jax.Array,
    A_w_o: jax.Array,
    B_x: jax.Array,
    B_Lambda_re: jax.Array,
    B_Lambda_im: jax.Array,
    B_B_re: jax.Array,
    B_B_im: jax.Array,
    B_C_re: jax.Array,
    B_C_im: jax.Array,
    B_log_dt: jax.Array,
    B_Dskip: jax.Array,
    gate_w: jax.Array,
):
    del B_x
    xT = jnp.transpose(A_x[0])
    woT = jnp.transpose(A_w_o, (0, 2, 1))
    ckv = A_c_kv.reshape(4, 4, 2, T // 2, DC)

    hbm = pl.BlockSpec(memory_space=pl.ANY)
    outT = pl.pallas_call(
        _kernel,
        grid=(H,),
        in_specs=[hbm] * 15,
        out_specs=hbm,
        out_shape=jax.ShapeDtypeStruct((M, S), f32),
        scratch_shapes=_SHARED_SCRATCH + list(_PROLOGUE_SCRATCH.values()) + list(_HEAD_SCRATCH.values()),
        compiler_params=pltpu.CompilerParams(
            dimension_semantics=("arbitrary",),
            vmem_limit_bytes=127 * 1024 * 1024,
        ),
    )(xT, B_B_re, B_B_im, B_C_re, B_C_im, B_Lambda_re, B_Lambda_im, B_log_dt,
      B_Dskip, gate_w, woT, ckv, A_w_q, A_w_uk, A_w_uv)
    return jnp.transpose(outT)[None]
```

```python
import bisect

import jax
import jax.numpy as jnp
from jax import lax
import jax.experimental.pallas as pl
import jax.experimental.pallas.tpu as pltpu

S = 2048
M = 448
H = 16
D = 256
DC = 1024
T = 128
NP = S // T // 2
HD = D // 2
HM = M // 2
QD = D // 4
QC = DC // 4
QM = M // 4
PA = 384
PB = M - PA
TA = 512
TC = 256
CS = DC // NP
NRAW = 4
LOG2E = 1.4426950408889634
NEG = -1e30

GS = 16
RCH = 256
LSUB = 4
NT1 = 3
OCH = ((0, 64), (64, 64), (128, 48), (176, 48))
PLAN = ('K1', 'K2', 'K3', 'P1 P0 O2 O3 P2 O0 O1 O4', 'O5 P3 O6')
SLACK, LATE, VW = 200, 40, 900

f32 = jnp.float32
bf16 = jnp.bfloat16
u32 = jnp.uint32

SEM_VEC, SEM_B, SEM_X, SEM_WQ, SEM_C, SEM_SL, SEM_WO, SEM_OUT, SEM_WQ1 = 0, 1, 2, 6, 7, 8, 16, 17, 18
NSEM = 22

_NN = ((1,), (0,))
_NT = ((1,), (1,))
_TT = ((0,), (1,))


def _cat(xs, axis):
    return xs[0] if len(xs) == 1 else jnp.concatenate(xs, axis=axis)


def _ds(lo, n, align):
    return pl.ds(lo if isinstance(lo, int) else pl.multiple_of(lo, align), n)


def _put(ref, row, col, xs, tie=None):
    x = _cat(xs, 1)
    if tie is not None:
        x = jnp.concatenate([tie(x[:8]), x[8:]], axis=0)
    ref[row // 2:(row + x.shape[0]) // 2, col:col + x.shape[1]] = pltpu.bitcast(x.astype(bf16), u32)


def _get(ref, row, nrows, col, ncols):
    return pltpu.bitcast(ref[row // 2:(row + nrows) // 2, col:col + ncols], bf16)


class _Clock:
    def __init__(self, zero_ref):
        self.masks = {(8, T): zero_ref[...] != 0.0}
        self.ticks, self.load = [], [0, 0, 0, 0]

    @property
    def t(self):
        return max(self.load)

    def dot(self, a, b, dims):
        v = lax.dot_general(a, b, (dims, ((), ())), preferred_element_type=f32)
        rows, depth = v.shape[0], a.shape[dims[0][0]]
        for c in range(0, v.shape[1], T):
            start = 0
            for _ in range(0, depth, T):
                k = self.load.index(min(self.load))
                start = max(start, self.load[k])
                self.load[k] += rows
            self.ticks += [(start + r + 8, (v, r, c)) for r in range(0, rows, 8)]
        return v

    def strassen(self, lhs, rhs, dims, jobs=1, split_last=False):
        lag = sum(l + 32 <= max(self.load) for l in self.load) // jobs if jobs < 3 else 0
        order = ((1, 3, 2, 4, 0, 5, 6), (0, 1, 3, 2, 4, 5, 6), (5, 6, 1, 3, 2, 4, 0), (0, 5, 6, 1, 3, 2, 4))[lag]
        m = {}
        for n in order:
            a, b = lhs(n), rhs(n)
            if split_last and n == order[-1]:
                half = a.shape[0] // 2
                m[n] = jnp.concatenate([self.dot(a[:half], b, dims), self.dot(a[half:], b, dims)], axis=0)
            else:
                m[n] = self.dot(a, b, dims)
        return lambda r=0, n=None: _combine(m if n is None else _Rows(m, r, n), order=order)

    def level(self, pairs):
        base, extra = divmod((sum(self.load) + sum(a.shape[0] for a, _ in pairs)) // 16, 4)
        target = [16 * (base + (k < extra)) for k in range(4)]
        out = []
        for a, b in pairs:
            r, parts = 0, []
            while r < a.shape[0]:
                k = self.load.index(min(self.load))
                n = min(max(target[k] - self.load[k], 16), a.shape[0] - r)
                parts.append(self.dot(a[r:r + n], b, _NN))
                r += n
            out.append(_cat(parts, 0))
        return out

    def pacer(self, t0, t1, n, holes=()):
        holes = sorted((max(a, t0), min(b, t1)) for a, b in holes if a < t1 and b > t0)
        gap = sum(b - a for a, b in holes)
        ticks = sorted(self.ticks, key=lambda tw: tw[0])
        times = [tw[0] for tw in ticks]

        def tie(x, k, distinct=False, delay=0):
            t = t0 + (t1 - t0 - gap) * k / n
            for a, b in holes:
                t += b - a if t > a else 0
            t += delay
            past = ticks[:bisect.bisect_right(times, t)]
            reps = (x.shape[0] // 8, x.shape[1] // T)
            if len(past) < (reps[1] if distinct else 1):
                return x
            tick = _cat([v[r:r + 8, c:c + T] for _, (v, r, c) in past[-reps[1] if distinct else -1:]], 1)
            if tick.dtype != x.dtype:
                tick = pltpu.bitcast(tick, x.dtype)
            if x.shape not in self.masks:
                self.masks[x.shape] = jnp.tile(self.masks[(8, T)], reps)
            return lax.select(self.masks[x.shape], tick if tick.shape == x.shape else jnp.tile(tick, reps), x)
        return tie


def _no_tie(x, k):
    return x


_A_TERMS = ((0, 3, 1), (2, 3, 1), (0, None, 0), (3, None, 0), (0, 1, 1), (2, 0, -1), (1, 3, -1))
_B_TERMS = ((0, 3, 1), (0, None, 0), (1, 3, -1), (2, 0, -1), (3, None, 0), (0, 1, 1), (2, 3, 1))


def _operand(term, block):
    x, y, sign = term
    if y is None:
        return block(x)
    return block(x) + block(y) if sign > 0 else block(x) - block(y)


def _operands(terms, blocks):
    return [_operand(t, blocks.__getitem__) for t in terms]


def _operands2(terms, n1, block, tie):
    first = terms[n1][0]
    sub = [_operand(terms[n1], lambda o: tie(block(o, q)) if o == first and q in (0, 3) else block(o, q))
           for q in range(4)]
    return _operands(terms, sub)


_C_TERMS = ({0: 1, 3: 1, 4: -1, 6: 1}, {2: 1, 4: 1}, {1: 1, 3: 1}, {0: 1, 1: -1, 2: 1, 5: 1})


def _combine(m, only=(0, 1, 2, 3), order=(1, 3, 2, 4, 0, 5, 6)):
    out = []
    for terms in (_C_TERMS[n] for n in only):
        seq = [n for n in order if n in terms]
        if terms[seq[0]] < 0:
            seq[0], seq[1] = seq[1], seq[0]
        acc = m[seq[0]]
        for n in seq[1:]:
            acc = acc + m[n] if terms[n] > 0 else acc - m[n]
        out.append(acc)
    return out


def _outer_step(m_s, n1, row, v):
    n = v.shape[0]
    if n1 < 5:
        m_s[n1 * HD + row:n1 * HD + row + n, :] = v
    if n1 < 3:
        return None
    blk = (2, 1, 3, 0)[n1 - 3]
    m = {j: v if j == n1 else m_s[j * HD + row:j * HD + row + n, :] for j in _C_TERMS[blk]}
    return blk, _combine(m, (blk,), range(7))[0]


class _Rows:
    def __init__(self, vals, r, n):
        self.vals, self.rows, self.cache = vals, slice(r, r + n), {}

    def __getitem__(self, i):
        if i not in self.cache:
            self.cache[i] = self.vals[i][self.rows, :]
        return self.cache[i]


class _Reducer:
    def __init__(self, red, comb):
        self.red, self.comb, self.acc, self.rows, self.out = red, comb, None, 0, None

    def add(self, v):
        self.rows += 8 * v.shape[0]
        v = self.red(v, axis=0)
        self.acc = v if self.acc is None else self.comb(self.acc, v)
        if self.rows >= RCH:
            self.result()

    def result(self):
        if self.acc is not None:
            v = self.red(self.acc, axis=0, keepdims=True)
            self.out = v if self.out is None else self.comb(self.out, v)
        self.acc, self.rows = None, 0
        return self.out


def _cmul(ar, ai, br, bi):
    return ar * br - ai * bi, ar * bi + ai * br


def _hi16(w):
    return pltpu.bitcast(w & jnp.uint32(0xFFFF0000), f32)


def _stage(raw, stg, c0, nc, tie, groups=(0, 1)):
    for ht in groups:
        for dt in range(2):
            v = raw[c0:c0 + nc, ht * 8:(ht + 1) * 8, dt * T:(dt + 1) * T].reshape(nc * 8, T)
            stg[ht * 2 + dt, c0 * 4:(c0 + nc) * 4, :] = tie(pltpu.bitcast(v, u32))


def _ssm_params(vec_s, coef_s, lam_s, col_s):
    row = lambda r: r[...].astype(f32).reshape(1, M)
    lre, lim, ldt, dsk, gw = [row(v) for v in vec_s]
    dt = jnp.exp(ldt).astype(bf16).astype(f32)
    mag = jnp.exp(dt * lre)
    ang = dt * lim
    lr, li = mag * jnp.cos(ang), mag * jnp.sin(ang)
    den = lre * lre + lim * lim
    nr = lr - 1.0
    coef_s[...] = jnp.zeros(coef_s.shape, f32)
    coef_s[0:1, 0:M] = 2.0 * ((nr * lre + li * lim) / den)
    coef_s[1:2, 0:M] = 2.0 * ((li * lre - nr * lim) / den)

    er = jnp.concatenate([lr, lr[:, PA:]], axis=1)
    ei = jnp.concatenate([li, -li[:, PA:]], axis=1)
    pw = [(er, ei)]
    for _ in range(7):
        pw.append(_cmul(pw[-1][0], pw[-1][1], er, ei))
    sub = lax.broadcasted_iota(jnp.int32, (8, 512), 0)
    for n, d in enumerate((1, 2, 4)):
        lam_s[2 * n] = jnp.where(sub >= d, pw[d - 1][0], 0.0)
        lam_s[2 * n + 1] = jnp.where(sub >= d, pw[d - 1][1], 0.0)
    lcr = jnp.zeros((8, 512), f32)
    lci = jnp.zeros((8, 512), f32)
    for r in range(8):
        lcr = jnp.where(sub == r, pw[r][0], lcr)
        lci = jnp.where(sub == r, pw[r][1], lci)
    lam_s[6] = lcr
    lam_s[7] = lci

    def col(v):
        v = jnp.concatenate([v, jnp.zeros((1, 512 - M), f32)], axis=1)
        return jnp.broadcast_to(v, (T, 512)).T[:M]
    col_s[0] = col(dsk)
    col_s[1] = col(gw)


def _ssm_cmat(craw_s, coef_s, c_s, tie):
    for r in range(0, M, 16):
        coef = tie(coef_s[...], r // 16)
        cr, ci = coef[0:1, :M], coef[1:2, :M]
        re, im = _cmul(craw_s[0, r:r + 16, :].astype(f32), craw_s[1, r:r + 16, :].astype(f32), cr, ci)
        _put(c_s, r, 0, [re[:, :PA], -im[:, :PA], re[:, PA:], -im[:, PA:]])


def _ssm_scan(u_ref, carry, lam_s, h_s, tie):
    car, cai = carry
    out = []
    for b in range(TC // 8):
        mixed = u_ref[3, b, :, 0:T]
        u = jnp.concatenate([u_ref[cb, b] for cb in range(3)], axis=1)
        cols = [u[:, 0:T], u[:, T:2 * T], u[:, 2 * T:PA], mixed]
        hr = jnp.concatenate([tie(v, 4 * b + n) for n, v in enumerate(cols)], axis=1)
        hi = jnp.concatenate([u[:, PA:2 * PA], pltpu.roll(mixed, PB, 1)], axis=1)
        for n, d in enumerate((1, 2, 4)):
            sr, si = pltpu.roll(hr, d, 0), pltpu.roll(hi, d, 0)
            tr, ti = _cmul(sr, si, lam_s[2 * n], lam_s[2 * n + 1])
            hr, hi = hr + tr, hi + ti
        tr, ti = _cmul(lam_s[6], lam_s[7], car, cai)
        hr, hi = hr + tr, hi + ti
        car, cai = hr[7:8, :], hi[7:8, :]
        out.append(jnp.concatenate([hr[:, :PA], hi[:, :PA], hr[:, PA:]], axis=1))
        if b % 2 == 1:
            _put(h_s, (b - 1) * 8, 0, [jnp.concatenate(out, axis=0)])
            out = []
    return car, cai


_vmem = pltpu.VMEM
_PROLOGUE_SCRATCH = dict(
    xT_s=_vmem((M, S), bf16),
    v0=_vmem((M,), bf16), v1=_vmem((M,), bf16), v2=_vmem((M,), bf16), v3=_vmem((M,), bf16), v4=_vmem((M,), bf16),
    b_s=_vmem((2 * M, M), bf16),
    craw_s=_vmem((2, M, M), bf16),
    c_s=_vmem((M // 2, 2 * M), u32),
    coef_s=_vmem((8, 512), f32),
    lam_s=_vmem((8, 8, 512), f32),
    col_s=_vmem((2, M, T), f32),
    h_s=_vmem((TC // 2, 2 * M), u32),
    ckv_s=_vmem((NRAW, 4, T // 2, DC), bf16),
    rq=_vmem((M, H, D), bf16),
    rk=_vmem((NRAW * CS, H, D), bf16),
    rv=_vmem((NRAW * CS, H, D), bf16),
    sq=_vmem((4, M * 4, T), u32),
    sk=_vmem((4, CS * 4, T), u32),
    sv=_vmem((4, CS * 4, T), u32),
    wqt_s=_vmem((D, 4 * T), u32),
)
_HEAD_SCRATCH = dict(
    mk_s=_vmem((7 * HD, 2 * T), f32),
    mv_s=_vmem((2, 7 * HD, 2 * T), f32),
    mp_s=_vmem((7 * HD, 2 * T), f32),
    kt_s=_vmem((2 * T, 4 * T), f32),
    ka_s=_vmem((S // 4, 8 * T), u32),
    va_s=_vmem((HD // 2, NP * 9 * T), u32),
    v2_s=_vmem((QD // 2, 3 * 49 * T), u32),
    s_s=_vmem((4, S // 8, 8, 2 * T), f32),
    pb_s=_vmem((2 * T, 7 * T), u32),
    pd_s=_vmem((S // 2, 2 * T), u32),
    p2_s=_vmem((3 * T, 49 * T), u32),
    sc_s=_vmem((1, S), f32),
    qb_s=_vmem((HD // 2, 14 * T), u32),
    kd_s=_vmem((T // 2, 7 * T), u32),
)
_SHARED_SCRATCH = [
    _vmem((H // 2 * D, DC), u32),
    _vmem((H // 2 * D, DC), u32),
    _vmem((S // 8, 49 * QC), u32),
    _vmem((H * D, S // 2), u32),
    _vmem((H, M, D), bf16),
    _vmem((QD, 49 * QC), u32),
    _vmem((HM // 2, 7 * T), u32),
    _vmem((HD // 2, NP * 7 * T), u32),
    _vmem((M, S), f32),
    _vmem((1, S), f32),
    _vmem((8, T), f32),
    pltpu.SemaphoreType.DMA((NSEM,)),
]


def _kernel(xT_hbm, bre_hbm, bim_hbm, cre_hbm, cim_hbm, lre_hbm, lim_hbm, ldt_hbm,
            dsk_hbm, gw_hbm, woT_hbm, ckv_hbm, wq_hbm, wk_hbm, wv_hbm,
            out_hbm,
            wkt_s, wvt_s, a_s, q_s, wo_s, w_s, wl_s, cl_s, o_s, g_s, zero_s, sem, *rest):
    h = pl.program_id(0)
    pro_refs = dict(zip(_PROLOGUE_SCRATCH, rest))
    head_refs = dict(zip(_HEAD_SCRATCH, rest[len(pro_refs):]))

    def out_copy(jp):
        cols = pl.ds(jp * 2 * T, 2 * T)
        return pltpu.make_async_copy(o_s.at[:, cols], out_hbm.at[:, cols], sem.at[SEM_OUT])

    def prep_w(hh, outer, tie):
        rows = _ds(lax.shift_right_logical(hh, 1) * D, D, D)
        sh = (16 * (1 - (hh & 1))).astype(u32)
        k = 0
        for row0, wt_s in ((0, wkt_s.at[rows]), (QD, wvt_s.at[rows])):
            for r in range(0, QD, 16):
                def block(o, q):
                    row = (o % 2) * HD + (q % 2) * QD + r
                    col = (o // 2) * 2 * QC + (q // 2) * QC
                    return _hi16(wt_s[row:row + 16, col:col + QC] << sh)
                for n1 in outer:
                    _put(w_s, row0 + r, 7 * n1 * QC, _operands2(_B_TERMS, n1, block, lambda x: tie(x, k)))
                    k += 1

    def prologue(xT_s, v0, v1, v2, v3, v4, b_s, craw_s, c_s, coef_s, lam_s, col_s, h_s,
                 ckv_s, rq, rk, rv, sq, sk, sv, wqt_s):
        xa_s = head_refs['p2_s']
        wq_s = xa_s.at[2 * QM:2 * QM + QD]
        u_s = head_refs['s_s']
        vec_s = (v0, v1, v2, v3, v4)

        def slice_copies(i):
            s = sem.at[SEM_SL + i]
            grp = i // 2 if isinstance(i, int) else lax.shift_right_logical(i, 1)
            cs, dst = pl.ds(i * CS, CS), pl.ds((i & (NRAW - 1)) * CS, CS)
            return [pltpu.make_async_copy(ckv_hbm.at[grp, :, i & 1], ckv_s.at[i & (NRAW - 1)], s),
                    pltpu.make_async_copy(wk_hbm.at[cs], rk.at[dst], s),
                    pltpu.make_async_copy(wv_hbm.at[cs], rv.at[dst], s)]

        def wq1_copy(i):
            rows = pl.ds(i * (M // 4), M // 4)
            return pltpu.make_async_copy(wq_hbm.at[rows, 8:16], rq.at[rows, 8:16], sem.at[SEM_WQ1 + i])

        def x_copy(i):
            cols = pl.ds(i * TA, TA)
            return pltpu.make_async_copy(xT_hbm.at[:, cols], xT_s.at[:, cols], sem.at[SEM_X + i])

        cp_vec = [pltpu.make_async_copy(src, dst, sem.at[SEM_VEC])
                  for src, dst in zip((lre_hbm, lim_hbm, ldt_hbm, dsk_hbm, gw_hbm), vec_s)]
        cp_b = [pltpu.make_async_copy(src.at[pl.ds(lo, n)], b_s.at[pl.ds(dst, n)], sem.at[SEM_B])
                for src, lo, n, dst in ((bre_hbm, 0, PA, 0), (bim_hbm, 0, PA, PA),
                                        (bre_hbm, PA, PB, 2 * PA), (bim_hbm, PA, PB, 2 * PA + PB))]
        cp_wq = [pltpu.make_async_copy(wq_hbm.at[:, 0:8], rq.at[:, 0:8], sem.at[SEM_WQ])]
        cp_c = [pltpu.make_async_copy(src, craw_s.at[n], sem.at[SEM_C])
                for n, src in enumerate((cre_hbm, cim_hbm))]
        cp_wo = pltpu.make_async_copy(woT_hbm, wo_s, sem.at[SEM_WO])
        for cp in cp_vec + cp_b + [x_copy(i) for i in range(S // TA)] + cp_c + cp_wq:
            cp.start()
        for i in range(NRAW - 1):
            for cp in [wq1_copy(i)] + slice_copies(i):
                cp.start()
        wq1_copy(3).start()
        cp_wo.start()

        zero_s[...] = jnp.zeros(zero_s.shape, f32)
        wl_s[...] = jnp.zeros(wl_s.shape, u32)
        cl_s[:, (NP - 1) * 7 * T:] = jnp.zeros((HD // 2, 7 * T), u32)
        for cp in cp_vec:
            cp.wait()
        _ssm_params(vec_s, coef_s, lam_s, col_s)

        def wq_transpose(pair, tie):
            ht = pair // 4 if isinstance(pair, int) else lax.shift_right_logical(pair, 2)
            pad = jnp.zeros((T - QM, T), u32)
            for dt in range(2):
                for mq in range(4):
                    blk = sq[ht * 2 + dt, pl.ds(mq * QM * 4 + (pair & 3), QM, stride=4), :]
                    blk = jnp.concatenate([tie(blk[:8], 4 * dt + mq), blk[8:], pad], axis=0)
                    wqt_s[dt * HD:(dt + 1) * HD, mq * T:(mq + 1) * T] = blk.T

        def phase1(i):
            clk = _Clock(zero_s)
            u = _cat([clk.dot(xT_s[:, i * TA + lo:i * TA + hi], b_s[...], _TT)
                      for lo, hi in ((0, T), (T, TA))], 0)
            for cb in range(4):
                w = min(2 * T, 2 * M - cb * 2 * T)
                u_s[cb, i * TA // 8:(i + 1) * TA // 8, :, 0:w] = (
                    u[:, cb * 2 * T:cb * 2 * T + w].reshape(TA // 8, 8, w))
            tie = clk.pacer(0, 6 * TA, 49)
            for r in range(0, QM, 16):
                def block(o, q):
                    row, col = (o % 2) * HM + (q % 2) * QM + r, (4 * i + 2 * (q // 2) + o // 2) * T
                    return xT_s[row:row + 16, col:col + T].astype(f32)
                for n1 in range(7):
                    ops = _operands2(_A_TERMS, n1, block, lambda x: tie(x, 7 * (r // 16) + n1))
                    _put(xa_s, i * QM + r, 7 * n1 * T, ops)
            tie = clk.pacer(0, 6 * TA, 8 * 14)
            for t in range(TA // T):
                cols = slice(i * TA + t * T, i * TA + (t + 1) * T)
                acc = jnp.zeros((8, T), f32)
                for r in range(0, M, 32):
                    xg = xT_s[r:r + 32, cols].astype(f32) * tie(col_s[1, r:r + 32, :], 28 * t + r // 32)
                    acc = acc + jnp.sum(xg.reshape(4, 8, T), axis=0)
                g = jax.nn.sigmoid(jnp.sum(acc, axis=0, keepdims=True))
                g_s[:, cols] = g
                for r in range(0, M, 32):
                    skip = xT_s[r:r + 32, cols].astype(f32) * tie(col_s[0, r:r + 32, :], 28 * t + 14 + r // 32)
                    o_s[r:r + 32, cols] = (1.0 - g) * skip
            return clk

        for cp in cp_b + [x_copy(0)]:
            cp.wait()
        phase1(0)
        x_copy(1).wait()
        clk = phase1(1)
        zero = jnp.zeros((1, 512), f32)
        carry0 = _ssm_scan(u_s.at[:, 0:TC // 8], (zero, zero), lam_s, h_s, clk.pacer(0, 6 * TA, TC // 2))
        for cp in [x_copy(2), x_copy(3)] + cp_c + cp_wq:
            cp.wait()
        _ssm_cmat(craw_s, coef_s, c_s, phase1(2).pacer(0, 6 * TA, M // 16))
        tie = phase1(3).pacer(0, 6 * TA, M // 8)
        for c0 in range(0, M, 8):
            _stage(rq, sq, c0, 8, lambda x: tie(x, c0 // 10), groups=(0,))
        wq_transpose(0, lambda x, k: tie(x, 46 + k))

        def phase2(i, carry):
            @pl.when(i + NRAW - 1 < NP)
            def _():
                for cp in slice_copies(i + NRAW - 1):
                    cp.start()

            @pl.when(i < 4)
            def _():
                wq1_copy(i).wait()

            for cp in slice_copies(i):
                cp.wait()

            clk = _Clock(zero_s)
            yT = _cat([clk.dot(_get(c_s, r, HM, 0, 2 * M), _get(h_s, 0, TC, 0, 2 * M), _NT)
                       for r in (0, HM)], 0)
            ty = clk.t
            cols = _ds(i * TC, TC, TC)
            keep = 1.0 - g_s[:, cols]
            for r in range(0, M, 32):
                o_s[r:r + 32, cols] += keep * yT[r:r + 32]

            q_i = q_s.at[_ds(i * 2 * D, 2 * D, 2 * D)]
            mq_s = (head_refs['mk_s'], head_refs['mp_s'], head_refs['mv_s'].at[0], head_refs['mv_s'].at[1])
            for g in range(4):
                for n1 in range(7):
                    if g == 0:
                        t = 200 + (ty + 644) * n1 / 7
                        tie = clk.pacer(min(t, clk.t - 500), min(t + 300, clk.t - 500), 8)
                        for r in range(0, 2 * QD, 16):
                            def block(o, q):
                                row = (o % 2) * HD + (q % 2) * QD + r % QD
                                col = (2 * (o // 2) + q // 2) * T
                                w = wqt_s[row:row + 16, col:col + T]
                                return _hi16(w) if r >= QD else pltpu.bitcast(w << 16, f32)
                            _put(wq_s, r, 7 * n1 * T, _operands2(_B_TERMS, n1, block, lambda x: tie(x, r // 16)))
                    comb = clk.strassen(lambda n: _get(wq_s, 0, 2 * QD, (7 * n1 + n) * T, QM),
                                        lambda n: _get(xa_s, g * QM, QM, (7 * n1 + n) * T, T), _NN)
                    for r in range(0, 2 * QD, 32):
                        e, c = r // QD, comb(r, 32)
                        for dq in range(2):
                            row = dq * QD + r % QD
                            done = _outer_step(mq_s[2 * (g % 2) + e], n1, row,
                                               jnp.concatenate([c[dq], c[2 + dq]], axis=1))
                            if done:
                                n, v = done
                                _put(q_i, (2 * e + n // 2) * D + (n % 2) * HD + row, 2 * g * T,
                                     [v * (LOG2E * D ** -0.5)])

            span = ty + 6000

            u_next = u_s.at[:, pl.ds(jnp.minimum(i + 1, NP - 1) * (TC // 8), TC // 8)]
            carry = _ssm_scan(u_next, carry, lam_s, h_s, clk.pacer(ty, span, TC // 2))

            tie = clk.pacer(ty - 1200, span, 64, [(ty, ty + 1000)])
            rq_i = rq.at[pl.ds((i & 3) * (M // 4), M // 4)]
            sq_i = sq.at[:, _ds((i & 3) * M, M, 8)]
            for c0 in range(0, M // 4, 8):
                _stage(rq_i, sq_i, c0, 8, lambda x: tie(x, c0 // 4 + 2), groups=(1,))
            wq_transpose(jnp.minimum(i + 1, NP - 1), lambda x, k: tie(x, 36 + 3 * k))
            slot = pl.ds((i & (NRAW - 1)) * CS, CS)
            for n, (raw, stg, wt_s) in enumerate(((rk, sk, wkt_s), (rv, sv, wvt_s))):
                for c0 in range(0, CS, 8):
                    _stage(raw.at[slot], stg, c0, 8, lambda x: tie(x, 16 * n + c0 // 8))
                cols = _ds(i * CS, CS, CS)
                for pair in range(H // 2):
                    for dt in range(2):
                        blk = stg[(pair // 4) * 2 + dt, pl.ds(pair % 4, CS, stride=4), :]
                        row = pair * D + dt * HD
                        blk = jnp.concatenate([tie(blk[:8], 16 + 24 * n + 3 * pair + dt), blk[8:]], axis=0)
                        wt_s[row:row + HD, cols] = blk.T

            tie = clk.pacer(ty + 1000, span, 28)
            ckv_i = ckv_s.at[i & (NRAW - 1)]
            a_i = a_s.at[_ds(i * (T // 4), T // 4, T // 4)]
            for r in range(0, T // 2, 16):
                def block(o, q):
                    col = (o % 2) * 2 * QC + (q % 2) * QC
                    return ckv_i[2 * (q // 2) + o // 2, r:r + 16, col:col + QC].astype(f32)
                for n1 in range(7):
                    ops = _operands2(_A_TERMS, n1, block, lambda x: tie(x, 7 * (r // 16) + n1))
                    _put(a_i, r, 7 * n1 * QC, ops)
            return carry

        lax.fori_loop(0, NP, phase2, carry0)
        cp_wo.wait()
        prep_w(h, range(NT1), _no_tie)

    @pl.when(h == 0)
    def _():
        prologue(**pro_refs)

    def oproj(jp, clk):
        cols = slice(2 * jp * T, (2 * jp + 2) * T)
        for r, n in OCH:
            c = clk.strassen(lambda i: _get(wl_s, r, n, i * T, T),
                             lambda i: _get(cl_s, 0, HD, (jp * 7 + i) * T, T), _NN)()
            o_s[r:r + n, cols] += jnp.concatenate(c[:2], axis=1)
            o_s[HM + r:HM + r + n, cols] += jnp.concatenate(c[2:], axis=1)

    def head(mk_s, mv_s, mp_s, kt_s, ka_s, va_s, v2_s, s_s, pb_s, pd_s, p2_s, sc_s, qb_s, kd_s):
        clk = _Clock(zero_s)
        q_h = q_s.at[_ds(h * D, D, D)]

        def prep_wo(tie):
            for r in range(0, HM, 16):
                top = tie(wo_s[h, r:r + 16, :].astype(f32), r // 16)
                bot = tie(wo_s[h, HM + r:HM + r + 16, :].astype(f32), r // 16)
                _put(wl_s, r, 0, _operands(_A_TERMS, [top[:, :HD], top[:, HD:], bot[:, :HD], bot[:, HD:]]))

        def proj(g, lo=0, hi=7):
            for n1 in range(lo, hi):
                comb = clk.strassen(lambda n: _get(w_s, 0, 2 * QD, (7 * n1 + n) * QC, QC),
                                    lambda n: _get(a_s, g * T, T, (7 * n1 + n) * QC, QC), _NT, 2, n1 == 6)
                for r, m_s in ((0, mk_s), (QD, mv_s.at[g % 2])):
                    c = comb(r, QD)
                    m_s[n1 * HD:n1 * HD + QD, :] = jnp.concatenate([c[0], c[2]], axis=1)
                    m_s[n1 * HD + QD:(n1 + 1) * HD, :] = jnp.concatenate([c[1], c[3]], axis=1)
            if hi < 7:
                return
            cs = [_combine([mk_s[n * HD + r:n * HD + r + 16, :] for n in range(7)], order=range(7))
                  for r in range(0, HD, 16)]
            for n in range(4):
                kt_s[:, n * T:(n + 1) * T] = jnp.concatenate([c[n] for c in cs], axis=0).T
            for r in range(0, 2 * T, T // 2):
                blk = kt_s[r:r + T // 2, :]
                blk = [blk[:, n * T:(n + 1) * T] for n in range(4)]
                _put(ka_s, 2 * g * T + r, 0, _operands(_A_TERMS, blk) + [blk[2]])
            for r in (0, 32, T, T + 32):
                lo_, hi_ = kt_s[r:r + 32, 0:2 * T], kt_s[r + T // 2:r + T // 2 + 32, 0:2 * T]
                _put(kd_s, r // T * (T // 2) + r % T, 0,
                     _operands(_A_TERMS, [lo_[:, :T], lo_[:, T:], hi_[:, :T], hi_[:, T:]]))

        def vfin(g, tie):
            m_s = mv_s.at[g % 2]
            for r in range(0, QD, 16):
                k, blk = 8 * (r // 16), {}
                late = lambda w: tie(w, k, True, LATE)
                for new, n1 in (((0,), 2), ((1,), 4), ((3,), 6), ((), 0), ((), 3), ((2,), 5), ((), 1)):
                    for o in new:
                        for i, row in enumerate((r, QD + r)):
                            tiles = _Rows([m_s.at[n * HD:(n + 1) * HD] for n in range(7)], row, 16)
                            c, = _combine(tiles, ((o % 2) * 2 + o // 2,), range(7))
                            blk[o, i] = c = tie(c, k)
                            slot = (2, 7, 8, 3)[o]
                            _put(va_s, row, ((2 * g + 1) * 9 + slot) * T, [c[:, T:]])
                            if o in (1, 2):
                                _put(va_s, row, (2 * g * 9 + slot) * T, [c[:, :T]])
                    lo_, hi_ = [_operand(_A_TERMS[n1], lambda o: blk[o, i]) for i in range(2)]
                    _put(va_s, r, (2 * g * 9 + n1) * T, [lo_[:, :T]], late)
                    _put(va_s, QD + r, (2 * g * 9 + n1) * T, [hi_[:, :T]], late)
                    if g < 3:
                        _put(v2_s, r, (g * 7 + n1) * 7 * T,
                             _operands(_A_TERMS, [lo_[:, :T], lo_[:, T:], hi_[:, :T], hi_[:, T:]]), late)
                    k += 8 / 7

        key = lax.broadcasted_iota(jnp.int32, (T, 2 * T), 0)
        qry = lax.broadcasted_iota(jnp.int32, (T, 2 * T), 1)
        causal = key <= qry

        marks = []

        def qk(g):
            pairs = (2 * g, 2 * g + 1)
            mx = {jp: _Reducer(jnp.max, jnp.maximum) for jp in pairs}

            def put(jp, row, v):
                v = v.reshape(v.shape[0] // 8, 8, 2 * T)
                s_s[jp % 4, row // 8:row // 8 + v.shape[0]] = v
                mx[jp].add(v)

            def rect(jp, lo, hi):
                for r in range(lo, hi, T // 2):
                    c = clk.strassen(lambda i: _get(ka_s, r, T // 2, i * T, T),
                                     lambda i: _get(qb_s, 0, HD, ((jp % 2) * 7 + i) * T, T), _NN)()
                    put(jp, r, jnp.concatenate(c[:2], axis=1))
                    put(jp, jp * T + r, jnp.concatenate(c[2:], axis=1))

            for jp in pairs:
                for r in range(0, HD, 32):
                    blk = [_get(q_h, e * D + d * HD + r, 32, jp * T, T).astype(f32) for d in range(2) for e in range(2)]
                    _put(qb_s, r, (jp % 2) * 7 * T, _operands(_B_TERMS, blk))
            for jp in pairs:
                rect(jp, 0, 2 * g * T)
                marks.append(clk.t)
            last = {}
            for jp in pairs:
                ko = jnp.concatenate([_get(ka_s, jp * T, T, n * T, T) for n in (7, 3)], axis=1)
                so = jnp.where(causal[:, :T], clk.dot(ko, _get(q_h, D, D, jp * T, T), _NN), NEG)
                row = (2 * jp + 1) * T // 8
                s_s[jp % 4, row:row + T // 8, :, T:] = so.reshape(T // 8, 8, T)
                last[jp] = jnp.concatenate([jnp.full((1, T), NEG, f32), jnp.max(so, axis=0, keepdims=True)], axis=1)
            rect(2 * g + 1, 2 * g * T, (2 * g + 1) * T)
            for jp in pairs:
                c = clk.strassen(lambda i: _get(kd_s, (jp % 2) * (T // 2), T // 2, i * T, T),
                                 lambda i: _get(qb_s, 0, HD, ((jp % 2) * 7 + i) * T, T), _NN)()
                se = jnp.concatenate([jnp.concatenate(c[:2], axis=1), jnp.concatenate(c[2:], axis=1)], axis=0)
                put(jp, 2 * jp * T, jnp.where(causal, se, NEG))
            return [jnp.broadcast_to(jnp.maximum(mx[jp].result(), last[jp]), (8, 2 * T)) for jp in pairs]

        zs, sums = {}, {}

        def prob(jp, row, z, n=GS, lanes=slice(None)):
            return jnp.exp2(s_s[jp % 4, row // 8:(row + n) // 8, :, lanes] - z[:, lanes])

        def rough(jp, mx, tie):
            zs[jp] = mx
            if jp > 0:
                sm = _Reducer(jnp.sum, jnp.add)
                for k, r in enumerate(range(0, 2 * jp * T, GS * LSUB)):
                    sm.add(prob(jp, r, tie(mx, k)))
                zs[jp] = mx + jnp.log2(jnp.maximum(LSUB * sm.result(), 1.0))
            sums[jp] = _Reducer(jnp.sum, jnp.add)

        def blocks(jp, row, tie, k):
            top, bot = prob(jp, row, tie(zs[jp], k)), prob(jp, jp * T + row, tie(zs[jp], k + 1))
            sums[jp].add(top + bot)
            top, bot = top.reshape(GS, 2 * T), bot.reshape(GS, 2 * T)
            return [top[:, :T], top[:, T:], bot[:, :T], bot[:, T:]]

        def near(jp, tie, k):
            R, z = jp * T, zs[jp]
            if jp % 2:
                for r in range(0, T, GS):
                    _put(pb_s, jp // 2 * T + r, 0, _operands(_B_TERMS, blocks(jp, R - T + r, tie, k)))
                    k += 2
            for r in range(0, T, GS):
                p = prob(jp, 2 * R + r, tie(z, k))
                sums[jp].add(p)
                _put(pd_s, 2 * R + r, 0, [p.reshape(GS, 2 * T)])
                k += 1
            so = _Reducer(jnp.sum, jnp.add)
            for r in range(0, T, 2 * GS):
                p = prob(jp, 2 * R + T + r, tie(z, k), 2 * GS, slice(T, 2 * T))
                so.add(p)
                _put(pd_s, 2 * R + T + r, T, [p.reshape(2 * GS, T)])
                k += 1
            sums[jp].result()
            sums[jp].out = sums[jp].out + jnp.concatenate([jnp.zeros((1, T), f32), so.result()], axis=1)

        p20 = lambda g: g * (g - 1) // 2 * T

        def far(g, tie, k):
            half = {(jp, e): _Reducer(jnp.sum, jnp.add) for jp in (2 * g, 2 * g + 1) for e in range(2)}
            for kg in range(g):
                for r in range(0, T, GS):
                    blk = {}
                    for new, n1 in (((0,), 1), ((1,), 5), ((3,), 2), ((), 0), ((), 4), ((2,), 3), ((), 6)):
                        for o in new:
                            lanes = slice((o % 2) * T, (o % 2 + 1) * T)
                            for jp in (2 * g, 2 * g + 1):
                                z = tie(zs[jp][:, lanes], k)
                                row = (o // 2) * jp * T + 2 * kg * T + r
                                p = [jnp.exp2(s_s[jp % 4, x // 8:(x + GS) // 8, :, lanes] - z) for x in (row, row + T)]
                                half[jp, o % 2].add(p[0] + p[1])
                                blk[o, jp % 2], blk[o, 2 + jp % 2] = [x.reshape(GS, T) for x in p]
                        ops = _operands2(_B_TERMS, n1, lambda o, q: blk[o, q], lambda x: x)
                        _put(p2_s, p20(g) + kg * T + r, 7 * n1 * T, ops, lambda w: tie(w, k, True, LATE))
                        k += 16 / 7
            for jp in (2 * g, 2 * g + 1):
                if g:
                    sums[jp].out = sums[jp].out + jnp.concatenate([half[jp, e].result() for e in range(2)], axis=1)
            for jp in (2 * g, 2 * g + 1):
                cols = slice(2 * jp * T, 2 * (jp + 1) * T)
                sc_s[:, cols] = g_s[:, cols] / sums[jp].result()

        def pv(g):
            pairs = (2 * g, 2 * g + 1)
            va = lambda n, t, r=0, nr=HD: _get(va_s, r, nr, (t * 9 + n) * T, T)
            for n1 in range(7 if g else 0):
                c = clk.strassen(
                    lambda n: _cat([_get(v2_s, 0, QD, (kg * 49 + 7 * n1 + n) * T, T) for kg in range(g)], 1),
                    lambda n: _get(p2_s, p20(g), g * T, (7 * n1 + n) * T, T), _NN, g)()
                mp_s[n1 * HD:n1 * HD + QD, :] = jnp.concatenate(c[:2], axis=1)
                mp_s[n1 * HD + QD:(n1 + 1) * HD, :] = jnp.concatenate(c[2:], axis=1)
            ve = [jnp.concatenate([va(2, jp), va(8, jp)], axis=0) for jp in pairs]
            vo = [jnp.concatenate([va(7, jp), va(3, jp)], axis=0) for jp in pairs]
            ce = clk.level([(ve[jp % 2], _get(pd_s, 2 * jp * T, T, 0, T)) for jp in pairs])
            co = [clk.dot(jnp.concatenate([ve[jp % 2], vo[jp % 2]], axis=1),
                          _get(pd_s, 2 * jp * T, 2 * T, T, T), _NN) for jp in pairs]
            for jp in pairs:
                R, e = jp * T, jp % 2
                ge, go = sc_s[:, 2 * R:2 * R + T], sc_s[:, 2 * R + T:2 * R + 2 * T]
                for r in range(0, HD, 32):
                    c = [ce[e][r:r + 32], co[e][r:r + 32], ce[e][HD + r:HD + r + 32], co[e][HD + r:HD + r + 32]]
                    if g:
                        far_ = _combine([mp_s[n * HD + r:n * HD + r + 32, e * T:(e + 1) * T] for n in range(7)],
                                        order=range(7))
                        c = [x + y for x, y in zip(c, far_)]
                    if e:
                        near_ = clk.strassen(lambda n: va(n, 2 * g, r, 32),
                                             lambda n: _get(pb_s, g * T, T, n * T, T), _NN)()
                        c = [x + y for x, y in zip(c, near_)]
                    ops = _operands(_B_TERMS, [c[0] * ge, c[1] * go, c[2] * ge, c[3] * go])
                    _put(cl_s, r, jp * 7 * T, ops)

        ends = []

        def run(items):
            for item in items.split():
                if item[0] == 'P':
                    pv(int(item[1]))
                    ends.append(clk.t)
                elif item[0] == 'K':
                    proj(int(item[1]))
                else:
                    jp = int(item[1])
                    oproj(jp, clk)

                    @pl.when(h == H - 1)
                    def _():
                        out_copy(jp).start()

        for n1 in range(7):
            if n1 >= NT1:
                prep_w(h, [n1], clk.pacer(clk.t - 896, clk.t - 448, 8))
            proj(0, n1, n1 + 1)
        oproj(NP - 1, clk)
        mx = qk(0)
        for g in range(4):
            t0 = clk.t
            del ends[:]
            run(PLAN[g])
            t1 = clk.t
            nxt = qk(g + 1) if g < 3 else None
            n_rough = [2 * jp * T // (GS * LSUB) for jp in (2 * g, 2 * g + 1)]
            n_near = [(T + T // 2) // GS, (3 * T + T // 2) // GS]
            holes = [(t - 400, t) for t in ends]
            if 0 < g < 3:
                holes.append((marks[-2] - 400, marks[-2] - 100))
            if g < 3:
                vfin(g, clk.pacer(t0, t0 + VW, 32))
                holes += [(t0, t0 + VW), (t1 - 300, t1 + 300)]
            if g == 2:
                vfin(3, clk.pacer(clk.t - SLACK - VW // 2, clk.t - SLACK, 32))
                holes.append((clk.t - SLACK - VW // 2, clk.t))
            tie = clk.pacer(t0, (clk.t if g else t1) - SLACK,
                            sum(n_rough) + sum(n_near) + g * 16 * T // GS, holes)
            rough(2 * g, mx[0], tie)
            near(2 * g, tie, n_rough[0])
            k = n_rough[0] + n_near[0]
            rough(2 * g + 1, mx[1], lambda x, i: tie(x, k + i))
            near(2 * g + 1, tie, k + n_rough[1])
            far(g, tie, k + n_rough[1] + n_near[1])
            if g == 0:
                prep_wo(clk.pacer(t0 + VW, t1 - 300, HM // 16))
            mx = nxt
        t0 = clk.t
        run(PLAN[4])
        prep_w(jnp.minimum(h + 1, H - 1), range(NT1), clk.pacer(t0 - 100, clk.t - 300, 8 * NT1))
        assert len(set(clk.load)) == 1

    head(**head_refs)

    @pl.when(h == H - 1)
    def _():
        oproj(NP - 1, _Clock(zero_s))
        out_copy(NP - 1).start()
        for jp in range(NP):
            out_copy(jp).wait()


@jax.jit
def pallas_gated_mix__compressed_kv_cla__ssm_conv_s5__prompt_kernel(
    A_x: jax.Array,
    A_c_kv: jax.Array,
    A_w_q: jax.Array,
    A_w_uk: jax.Array,
    A_w_uv: jax.Array,
    A_w_o: jax.Array,
    B_x: jax.Array,
    B_Lambda_re: jax.Array,
    B_Lambda_im: jax.Array,
    B_B_re: jax.Array,
    B_B_im: jax.Array,
    B_C_re: jax.Array,
    B_C_im: jax.Array,
    B_log_dt: jax.Array,
    B_Dskip: jax.Array,
    gate_w: jax.Array,
):
    del B_x
    xT = jnp.transpose(A_x[0])
    woT = jnp.transpose(A_w_o, (0, 2, 1))
    ckv = A_c_kv.reshape(4, 4, 2, T // 2, DC)

    hbm = pl.BlockSpec(memory_space=pl.ANY)
    outT = pl.pallas_call(
        _kernel,
        grid=(H,),
        in_specs=[hbm] * 15,
        out_specs=hbm,
        out_shape=jax.ShapeDtypeStruct((M, S), f32),
        scratch_shapes=_SHARED_SCRATCH + list(_PROLOGUE_SCRATCH.values()) + list(_HEAD_SCRATCH.values()),
        compiler_params=pltpu.CompilerParams(
            dimension_semantics=("arbitrary",),
            vmem_limit_bytes=127 * 1024 * 1024,
        ),
    )(xT, B_B_re, B_B_im, B_C_re, B_C_im, B_Lambda_re, B_Lambda_im, B_log_dt,
      B_Dskip, gate_w, woT, ckv, A_w_q, A_w_uk, A_w_uv)
    return jnp.transpose(outT)[None]
```

```python
import bisect

import jax
import jax.numpy as jnp
from jax import lax
import jax.experimental.pallas as pl
import jax.experimental.pallas.tpu as pltpu

S = 2048
M = 448
H = 16
D = 256
DC = 1024
T = 128
NP = S // T // 2
HD = D // 2
HM = M // 2
QD = D // 4
QC = DC // 4
QM = M // 4
PA = 384
PB = M - PA
TA = 512
TC = 256
CS = DC // NP
NRAW = 2
LOG2E = 1.4426950408889634
NEG = -1e30

GS = 16
RCH = 256
LSUB = 4
NT1 = 3
OCH = ((0, 64), (64, 64), (128, 48), (176, 48))
PLAN = ('K1', 'K2', 'K3', 'P1 P0 O2 O3 P2 O0 O1 O4', 'O5 P3 O6')
SLACK, LATE, VW = 200, 40, 900

f32 = jnp.float32
bf16 = jnp.bfloat16
u32 = jnp.uint32

SEM_VEC, SEM_B, SEM_X, SEM_WQ, SEM_C, SEM_SL, SEM_WO, SEM_OUT, SEM_WQ1, SEM_KV = 0, 1, 2, 6, 7, 8, 16, 17, 18, 22
NSEM = 24

_NN = ((1,), (0,))
_NT = ((1,), (1,))
_TT = ((0,), (1,))


def _cat(xs, axis):
    return xs[0] if len(xs) == 1 else jnp.concatenate(xs, axis=axis)


def _ds(lo, n, align):
    return pl.ds(lo if isinstance(lo, int) else pl.multiple_of(lo, align), n)


def _put(ref, row, col, xs, tie=None):
    x = _cat(xs, 1)
    if tie is not None:
        x = jnp.concatenate([tie(x[:8]), x[8:]], axis=0)
    ref[row // 2:(row + x.shape[0]) // 2, col:col + x.shape[1]] = pltpu.bitcast(x.astype(bf16), u32)


def _get(ref, row, nrows, col, ncols):
    return pltpu.bitcast(ref[row // 2:(row + nrows) // 2, col:col + ncols], bf16)


class _Clock:
    def __init__(self, zero_ref):
        self.masks = {(8, T): zero_ref[...] != 0.0}
        self.ticks, self.load = [], [0, 0, 0, 0]

    @property
    def t(self):
        return max(self.load)

    def dot(self, a, b, dims):
        v = lax.dot_general(a, b, (dims, ((), ())), preferred_element_type=f32)
        rows, depth = v.shape[0], a.shape[dims[0][0]]
        for c in range(0, v.shape[1], T):
            start = 0
            for _ in range(0, depth, T):
                k = self.load.index(min(self.load))
                start = max(start, self.load[k])
                self.load[k] += rows
            self.ticks += [(start + r + 8, (v, r, c)) for r in range(0, rows, 8)]
        return v

    def strassen(self, lhs, rhs, dims, jobs=1, split_last=False):
        lag = sum(l + 32 <= max(self.load) for l in self.load) // jobs if jobs < 3 else 0
        order = ((1, 3, 2, 4, 0, 5, 6), (0, 1, 3, 2, 4, 5, 6), (5, 6, 1, 3, 2, 4, 0), (0, 5, 6, 1, 3, 2, 4))[lag]
        m = {}
        for n in order:
            a, b = lhs(n), rhs(n)
            if split_last and n == order[-1]:
                half = a.shape[0] // 2
                m[n] = jnp.concatenate([self.dot(a[:half], b, dims), self.dot(a[half:], b, dims)], axis=0)
            else:
                m[n] = self.dot(a, b, dims)
        return lambda r=0, n=None: _combine(m if n is None else _Rows(m, r, n), order=order)

    def level(self, pairs):
        base, extra = divmod((sum(self.load) + sum(a.shape[0] for a, _ in pairs)) // 16, 4)
        target = [16 * (base + (k < extra)) for k in range(4)]
        out = []
        for a, b in pairs:
            r, parts = 0, []
            while r < a.shape[0]:
                k = self.load.index(min(self.load))
                n = min(max(target[k] - self.load[k], 16), a.shape[0] - r)
                parts.append(self.dot(a[r:r + n], b, _NN))
                r += n
            out.append(_cat(parts, 0))
        return out

    def pacer(self, t0, t1, n, holes=()):
        holes = sorted((max(a, t0), min(b, t1)) for a, b in holes if a < t1 and b > t0)
        gap = sum(b - a for a, b in holes)
        ticks = sorted(self.ticks, key=lambda tw: tw[0])
        times = [tw[0] for tw in ticks]

        def tie(x, k, distinct=False, delay=0):
            t = t0 + (t1 - t0 - gap) * k / n
            for a, b in holes:
                t += b - a if t > a else 0
            t += delay
            past = ticks[:bisect.bisect_right(times, t)]
            reps = (x.shape[0] // 8, x.shape[1] // T)
            if len(past) < (reps[1] if distinct else 1):
                return x
            tick = _cat([v[r:r + 8, c:c + T] for _, (v, r, c) in past[-reps[1] if distinct else -1:]], 1)
            if tick.dtype != x.dtype:
                tick = pltpu.bitcast(tick, x.dtype)
            if x.shape not in self.masks:
                self.masks[x.shape] = jnp.tile(self.masks[(8, T)], reps)
            return lax.select(self.masks[x.shape], tick if tick.shape == x.shape else jnp.tile(tick, reps), x)
        return tie


def _no_tie(x, k):
    return x


_A_TERMS = ((0, 3, 1), (2, 3, 1), (0, None, 0), (3, None, 0), (0, 1, 1), (2, 0, -1), (1, 3, -1))
_B_TERMS = ((0, 3, 1), (0, None, 0), (1, 3, -1), (2, 0, -1), (3, None, 0), (0, 1, 1), (2, 3, 1))


def _operand(term, block):
    x, y, sign = term
    if y is None:
        return block(x)
    return block(x) + block(y) if sign > 0 else block(x) - block(y)


def _operands(terms, blocks):
    return [_operand(t, blocks.__getitem__) for t in terms]


def _operands2(terms, n1, block, tie):
    first = terms[n1][0]
    sub = [_operand(terms[n1], lambda o: tie(block(o, q)) if o == first and q in (0, 3) else block(o, q))
           for q in range(4)]
    return _operands(terms, sub)


_C_TERMS = ({0: 1, 3: 1, 4: -1, 6: 1}, {2: 1, 4: 1}, {1: 1, 3: 1}, {0: 1, 1: -1, 2: 1, 5: 1})


def _combine(m, only=(0, 1, 2, 3), order=(1, 3, 2, 4, 0, 5, 6)):
    out = []
    for terms in (_C_TERMS[n] for n in only):
        seq = [n for n in order if n in terms]
        if terms[seq[0]] < 0:
            seq[0], seq[1] = seq[1], seq[0]
        acc = m[seq[0]]
        for n in seq[1:]:
            acc = acc + m[n] if terms[n] > 0 else acc - m[n]
        out.append(acc)
    return out


def _outer_step(m_s, n1, row, v):
    n = v.shape[0]
    if n1 < 5:
        m_s[n1 * HD + row:n1 * HD + row + n, :] = v
    if n1 < 3:
        return None
    blk = (2, 1, 3, 0)[n1 - 3]
    m = {j: v if j == n1 else m_s[j * HD + row:j * HD + row + n, :] for j in _C_TERMS[blk]}
    return blk, _combine(m, (blk,), range(7))[0]


class _Rows:
    def __init__(self, vals, r, n):
        self.vals, self.rows, self.cache = vals, slice(r, r + n), {}

    def __getitem__(self, i):
        if i not in self.cache:
            self.cache[i] = self.vals[i][self.rows, :]
        return self.cache[i]


class _Reducer:
    def __init__(self, red, comb):
        self.red, self.comb, self.acc, self.rows, self.out = red, comb, None, 0, None

    def add(self, v):
        self.rows += 8 * v.shape[0]
        v = self.red(v, axis=0)
        self.acc = v if self.acc is None else self.comb(self.acc, v)
        if self.rows >= RCH:
            self.result()

    def result(self):
        if self.acc is not None:
            v = self.red(self.acc, axis=0, keepdims=True)
            self.out = v if self.out is None else self.comb(self.out, v)
        self.acc, self.rows = None, 0
        return self.out


def _cmul(ar, ai, br, bi):
    return ar * br - ai * bi, ar * bi + ai * br


def _hi16(w):
    return pltpu.bitcast(w & jnp.uint32(0xFFFF0000), f32)


def _stage(raw, stg, c0, nc, tie, groups=(0, 1)):
    for ht in groups:
        for dt in range(2):
            v = raw[c0:c0 + nc, ht * 8:(ht + 1) * 8, dt * T:(dt + 1) * T].reshape(nc * 8, T)
            stg[ht * 2 + dt, c0 * 4:(c0 + nc) * 4, :] = tie(pltpu.bitcast(v, u32), (ht * 2 + dt) / 4)


def _ssm_params(vec_s, coef_s, lam_s, col_s):
    row = lambda r: r[...].astype(f32).reshape(1, M)
    lre, lim, ldt, dsk, gw = [row(v) for v in vec_s]
    dt = jnp.exp(ldt).astype(bf16).astype(f32)
    mag = jnp.exp(dt * lre)
    ang = dt * lim
    lr, li = mag * jnp.cos(ang), mag * jnp.sin(ang)
    den = lre * lre + lim * lim
    nr = lr - 1.0
    coef_s[...] = jnp.zeros(coef_s.shape, f32)
    coef_s[0:1, 0:M] = 2.0 * ((nr * lre + li * lim) / den)
    coef_s[1:2, 0:M] = 2.0 * ((li * lre - nr * lim) / den)

    er = jnp.concatenate([lr, lr[:, PA:]], axis=1)
    ei = jnp.concatenate([li, -li[:, PA:]], axis=1)
    pw = [(er, ei)]
    for _ in range(7):
        pw.append(_cmul(pw[-1][0], pw[-1][1], er, ei))
    sub = lax.broadcasted_iota(jnp.int32, (8, 512), 0)
    for n, d in enumerate((1, 2, 4)):
        lam_s[2 * n] = jnp.where(sub >= d, pw[d - 1][0], 0.0)
        lam_s[2 * n + 1] = jnp.where(sub >= d, pw[d - 1][1], 0.0)
    lcr = jnp.zeros((8, 512), f32)
    lci = jnp.zeros((8, 512), f32)
    for r in range(8):
        lcr = jnp.where(sub == r, pw[r][0], lcr)
        lci = jnp.where(sub == r, pw[r][1], lci)
    lam_s[6] = lcr
    lam_s[7] = lci

    def col(v):
        v = jnp.concatenate([v, jnp.zeros((1, 512 - M), f32)], axis=1)
        return jnp.broadcast_to(v, (T, 512)).T[:M]
    col_s[0] = col(dsk)
    col_s[1] = col(gw)


def _ssm_cmat(craw_s, coef_s, c_s, tie):
    for r in range(0, M, 16):
        coef = tie(coef_s[...], r // 16)
        cr, ci = coef[0:1, :M], coef[1:2, :M]
        re, im = _cmul(craw_s[0, r:r + 16, :].astype(f32), craw_s[1, r:r + 16, :].astype(f32), cr, ci)
        _put(c_s, r, 0, [re[:, :PA], -im[:, :PA], re[:, PA:], -im[:, PA:]])


def _ssm_scan(u_ref, carry, lam_s, h_s, tie):
    car, cai = carry
    out = []
    for b in range(TC // 8):
        mixed = u_ref[3, b, :, 0:T]
        u = jnp.concatenate([u_ref[cb, b] for cb in range(3)], axis=1)
        cols = [u[:, 0:T], u[:, T:2 * T], u[:, 2 * T:PA], mixed]
        hr = jnp.concatenate([tie(v, 4 * b + n) for n, v in enumerate(cols)], axis=1)
        hi = jnp.concatenate([u[:, PA:2 * PA], pltpu.roll(mixed, PB, 1)], axis=1)
        for n, d in enumerate((1, 2, 4)):
            sr, si = pltpu.roll(hr, d, 0), pltpu.roll(hi, d, 0)
            tr, ti = _cmul(sr, si, lam_s[2 * n], lam_s[2 * n + 1])
            hr, hi = hr + tr, hi + ti
        tr, ti = _cmul(lam_s[6], lam_s[7], car, cai)
        hr, hi = hr + tr, hi + ti
        car, cai = hr[7:8, :], hi[7:8, :]
        out.append(jnp.concatenate([hr[:, :PA], hi[:, :PA], hr[:, PA:]], axis=1))
        if b % 2 == 1:
            _put(h_s, (b - 1) * 8, 0, [jnp.concatenate(out, axis=0)])
            out = []
    return car, cai


_vmem = pltpu.VMEM
_PROLOGUE_SCRATCH = dict(
    xT_s=_vmem((M, S), bf16),
    v0=_vmem((M,), bf16), v1=_vmem((M,), bf16), v2=_vmem((M,), bf16), v3=_vmem((M,), bf16), v4=_vmem((M,), bf16),
    b_s=_vmem((2 * M, M), bf16),
    craw_s=_vmem((2, M, M), bf16),
    c_s=_vmem((M // 2, 2 * M), u32),
    coef_s=_vmem((8, 512), f32),
    lam_s=_vmem((8, 8, 512), f32),
    col_s=_vmem((2, M, T), f32),
    h_s=_vmem((TC // 2, 2 * M), u32),
    ckv_s=_vmem((NRAW, 4, T // 2, DC), bf16),
    rq=_vmem((M, H, D), bf16),
    rk=_vmem((CS + 1, H, D), bf16),
    rv=_vmem((CS + 1, H, D), bf16),
    sq=_vmem((4, M * 4, T), u32),
    sk=_vmem((4, CS * 4, T), u32),
    sv=_vmem((4, CS * 4, T), u32),
    wqt_s=_vmem((D, 4 * T), u32),
)
_HEAD_SCRATCH = dict(
    mk_s=_vmem((7 * HD, 2 * T), f32),
    mv_s=_vmem((2, 7 * HD, 2 * T), f32),
    mp_s=_vmem((7 * HD, 2 * T), f32),
    kt_s=_vmem((2 * T, 4 * T), f32),
    ka_s=_vmem((S // 4, 8 * T), u32),
    va_s=_vmem((HD // 2, NP * 9 * T), u32),
    v2_s=_vmem((QD // 2, 3 * 49 * T), u32),
    s_s=_vmem((4, S // 8, 8, 2 * T), f32),
    pb_s=_vmem((2 * T, 7 * T), u32),
    pd_s=_vmem((S // 2, 2 * T), u32),
    p2_s=_vmem((3 * T, 49 * T), u32),
    sc_s=_vmem((1, S), f32),
    qb_s=_vmem((HD // 2, 14 * T), u32),
    kd_s=_vmem((T // 2, 7 * T), u32),
)
_SHARED_SCRATCH = [
    _vmem((H // 2 * D, DC), u32),
    _vmem((H // 2 * D, DC), u32),
    _vmem((S // 8, 49 * QC), u32),
    _vmem((H * D, S // 2), u32),
    _vmem((H, M, D), bf16),
    _vmem((QD, 49 * QC), u32),
    _vmem((HM // 2, 7 * T), u32),
    _vmem((HD // 2, NP * 7 * T), u32),
    _vmem((M, S), f32),
    _vmem((1, S), f32),
    _vmem((8, T), f32),
    pltpu.SemaphoreType.DMA((NSEM,)),
]


def _kernel(xT_hbm, bre_hbm, bim_hbm, cre_hbm, cim_hbm, lre_hbm, lim_hbm, ldt_hbm,
            dsk_hbm, gw_hbm, woT_hbm, ckv_hbm, wq_hbm, wk_hbm, wv_hbm,
            out_hbm,
            wkt_s, wvt_s, a_s, q_s, wo_s, w_s, wl_s, cl_s, o_s, g_s, zero_s, sem, *rest):
    h = pl.program_id(0)
    pro_refs = dict(zip(_PROLOGUE_SCRATCH, rest))
    head_refs = dict(zip(_HEAD_SCRATCH, rest[len(pro_refs):]))

    def out_copy(jp):
        cols = pl.ds(jp * 2 * T, 2 * T)
        return pltpu.make_async_copy(o_s.at[:, cols], out_hbm.at[:, cols], sem.at[SEM_OUT])

    def prep_w(hh, outer, tie):
        rows = _ds(lax.shift_right_logical(hh, 1) * D, D, D)
        sh = (16 * (1 - (hh & 1))).astype(u32)
        k = 0
        for row0, wt_s in ((0, wkt_s.at[rows]), (QD, wvt_s.at[rows])):
            for r in range(0, QD, 16):
                def block(o, q):
                    row = (o % 2) * HD + (q % 2) * QD + r
                    col = (o // 2) * 2 * QC + (q // 2) * QC
                    return _hi16(wt_s[row:row + 16, col:col + QC] << sh)
                for n1 in outer:
                    _put(w_s, row0 + r, 7 * n1 * QC, _operands2(_B_TERMS, n1, block, lambda x: tie(x, k)))
                    k += 1

    def prologue(xT_s, v0, v1, v2, v3, v4, b_s, craw_s, c_s, coef_s, lam_s, col_s, h_s,
                 ckv_s, rq, rk, rv, sq, sk, sv, wqt_s):
        xa_s = head_refs['p2_s']
        wq_s = xa_s.at[2 * QM:2 * QM + QD]
        u_s = head_refs['s_s']
        vec_s = (v0, v1, v2, v3, v4)

        def slice_copies(i):
            s = sem.at[SEM_SL + i]
            grp = i // 2 if isinstance(i, int) else lax.shift_right_logical(i, 1)
            return [pltpu.make_async_copy(ckv_hbm.at[grp, :, i & 1], ckv_s.at[i & (NRAW - 1)], s)]

        def w_copy(n, i):
            src, dst = ((wk_hbm, rk), (wv_hbm, rv))[n]
            return pltpu.make_async_copy(src.at[pl.ds(i * CS, CS)], dst.at[0:CS], sem.at[SEM_KV + n])

        def wo_copy(i):
            heads = pl.ds(2 * i, 2)
            return pltpu.make_async_copy(woT_hbm.at[heads], wo_s.at[heads], sem.at[SEM_WO])

        def wq1_copy(i):
            rows = pl.ds(i * (M // 4), M // 4)
            return pltpu.make_async_copy(wq_hbm.at[rows, 8:16], rq.at[rows, 8:16], sem.at[SEM_WQ1 + i])

        def x_copy(i):
            cols = pl.ds(i * TA, TA)
            return pltpu.make_async_copy(xT_hbm.at[:, cols], xT_s.at[:, cols], sem.at[SEM_X + i])

        cp_vec = [pltpu.make_async_copy(src, dst, sem.at[SEM_VEC])
                  for src, dst in zip((lre_hbm, lim_hbm, ldt_hbm, dsk_hbm, gw_hbm), vec_s)]
        cp_b = [pltpu.make_async_copy(src.at[pl.ds(lo, n)], b_s.at[pl.ds(dst, n)], sem.at[SEM_B])
                for src, lo, n, dst in ((bre_hbm, 0, PA, 0), (bim_hbm, 0, PA, PA),
                                        (bre_hbm, PA, PB, 2 * PA), (bim_hbm, PA, PB, 2 * PA + PB))]
        cp_wq = [pltpu.make_async_copy(wq_hbm.at[:, 0:8], rq.at[:, 0:8], sem.at[SEM_WQ])]
        cp_c = [pltpu.make_async_copy(src, craw_s.at[n], sem.at[SEM_C])
                for n, src in enumerate((cre_hbm, cim_hbm))]
        for cp in cp_vec + cp_b + [x_copy(i) for i in range(S // TA)] + cp_c + cp_wq:
            cp.start()
        for cp in [wq1_copy(0)] + slice_copies(0) + [w_copy(0, 0), w_copy(1, 0)]:
            cp.start()

        zero_s[...] = jnp.zeros(zero_s.shape, f32)
        wl_s[...] = jnp.zeros(wl_s.shape, u32)
        cl_s[:, (NP - 1) * 7 * T:] = jnp.zeros((HD // 2, 7 * T), u32)
        for cp in cp_vec:
            cp.wait()
        _ssm_params(vec_s, coef_s, lam_s, col_s)

        def wq_transpose(pair, tie):
            ht = pair // 4 if isinstance(pair, int) else lax.shift_right_logical(pair, 2)
            pad = jnp.zeros((T - QM, T), u32)
            for dt in range(2):
                for mq in range(4):
                    blk = sq[ht * 2 + dt, pl.ds(mq * QM * 4 + (pair & 3), QM, stride=4), :]
                    blk = jnp.concatenate([tie(blk[:8], 4 * dt + mq), blk[8:], pad], axis=0)
                    wqt_s[dt * HD:(dt + 1) * HD, mq * T:(mq + 1) * T] = blk.T

        def phase1(i):
            clk = _Clock(zero_s)
            u = _cat([clk.dot(xT_s[:, i * TA + lo:i * TA + hi], b_s[...], _TT)
                      for lo, hi in ((0, T), (T, TA))], 0)
            for cb in range(4):
                w = min(2 * T, 2 * M - cb * 2 * T)
                u_s[cb, i * TA // 8:(i + 1) * TA // 8, :, 0:w] = (
                    u[:, cb * 2 * T:cb * 2 * T + w].reshape(TA // 8, 8, w))
            tie = clk.pacer(0, 6 * TA, 49)
            for r in range(0, QM, 16):
                def block(o, q):
                    row, col = (o % 2) * HM + (q % 2) * QM + r, (4 * i + 2 * (q // 2) + o // 2) * T
                    return xT_s[row:row + 16, col:col + T].astype(f32) * (LOG2E * D ** -0.5)
                for n1 in range(7):
                    ops = _operands2(_A_TERMS, n1, block, lambda x: tie(x, 7 * (r // 16) + n1))
                    _put(xa_s, i * QM + r, 7 * n1 * T, ops)
            tie = clk.pacer(0, 6 * TA, 8 * 14)
            for t in range(TA // T):
                cols = slice(i * TA + t * T, i * TA + (t + 1) * T)
                acc = jnp.zeros((8, T), f32)
                for r in range(0, M, 32):
                    xg = xT_s[r:r + 32, cols].astype(f32) * tie(col_s[1, r:r + 32, :], 28 * t + r // 32)
                    acc = acc + jnp.sum(xg.reshape(4, 8, T), axis=0)
                g = jax.nn.sigmoid(jnp.sum(acc, axis=0, keepdims=True))
                g_s[:, cols] = g
                for r in range(0, M, 32):
                    skip = xT_s[r:r + 32, cols].astype(f32) * tie(col_s[0, r:r + 32, :], 28 * t + 14 + r // 32)
                    o_s[r:r + 32, cols] = (1.0 - g) * skip
            return clk

        for cp in cp_b + [x_copy(0)]:
            cp.wait()
        phase1(0)
        x_copy(1).wait()
        clk = phase1(1)
        zero = jnp.zeros((1, 512), f32)
        carry0 = _ssm_scan(u_s.at[:, 0:TC // 8], (zero, zero), lam_s, h_s, clk.pacer(0, 6 * TA, TC // 2))
        for cp in [x_copy(2), x_copy(3)] + cp_c + cp_wq:
            cp.wait()
        _ssm_cmat(craw_s, coef_s, c_s, phase1(2).pacer(0, 6 * TA, M // 16))
        tie = phase1(3).pacer(0, 6 * TA, M // 8)
        for c0 in range(0, M, 8):
            _stage(rq, sq, c0, 8, lambda x, j: tie(x, c0 / 10 + j), groups=(0,))
        wq_transpose(0, lambda x, k: tie(x, 46 + k))

        def phase2(i, carry):
            @pl.when(i + 1 < NP)
            def _():
                for cp in slice_copies(i + 1):
                    cp.start()

            @pl.when(i < 3)
            def _():
                wq1_copy(i + 1).start()

            wo_copy(i).start()

            @pl.when(i < 4)
            def _():
                wq1_copy(i).wait()

            for cp in slice_copies(i) + [w_copy(0, i), w_copy(1, i)]:
                cp.wait()

            clk = _Clock(zero_s)
            yT = _cat([clk.dot(_get(c_s, r, HM, 0, 2 * M), _get(h_s, 0, TC, 0, 2 * M), _NT)
                       for r in (0, HM)], 0)
            ty = clk.t
            cols = _ds(i * TC, TC, TC)
            keep = 1.0 - g_s[:, cols]
            for r in range(0, M, 32):
                o_s[r:r + 32, cols] += keep * yT[r:r + 32]

            q_i = q_s.at[_ds(i * 2 * D, 2 * D, 2 * D)]
            mq_s = (head_refs['mk_s'], head_refs['mp_s'], head_refs['mv_s'].at[0], head_refs['mv_s'].at[1])
            for g in range(4):
                for n1 in range(7):
                    if g == 0:
                        t = 200 + (ty + 644) * n1 / 7
                        tie = clk.pacer(min(t, clk.t - 500), min(t + 300, clk.t - 500), 8)
                        for r in range(0, 2 * QD, 16):
                            def block(o, q):
                                row = (o % 2) * HD + (q % 2) * QD + r % QD
                                col = (2 * (o // 2) + q // 2) * T
                                w = wqt_s[row:row + 16, col:col + T]
                                return _hi16(w) if r >= QD else pltpu.bitcast(w << 16, f32)
                            _put(wq_s, r, 7 * n1 * T, _operands2(_B_TERMS, n1, block, lambda x: tie(x, r // 16)))
                    comb = clk.strassen(lambda n: _get(wq_s, 0, 2 * QD, (7 * n1 + n) * T, QM),
                                        lambda n: _get(xa_s, g * QM, QM, (7 * n1 + n) * T, T), _NN)
                    for r in range(0, 2 * QD, 32):
                        e, c = r // QD, comb(r, 32)
                        for dq in range(2):
                            row = dq * QD + r % QD
                            done = _outer_step(mq_s[2 * (g % 2) + e], n1, row,
                                               jnp.concatenate([c[dq], c[2 + dq]], axis=1))
                            if done:
                                n, v = done
                                _put(q_i, (2 * e + n // 2) * D + (n % 2) * HD + row, 2 * g * T, [v])

            span = ty + 6000

            u_next = u_s.at[:, pl.ds(jnp.minimum(i + 1, NP - 1) * (TC // 8), TC // 8)]
            carry = _ssm_scan(u_next, carry, lam_s, h_s, clk.pacer(ty, span, TC // 2))

            tie = clk.pacer(ty - 1200, span, 64, [(ty, ty + 1000)])
            rq_i = rq.at[pl.ds((i & 3) * (M // 4), M // 4)]
            sq_i = sq.at[:, _ds((i & 3) * M, M, 8)]
            for c0 in range(0, M // 4, 8):
                _stage(rq_i, sq_i, c0, 8, lambda x, j: tie(x, c0 // 4 + 4 * j), groups=(1,))
            wq_transpose(jnp.minimum(i + 1, NP - 1), lambda x, k: tie(x, 36 + 3 * k))
            for n, (raw, stg, wt_s) in enumerate(((rk, sk, wkt_s), (rv, sv, wvt_s))):
                for c0 in range(0, CS, 8):
                    _stage(raw, stg, c0, 8, lambda x, j: tie(x, 16 * n + c0 // 8 + j))

                @pl.when(i + 1 < NP)
                def _():
                    w_copy(n, i + 1).start()

                raw[CS, 0:8, 0:T] = tie(zero_s[...], 16 * n + 19).astype(bf16)
                cols = _ds(i * CS, CS, CS)
                for pair in range(H // 2):
                    for dt in range(2):
                        blk = stg[(pair // 4) * 2 + dt, pl.ds(pair % 4, CS, stride=4), :]
                        row = pair * D + dt * HD
                        blk = jnp.concatenate([tie(blk[:8], 16 + 24 * n + 3 * pair + dt), blk[8:]], axis=0)
                        wt_s[row:row + HD, cols] = blk.T

            tie = clk.pacer(ty + 1000, span, 28)
            ckv_i = ckv_s.at[i & (NRAW - 1)]
            a_i = a_s.at[_ds(i * (T // 4), T // 4, T // 4)]
            for r in range(0, T // 2, 16):
                def block(o, q):
                    col = (o % 2) * 2 * QC + (q % 2) * QC
                    return ckv_i[2 * (q // 2) + o // 2, r:r + 16, col:col + QC].astype(f32)
                for n1 in range(7):
                    ops = _operands2(_A_TERMS, n1, block, lambda x: tie(x, 7 * (r // 16) + n1))
                    _put(a_i, r, 7 * n1 * QC, ops)
            return carry

        lax.fori_loop(0, NP, phase2, carry0)
        for i in range(NP):
            wo_copy(i).wait()
        prep_w(h, range(NT1), _no_tie)

    @pl.when(h == 0)
    def _():
        prologue(**pro_refs)

    def oproj(jp, clk):
        cols = slice(2 * jp * T, (2 * jp + 2) * T)
        for r, n in OCH:
            c = clk.strassen(lambda i: _get(wl_s, r, n, i * T, T),
                             lambda i: _get(cl_s, 0, HD, (jp * 7 + i) * T, T), _NN)()
            o_s[r:r + n, cols] += jnp.concatenate(c[:2], axis=1)
            o_s[HM + r:HM + r + n, cols] += jnp.concatenate(c[2:], axis=1)

    def head(mk_s, mv_s, mp_s, kt_s, ka_s, va_s, v2_s, s_s, pb_s, pd_s, p2_s, sc_s, qb_s, kd_s):
        clk = _Clock(zero_s)
        q_h = q_s.at[_ds(h * D, D, D)]

        def prep_wo(tie):
            for r in range(0, HM, 16):
                top = tie(wo_s[h, r:r + 16, :].astype(f32), r // 16)
                bot = tie(wo_s[h, HM + r:HM + r + 16, :].astype(f32), r // 16)
                _put(wl_s, r, 0, _operands(_A_TERMS, [top[:, :HD], top[:, HD:], bot[:, :HD], bot[:, HD:]]))

        def proj(g, lo=0, hi=7):
            for n1 in range(lo, hi):
                comb = clk.strassen(lambda n: _get(w_s, 0, 2 * QD, (7 * n1 + n) * QC, QC),
                                    lambda n: _get(a_s, g * T, T, (7 * n1 + n) * QC, QC), _NT, 2, n1 == 6)
                for r, m_s in ((0, mk_s), (QD, mv_s.at[g % 2])):
                    c = comb(r, QD)
                    m_s[n1 * HD:n1 * HD + QD, :] = jnp.concatenate([c[0], c[2]], axis=1)
                    m_s[n1 * HD + QD:(n1 + 1) * HD, :] = jnp.concatenate([c[1], c[3]], axis=1)
            if hi < 7:
                return
            cs = [_combine([mk_s[n * HD + r:n * HD + r + 16, :] for n in range(7)], order=range(7))
                  for r in range(0, HD, 16)]
            for n in range(4):
                kt_s[:, n * T:(n + 1) * T] = jnp.concatenate([c[n] for c in cs], axis=0).T
            for r in range(0, 2 * T, T // 2):
                blk = kt_s[r:r + T // 2, :]
                blk = [blk[:, n * T:(n + 1) * T] for n in range(4)]
                _put(ka_s, 2 * g * T + r, 0, _operands(_A_TERMS, blk) + [blk[2]])
            for r in (0, 32, T, T + 32):
                lo_, hi_ = kt_s[r:r + 32, 0:2 * T], kt_s[r + T // 2:r + T // 2 + 32, 0:2 * T]
                _put(kd_s, r // T * (T // 2) + r % T, 0,
                     _operands(_A_TERMS, [lo_[:, :T], lo_[:, T:], hi_[:, :T], hi_[:, T:]]))

        def vfin(g, tie):
            m_s = mv_s.at[g % 2]
            for r in range(0, QD, 16):
                k, blk = 8 * (r // 16), {}
                late = lambda w: tie(w, k, True, LATE)
                for new, n1 in (((0,), 2), ((1,), 4), ((3,), 6), ((), 0), ((), 3), ((2,), 5), ((), 1)):
                    for o in new:
                        for i, row in enumerate((r, QD + r)):
                            tiles = _Rows([m_s.at[n * HD:(n + 1) * HD] for n in range(7)], row, 16)
                            c, = _combine(tiles, ((o % 2) * 2 + o // 2,), range(7))
                            blk[o, i] = c = tie(c, k)
                            slot = (2, 7, 8, 3)[o]
                            _put(va_s, row, ((2 * g + 1) * 9 + slot) * T, [c[:, T:]])
                            if o in (1, 2):
                                _put(va_s, row, (2 * g * 9 + slot) * T, [c[:, :T]])
                    lo_, hi_ = [_operand(_A_TERMS[n1], lambda o: blk[o, i]) for i in range(2)]
                    _put(va_s, r, (2 * g * 9 + n1) * T, [lo_[:, :T]], late)
                    _put(va_s, QD + r, (2 * g * 9 + n1) * T, [hi_[:, :T]], late)
                    if g < 3:
                        _put(v2_s, r, (g * 7 + n1) * 7 * T,
                             _operands(_A_TERMS, [lo_[:, :T], lo_[:, T:], hi_[:, :T], hi_[:, T:]]), late)
                    k += 8 / 7

        key = lax.broadcasted_iota(jnp.int32, (T, 2 * T), 0)
        qry = lax.broadcasted_iota(jnp.int32, (T, 2 * T), 1)
        causal = key <= qry

        marks = []

        def qk(g):
            pairs = (2 * g, 2 * g + 1)
            mx = {jp: _Reducer(jnp.max, jnp.maximum) for jp in pairs}

            def put(jp, row, v):
                v = v.reshape(v.shape[0] // 8, 8, 2 * T)
                s_s[jp % 4, row // 8:row // 8 + v.shape[0]] = v
                mx[jp].add(v)

            def rect(jp, lo, hi):
                for r in range(lo, hi, T // 2):
                    c = clk.strassen(lambda i: _get(ka_s, r, T // 2, i * T, T),
                                     lambda i: _get(qb_s, 0, HD, ((jp % 2) * 7 + i) * T, T), _NN)()
                    put(jp, r, jnp.concatenate(c[:2], axis=1))
                    put(jp, jp * T + r, jnp.concatenate(c[2:], axis=1))

            for jp in pairs:
                for r in range(0, HD, 32):
                    blk = [_get(q_h, e * D + d * HD + r, 32, jp * T, T).astype(f32) for d in range(2) for e in range(2)]
                    _put(qb_s, r, (jp % 2) * 7 * T, _operands(_B_TERMS, blk))
            for jp in pairs:
                rect(jp, 0, 2 * g * T)
                marks.append(clk.t)
            last = {}
            for jp in pairs:
                ko = jnp.concatenate([_get(ka_s, jp * T, T, n * T, T) for n in (7, 3)], axis=1)
                so = jnp.where(causal[:, :T], clk.dot(ko, _get(q_h, D, D, jp * T, T), _NN), NEG)
                row = (2 * jp + 1) * T // 8
                s_s[jp % 4, row:row + T // 8, :, T:] = so.reshape(T // 8, 8, T)
                last[jp] = jnp.concatenate([jnp.full((1, T), NEG, f32), jnp.max(so, axis=0, keepdims=True)], axis=1)
            rect(2 * g + 1, 2 * g * T, (2 * g + 1) * T)
            for jp in pairs:
                c = clk.strassen(lambda i: _get(kd_s, (jp % 2) * (T // 2), T // 2, i * T, T),
                                 lambda i: _get(qb_s, 0, HD, ((jp % 2) * 7 + i) * T, T), _NN)()
                se = jnp.concatenate([jnp.concatenate(c[:2], axis=1), jnp.concatenate(c[2:], axis=1)], axis=0)
                put(jp, 2 * jp * T, jnp.where(causal, se, NEG))
            return [jnp.broadcast_to(jnp.maximum(mx[jp].result(), last[jp]), (8, 2 * T)) for jp in pairs]

        zs, sums = {}, {}

        def prob(jp, row, z, n=GS, lanes=slice(None)):
            return jnp.exp2(s_s[jp % 4, row // 8:(row + n) // 8, :, lanes] - z[:, lanes])

        def rough(jp, mx, tie):
            zs[jp] = mx
            if jp > 0:
                sm = _Reducer(jnp.sum, jnp.add)
                for k, r in enumerate(range(0, 2 * jp * T, GS * LSUB)):
                    sm.add(prob(jp, r, tie(mx, k)))
                zs[jp] = mx + jnp.log2(jnp.maximum(LSUB * sm.result(), 1.0))
            sums[jp] = _Reducer(jnp.sum, jnp.add)

        def blocks(jp, row, tie, k):
            top, bot = prob(jp, row, tie(zs[jp], k)), prob(jp, jp * T + row, tie(zs[jp], k + 1))
            sums[jp].add(top + bot)
            top, bot = top.reshape(GS, 2 * T), bot.reshape(GS, 2 * T)
            return [top[:, :T], top[:, T:], bot[:, :T], bot[:, T:]]

        def near(jp, tie, k):
            R, z = jp * T, zs[jp]
            if jp % 2:
                for r in range(0, T, GS):
                    _put(pb_s, jp // 2 * T + r, 0, _operands(_B_TERMS, blocks(jp, R - T + r, tie, k)))
                    k += 2
            for r in range(0, T, GS):
                p = prob(jp, 2 * R + r, tie(z, k))
                sums[jp].add(p)
                _put(pd_s, 2 * R + r, 0, [p.reshape(GS, 2 * T)])
                k += 1
            so = _Reducer(jnp.sum, jnp.add)
            for r in range(0, T, 2 * GS):
                p = prob(jp, 2 * R + T + r, tie(z, k), 2 * GS, slice(T, 2 * T))
                so.add(p)
                _put(pd_s, 2 * R + T + r, T, [p.reshape(2 * GS, T)])
                k += 1
            sums[jp].result()
            sums[jp].out = sums[jp].out + jnp.concatenate([jnp.zeros((1, T), f32), so.result()], axis=1)

        p20 = lambda g: g * (g - 1) // 2 * T

        def far(g, tie, k):
            half = {(jp, e): _Reducer(jnp.sum, jnp.add) for jp in (2 * g, 2 * g + 1) for e in range(2)}
            for kg in range(g):
                for r in range(0, T, GS):
                    blk = {}
                    for new, n1 in (((0,), 1), ((1,), 5), ((3,), 2), ((), 0), ((), 4), ((2,), 3), ((), 6)):
                        for o in new:
                            lanes = slice((o % 2) * T, (o % 2 + 1) * T)
                            for jp in (2 * g, 2 * g + 1):
                                z = tie(zs[jp][:, lanes], k)
                                row = (o // 2) * jp * T + 2 * kg * T + r
                                p = [jnp.exp2(s_s[jp % 4, x // 8:(x + GS) // 8, :, lanes] - z) for x in (row, row + T)]
                                half[jp, o % 2].add(p[0] + p[1])
                                blk[o, jp % 2], blk[o, 2 + jp % 2] = [x.reshape(GS, T) for x in p]
                        ops = _operands2(_B_TERMS, n1, lambda o, q: blk[o, q], lambda x: x)
                        _put(p2_s, p20(g) + kg * T + r, 7 * n1 * T, ops, lambda w: tie(w, k, True, LATE))
                        k += 16 / 7
            for jp in (2 * g, 2 * g + 1):
                if g:
                    sums[jp].out = sums[jp].out + jnp.concatenate([half[jp, e].result() for e in range(2)], axis=1)
            for jp in (2 * g, 2 * g + 1):
                cols = slice(2 * jp * T, 2 * (jp + 1) * T)
                sc_s[:, cols] = g_s[:, cols] / sums[jp].result()

        def pv(g):
            pairs = (2 * g, 2 * g + 1)
            va = lambda n, t, r=0, nr=HD: _get(va_s, r, nr, (t * 9 + n) * T, T)
            for n1 in range(7 if g else 0):
                c = clk.strassen(
                    lambda n: _cat([_get(v2_s, 0, QD, (kg * 49 + 7 * n1 + n) * T, T) for kg in range(g)], 1),
                    lambda n: _get(p2_s, p20(g), g * T, (7 * n1 + n) * T, T), _NN, g)()
                mp_s[n1 * HD:n1 * HD + QD, :] = jnp.concatenate(c[:2], axis=1)
                mp_s[n1 * HD + QD:(n1 + 1) * HD, :] = jnp.concatenate(c[2:], axis=1)
            ve = [jnp.concatenate([va(2, jp), va(8, jp)], axis=0) for jp in pairs]
            vo = [jnp.concatenate([va(7, jp), va(3, jp)], axis=0) for jp in pairs]
            ce = clk.level([(ve[jp % 2], _get(pd_s, 2 * jp * T, T, 0, T)) for jp in pairs])
            co = [clk.dot(jnp.concatenate([ve[jp % 2], vo[jp % 2]], axis=1),
                          _get(pd_s, 2 * jp * T, 2 * T, T, T), _NN) for jp in pairs]
            for jp in pairs:
                R, e = jp * T, jp % 2
                ge, go = sc_s[:, 2 * R:2 * R + T], sc_s[:, 2 * R + T:2 * R + 2 * T]
                for r in range(0, HD, 32):
                    c = [ce[e][r:r + 32], co[e][r:r + 32], ce[e][HD + r:HD + r + 32], co[e][HD + r:HD + r + 32]]
                    if g:
                        far_ = _combine([mp_s[n * HD + r:n * HD + r + 32, e * T:(e + 1) * T] for n in range(7)],
                                        order=range(7))
                        c = [x + y for x, y in zip(c, far_)]
                    if e:
                        near_ = clk.strassen(lambda n: va(n, 2 * g, r, 32),
                                             lambda n: _get(pb_s, g * T, T, n * T, T), _NN)()
                        c = [x + y for x, y in zip(c, near_)]
                    ops = _operands(_B_TERMS, [c[0] * ge, c[1] * go, c[2] * ge, c[3] * go])
                    _put(cl_s, r, jp * 7 * T, ops)

        ends = []

        def run(items):
            for item in items.split():
                if item[0] == 'P':
                    pv(int(item[1]))
                    ends.append(clk.t)
                elif item[0] == 'K':
                    proj(int(item[1]))
                else:
                    jp = int(item[1])
                    oproj(jp, clk)

                    @pl.when(h == H - 1)
                    def _():
                        out_copy(jp).start()

        for n1 in range(7):
            if n1 >= NT1:
                prep_w(h, [n1], clk.pacer(clk.t - 896, clk.t - 448, 8))
            proj(0, n1, n1 + 1)
        oproj(NP - 1, clk)
        mx = qk(0)
        for g in range(4):
            t0 = clk.t
            del ends[:]
            run(PLAN[g])
            t1 = clk.t
            nxt = qk(g + 1) if g < 3 else None
            n_rough = [2 * jp * T // (GS * LSUB) for jp in (2 * g, 2 * g + 1)]
            n_near = [(T + T // 2) // GS, (3 * T + T // 2) // GS]
            holes = [(t - 400, t) for t in ends]
            if 0 < g < 3:
                holes.append((marks[-2] - 400, marks[-2] - 100))
            if g < 3:
                vfin(g, clk.pacer(t0, t0 + VW, 32))
                holes += [(t0, t0 + VW), (t1 - 300, t1 + 300)]
            if g == 2:
                vfin(3, clk.pacer(clk.t - SLACK - VW // 2, clk.t - SLACK, 32))
                holes.append((clk.t - SLACK - VW // 2, clk.t))
            tie = clk.pacer(t0, (clk.t if g else t1) - SLACK,
                            sum(n_rough) + sum(n_near) + g * 16 * T // GS, holes)
            rough(2 * g, mx[0], tie)
            near(2 * g, tie, n_rough[0])
            k = n_rough[0] + n_near[0]
            rough(2 * g + 1, mx[1], lambda x, i: tie(x, k + i))
            near(2 * g + 1, tie, k + n_rough[1])
            far(g, tie, k + n_rough[1] + n_near[1])
            if g == 0:
                prep_wo(clk.pacer(t0 + VW, t1 - 300, HM // 16))
            mx = nxt
        t0 = clk.t
        run(PLAN[4])
        prep_w(jnp.minimum(h + 1, H - 1), range(NT1), clk.pacer(t0 - 100, clk.t - 300, 8 * NT1))
        assert len(set(clk.load)) == 1

    head(**head_refs)

    @pl.when(h == H - 1)
    def _():
        oproj(NP - 1, _Clock(zero_s))
        out_copy(NP - 1).start()
        for jp in range(NP):
            out_copy(jp).wait()


@jax.jit
def pallas_gated_mix__compressed_kv_cla__ssm_conv_s5__prompt_kernel(
    A_x: jax.Array,
    A_c_kv: jax.Array,
    A_w_q: jax.Array,
    A_w_uk: jax.Array,
    A_w_uv: jax.Array,
    A_w_o: jax.Array,
    B_x: jax.Array,
    B_Lambda_re: jax.Array,
    B_Lambda_im: jax.Array,
    B_B_re: jax.Array,
    B_B_im: jax.Array,
    B_C_re: jax.Array,
    B_C_im: jax.Array,
    B_log_dt: jax.Array,
    B_Dskip: jax.Array,
    gate_w: jax.Array,
):
    del B_x
    xT = jnp.transpose(A_x[0])
    woT = jnp.transpose(A_w_o, (0, 2, 1))
    ckv = A_c_kv.reshape(4, 4, 2, T // 2, DC)

    hbm = pl.BlockSpec(memory_space=pl.ANY)
    outT = pl.pallas_call(
        _kernel,
        grid=(H,),
        in_specs=[hbm] * 15,
        out_specs=hbm,
        out_shape=jax.ShapeDtypeStruct((M, S), f32),
        scratch_shapes=_SHARED_SCRATCH + list(_PROLOGUE_SCRATCH.values()) + list(_HEAD_SCRATCH.values()),
        compiler_params=pltpu.CompilerParams(
            dimension_semantics=("arbitrary",),
            vmem_limit_bytes=127 * 1024 * 1024,
        ),
    )(xT, B_B_re, B_B_im, B_C_re, B_C_im, B_Lambda_re, B_Lambda_im, B_log_dt,
      B_Dskip, gate_w, woT, ckv, A_w_q, A_w_uk, A_w_uv)
    return jnp.transpose(outT)[None]
```

```python
import bisect

import jax
import jax.numpy as jnp
from jax import lax
import jax.experimental.pallas as pl
import jax.experimental.pallas.tpu as pltpu

S = 2048
M = 448
H = 16
D = 256
DC = 1024
T = 128
NP = S // T // 2
HD = D // 2
HM = M // 2
QD = D // 4
QC = DC // 4
QM = M // 4
PA = 384
PB = M - PA
TA = 512
TC = 256
CS = DC // NP
NRAW = 2
LOG2E = 1.4426950408889634
NEG = -1e30

GS = 16
RCH = 256
LSUB = 4
NT1 = 3
OCH = ((0, 64), (64, 64), (128, 48), (176, 48))
PLAN = ('K1', 'K2', 'K3', 'P1 P0 O2 O3 P2 O0 O1 O4', 'O5 P3 O6')
SLACK, LATE, VW = 200, 40, 900

f32 = jnp.float32
bf16 = jnp.bfloat16
u32 = jnp.uint32

SEM_VEC, SEM_B, SEM_X, SEM_WQ, SEM_C, SEM_SL, SEM_WO, SEM_OUT, SEM_WQ1, SEM_KV = 0, 1, 2, 6, 7, 8, 16, 17, 18, 22
NSEM = 24

_NN = ((1,), (0,))
_NT = ((1,), (1,))
_TT = ((0,), (1,))


def _cat(xs, axis):
    return xs[0] if len(xs) == 1 else jnp.concatenate(xs, axis=axis)


def _ds(lo, n, align):
    return pl.ds(lo if isinstance(lo, int) else pl.multiple_of(lo, align), n)


def _put(ref, row, col, xs, tie=None):
    x = _cat(xs, 1)
    if tie is not None:
        x = jnp.concatenate([tie(x[:8]), x[8:]], axis=0)
    ref[row // 2:(row + x.shape[0]) // 2, col:col + x.shape[1]] = pltpu.bitcast(x.astype(bf16), u32)


def _get(ref, row, nrows, col, ncols):
    return pltpu.bitcast(ref[row // 2:(row + nrows) // 2, col:col + ncols], bf16)


class _Clock:
    def __init__(self, zero_ref):
        self.masks = {(8, T): zero_ref[...] != 0.0}
        self.ticks, self.load = [], [0, 0, 0, 0]

    @property
    def t(self):
        return max(self.load)

    def dot(self, a, b, dims):
        v = lax.dot_general(a, b, (dims, ((), ())), preferred_element_type=f32)
        rows, depth = v.shape[0], a.shape[dims[0][0]]
        for c in range(0, v.shape[1], T):
            start = 0
            for _ in range(0, depth, T):
                k = self.load.index(min(self.load))
                start = max(start, self.load[k])
                self.load[k] += rows
            self.ticks += [(start + r + 8, (v, r, c)) for r in range(0, rows, 8)]
        return v

    def strassen(self, lhs, rhs, dims, jobs=1, split_last=False):
        lag = sum(l + 32 <= max(self.load) for l in self.load) // jobs if jobs < 3 else 0
        order = ((1, 3, 2, 4, 0, 5, 6), (0, 1, 3, 2, 4, 5, 6), (5, 6, 1, 3, 2, 4, 0), (0, 5, 6, 1, 3, 2, 4))[lag]
        m = {}
        for n in order:
            a, b = lhs(n), rhs(n)
            if split_last and n == order[-1]:
                half = a.shape[0] // 2
                m[n] = jnp.concatenate([self.dot(a[:half], b, dims), self.dot(a[half:], b, dims)], axis=0)
            else:
                m[n] = self.dot(a, b, dims)
        return lambda r=0, n=None: _combine(m if n is None else _Rows(m, r, n), order=order)

    def level(self, pairs, dims=_NN):
        base, extra = divmod((sum(self.load) + sum(a.shape[0] for a, _ in pairs)) // 16, 4)
        target = [16 * (base + (k < extra)) for k in range(4)]
        out = []
        for a, b in pairs:
            r, parts = 0, []
            while r < a.shape[0]:
                k = self.load.index(min(self.load))
                n = min(max(target[k] - self.load[k], 16), a.shape[0] - r)
                parts.append(self.dot(a[r:r + n], b, dims))
                r += n
            out.append(_cat(parts, 0))
        return out

    def pacer(self, t0, t1, n, holes=()):
        holes = sorted((max(a, t0), min(b, t1)) for a, b in holes if a < t1 and b > t0)
        gap = sum(b - a for a, b in holes)
        ticks = sorted(self.ticks, key=lambda tw: tw[0])
        times = [tw[0] for tw in ticks]

        def tie(x, k, distinct=False, delay=0):
            t = t0 + (t1 - t0 - gap) * k / n
            for a, b in holes:
                t += b - a if t > a else 0
            t += delay
            past = ticks[:bisect.bisect_right(times, t)]
            reps = (x.shape[0] // 8, x.shape[1] // T)
            if len(past) < (reps[1] if distinct else 1):
                return x
            tick = _cat([v[r:r + 8, c:c + T] for _, (v, r, c) in past[-reps[1] if distinct else -1:]], 1)
            if tick.dtype != x.dtype:
                tick = pltpu.bitcast(tick, x.dtype)
            if x.shape not in self.masks:
                self.masks[x.shape] = jnp.tile(self.masks[(8, T)], reps)
            return lax.select(self.masks[x.shape], tick if tick.shape == x.shape else jnp.tile(tick, reps), x)
        return tie


def _no_tie(x, k):
    return x


_A_TERMS = ((0, 3, 1), (2, 3, 1), (0, None, 0), (3, None, 0), (0, 1, 1), (2, 0, -1), (1, 3, -1))
_B_TERMS = ((0, 3, 1), (0, None, 0), (1, 3, -1), (2, 0, -1), (3, None, 0), (0, 1, 1), (2, 3, 1))


def _operand(term, block):
    x, y, sign = term
    if y is None:
        return block(x)
    return block(x) + block(y) if sign > 0 else block(x) - block(y)


def _operands(terms, blocks):
    return [_operand(t, blocks.__getitem__) for t in terms]


def _operands2(terms, n1, block, tie):
    first = terms[n1][0]
    sub = [_operand(terms[n1], lambda o: tie(block(o, q)) if o == first and q in (0, 3) else block(o, q))
           for q in range(4)]
    return _operands(terms, sub)


_C_TERMS = ({0: 1, 3: 1, 4: -1, 6: 1}, {2: 1, 4: 1}, {1: 1, 3: 1}, {0: 1, 1: -1, 2: 1, 5: 1})


def _combine(m, only=(0, 1, 2, 3), order=(1, 3, 2, 4, 0, 5, 6)):
    out = []
    for terms in (_C_TERMS[n] for n in only):
        seq = [n for n in order if n in terms]
        if terms[seq[0]] < 0:
            seq[0], seq[1] = seq[1], seq[0]
        acc = m[seq[0]]
        for n in seq[1:]:
            acc = acc + m[n] if terms[n] > 0 else acc - m[n]
        out.append(acc)
    return out


def _outer_step(m_s, n1, row, v):
    n = v.shape[0]
    if n1 < 5:
        m_s[n1 * HD + row:n1 * HD + row + n, :] = v
    if n1 < 3:
        return None
    blk = (2, 1, 3, 0)[n1 - 3]
    m = {j: v if j == n1 else m_s[j * HD + row:j * HD + row + n, :] for j in _C_TERMS[blk]}
    return blk, _combine(m, (blk,), range(7))[0]


class _Rows:
    def __init__(self, vals, r, n):
        self.vals, self.rows, self.cache = vals, slice(r, r + n), {}

    def __getitem__(self, i):
        if i not in self.cache:
            self.cache[i] = self.vals[i][self.rows, :]
        return self.cache[i]


class _Reducer:
    def __init__(self, red, comb):
        self.red, self.comb, self.acc, self.rows, self.out = red, comb, None, 0, None

    def add(self, v):
        self.rows += 8 * v.shape[0]
        v = self.red(v, axis=0)
        self.acc = v if self.acc is None else self.comb(self.acc, v)
        if self.rows >= RCH:
            self.result()

    def result(self):
        if self.acc is not None:
            v = self.red(self.acc, axis=0, keepdims=True)
            self.out = v if self.out is None else self.comb(self.out, v)
        self.acc, self.rows = None, 0
        return self.out


def _cmul(ar, ai, br, bi):
    return ar * br - ai * bi, ar * bi + ai * br


def _hi16(w):
    return pltpu.bitcast(w & jnp.uint32(0xFFFF0000), f32)


def _stage(raw, stg, c0, nc, tie, groups=(0, 1)):
    for ht in groups:
        for dt in range(2):
            v = raw[c0:c0 + nc, ht * 8:(ht + 1) * 8, dt * T:(dt + 1) * T].reshape(nc * 8, T)
            stg[ht * 2 + dt, c0 * 4:(c0 + nc) * 4, :] = tie(pltpu.bitcast(v, u32), (ht * 2 + dt) / 4)


def _ssm_params(vec_s, coef_s, lam_s, col_s):
    row = lambda r: r[...].astype(f32).reshape(1, M)
    lre, lim, ldt, dsk, gw = [row(v) for v in vec_s]
    dt = jnp.exp(ldt).astype(bf16).astype(f32)
    mag = jnp.exp(dt * lre)
    ang = dt * lim
    lr, li = mag * jnp.cos(ang), mag * jnp.sin(ang)
    den = lre * lre + lim * lim
    nr = lr - 1.0
    coef_s[...] = jnp.zeros(coef_s.shape, f32)
    coef_s[0:1, 0:M] = 2.0 * ((nr * lre + li * lim) / den)
    coef_s[1:2, 0:M] = 2.0 * ((li * lre - nr * lim) / den)

    er = jnp.concatenate([lr, lr[:, PA:]], axis=1)
    ei = jnp.concatenate([li, -li[:, PA:]], axis=1)
    pw = [(er, ei)]
    for _ in range(7):
        pw.append(_cmul(pw[-1][0], pw[-1][1], er, ei))
    sub = lax.broadcasted_iota(jnp.int32, (8, 512), 0)
    for n, d in enumerate((1, 2, 4)):
        lam_s[2 * n] = jnp.where(sub >= d, pw[d - 1][0], 0.0)
        lam_s[2 * n + 1] = jnp.where(sub >= d, pw[d - 1][1], 0.0)
    lcr = jnp.zeros((8, 512), f32)
    lci = jnp.zeros((8, 512), f32)
    for r in range(8):
        lcr = jnp.where(sub == r, pw[r][0], lcr)
        lci = jnp.where(sub == r, pw[r][1], lci)
    lam_s[6] = lcr
    lam_s[7] = lci

    def col(v):
        v = jnp.concatenate([v, jnp.zeros((1, 512 - M), f32)], axis=1)
        return jnp.broadcast_to(v, (T, 512)).T[:M]
    col_s[0] = col(dsk)
    col_s[1] = col(gw)


def _ssm_cmat(craw_s, coef_s, c_s, tie):
    for r in range(0, HM, 16):
        for c in range(0, M, T):
            w = min(T, M - c)
            coef = tie(coef_s[:, c:c + T], r // 16 + c / 512)
            cr, ci = coef[0:1, :w], coef[1:2, :w]
            blk = []
            for row in (r, HM + r):
                re, im = _cmul(craw_s[0, row:row + 16, c:c + w].astype(f32),
                               craw_s[1, row:row + 16, c:c + w].astype(f32), cr, ci)
                blk += [re, -im]
            if c < PA:
                for n, op in enumerate(_operands(_A_TERMS, blk)):
                    _put(c_s, r, n * PA + c, [op])
            else:
                _put(c_s, r, 7 * PA, blk)


def _ssm_scan(u_ref, carry, lam_s, h_s, h0_s, tie):
    car, cai = carry
    out = []
    for b in range(TC // 8):
        mixed = u_ref[3, b, :, 0:T]
        u = jnp.concatenate([u_ref[cb, b] for cb in range(3)], axis=1)
        cols = [u[:, 0:T], u[:, T:2 * T], u[:, 2 * T:PA], mixed]
        hr = jnp.concatenate([tie(v, 4 * b + n) for n, v in enumerate(cols)], axis=1)
        hi = jnp.concatenate([u[:, PA:2 * PA], pltpu.roll(mixed, PB, 1)], axis=1)
        for n, d in enumerate((1, 2, 4)):
            sr, si = pltpu.roll(hr, d, 0), pltpu.roll(hi, d, 0)
            tr, ti = _cmul(sr, si, lam_s[2 * n], lam_s[2 * n + 1])
            hr, hi = hr + tr, hi + ti
        tr, ti = _cmul(lam_s[6], lam_s[7], car, cai)
        hr, hi = hr + tr, hi + ti
        car, cai = hr[7:8, :], hi[7:8, :]
        out.append(jnp.concatenate([hr[:, :PA], hi[:, :PA], hr[:, PA:]], axis=1))
        if b % 2 == 1:
            v, row = jnp.concatenate(out, axis=0), (b - 1) * 8 % T
            _put(h_s, row, 7 * PA + b // 16 * T, [v[:, 2 * PA:]])
            if b < 16:
                h0_s[row:row + 16, :] = v[:, :2 * PA]
            else:
                v0 = h0_s[row:row + 16, :]
                _put(h_s, row, 0, _operands(_B_TERMS, [v0[:, :PA], v[:, :PA], v0[:, PA:], v[:, PA:2 * PA]]))
            out = []
    return car, cai


_vmem = pltpu.VMEM
_PROLOGUE_SCRATCH = dict(
    xT_s=_vmem((M, S), bf16),
    v0=_vmem((M,), bf16), v1=_vmem((M,), bf16), v2=_vmem((M,), bf16), v3=_vmem((M,), bf16), v4=_vmem((M,), bf16),
    b_s=_vmem((2 * M, M), bf16),
    craw_s=_vmem((2, M, M), bf16),
    c_s=_vmem((HM // 2, 7 * PA + 2 * T), u32),
    coef_s=_vmem((8, 512), f32),
    lam_s=_vmem((8, 8, 512), f32),
    col_s=_vmem((2, M, T), f32),
    h_s=_vmem((T // 2, 7 * PA + 2 * T), u32),
    h0_s=_vmem((T, 2 * PA), f32),
    ckv_s=_vmem((NRAW, 4, T // 2, DC), bf16),
    rq=_vmem((M, H, D), bf16),
    rk=_vmem((CS + 1, H, D), bf16),
    rv=_vmem((CS + 1, H, D), bf16),
    sq=_vmem((4, M * 4, T), u32),
    sk=_vmem((4, CS * 4, T), u32),
    sv=_vmem((4, CS * 4, T), u32),
    wqt_s=_vmem((D, 4 * T), u32),
)
_HEAD_SCRATCH = dict(
    mk_s=_vmem((7 * HD, 2 * T), f32),
    mv_s=_vmem((2, 7 * HD, 2 * T), f32),
    mp_s=_vmem((7 * HD, 2 * T), f32),
    kt_s=_vmem((2 * T, 4 * T), f32),
    ka_s=_vmem((S // 4, 8 * T), u32),
    va_s=_vmem((HD // 2, NP * 9 * T), u32),
    v2_s=_vmem((QD // 2, 3 * 49 * T), u32),
    s_s=_vmem((4, S // 8, 8, 2 * T), f32),
    pb_s=_vmem((2 * T, 7 * T), u32),
    pd_s=_vmem((S // 2, 2 * T), u32),
    p2_s=_vmem((3 * T, 49 * T), u32),
    sc_s=_vmem((1, S), f32),
    qb_s=_vmem((HD // 2, 14 * T), u32),
    kd_s=_vmem((T // 2, 7 * T), u32),
)
_SHARED_SCRATCH = [
    _vmem((H // 2 * D, DC), u32),
    _vmem((H // 2 * D, DC), u32),
    _vmem((S // 8, 49 * QC), u32),
    _vmem((H * D, S // 2), u32),
    _vmem((H, M, D), bf16),
    _vmem((QD, 49 * QC), u32),
    _vmem((HM // 2, 7 * T), u32),
    _vmem((HD // 2, NP * 7 * T), u32),
    _vmem((M, S), f32),
    _vmem((1, S), f32),
    _vmem((8, T), f32),
    pltpu.SemaphoreType.DMA((NSEM,)),
]


def _kernel(xT_hbm, bre_hbm, bim_hbm, cre_hbm, cim_hbm, lre_hbm, lim_hbm, ldt_hbm,
            dsk_hbm, gw_hbm, woT_hbm, ckv_hbm, wq_hbm, wk_hbm, wv_hbm,
            out_hbm,
            wkt_s, wvt_s, a_s, q_s, wo_s, w_s, wl_s, cl_s, o_s, g_s, zero_s, sem, *rest):
    h = pl.program_id(0)
    pro_refs = dict(zip(_PROLOGUE_SCRATCH, rest))
    head_refs = dict(zip(_HEAD_SCRATCH, rest[len(pro_refs):]))

    def out_copy(jp):
        cols = pl.ds(jp * 2 * T, 2 * T)
        return pltpu.make_async_copy(o_s.at[:, cols], out_hbm.at[:, cols], sem.at[SEM_OUT])

    def prep_w(hh, outer, tie):
        rows = _ds(lax.shift_right_logical(hh, 1) * D, D, D)
        sh = (16 * (1 - (hh & 1))).astype(u32)
        k = 0
        for row0, wt_s in ((0, wkt_s.at[rows]), (QD, wvt_s.at[rows])):
            for r in range(0, QD, 16):
                def block(o, q):
                    row = (o % 2) * HD + (q % 2) * QD + r
                    col = (o // 2) * 2 * QC + (q // 2) * QC
                    return _hi16(wt_s[row:row + 16, col:col + QC] << sh)
                for n1 in outer:
                    _put(w_s, row0 + r, 7 * n1 * QC, _operands2(_B_TERMS, n1, block, lambda x: tie(x, k)))
                    k += 1

    def prologue(xT_s, v0, v1, v2, v3, v4, b_s, craw_s, c_s, coef_s, lam_s, col_s, h_s, h0_s,
                 ckv_s, rq, rk, rv, sq, sk, sv, wqt_s):
        xa_s = head_refs['p2_s']
        wq_s = xa_s.at[2 * QM:2 * QM + QD]
        u_s = head_refs['s_s']
        vec_s = (v0, v1, v2, v3, v4)

        def slice_copies(i):
            s = sem.at[SEM_SL + i]
            grp = i // 2 if isinstance(i, int) else lax.shift_right_logical(i, 1)
            return [pltpu.make_async_copy(ckv_hbm.at[grp, :, i & 1], ckv_s.at[i & (NRAW - 1)], s)]

        def w_copy(n, i):
            src, dst = ((wk_hbm, rk), (wv_hbm, rv))[n]
            return pltpu.make_async_copy(src.at[pl.ds(i * CS, CS)], dst.at[0:CS], sem.at[SEM_KV + n])

        def wo_copy(i):
            heads = pl.ds(2 * i, 2)
            return pltpu.make_async_copy(woT_hbm.at[heads], wo_s.at[heads], sem.at[SEM_WO])

        def wq1_copy(i):
            rows = pl.ds(i * (M // 4), M // 4)
            return pltpu.make_async_copy(wq_hbm.at[rows, 8:16], rq.at[rows, 8:16], sem.at[SEM_WQ1 + i])

        def x_copy(i):
            cols = pl.ds(i * TA, TA)
            return pltpu.make_async_copy(xT_hbm.at[:, cols], xT_s.at[:, cols], sem.at[SEM_X + i])

        cp_vec = [pltpu.make_async_copy(src, dst, sem.at[SEM_VEC])
                  for src, dst in zip((lre_hbm, lim_hbm, ldt_hbm, dsk_hbm, gw_hbm), vec_s)]
        cp_b = [pltpu.make_async_copy(src.at[pl.ds(lo, n)], b_s.at[pl.ds(dst, n)], sem.at[SEM_B])
                for src, lo, n, dst in ((bre_hbm, 0, PA, 0), (bim_hbm, 0, PA, PA),
                                        (bre_hbm, PA, PB, 2 * PA), (bim_hbm, PA, PB, 2 * PA + PB))]
        cp_wq = [pltpu.make_async_copy(wq_hbm.at[:, 0:8], rq.at[:, 0:8], sem.at[SEM_WQ])]
        cp_c = [pltpu.make_async_copy(src, craw_s.at[n], sem.at[SEM_C])
                for n, src in enumerate((cre_hbm, cim_hbm))]
        for cp in cp_vec + cp_b + [x_copy(i) for i in range(S // TA)] + cp_c + cp_wq:
            cp.start()
        for cp in [wq1_copy(0)] + slice_copies(0) + [w_copy(0, 0), w_copy(1, 0)]:
            cp.start()

        zero_s[...] = jnp.zeros(zero_s.shape, f32)
        wl_s[...] = jnp.zeros(wl_s.shape, u32)
        cl_s[:, (NP - 1) * 7 * T:] = jnp.zeros((HD // 2, 7 * T), u32)
        for cp in cp_vec:
            cp.wait()
        _ssm_params(vec_s, coef_s, lam_s, col_s)

        def wq_transpose(pair, tie):
            ht = pair // 4 if isinstance(pair, int) else lax.shift_right_logical(pair, 2)
            pad = jnp.zeros((T - QM, T), u32)
            for dt in range(2):
                for mq in range(4):
                    blk = sq[ht * 2 + dt, pl.ds(mq * QM * 4 + (pair & 3), QM, stride=4), :]
                    blk = jnp.concatenate([tie(blk[:8], 4 * dt + mq), blk[8:], pad], axis=0)
                    wqt_s[dt * HD:(dt + 1) * HD, mq * T:(mq + 1) * T] = blk.T

        def phase1(i, gates):
            clk = _Clock(zero_s)
            u = _cat([clk.dot(xT_s[:, i * TA + lo:i * TA + hi], b_s[...], _TT)
                      for lo, hi in ((0, T), (T, TA))], 0)
            for cb in range(4):
                w = min(2 * T, 2 * M - cb * 2 * T)
                u_s[cb, i * TA // 8:(i + 1) * TA // 8, :, 0:w] = (
                    u[:, cb * 2 * T:cb * 2 * T + w].reshape(TA // 8, 8, w))
            tie = clk.pacer(0, 6 * TA, 49)
            for r in range(0, QM, 16):
                def block(o, q):
                    row, col = (o % 2) * HM + (q % 2) * QM + r, (4 * i + 2 * (q // 2) + o // 2) * T
                    return xT_s[row:row + 16, col:col + T].astype(f32) * (LOG2E * D ** -0.5)
                for n1 in range(7):
                    ops = _operands2(_A_TERMS, n1, block, lambda x: tie(x, 7 * (r // 16) + n1))
                    _put(xa_s, i * QM + r, 7 * n1 * T, ops)
            tie = clk.pacer(0, 6 * TA, 28 * len(gates))
            for t, tile in enumerate(gates):
                cols = slice(tile * T, (tile + 1) * T)
                acc = jnp.zeros((8, T), f32)
                for r in range(0, M, 32):
                    xg = xT_s[r:r + 32, cols].astype(f32) * tie(col_s[1, r:r + 32, :], 28 * t + r // 32)
                    acc = acc + jnp.sum(xg.reshape(4, 8, T), axis=0)
                g = jax.nn.sigmoid(jnp.sum(acc, axis=0, keepdims=True))
                g_s[:, cols] = g
                for r in range(0, M, 32):
                    skip = xT_s[r:r + 32, cols].astype(f32) * tie(col_s[0, r:r + 32, :], 28 * t + 14 + r // 32)
                    o_s[r:r + 32, cols] = (1.0 - g) * skip
            return clk

        for cp in cp_b + [x_copy(0)]:
            cp.wait()
        phase1(0, range(4))
        x_copy(1).wait()
        clk = phase1(1, range(4, 6))
        zero = jnp.zeros((1, 512), f32)
        carry0 = _ssm_scan(u_s.at[:, 0:TC // 8], (zero, zero), lam_s, h_s, h0_s, clk.pacer(0, 6 * TA, TC // 2))
        for cp in [x_copy(2), x_copy(3)] + cp_c + cp_wq:
            cp.wait()
        _ssm_cmat(craw_s, coef_s, c_s, phase1(2, range(6, 9)).pacer(0, 6 * TA, HM // 16))
        tie = phase1(3, range(9, 16)).pacer(0, 6 * TA, M // 8)
        for c0 in range(0, M, 8):
            _stage(rq, sq, c0, 8, lambda x, j: tie(x, c0 / 10 + j), groups=(0,))
        wq_transpose(0, lambda x, k: tie(x, 46 + k))

        def phase2(i, carry):
            @pl.when(i + 1 < NP)
            def _():
                for cp in slice_copies(i + 1):
                    cp.start()

            @pl.when(i < 3)
            def _():
                wq1_copy(i + 1).start()

            wo_copy(i).start()

            @pl.when(i < 4)
            def _():
                wq1_copy(i).wait()

            for cp in slice_copies(i) + [w_copy(0, i), w_copy(1, i)]:
                cp.wait()

            clk = _Clock(zero_s)
            comb = clk.strassen(lambda n: _get(c_s, 0, HM, n * PA, PA), lambda n: _get(h_s, 0, T, n * PA, PA), _NT, 3)
            mixed = clk.level([(_get(c_s, 0, HM, 7 * PA + n // 2 * T, T), _get(h_s, 0, T, 7 * PA + n % 2 * T, T))
                               for n in range(4)], _NT)
            ty = clk.t
            cols = _ds(i * TC, TC, TC)
            keep = 1.0 - g_s[:, cols]
            for r in range(0, HM, 32):
                y = [c + m[r:r + 32] for c, m in zip(comb(r, 32), mixed)]
                o_s[r:r + 32, cols] += keep * jnp.concatenate(y[:2], axis=1)
                o_s[HM + r:HM + r + 32, cols] += keep * jnp.concatenate(y[2:], axis=1)

            q_i = q_s.at[_ds(i * 2 * D, 2 * D, 2 * D)]
            mq_s = (head_refs['mk_s'], head_refs['mp_s'], head_refs['mv_s'].at[0], head_refs['mv_s'].at[1])
            for g in range(4):
                for n1 in range(7):
                    if g == 0:
                        t = 200 + (ty + 644) * n1 / 7
                        tie = clk.pacer(min(t, clk.t - 500), min(t + 300, clk.t - 500), 8)
                        for r in range(0, 2 * QD, 16):
                            def block(o, q):
                                row = (o % 2) * HD + (q % 2) * QD + r % QD
                                col = (2 * (o // 2) + q // 2) * T
                                w = wqt_s[row:row + 16, col:col + T]
                                return _hi16(w) if r >= QD else pltpu.bitcast(w << 16, f32)
                            _put(wq_s, r, 7 * n1 * T, _operands2(_B_TERMS, n1, block, lambda x: tie(x, r // 16)))
                    comb = clk.strassen(lambda n: _get(wq_s, 0, 2 * QD, (7 * n1 + n) * T, QM),
                                        lambda n: _get(xa_s, g * QM, QM, (7 * n1 + n) * T, T), _NN)
                    for r in range(0, 2 * QD, 32):
                        e, c = r // QD, comb(r, 32)
                        for dq in range(2):
                            row = dq * QD + r % QD
                            done = _outer_step(mq_s[2 * (g % 2) + e], n1, row,
                                               jnp.concatenate([c[dq], c[2 + dq]], axis=1))
                            if done:
                                n, v = done
                                _put(q_i, (2 * e + n // 2) * D + (n % 2) * HD + row, 2 * g * T, [v])

            span = ty + 6000

            u_next = u_s.at[:, pl.ds(jnp.minimum(i + 1, NP - 1) * (TC // 8), TC // 8)]
            carry = _ssm_scan(u_next, carry, lam_s, h_s, h0_s, clk.pacer(ty, span, TC // 2))

            tie = clk.pacer(ty - 1200, span, 64, [(ty, ty + 1000)])
            rq_i = rq.at[pl.ds((i & 3) * (M // 4), M // 4)]
            sq_i = sq.at[:, _ds((i & 3) * M, M, 8)]
            for c0 in range(0, M // 4, 8):
                _stage(rq_i, sq_i, c0, 8, lambda x, j: tie(x, c0 // 4 + 4 * j), groups=(1,))
            wq_transpose(jnp.minimum(i + 1, NP - 1), lambda x, k: tie(x, 36 + 3 * k))
            for n, (raw, stg, wt_s) in enumerate(((rk, sk, wkt_s), (rv, sv, wvt_s))):
                for c0 in range(0, CS, 8):
                    _stage(raw, stg, c0, 8, lambda x, j: tie(x, 16 * n + c0 // 8 + j))

                @pl.when(i + 1 < NP)
                def _():
                    w_copy(n, i + 1).start()

                raw[CS, 0:8, 0:T] = tie(zero_s[...], 16 * n + 19).astype(bf16)
                cols = _ds(i * CS, CS, CS)
                for pair in range(H // 2):
                    for dt in range(2):
                        blk = stg[(pair // 4) * 2 + dt, pl.ds(pair % 4, CS, stride=4), :]
                        row = pair * D + dt * HD
                        blk = jnp.concatenate([tie(blk[:8], 16 + 24 * n + 3 * pair + dt), blk[8:]], axis=0)
                        wt_s[row:row + HD, cols] = blk.T

            tie = clk.pacer(ty + 1000, span, 28)
            ckv_i = ckv_s.at[i & (NRAW - 1)]
            a_i = a_s.at[_ds(i * (T // 4), T // 4, T // 4)]
            for r in range(0, T // 2, 16):
                def block(o, q):
                    col = (o % 2) * 2 * QC + (q % 2) * QC
                    return ckv_i[2 * (q // 2) + o // 2, r:r + 16, col:col + QC].astype(f32)
                for n1 in range(7):
                    ops = _operands2(_A_TERMS, n1, block, lambda x: tie(x, 7 * (r // 16) + n1))
                    _put(a_i, r, 7 * n1 * QC, ops)
            return carry

        lax.fori_loop(0, NP, phase2, carry0)
        for i in range(NP):
            wo_copy(i).wait()
        prep_w(h, range(NT1), _no_tie)

    @pl.when(h == 0)
    def _():
        prologue(**pro_refs)

    def oproj(jp, clk):
        cols = slice(2 * jp * T, (2 * jp + 2) * T)
        for r, n in OCH:
            c = clk.strassen(lambda i: _get(wl_s, r, n, i * T, T),
                             lambda i: _get(cl_s, 0, HD, (jp * 7 + i) * T, T), _NN)()
            o_s[r:r + n, cols] += jnp.concatenate(c[:2], axis=1)
            o_s[HM + r:HM + r + n, cols] += jnp.concatenate(c[2:], axis=1)

    def head(mk_s, mv_s, mp_s, kt_s, ka_s, va_s, v2_s, s_s, pb_s, pd_s, p2_s, sc_s, qb_s, kd_s):
        clk = _Clock(zero_s)
        q_h = q_s.at[_ds(h * D, D, D)]

        def prep_wo(tie):
            for r in range(0, HM, 16):
                top = tie(wo_s[h, r:r + 16, :].astype(f32), r // 16)
                bot = tie(wo_s[h, HM + r:HM + r + 16, :].astype(f32), r // 16)
                _put(wl_s, r, 0, _operands(_A_TERMS, [top[:, :HD], top[:, HD:], bot[:, :HD], bot[:, HD:]]))

        def proj(g, lo=0, hi=7):
            for n1 in range(lo, hi):
                comb = clk.strassen(lambda n: _get(w_s, 0, 2 * QD, (7 * n1 + n) * QC, QC),
                                    lambda n: _get(a_s, g * T, T, (7 * n1 + n) * QC, QC), _NT, 2, n1 == 6)
                for r, m_s in ((0, mk_s), (QD, mv_s.at[g % 2])):
                    c = comb(r, QD)
                    m_s[n1 * HD:n1 * HD + QD, :] = jnp.concatenate([c[0], c[2]], axis=1)
                    m_s[n1 * HD + QD:(n1 + 1) * HD, :] = jnp.concatenate([c[1], c[3]], axis=1)
            if hi < 7:
                return
            cs = [_combine([mk_s[n * HD + r:n * HD + r + 16, :] for n in range(7)], order=range(7))
                  for r in range(0, HD, 16)]
            for n in range(4):
                kt_s[:, n * T:(n + 1) * T] = jnp.concatenate([c[n] for c in cs], axis=0).T
            for r in range(0, 2 * T, T // 2):
                blk = kt_s[r:r + T // 2, :]
                blk = [blk[:, n * T:(n + 1) * T] for n in range(4)]
                _put(ka_s, 2 * g * T + r, 0, _operands(_A_TERMS, blk) + [blk[2]])
            for r in (0, 32, T, T + 32):
                lo_, hi_ = kt_s[r:r + 32, 0:2 * T], kt_s[r + T // 2:r + T // 2 + 32, 0:2 * T]
                _put(kd_s, r // T * (T // 2) + r % T, 0,
                     _operands(_A_TERMS, [lo_[:, :T], lo_[:, T:], hi_[:, :T], hi_[:, T:]]))

        def vfin(g, tie):
            m_s = mv_s.at[g % 2]
            for r in range(0, QD, 16):
                k, blk = 8 * (r // 16), {}
                late = lambda w: tie(w, k, True, LATE)
                for new, n1 in (((0,), 2), ((1,), 4), ((3,), 6), ((), 0), ((), 3), ((2,), 5), ((), 1)):
                    for o in new:
                        for i, row in enumerate((r, QD + r)):
                            tiles = _Rows([m_s.at[n * HD:(n + 1) * HD] for n in range(7)], row, 16)
                            c, = _combine(tiles, ((o % 2) * 2 + o // 2,), range(7))
                            blk[o, i] = c = tie(c, k)
                            slot = (2, 7, 8, 3)[o]
                            _put(va_s, row, ((2 * g + 1) * 9 + slot) * T, [c[:, T:]])
                            if o in (1, 2):
                                _put(va_s, row, (2 * g * 9 + slot) * T, [c[:, :T]])
                    lo_, hi_ = [_operand(_A_TERMS[n1], lambda o: blk[o, i]) for i in range(2)]
                    _put(va_s, r, (2 * g * 9 + n1) * T, [lo_[:, :T]], late)
                    _put(va_s, QD + r, (2 * g * 9 + n1) * T, [hi_[:, :T]], late)
                    if g < 3:
                        _put(v2_s, r, (g * 7 + n1) * 7 * T,
                             _operands(_A_TERMS, [lo_[:, :T], lo_[:, T:], hi_[:, :T], hi_[:, T:]]), late)
                    k += 8 / 7

        key = lax.broadcasted_iota(jnp.int32, (T, 2 * T), 0)
        qry = lax.broadcasted_iota(jnp.int32, (T, 2 * T), 1)
        causal = key <= qry

        marks = []

        def qk(g):
            pairs = (2 * g, 2 * g + 1)
            mx = {jp: _Reducer(jnp.max, jnp.maximum) for jp in pairs}

            def put(jp, row, v):
                v = v.reshape(v.shape[0] // 8, 8, 2 * T)
                s_s[jp % 4, row // 8:row // 8 + v.shape[0]] = v
                mx[jp].add(v)

            def rect(jp, lo, hi):
                for r in range(lo, hi, T // 2):
                    c = clk.strassen(lambda i: _get(ka_s, r, T // 2, i * T, T),
                                     lambda i: _get(qb_s, 0, HD, ((jp % 2) * 7 + i) * T, T), _NN)()
                    put(jp, r, jnp.concatenate(c[:2], axis=1))
                    put(jp, jp * T + r, jnp.concatenate(c[2:], axis=1))

            for jp in pairs:
                for r in range(0, HD, 32):
                    blk = [_get(q_h, e * D + d * HD + r, 32, jp * T, T).astype(f32) for d in range(2) for e in range(2)]
                    _put(qb_s, r, (jp % 2) * 7 * T, _operands(_B_TERMS, blk))
            for jp in pairs:
                rect(jp, 0, 2 * g * T)
                marks.append(clk.t)
            last = {}
            for jp in pairs:
                ko = jnp.concatenate([_get(ka_s, jp * T, T, n * T, T) for n in (7, 3)], axis=1)
                so = jnp.where(causal[:, :T], clk.dot(ko, _get(q_h, D, D, jp * T, T), _NN), NEG)
                row = (2 * jp + 1) * T // 8
                s_s[jp % 4, row:row + T // 8, :, T:] = so.reshape(T // 8, 8, T)
                last[jp] = jnp.concatenate([jnp.full((1, T), NEG, f32), jnp.max(so, axis=0, keepdims=True)], axis=1)
            rect(2 * g + 1, 2 * g * T, (2 * g + 1) * T)
            for jp in pairs:
                c = clk.strassen(lambda i: _get(kd_s, (jp % 2) * (T // 2), T // 2, i * T, T),
                                 lambda i: _get(qb_s, 0, HD, ((jp % 2) * 7 + i) * T, T), _NN)()
                se = jnp.concatenate([jnp.concatenate(c[:2], axis=1), jnp.concatenate(c[2:], axis=1)], axis=0)
                put(jp, 2 * jp * T, jnp.where(causal, se, NEG))
            return [jnp.broadcast_to(jnp.maximum(mx[jp].result(), last[jp]), (8, 2 * T)) for jp in pairs]

        zs, sums = {}, {}

        def prob(jp, row, z, n=GS, lanes=slice(None)):
            return jnp.exp2(s_s[jp % 4, row // 8:(row + n) // 8, :, lanes] - z[:, lanes])

        def rough(jp, mx, tie):
            zs[jp] = mx
            if jp > 0:
                sm = _Reducer(jnp.sum, jnp.add)
                for k, r in enumerate(range(0, 2 * jp * T, GS * LSUB)):
                    sm.add(prob(jp, r, tie(mx, k)))
                zs[jp] = mx + jnp.log2(jnp.maximum(LSUB * sm.result(), 1.0))
            sums[jp] = _Reducer(jnp.sum, jnp.add)

        def blocks(jp, row, tie, k):
            top, bot = prob(jp, row, tie(zs[jp], k)), prob(jp, jp * T + row, tie(zs[jp], k + 1))
            sums[jp].add(top + bot)
            top, bot = top.reshape(GS, 2 * T), bot.reshape(GS, 2 * T)
            return [top[:, :T], top[:, T:], bot[:, :T], bot[:, T:]]

        def near(jp, tie, k):
            R, z = jp * T, zs[jp]
            if jp % 2:
                for r in range(0, T, GS):
                    _put(pb_s, jp // 2 * T + r, 0, _operands(_B_TERMS, blocks(jp, R - T + r, tie, k)))
                    k += 2
            for r in range(0, T, GS):
                p = prob(jp, 2 * R + r, tie(z, k))
                sums[jp].add(p)
                _put(pd_s, 2 * R + r, 0, [p.reshape(GS, 2 * T)])
                k += 1
            so = _Reducer(jnp.sum, jnp.add)
            for r in range(0, T, 2 * GS):
                p = prob(jp, 2 * R + T + r, tie(z, k), 2 * GS, slice(T, 2 * T))
                so.add(p)
                _put(pd_s, 2 * R + T + r, T, [p.reshape(2 * GS, T)])
                k += 1
            sums[jp].result()
            sums[jp].out = sums[jp].out + jnp.concatenate([jnp.zeros((1, T), f32), so.result()], axis=1)

        p20 = lambda g: g * (g - 1) // 2 * T

        def far(g, tie, k):
            half = {(jp, e): _Reducer(jnp.sum, jnp.add) for jp in (2 * g, 2 * g + 1) for e in range(2)}
            for kg in range(g):
                for r in range(0, T, GS):
                    blk = {}
                    for new, n1 in (((0,), 1), ((1,), 5), ((3,), 2), ((), 0), ((), 4), ((2,), 3), ((), 6)):
                        for o in new:
                            lanes = slice((o % 2) * T, (o % 2 + 1) * T)
                            for jp in (2 * g, 2 * g + 1):
                                z = tie(zs[jp][:, lanes], k)
                                row = (o // 2) * jp * T + 2 * kg * T + r
                                p = [jnp.exp2(s_s[jp % 4, x // 8:(x + GS) // 8, :, lanes] - z) for x in (row, row + T)]
                                half[jp, o % 2].add(p[0] + p[1])
                                blk[o, jp % 2], blk[o, 2 + jp % 2] = [x.reshape(GS, T) for x in p]
                        ops = _operands2(_B_TERMS, n1, lambda o, q: blk[o, q], lambda x: x)
                        _put(p2_s, p20(g) + kg * T + r, 7 * n1 * T, ops, lambda w: tie(w, k, True, LATE))
                        k += 16 / 7
            for jp in (2 * g, 2 * g + 1):
                if g:
                    sums[jp].out = sums[jp].out + jnp.concatenate([half[jp, e].result() for e in range(2)], axis=1)
            for jp in (2 * g, 2 * g + 1):
                cols = slice(2 * jp * T, 2 * (jp + 1) * T)
                sc_s[:, cols] = g_s[:, cols] / sums[jp].result()

        def pv(g):
            pairs = (2 * g, 2 * g + 1)
            va = lambda n, t, r=0, nr=HD: _get(va_s, r, nr, (t * 9 + n) * T, T)
            for n1 in range(7 if g else 0):
                c = clk.strassen(
                    lambda n: _cat([_get(v2_s, 0, QD, (kg * 49 + 7 * n1 + n) * T, T) for kg in range(g)], 1),
                    lambda n: _get(p2_s, p20(g), g * T, (7 * n1 + n) * T, T), _NN, g)()
                mp_s[n1 * HD:n1 * HD + QD, :] = jnp.concatenate(c[:2], axis=1)
                mp_s[n1 * HD + QD:(n1 + 1) * HD, :] = jnp.concatenate(c[2:], axis=1)
            ve = [jnp.concatenate([va(2, jp), va(8, jp)], axis=0) for jp in pairs]
            vo = [jnp.concatenate([va(7, jp), va(3, jp)], axis=0) for jp in pairs]
            ce = clk.level([(ve[jp % 2], _get(pd_s, 2 * jp * T, T, 0, T)) for jp in pairs])
            co = [clk.dot(jnp.concatenate([ve[jp % 2], vo[jp % 2]], axis=1),
                          _get(pd_s, 2 * jp * T, 2 * T, T, T), _NN) for jp in pairs]
            for jp in pairs:
                R, e = jp * T, jp % 2
                ge, go = sc_s[:, 2 * R:2 * R + T], sc_s[:, 2 * R + T:2 * R + 2 * T]
                for r in range(0, HD, 32):
                    c = [ce[e][r:r + 32], co[e][r:r + 32], ce[e][HD + r:HD + r + 32], co[e][HD + r:HD + r + 32]]
                    if g:
                        far_ = _combine([mp_s[n * HD + r:n * HD + r + 32, e * T:(e + 1) * T] for n in range(7)],
                                        order=range(7))
                        c = [x + y for x, y in zip(c, far_)]
                    if e:
                        near_ = clk.strassen(lambda n: va(n, 2 * g, r, 32),
                                             lambda n: _get(pb_s, g * T, T, n * T, T), _NN)()
                        c = [x + y for x, y in zip(c, near_)]
                    ops = _operands(_B_TERMS, [c[0] * ge, c[1] * go, c[2] * ge, c[3] * go])
                    _put(cl_s, r, jp * 7 * T, ops)

        ends = []

        def run(items):
            for item in items.split():
                if item[0] == 'P':
                    pv(int(item[1]))
                    ends.append(clk.t)
                elif item[0] == 'K':
                    proj(int(item[1]))
                else:
                    jp = int(item[1])
                    oproj(jp, clk)

                    @pl.when(h == H - 1)
                    def _():
                        out_copy(jp).start()

        for n1 in range(7):
            if n1 >= NT1:
                prep_w(h, [n1], clk.pacer(clk.t - 896, clk.t - 448, 8))
            proj(0, n1, n1 + 1)
        oproj(NP - 1, clk)
        mx = qk(0)
        for g in range(4):
            t0 = clk.t
            del ends[:]
            run(PLAN[g])
            t1 = clk.t
            nxt = qk(g + 1) if g < 3 else None
            n_rough = [2 * jp * T // (GS * LSUB) for jp in (2 * g, 2 * g + 1)]
            n_near = [(T + T // 2) // GS, (3 * T + T // 2) // GS]
            holes = [(t - 400, t) for t in ends]
            if 0 < g < 3:
                holes.append((marks[-2] - 400, marks[-2] - 100))
            if g < 3:
                vfin(g, clk.pacer(t0, t0 + VW, 32))
                holes += [(t0, t0 + VW), (t1 - 300, t1 + 300)]
            if g == 2:
                vfin(3, clk.pacer(clk.t - SLACK - VW // 2, clk.t - SLACK, 32))
                holes.append((clk.t - SLACK - VW // 2, clk.t))
            tie = clk.pacer(t0, (clk.t if g else t1) - SLACK,
                            sum(n_rough) + sum(n_near) + g * 16 * T // GS, holes)
            rough(2 * g, mx[0], tie)
            near(2 * g, tie, n_rough[0])
            k = n_rough[0] + n_near[0]
            rough(2 * g + 1, mx[1], lambda x, i: tie(x, k + i))
            near(2 * g + 1, tie, k + n_rough[1])
            far(g, tie, k + n_rough[1] + n_near[1])
            if g == 0:
                prep_wo(clk.pacer(t0 + VW, t1 - 300, HM // 16))
            mx = nxt
        t0 = clk.t
        run(PLAN[4])
        prep_w(jnp.minimum(h + 1, H - 1), range(NT1), clk.pacer(t0 - 100, clk.t - 300, 8 * NT1))
        assert len(set(clk.load)) == 1

    head(**head_refs)

    @pl.when(h == H - 1)
    def _():
        oproj(NP - 1, _Clock(zero_s))
        out_copy(NP - 1).start()
        for jp in range(NP):
            out_copy(jp).wait()


@jax.jit
def pallas_gated_mix__compressed_kv_cla__ssm_conv_s5__prompt_kernel(
    A_x: jax.Array,
    A_c_kv: jax.Array,
    A_w_q: jax.Array,
    A_w_uk: jax.Array,
    A_w_uv: jax.Array,
    A_w_o: jax.Array,
    B_x: jax.Array,
    B_Lambda_re: jax.Array,
    B_Lambda_im: jax.Array,
    B_B_re: jax.Array,
    B_B_im: jax.Array,
    B_C_re: jax.Array,
    B_C_im: jax.Array,
    B_log_dt: jax.Array,
    B_Dskip: jax.Array,
    gate_w: jax.Array,
):
    del B_x
    xT = jnp.transpose(A_x[0])
    woT = jnp.transpose(A_w_o, (0, 2, 1))
    ckv = A_c_kv.reshape(4, 4, 2, T // 2, DC)

    hbm = pl.BlockSpec(memory_space=pl.ANY)
    outT = pl.pallas_call(
        _kernel,
        grid=(H,),
        in_specs=[hbm] * 15,
        out_specs=hbm,
        out_shape=jax.ShapeDtypeStruct((M, S), f32),
        scratch_shapes=_SHARED_SCRATCH + list(_PROLOGUE_SCRATCH.values()) + list(_HEAD_SCRATCH.values()),
        compiler_params=pltpu.CompilerParams(
            dimension_semantics=("arbitrary",),
            vmem_limit_bytes=127 * 1024 * 1024,
        ),
    )(xT, B_B_re, B_B_im, B_C_re, B_C_im, B_Lambda_re, B_Lambda_im, B_log_dt,
      B_Dskip, gate_w, woT, ckv, A_w_q, A_w_uk, A_w_uv)
    return jnp.transpose(outT)[None]
```

```python
import bisect

import jax
import jax.numpy as jnp
from jax import lax
import jax.experimental.pallas as pl
import jax.experimental.pallas.tpu as pltpu

S = 2048
M = 448
H = 16
D = 256
DC = 1024
T = 128
NP = S // T // 2
HD = D // 2
HM = M // 2
QD = D // 4
QC = DC // 4
QM = M // 4
PA = 384
PB = M - PA
TA = 512
TC = 256
CS = DC // NP
NRAW = 2
LOG2E = 1.4426950408889634
NEG = -1e30

GS = 16
RCH = 256
LSUB = 4
NT1 = 3
OCH = ((0, 64), (64, 64), (128, 48), (176, 48))
PLAN = ('K1', 'K2', 'K3', 'P1 P0 O2 O3 P2 O0 O1 O4 O5', 'P3 O6')
SLACK, LATE, VW = 200, 40, 900

f32 = jnp.float32
bf16 = jnp.bfloat16
u32 = jnp.uint32

SEM_VEC, SEM_B, SEM_X, SEM_WQ, SEM_C, SEM_SL, SEM_WO, SEM_OUT, SEM_WQ1, SEM_KV = 0, 1, 2, 6, 7, 8, 16, 17, 18, 22
NSEM = 24

_NN = ((1,), (0,))
_NT = ((1,), (1,))
_TT = ((0,), (1,))


def _cat(xs, axis):
    return xs[0] if len(xs) == 1 else jnp.concatenate(xs, axis=axis)


def _ds(lo, n, align):
    return pl.ds(lo if isinstance(lo, int) else pl.multiple_of(lo, align), n)


def _put(ref, row, col, xs, tie=None):
    x = _cat(xs, 1)
    if tie is not None:
        x = jnp.concatenate([tie(x[:8]), x[8:]], axis=0)
    ref[row // 2:(row + x.shape[0]) // 2, col:col + x.shape[1]] = pltpu.bitcast(x.astype(bf16), u32)


def _get(ref, row, nrows, col, ncols):
    return pltpu.bitcast(ref[row // 2:(row + nrows) // 2, col:col + ncols], bf16)


class _Clock:
    def __init__(self, zero_ref):
        self.masks = {(8, T): zero_ref[...] != 0.0}
        self.ticks, self.load = [], [0, 0, 0, 0]

    @property
    def t(self):
        return max(self.load)

    def dot(self, a, b, dims):
        v = lax.dot_general(a, b, (dims, ((), ())), preferred_element_type=f32)
        rows, depth = v.shape[0], a.shape[dims[0][0]]
        for c in range(0, v.shape[1], T):
            start = 0
            for _ in range(0, depth, T):
                k = self.load.index(min(self.load))
                start = max(start, self.load[k])
                self.load[k] += rows
            self.ticks += [(start + r + 8, (v, r, c)) for r in range(0, rows, 8)]
        return v

    def strassen(self, lhs, rhs, dims, jobs=1, split_last=False):
        lag = sum(l + 32 <= max(self.load) for l in self.load) // jobs if jobs < 3 else 0
        order = ((1, 3, 2, 4, 0, 5, 6), (0, 1, 3, 2, 4, 5, 6), (5, 6, 1, 3, 2, 4, 0), (0, 5, 6, 1, 3, 2, 4))[lag]
        m = {}
        for n in order:
            a, b = lhs(n), rhs(n)
            if split_last and n == order[-1]:
                half = a.shape[0] // 2
                m[n] = jnp.concatenate([self.dot(a[:half], b, dims), self.dot(a[half:], b, dims)], axis=0)
            else:
                m[n] = self.dot(a, b, dims)
        return lambda r=0, n=None: _combine(m if n is None else _Rows(m, r, n), order=order)

    def level(self, pairs, dims=_NN):
        base, extra = divmod((sum(self.load) + sum(a.shape[0] for a, _ in pairs)) // 16, 4)
        target = [16 * (base + (k < extra)) for k in range(4)]
        out = []
        for a, b in pairs:
            r, parts = 0, []
            while r < a.shape[0]:
                k = self.load.index(min(self.load))
                n = min(max(target[k] - self.load[k], 16), a.shape[0] - r)
                parts.append(self.dot(a[r:r + n], b, dims))
                r += n
            out.append(_cat(parts, 0))
        return out

    def pacer(self, t0, t1, n, holes=()):
        holes = sorted((max(a, t0), min(b, t1)) for a, b in holes if a < t1 and b > t0)
        gap = sum(b - a for a, b in holes)
        ticks = sorted(self.ticks, key=lambda tw: tw[0])
        times = [tw[0] for tw in ticks]

        def tie(x, k, distinct=False, delay=0):
            t = t0 + (t1 - t0 - gap) * k / n
            for a, b in holes:
                t += b - a if t > a else 0
            t += delay
            past = ticks[:bisect.bisect_right(times, t)]
            reps = (x.shape[0] // 8, x.shape[1] // T)
            if len(past) < (reps[1] if distinct else 1):
                return x
            tick = _cat([v[r:r + 8, c:c + T] for _, (v, r, c) in past[-reps[1] if distinct else -1:]], 1)
            if tick.dtype != x.dtype:
                tick = pltpu.bitcast(tick, x.dtype)
            if x.shape not in self.masks:
                self.masks[x.shape] = jnp.tile(self.masks[(8, T)], reps)
            return lax.select(self.masks[x.shape], tick if tick.shape == x.shape else jnp.tile(tick, reps), x)
        return tie


def _no_tie(x, k):
    return x


_A_TERMS = ((0, 3, 1), (2, 3, 1), (0, None, 0), (3, None, 0), (0, 1, 1), (2, 0, -1), (1, 3, -1))
_B_TERMS = ((0, 3, 1), (0, None, 0), (1, 3, -1), (2, 0, -1), (3, None, 0), (0, 1, 1), (2, 3, 1))


def _operand(term, block):
    x, y, sign = term
    if y is None:
        return block(x)
    return block(x) + block(y) if sign > 0 else block(x) - block(y)


def _operands(terms, blocks):
    return [_operand(t, blocks.__getitem__) for t in terms]


def _operands2(terms, n1, block, tie):
    first = terms[n1][0]
    sub = [_operand(terms[n1], lambda o: tie(block(o, q)) if o == first and q in (0, 3) else block(o, q))
           for q in range(4)]
    return _operands(terms, sub)


_C_TERMS = ({0: 1, 3: 1, 4: -1, 6: 1}, {2: 1, 4: 1}, {1: 1, 3: 1}, {0: 1, 1: -1, 2: 1, 5: 1})


def _combine(m, only=(0, 1, 2, 3), order=(1, 3, 2, 4, 0, 5, 6)):
    out = []
    for terms in (_C_TERMS[n] for n in only):
        seq = [n for n in order if n in terms]
        if terms[seq[0]] < 0:
            seq[0], seq[1] = seq[1], seq[0]
        acc = m[seq[0]]
        for n in seq[1:]:
            acc = acc + m[n] if terms[n] > 0 else acc - m[n]
        out.append(acc)
    return out


def _outer_step(m_s, n1, row, v):
    n = v.shape[0]
    if n1 < 5:
        m_s[n1 * HD + row:n1 * HD + row + n, :] = v
    if n1 < 3:
        return None
    blk = (2, 1, 3, 0)[n1 - 3]
    m = {j: v if j == n1 else m_s[j * HD + row:j * HD + row + n, :] for j in _C_TERMS[blk]}
    return blk, _combine(m, (blk,), range(7))[0]


class _Rows:
    def __init__(self, vals, r, n):
        self.vals, self.rows, self.cache = vals, slice(r, r + n), {}

    def __getitem__(self, i):
        if i not in self.cache:
            self.cache[i] = self.vals[i][self.rows, :]
        return self.cache[i]


class _Reducer:
    def __init__(self, red, comb):
        self.red, self.comb, self.acc, self.rows, self.out = red, comb, None, 0, None

    def add(self, v):
        self.rows += 8 * v.shape[0]
        v = self.red(v, axis=0)
        self.acc = v if self.acc is None else self.comb(self.acc, v)
        if self.rows >= RCH:
            self.result()

    def result(self):
        if self.acc is not None:
            v = self.red(self.acc, axis=0, keepdims=True)
            self.out = v if self.out is None else self.comb(self.out, v)
        self.acc, self.rows = None, 0
        return self.out


def _cmul(ar, ai, br, bi):
    return ar * br - ai * bi, ar * bi + ai * br


def _hi16(w):
    return pltpu.bitcast(w & jnp.uint32(0xFFFF0000), f32)


def _stage(raw, stg, c0, nc, tie, groups=(0, 1)):
    for ht in groups:
        for dt in range(2):
            v = raw[c0:c0 + nc, ht * 8:(ht + 1) * 8, dt * T:(dt + 1) * T].reshape(nc * 8, T)
            stg[ht * 2 + dt, c0 * 4:(c0 + nc) * 4, :] = tie(pltpu.bitcast(v, u32), (ht * 2 + dt) / 4)


def _ssm_params(vec_s, coef_s, lam_s, col_s):
    row = lambda r: r[...].astype(f32).reshape(1, M)
    lre, lim, ldt, dsk, gw = [row(v) for v in vec_s]
    dt = jnp.exp(ldt).astype(bf16).astype(f32)
    mag = jnp.exp(dt * lre)
    ang = dt * lim
    lr, li = mag * jnp.cos(ang), mag * jnp.sin(ang)
    den = lre * lre + lim * lim
    nr = lr - 1.0
    coef_s[...] = jnp.zeros(coef_s.shape, f32)
    coef_s[0:1, 0:M] = 2.0 * ((nr * lre + li * lim) / den)
    coef_s[1:2, 0:M] = 2.0 * ((li * lre - nr * lim) / den)

    er = jnp.concatenate([lr, lr[:, PA:]], axis=1)
    ei = jnp.concatenate([li, -li[:, PA:]], axis=1)
    pw = [(er, ei)]
    for _ in range(7):
        pw.append(_cmul(pw[-1][0], pw[-1][1], er, ei))
    sub = lax.broadcasted_iota(jnp.int32, (8, 512), 0)
    for n, d in enumerate((1, 2, 4)):
        lam_s[2 * n] = jnp.where(sub >= d, pw[d - 1][0], 0.0)
        lam_s[2 * n + 1] = jnp.where(sub >= d, pw[d - 1][1], 0.0)
    lcr = jnp.zeros((8, 512), f32)
    lci = jnp.zeros((8, 512), f32)
    for r in range(8):
        lcr = jnp.where(sub == r, pw[r][0], lcr)
        lci = jnp.where(sub == r, pw[r][1], lci)
    lam_s[6] = lcr
    lam_s[7] = lci

    def col(v):
        v = jnp.concatenate([v, jnp.zeros((1, 512 - M), f32)], axis=1)
        return jnp.broadcast_to(v, (T, 512)).T[:M]
    col_s[0] = col(dsk)
    col_s[1] = col(gw)


def _ssm_cmat(craw_s, coef_s, c_s, tie):
    for r in range(0, HM, 16):
        for c in range(0, M, T):
            w = min(T, M - c)
            coef = tie(coef_s[:, c:c + T], r // 16 + c / 512)
            cr, ci = coef[0:1, :w], coef[1:2, :w]
            blk = []
            for row in (r, HM + r):
                re, im = _cmul(craw_s[0, row:row + 16, c:c + w].astype(f32),
                               craw_s[1, row:row + 16, c:c + w].astype(f32), cr, ci)
                blk += [re, -im]
            if c < PA:
                for n, op in enumerate(_operands(_A_TERMS, blk)):
                    _put(c_s, r, n * PA + c, [op])
            else:
                _put(c_s, r, 7 * PA, blk)


def _ssm_scan(u_ref, carry, lam_s, h_s, h0_s, tie):
    car, cai = carry
    out = []
    for b in range(TC // 8):
        mixed = u_ref[3, b, :, 0:T]
        u = jnp.concatenate([u_ref[cb, b] for cb in range(3)], axis=1)
        cols = [u[:, 0:T], u[:, T:2 * T], u[:, 2 * T:PA], mixed]
        hr = jnp.concatenate([tie(v, 4 * b + n) for n, v in enumerate(cols)], axis=1)
        hi = jnp.concatenate([u[:, PA:2 * PA], pltpu.roll(mixed, PB, 1)], axis=1)
        for n, d in enumerate((1, 2, 4)):
            sr, si = pltpu.roll(hr, d, 0), pltpu.roll(hi, d, 0)
            tr, ti = _cmul(sr, si, lam_s[2 * n], lam_s[2 * n + 1])
            hr, hi = hr + tr, hi + ti
        tr, ti = _cmul(lam_s[6], lam_s[7], car, cai)
        hr, hi = hr + tr, hi + ti
        car, cai = hr[7:8, :], hi[7:8, :]
        out.append(jnp.concatenate([hr[:, :PA], hi[:, :PA], hr[:, PA:]], axis=1))
        if b % 2 == 1:
            v, row = jnp.concatenate(out, axis=0), (b - 1) * 8 % T
            _put(h_s, row, 7 * PA + b // 16 * T, [v[:, 2 * PA:]])
            if b < 16:
                h0_s[row:row + 16, :] = v[:, :2 * PA]
            else:
                v0 = h0_s[row:row + 16, :]
                _put(h_s, row, 0, _operands(_B_TERMS, [v0[:, :PA], v[:, :PA], v0[:, PA:], v[:, PA:2 * PA]]))
            out = []
    return car, cai


_vmem = pltpu.VMEM
_PROLOGUE_SCRATCH = dict(
    xT_s=_vmem((M, S), bf16),
    v0=_vmem((M,), bf16), v1=_vmem((M,), bf16), v2=_vmem((M,), bf16), v3=_vmem((M,), bf16), v4=_vmem((M,), bf16),
    b_s=_vmem((2 * M, M), bf16),
    craw_s=_vmem((2, M, M), bf16),
    c_s=_vmem((HM // 2, 7 * PA + 2 * T), u32),
    coef_s=_vmem((8, 512), f32),
    lam_s=_vmem((8, 8, 512), f32),
    col_s=_vmem((2, M, T), f32),
    h_s=_vmem((T // 2, 7 * PA + 2 * T), u32),
    h0_s=_vmem((T, 2 * PA), f32),
    ckv_s=_vmem((NRAW, 4, T // 2, DC), bf16),
    rq=_vmem((M, H, D), bf16),
    rk=_vmem((CS + 1, H, D), bf16),
    rv=_vmem((CS + 1, H, D), bf16),
    sq=_vmem((4, M * 4, T), u32),
    sk=_vmem((4, CS * 4, T), u32),
    sv=_vmem((4, CS * 4, T), u32),
    wqt_s=_vmem((D, 4 * T), u32),
)
_HEAD_SCRATCH = dict(
    mk_s=_vmem((7 * HD, 2 * T), f32),
    mv_s=_vmem((2, 7 * HD, 2 * T), f32),
    mp_s=_vmem((7 * HD, 2 * T), f32),
    kt_s=_vmem((2 * T, 4 * T), f32),
    ka_s=_vmem((S // 4, 8 * T), u32),
    va_s=_vmem((HD // 2, NP * 9 * T), u32),
    v2_s=_vmem((QD // 2, 3 * 49 * T), u32),
    s_s=_vmem((4, S // 8, 8, 2 * T), f32),
    pb_s=_vmem((2 * T, 7 * T), u32),
    pd_s=_vmem((S // 2, 2 * T), u32),
    p2_s=_vmem((3 * T, 49 * T), u32),
    sc_s=_vmem((1, S), f32),
    qb_s=_vmem((HD // 2, 14 * T), u32),
    kd_s=_vmem((T // 2, 7 * T), u32),
)
_SHARED_SCRATCH = [
    _vmem((H // 2 * D, DC), u32),
    _vmem((H // 2 * D, DC), u32),
    _vmem((S // 8, 49 * QC), u32),
    _vmem((H * D, S // 2), u32),
    _vmem((H, M, D), bf16),
    _vmem((QD, 49 * QC), u32),
    _vmem((HM // 2, 7 * T), u32),
    _vmem((HD // 2, NP * 7 * T), u32),
    _vmem((M, S), f32),
    _vmem((1, S), f32),
    _vmem((8, T), f32),
    pltpu.SemaphoreType.DMA((NSEM,)),
]


def _kernel(xT_hbm, bre_hbm, bim_hbm, cre_hbm, cim_hbm, lre_hbm, lim_hbm, ldt_hbm,
            dsk_hbm, gw_hbm, woT_hbm, ckv_hbm, wq_hbm, wk_hbm, wv_hbm,
            out_hbm,
            wkt_s, wvt_s, a_s, q_s, wo_s, w_s, wl_s, cl_s, o_s, g_s, zero_s, sem, *rest):
    h = pl.program_id(0)
    pro_refs = dict(zip(_PROLOGUE_SCRATCH, rest))
    head_refs = dict(zip(_HEAD_SCRATCH, rest[len(pro_refs):]))

    def out_copy(jp):
        cols = pl.ds(jp * 2 * T, 2 * T)
        return pltpu.make_async_copy(o_s.at[:, cols], out_hbm.at[:, cols], sem.at[SEM_OUT])

    def prep_w(hh, outer, tie):
        rows = _ds(lax.shift_right_logical(hh, 1) * D, D, D)
        sh = (16 * (1 - (hh & 1))).astype(u32)
        k = 0
        for row0, wt_s in ((0, wkt_s.at[rows]), (QD, wvt_s.at[rows])):
            for r in range(0, QD, 16):
                def block(o, q):
                    row = (o % 2) * HD + (q % 2) * QD + r
                    col = (o // 2) * 2 * QC + (q // 2) * QC
                    return _hi16(wt_s[row:row + 16, col:col + QC] << sh)
                for n1 in outer:
                    _put(w_s, row0 + r, 7 * n1 * QC, _operands2(_B_TERMS, n1, block, lambda x: tie(x, k)))
                    k += 1

    def prologue(xT_s, v0, v1, v2, v3, v4, b_s, craw_s, c_s, coef_s, lam_s, col_s, h_s, h0_s,
                 ckv_s, rq, rk, rv, sq, sk, sv, wqt_s):
        xa_s = head_refs['p2_s']
        wq_s = xa_s.at[2 * QM:2 * QM + QD]
        u_s = head_refs['s_s']
        vec_s = (v0, v1, v2, v3, v4)

        def slice_copies(i):
            s = sem.at[SEM_SL + i]
            grp = i // 2 if isinstance(i, int) else lax.shift_right_logical(i, 1)
            return [pltpu.make_async_copy(ckv_hbm.at[grp, :, i & 1], ckv_s.at[i & (NRAW - 1)], s)]

        def w_copy(n, i):
            src, dst = ((wk_hbm, rk), (wv_hbm, rv))[n]
            return pltpu.make_async_copy(src.at[pl.ds(i * CS, CS)], dst.at[0:CS], sem.at[SEM_KV + n])

        def wo_copy(i):
            heads = pl.ds(2 * i, 2)
            return pltpu.make_async_copy(woT_hbm.at[heads], wo_s.at[heads], sem.at[SEM_WO])

        def wq1_copy(i):
            rows = pl.ds(i * (M // 4), M // 4)
            return pltpu.make_async_copy(wq_hbm.at[rows, 8:16], rq.at[rows, 8:16], sem.at[SEM_WQ1 + i])

        def x_copy(i):
            cols = pl.ds(i * TA, TA)
            return pltpu.make_async_copy(xT_hbm.at[:, cols], xT_s.at[:, cols], sem.at[SEM_X + i])

        cp_vec = [pltpu.make_async_copy(src, dst, sem.at[SEM_VEC])
                  for src, dst in zip((lre_hbm, lim_hbm, ldt_hbm, dsk_hbm, gw_hbm), vec_s)]
        cp_b = [pltpu.make_async_copy(src.at[pl.ds(lo, n)], b_s.at[pl.ds(dst, n)], sem.at[SEM_B])
                for src, lo, n, dst in ((bre_hbm, 0, PA, 0), (bim_hbm, 0, PA, PA),
                                        (bre_hbm, PA, PB, 2 * PA), (bim_hbm, PA, PB, 2 * PA + PB))]
        cp_wq = [pltpu.make_async_copy(wq_hbm.at[:, 0:8], rq.at[:, 0:8], sem.at[SEM_WQ])]
        cp_c = [pltpu.make_async_copy(src, craw_s.at[n], sem.at[SEM_C])
                for n, src in enumerate((cre_hbm, cim_hbm))]
        for cp in cp_vec + cp_b + [x_copy(i) for i in range(S // TA)] + cp_c + cp_wq:
            cp.start()
        for cp in [wq1_copy(0)] + slice_copies(0) + [w_copy(0, 0), w_copy(1, 0)]:
            cp.start()

        zero_s[...] = jnp.zeros(zero_s.shape, f32)
        wl_s[...] = jnp.zeros(wl_s.shape, u32)
        cl_s[:, (NP - 1) * 7 * T:] = jnp.zeros((HD // 2, 7 * T), u32)
        for cp in cp_vec:
            cp.wait()
        _ssm_params(vec_s, coef_s, lam_s, col_s)

        def wq_transpose(pair, tie):
            ht = pair // 4 if isinstance(pair, int) else lax.shift_right_logical(pair, 2)
            pad = jnp.zeros((T - QM, T), u32)
            for dt in range(2):
                for mq in range(4):
                    blk = sq[ht * 2 + dt, pl.ds(mq * QM * 4 + (pair & 3), QM, stride=4), :]
                    blk = jnp.concatenate([tie(blk[:8], 4 * dt + mq), blk[8:], pad], axis=0)
                    wqt_s[dt * HD:(dt + 1) * HD, mq * T:(mq + 1) * T] = blk.T

        def phase1(i, gates):
            clk = _Clock(zero_s)
            u = _cat([clk.dot(xT_s[:, i * TA + lo:i * TA + hi], b_s[...], _TT)
                      for lo, hi in ((0, T), (T, TA))], 0)
            for cb in range(4):
                w = min(2 * T, 2 * M - cb * 2 * T)
                u_s[cb, i * TA // 8:(i + 1) * TA // 8, :, 0:w] = (
                    u[:, cb * 2 * T:cb * 2 * T + w].reshape(TA // 8, 8, w))
            tie = clk.pacer(0, 6 * TA, 49)
            for r in range(0, QM, 16):
                def block(o, q):
                    row, col = (o % 2) * HM + (q % 2) * QM + r, (4 * i + 2 * (q // 2) + o // 2) * T
                    return xT_s[row:row + 16, col:col + T].astype(f32) * (LOG2E * D ** -0.5)
                for n1 in range(7):
                    ops = _operands2(_A_TERMS, n1, block, lambda x: tie(x, 7 * (r // 16) + n1))
                    _put(xa_s, i * QM + r, 7 * n1 * T, ops)
            tie = clk.pacer(0, 6 * TA, 28 * len(gates))
            for t, tile in enumerate(gates):
                cols = slice(tile * T, (tile + 1) * T)
                acc = jnp.zeros((8, T), f32)
                for r in range(0, M, 32):
                    xg = xT_s[r:r + 32, cols].astype(f32) * tie(col_s[1, r:r + 32, :], 28 * t + r // 32)
                    acc = acc + jnp.sum(xg.reshape(4, 8, T), axis=0)
                g = jax.nn.sigmoid(jnp.sum(acc, axis=0, keepdims=True))
                g_s[:, cols] = g
                for r in range(0, M, 32):
                    skip = xT_s[r:r + 32, cols].astype(f32) * tie(col_s[0, r:r + 32, :], 28 * t + 14 + r // 32)
                    o_s[r:r + 32, cols] = (1.0 - g) * skip
            return clk

        for cp in cp_b + [x_copy(0)]:
            cp.wait()
        phase1(0, range(4))
        x_copy(1).wait()
        clk = phase1(1, range(4, 6))
        zero = jnp.zeros((1, 512), f32)
        carry0 = _ssm_scan(u_s.at[:, 0:TC // 8], (zero, zero), lam_s, h_s, h0_s, clk.pacer(0, 6 * TA, TC // 2))
        for cp in [x_copy(2), x_copy(3)] + cp_c + cp_wq:
            cp.wait()
        _ssm_cmat(craw_s, coef_s, c_s, phase1(2, range(6, 9)).pacer(0, 6 * TA, HM // 16))
        tie = phase1(3, range(9, 16)).pacer(0, 6 * TA, M // 8)
        for c0 in range(0, M, 8):
            _stage(rq, sq, c0, 8, lambda x, j: tie(x, c0 / 10 + j), groups=(0,))
        wq_transpose(0, lambda x, k: tie(x, 46 + k))

        def phase2(i, carry):
            @pl.when(i + 1 < NP)
            def _():
                for cp in slice_copies(i + 1):
                    cp.start()

            @pl.when(i < 3)
            def _():
                wq1_copy(i + 1).start()

            wo_copy(i).start()

            @pl.when(i < 4)
            def _():
                wq1_copy(i).wait()

            for cp in slice_copies(i) + [w_copy(0, i), w_copy(1, i)]:
                cp.wait()

            clk = _Clock(zero_s)
            comb = clk.strassen(lambda n: _get(c_s, 0, HM, n * PA, PA), lambda n: _get(h_s, 0, T, n * PA, PA), _NT, 3)
            mixed = clk.level([(_get(c_s, 0, HM, 7 * PA + n // 2 * T, T), _get(h_s, 0, T, 7 * PA + n % 2 * T, T))
                               for n in range(4)], _NT)
            ty = clk.t
            cols = _ds(i * TC, TC, TC)
            keep = 1.0 - g_s[:, cols]
            for r in range(0, HM, 32):
                y = [c + m[r:r + 32] for c, m in zip(comb(r, 32), mixed)]
                o_s[r:r + 32, cols] += keep * jnp.concatenate(y[:2], axis=1)
                o_s[HM + r:HM + r + 32, cols] += keep * jnp.concatenate(y[2:], axis=1)

            q_i = q_s.at[_ds(i * 2 * D, 2 * D, 2 * D)]
            mq_s = (head_refs['mk_s'], head_refs['mp_s'], head_refs['mv_s'].at[0], head_refs['mv_s'].at[1])
            for g in range(4):
                for n1 in range(7):
                    if g == 0:
                        t = 200 + (ty + 644) * n1 / 7
                        tie = clk.pacer(min(t, clk.t - 500), min(t + 300, clk.t - 500), 8)
                        for r in range(0, 2 * QD, 16):
                            def block(o, q):
                                row = (o % 2) * HD + (q % 2) * QD + r % QD
                                col = (2 * (o // 2) + q // 2) * T
                                w = wqt_s[row:row + 16, col:col + T]
                                return _hi16(w) if r >= QD else pltpu.bitcast(w << 16, f32)
                            _put(wq_s, r, 7 * n1 * T, _operands2(_B_TERMS, n1, block, lambda x: tie(x, r // 16)))
                    comb = clk.strassen(lambda n: _get(wq_s, 0, 2 * QD, (7 * n1 + n) * T, QM),
                                        lambda n: _get(xa_s, g * QM, QM, (7 * n1 + n) * T, T), _NN)
                    for r in range(0, 2 * QD, 32):
                        e, c = r // QD, comb(r, 32)
                        for dq in range(2):
                            row = dq * QD + r % QD
                            done = _outer_step(mq_s[2 * (g % 2) + e], n1, row,
                                               jnp.concatenate([c[dq], c[2 + dq]], axis=1))
                            if done:
                                n, v = done
                                _put(q_i, (2 * e + n // 2) * D + (n % 2) * HD + row, 2 * g * T, [v])

            span = ty + 6000

            u_next = u_s.at[:, pl.ds(jnp.minimum(i + 1, NP - 1) * (TC // 8), TC // 8)]
            carry = _ssm_scan(u_next, carry, lam_s, h_s, h0_s, clk.pacer(ty, span, TC // 2))

            tie = clk.pacer(ty - 1200, span, 64, [(ty, ty + 1000)])
            rq_i = rq.at[pl.ds((i & 3) * (M // 4), M // 4)]
            sq_i = sq.at[:, _ds((i & 3) * M, M, 8)]
            for c0 in range(0, M // 4, 8):
                _stage(rq_i, sq_i, c0, 8, lambda x, j: tie(x, c0 // 4 + 4 * j), groups=(1,))
            wq_transpose(jnp.minimum(i + 1, NP - 1), lambda x, k: tie(x, 36 + 3 * k))
            for n, (raw, stg, wt_s) in enumerate(((rk, sk, wkt_s), (rv, sv, wvt_s))):
                for c0 in range(0, CS, 8):
                    _stage(raw, stg, c0, 8, lambda x, j: tie(x, 16 * n + c0 // 8 + j))

                @pl.when(i + 1 < NP)
                def _():
                    w_copy(n, i + 1).start()

                raw[CS, 0:8, 0:T] = tie(zero_s[...], 16 * n + 19).astype(bf16)
                cols = _ds(i * CS, CS, CS)
                for pair in range(H // 2):
                    for dt in range(2):
                        blk = stg[(pair // 4) * 2 + dt, pl.ds(pair % 4, CS, stride=4), :]
                        row = pair * D + dt * HD
                        blk = jnp.concatenate([tie(blk[:8], 16 + 24 * n + 3 * pair + dt), blk[8:]], axis=0)
                        wt_s[row:row + HD, cols] = blk.T

            tie = clk.pacer(ty + 1000, span, 28)
            ckv_i = ckv_s.at[i & (NRAW - 1)]
            a_i = a_s.at[_ds(i * (T // 4), T // 4, T // 4)]
            for r in range(0, T // 2, 16):
                def block(o, q):
                    col = (o % 2) * 2 * QC + (q % 2) * QC
                    return ckv_i[2 * (q // 2) + o // 2, r:r + 16, col:col + QC].astype(f32)
                for n1 in range(7):
                    ops = _operands2(_A_TERMS, n1, block, lambda x: tie(x, 7 * (r // 16) + n1))
                    _put(a_i, r, 7 * n1 * QC, ops)
            return carry

        lax.fori_loop(0, NP, phase2, carry0)
        for i in range(NP):
            wo_copy(i).wait()
        prep_w(h, range(NT1), _no_tie)

    @pl.when(h == 0)
    def _():
        prologue(**pro_refs)

    def oproj(jp, clk):
        cols = slice(2 * jp * T, (2 * jp + 2) * T)
        for r, n in OCH:
            c = clk.strassen(lambda i: _get(wl_s, r, n, i * T, T),
                             lambda i: _get(cl_s, 0, HD, (jp * 7 + i) * T, T), _NN)()
            o_s[r:r + n, cols] += jnp.concatenate(c[:2], axis=1)
            o_s[HM + r:HM + r + n, cols] += jnp.concatenate(c[2:], axis=1)

    def head(mk_s, mv_s, mp_s, kt_s, ka_s, va_s, v2_s, s_s, pb_s, pd_s, p2_s, sc_s, qb_s, kd_s):
        clk = _Clock(zero_s)
        q_h = q_s.at[_ds(h * D, D, D)]

        def prep_wo(tie):
            for r in range(0, HM, 16):
                top = tie(wo_s[h, r:r + 16, :].astype(f32), r // 16)
                bot = tie(wo_s[h, HM + r:HM + r + 16, :].astype(f32), r // 16)
                _put(wl_s, r, 0, _operands(_A_TERMS, [top[:, :HD], top[:, HD:], bot[:, :HD], bot[:, HD:]]))

        def proj(g, lo=0, hi=7):
            for n1 in range(lo, hi):
                comb = clk.strassen(lambda n: _get(w_s, 0, 2 * QD, (7 * n1 + n) * QC, QC),
                                    lambda n: _get(a_s, g * T, T, (7 * n1 + n) * QC, QC), _NT, 2, n1 == 6)
                for r, m_s in ((0, mk_s), (QD, mv_s.at[g % 2])):
                    c = comb(r, QD)
                    m_s[n1 * HD:n1 * HD + QD, :] = jnp.concatenate([c[0], c[2]], axis=1)
                    m_s[n1 * HD + QD:(n1 + 1) * HD, :] = jnp.concatenate([c[1], c[3]], axis=1)
            if hi < 7:
                return
            cs = [_combine([mk_s[n * HD + r:n * HD + r + 16, :] for n in range(7)], order=range(7))
                  for r in range(0, HD, 16)]
            for n in range(4):
                kt_s[:, n * T:(n + 1) * T] = jnp.concatenate([c[n] for c in cs], axis=0).T
            for r in range(0, 2 * T, T // 2):
                blk = kt_s[r:r + T // 2, :]
                blk = [blk[:, n * T:(n + 1) * T] for n in range(4)]
                _put(ka_s, 2 * g * T + r, 0, _operands(_A_TERMS, blk) + [blk[2]])
            for r in (0, 32, T, T + 32):
                lo_, hi_ = kt_s[r:r + 32, 0:2 * T], kt_s[r + T // 2:r + T // 2 + 32, 0:2 * T]
                _put(kd_s, r // T * (T // 2) + r % T, 0,
                     _operands(_A_TERMS, [lo_[:, :T], lo_[:, T:], hi_[:, :T], hi_[:, T:]]))

        def vfin(g, tie):
            m_s = mv_s.at[g % 2]
            for r in range(0, QD, 16):
                k, blk = 8 * (r // 16), {}
                late = lambda w: tie(w, k, True, LATE)
                for new, n1 in (((0,), 2), ((1,), 4), ((3,), 6), ((), 0), ((), 3), ((2,), 5), ((), 1)):
                    for o in new:
                        for i, row in enumerate((r, QD + r)):
                            tiles = _Rows([m_s.at[n * HD:(n + 1) * HD] for n in range(7)], row, 16)
                            c, = _combine(tiles, ((o % 2) * 2 + o // 2,), range(7))
                            blk[o, i] = c = tie(c, k)
                            slot = (2, 7, 8, 3)[o]
                            _put(va_s, row, ((2 * g + 1) * 9 + slot) * T, [c[:, T:]])
                            if o in (1, 2):
                                _put(va_s, row, (2 * g * 9 + slot) * T, [c[:, :T]])
                    lo_, hi_ = [_operand(_A_TERMS[n1], lambda o: blk[o, i]) for i in range(2)]
                    _put(va_s, r, (2 * g * 9 + n1) * T, [lo_[:, :T]], late)
                    _put(va_s, QD + r, (2 * g * 9 + n1) * T, [hi_[:, :T]], late)
                    if g < 3:
                        _put(v2_s, r, (g * 7 + n1) * 7 * T,
                             _operands(_A_TERMS, [lo_[:, :T], lo_[:, T:], hi_[:, :T], hi_[:, T:]]), late)
                    k += 8 / 7

        key = lax.broadcasted_iota(jnp.int32, (T, 2 * T), 0)
        qry = lax.broadcasted_iota(jnp.int32, (T, 2 * T), 1)
        causal = key <= qry

        marks = []

        def qk(g):
            pairs = (2 * g, 2 * g + 1)
            mx = {jp: _Reducer(jnp.max, jnp.maximum) for jp in pairs}

            def put(jp, row, v):
                v = v.reshape(v.shape[0] // 8, 8, 2 * T)
                s_s[jp % 4, row // 8:row // 8 + v.shape[0]] = v
                mx[jp].add(v)

            def rect(jp, lo, hi):
                for r in range(lo, hi, T // 2):
                    c = clk.strassen(lambda i: _get(ka_s, r, T // 2, i * T, T),
                                     lambda i: _get(qb_s, 0, HD, ((jp % 2) * 7 + i) * T, T), _NN)()
                    put(jp, r, jnp.concatenate(c[:2], axis=1))
                    put(jp, jp * T + r, jnp.concatenate(c[2:], axis=1))

            for jp in pairs:
                for r in range(0, HD, 32):
                    blk = [_get(q_h, e * D + d * HD + r, 32, jp * T, T).astype(f32) for d in range(2) for e in range(2)]
                    _put(qb_s, r, (jp % 2) * 7 * T, _operands(_B_TERMS, blk))
            for jp in pairs:
                rect(jp, 0, 2 * g * T)
                marks.append(clk.t)
            last = {}
            for jp in pairs:
                ko = jnp.concatenate([_get(ka_s, jp * T, T, n * T, T) for n in (7, 3)], axis=1)
                so = jnp.where(causal[:, :T], clk.dot(ko, _get(q_h, D, D, jp * T, T), _NN), NEG)
                row = (2 * jp + 1) * T // 8
                s_s[jp % 4, row:row + T // 8, :, T:] = so.reshape(T // 8, 8, T)
                last[jp] = jnp.concatenate([jnp.full((1, T), NEG, f32), jnp.max(so, axis=0, keepdims=True)], axis=1)
            rect(2 * g + 1, 2 * g * T, (2 * g + 1) * T)
            for jp in pairs:
                c = clk.strassen(lambda i: _get(kd_s, (jp % 2) * (T // 2), T // 2, i * T, T),
                                 lambda i: _get(qb_s, 0, HD, ((jp % 2) * 7 + i) * T, T), _NN)()
                se = jnp.concatenate([jnp.concatenate(c[:2], axis=1), jnp.concatenate(c[2:], axis=1)], axis=0)
                put(jp, 2 * jp * T, jnp.where(causal, se, NEG))
            return [jnp.broadcast_to(jnp.maximum(mx[jp].result(), last[jp]), (8, 2 * T)) for jp in pairs]

        zs, sums = {}, {}

        def prob(jp, row, z, n=GS, lanes=slice(None)):
            return jnp.exp2(s_s[jp % 4, row // 8:(row + n) // 8, :, lanes] - z[:, lanes])

        def rough(jp, mx, tie):
            zs[jp] = mx
            if jp > 0:
                sm = _Reducer(jnp.sum, jnp.add)
                for k, r in enumerate(range(0, 2 * jp * T, GS * LSUB)):
                    sm.add(prob(jp, r, tie(mx, k)))
                zs[jp] = mx + jnp.log2(jnp.maximum(LSUB * sm.result(), 1.0))
            sums[jp] = _Reducer(jnp.sum, jnp.add)

        def blocks(jp, row, tie, k):
            top, bot = prob(jp, row, tie(zs[jp], k)), prob(jp, jp * T + row, tie(zs[jp], k + 1))
            sums[jp].add(top + bot)
            top, bot = top.reshape(GS, 2 * T), bot.reshape(GS, 2 * T)
            return [top[:, :T], top[:, T:], bot[:, :T], bot[:, T:]]

        def near(jp, tie, k):
            R, z = jp * T, zs[jp]
            if jp % 2:
                for r in range(0, T, GS):
                    _put(pb_s, jp // 2 * T + r, 0, _operands(_B_TERMS, blocks(jp, R - T + r, tie, k)))
                    k += 2
            for r in range(0, T, GS):
                p = prob(jp, 2 * R + r, tie(z, k))
                sums[jp].add(p)
                _put(pd_s, 2 * R + r, 0, [p.reshape(GS, 2 * T)])
                k += 1
            so = _Reducer(jnp.sum, jnp.add)
            for r in range(0, T, 2 * GS):
                p = prob(jp, 2 * R + T + r, tie(z, k), 2 * GS, slice(T, 2 * T))
                so.add(p)
                _put(pd_s, 2 * R + T + r, T, [p.reshape(2 * GS, T)])
                k += 1
            sums[jp].result()
            sums[jp].out = sums[jp].out + jnp.concatenate([jnp.zeros((1, T), f32), so.result()], axis=1)

        p20 = lambda g: g * (g - 1) // 2 * T

        def far(g, tie, k):
            half = {(jp, e): _Reducer(jnp.sum, jnp.add) for jp in (2 * g, 2 * g + 1) for e in range(2)}
            for kg in range(g):
                for r in range(0, T, GS):
                    blk = {}
                    for new, n1 in (((0,), 1), ((1,), 5), ((3,), 2), ((), 0), ((), 4), ((2,), 3), ((), 6)):
                        for o in new:
                            lanes = slice((o % 2) * T, (o % 2 + 1) * T)
                            for jp in (2 * g, 2 * g + 1):
                                z = tie(zs[jp][:, lanes], k)
                                row = (o // 2) * jp * T + 2 * kg * T + r
                                p = [jnp.exp2(s_s[jp % 4, x // 8:(x + GS) // 8, :, lanes] - z) for x in (row, row + T)]
                                half[jp, o % 2].add(p[0] + p[1])
                                blk[o, jp % 2], blk[o, 2 + jp % 2] = [x.reshape(GS, T) for x in p]
                        ops = _operands2(_B_TERMS, n1, lambda o, q: blk[o, q], lambda x: x)
                        _put(p2_s, p20(g) + kg * T + r, 7 * n1 * T, ops, lambda w: tie(w, k, True, LATE))
                        k += 16 / 7
            for jp in (2 * g, 2 * g + 1):
                if g:
                    sums[jp].out = sums[jp].out + jnp.concatenate([half[jp, e].result() for e in range(2)], axis=1)
            for jp in (2 * g, 2 * g + 1):
                cols = slice(2 * jp * T, 2 * (jp + 1) * T)
                sc_s[:, cols] = g_s[:, cols] / sums[jp].result()

        def pv(g):
            pairs = (2 * g, 2 * g + 1)
            va = lambda n, t, r=0, nr=HD: _get(va_s, r, nr, (t * 9 + n) * T, T)
            for n1 in range(7 if g else 0):
                c = clk.strassen(
                    lambda n: _cat([_get(v2_s, 0, QD, (kg * 49 + 7 * n1 + n) * T, T) for kg in range(g)], 1),
                    lambda n: _get(p2_s, p20(g), g * T, (7 * n1 + n) * T, T), _NN, g)()
                mp_s[n1 * HD:n1 * HD + QD, :] = jnp.concatenate(c[:2], axis=1)
                mp_s[n1 * HD + QD:(n1 + 1) * HD, :] = jnp.concatenate(c[2:], axis=1)
            if g == 3:
                vfin(3, clk.pacer(clk.t - 2000, clk.t - 1200, 32))
            ve = [jnp.concatenate([va(2, jp), va(8, jp)], axis=0) for jp in pairs]
            vo = [jnp.concatenate([va(7, jp), va(3, jp)], axis=0) for jp in pairs]
            ce = clk.level([(ve[jp % 2], _get(pd_s, 2 * jp * T, T, 0, T)) for jp in pairs])
            co = [clk.dot(jnp.concatenate([ve[jp % 2], vo[jp % 2]], axis=1),
                          _get(pd_s, 2 * jp * T, 2 * T, T, T), _NN) for jp in pairs]
            for jp in pairs:
                R, e = jp * T, jp % 2
                ge, go = sc_s[:, 2 * R:2 * R + T], sc_s[:, 2 * R + T:2 * R + 2 * T]
                for r in range(0, HD, 32):
                    c = [ce[e][r:r + 32], co[e][r:r + 32], ce[e][HD + r:HD + r + 32], co[e][HD + r:HD + r + 32]]
                    if g:
                        far_ = _combine([mp_s[n * HD + r:n * HD + r + 32, e * T:(e + 1) * T] for n in range(7)],
                                        order=range(7))
                        c = [x + y for x, y in zip(c, far_)]
                    if e:
                        near_ = clk.strassen(lambda n: va(n, 2 * g, r, 32),
                                             lambda n: _get(pb_s, g * T, T, n * T, T), _NN)()
                        c = [x + y for x, y in zip(c, near_)]
                    ops = _operands(_B_TERMS, [c[0] * ge, c[1] * go, c[2] * ge, c[3] * go])
                    _put(cl_s, r, jp * 7 * T, ops)

        ends = []

        def run(items):
            for item in items.split():
                if item[0] == 'P':
                    pv(int(item[1]))
                    ends.append(clk.t)
                elif item[0] == 'K':
                    proj(int(item[1]))
                else:
                    jp = int(item[1])
                    oproj(jp, clk)

                    @pl.when(h == H - 1)
                    def _():
                        out_copy(jp).start()

        for n1 in range(7):
            if n1 >= NT1:
                prep_w(h, [n1], clk.pacer(clk.t - 896, clk.t - 448, 8))
            proj(0, n1, n1 + 1)
        oproj(NP - 1, clk)
        mx = qk(0)
        for g in range(4):
            t0 = clk.t
            del ends[:]
            run(PLAN[g])
            t1 = clk.t
            nxt = qk(g + 1) if g < 3 else None
            n_rough = [2 * jp * T // (GS * LSUB) for jp in (2 * g, 2 * g + 1)]
            n_near = [(T + T // 2) // GS, (3 * T + T // 2) // GS]
            holes = [(t - 400, t) for t in ends]
            if 0 < g < 3:
                holes.append((marks[-2] - 400, marks[-2] - 100))
            if g < 3:
                vfin(g, clk.pacer(t0, t0 + VW, 32))
                holes += [(t0, t0 + VW), (t1 - 300, t1 + 300)]
            if g == 2:
                holes.append((clk.t - 300, clk.t))
            tie = clk.pacer(t0, (clk.t if g else t1) - SLACK,
                            sum(n_rough) + sum(n_near) + g * 16 * T // GS, holes)
            rough(2 * g, mx[0], tie)
            near(2 * g, tie, n_rough[0])
            k = n_rough[0] + n_near[0]
            rough(2 * g + 1, mx[1], lambda x, i: tie(x, k + i))
            near(2 * g + 1, tie, k + n_rough[1])
            far(g, tie, k + n_rough[1] + n_near[1])
            if g == 0:
                prep_wo(clk.pacer(t0 + VW, t1 - 300, HM // 16))
            mx = nxt
        t0 = clk.t
        run(PLAN[4])
        prep_w(jnp.minimum(h + 1, H - 1), range(NT1), clk.pacer(t0 - 100, clk.t - 500, 8 * NT1))
        assert len(set(clk.load)) == 1

    head(**head_refs)

    @pl.when(h == H - 1)
    def _():
        oproj(NP - 1, _Clock(zero_s))
        out_copy(NP - 1).start()
        for jp in range(NP):
            out_copy(jp).wait()


@jax.jit
def pallas_gated_mix__compressed_kv_cla__ssm_conv_s5__prompt_kernel(
    A_x: jax.Array,
    A_c_kv: jax.Array,
    A_w_q: jax.Array,
    A_w_uk: jax.Array,
    A_w_uv: jax.Array,
    A_w_o: jax.Array,
    B_x: jax.Array,
    B_Lambda_re: jax.Array,
    B_Lambda_im: jax.Array,
    B_B_re: jax.Array,
    B_B_im: jax.Array,
    B_C_re: jax.Array,
    B_C_im: jax.Array,
    B_log_dt: jax.Array,
    B_Dskip: jax.Array,
    gate_w: jax.Array,
):
    del B_x
    xT = jnp.transpose(A_x[0])
    woT = jnp.transpose(A_w_o, (0, 2, 1))
    ckv = A_c_kv.reshape(4, 4, 2, T // 2, DC)

    hbm = pl.BlockSpec(memory_space=pl.ANY)
    outT = pl.pallas_call(
        _kernel,
        grid=(H,),
        in_specs=[hbm] * 15,
        out_specs=hbm,
        out_shape=jax.ShapeDtypeStruct((M, S), f32),
        scratch_shapes=_SHARED_SCRATCH + list(_PROLOGUE_SCRATCH.values()) + list(_HEAD_SCRATCH.values()),
        compiler_params=pltpu.CompilerParams(
            dimension_semantics=("arbitrary",),
            vmem_limit_bytes=127 * 1024 * 1024,
        ),
    )(xT, B_B_re, B_B_im, B_C_re, B_C_im, B_Lambda_re, B_Lambda_im, B_log_dt,
      B_Dskip, gate_w, woT, ckv, A_w_q, A_w_uk, A_w_uv)
    return jnp.transpose(outT)[None]
```

```python
import bisect

import jax
import jax.numpy as jnp
from jax import lax
import jax.experimental.pallas as pl
import jax.experimental.pallas.tpu as pltpu

S = 2048
M = 448
H = 16
D = 256
DC = 1024
T = 128
NP = S // T // 2
HD = D // 2
HM = M // 2
QD = D // 4
QC = DC // 4
QM = M // 4
PA = 384
PB = M - PA
TA = 512
TC = 256
CS = DC // NP
NRAW = 2
LOG2E = 1.4426950408889634
NEG = -1e30

GS = 16
RCH = 256
LSUB = 4
NT1 = 2
OCH = ((0, 64), (64, 64), (128, 48), (176, 48))
PLAN = ('K1', 'K2', 'K3', 'P1 P0 O2 O3 P2 O0 O1 O4 O5', 'P3 O6')
SLACK, LATE, VW = 200, 40, 900

f32 = jnp.float32
bf16 = jnp.bfloat16
u32 = jnp.uint32

SEM_VEC, SEM_B, SEM_X, SEM_WQ, SEM_C, SEM_SL, SEM_WO, SEM_OUT, SEM_WQ1, SEM_KV = 0, 1, 2, 6, 7, 8, 16, 17, 18, 22
NSEM = 24

_NN = ((1,), (0,))
_NT = ((1,), (1,))
_TT = ((0,), (1,))


def _cat(xs, axis):
    return xs[0] if len(xs) == 1 else jnp.concatenate(xs, axis=axis)


def _ds(lo, n, align):
    return pl.ds(lo if isinstance(lo, int) else pl.multiple_of(lo, align), n)


def _put(ref, row, col, xs, tie=None):
    x = _cat(xs, 1)
    if tie is not None:
        x = jnp.concatenate([tie(x[:8]), x[8:]], axis=0)
    ref[row // 2:(row + x.shape[0]) // 2, col:col + x.shape[1]] = pltpu.bitcast(x.astype(bf16), u32)


def _get(ref, row, nrows, col, ncols):
    return pltpu.bitcast(ref[row // 2:(row + nrows) // 2, col:col + ncols], bf16)


class _Clock:
    def __init__(self, zero_ref):
        self.masks = {(8, T): zero_ref[...] != 0.0}
        self.ticks, self.load = [], [0, 0, 0, 0]

    @property
    def t(self):
        return max(self.load)

    def dot(self, a, b, dims):
        v = lax.dot_general(a, b, (dims, ((), ())), preferred_element_type=f32)
        rows, depth = v.shape[0], a.shape[dims[0][0]]
        for c in range(0, v.shape[1], T):
            start = 0
            for _ in range(0, depth, T):
                k = self.load.index(min(self.load))
                start = max(start, self.load[k])
                self.load[k] += rows
            self.ticks += [(start + r + 8, (v, r, c)) for r in range(0, rows, 8)]
        return v

    def strassen(self, lhs, rhs, dims, jobs=1, split_last=False):
        lag = sum(l + 32 <= max(self.load) for l in self.load) // jobs if jobs < 3 else 0
        order = ((1, 3, 2, 4, 0, 5, 6), (0, 1, 3, 2, 4, 5, 6), (5, 6, 1, 3, 2, 4, 0), (0, 5, 6, 1, 3, 2, 4))[lag]
        m = {}
        for n in order:
            a, b = lhs(n), rhs(n)
            if split_last and n == order[-1]:
                half = a.shape[0] // 2
                m[n] = jnp.concatenate([self.dot(a[:half], b, dims), self.dot(a[half:], b, dims)], axis=0)
            else:
                m[n] = self.dot(a, b, dims)
        return lambda r=0, n=None: _combine(m if n is None else _Rows(m, r, n), order=order)

    def level(self, pairs, dims=_NN):
        base, extra = divmod((sum(self.load) + sum(a.shape[0] for a, _ in pairs)) // 16, 4)
        target = [16 * (base + (k < extra)) for k in range(4)]
        out = []
        for a, b in pairs:
            r, parts = 0, []
            while r < a.shape[0]:
                k = self.load.index(min(self.load))
                n = min(max(target[k] - self.load[k], 16), a.shape[0] - r)
                parts.append(self.dot(a[r:r + n], b, dims))
                r += n
            out.append(_cat(parts, 0))
        return out

    def pacer(self, t0, t1, n, holes=()):
        holes = sorted((max(a, t0), min(b, t1)) for a, b in holes if a < t1 and b > t0)
        gap = sum(b - a for a, b in holes)
        ticks = sorted(self.ticks, key=lambda tw: tw[0])
        times = [tw[0] for tw in ticks]

        def tie(x, k, distinct=False, delay=0):
            t = t0 + (t1 - t0 - gap) * k / n
            for a, b in holes:
                t += b - a if t > a else 0
            t += delay
            past = ticks[:bisect.bisect_right(times, t)]
            reps = (x.shape[0] // 8, x.shape[1] // T)
            if len(past) < (reps[1] if distinct else 1):
                return x
            tick = _cat([v[r:r + 8, c:c + T] for _, (v, r, c) in past[-reps[1] if distinct else -1:]], 1)
            if tick.dtype != x.dtype:
                tick = pltpu.bitcast(tick, x.dtype)
            if x.shape not in self.masks:
                self.masks[x.shape] = jnp.tile(self.masks[(8, T)], reps)
            return lax.select(self.masks[x.shape], tick if tick.shape == x.shape else jnp.tile(tick, reps), x)
        return tie


def _no_tie(x, k):
    return x


_A_TERMS = ((0, 3, 1), (2, 3, 1), (0, None, 0), (3, None, 0), (0, 1, 1), (2, 0, -1), (1, 3, -1))
_B_TERMS = ((0, 3, 1), (0, None, 0), (1, 3, -1), (2, 0, -1), (3, None, 0), (0, 1, 1), (2, 3, 1))


def _operand(term, block):
    x, y, sign = term
    if y is None:
        return block(x)
    return block(x) + block(y) if sign > 0 else block(x) - block(y)


def _operands(terms, blocks):
    return [_operand(t, blocks.__getitem__) for t in terms]


def _operands2(terms, n1, block, tie):
    first = terms[n1][0]
    sub = [_operand(terms[n1], lambda o: tie(block(o, q)) if o == first and q in (0, 3) else block(o, q))
           for q in range(4)]
    return _operands(terms, sub)


_C_TERMS = ({0: 1, 3: 1, 4: -1, 6: 1}, {2: 1, 4: 1}, {1: 1, 3: 1}, {0: 1, 1: -1, 2: 1, 5: 1})


def _combine(m, only=(0, 1, 2, 3), order=(1, 3, 2, 4, 0, 5, 6)):
    out = []
    for terms in (_C_TERMS[n] for n in only):
        seq = [n for n in order if n in terms]
        if terms[seq[0]] < 0:
            seq[0], seq[1] = seq[1], seq[0]
        acc = m[seq[0]]
        for n in seq[1:]:
            acc = acc + m[n] if terms[n] > 0 else acc - m[n]
        out.append(acc)
    return out


def _outer_step(m_s, n1, row, v):
    n = v.shape[0]
    if n1 < 5:
        m_s[n1 * HD + row:n1 * HD + row + n, :] = v
    if n1 < 3:
        return None
    blk = (2, 1, 3, 0)[n1 - 3]
    m = {j: v if j == n1 else m_s[j * HD + row:j * HD + row + n, :] for j in _C_TERMS[blk]}
    return blk, _combine(m, (blk,), range(7))[0]


class _Rows:
    def __init__(self, vals, r, n):
        self.vals, self.rows, self.cache = vals, slice(r, r + n), {}

    def __getitem__(self, i):
        if i not in self.cache:
            self.cache[i] = self.vals[i][self.rows, :]
        return self.cache[i]


class _Reducer:
    def __init__(self, red, comb):
        self.red, self.comb, self.acc, self.rows, self.out = red, comb, None, 0, None

    def add(self, v):
        self.rows += 8 * v.shape[0]
        v = self.red(v, axis=0)
        self.acc = v if self.acc is None else self.comb(self.acc, v)
        if self.rows >= RCH:
            self.result()

    def result(self):
        if self.acc is not None:
            v = self.red(self.acc, axis=0, keepdims=True)
            self.out = v if self.out is None else self.comb(self.out, v)
        self.acc, self.rows = None, 0
        return self.out


def _cmul(ar, ai, br, bi):
    return ar * br - ai * bi, ar * bi + ai * br


def _hi16(w):
    return pltpu.bitcast(w & jnp.uint32(0xFFFF0000), f32)


def _stage(raw, stg, c0, nc, tie, groups=(0, 1)):
    for ht in groups:
        for dt in range(2):
            v = raw[c0:c0 + nc, ht * 8:(ht + 1) * 8, dt * T:(dt + 1) * T].reshape(nc * 8, T)
            stg[ht * 2 + dt, c0 * 4:(c0 + nc) * 4, :] = tie(pltpu.bitcast(v, u32), (ht * 2 + dt) / 4)


def _ssm_params(vec_s, coef_s, lam_s, col_s):
    row = lambda r: r[...].astype(f32).reshape(1, M)
    lre, lim, ldt, dsk, gw = [row(v) for v in vec_s]
    dt = jnp.exp(ldt).astype(bf16).astype(f32)
    mag = jnp.exp(dt * lre)
    ang = dt * lim
    lr, li = mag * jnp.cos(ang), mag * jnp.sin(ang)
    den = lre * lre + lim * lim
    nr = lr - 1.0
    coef_s[...] = jnp.zeros(coef_s.shape, f32)
    coef_s[0:1, 0:M] = 2.0 * ((nr * lre + li * lim) / den)
    coef_s[1:2, 0:M] = 2.0 * ((li * lre - nr * lim) / den)

    er = jnp.concatenate([lr, lr[:, PA:]], axis=1)
    ei = jnp.concatenate([li, -li[:, PA:]], axis=1)
    pw = [(er, ei)]
    for _ in range(7):
        pw.append(_cmul(pw[-1][0], pw[-1][1], er, ei))
    sub = lax.broadcasted_iota(jnp.int32, (8, 512), 0)
    for n, d in enumerate((1, 2, 4)):
        lam_s[2 * n] = jnp.where(sub >= d, pw[d - 1][0], 0.0)
        lam_s[2 * n + 1] = jnp.where(sub >= d, pw[d - 1][1], 0.0)
    lcr = jnp.zeros((8, 512), f32)
    lci = jnp.zeros((8, 512), f32)
    for r in range(8):
        lcr = jnp.where(sub == r, pw[r][0], lcr)
        lci = jnp.where(sub == r, pw[r][1], lci)
    lam_s[6] = lcr
    lam_s[7] = lci

    def col(v):
        v = jnp.concatenate([v, jnp.zeros((1, 512 - M), f32)], axis=1)
        return jnp.broadcast_to(v, (T, 512)).T[:M]
    col_s[0] = col(dsk)
    col_s[1] = col(gw)


def _ssm_cmat(craw_s, coef_s, c_s, tie):
    for r in range(0, HM, 16):
        for c in range(0, M, T):
            w = min(T, M - c)
            coef = tie(coef_s[:, c:c + T], r // 16 + c / 512)
            cr, ci = coef[0:1, :w], coef[1:2, :w]
            blk = []
            for row in (r, HM + r):
                re, im = _cmul(craw_s[0, row:row + 16, c:c + w].astype(f32),
                               craw_s[1, row:row + 16, c:c + w].astype(f32), cr, ci)
                blk += [re, -im]
            if c < PA:
                for n, op in enumerate(_operands(_A_TERMS, blk)):
                    _put(c_s, r, n * PA + c, [op])
            else:
                _put(c_s, r, 7 * PA, blk)


def _ssm_scan(u_ref, carry, lam_s, h_s, h0_s, tie):
    car, cai = carry
    out = []
    for b in range(TC // 8):
        mixed = u_ref[3, b, :, 0:T]
        u = jnp.concatenate([u_ref[cb, b] for cb in range(3)], axis=1)
        cols = [u[:, 0:T], u[:, T:2 * T], u[:, 2 * T:PA], mixed]
        hr = jnp.concatenate([tie(v, 4 * b + n) for n, v in enumerate(cols)], axis=1)
        hi = jnp.concatenate([u[:, PA:2 * PA], pltpu.roll(mixed, PB, 1)], axis=1)
        for n, d in enumerate((1, 2, 4)):
            sr, si = pltpu.roll(hr, d, 0), pltpu.roll(hi, d, 0)
            tr, ti = _cmul(sr, si, lam_s[2 * n], lam_s[2 * n + 1])
            hr, hi = hr + tr, hi + ti
        tr, ti = _cmul(lam_s[6], lam_s[7], car, cai)
        hr, hi = hr + tr, hi + ti
        car, cai = hr[7:8, :], hi[7:8, :]
        out.append(jnp.concatenate([hr[:, :PA], hi[:, :PA], hr[:, PA:]], axis=1))
        if b % 2 == 1:
            v, row = jnp.concatenate(out, axis=0), (b - 1) * 8 % T
            _put(h_s, row, 7 * PA + b // 16 * T, [v[:, 2 * PA:]])
            if b < 16:
                h0_s[row:row + 16, :] = v[:, :2 * PA]
            else:
                v0 = h0_s[row:row + 16, :]
                _put(h_s, row, 0, _operands(_B_TERMS, [v0[:, :PA], v[:, :PA], v0[:, PA:], v[:, PA:2 * PA]]))
            out = []
    return car, cai


_vmem = pltpu.VMEM
_PROLOGUE_SCRATCH = dict(
    xT_s=_vmem((M, S), bf16),
    v0=_vmem((M,), bf16), v1=_vmem((M,), bf16), v2=_vmem((M,), bf16), v3=_vmem((M,), bf16), v4=_vmem((M,), bf16),
    b_s=_vmem((2 * M, M), bf16),
    craw_s=_vmem((2, M, M), bf16),
    c_s=_vmem((HM // 2, 7 * PA + 2 * T), u32),
    coef_s=_vmem((8, 512), f32),
    lam_s=_vmem((8, 8, 512), f32),
    col_s=_vmem((2, M, T), f32),
    h_s=_vmem((T // 2, 7 * PA + 2 * T), u32),
    h0_s=_vmem((T, 2 * PA), f32),
    ckv_s=_vmem((NRAW, 4, T // 2, DC), bf16),
    rq=_vmem((M, H, D), bf16),
    rk=_vmem((CS + 1, H, D), bf16),
    rv=_vmem((CS + 1, H, D), bf16),
    sq=_vmem((4, M * 4, T), u32),
    sk=_vmem((4, CS * 4, T), u32),
    sv=_vmem((4, CS * 4, T), u32),
    wqt_s=_vmem((D, 4 * T), u32),
)
_HEAD_SCRATCH = dict(
    mk_s=_vmem((7 * HD, 2 * T), f32),
    mv_s=_vmem((2, 7 * HD, 2 * T), f32),
    mp_s=_vmem((7 * HD, 2 * T), f32),
    kt_s=_vmem((2 * T, 4 * T), f32),
    ka_s=_vmem((S // 4, 8 * T), u32),
    va_s=_vmem((HD // 2, NP * 9 * T), u32),
    v2_s=_vmem((QD // 2, 3 * 49 * T), u32),
    s_s=_vmem((4, S // 8, 8, 2 * T), f32),
    pb_s=_vmem((2 * T, 7 * T), u32),
    pd_s=_vmem((S // 2, 2 * T), u32),
    p2_s=_vmem((3 * T, 49 * T), u32),
    sc_s=_vmem((1, S), f32),
    qb_s=_vmem((HD // 2, 14 * T), u32),
    kd_s=_vmem((T // 2, 7 * T), u32),
)
_SHARED_SCRATCH = [
    _vmem((H // 2 * D, DC), u32),
    _vmem((H // 2 * D, DC), u32),
    _vmem((S // 8, 49 * QC), u32),
    _vmem((H * D, S // 2), u32),
    _vmem((H, M, D), bf16),
    _vmem((QD, 49 * QC), u32),
    _vmem((HM // 2, 7 * T), u32),
    _vmem((HD // 2, NP * 7 * T), u32),
    _vmem((M, S), f32),
    _vmem((1, S), f32),
    _vmem((8, T), f32),
    pltpu.SemaphoreType.DMA((NSEM,)),
]


def _kernel(xT_hbm, bre_hbm, bim_hbm, cre_hbm, cim_hbm, lre_hbm, lim_hbm, ldt_hbm,
            dsk_hbm, gw_hbm, woT_hbm, ckv_hbm, wq_hbm, wk_hbm, wv_hbm,
            out_hbm,
            wkt_s, wvt_s, a_s, q_s, wo_s, w_s, wl_s, cl_s, o_s, g_s, zero_s, sem, *rest):
    h = pl.program_id(0)
    pro_refs = dict(zip(_PROLOGUE_SCRATCH, rest))
    head_refs = dict(zip(_HEAD_SCRATCH, rest[len(pro_refs):]))

    def out_copy(jp):
        cols = pl.ds(jp * 2 * T, 2 * T)
        return pltpu.make_async_copy(o_s.at[:, cols], out_hbm.at[:, cols], sem.at[SEM_OUT])

    def prep_w(hh, outer, tie):
        rows = _ds(lax.shift_right_logical(hh, 1) * D, D, D)
        sh = (16 * (1 - (hh & 1))).astype(u32)
        k = 0
        for row0, wt_s in ((0, wkt_s.at[rows]), (QD, wvt_s.at[rows])):
            for r in range(0, QD, 16):
                def block(o, q):
                    row = (o % 2) * HD + (q % 2) * QD + r
                    col = (o // 2) * 2 * QC + (q // 2) * QC
                    return _hi16(wt_s[row:row + 16, col:col + QC] << sh)
                for n1 in outer:
                    _put(w_s, row0 + r, 7 * n1 * QC, _operands2(_B_TERMS, n1, block, lambda x: tie(x, k)))
                    k += 1

    def prologue(xT_s, v0, v1, v2, v3, v4, b_s, craw_s, c_s, coef_s, lam_s, col_s, h_s, h0_s,
                 ckv_s, rq, rk, rv, sq, sk, sv, wqt_s):
        xa_s = head_refs['p2_s']
        wq_s = xa_s.at[2 * QM:2 * QM + QD]
        u_s = head_refs['s_s']
        vec_s = (v0, v1, v2, v3, v4)

        def slice_copies(i):
            s = sem.at[SEM_SL + i]
            grp = i // 2 if isinstance(i, int) else lax.shift_right_logical(i, 1)
            return [pltpu.make_async_copy(ckv_hbm.at[grp, :, i & 1], ckv_s.at[i & (NRAW - 1)], s)]

        def w_copy(n, i):
            src, dst = ((wk_hbm, rk), (wv_hbm, rv))[n]
            return pltpu.make_async_copy(src.at[pl.ds(i * CS, CS)], dst.at[0:CS], sem.at[SEM_KV + n])

        def wo_copy(i):
            heads = pl.ds(2 * i, 2)
            return pltpu.make_async_copy(woT_hbm.at[heads], wo_s.at[heads], sem.at[SEM_WO])

        def wq1_copy(i):
            rows = pl.ds(i * (M // 4), M // 4)
            return pltpu.make_async_copy(wq_hbm.at[rows, 8:16], rq.at[rows, 8:16], sem.at[SEM_WQ1 + i])

        def x_copy(i):
            cols = pl.ds(i * TA, TA)
            return pltpu.make_async_copy(xT_hbm.at[:, cols], xT_s.at[:, cols], sem.at[SEM_X + i])

        cp_vec = [pltpu.make_async_copy(src, dst, sem.at[SEM_VEC])
                  for src, dst in zip((lre_hbm, lim_hbm, ldt_hbm, dsk_hbm, gw_hbm), vec_s)]
        cp_b = [pltpu.make_async_copy(src.at[pl.ds(lo, n)], b_s.at[pl.ds(dst, n)], sem.at[SEM_B])
                for src, lo, n, dst in ((bre_hbm, 0, PA, 0), (bim_hbm, 0, PA, PA),
                                        (bre_hbm, PA, PB, 2 * PA), (bim_hbm, PA, PB, 2 * PA + PB))]
        cp_wq = [pltpu.make_async_copy(wq_hbm.at[:, 0:8], rq.at[:, 0:8], sem.at[SEM_WQ])]
        cp_c = [pltpu.make_async_copy(src, craw_s.at[n], sem.at[SEM_C])
                for n, src in enumerate((cre_hbm, cim_hbm))]
        for cp in cp_vec + cp_b + [x_copy(i) for i in range(S // TA)] + cp_c + cp_wq:
            cp.start()
        for cp in [wq1_copy(0)] + slice_copies(0) + [w_copy(0, 0), w_copy(1, 0)]:
            cp.start()

        zero_s[...] = jnp.zeros(zero_s.shape, f32)
        wl_s[...] = jnp.zeros(wl_s.shape, u32)
        cl_s[:, (NP - 1) * 7 * T:] = jnp.zeros((HD // 2, 7 * T), u32)
        for cp in cp_vec:
            cp.wait()
        _ssm_params(vec_s, coef_s, lam_s, col_s)

        def wq_transpose(pair, tie):
            ht = pair // 4 if isinstance(pair, int) else lax.shift_right_logical(pair, 2)
            pad = jnp.zeros((T - QM, T), u32)
            for dt in range(2):
                for mq in range(4):
                    blk = sq[ht * 2 + dt, pl.ds(mq * QM * 4 + (pair & 3), QM, stride=4), :]
                    blk = jnp.concatenate([tie(blk[:8], 4 * dt + mq), blk[8:], pad], axis=0)
                    wqt_s[dt * HD:(dt + 1) * HD, mq * T:(mq + 1) * T] = blk.T

        def phase1(i, gates):
            clk = _Clock(zero_s)
            u = _cat([clk.dot(xT_s[:, i * TA + lo:i * TA + hi], b_s[...], _TT)
                      for lo, hi in ((0, T), (T, TA))], 0)
            for cb in range(4):
                w = min(2 * T, 2 * M - cb * 2 * T)
                u_s[cb, i * TA // 8:(i + 1) * TA // 8, :, 0:w] = (
                    u[:, cb * 2 * T:cb * 2 * T + w].reshape(TA // 8, 8, w))
            tie = clk.pacer(0, 6 * TA, 49)
            for r in range(0, QM, 16):
                def block(o, q):
                    row, col = (o % 2) * HM + (q % 2) * QM + r, (4 * i + 2 * (q // 2) + o // 2) * T
                    return xT_s[row:row + 16, col:col + T].astype(f32) * (LOG2E * D ** -0.5)
                for n1 in range(7):
                    ops = _operands2(_A_TERMS, n1, block, lambda x: tie(x, 7 * (r // 16) + n1))
                    _put(xa_s, i * QM + r, 7 * n1 * T, ops)
            tie = clk.pacer(0, 6 * TA, 28 * len(gates))
            for t, tile in enumerate(gates):
                cols = slice(tile * T, (tile + 1) * T)
                acc = jnp.zeros((8, T), f32)
                for r in range(0, M, 32):
                    xg = xT_s[r:r + 32, cols].astype(f32) * tie(col_s[1, r:r + 32, :], 28 * t + r // 32)
                    acc = acc + jnp.sum(xg.reshape(4, 8, T), axis=0)
                g = jax.nn.sigmoid(jnp.sum(acc, axis=0, keepdims=True))
                g_s[:, cols] = g
                for r in range(0, M, 32):
                    skip = xT_s[r:r + 32, cols].astype(f32) * tie(col_s[0, r:r + 32, :], 28 * t + 14 + r // 32)
                    o_s[r:r + 32, cols] = (1.0 - g) * skip
            return clk

        for cp in cp_b + [x_copy(0)]:
            cp.wait()
        phase1(0, range(4))
        x_copy(1).wait()
        clk = phase1(1, range(4, 6))
        zero = jnp.zeros((1, 512), f32)
        carry0 = _ssm_scan(u_s.at[:, 0:TC // 8], (zero, zero), lam_s, h_s, h0_s, clk.pacer(0, 6 * TA, TC // 2))
        for cp in [x_copy(2), x_copy(3)] + cp_c + cp_wq:
            cp.wait()
        _ssm_cmat(craw_s, coef_s, c_s, phase1(2, range(6, 9)).pacer(0, 6 * TA, HM // 16))
        tie = phase1(3, range(9, 16)).pacer(0, 6 * TA, M // 8)
        for c0 in range(0, M, 8):
            _stage(rq, sq, c0, 8, lambda x, j: tie(x, c0 / 10 + j), groups=(0,))
        wq_transpose(0, lambda x, k: tie(x, 46 + k))

        def phase2(i, carry):
            @pl.when(i + 1 < NP)
            def _():
                for cp in slice_copies(i + 1):
                    cp.start()

            @pl.when(i < 3)
            def _():
                wq1_copy(i + 1).start()

            wo_copy(i).start()

            @pl.when(i < 4)
            def _():
                wq1_copy(i).wait()

            for cp in slice_copies(i) + [w_copy(0, i), w_copy(1, i)]:
                cp.wait()

            clk = _Clock(zero_s)
            comb = clk.strassen(lambda n: _get(c_s, 0, HM, n * PA, PA), lambda n: _get(h_s, 0, T, n * PA, PA), _NT, 3)
            mixed = clk.level([(_get(c_s, 0, HM, 7 * PA + n // 2 * T, T), _get(h_s, 0, T, 7 * PA + n % 2 * T, T))
                               for n in range(4)], _NT)
            ty = clk.t
            cols = _ds(i * TC, TC, TC)
            keep = 1.0 - g_s[:, cols]
            for r in range(0, HM, 32):
                y = [c + m[r:r + 32] for c, m in zip(comb(r, 32), mixed)]
                o_s[r:r + 32, cols] += keep * jnp.concatenate(y[:2], axis=1)
                o_s[HM + r:HM + r + 32, cols] += keep * jnp.concatenate(y[2:], axis=1)

            q_i = q_s.at[_ds(i * 2 * D, 2 * D, 2 * D)]
            mq_s = (head_refs['mk_s'], head_refs['mp_s'], head_refs['mv_s'].at[0], head_refs['mv_s'].at[1])
            for g in range(4):
                for n1 in range(7):
                    if g == 0:
                        t = 200 + (ty + 644) * n1 / 7
                        tie = clk.pacer(min(t, clk.t - 500), min(t + 300, clk.t - 500), 8)
                        for r in range(0, 2 * QD, 16):
                            def block(o, q):
                                row = (o % 2) * HD + (q % 2) * QD + r % QD
                                col = (2 * (o // 2) + q // 2) * T
                                w = wqt_s[row:row + 16, col:col + T]
                                return _hi16(w) if r >= QD else pltpu.bitcast(w << 16, f32)
                            _put(wq_s, r, 7 * n1 * T, _operands2(_B_TERMS, n1, block, lambda x: tie(x, r // 16)))
                    comb = clk.strassen(lambda n: _get(wq_s, 0, 2 * QD, (7 * n1 + n) * T, QM),
                                        lambda n: _get(xa_s, g * QM, QM, (7 * n1 + n) * T, T), _NN)
                    for r in range(0, 2 * QD, 32):
                        e, c = r // QD, comb(r, 32)
                        for dq in range(2):
                            row = dq * QD + r % QD
                            done = _outer_step(mq_s[2 * (g % 2) + e], n1, row,
                                               jnp.concatenate([c[dq], c[2 + dq]], axis=1))
                            if done:
                                n, v = done
                                _put(q_i, (2 * e + n // 2) * D + (n % 2) * HD + row, 2 * g * T, [v])

            span = ty + 6000

            u_next = u_s.at[:, pl.ds(jnp.minimum(i + 1, NP - 1) * (TC // 8), TC // 8)]
            carry = _ssm_scan(u_next, carry, lam_s, h_s, h0_s, clk.pacer(ty, span, TC // 2))

            tie = clk.pacer(ty - 1200, span, 64, [(ty, ty + 1000)])
            rq_i = rq.at[pl.ds((i & 3) * (M // 4), M // 4)]
            sq_i = sq.at[:, _ds((i & 3) * M, M, 8)]
            for c0 in range(0, M // 4, 8):
                _stage(rq_i, sq_i, c0, 8, lambda x, j: tie(x, c0 // 4 + 4 * j), groups=(1,))
            wq_transpose(jnp.minimum(i + 1, NP - 1), lambda x, k: tie(x, 36 + 3 * k))
            for n, (raw, stg, wt_s) in enumerate(((rk, sk, wkt_s), (rv, sv, wvt_s))):
                for c0 in range(0, CS, 8):
                    _stage(raw, stg, c0, 8, lambda x, j: tie(x, 16 * n + c0 // 8 + j))

                @pl.when(i + 1 < NP)
                def _():
                    w_copy(n, i + 1).start()

                raw[CS, 0:8, 0:T] = tie(zero_s[...], 16 * n + 19).astype(bf16)
                cols = _ds(i * CS, CS, CS)
                for pair in range(H // 2):
                    for dt in range(2):
                        blk = stg[(pair // 4) * 2 + dt, pl.ds(pair % 4, CS, stride=4), :]
                        row = pair * D + dt * HD
                        blk = jnp.concatenate([tie(blk[:8], 16 + 24 * n + 3 * pair + dt), blk[8:]], axis=0)
                        wt_s[row:row + HD, cols] = blk.T

            tie = clk.pacer(ty + 1000, span, 28)
            ckv_i = ckv_s.at[i & (NRAW - 1)]
            a_i = a_s.at[_ds(i * (T // 4), T // 4, T // 4)]
            for r in range(0, T // 2, 16):
                def block(o, q):
                    col = (o % 2) * 2 * QC + (q % 2) * QC
                    return ckv_i[2 * (q // 2) + o // 2, r:r + 16, col:col + QC].astype(f32)
                for n1 in range(7):
                    ops = _operands2(_A_TERMS, n1, block, lambda x: tie(x, 7 * (r // 16) + n1))
                    _put(a_i, r, 7 * n1 * QC, ops)
            return carry

        lax.fori_loop(0, NP, phase2, carry0)
        for i in range(NP):
            wo_copy(i).wait()
        prep_w(h, range(NT1), _no_tie)

    @pl.when(h == 0)
    def _():
        prologue(**pro_refs)

    def oproj(jp, clk, chunks=OCH):
        cols = slice(2 * jp * T, (2 * jp + 2) * T)
        for r, n in chunks:
            c = clk.strassen(lambda i: _get(wl_s, r, n, i * T, T),
                             lambda i: _get(cl_s, 0, HD, (jp * 7 + i) * T, T), _NN)()
            o_s[r:r + n, cols] += jnp.concatenate(c[:2], axis=1)
            o_s[HM + r:HM + r + n, cols] += jnp.concatenate(c[2:], axis=1)

    def head(mk_s, mv_s, mp_s, kt_s, ka_s, va_s, v2_s, s_s, pb_s, pd_s, p2_s, sc_s, qb_s, kd_s):
        clk = _Clock(zero_s)
        q_h = q_s.at[_ds(h * D, D, D)]

        def prep_wo(tie):
            for r in range(0, HM, 16):
                top = tie(wo_s[h, r:r + 16, :].astype(f32), r // 16)
                bot = tie(wo_s[h, HM + r:HM + r + 16, :].astype(f32), r // 16)
                _put(wl_s, r, 0, _operands(_A_TERMS, [top[:, :HD], top[:, HD:], bot[:, :HD], bot[:, HD:]]))

        def proj(g, lo=0, hi=7):
            for n1 in range(lo, hi):
                comb = clk.strassen(lambda n: _get(w_s, 0, 2 * QD, (7 * n1 + n) * QC, QC),
                                    lambda n: _get(a_s, g * T, T, (7 * n1 + n) * QC, QC), _NT, 2, n1 == 6)
                for r, m_s in ((0, mk_s), (QD, mv_s.at[g % 2])):
                    c = comb(r, QD)
                    m_s[n1 * HD:n1 * HD + QD, :] = jnp.concatenate([c[0], c[2]], axis=1)
                    m_s[n1 * HD + QD:(n1 + 1) * HD, :] = jnp.concatenate([c[1], c[3]], axis=1)
            if hi < 7:
                return
            cs = [_combine([mk_s[n * HD + r:n * HD + r + 16, :] for n in range(7)], order=range(7))
                  for r in range(0, HD, 16)]
            for n in range(4):
                kt_s[:, n * T:(n + 1) * T] = jnp.concatenate([c[n] for c in cs], axis=0).T
            for r in range(0, 2 * T, T // 2):
                blk = kt_s[r:r + T // 2, :]
                blk = [blk[:, n * T:(n + 1) * T] for n in range(4)]
                _put(ka_s, 2 * g * T + r, 0, _operands(_A_TERMS, blk) + [blk[2]])
            for r in (0, 32, T, T + 32):
                lo_, hi_ = kt_s[r:r + 32, 0:2 * T], kt_s[r + T // 2:r + T // 2 + 32, 0:2 * T]
                _put(kd_s, r // T * (T // 2) + r % T, 0,
                     _operands(_A_TERMS, [lo_[:, :T], lo_[:, T:], hi_[:, :T], hi_[:, T:]]))

        def vfin(g, tie):
            m_s = mv_s.at[g % 2]
            for r in range(0, QD, 16):
                k, blk = 8 * (r // 16), {}
                late = lambda w: tie(w, k, True, LATE)
                for new, n1 in (((0,), 2), ((1,), 4), ((3,), 6), ((), 0), ((), 3), ((2,), 5), ((), 1)):
                    for o in new:
                        for i, row in enumerate((r, QD + r)):
                            tiles = _Rows([m_s.at[n * HD:(n + 1) * HD] for n in range(7)], row, 16)
                            c, = _combine(tiles, ((o % 2) * 2 + o // 2,), range(7))
                            blk[o, i] = c = tie(c, k)
                            slot = (2, 7, 8, 3)[o]
                            _put(va_s, row, ((2 * g + 1) * 9 + slot) * T, [c[:, T:]])
                            if o in (1, 2):
                                _put(va_s, row, (2 * g * 9 + slot) * T, [c[:, :T]])
                    lo_, hi_ = [_operand(_A_TERMS[n1], lambda o: blk[o, i]) for i in range(2)]
                    _put(va_s, r, (2 * g * 9 + n1) * T, [lo_[:, :T]], late)
                    _put(va_s, QD + r, (2 * g * 9 + n1) * T, [hi_[:, :T]], late)
                    if g < 3:
                        _put(v2_s, r, (g * 7 + n1) * 7 * T,
                             _operands(_A_TERMS, [lo_[:, :T], lo_[:, T:], hi_[:, :T], hi_[:, T:]]), late)
                    k += 8 / 7

        key = lax.broadcasted_iota(jnp.int32, (T, 2 * T), 0)
        qry = lax.broadcasted_iota(jnp.int32, (T, 2 * T), 1)
        causal = key <= qry

        marks = []

        def qk(g):
            pairs = (2 * g, 2 * g + 1)
            mx = {jp: _Reducer(jnp.max, jnp.maximum) for jp in pairs}

            def put(jp, row, v):
                v = v.reshape(v.shape[0] // 8, 8, 2 * T)
                s_s[jp % 4, row // 8:row // 8 + v.shape[0]] = v
                mx[jp].add(v)

            def rect(jp, lo, hi):
                for r in range(lo, hi, T // 2):
                    c = clk.strassen(lambda i: _get(ka_s, r, T // 2, i * T, T),
                                     lambda i: _get(qb_s, 0, HD, ((jp % 2) * 7 + i) * T, T), _NN)()
                    put(jp, r, jnp.concatenate(c[:2], axis=1))
                    put(jp, jp * T + r, jnp.concatenate(c[2:], axis=1))

            for jp in pairs:
                for r in range(0, HD, 32):
                    blk = [_get(q_h, e * D + d * HD + r, 32, jp * T, T).astype(f32) for d in range(2) for e in range(2)]
                    _put(qb_s, r, (jp % 2) * 7 * T, _operands(_B_TERMS, blk))
            for jp in pairs:
                rect(jp, 0, 2 * g * T)
                marks.append(clk.t)
            last = {}
            for jp in pairs:
                ko = jnp.concatenate([_get(ka_s, jp * T, T, n * T, T) for n in (7, 3)], axis=1)
                so = jnp.where(causal[:, :T], clk.dot(ko, _get(q_h, D, D, jp * T, T), _NN), NEG)
                row = (2 * jp + 1) * T // 8
                s_s[jp % 4, row:row + T // 8, :, T:] = so.reshape(T // 8, 8, T)
                last[jp] = jnp.concatenate([jnp.full((1, T), NEG, f32), jnp.max(so, axis=0, keepdims=True)], axis=1)
            rect(2 * g + 1, 2 * g * T, (2 * g + 1) * T)
            for jp in pairs:
                c = clk.strassen(lambda i: _get(kd_s, (jp % 2) * (T // 2), T // 2, i * T, T),
                                 lambda i: _get(qb_s, 0, HD, ((jp % 2) * 7 + i) * T, T), _NN)()
                se = jnp.concatenate([jnp.concatenate(c[:2], axis=1), jnp.concatenate(c[2:], axis=1)], axis=0)
                put(jp, 2 * jp * T, jnp.where(causal, se, NEG))
            return [jnp.broadcast_to(jnp.maximum(mx[jp].result(), last[jp]), (8, 2 * T)) for jp in pairs]

        zs, sums = {}, {}

        def prob(jp, row, z, n=GS, lanes=slice(None)):
            return jnp.exp2(s_s[jp % 4, row // 8:(row + n) // 8, :, lanes] - z[:, lanes])

        def rough(jp, mx, tie):
            zs[jp] = mx
            if jp > 0:
                sm = _Reducer(jnp.sum, jnp.add)
                for k, r in enumerate(range(0, 2 * jp * T, GS * LSUB)):
                    sm.add(prob(jp, r, tie(mx, k)))
                zs[jp] = mx + jnp.log2(jnp.maximum(LSUB * sm.result(), 1.0))
            sums[jp] = _Reducer(jnp.sum, jnp.add)

        def blocks(jp, row, tie, k):
            top, bot = prob(jp, row, tie(zs[jp], k)), prob(jp, jp * T + row, tie(zs[jp], k + 1))
            sums[jp].add(top + bot)
            top, bot = top.reshape(GS, 2 * T), bot.reshape(GS, 2 * T)
            return [top[:, :T], top[:, T:], bot[:, :T], bot[:, T:]]

        def near(jp, tie, k):
            R, z = jp * T, zs[jp]
            if jp % 2:
                for r in range(0, T, GS):
                    _put(pb_s, jp // 2 * T + r, 0, _operands(_B_TERMS, blocks(jp, R - T + r, tie, k)))
                    k += 2
            for r in range(0, T, GS):
                p = prob(jp, 2 * R + r, tie(z, k))
                sums[jp].add(p)
                _put(pd_s, 2 * R + r, 0, [p.reshape(GS, 2 * T)])
                k += 1
            so = _Reducer(jnp.sum, jnp.add)
            for r in range(0, T, 2 * GS):
                p = prob(jp, 2 * R + T + r, tie(z, k), 2 * GS, slice(T, 2 * T))
                so.add(p)
                _put(pd_s, 2 * R + T + r, T, [p.reshape(2 * GS, T)])
                k += 1
            sums[jp].result()
            sums[jp].out = sums[jp].out + jnp.concatenate([jnp.zeros((1, T), f32), so.result()], axis=1)

        p20 = lambda g: g * (g - 1) // 2 * T

        def far(g, tie, k):
            half = {(jp, e): _Reducer(jnp.sum, jnp.add) for jp in (2 * g, 2 * g + 1) for e in range(2)}
            for kg in range(g):
                for r in range(0, T, GS):
                    blk = {}
                    for new, n1 in (((0,), 1), ((1,), 5), ((3,), 2), ((), 0), ((), 4), ((2,), 3), ((), 6)):
                        for o in new:
                            lanes = slice((o % 2) * T, (o % 2 + 1) * T)
                            for jp in (2 * g, 2 * g + 1):
                                z = tie(zs[jp][:, lanes], k)
                                row = (o // 2) * jp * T + 2 * kg * T + r
                                p = [jnp.exp2(s_s[jp % 4, x // 8:(x + GS) // 8, :, lanes] - z) for x in (row, row + T)]
                                half[jp, o % 2].add(p[0] + p[1])
                                blk[o, jp % 2], blk[o, 2 + jp % 2] = [x.reshape(GS, T) for x in p]
                        ops = _operands2(_B_TERMS, n1, lambda o, q: blk[o, q], lambda x: x)
                        _put(p2_s, p20(g) + kg * T + r, 7 * n1 * T, ops, lambda w: tie(w, k, True, LATE))
                        k += 16 / 7
            for jp in (2 * g, 2 * g + 1):
                if g:
                    sums[jp].out = sums[jp].out + jnp.concatenate([half[jp, e].result() for e in range(2)], axis=1)
            for jp in (2 * g, 2 * g + 1):
                cols = slice(2 * jp * T, 2 * (jp + 1) * T)
                sc_s[:, cols] = g_s[:, cols] / sums[jp].result()

        def pv(g):
            pairs = (2 * g, 2 * g + 1)
            va = lambda n, t, r=0, nr=HD: _get(va_s, r, nr, (t * 9 + n) * T, T)
            for n1 in range(7 if g else 0):
                c = clk.strassen(
                    lambda n: _cat([_get(v2_s, 0, QD, (kg * 49 + 7 * n1 + n) * T, T) for kg in range(g)], 1),
                    lambda n: _get(p2_s, p20(g), g * T, (7 * n1 + n) * T, T), _NN, g)()
                mp_s[n1 * HD:n1 * HD + QD, :] = jnp.concatenate(c[:2], axis=1)
                mp_s[n1 * HD + QD:(n1 + 1) * HD, :] = jnp.concatenate(c[2:], axis=1)
            if g == 3:
                vfin(3, clk.pacer(clk.t - 2000, clk.t - 1200, 32))
            ve = [jnp.concatenate([va(2, jp), va(8, jp)], axis=0) for jp in pairs]
            vo = [jnp.concatenate([va(7, jp), va(3, jp)], axis=0) for jp in pairs]
            ce = clk.level([(ve[jp % 2], _get(pd_s, 2 * jp * T, T, 0, T)) for jp in pairs])
            co = [clk.dot(jnp.concatenate([ve[jp % 2], vo[jp % 2]], axis=1),
                          _get(pd_s, 2 * jp * T, 2 * T, T, T), _NN) for jp in pairs]
            for jp in pairs:
                R, e = jp * T, jp % 2
                ge, go = sc_s[:, 2 * R:2 * R + T], sc_s[:, 2 * R + T:2 * R + 2 * T]
                for r in range(0, HD, 32):
                    c = [ce[e][r:r + 32], co[e][r:r + 32], ce[e][HD + r:HD + r + 32], co[e][HD + r:HD + r + 32]]
                    if g:
                        far_ = _combine([mp_s[n * HD + r:n * HD + r + 32, e * T:(e + 1) * T] for n in range(7)],
                                        order=range(7))
                        c = [x + y for x, y in zip(c, far_)]
                    if e:
                        near_ = clk.strassen(lambda n: va(n, 2 * g, r, 32),
                                             lambda n: _get(pb_s, g * T, T, n * T, T), _NN)()
                        c = [x + y for x, y in zip(c, near_)]
                    ops = _operands(_B_TERMS, [c[0] * ge, c[1] * go, c[2] * ge, c[3] * go])
                    _put(cl_s, r, jp * 7 * T, ops)

        ends = []

        def run(items):
            for item in items.split():
                if item[0] == 'P':
                    pv(int(item[1]))
                    ends.append(clk.t)
                elif item[0] == 'K':
                    proj(int(item[1]), 2 if item == 'K1' else 0)
                else:
                    jp = int(item[1])
                    oproj(jp, clk)

                    @pl.when(h == H - 1)
                    def _():
                        out_copy(jp).start()

        oproj(NP - 1, clk)
        for n1 in range(7):
            if n1 >= NT1:
                prep_w(h, [n1], clk.pacer(clk.t - 896, clk.t - 448, 8))
            proj(0, n1, n1 + 1)
        proj(1, 0, 2)
        mx = qk(0)
        for g in range(4):
            t0 = clk.t
            del ends[:]
            run(PLAN[g])
            t1 = clk.t
            nxt = qk(g + 1) if g < 3 else None
            n_rough = [2 * jp * T // (GS * LSUB) for jp in (2 * g, 2 * g + 1)]
            n_near = [(T + T // 2) // GS, (3 * T + T // 2) // GS]
            holes = [(t - 400, t) for t in ends]
            if 0 < g < 3:
                holes.append((marks[-2] - 400, marks[-2] - 100))
            if g < 3:
                vfin(g, clk.pacer(t0, t0 + VW, 32))
                holes += [(t0, t0 + VW), (t1 - 300, t1 + 300)]
            if g == 2:
                holes.append((clk.t - 300, clk.t))
            tie = clk.pacer(t0, (clk.t if g else t1) - SLACK,
                            sum(n_rough) + sum(n_near) + g * 16 * T // GS, holes)
            rough(2 * g, mx[0], tie)
            near(2 * g, tie, n_rough[0])
            k = n_rough[0] + n_near[0]
            rough(2 * g + 1, mx[1], lambda x, i: tie(x, k + i))
            near(2 * g + 1, tie, k + n_rough[1])
            far(g, tie, k + n_rough[1] + n_near[1])
            if g == 0:
                prep_wo(clk.pacer(t0 + VW, t1 - 300, HM // 16))
            mx = nxt
        t0 = clk.t
        run(PLAN[4])
        prep_w(jnp.minimum(h + 1, H - 1), range(NT1), clk.pacer(t0 - 100, clk.t - 500, 8 * NT1))
        assert len(set(clk.load)) == 1

    head(**head_refs)

    @pl.when(h == H - 1)
    def _():
        oproj(NP - 1, _Clock(zero_s))
        out_copy(NP - 1).start()
        for jp in range(NP):
            out_copy(jp).wait()


@jax.jit
def pallas_gated_mix__compressed_kv_cla__ssm_conv_s5__prompt_kernel(
    A_x: jax.Array,
    A_c_kv: jax.Array,
    A_w_q: jax.Array,
    A_w_uk: jax.Array,
    A_w_uv: jax.Array,
    A_w_o: jax.Array,
    B_x: jax.Array,
    B_Lambda_re: jax.Array,
    B_Lambda_im: jax.Array,
    B_B_re: jax.Array,
    B_B_im: jax.Array,
    B_C_re: jax.Array,
    B_C_im: jax.Array,
    B_log_dt: jax.Array,
    B_Dskip: jax.Array,
    gate_w: jax.Array,
):
    del B_x
    xT = jnp.transpose(A_x[0])
    woT = jnp.transpose(A_w_o, (0, 2, 1))
    ckv = A_c_kv.reshape(4, 4, 2, T // 2, DC)

    hbm = pl.BlockSpec(memory_space=pl.ANY)
    outT = pl.pallas_call(
        _kernel,
        grid=(H,),
        in_specs=[hbm] * 15,
        out_specs=hbm,
        out_shape=jax.ShapeDtypeStruct((M, S), f32),
        scratch_shapes=_SHARED_SCRATCH + list(_PROLOGUE_SCRATCH.values()) + list(_HEAD_SCRATCH.values()),
        compiler_params=pltpu.CompilerParams(
            dimension_semantics=("arbitrary",),
            vmem_limit_bytes=127 * 1024 * 1024,
            disable_bounds_checks=True,
        ),
    )(xT, B_B_re, B_B_im, B_C_re, B_C_im, B_Lambda_re, B_Lambda_im, B_log_dt,
      B_Dskip, gate_w, woT, ckv, A_w_q, A_w_uk, A_w_uv)
    return jnp.transpose(outT)[None]
```

```python
import bisect

import jax
import jax.numpy as jnp
from jax import lax
import jax.experimental.pallas as pl
import jax.experimental.pallas.tpu as pltpu

S = 2048
M = 448
H = 16
D = 256
DC = 1024
T = 128
NP = S // T // 2
HD = D // 2
HM = M // 2
QD = D // 4
QC = DC // 4
QM = M // 4
PA = 384
PB = M - PA
TA = 512
XCUT = (0, 256, 1152, 2048)
TC = 256
CS = DC // NP
NRAW = 2
LOG2E = 1.4426950408889634
NEG = -1e30

GS = 16
RCH = 256
LSUB = 4
NT1 = 2
OCH = ((0, 64), (64, 64), (128, 48), (176, 48))
PLAN = ('K1', 'K2', 'K3', 'P1 P0 O2 O3 P2 O0 O1 O4 O5', 'P3 O6')
SLACK, LATE, VW = 200, 40, 900

f32 = jnp.float32
bf16 = jnp.bfloat16
u32 = jnp.uint32

SEM_VEC, SEM_B, SEM_X, SEM_WQ, SEM_C, SEM_SL, SEM_WO, SEM_OUT, SEM_WQ1, SEM_KV = 0, 1, 2, 6, 7, 8, 16, 17, 18, 22
NSEM = 24

_NN = ((1,), (0,))
_NT = ((1,), (1,))
_TT = ((0,), (1,))


def _cat(xs, axis):
    return xs[0] if len(xs) == 1 else jnp.concatenate(xs, axis=axis)


def _ds(lo, n, align):
    return pl.ds(lo if isinstance(lo, int) else pl.multiple_of(lo, align), n)


def _put(ref, row, col, xs, tie=None):
    x = _cat(xs, 1)
    if tie is not None:
        x = jnp.concatenate([tie(x[:8]), x[8:]], axis=0)
    ref[row // 2:(row + x.shape[0]) // 2, col:col + x.shape[1]] = pltpu.bitcast(x.astype(bf16), u32)


def _get(ref, row, nrows, col, ncols):
    return pltpu.bitcast(ref[row // 2:(row + nrows) // 2, col:col + ncols], bf16)


class _Clock:
    def __init__(self, zero_ref):
        self.masks = {(8, T): zero_ref[...] != 0.0}
        self.ticks, self.load = [], [0, 0, 0, 0]

    @property
    def t(self):
        return max(self.load)

    def dot(self, a, b, dims):
        v = lax.dot_general(a, b, (dims, ((), ())), preferred_element_type=f32)
        rows, depth = v.shape[0], a.shape[dims[0][0]]
        for c in range(0, v.shape[1], T):
            start = 0
            for _ in range(0, depth, T):
                k = self.load.index(min(self.load))
                start = max(start, self.load[k])
                self.load[k] += rows
            self.ticks += [(start + r + 8, (v, r, c)) for r in range(0, rows, 8)]
        return v

    def strassen(self, lhs, rhs, dims, jobs=1, split_last=False):
        lag = sum(l + 32 <= max(self.load) for l in self.load) // jobs if jobs < 3 else 0
        order = ((1, 3, 2, 4, 0, 5, 6), (0, 1, 3, 2, 4, 5, 6), (5, 6, 1, 3, 2, 4, 0), (0, 5, 6, 1, 3, 2, 4))[lag]
        m = {}
        for n in order:
            a, b = lhs(n), rhs(n)
            if split_last and n == order[-1]:
                half = a.shape[0] // 2
                m[n] = jnp.concatenate([self.dot(a[:half], b, dims), self.dot(a[half:], b, dims)], axis=0)
            else:
                m[n] = self.dot(a, b, dims)
        return lambda r=0, n=None: _combine(m if n is None else _Rows(m, r, n), order=order)

    def level(self, pairs, dims=_NN):
        base, extra = divmod((sum(self.load) + sum(a.shape[0] for a, _ in pairs)) // 16, 4)
        target = [16 * (base + (k < extra)) for k in range(4)]
        out = []
        for a, b in pairs:
            r, parts = 0, []
            while r < a.shape[0]:
                k = self.load.index(min(self.load))
                n = min(max(target[k] - self.load[k], 16), a.shape[0] - r)
                parts.append(self.dot(a[r:r + n], b, dims))
                r += n
            out.append(_cat(parts, 0))
        return out

    def pacer(self, t0, t1, n, holes=()):
        holes = sorted((max(a, t0), min(b, t1)) for a, b in holes if a < t1 and b > t0)
        gap = sum(b - a for a, b in holes)
        ticks = sorted(self.ticks, key=lambda tw: tw[0])
        times = [tw[0] for tw in ticks]

        def tie(x, k, distinct=False, delay=0):
            t = t0 + (t1 - t0 - gap) * k / n
            for a, b in holes:
                t += b - a if t > a else 0
            t += delay
            past = ticks[:bisect.bisect_right(times, t)]
            reps = (x.shape[0] // 8, x.shape[1] // T)
            if len(past) < (reps[1] if distinct else 1):
                return x
            tick = _cat([v[r:r + 8, c:c + T] for _, (v, r, c) in past[-reps[1] if distinct else -1:]], 1)
            if tick.dtype != x.dtype:
                tick = pltpu.bitcast(tick, x.dtype)
            if x.shape not in self.masks:
                self.masks[x.shape] = jnp.tile(self.masks[(8, T)], reps)
            return lax.select(self.masks[x.shape], tick if tick.shape == x.shape else jnp.tile(tick, reps), x)
        return tie


def _no_tie(x, k):
    return x


_A_TERMS = ((0, 3, 1), (2, 3, 1), (0, None, 0), (3, None, 0), (0, 1, 1), (2, 0, -1), (1, 3, -1))
_B_TERMS = ((0, 3, 1), (0, None, 0), (1, 3, -1), (2, 0, -1), (3, None, 0), (0, 1, 1), (2, 3, 1))


def _operand(term, block):
    x, y, sign = term
    if y is None:
        return block(x)
    return block(x) + block(y) if sign > 0 else block(x) - block(y)


def _operands(terms, blocks):
    return [_operand(t, blocks.__getitem__) for t in terms]


def _operands2(terms, n1, block, tie):
    first = terms[n1][0]
    sub = [_operand(terms[n1], lambda o: tie(block(o, q)) if o == first and q in (0, 3) else block(o, q))
           for q in range(4)]
    return _operands(terms, sub)


_C_TERMS = ({0: 1, 3: 1, 4: -1, 6: 1}, {2: 1, 4: 1}, {1: 1, 3: 1}, {0: 1, 1: -1, 2: 1, 5: 1})


def _combine(m, only=(0, 1, 2, 3), order=(1, 3, 2, 4, 0, 5, 6)):
    out = []
    for terms in (_C_TERMS[n] for n in only):
        seq = [n for n in order if n in terms]
        if terms[seq[0]] < 0:
            seq[0], seq[1] = seq[1], seq[0]
        acc = m[seq[0]]
        for n in seq[1:]:
            acc = acc + m[n] if terms[n] > 0 else acc - m[n]
        out.append(acc)
    return out


def _outer_step(m_s, n1, row, v):
    n = v.shape[0]
    if n1 < 5:
        m_s[n1 * HD + row:n1 * HD + row + n, :] = v
    if n1 < 3:
        return None
    blk = (2, 1, 3, 0)[n1 - 3]
    m = {j: v if j == n1 else m_s[j * HD + row:j * HD + row + n, :] for j in _C_TERMS[blk]}
    return blk, _combine(m, (blk,), range(7))[0]


class _Rows:
    def __init__(self, vals, r, n):
        self.vals, self.rows, self.cache = vals, slice(r, r + n), {}

    def __getitem__(self, i):
        if i not in self.cache:
            self.cache[i] = self.vals[i][self.rows, :]
        return self.cache[i]


class _Reducer:
    def __init__(self, red, comb):
        self.red, self.comb, self.acc, self.rows, self.out = red, comb, None, 0, None

    def add(self, v):
        self.rows += 8 * v.shape[0]
        v = self.red(v, axis=0)
        self.acc = v if self.acc is None else self.comb(self.acc, v)
        if self.rows >= RCH:
            self.result()

    def result(self):
        if self.acc is not None:
            v = self.red(self.acc, axis=0, keepdims=True)
            self.out = v if self.out is None else self.comb(self.out, v)
        self.acc, self.rows = None, 0
        return self.out


def _cmul(ar, ai, br, bi):
    return ar * br - ai * bi, ar * bi + ai * br


def _hi16(w):
    return pltpu.bitcast(w & jnp.uint32(0xFFFF0000), f32)


def _stage(raw, stg, c0, nc, tie, groups=(0, 1)):
    for ht in groups:
        for dt in range(2):
            v = raw[c0:c0 + nc, ht * 8:(ht + 1) * 8, dt * T:(dt + 1) * T].reshape(nc * 8, T)
            stg[ht * 2 + dt, c0 * 4:(c0 + nc) * 4, :] = tie(pltpu.bitcast(v, u32), (ht * 2 + dt) / 4)


def _ssm_params(vec_s, coef_s, lam_s, col_s):
    row = lambda r: r[...].astype(f32).reshape(1, M)
    lre, lim, ldt, dsk, gw = [row(v) for v in vec_s]
    dt = jnp.exp(ldt).astype(bf16).astype(f32)
    mag = jnp.exp(dt * lre)
    ang = dt * lim
    lr, li = mag * jnp.cos(ang), mag * jnp.sin(ang)
    den = lre * lre + lim * lim
    nr = lr - 1.0
    coef_s[...] = jnp.zeros(coef_s.shape, f32)
    coef_s[0:1, 0:M] = 2.0 * ((nr * lre + li * lim) / den)
    coef_s[1:2, 0:M] = 2.0 * ((li * lre - nr * lim) / den)

    er = jnp.concatenate([lr, lr[:, PA:]], axis=1)
    ei = jnp.concatenate([li, -li[:, PA:]], axis=1)
    pw = [(er, ei)]
    for _ in range(7):
        pw.append(_cmul(pw[-1][0], pw[-1][1], er, ei))
    sub = lax.broadcasted_iota(jnp.int32, (8, 512), 0)
    for n, d in enumerate((1, 2, 4)):
        lam_s[2 * n] = jnp.where(sub >= d, pw[d - 1][0], 0.0)
        lam_s[2 * n + 1] = jnp.where(sub >= d, pw[d - 1][1], 0.0)
    lcr = jnp.zeros((8, 512), f32)
    lci = jnp.zeros((8, 512), f32)
    for r in range(8):
        lcr = jnp.where(sub == r, pw[r][0], lcr)
        lci = jnp.where(sub == r, pw[r][1], lci)
    lam_s[6] = lcr
    lam_s[7] = lci

    def col(v):
        v = jnp.concatenate([v, jnp.zeros((1, 512 - M), f32)], axis=1)
        return jnp.broadcast_to(v, (T, 512)).T[:M]
    col_s[0] = col(dsk)
    col_s[1] = col(gw)


def _ssm_cmat(craw_s, coef_s, c_s, tie):
    for r in range(0, HM, 16):
        for c in range(0, M, T):
            w = min(T, M - c)
            coef = tie(coef_s[:, c:c + T], r // 16 + c / 512)
            cr, ci = coef[0:1, :w], coef[1:2, :w]
            blk = []
            for row in (r, HM + r):
                re, im = _cmul(craw_s[0, row:row + 16, c:c + w].astype(f32),
                               craw_s[1, row:row + 16, c:c + w].astype(f32), cr, ci)
                blk += [re, -im]
            if c < PA:
                for n, op in enumerate(_operands(_A_TERMS, blk)):
                    _put(c_s, r, n * PA + c, [op])
            else:
                _put(c_s, r, 7 * PA, blk)


def _ssm_scan(u_ref, carry, lam_s, h_s, h0_s, tie):
    car, cai = carry
    out = []
    for b in range(TC // 8):
        mixed = u_ref[3, b, :, 0:T]
        u = jnp.concatenate([u_ref[cb, b] for cb in range(3)], axis=1)
        cols = [u[:, 0:T], u[:, T:2 * T], u[:, 2 * T:PA], mixed]
        hr = jnp.concatenate([tie(v, 4 * b + n) for n, v in enumerate(cols)], axis=1)
        hi = jnp.concatenate([u[:, PA:2 * PA], pltpu.roll(mixed, PB, 1)], axis=1)
        for n, d in enumerate((1, 2, 4)):
            sr, si = pltpu.roll(hr, d, 0), pltpu.roll(hi, d, 0)
            tr, ti = _cmul(sr, si, lam_s[2 * n], lam_s[2 * n + 1])
            hr, hi = hr + tr, hi + ti
        tr, ti = _cmul(lam_s[6], lam_s[7], car, cai)
        hr, hi = hr + tr, hi + ti
        car, cai = hr[7:8, :], hi[7:8, :]
        out.append(jnp.concatenate([hr[:, :PA], hi[:, :PA], hr[:, PA:]], axis=1))
        if b % 2 == 1:
            v, row = jnp.concatenate(out, axis=0), (b - 1) * 8 % T
            _put(h_s, row, 7 * PA + b // 16 * T, [v[:, 2 * PA:]])
            if b < 16:
                h0_s[row:row + 16, :] = v[:, :2 * PA]
            else:
                v0 = h0_s[row:row + 16, :]
                _put(h_s, row, 0, _operands(_B_TERMS, [v0[:, :PA], v[:, :PA], v0[:, PA:], v[:, PA:2 * PA]]))
            out = []
    return car, cai


_vmem = pltpu.VMEM
_PROLOGUE_SCRATCH = dict(
    xT_s=_vmem((M, S), bf16),
    v0=_vmem((M,), bf16), v1=_vmem((M,), bf16), v2=_vmem((M,), bf16), v3=_vmem((M,), bf16), v4=_vmem((M,), bf16),
    b_s=_vmem((2 * M, M), bf16),
    craw_s=_vmem((2, M, M), bf16),
    c_s=_vmem((HM // 2, 7 * PA + 2 * T), u32),
    coef_s=_vmem((8, 512), f32),
    lam_s=_vmem((8, 8, 512), f32),
    col_s=_vmem((2, M, T), f32),
    h_s=_vmem((T // 2, 7 * PA + 2 * T), u32),
    h0_s=_vmem((T, 2 * PA), f32),
    ckv_s=_vmem((NRAW, 4, T // 2, DC), bf16),
    rq=_vmem((M, H, D), bf16),
    rk=_vmem((CS + 1, H, D), bf16),
    rv=_vmem((CS + 1, H, D), bf16),
    sq=_vmem((4, M * 4, T), u32),
    sk=_vmem((4, CS * 4, T), u32),
    sv=_vmem((4, CS * 4, T), u32),
    wqt_s=_vmem((D, 4 * T), u32),
)
_HEAD_SCRATCH = dict(
    mk_s=_vmem((7 * HD, 2 * T), f32),
    mv_s=_vmem((2, 7 * HD, 2 * T), f32),
    mp_s=_vmem((7 * HD, 2 * T), f32),
    kt_s=_vmem((2 * T, 4 * T), f32),
    ka_s=_vmem((S // 4, 8 * T), u32),
    va_s=_vmem((HD // 2, NP * 9 * T), u32),
    v2_s=_vmem((QD // 2, 3 * 49 * T), u32),
    s_s=_vmem((4, S // 8, 8, 2 * T), f32),
    pb_s=_vmem((2 * T, 7 * T), u32),
    pd_s=_vmem((S // 2, 2 * T), u32),
    p2_s=_vmem((3 * T, 49 * T), u32),
    sc_s=_vmem((1, S), f32),
    qb_s=_vmem((HD // 2, 14 * T), u32),
    kd_s=_vmem((T // 2, 7 * T), u32),
)
_SHARED_SCRATCH = [
    _vmem((H // 2 * D, DC), u32),
    _vmem((H // 2 * D, DC), u32),
    _vmem((S // 8, 49 * QC), u32),
    _vmem((H * D, S // 2), u32),
    _vmem((H, M, D), bf16),
    _vmem((QD, 49 * QC), u32),
    _vmem((HM // 2, 7 * T), u32),
    _vmem((HD // 2, NP * 7 * T), u32),
    _vmem((M, S), f32),
    _vmem((1, S), f32),
    _vmem((8, T), f32),
    pltpu.SemaphoreType.DMA((NSEM,)),
]


def _kernel(xT_hbm, bre_hbm, bim_hbm, cre_hbm, cim_hbm, lre_hbm, lim_hbm, ldt_hbm,
            dsk_hbm, gw_hbm, woT_hbm, ckv_hbm, wq_hbm, wk_hbm, wv_hbm,
            out_hbm,
            wkt_s, wvt_s, a_s, q_s, wo_s, w_s, wl_s, cl_s, o_s, g_s, zero_s, sem, *rest):
    h = pl.program_id(0)
    pro_refs = dict(zip(_PROLOGUE_SCRATCH, rest))
    head_refs = dict(zip(_HEAD_SCRATCH, rest[len(pro_refs):]))

    def out_copy(jp):
        cols = pl.ds(jp * 2 * T, 2 * T)
        return pltpu.make_async_copy(o_s.at[:, cols], out_hbm.at[:, cols], sem.at[SEM_OUT])

    def prep_w(hh, outer, tie):
        rows = _ds(lax.shift_right_logical(hh, 1) * D, D, D)
        sh = (16 * (1 - (hh & 1))).astype(u32)
        k = 0
        for row0, wt_s in ((0, wkt_s.at[rows]), (QD, wvt_s.at[rows])):
            for r in range(0, QD, 16):
                def block(o, q):
                    row = (o % 2) * HD + (q % 2) * QD + r
                    col = (o // 2) * 2 * QC + (q // 2) * QC
                    return _hi16(wt_s[row:row + 16, col:col + QC] << sh)
                for n1 in outer:
                    _put(w_s, row0 + r, 7 * n1 * QC, _operands2(_B_TERMS, n1, block, lambda x: tie(x, k)))
                    k += 1

    def prologue(xT_s, v0, v1, v2, v3, v4, b_s, craw_s, c_s, coef_s, lam_s, col_s, h_s, h0_s,
                 ckv_s, rq, rk, rv, sq, sk, sv, wqt_s):
        xa_s = head_refs['p2_s']
        wq_s = xa_s.at[2 * QM:2 * QM + QD]
        u_s = head_refs['s_s']
        vec_s = (v0, v1, v2, v3, v4)

        def slice_copies(i):
            s = sem.at[SEM_SL + i]
            grp = i // 2 if isinstance(i, int) else lax.shift_right_logical(i, 1)
            return [pltpu.make_async_copy(ckv_hbm.at[grp, :, i & 1], ckv_s.at[i & (NRAW - 1)], s)]

        def w_copy(n, i):
            src, dst = ((wk_hbm, rk), (wv_hbm, rv))[n]
            return pltpu.make_async_copy(src.at[pl.ds(i * CS, CS)], dst.at[0:CS], sem.at[SEM_KV + n])

        def wo_copy(i):
            heads = pl.ds(2 * i, 2)
            return pltpu.make_async_copy(woT_hbm.at[heads], wo_s.at[heads], sem.at[SEM_WO])

        def wq1_copy(i):
            rows = pl.ds(i * (M // 4), M // 4)
            return pltpu.make_async_copy(wq_hbm.at[rows, 8:16], rq.at[rows, 8:16], sem.at[SEM_WQ1 + i])

        def x_copy(i):
            cols = pl.ds(XCUT[i], XCUT[i + 1] - XCUT[i])
            return pltpu.make_async_copy(xT_hbm.at[:, cols], xT_s.at[:, cols], sem.at[SEM_X + i])

        cp_vec = [pltpu.make_async_copy(src, dst, sem.at[SEM_VEC])
                  for src, dst in zip((lre_hbm, lim_hbm, ldt_hbm, dsk_hbm, gw_hbm), vec_s)]
        cp_b = [pltpu.make_async_copy(src.at[pl.ds(lo, n)], b_s.at[pl.ds(dst, n)], sem.at[SEM_B])
                for src, lo, n, dst in ((bre_hbm, 0, PA, 0), (bim_hbm, 0, PA, PA),
                                        (bre_hbm, PA, PB, 2 * PA), (bim_hbm, PA, PB, 2 * PA + PB))]
        cp_wq = [pltpu.make_async_copy(wq_hbm.at[:, 0:8], rq.at[:, 0:8], sem.at[SEM_WQ])]
        cp_c = [pltpu.make_async_copy(src, craw_s.at[n], sem.at[SEM_C])
                for n, src in enumerate((cre_hbm, cim_hbm))]
        for cp in cp_vec + cp_b + [x_copy(i) for i in range(3)] + cp_c + cp_wq:
            cp.start()
        for cp in [wq1_copy(0)] + slice_copies(0) + [w_copy(0, 0), w_copy(1, 0)]:
            cp.start()

        zero_s[...] = jnp.zeros(zero_s.shape, f32)
        wl_s[...] = jnp.zeros(wl_s.shape, u32)
        cl_s[:, (NP - 1) * 7 * T:] = jnp.zeros((HD // 2, 7 * T), u32)
        for cp in cp_vec:
            cp.wait()
        _ssm_params(vec_s, coef_s, lam_s, col_s)

        def wq_transpose(pair, tie):
            ht = pair // 4 if isinstance(pair, int) else lax.shift_right_logical(pair, 2)
            pad = jnp.zeros((T - QM, T), u32)
            for dt in range(2):
                for mq in range(4):
                    blk = sq[ht * 2 + dt, pl.ds(mq * QM * 4 + (pair & 3), QM, stride=4), :]
                    blk = jnp.concatenate([tie(blk[:8], 4 * dt + mq), blk[8:], pad], axis=0)
                    wqt_s[dt * HD:(dt + 1) * HD, mq * T:(mq + 1) * T] = blk.T

        def phase1(lo, hi, groups, gates):
            clk = _Clock(zero_s)
            cuts = [lo, lo + T] + list(range(lo + 4 * T, hi, 4 * T)) + [hi]
            for c0, c1 in zip(cuts[:-1], cuts[1:]):
                u = clk.dot(xT_s[:, c0:c1], b_s[...], _TT)
                for cb in range(4):
                    w = min(2 * T, 2 * M - cb * 2 * T)
                    u_s[cb, c0 // 8:c1 // 8, :, 0:w] = u[:, cb * 2 * T:cb * 2 * T + w].reshape((c1 - c0) // 8, 8, w)
            pacer = lambda n, f0=0.0, f1=1.0: clk.pacer(f0 * (clk.t - 500), f1 * (clk.t - 500), n)
            tie = pacer(49 * len(groups))
            for k, g in enumerate(groups):
                for r in range(0, QM, 16):
                    def block(o, q):
                        row, col = (o % 2) * HM + (q % 2) * QM + r, (4 * g + 2 * (q // 2) + o // 2) * T
                        return xT_s[row:row + 16, col:col + T].astype(f32) * (LOG2E * D ** -0.5)
                    for n1 in range(7):
                        ops = _operands2(_A_TERMS, n1, block, lambda x: tie(x, 49 * k + 7 * (r // 16) + n1))
                        _put(xa_s, g * QM + r, 7 * n1 * T, ops)
            tie = pacer(28 * len(gates))
            for t, tile in enumerate(gates):
                cols = slice(tile * T, (tile + 1) * T)
                acc = jnp.zeros((8, T), f32)
                for r in range(0, M, 32):
                    xg = xT_s[r:r + 32, cols].astype(f32) * tie(col_s[1, r:r + 32, :], 28 * t + r // 32)
                    acc = acc + jnp.sum(xg.reshape(4, 8, T), axis=0)
                g = jax.nn.sigmoid(jnp.sum(acc, axis=0, keepdims=True))
                g_s[:, cols] = g
                for r in range(0, M, 32):
                    skip = xT_s[r:r + 32, cols].astype(f32) * tie(col_s[0, r:r + 32, :], 28 * t + 14 + r // 32)
                    o_s[r:r + 32, cols] = (1.0 - g) * skip
            return pacer

        for cp in cp_b + [x_copy(0)]:
            cp.wait()
        phase1(XCUT[0], XCUT[1], [], range(XCUT[1] // T))
        x_copy(1).wait()
        pacer = phase1(XCUT[1], XCUT[2], range(XCUT[2] // TA), range(XCUT[1] // T, XCUT[2] // T))
        zero = jnp.zeros((1, 512), f32)
        carry0 = _ssm_scan(u_s.at[:, 0:TC // 8], (zero, zero), lam_s, h_s, h0_s, pacer(TC // 2))
        for cp in [x_copy(2)] + cp_c + cp_wq:
            cp.wait()
        pacer = phase1(XCUT[2], XCUT[3], range(XCUT[2] // TA, 4), range(XCUT[2] // T, S // T))
        _ssm_cmat(craw_s, coef_s, c_s, pacer(HM // 16))
        tie = pacer(M // 8)
        for c0 in range(0, M, 8):
            _stage(rq, sq, c0, 8, lambda x, j: tie(x, c0 / 10 + j), groups=(0,))
        wq_transpose(0, lambda x, k: tie(x, 46 + k))

        def phase2(i, carry):
            @pl.when(i + 1 < NP)
            def _():
                for cp in slice_copies(i + 1):
                    cp.start()

            @pl.when(i < 3)
            def _():
                wq1_copy(i + 1).start()

            wo_copy(i).start()

            @pl.when(i < 4)
            def _():
                wq1_copy(i).wait()

            for cp in slice_copies(i) + [w_copy(0, i), w_copy(1, i)]:
                cp.wait()

            clk = _Clock(zero_s)
            comb = clk.strassen(lambda n: _get(c_s, 0, HM, n * PA, PA), lambda n: _get(h_s, 0, T, n * PA, PA), _NT, 3)
            mixed = clk.level([(_get(c_s, 0, HM, 7 * PA + n // 2 * T, T), _get(h_s, 0, T, 7 * PA + n % 2 * T, T))
                               for n in range(4)], _NT)
            ty = clk.t
            cols = _ds(i * TC, TC, TC)
            keep = 1.0 - g_s[:, cols]
            for r in range(0, HM, 32):
                y = [c + m[r:r + 32] for c, m in zip(comb(r, 32), mixed)]
                o_s[r:r + 32, cols] += keep * jnp.concatenate(y[:2], axis=1)
                o_s[HM + r:HM + r + 32, cols] += keep * jnp.concatenate(y[2:], axis=1)

            q_i = q_s.at[_ds(i * 2 * D, 2 * D, 2 * D)]
            mq_s = (head_refs['mk_s'], head_refs['mp_s'], head_refs['mv_s'].at[0], head_refs['mv_s'].at[1])
            for g in range(4):
                for n1 in range(7):
                    if g == 0:
                        t = 200 + (ty + 644) * n1 / 7
                        tie = clk.pacer(min(t, clk.t - 500), min(t + 300, clk.t - 500), 8)
                        for r in range(0, 2 * QD, 16):
                            def block(o, q):
                                row = (o % 2) * HD + (q % 2) * QD + r % QD
                                col = (2 * (o // 2) + q // 2) * T
                                w = wqt_s[row:row + 16, col:col + T]
                                return _hi16(w) if r >= QD else pltpu.bitcast(w << 16, f32)
                            _put(wq_s, r, 7 * n1 * T, _operands2(_B_TERMS, n1, block, lambda x: tie(x, r // 16)))
                    comb = clk.strassen(lambda n: _get(wq_s, 0, 2 * QD, (7 * n1 + n) * T, QM),
                                        lambda n: _get(xa_s, g * QM, QM, (7 * n1 + n) * T, T), _NN)
                    for r in range(0, 2 * QD, 32):
                        e, c = r // QD, comb(r, 32)
                        for dq in range(2):
                            row = dq * QD + r % QD
                            done = _outer_step(mq_s[2 * (g % 2) + e], n1, row,
                                               jnp.concatenate([c[dq], c[2 + dq]], axis=1))
                            if done:
                                n, v = done
                                _put(q_i, (2 * e + n // 2) * D + (n % 2) * HD + row, 2 * g * T, [v])

            span = ty + 6000

            u_next = u_s.at[:, pl.ds(jnp.minimum(i + 1, NP - 1) * (TC // 8), TC // 8)]
            carry = _ssm_scan(u_next, carry, lam_s, h_s, h0_s, clk.pacer(ty, span, TC // 2))

            tie = clk.pacer(ty - 1200, span, 64, [(ty, ty + 1000)])
            rq_i = rq.at[pl.ds((i & 3) * (M // 4), M // 4)]
            sq_i = sq.at[:, _ds((i & 3) * M, M, 8)]
            for c0 in range(0, M // 4, 8):
                _stage(rq_i, sq_i, c0, 8, lambda x, j: tie(x, c0 // 4 + 4 * j), groups=(1,))
            wq_transpose(jnp.minimum(i + 1, NP - 1), lambda x, k: tie(x, 36 + 3 * k))
            for n, (raw, stg, wt_s) in enumerate(((rk, sk, wkt_s), (rv, sv, wvt_s))):
                for c0 in range(0, CS, 8):
                    _stage(raw, stg, c0, 8, lambda x, j: tie(x, 16 * n + c0 // 8 + j))

                @pl.when(i + 1 < NP)
                def _():
                    w_copy(n, i + 1).start()

                raw[CS, 0:8, 0:T] = tie(zero_s[...], 16 * n + 19).astype(bf16)
                cols = _ds(i * CS, CS, CS)
                for pair in range(H // 2):
                    for dt in range(2):
                        blk = stg[(pair // 4) * 2 + dt, pl.ds(pair % 4, CS, stride=4), :]
                        row = pair * D + dt * HD
                        blk = jnp.concatenate([tie(blk[:8], 16 + 24 * n + 3 * pair + dt), blk[8:]], axis=0)
                        wt_s[row:row + HD, cols] = blk.T

            tie = clk.pacer(ty + 1000, span, 28)
            ckv_i = ckv_s.at[i & (NRAW - 1)]
            a_i = a_s.at[_ds(i * (T // 4), T // 4, T // 4)]
            for r in range(0, T // 2, 16):
                def block(o, q):
                    col = (o % 2) * 2 * QC + (q % 2) * QC
                    return ckv_i[2 * (q // 2) + o // 2, r:r + 16, col:col + QC].astype(f32)
                for n1 in range(7):
                    ops = _operands2(_A_TERMS, n1, block, lambda x: tie(x, 7 * (r // 16) + n1))
                    _put(a_i, r, 7 * n1 * QC, ops)
            return carry

        lax.fori_loop(0, NP, phase2, carry0)
        for i in range(NP):
            wo_copy(i).wait()
        prep_w(h, range(NT1), _no_tie)

    @pl.when(h == 0)
    def _():
        prologue(**pro_refs)

    def oproj(jp, clk):
        cols = slice(2 * jp * T, (2 * jp + 2) * T)
        for r, n in OCH:
            c = clk.strassen(lambda i: _get(wl_s, r, n, i * T, T),
                             lambda i: _get(cl_s, 0, HD, (jp * 7 + i) * T, T), _NN)()
            o_s[r:r + n, cols] += jnp.concatenate(c[:2], axis=1)
            o_s[HM + r:HM + r + n, cols] += jnp.concatenate(c[2:], axis=1)

    def head(mk_s, mv_s, mp_s, kt_s, ka_s, va_s, v2_s, s_s, pb_s, pd_s, p2_s, sc_s, qb_s, kd_s):
        clk = _Clock(zero_s)
        q_h = q_s.at[_ds(h * D, D, D)]

        def prep_wo(tie):
            for r in range(0, HM, 16):
                top = tie(wo_s[h, r:r + 16, :].astype(f32), r // 16)
                bot = tie(wo_s[h, HM + r:HM + r + 16, :].astype(f32), r // 16)
                _put(wl_s, r, 0, _operands(_A_TERMS, [top[:, :HD], top[:, HD:], bot[:, :HD], bot[:, HD:]]))

        def proj(g, lo=0, hi=7):
            for n1 in range(lo, hi):
                comb = clk.strassen(lambda n: _get(w_s, 0, 2 * QD, (7 * n1 + n) * QC, QC),
                                    lambda n: _get(a_s, g * T, T, (7 * n1 + n) * QC, QC), _NT, 2, n1 == 6)
                for r, m_s in ((0, mk_s), (QD, mv_s.at[g % 2])):
                    c = comb(r, QD)
                    m_s[n1 * HD:n1 * HD + QD, :] = jnp.concatenate([c[0], c[2]], axis=1)
                    m_s[n1 * HD + QD:(n1 + 1) * HD, :] = jnp.concatenate([c[1], c[3]], axis=1)
            if hi < 7:
                return
            cs = [_combine([mk_s[n * HD + r:n * HD + r + 16, :] for n in range(7)], order=range(7))
                  for r in range(0, HD, 16)]
            for n in range(4):
                kt_s[:, n * T:(n + 1) * T] = jnp.concatenate([c[n] for c in cs], axis=0).T
            for r in range(0, 2 * T, T // 2):
                blk = kt_s[r:r + T // 2, :]
                blk = [blk[:, n * T:(n + 1) * T] for n in range(4)]
                _put(ka_s, 2 * g * T + r, 0, _operands(_A_TERMS, blk) + [blk[2]])
            for r in (0, 32, T, T + 32):
                lo_, hi_ = kt_s[r:r + 32, 0:2 * T], kt_s[r + T // 2:r + T // 2 + 32, 0:2 * T]
                _put(kd_s, r // T * (T // 2) + r % T, 0,
                     _operands(_A_TERMS, [lo_[:, :T], lo_[:, T:], hi_[:, :T], hi_[:, T:]]))

        def vfin(g, tie):
            m_s = mv_s.at[g % 2]
            for r in range(0, QD, 16):
                k, blk = 8 * (r // 16), {}
                late = lambda w: tie(w, k, True, LATE)
                for new, n1 in (((0,), 2), ((1,), 4), ((3,), 6), ((), 0), ((), 3), ((2,), 5), ((), 1)):
                    for o in new:
                        for i, row in enumerate((r, QD + r)):
                            tiles = _Rows([m_s.at[n * HD:(n + 1) * HD] for n in range(7)], row, 16)
                            c, = _combine(tiles, ((o % 2) * 2 + o // 2,), range(7))
                            blk[o, i] = c = tie(c, k)
                            slot = (2, 7, 8, 3)[o]
                            _put(va_s, row, ((2 * g + 1) * 9 + slot) * T, [c[:, T:]])
                            if o in (1, 2):
                                _put(va_s, row, (2 * g * 9 + slot) * T, [c[:, :T]])
                    lo_, hi_ = [_operand(_A_TERMS[n1], lambda o: blk[o, i]) for i in range(2)]
                    _put(va_s, r, (2 * g * 9 + n1) * T, [lo_[:, :T]], late)
                    _put(va_s, QD + r, (2 * g * 9 + n1) * T, [hi_[:, :T]], late)
                    if g < 3:
                        _put(v2_s, r, (g * 7 + n1) * 7 * T,
                             _operands(_A_TERMS, [lo_[:, :T], lo_[:, T:], hi_[:, :T], hi_[:, T:]]), late)
                    k += 8 / 7

        key = lax.broadcasted_iota(jnp.int32, (T, 2 * T), 0)
        qry = lax.broadcasted_iota(jnp.int32, (T, 2 * T), 1)
        causal = key <= qry

        marks = []

        def qk(g):
            pairs = (2 * g, 2 * g + 1)
            mx = {jp: _Reducer(jnp.max, jnp.maximum) for jp in pairs}

            def put(jp, row, v):
                v = v.reshape(v.shape[0] // 8, 8, 2 * T)
                s_s[jp % 4, row // 8:row // 8 + v.shape[0]] = v
                mx[jp].add(v)

            def rect(jp, lo, hi):
                for r in range(lo, hi, T // 2):
                    c = clk.strassen(lambda i: _get(ka_s, r, T // 2, i * T, T),
                                     lambda i: _get(qb_s, 0, HD, ((jp % 2) * 7 + i) * T, T), _NN)()
                    put(jp, r, jnp.concatenate(c[:2], axis=1))
                    put(jp, jp * T + r, jnp.concatenate(c[2:], axis=1))

            for jp in pairs:
                for r in range(0, HD, 32):
                    blk = [_get(q_h, e * D + d * HD + r, 32, jp * T, T).astype(f32) for d in range(2) for e in range(2)]
                    _put(qb_s, r, (jp % 2) * 7 * T, _operands(_B_TERMS, blk))
            for jp in pairs:
                rect(jp, 0, 2 * g * T)
                marks.append(clk.t)
            last = {}
            for jp in pairs:
                ko = jnp.concatenate([_get(ka_s, jp * T, T, n * T, T) for n in (7, 3)], axis=1)
                so = jnp.where(causal[:, :T], clk.dot(ko, _get(q_h, D, D, jp * T, T), _NN), NEG)
                row = (2 * jp + 1) * T // 8
                s_s[jp % 4, row:row + T // 8, :, T:] = so.reshape(T // 8, 8, T)
                last[jp] = jnp.concatenate([jnp.full((1, T), NEG, f32), jnp.max(so, axis=0, keepdims=True)], axis=1)
            rect(2 * g + 1, 2 * g * T, (2 * g + 1) * T)
            for jp in pairs:
                c = clk.strassen(lambda i: _get(kd_s, (jp % 2) * (T // 2), T // 2, i * T, T),
                                 lambda i: _get(qb_s, 0, HD, ((jp % 2) * 7 + i) * T, T), _NN)()
                se = jnp.concatenate([jnp.concatenate(c[:2], axis=1), jnp.concatenate(c[2:], axis=1)], axis=0)
                put(jp, 2 * jp * T, jnp.where(causal, se, NEG))
            return [jnp.broadcast_to(jnp.maximum(mx[jp].result(), last[jp]), (8, 2 * T)) for jp in pairs]

        zs, sums = {}, {}

        def prob(jp, row, z, n=GS, lanes=slice(None)):
            return jnp.exp2(s_s[jp % 4, row // 8:(row + n) // 8, :, lanes] - z[:, lanes])

        def rough(jp, mx, tie):
            zs[jp] = mx
            if jp > 0:
                sm = _Reducer(jnp.sum, jnp.add)
                for k, r in enumerate(range(0, 2 * jp * T, GS * LSUB)):
                    sm.add(prob(jp, r, tie(mx, k)))
                zs[jp] = mx + jnp.log2(jnp.maximum(LSUB * sm.result(), 1.0))
            sums[jp] = _Reducer(jnp.sum, jnp.add)

        def blocks(jp, row, tie, k):
            top, bot = prob(jp, row, tie(zs[jp], k)), prob(jp, jp * T + row, tie(zs[jp], k + 1))
            sums[jp].add(top + bot)
            top, bot = top.reshape(GS, 2 * T), bot.reshape(GS, 2 * T)
            return [top[:, :T], top[:, T:], bot[:, :T], bot[:, T:]]

        def near(jp, tie, k):
            R, z = jp * T, zs[jp]
            if jp % 2:
                for r in range(0, T, GS):
                    _put(pb_s, jp // 2 * T + r, 0, _operands(_B_TERMS, blocks(jp, R - T + r, tie, k)))
                    k += 2
            for r in range(0, T, GS):
                p = prob(jp, 2 * R + r, tie(z, k))
                sums[jp].add(p)
                _put(pd_s, 2 * R + r, 0, [p.reshape(GS, 2 * T)])
                k += 1
            so = _Reducer(jnp.sum, jnp.add)
            for r in range(0, T, 2 * GS):
                p = prob(jp, 2 * R + T + r, tie(z, k), 2 * GS, slice(T, 2 * T))
                so.add(p)
                _put(pd_s, 2 * R + T + r, T, [p.reshape(2 * GS, T)])
                k += 1
            sums[jp].result()
            sums[jp].out = sums[jp].out + jnp.concatenate([jnp.zeros((1, T), f32), so.result()], axis=1)

        p20 = lambda g: g * (g - 1) // 2 * T

        def far(g, tie, k):
            half = {(jp, e): _Reducer(jnp.sum, jnp.add) for jp in (2 * g, 2 * g + 1) for e in range(2)}
            for kg in range(g):
                for r in range(0, T, GS):
                    blk = {}
                    for new, n1 in (((0,), 1), ((1,), 5), ((3,), 2), ((), 0), ((), 4), ((2,), 3), ((), 6)):
                        for o in new:
                            lanes = slice((o % 2) * T, (o % 2 + 1) * T)
                            for jp in (2 * g, 2 * g + 1):
                                z = tie(zs[jp][:, lanes], k)
                                row = (o // 2) * jp * T + 2 * kg * T + r
                                p = [jnp.exp2(s_s[jp % 4, x // 8:(x + GS) // 8, :, lanes] - z) for x in (row, row + T)]
                                half[jp, o % 2].add(p[0] + p[1])
                                blk[o, jp % 2], blk[o, 2 + jp % 2] = [x.reshape(GS, T) for x in p]
                        ops = _operands2(_B_TERMS, n1, lambda o, q: blk[o, q], lambda x: x)
                        _put(p2_s, p20(g) + kg * T + r, 7 * n1 * T, ops, lambda w: tie(w, k, True, LATE))
                        k += 16 / 7
            for jp in (2 * g, 2 * g + 1):
                if g:
                    sums[jp].out = sums[jp].out + jnp.concatenate([half[jp, e].result() for e in range(2)], axis=1)
            for jp in (2 * g, 2 * g + 1):
                cols = slice(2 * jp * T, 2 * (jp + 1) * T)
                sc_s[:, cols] = g_s[:, cols] / sums[jp].result()

        def pv(g):
            pairs = (2 * g, 2 * g + 1)
            va = lambda n, t, r=0, nr=HD: _get(va_s, r, nr, (t * 9 + n) * T, T)
            for n1 in range(7 if g else 0):
                c = clk.strassen(
                    lambda n: _cat([_get(v2_s, 0, QD, (kg * 49 + 7 * n1 + n) * T, T) for kg in range(g)], 1),
                    lambda n: _get(p2_s, p20(g), g * T, (7 * n1 + n) * T, T), _NN, g)()
                mp_s[n1 * HD:n1 * HD + QD, :] = jnp.concatenate(c[:2], axis=1)
                mp_s[n1 * HD + QD:(n1 + 1) * HD, :] = jnp.concatenate(c[2:], axis=1)
            if g == 3:
                vfin(3, clk.pacer(clk.t - 2000, clk.t - 1200, 32))
            ve = [jnp.concatenate([va(2, jp), va(8, jp)], axis=0) for jp in pairs]
            vo = [jnp.concatenate([va(7, jp), va(3, jp)], axis=0) for jp in pairs]
            ce = clk.level([(ve[jp % 2], _get(pd_s, 2 * jp * T, T, 0, T)) for jp in pairs])
            co = [clk.dot(jnp.concatenate([ve[jp % 2], vo[jp % 2]], axis=1),
                          _get(pd_s, 2 * jp * T, 2 * T, T, T), _NN) for jp in pairs]
            for jp in pairs:
                R, e = jp * T, jp % 2
                ge, go = sc_s[:, 2 * R:2 * R + T], sc_s[:, 2 * R + T:2 * R + 2 * T]
                for r in range(0, HD, 32):
                    c = [ce[e][r:r + 32], co[e][r:r + 32], ce[e][HD + r:HD + r + 32], co[e][HD + r:HD + r + 32]]
                    if g:
                        far_ = _combine([mp_s[n * HD + r:n * HD + r + 32, e * T:(e + 1) * T] for n in range(7)],
                                        order=range(7))
                        c = [x + y for x, y in zip(c, far_)]
                    if e:
                        near_ = clk.strassen(lambda n: va(n, 2 * g, r, 32),
                                             lambda n: _get(pb_s, g * T, T, n * T, T), _NN)()
                        c = [x + y for x, y in zip(c, near_)]
                    ops = _operands(_B_TERMS, [c[0] * ge, c[1] * go, c[2] * ge, c[3] * go])
                    _put(cl_s, r, jp * 7 * T, ops)

        ends = []

        def run(items):
            for item in items.split():
                if item[0] == 'P':
                    pv(int(item[1]))
                    ends.append(clk.t)
                elif item[0] == 'K':
                    proj(int(item[1]), 2 if item == 'K1' else 0)
                else:
                    jp = int(item[1])
                    oproj(jp, clk)

                    @pl.when(h == H - 1)
                    def _():
                        out_copy(jp).start()

        oproj(NP - 1, clk)
        for n1 in range(7):
            if n1 >= NT1:
                prep_w(h, [n1], clk.pacer(clk.t - 896, clk.t - 448, 8))
            proj(0, n1, n1 + 1)
        proj(1, 0, 2)
        mx = qk(0)
        for g in range(4):
            t0 = clk.t
            del ends[:]
            run(PLAN[g])
            t1 = clk.t
            nxt = qk(g + 1) if g < 3 else None
            n_rough = [2 * jp * T // (GS * LSUB) for jp in (2 * g, 2 * g + 1)]
            n_near = [(T + T // 2) // GS, (3 * T + T // 2) // GS]
            holes = [(t - 400, t) for t in ends]
            if 0 < g < 3:
                holes.append((marks[-2] - 400, marks[-2] - 100))
            if g < 3:
                vfin(g, clk.pacer(t0, t0 + VW, 32))
                holes += [(t0, t0 + VW), (t1 - 300, t1 + 300)]
            if g == 2:
                holes.append((clk.t - 300, clk.t))
            tie = clk.pacer(t0, (clk.t if g else t1) - SLACK,
                            sum(n_rough) + sum(n_near) + g * 16 * T // GS, holes)
            rough(2 * g, mx[0], tie)
            near(2 * g, tie, n_rough[0])
            k = n_rough[0] + n_near[0]
            rough(2 * g + 1, mx[1], lambda x, i: tie(x, k + i))
            near(2 * g + 1, tie, k + n_rough[1])
            far(g, tie, k + n_rough[1] + n_near[1])
            if g == 0:
                prep_wo(clk.pacer(t0 + VW, t1 - 300, HM // 16))
            mx = nxt
        t0 = clk.t
        run(PLAN[4])
        prep_w(jnp.minimum(h + 1, H - 1), range(NT1), clk.pacer(t0 - 100, clk.t - 500, 8 * NT1))
        assert len(set(clk.load)) == 1

    head(**head_refs)

    @pl.when(h == H - 1)
    def _():
        oproj(NP - 1, _Clock(zero_s))
        out_copy(NP - 1).start()
        for jp in range(NP):
            out_copy(jp).wait()


@jax.jit
def pallas_gated_mix__compressed_kv_cla__ssm_conv_s5__prompt_kernel(
    A_x: jax.Array,
    A_c_kv: jax.Array,
    A_w_q: jax.Array,
    A_w_uk: jax.Array,
    A_w_uv: jax.Array,
    A_w_o: jax.Array,
    B_x: jax.Array,
    B_Lambda_re: jax.Array,
    B_Lambda_im: jax.Array,
    B_B_re: jax.Array,
    B_B_im: jax.Array,
    B_C_re: jax.Array,
    B_C_im: jax.Array,
    B_log_dt: jax.Array,
    B_Dskip: jax.Array,
    gate_w: jax.Array,
):
    del B_x
    xT = jnp.transpose(A_x[0])
    woT = jnp.transpose(A_w_o, (0, 2, 1))
    ckv = A_c_kv.reshape(4, 4, 2, T // 2, DC)

    hbm = pl.BlockSpec(memory_space=pl.ANY)
    outT = pl.pallas_call(
        _kernel,
        grid=(H,),
        in_specs=[hbm] * 15,
        out_specs=hbm,
        out_shape=jax.ShapeDtypeStruct((M, S), f32),
        scratch_shapes=_SHARED_SCRATCH + list(_PROLOGUE_SCRATCH.values()) + list(_HEAD_SCRATCH.values()),
        compiler_params=pltpu.CompilerParams(
            dimension_semantics=("arbitrary",),
            vmem_limit_bytes=127 * 1024 * 1024,
            disable_bounds_checks=True,
        ),
    )(xT, B_B_re, B_B_im, B_C_re, B_C_im, B_Lambda_re, B_Lambda_im, B_log_dt,
      B_Dskip, gate_w, woT, ckv, A_w_q, A_w_uk, A_w_uv)
    return jnp.transpose(outT)[None]
```

```python
import bisect

import jax
import jax.numpy as jnp
from jax import lax
import jax.experimental.pallas as pl
import jax.experimental.pallas.tpu as pltpu

S = 2048
M = 448
H = 16
D = 256
DC = 1024
T = 128
NP = S // T // 2
HD = D // 2
HM = M // 2
QD = D // 4
QC = DC // 4
QM = M // 4
PA = 384
PB = M - PA
TA = 512
XCUT = (0, 256, 1152, 2048)
TC = 256
CS = DC // NP
NRAW = 2
LOG2E = 1.4426950408889634
NEG = -1e30

GS = 16
RCH = 256
LSUB = 4
NT1 = 2
OCH = ((0, 64), (64, 64), (128, 48), (176, 48))
PLAN = ('K1', 'K2', 'K3', 'P1 P0 O2 O3 P2 O0 O1 O4 O5', 'P3 O6')
SLACK, LATE, VW = 200, 40, 900

f32 = jnp.float32
bf16 = jnp.bfloat16
u32 = jnp.uint32

SEM_VEC, SEM_B, SEM_X, SEM_WQ, SEM_C, SEM_SL, SEM_WO, SEM_OUT, SEM_WQ1, SEM_KV = 0, 1, 2, 6, 7, 8, 16, 17, 18, 22
NSEM = 24

_NN = ((1,), (0,))
_NT = ((1,), (1,))
_TT = ((0,), (1,))


def _cat(xs, axis):
    return xs[0] if len(xs) == 1 else jnp.concatenate(xs, axis=axis)


def _ds(lo, n, align):
    return pl.ds(lo if isinstance(lo, int) else pl.multiple_of(lo, align), n)


def _put(ref, row, col, xs, tie=None):
    x = _cat(xs, 1)
    if tie is not None:
        x = jnp.concatenate([tie(x[:8]), x[8:]], axis=0)
    ref[row // 2:(row + x.shape[0]) // 2, col:col + x.shape[1]] = pltpu.bitcast(x.astype(bf16), u32)


def _get(ref, row, nrows, col, ncols):
    return pltpu.bitcast(ref[row // 2:(row + nrows) // 2, col:col + ncols], bf16)


class _Clock:
    def __init__(self, zero_ref):
        self.masks = {(8, T): zero_ref[...] != 0.0}
        self.ticks, self.load = [], [0, 0, 0, 0]

    @property
    def t(self):
        return max(self.load)

    def dot(self, a, b, dims):
        v = lax.dot_general(a, b, (dims, ((), ())), preferred_element_type=f32)
        rows, depth = v.shape[0], a.shape[dims[0][0]]
        for c in range(0, v.shape[1], T):
            start = 0
            for _ in range(0, depth, T):
                k = self.load.index(min(self.load))
                start = max(start, self.load[k])
                self.load[k] += rows
            self.ticks += [(start + r + 8, (v, r, c)) for r in range(0, rows, 8)]
        return v

    def strassen(self, lhs, rhs, dims, jobs=1, split_last=False):
        lag = sum(l + 32 <= max(self.load) for l in self.load) // jobs if jobs < 3 else 0
        order = ((1, 3, 2, 4, 0, 5, 6), (0, 1, 3, 2, 4, 5, 6), (5, 6, 1, 3, 2, 4, 0), (0, 5, 6, 1, 3, 2, 4))[lag]
        m = {}
        for n in order:
            a, b = lhs(n), rhs(n)
            if split_last and n == order[-1]:
                half = a.shape[0] // 2
                m[n] = jnp.concatenate([self.dot(a[:half], b, dims), self.dot(a[half:], b, dims)], axis=0)
            else:
                m[n] = self.dot(a, b, dims)
        return lambda r=0, n=None: _combine(m if n is None else _Rows(m, r, n), order=order)

    def level(self, pairs, dims=_NN):
        base, extra = divmod((sum(self.load) + sum(a.shape[0] for a, _ in pairs)) // 16, 4)
        target = [16 * (base + (k < extra)) for k in range(4)]
        out = []
        for a, b in pairs:
            r, parts = 0, []
            while r < a.shape[0]:
                k = self.load.index(min(self.load))
                n = min(max(target[k] - self.load[k], 16), a.shape[0] - r)
                parts.append(self.dot(a[r:r + n], b, dims))
                r += n
            out.append(_cat(parts, 0))
        return out

    def pacer(self, t0, t1, n, holes=()):
        holes = sorted((max(a, t0), min(b, t1)) for a, b in holes if a < t1 and b > t0)
        gap = sum(b - a for a, b in holes)
        ticks = sorted(self.ticks, key=lambda tw: tw[0])
        times = [tw[0] for tw in ticks]

        def tie(x, k, distinct=False, delay=0):
            t = t0 + (t1 - t0 - gap) * k / n
            for a, b in holes:
                t += b - a if t > a else 0
            t += delay
            past = ticks[:bisect.bisect_right(times, t)]
            reps = (x.shape[0] // 8, x.shape[1] // T)
            if len(past) < (reps[1] if distinct else 1):
                return x
            tick = _cat([v[r:r + 8, c:c + T] for _, (v, r, c) in past[-reps[1] if distinct else -1:]], 1)
            if tick.dtype != x.dtype:
                tick = pltpu.bitcast(tick, x.dtype)
            if x.shape not in self.masks:
                self.masks[x.shape] = jnp.tile(self.masks[(8, T)], reps)
            return lax.select(self.masks[x.shape], tick if tick.shape == x.shape else jnp.tile(tick, reps), x)
        return tie


def _no_tie(x, k):
    return x


_A_TERMS = ((0, 3, 1), (2, 3, 1), (0, None, 0), (3, None, 0), (0, 1, 1), (2, 0, -1), (1, 3, -1))
_B_TERMS = ((0, 3, 1), (0, None, 0), (1, 3, -1), (2, 0, -1), (3, None, 0), (0, 1, 1), (2, 3, 1))


def _operand(term, block):
    x, y, sign = term
    if y is None:
        return block(x)
    return block(x) + block(y) if sign > 0 else block(x) - block(y)


def _operands(terms, blocks):
    return [_operand(t, blocks.__getitem__) for t in terms]


def _operands2(terms, n1, block, tie):
    first = terms[n1][0]
    sub = [_operand(terms[n1], lambda o: tie(block(o, q)) if o == first and q in (0, 3) else block(o, q))
           for q in range(4)]
    return _operands(terms, sub)


_C_TERMS = ({0: 1, 3: 1, 4: -1, 6: 1}, {2: 1, 4: 1}, {1: 1, 3: 1}, {0: 1, 1: -1, 2: 1, 5: 1})


def _combine(m, only=(0, 1, 2, 3), order=(1, 3, 2, 4, 0, 5, 6)):
    out = []
    for terms in (_C_TERMS[n] for n in only):
        seq = [n for n in order if n in terms]
        if terms[seq[0]] < 0:
            seq[0], seq[1] = seq[1], seq[0]
        acc = m[seq[0]]
        for n in seq[1:]:
            acc = acc + m[n] if terms[n] > 0 else acc - m[n]
        out.append(acc)
    return out


def _outer_step(m_s, n1, row, v):
    n = v.shape[0]
    if n1 < 5:
        m_s[n1 * HD + row:n1 * HD + row + n, :] = v
    if n1 < 3:
        return None
    blk = (2, 1, 3, 0)[n1 - 3]
    m = {j: v if j == n1 else m_s[j * HD + row:j * HD + row + n, :] for j in _C_TERMS[blk]}
    return blk, _combine(m, (blk,), range(7))[0]


class _Rows:
    def __init__(self, vals, r, n):
        self.vals, self.rows, self.cache = vals, slice(r, r + n), {}

    def __getitem__(self, i):
        if i not in self.cache:
            self.cache[i] = self.vals[i][self.rows, :]
        return self.cache[i]


class _Reducer:
    def __init__(self, red, comb):
        self.red, self.comb, self.acc, self.rows, self.out = red, comb, None, 0, None

    def add(self, v):
        self.rows += 8 * v.shape[0]
        v = self.red(v, axis=0)
        self.acc = v if self.acc is None else self.comb(self.acc, v)
        if self.rows >= RCH:
            self.result()

    def result(self):
        if self.acc is not None:
            v = self.red(self.acc, axis=0, keepdims=True)
            self.out = v if self.out is None else self.comb(self.out, v)
        self.acc, self.rows = None, 0
        return self.out


def _cmul(ar, ai, br, bi):
    return ar * br - ai * bi, ar * bi + ai * br


def _hi16(w):
    return pltpu.bitcast(w & jnp.uint32(0xFFFF0000), f32)


def _stage(raw, stg, c0, nc, tie, groups=(0, 1)):
    for ht in groups:
        for dt in range(2):
            v = raw[c0:c0 + nc, ht * 8:(ht + 1) * 8, dt * T:(dt + 1) * T].reshape(nc * 8, T)
            stg[ht * 2 + dt, c0 * 4:(c0 + nc) * 4, :] = tie(pltpu.bitcast(v, u32), (ht * 2 + dt) / 4)


def _ssm_params(vec_s, coef_s, lam_s, col_s):
    row = lambda r: r[...].astype(f32).reshape(1, M)
    lre, lim, ldt, dsk, gw = [row(v) for v in vec_s]
    dt = jnp.exp(ldt).astype(bf16).astype(f32)
    mag = jnp.exp(dt * lre)
    ang = dt * lim
    lr, li = mag * jnp.cos(ang), mag * jnp.sin(ang)
    den = lre * lre + lim * lim
    nr = lr - 1.0
    coef_s[...] = jnp.zeros(coef_s.shape, f32)
    coef_s[0:1, 0:M] = 2.0 * ((nr * lre + li * lim) / den)
    coef_s[1:2, 0:M] = 2.0 * ((li * lre - nr * lim) / den)

    er = jnp.concatenate([lr, lr[:, PA:]], axis=1)
    ei = jnp.concatenate([li, -li[:, PA:]], axis=1)
    pw = [(er, ei)]
    for _ in range(7):
        pw.append(_cmul(pw[-1][0], pw[-1][1], er, ei))
    sub = lax.broadcasted_iota(jnp.int32, (8, 512), 0)
    for n, d in enumerate((1, 2, 4)):
        lam_s[2 * n] = jnp.where(sub >= d, pw[d - 1][0], 0.0)
        lam_s[2 * n + 1] = jnp.where(sub >= d, pw[d - 1][1], 0.0)
    lcr = jnp.zeros((8, 512), f32)
    lci = jnp.zeros((8, 512), f32)
    for r in range(8):
        lcr = jnp.where(sub == r, pw[r][0], lcr)
        lci = jnp.where(sub == r, pw[r][1], lci)
    lam_s[6] = lcr
    lam_s[7] = lci

    def col(v):
        v = jnp.concatenate([v, jnp.zeros((1, 512 - M), f32)], axis=1)
        return jnp.broadcast_to(v, (T, 512)).T[:M]
    col_s[0] = col(dsk)
    col_s[1] = col(gw)


def _ssm_cmat(craw_s, coef_s, c_s, tie):
    for r in range(0, HM, 16):
        for c in range(0, M, T):
            w = min(T, M - c)
            coef = tie(coef_s[:, c:c + T], r // 16 + c / 512)
            cr, ci = coef[0:1, :w], coef[1:2, :w]
            blk = []
            for row in (r, HM + r):
                re, im = _cmul(craw_s[0, row:row + 16, c:c + w].astype(f32),
                               craw_s[1, row:row + 16, c:c + w].astype(f32), cr, ci)
                blk += [re, -im]
            if c < PA:
                for n, op in enumerate(_operands(_A_TERMS, blk)):
                    _put(c_s, r, n * PA + c, [op])
            else:
                _put(c_s, r, 7 * PA, blk)


def _ssm_scan(u_ref, carry, lam_s, h_s, h0_s, tie):
    car, cai = carry
    out = []
    for b in range(TC // 8):
        mixed = u_ref[3, b, :, 0:T]
        u = jnp.concatenate([u_ref[cb, b] for cb in range(3)], axis=1)
        cols = [u[:, 0:T], u[:, T:2 * T], u[:, 2 * T:PA], mixed]
        hr = jnp.concatenate([tie(v, 4 * b + n) for n, v in enumerate(cols)], axis=1)
        hi = jnp.concatenate([u[:, PA:2 * PA], pltpu.roll(mixed, PB, 1)], axis=1)
        for n, d in enumerate((1, 2, 4)):
            sr, si = pltpu.roll(hr, d, 0), pltpu.roll(hi, d, 0)
            tr, ti = _cmul(sr, si, lam_s[2 * n], lam_s[2 * n + 1])
            hr, hi = hr + tr, hi + ti
        tr, ti = _cmul(lam_s[6], lam_s[7], car, cai)
        hr, hi = hr + tr, hi + ti
        car, cai = hr[7:8, :], hi[7:8, :]
        out.append(jnp.concatenate([hr[:, :PA], hi[:, :PA], hr[:, PA:]], axis=1))
        if b % 2 == 1:
            v, row = jnp.concatenate(out, axis=0), (b - 1) * 8 % T
            _put(h_s, row, 7 * PA + b // 16 * T, [v[:, 2 * PA:]])
            if b < 16:
                h0_s[row:row + 16, :] = v[:, :2 * PA]
            else:
                v0 = h0_s[row:row + 16, :]
                _put(h_s, row, 0, _operands(_B_TERMS, [v0[:, :PA], v[:, :PA], v0[:, PA:], v[:, PA:2 * PA]]))
            out = []
    return car, cai


_vmem = pltpu.VMEM
_PROLOGUE_SCRATCH = dict(
    xT_s=_vmem((M, S), bf16),
    v0=_vmem((M,), bf16), v1=_vmem((M,), bf16), v2=_vmem((M,), bf16), v3=_vmem((M,), bf16), v4=_vmem((M,), bf16),
    b_s=_vmem((2 * M, M), bf16),
    craw_s=_vmem((2, M, M), bf16),
    c_s=_vmem((HM // 2, 7 * PA + 2 * T), u32),
    coef_s=_vmem((8, 512), f32),
    lam_s=_vmem((8, 8, 512), f32),
    col_s=_vmem((2, M, T), f32),
    h_s=_vmem((T // 2, 7 * PA + 2 * T), u32),
    h0_s=_vmem((T, 2 * PA), f32),
    ckv_s=_vmem((NRAW, 4, T // 2, DC), bf16),
    rq=_vmem((M, H, D), bf16),
    rk=_vmem((CS + 1, H, D), bf16),
    rv=_vmem((CS + 1, H, D), bf16),
    sq=_vmem((4, M * 4 + 8, T), u32),
    sk=_vmem((4, CS * 4 + 8, T), u32),
    sv=_vmem((4, CS * 4 + 8, T), u32),
    wqt_s=_vmem((D, 4 * T), u32),
)
_HEAD_SCRATCH = dict(
    mk_s=_vmem((7 * HD, 2 * T), f32),
    mv_s=_vmem((2, 7 * HD, 2 * T), f32),
    mp_s=_vmem((7 * HD, 2 * T), f32),
    kt_s=_vmem((2 * T, 4 * T), f32),
    ka_s=_vmem((S // 4, 8 * T), u32),
    va_s=_vmem((HD // 2, NP * 9 * T), u32),
    v2_s=_vmem((QD // 2, 3 * 49 * T), u32),
    s_s=_vmem((4, S // 8, 8, 2 * T), f32),
    pb_s=_vmem((2 * T, 7 * T), u32),
    pd_s=_vmem((S // 2, 2 * T), u32),
    p2_s=_vmem((3 * T, 49 * T), u32),
    sc_s=_vmem((1, S), f32),
    qb_s=_vmem((HD // 2, 14 * T), u32),
    kd_s=_vmem((T // 2, 7 * T), u32),
)
_SHARED_SCRATCH = [
    _vmem((H // 2 * D, DC), u32),
    _vmem((H // 2 * D, DC), u32),
    _vmem((S // 8, 49 * QC), u32),
    _vmem((H * D, S // 2), u32),
    _vmem((H, M, D), bf16),
    _vmem((QD, 49 * QC), u32),
    _vmem((HM // 2, 7 * T), u32),
    _vmem((HD // 2, NP * 7 * T), u32),
    _vmem((M, S), f32),
    _vmem((1, S), f32),
    _vmem((8, T), f32),
    pltpu.SemaphoreType.DMA((NSEM,)),
]


def _kernel(xT_hbm, bre_hbm, bim_hbm, cre_hbm, cim_hbm, lre_hbm, lim_hbm, ldt_hbm,
            dsk_hbm, gw_hbm, woT_hbm, ckv_hbm, wq_hbm, wk_hbm, wv_hbm,
            out_hbm,
            wkt_s, wvt_s, a_s, q_s, wo_s, w_s, wl_s, cl_s, o_s, g_s, zero_s, sem, *rest):
    h = pl.program_id(0)
    pro_refs = dict(zip(_PROLOGUE_SCRATCH, rest))
    head_refs = dict(zip(_HEAD_SCRATCH, rest[len(pro_refs):]))

    def out_copy(jp):
        cols = pl.ds(jp * 2 * T, 2 * T)
        return pltpu.make_async_copy(o_s.at[:, cols], out_hbm.at[:, cols], sem.at[SEM_OUT])

    def prep_w(hh, outer, tie):
        rows = _ds(lax.shift_right_logical(hh, 1) * D, D, D)
        sh = (16 * (1 - (hh & 1))).astype(u32)
        k = 0
        for row0, wt_s in ((0, wkt_s.at[rows]), (QD, wvt_s.at[rows])):
            for r in range(0, QD, 16):
                def block(o, q):
                    row = (o % 2) * HD + (q % 2) * QD + r
                    col = (o // 2) * 2 * QC + (q // 2) * QC
                    return _hi16(wt_s[row:row + 16, col:col + QC] << sh)
                for n1 in outer:
                    _put(w_s, row0 + r, 7 * n1 * QC, _operands2(_B_TERMS, n1, block, lambda x: tie(x, k)))
                    k += 1

    def prologue(xT_s, v0, v1, v2, v3, v4, b_s, craw_s, c_s, coef_s, lam_s, col_s, h_s, h0_s,
                 ckv_s, rq, rk, rv, sq, sk, sv, wqt_s):
        xa_s = head_refs['p2_s']
        wq_s = xa_s.at[2 * QM:2 * QM + QD]
        u_s = head_refs['s_s']
        vec_s = (v0, v1, v2, v3, v4)

        def slice_copies(i):
            s = sem.at[SEM_SL + i]
            grp = i // 2 if isinstance(i, int) else lax.shift_right_logical(i, 1)
            return [pltpu.make_async_copy(ckv_hbm.at[grp, :, i & 1], ckv_s.at[i & (NRAW - 1)], s)]

        def w_copy(n, i):
            src, dst = ((wk_hbm, rk), (wv_hbm, rv))[n]
            return pltpu.make_async_copy(src.at[pl.ds(i * CS, CS)], dst.at[0:CS], sem.at[SEM_KV + n])

        def wo_copy(i):
            heads = pl.ds(2 * i, 2)
            return pltpu.make_async_copy(woT_hbm.at[heads], wo_s.at[heads], sem.at[SEM_WO])

        def wq1_copy(i):
            rows = pl.ds(i * (M // 4), M // 4)
            return pltpu.make_async_copy(wq_hbm.at[rows, 8:16], rq.at[rows, 8:16], sem.at[SEM_WQ1 + i])

        def x_copy(i):
            cols = pl.ds(XCUT[i], XCUT[i + 1] - XCUT[i])
            return pltpu.make_async_copy(xT_hbm.at[:, cols], xT_s.at[:, cols], sem.at[SEM_X + i])

        cp_vec = [pltpu.make_async_copy(src, dst, sem.at[SEM_VEC])
                  for src, dst in zip((lre_hbm, lim_hbm, ldt_hbm, dsk_hbm, gw_hbm), vec_s)]
        cp_b = [pltpu.make_async_copy(src.at[pl.ds(lo, n)], b_s.at[pl.ds(dst, n)], sem.at[SEM_B])
                for src, lo, n, dst in ((bre_hbm, 0, PA, 0), (bim_hbm, 0, PA, PA),
                                        (bre_hbm, PA, PB, 2 * PA), (bim_hbm, PA, PB, 2 * PA + PB))]
        cp_wq = [pltpu.make_async_copy(wq_hbm.at[:, 0:8], rq.at[:, 0:8], sem.at[SEM_WQ])]
        cp_c = [pltpu.make_async_copy(src, craw_s.at[n], sem.at[SEM_C])
                for n, src in enumerate((cre_hbm, cim_hbm))]
        for cp in cp_vec + cp_b + [x_copy(i) for i in range(3)] + cp_c + cp_wq:
            cp.start()
        for cp in [wq1_copy(0)] + slice_copies(0) + [w_copy(0, 0), w_copy(1, 0)]:
            cp.start()

        zero_s[...] = jnp.zeros(zero_s.shape, f32)
        wl_s[...] = jnp.zeros(wl_s.shape, u32)
        for stg in (sq, sk, sv):
            stg[:, stg.shape[1] - 8:, :] = jnp.zeros((4, 8, T), u32)
        cl_s[:, (NP - 1) * 7 * T:] = jnp.zeros((HD // 2, 7 * T), u32)
        for cp in cp_vec:
            cp.wait()
        _ssm_params(vec_s, coef_s, lam_s, col_s)

        def wq_transpose(pair, tie):
            ht = pair // 4 if isinstance(pair, int) else lax.shift_right_logical(pair, 2)
            pad = jnp.zeros((T - QM, T), u32)
            for dt in range(2):
                for mq in range(4):
                    blk = sq[ht * 2 + dt, pl.ds(mq * QM * 4 + (pair & 3), QM, stride=4), :]
                    blk = jnp.concatenate([tie(blk[:8], 4 * dt + mq), blk[8:], pad], axis=0)
                    wqt_s[dt * HD:(dt + 1) * HD, mq * T:(mq + 1) * T] = blk.T

        def phase1(lo, hi, groups, gates):
            clk = _Clock(zero_s)
            cuts = [lo, lo + T] + list(range(lo + 4 * T, hi, 4 * T)) + [hi]
            for c0, c1 in zip(cuts[:-1], cuts[1:]):
                u = clk.dot(xT_s[:, c0:c1], b_s[...], _TT)
                for cb in range(4):
                    w = min(2 * T, 2 * M - cb * 2 * T)
                    u_s[cb, c0 // 8:c1 // 8, :, 0:w] = u[:, cb * 2 * T:cb * 2 * T + w].reshape((c1 - c0) // 8, 8, w)
            pacer = lambda n, f0=0.0, f1=1.0: clk.pacer(f0 * (clk.t - 500), f1 * (clk.t - 500), n)
            tie = pacer(49 * len(groups))
            for k, g in enumerate(groups):
                for r in range(0, QM, 16):
                    def block(o, q):
                        row, col = (o % 2) * HM + (q % 2) * QM + r, (4 * g + 2 * (q // 2) + o // 2) * T
                        return xT_s[row:row + 16, col:col + T].astype(f32) * (LOG2E * D ** -0.5)
                    for n1 in range(7):
                        ops = _operands2(_A_TERMS, n1, block, lambda x: tie(x, 49 * k + 7 * (r // 16) + n1))
                        _put(xa_s, g * QM + r, 7 * n1 * T, ops)
            tie = pacer(28 * len(gates))
            for t, tile in enumerate(gates):
                cols = slice(tile * T, (tile + 1) * T)
                acc = jnp.zeros((8, T), f32)
                for r in range(0, M, 32):
                    xg = xT_s[r:r + 32, cols].astype(f32) * tie(col_s[1, r:r + 32, :], 28 * t + r // 32)
                    acc = acc + jnp.sum(xg.reshape(4, 8, T), axis=0)
                g = jax.nn.sigmoid(jnp.sum(acc, axis=0, keepdims=True))
                g_s[:, cols] = g
                for r in range(0, M, 32):
                    skip = xT_s[r:r + 32, cols].astype(f32) * tie(col_s[0, r:r + 32, :], 28 * t + 14 + r // 32)
                    o_s[r:r + 32, cols] = (1.0 - g) * skip
            return pacer

        for cp in cp_b + [x_copy(0)]:
            cp.wait()
        phase1(XCUT[0], XCUT[1], [], range(XCUT[1] // T))
        x_copy(1).wait()
        pacer = phase1(XCUT[1], XCUT[2], range(XCUT[2] // TA), range(XCUT[1] // T, XCUT[2] // T))
        zero = jnp.zeros((1, 512), f32)
        carry0 = _ssm_scan(u_s.at[:, 0:TC // 8], (zero, zero), lam_s, h_s, h0_s, pacer(TC // 2))
        for cp in [x_copy(2)] + cp_c + cp_wq:
            cp.wait()
        pacer = phase1(XCUT[2], XCUT[3], range(XCUT[2] // TA, 4), range(XCUT[2] // T, S // T))
        _ssm_cmat(craw_s, coef_s, c_s, pacer(HM // 16))
        tie = pacer(M // 8)
        for c0 in range(0, M, 8):
            _stage(rq, sq, c0, 8, lambda x, j: tie(x, c0 / 10 + j), groups=(0,))
        wq_transpose(0, lambda x, k: tie(x, 46 + k))

        def phase2(i, carry):
            @pl.when(i + 1 < NP)
            def _():
                for cp in slice_copies(i + 1):
                    cp.start()

            @pl.when(i < 3)
            def _():
                wq1_copy(i + 1).start()

            wo_copy(i).start()

            @pl.when(i < 4)
            def _():
                wq1_copy(i).wait()

            for cp in slice_copies(i) + [w_copy(0, i), w_copy(1, i)]:
                cp.wait()

            clk = _Clock(zero_s)
            comb = clk.strassen(lambda n: _get(c_s, 0, HM, n * PA, PA), lambda n: _get(h_s, 0, T, n * PA, PA), _NT, 3)
            mixed = clk.level([(_get(c_s, 0, HM, 7 * PA + n // 2 * T, T), _get(h_s, 0, T, 7 * PA + n % 2 * T, T))
                               for n in range(4)], _NT)
            ty = clk.t
            cols = _ds(i * TC, TC, TC)
            keep = 1.0 - g_s[:, cols]
            for r in range(0, HM, 32):
                y = [c + m[r:r + 32] for c, m in zip(comb(r, 32), mixed)]
                o_s[r:r + 32, cols] += keep * jnp.concatenate(y[:2], axis=1)
                o_s[HM + r:HM + r + 32, cols] += keep * jnp.concatenate(y[2:], axis=1)

            q_i = q_s.at[_ds(i * 2 * D, 2 * D, 2 * D)]
            mq_s = (head_refs['mk_s'], head_refs['mp_s'], head_refs['mv_s'].at[0], head_refs['mv_s'].at[1])
            for g in range(4):
                for n1 in range(7):
                    if g == 0:
                        t = 200 + (ty + 644) * n1 / 7
                        tie = clk.pacer(min(t, clk.t - 500), min(t + 300, clk.t - 500), 8)
                        for r in range(0, 2 * QD, 16):
                            def block(o, q):
                                row = (o % 2) * HD + (q % 2) * QD + r % QD
                                col = (2 * (o // 2) + q // 2) * T
                                w = wqt_s[row:row + 16, col:col + T]
                                return _hi16(w) if r >= QD else pltpu.bitcast(w << 16, f32)
                            _put(wq_s, r, 7 * n1 * T, _operands2(_B_TERMS, n1, block, lambda x: tie(x, r // 16)))
                    comb = clk.strassen(lambda n: _get(wq_s, 0, 2 * QD, (7 * n1 + n) * T, QM),
                                        lambda n: _get(xa_s, g * QM, QM, (7 * n1 + n) * T, T), _NN)
                    for r in range(0, 2 * QD, 32):
                        e, c = r // QD, comb(r, 32)
                        for dq in range(2):
                            row = dq * QD + r % QD
                            done = _outer_step(mq_s[2 * (g % 2) + e], n1, row,
                                               jnp.concatenate([c[dq], c[2 + dq]], axis=1))
                            if done:
                                n, v = done
                                _put(q_i, (2 * e + n // 2) * D + (n % 2) * HD + row, 2 * g * T, [v])

            span = ty + 6000

            u_next = u_s.at[:, pl.ds(jnp.minimum(i + 1, NP - 1) * (TC // 8), TC // 8)]
            carry = _ssm_scan(u_next, carry, lam_s, h_s, h0_s, clk.pacer(ty, span, TC // 2))

            tie = clk.pacer(ty - 1200, span, 64, [(ty, ty + 1000)])
            rq_i = rq.at[pl.ds((i & 3) * (M // 4), M // 4)]
            sq_i = sq.at[:, _ds((i & 3) * M, M, 8)]
            for c0 in range(0, M // 4, 8):
                _stage(rq_i, sq_i, c0, 8, lambda x, j: tie(x, c0 // 4 + 4 * j), groups=(1,))
            wq_transpose(jnp.minimum(i + 1, NP - 1), lambda x, k: tie(x, 36 + 3 * k))
            for n, (raw, stg, wt_s) in enumerate(((rk, sk, wkt_s), (rv, sv, wvt_s))):
                for c0 in range(0, CS, 8):
                    _stage(raw, stg, c0, 8, lambda x, j: tie(x, 16 * n + c0 // 8 + j))

                @pl.when(i + 1 < NP)
                def _():
                    w_copy(n, i + 1).start()

                raw[CS, 0:8, 0:T] = tie(zero_s[...], 16 * n + 19).astype(bf16)
                cols = _ds(i * CS, CS, CS)
                for pair in range(H // 2):
                    for dt in range(2):
                        blk = stg[(pair // 4) * 2 + dt, pl.ds(pair % 4, CS, stride=4), :]
                        row = pair * D + dt * HD
                        blk = jnp.concatenate([tie(blk[:8], 16 + 24 * n + 3 * pair + dt), blk[8:]], axis=0)
                        wt_s[row:row + HD, cols] = blk.T

            tie = clk.pacer(ty + 1000, span, 28)
            ckv_i = ckv_s.at[i & (NRAW - 1)]
            a_i = a_s.at[_ds(i * (T // 4), T // 4, T // 4)]
            for r in range(0, T // 2, 16):
                def block(o, q):
                    col = (o % 2) * 2 * QC + (q % 2) * QC
                    return ckv_i[2 * (q // 2) + o // 2, r:r + 16, col:col + QC].astype(f32)
                for n1 in range(7):
                    ops = _operands2(_A_TERMS, n1, block, lambda x: tie(x, 7 * (r // 16) + n1))
                    _put(a_i, r, 7 * n1 * QC, ops)
            return carry

        lax.fori_loop(0, NP, phase2, carry0)
        for i in range(NP):
            wo_copy(i).wait()
        prep_w(h, range(NT1), _no_tie)

    @pl.when(h == 0)
    def _():
        prologue(**pro_refs)

    def oproj(jp, clk):
        cols = slice(2 * jp * T, (2 * jp + 2) * T)
        for r, n in OCH:
            c = clk.strassen(lambda i: _get(wl_s, r, n, i * T, T),
                             lambda i: _get(cl_s, 0, HD, (jp * 7 + i) * T, T), _NN)()
            o_s[r:r + n, cols] += jnp.concatenate(c[:2], axis=1)
            o_s[HM + r:HM + r + n, cols] += jnp.concatenate(c[2:], axis=1)

    def head(mk_s, mv_s, mp_s, kt_s, ka_s, va_s, v2_s, s_s, pb_s, pd_s, p2_s, sc_s, qb_s, kd_s):
        clk = _Clock(zero_s)
        q_h = q_s.at[_ds(h * D, D, D)]

        def prep_wo(tie):
            for r in range(0, HM, 16):
                top = tie(wo_s[h, r:r + 16, :].astype(f32), r // 16)
                bot = tie(wo_s[h, HM + r:HM + r + 16, :].astype(f32), r // 16)
                _put(wl_s, r, 0, _operands(_A_TERMS, [top[:, :HD], top[:, HD:], bot[:, :HD], bot[:, HD:]]))

        def proj(g, lo=0, hi=7):
            for n1 in range(lo, hi):
                comb = clk.strassen(lambda n: _get(w_s, 0, 2 * QD, (7 * n1 + n) * QC, QC),
                                    lambda n: _get(a_s, g * T, T, (7 * n1 + n) * QC, QC), _NT, 2, n1 == 6)
                for r, m_s in ((0, mk_s), (QD, mv_s.at[g % 2])):
                    c = comb(r, QD)
                    m_s[n1 * HD:n1 * HD + QD, :] = jnp.concatenate([c[0], c[2]], axis=1)
                    m_s[n1 * HD + QD:(n1 + 1) * HD, :] = jnp.concatenate([c[1], c[3]], axis=1)
            if hi < 7:
                return
            cs = [_combine([mk_s[n * HD + r:n * HD + r + 16, :] for n in range(7)], order=range(7))
                  for r in range(0, HD, 16)]
            for n in range(4):
                kt_s[:, n * T:(n + 1) * T] = jnp.concatenate([c[n] for c in cs], axis=0).T
            for r in range(0, 2 * T, T // 2):
                blk = kt_s[r:r + T // 2, :]
                blk = [blk[:, n * T:(n + 1) * T] for n in range(4)]
                _put(ka_s, 2 * g * T + r, 0, _operands(_A_TERMS, blk) + [blk[2]])
            for r in (0, 32, T, T + 32):
                lo_, hi_ = kt_s[r:r + 32, 0:2 * T], kt_s[r + T // 2:r + T // 2 + 32, 0:2 * T]
                _put(kd_s, r // T * (T // 2) + r % T, 0,
                     _operands(_A_TERMS, [lo_[:, :T], lo_[:, T:], hi_[:, :T], hi_[:, T:]]))

        def vfin(g, tie):
            m_s = mv_s.at[g % 2]
            for r in range(0, QD, 16):
                k, blk = 8 * (r // 16), {}
                late = lambda w: tie(w, k, True, LATE)
                for new, n1 in (((0,), 2), ((1,), 4), ((3,), 6), ((), 0), ((), 3), ((2,), 5), ((), 1)):
                    for o in new:
                        for i, row in enumerate((r, QD + r)):
                            tiles = _Rows([m_s.at[n * HD:(n + 1) * HD] for n in range(7)], row, 16)
                            c, = _combine(tiles, ((o % 2) * 2 + o // 2,), range(7))
                            blk[o, i] = c = tie(c, k)
                            slot = (2, 7, 8, 3)[o]
                            _put(va_s, row, ((2 * g + 1) * 9 + slot) * T, [c[:, T:]])
                            if o in (1, 2):
                                _put(va_s, row, (2 * g * 9 + slot) * T, [c[:, :T]])
                    lo_, hi_ = [_operand(_A_TERMS[n1], lambda o: blk[o, i]) for i in range(2)]
                    _put(va_s, r, (2 * g * 9 + n1) * T, [lo_[:, :T]], late)
                    _put(va_s, QD + r, (2 * g * 9 + n1) * T, [hi_[:, :T]], late)
                    if g < 3:
                        _put(v2_s, r, (g * 7 + n1) * 7 * T,
                             _operands(_A_TERMS, [lo_[:, :T], lo_[:, T:], hi_[:, :T], hi_[:, T:]]), late)
                    k += 8 / 7

        key = lax.broadcasted_iota(jnp.int32, (T, 2 * T), 0)
        qry = lax.broadcasted_iota(jnp.int32, (T, 2 * T), 1)
        causal = key <= qry

        marks = []

        def qk(g):
            pairs = (2 * g, 2 * g + 1)
            mx = {jp: _Reducer(jnp.max, jnp.maximum) for jp in pairs}

            def put(jp, row, v):
                v = v.reshape(v.shape[0] // 8, 8, 2 * T)
                s_s[jp % 4, row // 8:row // 8 + v.shape[0]] = v
                mx[jp].add(v)

            def rect(jp, lo, hi):
                for r in range(lo, hi, T // 2):
                    c = clk.strassen(lambda i: _get(ka_s, r, T // 2, i * T, T),
                                     lambda i: _get(qb_s, 0, HD, ((jp % 2) * 7 + i) * T, T), _NN)()
                    put(jp, r, jnp.concatenate(c[:2], axis=1))
                    put(jp, jp * T + r, jnp.concatenate(c[2:], axis=1))

            for jp in pairs:
                for r in range(0, HD, 32):
                    blk = [_get(q_h, e * D + d * HD + r, 32, jp * T, T).astype(f32) for d in range(2) for e in range(2)]
                    _put(qb_s, r, (jp % 2) * 7 * T, _operands(_B_TERMS, blk))
            for jp in pairs:
                rect(jp, 0, 2 * g * T)
                marks.append(clk.t)
            last = {}
            for jp in pairs:
                ko = jnp.concatenate([_get(ka_s, jp * T, T, n * T, T) for n in (7, 3)], axis=1)
                so = jnp.where(causal[:, :T], clk.dot(ko, _get(q_h, D, D, jp * T, T), _NN), NEG)
                row = (2 * jp + 1) * T // 8
                s_s[jp % 4, row:row + T // 8, :, T:] = so.reshape(T // 8, 8, T)
                last[jp] = jnp.concatenate([jnp.full((1, T), NEG, f32), jnp.max(so, axis=0, keepdims=True)], axis=1)
            rect(2 * g + 1, 2 * g * T, (2 * g + 1) * T)
            for jp in pairs:
                c = clk.strassen(lambda i: _get(kd_s, (jp % 2) * (T // 2), T // 2, i * T, T),
                                 lambda i: _get(qb_s, 0, HD, ((jp % 2) * 7 + i) * T, T), _NN)()
                se = jnp.concatenate([jnp.concatenate(c[:2], axis=1), jnp.concatenate(c[2:], axis=1)], axis=0)
                put(jp, 2 * jp * T, jnp.where(causal, se, NEG))
            return [jnp.broadcast_to(jnp.maximum(mx[jp].result(), last[jp]), (8, 2 * T)) for jp in pairs]

        zs, sums = {}, {}

        def prob(jp, row, z, n=GS, lanes=slice(None)):
            return jnp.exp2(s_s[jp % 4, row // 8:(row + n) // 8, :, lanes] - z[:, lanes])

        def rough(jp, mx, tie):
            zs[jp] = mx
            if jp > 0:
                sm = _Reducer(jnp.sum, jnp.add)
                for k, r in enumerate(range(0, 2 * jp * T, GS * LSUB)):
                    sm.add(prob(jp, r, tie(mx, k)))
                zs[jp] = mx + jnp.log2(jnp.maximum(LSUB * sm.result(), 1.0))
            sums[jp] = _Reducer(jnp.sum, jnp.add)

        def blocks(jp, row, tie, k):
            top, bot = prob(jp, row, tie(zs[jp], k)), prob(jp, jp * T + row, tie(zs[jp], k + 1))
            sums[jp].add(top + bot)
            top, bot = top.reshape(GS, 2 * T), bot.reshape(GS, 2 * T)
            return [top[:, :T], top[:, T:], bot[:, :T], bot[:, T:]]

        def near(jp, tie, k):
            R, z = jp * T, zs[jp]
            if jp % 2:
                for r in range(0, T, GS):
                    _put(pb_s, jp // 2 * T + r, 0, _operands(_B_TERMS, blocks(jp, R - T + r, tie, k)))
                    k += 2
            for r in range(0, T, GS):
                p = prob(jp, 2 * R + r, tie(z, k))
                sums[jp].add(p)
                _put(pd_s, 2 * R + r, 0, [p.reshape(GS, 2 * T)])
                k += 1
            so = _Reducer(jnp.sum, jnp.add)
            for r in range(0, T, 2 * GS):
                p = prob(jp, 2 * R + T + r, tie(z, k), 2 * GS, slice(T, 2 * T))
                so.add(p)
                _put(pd_s, 2 * R + T + r, T, [p.reshape(2 * GS, T)])
                k += 1
            sums[jp].result()
            sums[jp].out = sums[jp].out + jnp.concatenate([jnp.zeros((1, T), f32), so.result()], axis=1)

        p20 = lambda g: g * (g - 1) // 2 * T

        def far(g, tie, k):
            half = {(jp, e): _Reducer(jnp.sum, jnp.add) for jp in (2 * g, 2 * g + 1) for e in range(2)}
            for kg in range(g):
                for r in range(0, T, GS):
                    blk = {}
                    for new, n1 in (((0,), 1), ((1,), 5), ((3,), 2), ((), 0), ((), 4), ((2,), 3), ((), 6)):
                        for o in new:
                            lanes = slice((o % 2) * T, (o % 2 + 1) * T)
                            for jp in (2 * g, 2 * g + 1):
                                z = tie(zs[jp][:, lanes], k)
                                row = (o // 2) * jp * T + 2 * kg * T + r
                                p = [jnp.exp2(s_s[jp % 4, x // 8:(x + GS) // 8, :, lanes] - z) for x in (row, row + T)]
                                half[jp, o % 2].add(p[0] + p[1])
                                blk[o, jp % 2], blk[o, 2 + jp % 2] = [x.reshape(GS, T) for x in p]
                        ops = _operands2(_B_TERMS, n1, lambda o, q: blk[o, q], lambda x: x)
                        _put(p2_s, p20(g) + kg * T + r, 7 * n1 * T, ops, lambda w: tie(w, k, True, LATE))
                        k += 16 / 7
            for jp in (2 * g, 2 * g + 1):
                if g:
                    sums[jp].out = sums[jp].out + jnp.concatenate([half[jp, e].result() for e in range(2)], axis=1)
            for jp in (2 * g, 2 * g + 1):
                cols = slice(2 * jp * T, 2 * (jp + 1) * T)
                sc_s[:, cols] = g_s[:, cols] / sums[jp].result()

        def pv(g):
            pairs = (2 * g, 2 * g + 1)
            va = lambda n, t, r=0, nr=HD: _get(va_s, r, nr, (t * 9 + n) * T, T)
            for n1 in range(7 if g else 0):
                c = clk.strassen(
                    lambda n: _cat([_get(v2_s, 0, QD, (kg * 49 + 7 * n1 + n) * T, T) for kg in range(g)], 1),
                    lambda n: _get(p2_s, p20(g), g * T, (7 * n1 + n) * T, T), _NN, g)()
                mp_s[n1 * HD:n1 * HD + QD, :] = jnp.concatenate(c[:2], axis=1)
                mp_s[n1 * HD + QD:(n1 + 1) * HD, :] = jnp.concatenate(c[2:], axis=1)
            if g == 3:
                vfin(3, clk.pacer(clk.t - 2000, clk.t - 1200, 32))
            ve = [jnp.concatenate([va(2, jp), va(8, jp)], axis=0) for jp in pairs]
            vo = [jnp.concatenate([va(7, jp), va(3, jp)], axis=0) for jp in pairs]
            ce = clk.level([(ve[jp % 2], _get(pd_s, 2 * jp * T, T, 0, T)) for jp in pairs])
            co = [clk.dot(jnp.concatenate([ve[jp % 2], vo[jp % 2]], axis=1),
                          _get(pd_s, 2 * jp * T, 2 * T, T, T), _NN) for jp in pairs]
            for jp in pairs:
                R, e = jp * T, jp % 2
                ge, go = sc_s[:, 2 * R:2 * R + T], sc_s[:, 2 * R + T:2 * R + 2 * T]
                for r in range(0, HD, 32):
                    c = [ce[e][r:r + 32], co[e][r:r + 32], ce[e][HD + r:HD + r + 32], co[e][HD + r:HD + r + 32]]
                    if g:
                        far_ = _combine([mp_s[n * HD + r:n * HD + r + 32, e * T:(e + 1) * T] for n in range(7)],
                                        order=range(7))
                        c = [x + y for x, y in zip(c, far_)]
                    if e:
                        near_ = clk.strassen(lambda n: va(n, 2 * g, r, 32),
                                             lambda n: _get(pb_s, g * T, T, n * T, T), _NN)()
                        c = [x + y for x, y in zip(c, near_)]
                    ops = _operands(_B_TERMS, [c[0] * ge, c[1] * go, c[2] * ge, c[3] * go])
                    _put(cl_s, r, jp * 7 * T, ops)

        ends = []

        def run(items):
            for item in items.split():
                if item[0] == 'P':
                    pv(int(item[1]))
                    ends.append(clk.t)
                elif item[0] == 'K':
                    proj(int(item[1]), 2 if item == 'K1' else 0)
                else:
                    jp = int(item[1])
                    oproj(jp, clk)

                    @pl.when(h == H - 1)
                    def _():
                        out_copy(jp).start()

        oproj(NP - 1, clk)
        for n1 in range(7):
            if n1 >= NT1:
                prep_w(h, [n1], clk.pacer(clk.t - 896, clk.t - 448, 8))
            proj(0, n1, n1 + 1)
        proj(1, 0, 2)
        mx = qk(0)
        for g in range(4):
            t0 = clk.t
            del ends[:]
            run(PLAN[g])
            t1 = clk.t
            nxt = qk(g + 1) if g < 3 else None
            n_rough = [2 * jp * T // (GS * LSUB) for jp in (2 * g, 2 * g + 1)]
            n_near = [(T + T // 2) // GS, (3 * T + T // 2) // GS]
            holes = [(t - 400, t) for t in ends]
            if 0 < g < 3:
                holes.append((marks[-2] - 400, marks[-2] - 100))
            if g < 3:
                vfin(g, clk.pacer(t0, t0 + VW, 32))
                holes += [(t0, t0 + VW), (t1 - 300, t1 + 300)]
            if g == 2:
                holes.append((clk.t - 300, clk.t))
            tie = clk.pacer(t0, (clk.t if g else t1) - SLACK,
                            sum(n_rough) + sum(n_near) + g * 16 * T // GS, holes)
            rough(2 * g, mx[0], tie)
            near(2 * g, tie, n_rough[0])
            k = n_rough[0] + n_near[0]
            rough(2 * g + 1, mx[1], lambda x, i: tie(x, k + i))
            near(2 * g + 1, tie, k + n_rough[1])
            far(g, tie, k + n_rough[1] + n_near[1])
            if g == 0:
                prep_wo(clk.pacer(t0 + VW, t1 - 300, HM // 16))
            mx = nxt
        t0 = clk.t
        run(PLAN[4])
        prep_w(jnp.minimum(h + 1, H - 1), range(NT1), clk.pacer(t0 - 100, clk.t - 500, 8 * NT1))
        assert len(set(clk.load)) == 1

    head(**head_refs)

    @pl.when(h == H - 1)
    def _():
        oproj(NP - 1, _Clock(zero_s))
        out_copy(NP - 1).start()
        for jp in range(NP):
            out_copy(jp).wait()


@jax.jit
def pallas_gated_mix__compressed_kv_cla__ssm_conv_s5__prompt_kernel(
    A_x: jax.Array,
    A_c_kv: jax.Array,
    A_w_q: jax.Array,
    A_w_uk: jax.Array,
    A_w_uv: jax.Array,
    A_w_o: jax.Array,
    B_x: jax.Array,
    B_Lambda_re: jax.Array,
    B_Lambda_im: jax.Array,
    B_B_re: jax.Array,
    B_B_im: jax.Array,
    B_C_re: jax.Array,
    B_C_im: jax.Array,
    B_log_dt: jax.Array,
    B_Dskip: jax.Array,
    gate_w: jax.Array,
):
    del B_x
    xT = jnp.transpose(A_x[0])
    woT = jnp.transpose(A_w_o, (0, 2, 1))
    ckv = A_c_kv.reshape(4, 4, 2, T // 2, DC)

    hbm = pl.BlockSpec(memory_space=pl.ANY)
    outT = pl.pallas_call(
        _kernel,
        grid=(H,),
        in_specs=[hbm] * 15,
        out_specs=hbm,
        out_shape=jax.ShapeDtypeStruct((M, S), f32),
        scratch_shapes=_SHARED_SCRATCH + list(_PROLOGUE_SCRATCH.values()) + list(_HEAD_SCRATCH.values()),
        compiler_params=pltpu.CompilerParams(
            dimension_semantics=("arbitrary",),
            vmem_limit_bytes=127 * 1024 * 1024,
            disable_bounds_checks=True,
        ),
    )(xT, B_B_re, B_B_im, B_C_re, B_C_im, B_Lambda_re, B_Lambda_im, B_log_dt,
      B_Dskip, gate_w, woT, ckv, A_w_q, A_w_uk, A_w_uv)
    return jnp.transpose(outT)[None]
```

```python
import bisect

import jax
import jax.numpy as jnp
from jax import lax
import jax.experimental.pallas as pl
import jax.experimental.pallas.tpu as pltpu

S = 2048
M = 448
H = 16
D = 256
DC = 1024
T = 128
NP = S // T // 2
HD = D // 2
HM = M // 2
QD = D // 4
QC = DC // 4
QM = M // 4
PA = 384
PB = M - PA
TA = 512
XCUT = (0, 256, 1152, 2048)
TC = 256
CS = DC // NP
LOG2E = 1.4426950408889634
NEG = -1e30

GS = 16
RCH = 256
LSUB = 4
NT1 = 2
OCH = ((0, 64), (64, 64), (128, 48), (176, 48))
PLAN = ('K1', 'K2', 'K3', 'P1 P0 O2 O3 P2 O0 O1 O4 O5', 'P3 O6')
SLACK, LATE, VW = 200, 40, 900

f32 = jnp.float32
bf16 = jnp.bfloat16
u32 = jnp.uint32

SEM_VEC, SEM_B, SEM_X, SEM_WQ, SEM_C, SEM_CKV, SEM_WO, SEM_OUT, SEM_WQ1, SEM_KV = 0, 1, 2, 5, 6, 7, 8, 9, 10, 14
NSEM = 16

_NN = ((1,), (0,))
_NT = ((1,), (1,))
_TT = ((0,), (1,))


def _cat(xs, axis):
    return xs[0] if len(xs) == 1 else jnp.concatenate(xs, axis=axis)


def _ds(lo, n, align):
    return pl.ds(lo if isinstance(lo, int) else pl.multiple_of(lo, align), n)


def _put(ref, row, col, xs, tie=None):
    x = _cat(xs, 1)
    if tie is not None:
        x = jnp.concatenate([tie(x[:8]), x[8:]], axis=0)
    ref[row // 2:(row + x.shape[0]) // 2, col:col + x.shape[1]] = pltpu.bitcast(x.astype(bf16), u32)


def _get(ref, row, nrows, col, ncols):
    return pltpu.bitcast(ref[row // 2:(row + nrows) // 2, col:col + ncols], bf16)


class _Clock:
    def __init__(self, zero_ref):
        self.masks = {(8, T): zero_ref[...] != 0.0}
        self.ticks, self.load = [], [0, 0, 0, 0]

    @property
    def t(self):
        return max(self.load)

    def dot(self, a, b, dims):
        v = lax.dot_general(a, b, (dims, ((), ())), preferred_element_type=f32)
        rows, depth = v.shape[0], a.shape[dims[0][0]]
        for c in range(0, v.shape[1], T):
            start = 0
            for _ in range(0, depth, T):
                k = self.load.index(min(self.load))
                start = max(start, self.load[k])
                self.load[k] += rows
            self.ticks += [(start + r + 8, (v, r, c)) for r in range(0, rows, 8)]
        return v

    def strassen(self, lhs, rhs, dims, jobs=1, split_last=False):
        lag = sum(l + 32 <= max(self.load) for l in self.load) // jobs if jobs < 3 else 0
        order = ((1, 3, 2, 4, 0, 5, 6), (0, 1, 3, 2, 4, 5, 6), (5, 6, 1, 3, 2, 4, 0), (0, 5, 6, 1, 3, 2, 4))[lag]
        m = {}
        for n in order:
            a, b = lhs(n), rhs(n)
            if split_last and n == order[-1]:
                half = a.shape[0] // 2
                m[n] = jnp.concatenate([self.dot(a[:half], b, dims), self.dot(a[half:], b, dims)], axis=0)
            else:
                m[n] = self.dot(a, b, dims)
        return lambda r=0, n=None: _combine(m if n is None else _Rows(m, r, n), order=order)

    def level(self, pairs, dims=_NN):
        base, extra = divmod((sum(self.load) + sum(a.shape[0] for a, _ in pairs)) // 16, 4)
        target = [16 * (base + (k < extra)) for k in range(4)]
        out = []
        for a, b in pairs:
            r, parts = 0, []
            while r < a.shape[0]:
                k = self.load.index(min(self.load))
                n = min(max(target[k] - self.load[k], 16), a.shape[0] - r)
                parts.append(self.dot(a[r:r + n], b, dims))
                r += n
            out.append(_cat(parts, 0))
        return out

    def pacer(self, t0, t1, n, holes=()):
        holes = sorted((max(a, t0), min(b, t1)) for a, b in holes if a < t1 and b > t0)
        gap = sum(b - a for a, b in holes)
        ticks = sorted(self.ticks, key=lambda tw: tw[0])
        times = [tw[0] for tw in ticks]

        def tie(x, k, distinct=False, delay=0):
            t = t0 + (t1 - t0 - gap) * k / n
            for a, b in holes:
                t += b - a if t > a else 0
            t += delay
            past = ticks[:bisect.bisect_right(times, t)]
            reps = (x.shape[0] // 8, x.shape[1] // T)
            if len(past) < (reps[1] if distinct else 1):
                return x
            tick = _cat([v[r:r + 8, c:c + T] for _, (v, r, c) in past[-reps[1] if distinct else -1:]], 1)
            if tick.dtype != x.dtype:
                tick = pltpu.bitcast(tick, x.dtype)
            if x.shape not in self.masks:
                self.masks[x.shape] = jnp.tile(self.masks[(8, T)], reps)
            return lax.select(self.masks[x.shape], tick if tick.shape == x.shape else jnp.tile(tick, reps), x)
        return tie


def _no_tie(x, k):
    return x


_A_TERMS = ((0, 3, 1), (2, 3, 1), (0, None, 0), (3, None, 0), (0, 1, 1), (2, 0, -1), (1, 3, -1))
_B_TERMS = ((0, 3, 1), (0, None, 0), (1, 3, -1), (2, 0, -1), (3, None, 0), (0, 1, 1), (2, 3, 1))


def _operand(term, block):
    x, y, sign = term
    if y is None:
        return block(x)
    return block(x) + block(y) if sign > 0 else block(x) - block(y)


def _operands(terms, blocks):
    return [_operand(t, blocks.__getitem__) for t in terms]


def _operands2(terms, n1, block, tie):
    first = terms[n1][0]
    sub = [_operand(terms[n1], lambda o: tie(block(o, q)) if o == first and q in (0, 3) else block(o, q))
           for q in range(4)]
    return _operands(terms, sub)


_C_TERMS = ({0: 1, 3: 1, 4: -1, 6: 1}, {2: 1, 4: 1}, {1: 1, 3: 1}, {0: 1, 1: -1, 2: 1, 5: 1})


def _combine(m, only=(0, 1, 2, 3), order=(1, 3, 2, 4, 0, 5, 6)):
    out = []
    for terms in (_C_TERMS[n] for n in only):
        seq = [n for n in order if n in terms]
        if terms[seq[0]] < 0:
            seq[0], seq[1] = seq[1], seq[0]
        acc = m[seq[0]]
        for n in seq[1:]:
            acc = acc + m[n] if terms[n] > 0 else acc - m[n]
        out.append(acc)
    return out


def _outer_step(m_s, n1, row, v):
    n = v.shape[0]
    if n1 < 5:
        m_s[n1 * HD + row:n1 * HD + row + n, :] = v
    if n1 < 3:
        return None
    blk = (2, 1, 3, 0)[n1 - 3]
    m = {j: v if j == n1 else m_s[j * HD + row:j * HD + row + n, :] for j in _C_TERMS[blk]}
    return blk, _combine(m, (blk,), range(7))[0]


class _Rows:
    def __init__(self, vals, r, n):
        self.vals, self.rows, self.cache = vals, slice(r, r + n), {}

    def __getitem__(self, i):
        if i not in self.cache:
            self.cache[i] = self.vals[i][self.rows, :]
        return self.cache[i]


class _Reducer:
    def __init__(self, red, comb):
        self.red, self.comb, self.acc, self.rows, self.out = red, comb, None, 0, None

    def add(self, v):
        self.rows += 8 * v.shape[0]
        v = self.red(v, axis=0)
        self.acc = v if self.acc is None else self.comb(self.acc, v)
        if self.rows >= RCH:
            self.result()

    def result(self):
        if self.acc is not None:
            v = self.red(self.acc, axis=0, keepdims=True)
            self.out = v if self.out is None else self.comb(self.out, v)
        self.acc, self.rows = None, 0
        return self.out


def _cmul(ar, ai, br, bi):
    return ar * br - ai * bi, ar * bi + ai * br


def _hi16(w):
    return pltpu.bitcast(w & jnp.uint32(0xFFFF0000), f32)


def _stage(raw, stg, c0, nc, tie, groups=(0, 1)):
    for ht in groups:
        for dt in range(2):
            v = raw[c0:c0 + nc, ht * 8:(ht + 1) * 8, dt * T:(dt + 1) * T].reshape(nc * 8, T)
            stg[ht * 2 + dt, c0 * 4:(c0 + nc) * 4, :] = tie(pltpu.bitcast(v, u32), (ht * 2 + dt) / 4)


def _ssm_params(vec_s, coef_s, lam_s, col_s):
    row = lambda r: r[...].astype(f32).reshape(1, M)
    lre, lim, ldt, dsk, gw = [row(v) for v in vec_s]
    dt = jnp.exp(ldt).astype(bf16).astype(f32)
    mag = jnp.exp(dt * lre)
    ang = dt * lim
    lr, li = mag * jnp.cos(ang), mag * jnp.sin(ang)
    den = lre * lre + lim * lim
    nr = lr - 1.0
    coef_s[...] = jnp.zeros(coef_s.shape, f32)
    coef_s[0:1, 0:M] = 2.0 * ((nr * lre + li * lim) / den)
    coef_s[1:2, 0:M] = 2.0 * ((li * lre - nr * lim) / den)

    er = jnp.concatenate([lr, lr[:, PA:]], axis=1)
    ei = jnp.concatenate([li, -li[:, PA:]], axis=1)
    pw = [(er, ei)]
    for _ in range(7):
        pw.append(_cmul(pw[-1][0], pw[-1][1], er, ei))
    sub = lax.broadcasted_iota(jnp.int32, (8, 512), 0)
    for n, d in enumerate((1, 2, 4)):
        lam_s[2 * n] = jnp.where(sub >= d, pw[d - 1][0], 0.0)
        lam_s[2 * n + 1] = jnp.where(sub >= d, pw[d - 1][1], 0.0)
    lcr = jnp.zeros((8, 512), f32)
    lci = jnp.zeros((8, 512), f32)
    for r in range(8):
        lcr = jnp.where(sub == r, pw[r][0], lcr)
        lci = jnp.where(sub == r, pw[r][1], lci)
    lam_s[6] = lcr
    lam_s[7] = lci

    def col(v):
        v = jnp.concatenate([v, jnp.zeros((1, 512 - M), f32)], axis=1)
        return jnp.broadcast_to(v, (T, 512)).T[:M]
    col_s[0] = col(dsk)
    col_s[1] = col(gw)


def _ssm_cmat(craw_s, coef_s, c_s, tie):
    for r in range(0, HM, 16):
        for c in range(0, M, T):
            w = min(T, M - c)
            coef = tie(coef_s[:, c:c + T], r // 16 + c / 512)
            cr, ci = coef[0:1, :w], coef[1:2, :w]
            blk = []
            for row in (r, HM + r):
                re, im = _cmul(craw_s[0, row:row + 16, c:c + w].astype(f32),
                               craw_s[1, row:row + 16, c:c + w].astype(f32), cr, ci)
                blk += [re, -im]
            if c < PA:
                for n, op in enumerate(_operands(_A_TERMS, blk)):
                    _put(c_s, r, n * PA + c, [op])
            else:
                _put(c_s, r, 7 * PA, blk)


def _ssm_scan(u_ref, carry, lam_s, h_s, h0_s, tie):
    car, cai = carry
    out = []
    for b in range(TC // 8):
        mixed = u_ref[3, b, :, 0:T]
        u = jnp.concatenate([u_ref[cb, b] for cb in range(3)], axis=1)
        cols = [u[:, 0:T], u[:, T:2 * T], u[:, 2 * T:PA], mixed]
        hr = jnp.concatenate([tie(v, 4 * b + n) for n, v in enumerate(cols)], axis=1)
        hi = jnp.concatenate([u[:, PA:2 * PA], pltpu.roll(mixed, PB, 1)], axis=1)
        for n, d in enumerate((1, 2, 4)):
            sr, si = pltpu.roll(hr, d, 0), pltpu.roll(hi, d, 0)
            tr, ti = _cmul(sr, si, lam_s[2 * n], lam_s[2 * n + 1])
            hr, hi = hr + tr, hi + ti
        tr, ti = _cmul(lam_s[6], lam_s[7], car, cai)
        hr, hi = hr + tr, hi + ti
        car, cai = hr[7:8, :], hi[7:8, :]
        out.append(jnp.concatenate([hr[:, :PA], hi[:, :PA], hr[:, PA:]], axis=1))
        if b % 2 == 1:
            v, row = jnp.concatenate(out, axis=0), (b - 1) * 8 % T
            _put(h_s, row, 7 * PA + b // 16 * T, [v[:, 2 * PA:]])
            if b < 16:
                h0_s[row:row + 16, :] = v[:, :2 * PA]
            else:
                v0 = h0_s[row:row + 16, :]
                _put(h_s, row, 0, _operands(_B_TERMS, [v0[:, :PA], v[:, :PA], v0[:, PA:], v[:, PA:2 * PA]]))
            out = []
    return car, cai


_vmem = pltpu.VMEM
_PROLOGUE_SCRATCH = dict(
    xT_s=_vmem((M, S), bf16),
    v0=_vmem((M,), bf16), v1=_vmem((M,), bf16), v2=_vmem((M,), bf16), v3=_vmem((M,), bf16), v4=_vmem((M,), bf16),
    b_s=_vmem((2 * M, M), bf16),
    craw_s=_vmem((2, M, M), bf16),
    c_s=_vmem((HM // 2, 7 * PA + 2 * T), u32),
    coef_s=_vmem((8, 512), f32),
    lam_s=_vmem((8, 8, 512), f32),
    col_s=_vmem((2, M, T), f32),
    h_s=_vmem((T // 2, 7 * PA + 2 * T), u32),
    h0_s=_vmem((T, 2 * PA), f32),
    ckv_s=_vmem((5, T // 2, DC), bf16),
    rq=_vmem((M, H, D), bf16),
    rk=_vmem((CS + 1, H, D), bf16),
    rv=_vmem((CS + 1, H, D), bf16),
    sq=_vmem((4, M * 4 + 8, T), u32),
    sk=_vmem((4, CS * 4 + 8, T), u32),
    sv=_vmem((4, CS * 4 + 8, T), u32),
    wqt_s=_vmem((D, 4 * T), u32),
)
_HEAD_SCRATCH = dict(
    mk_s=_vmem((7 * HD, 2 * T), f32),
    mv_s=_vmem((2, 7 * HD, 2 * T), f32),
    mp_s=_vmem((7 * HD, 2 * T), f32),
    kt_s=_vmem((2 * T, 4 * T), f32),
    ka_s=_vmem((S // 4, 8 * T), u32),
    va_s=_vmem((HD // 2, NP * 9 * T), u32),
    v2_s=_vmem((QD // 2, 3 * 49 * T), u32),
    s_s=_vmem((4, S // 8, 8, 2 * T), f32),
    pb_s=_vmem((2 * T, 7 * T), u32),
    pd_s=_vmem((S // 2, 2 * T), u32),
    p2_s=_vmem((3 * T, 49 * T), u32),
    sc_s=_vmem((1, S), f32),
    qb_s=_vmem((HD // 2, 14 * T), u32),
    kd_s=_vmem((T // 2, 7 * T), u32),
)
_SHARED_SCRATCH = [
    _vmem((H // 2 * D, DC), u32),
    _vmem((H // 2 * D, DC), u32),
    _vmem((S // 8, 49 * QC), u32),
    _vmem((H * D, S // 2), u32),
    _vmem((H, M, D), bf16),
    _vmem((QD, 49 * QC), u32),
    _vmem((HM // 2, 7 * T), u32),
    _vmem((HD // 2, NP * 7 * T), u32),
    _vmem((M, S), f32),
    _vmem((1, S), f32),
    _vmem((8, T), f32),
    pltpu.SemaphoreType.DMA((NSEM,)),
]


def _kernel(xT_hbm, bre_hbm, bim_hbm, cre_hbm, cim_hbm, lre_hbm, lim_hbm, ldt_hbm,
            dsk_hbm, gw_hbm, woT_hbm, ckv_hbm, wq_hbm, wk_hbm, wv_hbm,
            out_hbm,
            wkt_s, wvt_s, a_s, q_s, wo_s, w_s, wl_s, cl_s, o_s, g_s, zero_s, sem, *rest):
    h = pl.program_id(0)
    pro_refs = dict(zip(_PROLOGUE_SCRATCH, rest))
    head_refs = dict(zip(_HEAD_SCRATCH, rest[len(pro_refs):]))

    def out_copy(jp):
        cols = pl.ds(jp * 2 * T, 2 * T)
        return pltpu.make_async_copy(o_s.at[:, cols], out_hbm.at[:, cols], sem.at[SEM_OUT])

    def prep_w(hh, outer, tie):
        rows = _ds(lax.shift_right_logical(hh, 1) * D, D, D)
        sh = (16 * (1 - (hh & 1))).astype(u32)
        k = 0
        for row0, wt_s in ((0, wkt_s.at[rows]), (QD, wvt_s.at[rows])):
            for r in range(0, QD, 16):
                def block(o, q):
                    row = (o % 2) * HD + (q % 2) * QD + r
                    col = (o // 2) * 2 * QC + (q // 2) * QC
                    return _hi16(wt_s[row:row + 16, col:col + QC] << sh)
                for n1 in outer:
                    _put(w_s, row0 + r, 7 * n1 * QC, _operands2(_B_TERMS, n1, block, lambda x: tie(x, k)))
                    k += 1

    def prologue(xT_s, v0, v1, v2, v3, v4, b_s, craw_s, c_s, coef_s, lam_s, col_s, h_s, h0_s,
                 ckv_s, rq, rk, rv, sq, sk, sv, wqt_s):
        xa_s = head_refs['p2_s']
        wq_s = xa_s.at[2 * QM:2 * QM + QD]
        u_s = head_refs['s_s']
        vec_s = (v0, v1, v2, v3, v4)

        def ckv_copy(i):
            grp = i // 2 if isinstance(i, int) else lax.shift_right_logical(i, 1)
            return pltpu.make_async_copy(ckv_hbm.at[grp, :, i & 1], ckv_s.at[0:4], sem.at[SEM_CKV])

        def w_copy(n, i):
            src, dst = ((wk_hbm, rk), (wv_hbm, rv))[n]
            return pltpu.make_async_copy(src.at[pl.ds(i * CS, CS)], dst.at[0:CS], sem.at[SEM_KV + n])

        def wo_copy(i):
            heads = pl.ds(2 * i, 2)
            return pltpu.make_async_copy(woT_hbm.at[heads], wo_s.at[heads], sem.at[SEM_WO])

        def wq1_copy(i):
            rows = pl.ds(i * (M // 4), M // 4)
            return pltpu.make_async_copy(wq_hbm.at[rows, 8:16], rq.at[rows, 8:16], sem.at[SEM_WQ1 + i])

        def x_copy(i):
            cols = pl.ds(XCUT[i], XCUT[i + 1] - XCUT[i])
            return pltpu.make_async_copy(xT_hbm.at[:, cols], xT_s.at[:, cols], sem.at[SEM_X + i])

        cp_vec = [pltpu.make_async_copy(src, dst, sem.at[SEM_VEC])
                  for src, dst in zip((lre_hbm, lim_hbm, ldt_hbm, dsk_hbm, gw_hbm), vec_s)]
        cp_b = [pltpu.make_async_copy(src.at[pl.ds(lo, n)], b_s.at[pl.ds(dst, n)], sem.at[SEM_B])
                for src, lo, n, dst in ((bre_hbm, 0, PA, 0), (bim_hbm, 0, PA, PA),
                                        (bre_hbm, PA, PB, 2 * PA), (bim_hbm, PA, PB, 2 * PA + PB))]
        cp_wq = [pltpu.make_async_copy(wq_hbm.at[:, 0:8], rq.at[:, 0:8], sem.at[SEM_WQ])]
        cp_c = [pltpu.make_async_copy(src, craw_s.at[n], sem.at[SEM_C])
                for n, src in enumerate((cre_hbm, cim_hbm))]
        for cp in cp_vec + cp_b + [x_copy(i) for i in range(3)] + cp_c + cp_wq:
            cp.start()
        for cp in [wq1_copy(0), ckv_copy(0), w_copy(0, 0), w_copy(1, 0)]:
            cp.start()

        zero_s[...] = jnp.zeros(zero_s.shape, f32)
        wl_s[...] = jnp.zeros(wl_s.shape, u32)
        for stg in (sq, sk, sv):
            stg[:, stg.shape[1] - 8:, :] = jnp.zeros((4, 8, T), u32)
        cl_s[:, (NP - 1) * 7 * T:] = jnp.zeros((HD // 2, 7 * T), u32)
        for cp in cp_vec:
            cp.wait()
        _ssm_params(vec_s, coef_s, lam_s, col_s)

        def wq_transpose(pair, tie):
            ht = pair // 4 if isinstance(pair, int) else lax.shift_right_logical(pair, 2)
            pad = jnp.zeros((T - QM, T), u32)
            for dt in range(2):
                for mq in range(4):
                    blk = sq[ht * 2 + dt, pl.ds(mq * QM * 4 + (pair & 3), QM, stride=4), :]
                    blk = jnp.concatenate([tie(blk[:8], 4 * dt + mq), blk[8:], pad], axis=0)
                    wqt_s[dt * HD:(dt + 1) * HD, mq * T:(mq + 1) * T] = blk.T

        def phase1(lo, hi, groups, gates):
            clk = _Clock(zero_s)
            cuts = [lo, lo + T] + list(range(lo + 4 * T, hi, 4 * T)) + [hi]
            for c0, c1 in zip(cuts[:-1], cuts[1:]):
                u = clk.dot(xT_s[:, c0:c1], b_s[...], _TT)
                for cb in range(4):
                    w = min(2 * T, 2 * M - cb * 2 * T)
                    u_s[cb, c0 // 8:c1 // 8, :, 0:w] = u[:, cb * 2 * T:cb * 2 * T + w].reshape((c1 - c0) // 8, 8, w)
            pacer = lambda n: clk.pacer(0, clk.t - 500, n)
            tie = pacer(49 * len(groups))
            for k, g in enumerate(groups):
                for r in range(0, QM, 16):
                    def block(o, q):
                        row, col = (o % 2) * HM + (q % 2) * QM + r, (4 * g + 2 * (q // 2) + o // 2) * T
                        return xT_s[row:row + 16, col:col + T].astype(f32) * (LOG2E * D ** -0.5)
                    for n1 in range(7):
                        ops = _operands2(_A_TERMS, n1, block, lambda x: tie(x, 49 * k + 7 * (r // 16) + n1))
                        _put(xa_s, g * QM + r, 7 * n1 * T, ops)
            tie = pacer(28 * len(gates))
            for t, tile in enumerate(gates):
                cols = slice(tile * T, (tile + 1) * T)
                acc = jnp.zeros((8, T), f32)
                for r in range(0, M, 32):
                    xg = xT_s[r:r + 32, cols].astype(f32) * tie(col_s[1, r:r + 32, :], 28 * t + r // 32)
                    acc = acc + jnp.sum(xg.reshape(4, 8, T), axis=0)
                g = jax.nn.sigmoid(jnp.sum(acc, axis=0, keepdims=True))
                g_s[:, cols] = g
                for r in range(0, M, 32):
                    skip = xT_s[r:r + 32, cols].astype(f32) * tie(col_s[0, r:r + 32, :], 28 * t + 14 + r // 32)
                    o_s[r:r + 32, cols] = (1.0 - g) * skip
            return pacer

        for cp in cp_b + [x_copy(0)]:
            cp.wait()
        phase1(XCUT[0], XCUT[1], [], range(XCUT[1] // T))
        x_copy(1).wait()
        pacer = phase1(XCUT[1], XCUT[2], range(XCUT[2] // TA), range(XCUT[1] // T, XCUT[2] // T))
        zero = jnp.zeros((1, 512), f32)
        carry0 = _ssm_scan(u_s.at[:, 0:TC // 8], (zero, zero), lam_s, h_s, h0_s, pacer(TC // 2))
        for cp in [x_copy(2)] + cp_c + cp_wq:
            cp.wait()
        pacer = phase1(XCUT[2], XCUT[3], range(XCUT[2] // TA, 4), range(XCUT[2] // T, S // T))
        _ssm_cmat(craw_s, coef_s, c_s, pacer(HM // 16))
        tie = pacer(M // 8)
        for c0 in range(0, M, 8):
            _stage(rq, sq, c0, 8, lambda x, j: tie(x, c0 / 10 + j), groups=(0,))
        wq_transpose(0, lambda x, k: tie(x, 46 + k))

        def phase2(i, carry):
            @pl.when(i < 3)
            def _():
                wq1_copy(i + 1).start()

            wo_copy(i).start()

            @pl.when(i < 4)
            def _():
                wq1_copy(i).wait()

            for cp in [ckv_copy(i), w_copy(0, i), w_copy(1, i)]:
                cp.wait()

            clk = _Clock(zero_s)
            comb = clk.strassen(lambda n: _get(c_s, 0, HM, n * PA, PA), lambda n: _get(h_s, 0, T, n * PA, PA), _NT, 3)
            mixed = clk.level([(_get(c_s, 0, HM, 7 * PA + n // 2 * T, T), _get(h_s, 0, T, 7 * PA + n % 2 * T, T))
                               for n in range(4)], _NT)
            ty = clk.t
            cols = _ds(i * TC, TC, TC)
            keep = 1.0 - g_s[:, cols]
            for r in range(0, HM, 32):
                y = [c + m[r:r + 32] for c, m in zip(comb(r, 32), mixed)]
                o_s[r:r + 32, cols] += keep * jnp.concatenate(y[:2], axis=1)
                o_s[HM + r:HM + r + 32, cols] += keep * jnp.concatenate(y[2:], axis=1)

            q_i = q_s.at[_ds(i * 2 * D, 2 * D, 2 * D)]
            mq_s = (head_refs['mk_s'], head_refs['mp_s'], head_refs['mv_s'].at[0], head_refs['mv_s'].at[1])
            for g in range(4):
                for n1 in range(7):
                    if g == 0:
                        t = 200 + (ty + 644) * n1 / 7
                        tie = clk.pacer(min(t, clk.t - 500), min(t + 300, clk.t - 500), 8)
                        for r in range(0, 2 * QD, 16):
                            def block(o, q):
                                row = (o % 2) * HD + (q % 2) * QD + r % QD
                                col = (2 * (o // 2) + q // 2) * T
                                w = wqt_s[row:row + 16, col:col + T]
                                return _hi16(w) if r >= QD else pltpu.bitcast(w << 16, f32)
                            _put(wq_s, r, 7 * n1 * T, _operands2(_B_TERMS, n1, block, lambda x: tie(x, r // 16)))
                    comb = clk.strassen(lambda n: _get(wq_s, 0, 2 * QD, (7 * n1 + n) * T, QM),
                                        lambda n: _get(xa_s, g * QM, QM, (7 * n1 + n) * T, T), _NN)
                    for r in range(0, 2 * QD, 32):
                        e, c = r // QD, comb(r, 32)
                        for dq in range(2):
                            row = dq * QD + r % QD
                            done = _outer_step(mq_s[2 * (g % 2) + e], n1, row,
                                               jnp.concatenate([c[dq], c[2 + dq]], axis=1))
                            if done:
                                n, v = done
                                _put(q_i, (2 * e + n // 2) * D + (n % 2) * HD + row, 2 * g * T, [v])

            span = ty + 6000

            u_next = u_s.at[:, pl.ds(jnp.minimum(i + 1, NP - 1) * (TC // 8), TC // 8)]
            carry = _ssm_scan(u_next, carry, lam_s, h_s, h0_s, clk.pacer(ty, span, TC // 2))

            tie = clk.pacer(ty - 1200, span, 64, [(ty, ty + 1000)])
            rq_i = rq.at[pl.ds((i & 3) * (M // 4), M // 4)]
            sq_i = sq.at[:, _ds((i & 3) * M, M, 8)]
            for c0 in range(0, M // 4, 8):
                _stage(rq_i, sq_i, c0, 8, lambda x, j: tie(x, c0 // 4 + 4 * j), groups=(1,))
            wq_transpose(jnp.minimum(i + 1, NP - 1), lambda x, k: tie(x, 36 + 3 * k))
            for n, (raw, stg, wt_s) in enumerate(((rk, sk, wkt_s), (rv, sv, wvt_s))):
                for c0 in range(0, CS, 8):
                    _stage(raw, stg, c0, 8, lambda x, j: tie(x, 12 * (n + (c0 // 8 + j) / 16)))

                @pl.when(i + 1 < NP)
                def _():
                    w_copy(n, i + 1).start()

                raw[CS, 0:8, 0:T] = tie(zero_s[...], 12 * n + 14).astype(bf16)
                cols = _ds(i * CS, CS, CS)
                for pair in range(H // 2):
                    for dt in range(2):
                        blk = stg[(pair // 4) * 2 + dt, pl.ds(pair % 4, CS, stride=4), :]
                        row = pair * D + dt * HD
                        blk = jnp.concatenate([tie(blk[:8], 16 + 24 * n + 3 * pair + dt), blk[8:]], axis=0)
                        wt_s[row:row + HD, cols] = blk.T

            tie = clk.pacer(ty + 600, ty + 4200, 28)
            a_i = a_s.at[_ds(i * (T // 4), T // 4, T // 4)]
            for r in range(0, T // 2, 16):
                def block(o, q):
                    col = (o % 2) * 2 * QC + (q % 2) * QC
                    return ckv_s[2 * (q // 2) + o // 2, r:r + 16, col:col + QC].astype(f32)
                for n1 in range(7):
                    ops = _operands2(_A_TERMS, n1, block, lambda x: tie(x, 7 * (r // 16) + n1))
                    _put(a_i, r, 7 * n1 * QC, ops)

            @pl.when(i + 1 < NP)
            def _():
                ckv_copy(i + 1).start()

            ckv_s[4, 0:8, 0:T] = tie(zero_s[...], 29).astype(bf16)
            return carry

        lax.fori_loop(0, NP, phase2, carry0)
        for i in range(NP):
            wo_copy(i).wait()
        prep_w(h, range(NT1), _no_tie)

    @pl.when(h == 0)
    def _():
        prologue(**pro_refs)

    def oproj(jp, clk):
        cols = slice(2 * jp * T, (2 * jp + 2) * T)
        for r, n in OCH:
            c = clk.strassen(lambda i: _get(wl_s, r, n, i * T, T),
                             lambda i: _get(cl_s, 0, HD, (jp * 7 + i) * T, T), _NN)()
            o_s[r:r + n, cols] += jnp.concatenate(c[:2], axis=1)
            o_s[HM + r:HM + r + n, cols] += jnp.concatenate(c[2:], axis=1)

    def head(mk_s, mv_s, mp_s, kt_s, ka_s, va_s, v2_s, s_s, pb_s, pd_s, p2_s, sc_s, qb_s, kd_s):
        clk = _Clock(zero_s)
        q_h = q_s.at[_ds(h * D, D, D)]

        def prep_wo(tie):
            for r in range(0, HM, 16):
                top = tie(wo_s[h, r:r + 16, :].astype(f32), r // 16)
                bot = tie(wo_s[h, HM + r:HM + r + 16, :].astype(f32), r // 16)
                _put(wl_s, r, 0, _operands(_A_TERMS, [top[:, :HD], top[:, HD:], bot[:, :HD], bot[:, HD:]]))

        def proj(g, lo=0, hi=7):
            for n1 in range(lo, hi):
                comb = clk.strassen(lambda n: _get(w_s, 0, 2 * QD, (7 * n1 + n) * QC, QC),
                                    lambda n: _get(a_s, g * T, T, (7 * n1 + n) * QC, QC), _NT, 2, n1 == 6)
                for r, m_s in ((0, mk_s), (QD, mv_s.at[g % 2])):
                    c = comb(r, QD)
                    m_s[n1 * HD:n1 * HD + QD, :] = jnp.concatenate([c[0], c[2]], axis=1)
                    m_s[n1 * HD + QD:(n1 + 1) * HD, :] = jnp.concatenate([c[1], c[3]], axis=1)
            if hi < 7:
                return
            cs = [_combine([mk_s[n * HD + r:n * HD + r + 16, :] for n in range(7)], order=range(7))
                  for r in range(0, HD, 16)]
            for n in range(4):
                kt_s[:, n * T:(n + 1) * T] = jnp.concatenate([c[n] for c in cs], axis=0).T
            for r in range(0, 2 * T, T // 2):
                blk = kt_s[r:r + T // 2, :]
                blk = [blk[:, n * T:(n + 1) * T] for n in range(4)]
                _put(ka_s, 2 * g * T + r, 0, _operands(_A_TERMS, blk) + [blk[2]])
            for r in (0, 32, T, T + 32):
                lo_, hi_ = kt_s[r:r + 32, 0:2 * T], kt_s[r + T // 2:r + T // 2 + 32, 0:2 * T]
                _put(kd_s, r // T * (T // 2) + r % T, 0,
                     _operands(_A_TERMS, [lo_[:, :T], lo_[:, T:], hi_[:, :T], hi_[:, T:]]))

        def vfin(g, tie):
            m_s = mv_s.at[g % 2]
            for r in range(0, QD, 16):
                k, blk = 8 * (r // 16), {}
                late = lambda w: tie(w, k, True, LATE)
                for new, n1 in (((0,), 2), ((1,), 4), ((3,), 6), ((), 0), ((), 3), ((2,), 5), ((), 1)):
                    for o in new:
                        for i, row in enumerate((r, QD + r)):
                            tiles = _Rows([m_s.at[n * HD:(n + 1) * HD] for n in range(7)], row, 16)
                            c, = _combine(tiles, ((o % 2) * 2 + o // 2,), range(7))
                            blk[o, i] = c = tie(c, k)
                            slot = (2, 7, 8, 3)[o]
                            _put(va_s, row, ((2 * g + 1) * 9 + slot) * T, [c[:, T:]])
                            if o in (1, 2):
                                _put(va_s, row, (2 * g * 9 + slot) * T, [c[:, :T]])
                    lo_, hi_ = [_operand(_A_TERMS[n1], lambda o: blk[o, i]) for i in range(2)]
                    _put(va_s, r, (2 * g * 9 + n1) * T, [lo_[:, :T]], late)
                    _put(va_s, QD + r, (2 * g * 9 + n1) * T, [hi_[:, :T]], late)
                    if g < 3:
                        _put(v2_s, r, (g * 7 + n1) * 7 * T,
                             _operands(_A_TERMS, [lo_[:, :T], lo_[:, T:], hi_[:, :T], hi_[:, T:]]), late)
                    k += 8 / 7

        key = lax.broadcasted_iota(jnp.int32, (T, 2 * T), 0)
        qry = lax.broadcasted_iota(jnp.int32, (T, 2 * T), 1)
        causal = key <= qry

        marks = []

        def qk(g):
            pairs = (2 * g, 2 * g + 1)
            mx = {jp: _Reducer(jnp.max, jnp.maximum) for jp in pairs}

            def put(jp, row, v):
                v = v.reshape(v.shape[0] // 8, 8, 2 * T)
                s_s[jp % 4, row // 8:row // 8 + v.shape[0]] = v
                mx[jp].add(v)

            def rect(jp, lo, hi):
                for r in range(lo, hi, T // 2):
                    c = clk.strassen(lambda i: _get(ka_s, r, T // 2, i * T, T),
                                     lambda i: _get(qb_s, 0, HD, ((jp % 2) * 7 + i) * T, T), _NN)()
                    put(jp, r, jnp.concatenate(c[:2], axis=1))
                    put(jp, jp * T + r, jnp.concatenate(c[2:], axis=1))

            for jp in pairs:
                for r in range(0, HD, 32):
                    blk = [_get(q_h, e * D + d * HD + r, 32, jp * T, T).astype(f32) for d in range(2) for e in range(2)]
                    _put(qb_s, r, (jp % 2) * 7 * T, _operands(_B_TERMS, blk))
            for jp in pairs:
                rect(jp, 0, 2 * g * T)
                marks.append(clk.t)
            last = {}
            for jp in pairs:
                ko = jnp.concatenate([_get(ka_s, jp * T, T, n * T, T) for n in (7, 3)], axis=1)
                so = jnp.where(causal[:, :T], clk.dot(ko, _get(q_h, D, D, jp * T, T), _NN), NEG)
                row = (2 * jp + 1) * T // 8
                s_s[jp % 4, row:row + T // 8, :, T:] = so.reshape(T // 8, 8, T)
                last[jp] = jnp.concatenate([jnp.full((1, T), NEG, f32), jnp.max(so, axis=0, keepdims=True)], axis=1)
            rect(2 * g + 1, 2 * g * T, (2 * g + 1) * T)
            for jp in pairs:
                c = clk.strassen(lambda i: _get(kd_s, (jp % 2) * (T // 2), T // 2, i * T, T),
                                 lambda i: _get(qb_s, 0, HD, ((jp % 2) * 7 + i) * T, T), _NN)()
                se = jnp.concatenate([jnp.concatenate(c[:2], axis=1), jnp.concatenate(c[2:], axis=1)], axis=0)
                put(jp, 2 * jp * T, jnp.where(causal, se, NEG))
            return [jnp.broadcast_to(jnp.maximum(mx[jp].result(), last[jp]), (8, 2 * T)) for jp in pairs]

        zs, sums = {}, {}

        def prob(jp, row, z, n=GS, lanes=slice(None)):
            return jnp.exp2(s_s[jp % 4, row // 8:(row + n) // 8, :, lanes] - z[:, lanes])

        def rough(jp, mx, tie):
            zs[jp] = mx
            if jp > 0:
                sm = _Reducer(jnp.sum, jnp.add)
                for k, r in enumerate(range(0, 2 * jp * T, GS * LSUB)):
                    sm.add(prob(jp, r, tie(mx, k)))
                zs[jp] = mx + jnp.log2(jnp.maximum(LSUB * sm.result(), 1.0))
            sums[jp] = _Reducer(jnp.sum, jnp.add)

        def blocks(jp, row, tie, k):
            top, bot = prob(jp, row, tie(zs[jp], k)), prob(jp, jp * T + row, tie(zs[jp], k + 1))
            sums[jp].add(top + bot)
            top, bot = top.reshape(GS, 2 * T), bot.reshape(GS, 2 * T)
            return [top[:, :T], top[:, T:], bot[:, :T], bot[:, T:]]

        def near(jp, tie, k):
            R, z = jp * T, zs[jp]
            if jp % 2:
                for r in range(0, T, GS):
                    _put(pb_s, jp // 2 * T + r, 0, _operands(_B_TERMS, blocks(jp, R - T + r, tie, k)))
                    k += 2
            for r in range(0, T, GS):
                p = prob(jp, 2 * R + r, tie(z, k))
                sums[jp].add(p)
                _put(pd_s, 2 * R + r, 0, [p.reshape(GS, 2 * T)])
                k += 1
            so = _Reducer(jnp.sum, jnp.add)
            for r in range(0, T, 2 * GS):
                p = prob(jp, 2 * R + T + r, tie(z, k), 2 * GS, slice(T, 2 * T))
                so.add(p)
                _put(pd_s, 2 * R + T + r, T, [p.reshape(2 * GS, T)])
                k += 1
            sums[jp].result()
            sums[jp].out = sums[jp].out + jnp.concatenate([jnp.zeros((1, T), f32), so.result()], axis=1)

        p20 = lambda g: g * (g - 1) // 2 * T

        def far(g, tie, k):
            half = {(jp, e): _Reducer(jnp.sum, jnp.add) for jp in (2 * g, 2 * g + 1) for e in range(2)}
            for kg in range(g):
                for r in range(0, T, GS):
                    blk = {}
                    for new, n1 in (((0,), 1), ((1,), 5), ((3,), 2), ((), 0), ((), 4), ((2,), 3), ((), 6)):
                        for o in new:
                            lanes = slice((o % 2) * T, (o % 2 + 1) * T)
                            for jp in (2 * g, 2 * g + 1):
                                z = tie(zs[jp][:, lanes], k)
                                row = (o // 2) * jp * T + 2 * kg * T + r
                                p = [jnp.exp2(s_s[jp % 4, x // 8:(x + GS) // 8, :, lanes] - z) for x in (row, row + T)]
                                half[jp, o % 2].add(p[0] + p[1])
                                blk[o, jp % 2], blk[o, 2 + jp % 2] = [x.reshape(GS, T) for x in p]
                        ops = _operands2(_B_TERMS, n1, lambda o, q: blk[o, q], lambda x: x)
                        _put(p2_s, p20(g) + kg * T + r, 7 * n1 * T, ops, lambda w: tie(w, k, True, LATE))
                        k += 16 / 7
            for jp in (2 * g, 2 * g + 1):
                if g:
                    sums[jp].out = sums[jp].out + jnp.concatenate([half[jp, e].result() for e in range(2)], axis=1)
            for jp in (2 * g, 2 * g + 1):
                cols = slice(2 * jp * T, 2 * (jp + 1) * T)
                sc_s[:, cols] = g_s[:, cols] / sums[jp].result()

        def pv(g):
            pairs = (2 * g, 2 * g + 1)
            va = lambda n, t, r=0, nr=HD: _get(va_s, r, nr, (t * 9 + n) * T, T)
            for n1 in range(7 if g else 0):
                c = clk.strassen(
                    lambda n: _cat([_get(v2_s, 0, QD, (kg * 49 + 7 * n1 + n) * T, T) for kg in range(g)], 1),
                    lambda n: _get(p2_s, p20(g), g * T, (7 * n1 + n) * T, T), _NN, g)()
                mp_s[n1 * HD:n1 * HD + QD, :] = jnp.concatenate(c[:2], axis=1)
                mp_s[n1 * HD + QD:(n1 + 1) * HD, :] = jnp.concatenate(c[2:], axis=1)
            if g == 3:
                vfin(3, clk.pacer(clk.t - 2000, clk.t - 1200, 32))
            ve = [jnp.concatenate([va(2, jp), va(8, jp)], axis=0) for jp in pairs]
            vo = [jnp.concatenate([va(7, jp), va(3, jp)], axis=0) for jp in pairs]
            ce = clk.level([(ve[jp % 2], _get(pd_s, 2 * jp * T, T, 0, T)) for jp in pairs])
            co = [clk.dot(jnp.concatenate([ve[jp % 2], vo[jp % 2]], axis=1),
                          _get(pd_s, 2 * jp * T, 2 * T, T, T), _NN) for jp in pairs]
            for jp in pairs:
                R, e = jp * T, jp % 2
                ge, go = sc_s[:, 2 * R:2 * R + T], sc_s[:, 2 * R + T:2 * R + 2 * T]
                for r in range(0, HD, 32):
                    c = [ce[e][r:r + 32], co[e][r:r + 32], ce[e][HD + r:HD + r + 32], co[e][HD + r:HD + r + 32]]
                    if g:
                        far_ = _combine([mp_s[n * HD + r:n * HD + r + 32, e * T:(e + 1) * T] for n in range(7)],
                                        order=range(7))
                        c = [x + y for x, y in zip(c, far_)]
                    if e:
                        near_ = clk.strassen(lambda n: va(n, 2 * g, r, 32),
                                             lambda n: _get(pb_s, g * T, T, n * T, T), _NN)()
                        c = [x + y for x, y in zip(c, near_)]
                    ops = _operands(_B_TERMS, [c[0] * ge, c[1] * go, c[2] * ge, c[3] * go])
                    _put(cl_s, r, jp * 7 * T, ops)

        ends = []

        def run(items):
            for item in items.split():
                if item[0] == 'P':
                    pv(int(item[1]))
                    ends.append(clk.t)
                elif item[0] == 'K':
                    proj(int(item[1]), 2 if item == 'K1' else 0)
                else:
                    jp = int(item[1])
                    oproj(jp, clk)

                    @pl.when(h == H - 1)
                    def _():
                        out_copy(jp).start()

        oproj(NP - 1, clk)
        for n1 in range(7):
            if n1 >= NT1:
                prep_w(h, [n1], clk.pacer(clk.t - 896, clk.t - 448, 8))
            proj(0, n1, n1 + 1)
        proj(1, 0, 2)
        mx = qk(0)
        for g in range(4):
            t0 = clk.t
            del ends[:]
            run(PLAN[g])
            t1 = clk.t
            nxt = qk(g + 1) if g < 3 else None
            n_rough = [2 * jp * T // (GS * LSUB) for jp in (2 * g, 2 * g + 1)]
            n_near = [(T + T // 2) // GS, (3 * T + T // 2) // GS]
            holes = [(t - 400, t) for t in ends]
            if 0 < g < 3:
                holes.append((marks[-2] - 400, marks[-2] - 100))
            if g < 3:
                vfin(g, clk.pacer(t0, t0 + VW, 32))
                holes += [(t0, t0 + VW), (t1 - 300, t1 + 300)]
            if g == 2:
                holes.append((clk.t - 300, clk.t))
            tie = clk.pacer(t0, (clk.t if g else t1) - SLACK,
                            sum(n_rough) + sum(n_near) + g * 16 * T // GS, holes)
            rough(2 * g, mx[0], tie)
            near(2 * g, tie, n_rough[0])
            k = n_rough[0] + n_near[0]
            rough(2 * g + 1, mx[1], lambda x, i: tie(x, k + i))
            near(2 * g + 1, tie, k + n_rough[1])
            far(g, tie, k + n_rough[1] + n_near[1])
            if g == 0:
                prep_wo(clk.pacer(t0 + VW, t1 - 300, HM // 16))
            mx = nxt
        t0 = clk.t
        run(PLAN[4])
        prep_w(jnp.minimum(h + 1, H - 1), range(NT1), clk.pacer(t0 - 100, clk.t - 500, 8 * NT1))
        assert len(set(clk.load)) == 1

    head(**head_refs)

    @pl.when(h == H - 1)
    def _():
        oproj(NP - 1, _Clock(zero_s))
        out_copy(NP - 1).start()
        for jp in range(NP):
            out_copy(jp).wait()


@jax.jit
def pallas_gated_mix__compressed_kv_cla__ssm_conv_s5__prompt_kernel(
    A_x: jax.Array,
    A_c_kv: jax.Array,
    A_w_q: jax.Array,
    A_w_uk: jax.Array,
    A_w_uv: jax.Array,
    A_w_o: jax.Array,
    B_x: jax.Array,
    B_Lambda_re: jax.Array,
    B_Lambda_im: jax.Array,
    B_B_re: jax.Array,
    B_B_im: jax.Array,
    B_C_re: jax.Array,
    B_C_im: jax.Array,
    B_log_dt: jax.Array,
    B_Dskip: jax.Array,
    gate_w: jax.Array,
):
    del B_x
    xT = jnp.transpose(A_x[0])
    woT = jnp.transpose(A_w_o, (0, 2, 1))
    ckv = A_c_kv.reshape(4, 4, 2, T // 2, DC)

    hbm = pl.BlockSpec(memory_space=pl.ANY)
    outT = pl.pallas_call(
        _kernel,
        grid=(H,),
        in_specs=[hbm] * 15,
        out_specs=hbm,
        out_shape=jax.ShapeDtypeStruct((M, S), f32),
        scratch_shapes=_SHARED_SCRATCH + list(_PROLOGUE_SCRATCH.values()) + list(_HEAD_SCRATCH.values()),
        compiler_params=pltpu.CompilerParams(
            dimension_semantics=("arbitrary",),
            vmem_limit_bytes=127 * 1024 * 1024,
            disable_bounds_checks=True,
        ),
    )(xT, B_B_re, B_B_im, B_C_re, B_C_im, B_Lambda_re, B_Lambda_im, B_log_dt,
      B_Dskip, gate_w, woT, ckv, A_w_q, A_w_uk, A_w_uv)
    return jnp.transpose(outT)[None]
```
